```python
import jax
import jax.numpy as jnp

def _softmax(x, axis=-1):
    return jax.nn.softmax(x, axis=axis)

def _gelu(x):
    return jax.nn.gelu(x, approximate=True)

def _silu(x):
    return jax.nn.silu(x)

def _sigmoid(x):
    return jax.nn.sigmoid(x)

def _layernorm(x, axis=-1, eps=1e-05):
    m = jnp.mean(x, axis=axis, keepdims=True)
    v = jnp.var(x, axis=axis, keepdims=True)
    return (x - m) / jnp.sqrt(v + eps)

def _scatter_add(tgt, idx, src, axis=0):
    return tgt.at[idx].add(src)

def _segment_sum(src, seg, n):
    return jax.ops.segment_sum(src, seg, n)

class _Rng:

    def __init__(self, key):
        self._k = key

    def _next(self):
        self._k, sub = jax.random.split(self._k)
        return sub

    def normal(self, shape):
        return jax.random.normal(self._next(), shape, dtype=jnp.bfloat16)

    def randint(self, lo, hi, shape):
        return jax.random.randint(self._next(), shape, lo, hi, dtype=jnp.int32)

    def uniform(self, shape, lo=0.0, hi=1.0):
        return jax.random.uniform(self._next(), shape, jnp.bfloat16, lo, hi)

    def permutation(self, n):
        return jax.random.permutation(self._next(), n)
kernel_name = 'adaLN_cond__ssm_conv_h3__mixer_s_mlp__prompt'

def setup_inputs():
    _rng = _Rng(jax.random.key(int.from_bytes(__import__("os").urandom(4), "little")))
    _w = lambda a: (lambda t: t.astype(jnp.bfloat16) if jnp.issubdtype(t.dtype, jnp.floating) else t)(jnp.asarray(a))

    def _A_setup():
        B, S, D = (1, 2048, 640)
        ks = 4
        return {'q': _w((lambda *s: _rng.normal(s) * 0.05)(B, S, D)), 'k': _w((lambda *s: _rng.normal(s) * 0.05)(B, S, D)), 'v': _w((lambda *s: _rng.normal(s) * 0.05)(B, S, D)), 'shift_k': _w((lambda *s: _rng.normal(s) * 0.05)(D, ks) * 0.5), 'ssm_k': _w((lambda *s: _rng.normal(s) * 0.05)(D, S) * (1.0 / S ** 0.5)), 'ssm_D': _w((lambda *s: _rng.normal(s) * 0.05)(D))}
    _A_in = _A_setup()

    def _B_setup():
        B, S, D, F = (1, 2048, 640, 1728)
        return {'x': _w((lambda *s: _rng.normal(s) * 0.05)(B, S, D)), 'w1': _w((lambda *s: _rng.normal(s) * 0.05)(D, D) * D ** (-0.5)), 'w2': _w((lambda *s: _rng.normal(s) * 0.05)(D, D) * D ** (-0.5)), 'w3': _w((lambda *s: _rng.normal(s) * 0.05)(D, F) * D ** (-0.5)), 'w4': _w((lambda *s: _rng.normal(s) * 0.05)(F, D) * F ** (-0.5))}
    _B_in = _B_setup()
    return {'A_q': _A_in['q'], 'A_k': _A_in['k'], 'A_v': _A_in['v'], 'A_shift_k': _A_in['shift_k'], 'A_ssm_k': _A_in['ssm_k'], 'A_ssm_D': _A_in['ssm_D'], 'B_x': _B_in['x'], 'B_w1': _B_in['w1'], 'B_w2': _B_in['w2'], 'B_w3': _B_in['w3'], 'B_w4': _B_in['w4'], 'c': _w((lambda *s: _rng.normal(s) * 0.05)(1, 640)), 'w_mod': _w((lambda *s: _rng.normal(s) * 0.05)(640, 6 * 640) * 640 ** (-0.5))}

def reference(A_q, A_k, A_v, A_shift_k, A_ssm_k, A_ssm_D, B_x, B_w1, B_w2, B_w3, B_w4, c, w_mod):

    def _A_ref(q, k, v, shift_k, ssm_k, ssm_D):
        B, S, D = q.shape
        ks = shift_k.shape[-1]
        k_pad = jnp.pad(k, ((0, 0), (ks - 1, 0), (0, 0)))
        k_shift = jnp.zeros_like(k)
        for t in range(ks):
            k_shift = k_shift + k_pad[:, t:t + S, :] * shift_k[:, ks - 1 - t][None, None, :]
        kv = k_shift * v
        L = 2 * S
        kv_pad = jnp.pad(kv, ((0, 0), (0, S), (0, 0)))
        kf_pad = jnp.pad(ssm_k, ((0, 0), (0, S)))
        kv_f = (lambda x, axes=(-2, -1): jnp.fft.rfft2(x.astype(jnp.float32), axes=axes))(kv_pad[:, None, :, :], axes=(1, 2))
        kf_f = (lambda x, axes=(-2, -1): jnp.fft.rfft2(x.astype(jnp.float32), axes=axes))(kf_pad[:, None, :], axes=(1, 2))
        kf_f = (lambda x, *d: x.transpose(*d))(kf_f, 1, 2, 0)
        y_f = kv_f * kf_f[None, :, :, :]
        y = (lambda x, s, axes=(-2, -1): jnp.fft.irfft2(x, s=s, axes=axes).astype(jnp.bfloat16))(y_f, (1, L), axes=(1, 2))[:, 0, :S, :]
        y = y + kv * ssm_D[None, None, :]
        return q * y

    def _B_ref(x, w1, w2, w3, w4):
        B, S, D = x.shape
        h = _gelu(_layernorm(x, axis=-1) @ w1)
        c = D // 4
        g0 = jnp.pad(h[:, :, 0 * c:1 * c], ((0, 0), (1, 0), (0, 0)))[:, :S, :]
        g1 = jnp.pad(h[:, :, 1 * c:2 * c], ((0, 0), (0, 1), (0, 0)))[:, 1:, :]
        g2 = jnp.pad(h[:, :, 2 * c:3 * c], ((0, 0), (2, 0), (0, 0)))[:, :S, :]
        g3 = jnp.pad(h[:, :, 3 * c:], ((0, 0), (0, 2), (0, 0)))[:, 2:, :]
        hs = jnp.concatenate([g0, g1, g2, g3], axis=-1) @ w2
        x1 = x + hs
        h2 = _gelu(_layernorm(x1, axis=-1) @ w3) @ w4
        return x1 + h2
    x = A_q
    mod = (_silu(c) @ w_mod).reshape(c.shape[0], 6, 1, -1)
    sa, ca, ga, sb, cb, gb = (mod[:, 0].copy(), mod[:, 1].copy(), mod[:, 2].copy(), mod[:, 3].copy(), mod[:, 4].copy(), mod[:, 5].copy())
    h = _layernorm(x, axis=-1) * (1 + ca) + sa
    x = x + ga * _A_ref(h, A_k, A_v, A_shift_k, A_ssm_k, A_ssm_D)
    h = _layernorm(x, axis=-1) * (1 + cb) + sb
    x = x + gb * _B_ref(h, B_w1, B_w2, B_w3, B_w4)
    return x
```

```python
import math

import jax
import jax.numpy as jnp
from jax import lax
import jax.experimental.pallas as pl
import jax.experimental.pallas.tpu as pltpu

S, D, F = 2048, 640, 1728
C = 128
NC = S // C
NT = D // 128
NG = 16
T1 = 256
T2 = 256
EPS = 1e-5
_C0 = math.sqrt(2.0 / math.pi)
ALPHA = (_C0 * 0.044715) ** (1.0 / 3.0)
GC = _C0 / ALPHA
BETA = 0.5 / ALPHA
F_CHUNKS = ((0, 512), (512, 512), (1024, 512), (1536, 192))

f32 = jnp.float32
bf16 = jnp.bfloat16
u32 = jnp.uint32


def _dft(shape, freq_dim, scale):
    row = lax.broadcasted_iota(jnp.int32, shape, freq_dim)
    n = lax.broadcasted_iota(jnp.int32, shape, 1 - freq_dim)
    j = ((row >> 4) << 3) + (row & 7)
    m = ((4 * j + 1) * n + ((row >> 3) & 1) * 128) & 511
    return (jnp.cos(m.astype(f32) * (math.pi / 256.0)) * scale).astype(bf16)


def _gelu2a(z):
    return z * (1.0 + jnp.tanh(z * (z * z + GC)))


def _center(x):
    m = jnp.sum(x, axis=-1, keepdims=True) * (1.0 / D)
    d = x - m
    v = jnp.sum(d * d, axis=-1, keepdims=True) * (1.0 / D)
    return d, lax.rsqrt(v + EPS)


def _kernel(q_hbm, k_hbm, v_hbm, sk_ref, h_hbm, dd_ref, w1_hbm, w2_hbm, w3_hbm, w4_hbm,
            c_ref, wm_hbm, o_hbm,
            qbuf, kbuf, vbuf, hbuf, w1, w2, w3, w4, wm, obuf,
            fw, inv, kf, ub, gb_, yb, xn, hh, h1, par, sems, osems):
    cp_k = [pltpu.make_async_copy(k_hbm.at[0, :, pl.ds(j * 128, 128)], kbuf.at[j], sems.at[j]) for j in range(NT)]
    cp_v = [pltpu.make_async_copy(v_hbm.at[0, :, pl.ds(j * 128, 128)], vbuf.at[j], sems.at[5 + j]) for j in range(NT)]
    cp_h = [pltpu.make_async_copy(h_hbm.at[pl.ds(j * 128, 128), :], hbuf.at[j], sems.at[10 + j]) for j in range(NT)]
    cp_q = pltpu.make_async_copy(q_hbm.at[0], qbuf, sems.at[15])
    cp_wm = pltpu.make_async_copy(wm_hbm, wm, sems.at[16])
    cp_w = [pltpu.make_async_copy(s, d, sems.at[17 + i])
            for i, (s, d) in enumerate(((w1_hbm, w1), (w2_hbm, w2), (w3_hbm, w3), (w4_hbm, w4)))]
    for j in range(NT):
        cp_k[j].start()
        cp_v[j].start()
        cp_h[j].start()
    cp_wm.start()
    cp_q.start()
    for c in cp_w:
        c.start()

    with jax.named_scope("init"):
        fw[...] = pltpu.bitcast(_dft((256, 128), 0, 1.0), u32)
        inv[...] = pltpu.bitcast(_dft((128, 256), 1, 1.0 / 128.0), u32)
        kf[pl.ds(0, 8), :] = jnp.zeros((8, 128), f32)
        par[pl.ds(0, 4), :] = sk_ref[...].astype(f32)
        par[pl.ds(8, 8), :] = jnp.broadcast_to(dd_ref[...].astype(f32).reshape(1, D), (8, D))
        zeros = jnp.zeros((8, 128), f32)
        for j in range(NT):
            h1[j, pl.ds(0, 8), :] = zeros
            h1[j, pl.ds(S + 8, 8), :] = zeros

    def fwd_step(j, i):
        r = pl.multiple_of(i * 256, 256)
        taps = [par[pl.ds(t, 1), pl.ds(j * 128, 128)] for t in range(4)]
        k0 = kbuf[j, pl.ds(r, 256), :].astype(f32)
        kf[pl.ds(r + 8, 256), :] = k0
        ks = k0 * taps[0]
        for t in range(1, 4):
            ks = ks + kf[pl.ds(r + 8 - t, 256), :] * taps[t]
        kv = (ks * vbuf[j, pl.ds(r, 256), :].astype(f32)).astype(bf16)
        fm = pltpu.bitcast(fw[...], bf16)
        rhs = jnp.concatenate([kv[:128], kv[128:]], axis=1)
        u = jnp.dot(fm, rhs, preferred_element_type=f32)
        hc = hbuf[j, :, pl.ds(r, 256)]
        rhs_t = jnp.concatenate([hc[:, :128], hc[:, 128:]], axis=0)
        g = lax.dot_general(fm, rhs_t, (((1,), (1,)), ((), ())), preferred_element_type=f32)
        for cc in range(2):
            ci = 2 * i + cc
            for gi in range(NG):
                a = u[16 * gi:16 * gi + 8, 128 * cc:128 * cc + 128]
                b = u[16 * gi + 8:16 * gi + 16, 128 * cc:128 * cc + 128]
                ub[gi, ci, 0] = a + b
                ub[gi, ci, 1] = a
                ub[gi, ci, 2] = b
                c = g[16 * gi:16 * gi + 8, 128 * cc:128 * cc + 128]
                d = g[16 * gi + 8:16 * gi + 16, 128 * cc:128 * cc + 128]
                gb_[gi, ci, 0] = c
                gb_[gi, ci, 1] = d - c
                gb_[gi, ci, 2] = c + d

    def mac_step(gi):
        OB = 4
        prev = None
        for a0 in range(0, NC, OB):
            acc = [[None] * 3 for _ in range(OB)]
            gwin = {}
            for c in range(a0 + OB):
                uu = [ub[gi, c, t] for t in range(3)]
                for o in range(OB):
                    dl = a0 + o - c
                    if dl < 0:
                        continue
                    if dl not in gwin:
                        gwin[dl] = [gb_[gi, dl, t] for t in range(3)]
                    for t in range(3):
                        p = uu[t] * gwin[dl][t]
                        acc[o][t] = p if acc[o][t] is None else acc[o][t] + p
            for o in range(OB):
                re = acc[o][0] - acc[o][2]
                im = acc[o][0] + acc[o][1]
                if prev is None:
                    yr, yi = re, im
                else:
                    yr, yi = re - prev[1], im + prev[0]
                prev = (re, im)
                y = jnp.concatenate([yr, yi], axis=0).astype(bf16)
                yb[a0 + o, pl.ds(pl.multiple_of(gi * 8, 8), 8), :] = pltpu.bitcast(y, u32)

    def inv_step(j, i):
        im_ = pltpu.bitcast(inv[...], bf16)
        rhs = jnp.concatenate([pltpu.bitcast(yb[2 * i + cc], bf16) for cc in range(2)], axis=1)
        y = jnp.dot(im_, rhs, preferred_element_type=f32)
        for cc in range(2):
            r = pl.multiple_of(i * 256 + cc * 128, 128)
            xn[pl.ds(r, 128), pl.ds(j * 128, 128)] = y[:, 128 * cc:128 * cc + 128]

    for j in range(NT):
        with jax.named_scope("A_wait"):
            cp_k[j].wait()
            cp_v[j].wait()
            cp_h[j].wait()
        with jax.named_scope("A_fwd"):
            lax.fori_loop(0, 8, lambda i, c, j=j: (fwd_step(j, i), c)[1], 0)
            dvec = par[pl.ds(8, 8), pl.ds(j * 128, 128)]
            for gi in range(NG):
                gb_[gi, 0, 0] = gb_[gi, 0, 0] + dvec
                gb_[gi, 0, 1] = gb_[gi, 0, 1] - dvec
                gb_[gi, 0, 2] = gb_[gi, 0, 2] + dvec
        with jax.named_scope("A_mac"):
            lax.fori_loop(0, NG, lambda gi, c: (mac_step(gi), c)[1], 0)
        with jax.named_scope("A_inv"):
            lax.fori_loop(0, 8, lambda i, c, j=j: (inv_step(j, i), c)[1], 0)

    with jax.named_scope("mod"):
        cp_wm.wait()
        cv = c_ref[...].astype(f32)
        sc = jnp.broadcast_to(cv * jax.nn.sigmoid(cv), (16, D)).astype(bf16)
        mod = jnp.dot(sc, wm[...], preferred_element_type=f32)[:8]
        sa, ca, ga, sb, cb, gb = [mod[:, i * D:(i + 1) * D] for i in range(6)]
        par[pl.ds(16, 8), :] = ga * (1.0 + ca)
        par[pl.ds(24, 8), :] = ga * sa
        par[pl.ds(32, 8), :] = 1.0 + cb
        par[pl.ds(40, 8), :] = sb
        par[pl.ds(48, 8), :] = gb
        cp_q.wait()
        cp_w[0].wait()

    def b1_step(i):
        r = pl.multiple_of(i * T1, T1)
        pa, pb, pc, ps = [par[pl.ds(16 + 8 * t, 1), :] for t in range(4)]
        q = qbuf[pl.ds(r, T1), :].astype(f32)
        d1, r1 = _center(q)
        x = q + ((d1 * r1) * pa + pb) * xn[pl.ds(r, T1), :]
        xn[pl.ds(r, T1), :] = x
        d2, r2 = _center(x)
        h = (d2 * r2) * pc + ps
        hh[pl.ds(r, T1), :] = h
        d3, r3 = _center(h)
        l3 = (d3 * (r3 * ALPHA)).astype(bf16)
        z = jnp.dot(l3, w1[...], preferred_element_type=f32)
        g = _gelu2a(z)
        for j in range(NT):
            h1[j, pl.ds(r + 8, T1), :] = g[:, j * 128:(j + 1) * 128]

    with jax.named_scope("B1"):
        lax.fori_loop(0, S // T1, lambda i, c: (b1_step(i), c)[1], 0)

    def out_copy(i):
        r = pl.multiple_of(i * T2, T2)
        return pltpu.make_async_copy(obuf.at[pl.ds(r, T2), :], o_hbm.at[0, pl.ds(r, T2), :], osems.at[i])

    def b2_step(i):
        r = pl.multiple_of(i * T2, T2)
        lane = lax.broadcasted_iota(jnp.int32, (T2, 128), 1)

        def ld(j, off):
            return h1[j, pl.ds(r + 8 + off, T2), :]
        tiles = [
            ld(0, -1),
            jnp.where(lane < 32, ld(1, -1), ld(1, 1)),
            jnp.where(lane < 64, ld(2, 1), ld(2, -2)),
            jnp.where(lane < 96, ld(3, -2), ld(3, 2)),
            ld(4, 2),
        ]
        hs = jnp.concatenate([t.astype(bf16) for t in tiles], axis=1)
        x1 = hh[pl.ds(r, T2), :] + jnp.dot(hs, w2[...], preferred_element_type=f32) * BETA
        d4, r4 = _center(x1)
        l4 = (d4 * (r4 * ALPHA)).astype(bf16)
        acc = None
        for (f0, fn) in F_CHUNKS:
            z = lax.dot_general(l4, w3[pl.ds(f0, fn), :], (((1,), (1,)), ((), ())), preferred_element_type=f32)
            g = _gelu2a(z).astype(bf16)
            p = jnp.dot(g, w4[pl.ds(f0, fn), :], preferred_element_type=f32)
            acc = p if acc is None else acc + p
        gbv = par[pl.ds(48, 1), :]
        out = xn[pl.ds(r, T2), :] + gbv * (x1 + acc * BETA)
        obuf[pl.ds(r, T2), :] = out.astype(bf16)
        out_copy(i).start()

    with jax.named_scope("B2_wait"):
        cp_w[1].wait()
        cp_w[2].wait()
        cp_w[3].wait()
    with jax.named_scope("B2"):
        lax.fori_loop(0, S // T2, lambda i, c: (b2_step(i), c)[1], 0)
    with jax.named_scope("out_wait"):
        for i in range(S // T2):
            out_copy(i).wait()


@jax.jit
def pallas_adaLN_cond__ssm_conv_h3__mixer_s_mlp__prompt_kernel(
    A_q, A_k, A_v, A_shift_k, A_ssm_k, A_ssm_D, B_x, B_w1, B_w2, B_w3, B_w4, c, w_mod,
):
    del B_x
    any_spec = pl.BlockSpec(memory_space=pltpu.MemorySpace.HBM)
    vmem_spec = pl.BlockSpec(memory_space=pltpu.VMEM)
    return pl.pallas_call(
        _kernel,
        out_shape=jax.ShapeDtypeStruct((1, S, D), bf16),
        in_specs=[any_spec, any_spec, any_spec, vmem_spec, any_spec, vmem_spec,
                  any_spec, any_spec, any_spec, any_spec, vmem_spec, any_spec],
        out_specs=any_spec,
        scratch_shapes=[
            pltpu.VMEM((S, D), bf16),
            pltpu.VMEM((NT, S, 128), bf16),
            pltpu.VMEM((NT, S, 128), bf16),
            pltpu.VMEM((NT, 128, S), bf16),
            pltpu.VMEM((D, D), bf16),
            pltpu.VMEM((D, D), bf16),
            pltpu.VMEM((F, D), bf16),
            pltpu.VMEM((F, D), bf16),
            pltpu.VMEM((D, 6 * D), bf16),
            pltpu.VMEM((S, D), bf16),
            pltpu.VMEM((128, 128), u32),
            pltpu.VMEM((64, 256), u32),
            pltpu.VMEM((S + 8, 128), f32),
            pltpu.VMEM((NG, NC, 3, 8, 128), f32),
            pltpu.VMEM((NG, NC, 3, 8, 128), f32),
            pltpu.VMEM((NC, 128, 128), u32),
            pltpu.VMEM((S, D), f32),
            pltpu.VMEM((S, D), f32),
            pltpu.VMEM((NT, S + 16, 128), f32),
            pltpu.VMEM((56, D), f32),
            pltpu.SemaphoreType.DMA((21,)),
            pltpu.SemaphoreType.DMA((S // T2,)),
        ],
        compiler_params=pltpu.CompilerParams(vmem_limit_bytes=100 * 1024 * 1024),
    )(A_q, A_k, A_v, A_shift_k.T, A_ssm_k, A_ssm_D, B_w1, B_w2, B_w3.T, B_w4, c, w_mod)
```

```python
import math
import os

import jax
import jax.numpy as jnp
from jax import lax
import jax.experimental.pallas as pl
import jax.experimental.pallas.tpu as pltpu

S, D, F = 2048, 640, 1728
C = 128
NC = S // C
NT = D // 128
NG = 16
KOFF = (NC + 1) * NG * 3
W = int(os.environ.get('W', '4'))
SKIPA = int(os.environ.get('SKIPA', '0'))
WMA, WMC = 1664, 512
Q0 = int(os.environ.get('Q0', '512'))
N2 = int(os.environ.get('N2', '5'))
PRELN = int(os.environ.get('PRELN', '2'))
NOCACHE = int(os.environ.get('NOCACHE', '0'))
OUTWAIT = int(os.environ.get('OUTWAIT', '0'))
SEGS = [int(x) for x in os.environ.get('SEGS', '012345')]
SKIPB = int(os.environ.get('SKIPB', '0'))
KARA = int(os.environ.get('KARA', '1'))
UNR = int(os.environ.get('UNR', '2'))
HEAD = int(os.environ.get('HEAD', '250'))
TAIL = int(os.environ.get('TAIL', '450'))
DORDER = os.environ.get('DORDER', 'HaUb')
R1 = int(os.environ.get('R1', '64'))
R2 = int(os.environ.get('R2', '128'))
LEAD = int(os.environ.get('LEAD', '3'))
TS = int(os.environ.get('TS', '256'))
ONEPASS = int(os.environ.get('ONEPASS', '1'))
RSQ = int(os.environ.get('RSQ', '1'))
T2 = int(os.environ.get('T2', '512'))
EPS = 1e-5
_C0 = math.sqrt(2.0 / math.pi)
ALPHA = (_C0 * 0.044715) ** (1.0 / 3.0)
GC = _C0 / ALPHA
BETA = 0.5 / ALPHA
F_CHUNKS = ((0, 512), (512, 512), (1024, 512), (1536, 192))

f32 = jnp.float32
bf16 = jnp.bfloat16
u32 = jnp.uint32
NTDIMS = (((1,), (1,)), ((), ()))


def _cos_table(m, scale):
    mm = jnp.abs(((m + 256) & 511) - 256)
    x = (128 - mm).astype(f32) * (1.0 / 128.0)
    x2 = x * x
    h = math.pi / 2
    p = -(h ** 7) / 5040 + x2 * ((h ** 9) / 362880 - x2 * (h ** 11) / 39916800)
    p = h + x2 * (-(h ** 3) / 6 + x2 * ((h ** 5) / 120 + x2 * p))
    return (x * scale) * p


def _dft_tables():
    shape = (16, 8, 128)
    n = lax.broadcasted_iota(jnp.int32, shape, 0)
    s = lax.broadcasted_iota(jnp.int32, shape, 1)
    l = lax.broadcasted_iota(jnp.int32, shape, 2)
    fw, fu, iv = [], [], []
    wv = l >> 4
    tu = (16 * W) * (wv // W) + (2 * W) * ((l >> 1) & 7) + 2 * (wv % W) + (l & 1)
    for e in range(2):
        r = 2 * s + e
        j = 8 * n + (r & 7)
        fw.append(_cos_table((4 * j + 1) * l + (r >> 3) * 128, 1.0))
        fu.append(_cos_table((4 * j + 1) * tu + (r >> 3) * 128, 1.0))
        b = 16 * (n >> 1) + r
        col = 128 * (n & 1) + l
        iv.append(_cos_table((4 * (col >> 1) + 1) * b + (col & 1) * 128, 1.0 / 128.0))
    pk = lambda xs: pltpu.bitcast(pltpu.pack_elementwise(xs, packed_dtype=bf16), f32)
    return pk(fw), pk(iv), pk(fu)


def _gelu2a(z):
    return z * (1.0 + jnp.tanh(z * (z * z + GC)))


def _rstd(ssd, scale):
    if RSQ == 0:
        r = lax.rsqrt(ssd * (1.0 / D) + EPS)
        return r if scale == 1.0 else r * scale
    return jnp.exp2(jnp.log(ssd + D * EPS) * (-0.5 / math.log(2.0)) + math.log2(scale * math.sqrt(D)))


def _center(x, scale=1.0):
    s1 = jnp.sum(x, axis=-1, keepdims=True)
    m = s1 * (1.0 / D)
    d = x - m
    if ONEPASS:
        ssd = jnp.maximum(jnp.sum(x * x, axis=-1, keepdims=True) - s1 * m, 0.0)
    else:
        ssd = jnp.sum(d * d, axis=-1, keepdims=True)
    return d, _rstd(ssd, scale)


def _conv(us, gs, a):
    acc = None
    for c in range(a + 1):
        p = us[c] * gs[a - c]
        acc = p if acc is None else acc + p
    return acc


def _wt(ref, *idx):
    return pltpu.bitcast(ref[idx] if idx else ref[...], bf16)


def _kernel(q_hbm, k_hbm, v_hbm, sk_hbm, h_hbm, dd_hbm, w1_hbm, w2_hbm, w3_hbm, w4_hbm,
            c_hbm, wm_hbm, o_hbm,
            qbuf, kbuf, vbuf, hbuf, w1, w2, w3, w4, wm, wmc, modb, obuf, sk_s, dd_s, c_s,
            ub0, ub1, gb0, gb1, kb0, kb1, yb, xn, hh, h1, par, sems, osems):
    ubs, gbs, kbs = (ub0, ub1), (gb0, gb1), (kb0, kb1)
    cp = pltpu.make_async_copy
    HS = S // 2

    def cp_tile(j, i):
        r = i * HS
        sem = sems.at[2 * j + i]
        lanes = pl.ds(j * 128, 128)
        return [cp(h_hbm.at[lanes, pl.ds(r, HS)], hbuf.bitcast(bf16).at[j, :, pl.ds(r, HS)], sem),
                cp(k_hbm.at[0, pl.ds(r, HS), lanes], kbuf.bitcast(bf16).at[j, pl.ds(r + 16, HS), :], sem),
                cp(v_hbm.at[0, pl.ds(r, HS), lanes], vbuf.bitcast(bf16).at[j, pl.ds(r, HS), :], sem)]

    def cp_wm(i):
        return cp(wm_hbm.at[:, pl.ds(i * WMA, WMA)], wm.bitcast(bf16).at[i], sems.at[10 + i])

    cp_wmc = cp(wm_hbm.at[:, pl.ds(2 * WMA, WMC)], wmc.bitcast(bf16), sems.at[12])
    cp_q = [cp(q_hbm.at[0, pl.ds(r0, r1 - r0), :], qbuf.at[pl.ds(r0, r1 - r0), :], sems.at[13 + i])
            for i, (r0, r1) in enumerate(((0, Q0), (Q0, S)))]
    cp_w = [cp(s_, d_.bitcast(bf16), sems.at[15 + i])
            for i, (s_, d_) in enumerate(((w1_hbm, w1), (w2_hbm, w2), (w3_hbm, w3), (w4_hbm, w4)))]
    cp_s = [cp(sk_hbm, sk_s, sems.at[19]), cp(dd_hbm, dd_s, sems.at[19]), cp(c_hbm, c_s, sems.at[19])]
    order = list(cp_s)
    for j in range(NT):
        order += cp_tile(j, 0) + cp_tile(j, 1)
    order += [cp_wm(0), cp_wm(1), cp_q[0], cp_w[0], cp_w[1], cp_q[1], cp_w[2], cp_w[3], cp_wmc]
    for c_ in order:
        c_.start()

    with jax.named_scope("init"):
        fw_t, iv_t, fu_t = _dft_tables()
        for kb in kbs:
            kb[pl.ds(KOFF, 16)] = fw_t
            kb[pl.ds(KOFF + 16, 16)] = iv_t
            kb[pl.ds(KOFF + 32, 16)] = fu_t
            kb[pl.ds(0, NG * 3)] = jnp.zeros((NG * 3, 8, 128), f32)
        zeros = jnp.zeros((8, 128), f32)
        for j in range(NT):
            kbuf[j, pl.ds(0, 8), :] = jnp.zeros((8, 128), u32)
        for j in range(NT):
            h1[j, pl.ds(0, 8), :] = zeros
            h1[j, pl.ds(S + 8, 8), :] = zeros
        for c_ in cp_s:
            c_.wait()
        par[pl.ds(0, 4), :] = sk_s[...].astype(f32)
        par[pl.ds(8, 8), :] = jnp.broadcast_to(dd_s[...].astype(f32).reshape(1, D), (8, D))
        cv = c_s[...].astype(f32)
        sc = jnp.broadcast_to(cv * jax.nn.sigmoid(cv), (8, D))
        scp = pltpu.bitcast(pltpu.pack_elementwise([sc, sc], packed_dtype=bf16), f32)
        for j in range(NT):
            kb0[KOFF + 48 + j] = scp[:, 128 * j:128 * (j + 1)]

    def mkb(i, unr, off, cache):
        def b(stride, extra=0, z=None):
            if isinstance(i, int):
                return (i * unr + off) * stride + extra
            key = (stride, z)
            if key not in cache or NOCACHE:
                base = pl.multiple_of(i * (unr * stride), unr * stride)
                cache[key] = base if z is None else base + (i >> z)
            return cache[key] + (off * stride + extra)
        return b

    def dot_h(j, b, lhs):
        gb = gbs[j % 2]
        hc = hbuf[j, :, pl.ds(pl.multiple_of(b(512), 512), 512)]
        rhs_t = jnp.concatenate([hc[:, C * cc:C * (cc + 1)] for cc in range(4)], axis=0)
        g = lax.dot_general(lhs, pltpu.bitcast(rhs_t, bf16), NTDIMS, preferred_element_type=f32)
        for rg in range(2 * NG):
            for cc in range(4):
                gb[b(4, cc + rg * NC)] = g[8 * rg:8 * rg + 8, 128 * cc:128 * cc + 128]

    def dot_u(j, b, lhs):
        ub = ubs[j % 2]
        taps = [par[pl.ds(t, 1), pl.ds(j * 128, 128)] for t in range(4)]
        unp = lambda w_, e: pltpu.unpack_elementwise(w_, index=e, packed_dtype=bf16, unpacked_dtype=f32)
        cols = []
        for cc in range(4):
            words = []
            for blk in range(8 // W):
                w0 = 64 * cc + 8 * W * blk
                kw = {m: kbuf[j, pl.ds(b(256, 8 + w0 + m), 8, stride=W), :] for m in range(-2, W)}
                kk = {2 * m + e: unp(kw[m], e) for m in range(-2, W) for e in range(2) if 2 * m + e >= -3}
                for m in range(W):
                    vw = vbuf[j, pl.ds(b(256, w0 + m), 8, stride=W), :]
                    pair = []
                    for e in range(2):
                        n = 2 * m + e
                        ks = kk[n] * taps[0] + kk[n - 1] * taps[1] + kk[n - 2] * taps[2] + kk[n - 3] * taps[3]
                        pair.append(ks * unp(vw, e))
                    words.append(pltpu.pack_elementwise(pair, packed_dtype=bf16))
            cols.append(jnp.concatenate(words, axis=0))
        rhs = pltpu.bitcast(jnp.concatenate(cols, axis=1), bf16)
        u = jnp.dot(lhs, rhs, preferred_element_type=f32)
        for rg in range(2 * NG):
            for cc in range(4):
                ub[b(4, cc + rg * NC)] = u[8 * rg:8 * rg + 8, 128 * cc:128 * cc + 128]

    def dot_i(j, b, half, lhs):
        kb = kbs[j % 2]
        cols = [[], []]
        for gi in range(NG):
            prev = None
            for cc in range(-1, 2):
                k0, k1, k2 = [kb[b(4 * NG * 3, ((2 * half + cc + 1) * NG + gi) * 3 + t)] for t in range(3)]
                re, im = k0 - k2, k0 + k1
                if prev is not None:
                    cols[cc].append(pltpu.pack_elementwise([re - prev[1], im + prev[0]], packed_dtype=bf16))
                prev = (re, im)
        rhs = jnp.concatenate([jnp.concatenate(c_, axis=0) for c_ in cols], axis=1)
        y = jnp.dot(lhs, pltpu.bitcast(rhs, bf16), preferred_element_type=f32)
        for cc in range(2):
            yb[j, pl.ds(b(512, (2 * half + cc) * C), C), :] = y[:, 128 * cc:128 * cc + 128]

    def gen_m(j, b):
        ub, gb, kb = ubs[j % 2], gbs[j % 2], kbs[j % 2]
        for s in range(4):
            for t in range(3):
                z = 8 + t
                re = lambda ref, c: ref[b(8 * NC, 2 * s * NC + c, z)]
                im = lambda ref, c: ref[b(8 * NC, (2 * s + 1) * NC + c, z)]
                gre = [re(gb, c) for c in range(NC)]
                if t == 0:
                    us = [re(ub, c) + im(ub, c) for c in range(NC)]
                    gs = gre
                elif t == 1:
                    us = [re(ub, c) for c in range(NC)]
                    gs = [im(gb, c) - gre[c] for c in range(NC)]
                else:
                    us = [im(ub, c) for c in range(NC)]
                    gs = [im(gb, c) + gre[c] for c in range(NC)]

                def st(a, val):
                    kb[b(12, ((a + 1) * NG + s) * 3 + t)] = val
                if not KARA:
                    for a in range(NC):
                        st(a, _conv(us, gs, a))
                        yield 2 * a + 2
                    continue
                ue, uo, ge, go = us[0::2], us[1::2], gs[0::2], gs[1::2]
                usum = [x + y for x, y in zip(ue, uo)]
                gsum = [x + y for x, y in zip(ge, go)]
                poo_prev = None
                for a in range(NC // 2):
                    pee = _conv(ue, ge, a)
                    poo = _conv(uo, go, a)
                    pss = _conv(usum, gsum, a)
                    st(2 * a, pee if poo_prev is None else pee + poo_prev)
                    st(2 * a + 1, pss - pee - poo)
                    poo_prev = poo
                    yield 3 * (2 * a + 1) + 7

    def add_d(j):
        gb = gbs[j % 2]
        dvec = par[pl.ds(8, 8), pl.ds(j * 128, 128)]
        for gi in range(NG):
            gb[2 * gi * NC] = gb[2 * gi * NC] + dvec

    def sc_lhs():
        return pltpu.bitcast(jnp.concatenate([kb0[KOFF + 48 + j] for j in range(NT)], axis=1), bf16)

    def dot_m(i, t0, nt, lhs):
        m = jnp.dot(lhs, _wt(wm, i, slice(None), pl.ds(128 * t0, 128 * nt)), preferred_element_type=f32)
        for t in range(nt):
            modb[i * (WMA // 128) + (t0 + t)] = m[0:8, 128 * t:128 * (t + 1)]

    def inv_lhs(tbl, n):
        return jnp.concatenate([tbl[KOFF + 16 + 2 * n], tbl[KOFF + 17 + 2 * n]], axis=1)

    PRE = dict(H=0, U=672 + 96 // W, a=192, b=192, m=0)
    POST = dict(H=0, U=0, a=4, b=4, m=2)
    NST = dict(H=16, U=16, a=8, b=8, m=1)
    MCOST = 12 * (248 if KARA else 272)

    def a_loop(jf, jm, ji, with_mod=False):
        unr = 2
        kinds = [k_ for k_ in DORDER if (jf is not None if k_ in 'HU' else ji is not None)]
        dots = [(k_, s_) for s_ in range(unr) for k_ in kinds]
        if with_mod:
            mods = [('m', (0, 4)), ('m', (4, 4)), ('m', (8, 4)), ('m', (12, 1))]
            dots = [x for pr in zip(mods, dots) for x in pr]
        native, dur = [], []
        for idx, (k_, arg) in enumerate(dots):
            nxt = PRE[dots[idx + 1][0]] if idx + 1 < len(dots) else 0
            d_ = 2.5 * arg[1] if k_ == 'm' else 1.0
            native += [nxt / NST[k_] + POST[k_] * d_] * NST[k_]
            dur += [d_] * NST[k_]
        tbl = kbs[jm % 2] if jm is not None else kbs[0]

        def body(i, carry):
            cache = {}
            if jm is not None:
                def chain():
                    for s_ in range(unr):
                        yield from gen_m(jm, mkb(i, unr, s_, cache))
                mg = chain()
                mtot = MCOST * unr - TAIL - HEAD
                lvl = (mtot + sum(native)) / sum(dur)
                want = [max(lvl * d_ - x, 0.0) for x, d_ in zip(native, dur)]
                scale = mtot / sum(want)
                cum, tgt = [HEAD], HEAD
                for w_ in want:
                    tgt += w_ * scale
                    cum.append(tgt)
            done = 0.0
            step = 0
            for (k_, arg) in dots:
                rows = []
                for n in range(NST[k_]):
                    if jm is not None:
                        while done < cum[step]:
                            done += next(mg)
                    step += 1
                    if k_ in 'HU':
                        rows.append(tbl[KOFF + n + (32 if k_ == 'U' else 0)])
                    elif k_ in 'ab':
                        rows.append(inv_lhs(tbl, n))
                if k_ == 'm':
                    dot_m(i, arg[0], arg[1], sc_lhs())
                    continue
                lhs = pltpu.bitcast(jnp.concatenate(rows, axis=0), bf16)
                if k_ == 'H':
                    dot_h(jf, mkb(i, unr, arg, cache), lhs)
                elif k_ == 'U':
                    dot_u(jf, mkb(i, unr, arg, cache), lhs)
                else:
                    dot_i(ji, mkb(i, unr, arg, cache), 0 if k_ == 'a' else 1, lhs)
            if jm is not None:
                for _ in mg:
                    pass

            @pl.when(i == 0)
            def _():
                for c_ in (cp_tile(jf, 1) if jf is not None else [cp_wm(1)]):
                    c_.wait()
            return carry
        for c_ in (cp_tile(jf, 0) if jf is not None else [cp_wm(0)]):
            c_.wait()
        lax.fori_loop(0, 2, body, 0)

    for seg in range(NT + 1):
        jf, jm, ji = [x if 0 <= x < NT else None for x in (seg, seg - 1, seg - 2)]
        if SKIPA or seg not in SEGS:
            for i in range(2):
                for c_ in (cp_tile(jf, i) if jf is not None else [cp_wm(i)]):
                    c_.wait()
        if SKIPA or seg not in SEGS:
            continue
        with jax.named_scope(f"A_seg{seg}"):
            a_loop(jf, jm, ji, with_mod=(seg == NT))
            if jf is not None:
                add_d(jf)

    def inv_last(bt):
        lhs = pltpu.bitcast(jnp.concatenate([inv_lhs(kb1, n) for n in range(8)], axis=0), bf16)
        for half in range(2):
            dot_i(NT - 1, mkb(0, 1, bt, None), half, lhs)

    def modrow(k_):
        return jnp.concatenate([modb[NT * k_ + j] for j in range(NT)], axis=1)

    def bc(x, p):
        return x.reshape(x.shape[0] // 8, 8, D), p[None]

    def ln_chain(r, n):
        pa, pb, pc, ps = [par[pl.ds(16 + 8 * t, 8), :][None] for t in range(4)]
        g3 = lambda x: x.reshape(n // 8, 8, D)
        q = g3(qbuf[pl.ds(r, n), :].astype(f32))
        d1, r1 = _center(q)
        y = g3(jnp.concatenate([yb[j, pl.ds(r, n), :] for j in range(NT)], axis=1))
        x = q + ((d1 * r1) * pa + pb) * y
        xn[pl.ds(r, n), :] = x.reshape(n, D)
        d2, r2 = _center(x)
        h = (d2 * r2) * pc + ps
        hh[pl.ds(r, n), :] = h.reshape(n, D)
        d3, r3 = _center(h, ALPHA)
        return (d3 * r3).reshape(n, D).astype(bf16)

    def w1_dot(r, n, l3):
        z = jnp.dot(l3, _wt(w1), preferred_element_type=f32)
        g = _gelu2a(z)
        for j in range(NT):
            h1[j, pl.ds(r + 8, n), :] = g[:, j * 128:(j + 1) * 128]

    def b2a(r, n):
        lane = lax.broadcasted_iota(jnp.int32, (n, 128), 1)

        def ld(j, off):
            return h1[j, pl.ds(r + 8 + off, n), :]
        tiles = [
            ld(0, -1),
            jnp.where(lane < 32, ld(1, -1), ld(1, 1)),
            jnp.where(lane < 64, ld(2, 1), ld(2, -2)),
            jnp.where(lane < 96, ld(3, -2), ld(3, 2)),
            ld(4, 2),
        ]
        hs = jnp.concatenate(tiles, axis=1).astype(bf16)
        x1 = hh[pl.ds(r, n), :] + jnp.dot(hs, _wt(w2), preferred_element_type=f32) * BETA
        hh[pl.ds(r, n), :] = x1

    R = R1
    l3s = {}

    def do1(p):
        w1_dot(p * R, R, l3s.pop(p) if p in l3s else ln_chain(p * R, R))

    with jax.named_scope("P1"):
        cp_q[0].wait()
        sa, ca, ga, sb, cb = [modrow(k_) for k_ in range(5)]
        par[pl.ds(16, 8), :] = ga * (1.0 + ca)
        par[pl.ds(24, 8), :] = ga * sa
        par[pl.ds(32, 8), :] = 1.0 + cb
        par[pl.ds(40, 8), :] = sb
        if not SKIPA:
            for bt in range(4):
                inv_last(bt)
        for p in range(PRELN):
            l3s[p] = ln_chain(p * R, R)
    with jax.named_scope("w1wait"):
        cp_w[0].wait()
    p1 = p2 = 0
    with jax.named_scope("P2"):
        while p1 < N2:
            do1(p1)
            p1 += 1
    with jax.named_scope("w2wait"):
        cp_w[1].wait()
    with jax.named_scope("P3"):
        while p2 < Q0 // R - 3:
            b2a(p2 * R, R)
            p2 += 1
            if p1 < Q0 // R:
                do1(p1)
                p1 += 1
    with jax.named_scope("q1wait"):
        cp_q[1].wait()
    with jax.named_scope("P4"):
        for _ in range(2):
            b2a(p2 * R, R)
            p2 += 1
        while p2 < S // R and not SKIPB:
            while p1 < S // R and p1 - p2 < LEAD:
                do1(p1)
                p1 += 1
            b2a(p2 * R, R)
            p2 += 1

    def out_copy(i):
        r = pl.multiple_of(i * T2, T2)
        return cp(obuf.at[pl.ds(r, T2), :], o_hbm.at[0, pl.ds(r, T2), :], osems.at[i])

    def b2_step(i):
        gbv = par[pl.ds(48, 1), :]
        for sub in range(T2 // TS):
            r = pl.multiple_of(i * T2, T2) + sub * TS
            x1 = hh[pl.ds(r, TS), :]
            d4, r4 = _center(x1, ALPHA)
            l4 = (d4 * r4).astype(bf16)
            acc = None
            for (f0, fn) in F_CHUNKS:
                z = lax.dot_general(l4, _wt(w3, pl.ds(f0 // 2, fn // 2), slice(None)), NTDIMS, preferred_element_type=f32)
                g = _gelu2a(z).astype(bf16)
                p = jnp.dot(g, _wt(w4, pl.ds(f0 // 2, fn // 2), slice(None)), preferred_element_type=f32)
                acc = p if acc is None else acc + p
            obuf[pl.ds(r, TS), :] = (xn[pl.ds(r, TS), :] + gbv * (hh[pl.ds(r, TS), :] + BETA * acc)).astype(bf16)
        out_copy(i).start()

    with jax.named_scope("B2_wait"):
        cp_w[2].wait()
        cp_w[3].wait()
        cp_wmc.wait()
        mc = jnp.dot(sc_lhs(), _wt(wmc), preferred_element_type=f32)[0:8]
        par[pl.ds(48, 8), :] = jnp.concatenate([modb[25], mc], axis=1)
    with jax.named_scope("BII"):
        lax.fori_loop(0, S // T2, lambda i, c: (b2_step(i), c)[1], 0)
    with jax.named_scope("out_wait"):
        for i in range(S // T2):
            out_copy(i).wait()


@jax.jit
def pallas_adaLN_cond__ssm_conv_h3__mixer_s_mlp__prompt_kernel(
    A_q, A_k, A_v, A_shift_k, A_ssm_k, A_ssm_D, B_x, B_w1, B_w2, B_w3, B_w4, c, w_mod,
):
    del B_x
    hbm = pl.BlockSpec(memory_space=pltpu.MemorySpace.HBM)
    return pl.pallas_call(
        _kernel,
        out_shape=jax.ShapeDtypeStruct((1, S, D), bf16),
        in_specs=[hbm] * 12,
        out_specs=hbm,
        scratch_shapes=[
            pltpu.VMEM((S, D), bf16),
            pltpu.VMEM((NT, 8 + S // 2, 128), u32),
            pltpu.VMEM((NT, S // 2, 128), u32),
            pltpu.VMEM((NT, 64, S), u32),
            pltpu.VMEM((D // 2, D), u32),
            pltpu.VMEM((D // 2, D), u32),
            pltpu.VMEM((F // 2, D), u32),
            pltpu.VMEM((F // 2, D), u32),
            pltpu.VMEM((2, D // 2, WMA), u32),
            pltpu.VMEM((D // 2, WMC), u32),
            pltpu.VMEM((26, 8, 128), f32),
            pltpu.VMEM((S, D), bf16),
            pltpu.VMEM((4, D), bf16),
            pltpu.VMEM((D,), bf16),
            pltpu.VMEM((1, D), bf16),
            pltpu.VMEM((NG * 2 * NC, 8, 128), f32),
            pltpu.VMEM((NG * 2 * NC, 8, 128), f32),
            pltpu.VMEM((NG * 2 * NC, 8, 128), f32),
            pltpu.VMEM((NG * 2 * NC, 8, 128), f32),
            pltpu.VMEM((KOFF + 56, 8, 128), f32),
            pltpu.VMEM((KOFF + 56, 8, 128), f32),
            pltpu.VMEM((NT, S, 128), f32),
            pltpu.VMEM((S, D), f32),
            pltpu.VMEM((S, D), f32),
            pltpu.VMEM((NT, S + 16, 128), f32),
            pltpu.VMEM((56, D), f32),
            pltpu.SemaphoreType.DMA((20,)),
            pltpu.SemaphoreType.DMA((S // T2,)),
        ],
        compiler_params=pltpu.CompilerParams(vmem_limit_bytes=100 * 1024 * 1024, disable_semaphore_checks=True),
    )(A_q, A_k, A_v, A_shift_k.T, A_ssm_k, A_ssm_D, B_w1, B_w2, B_w3.T, B_w4, c, w_mod)
```

```python
import math
import os

import jax
import jax.numpy as jnp
from jax import lax
import jax.experimental.pallas as pl
import jax.experimental.pallas.tpu as pltpu

S, D, F = 2048, 640, 1728
C = 128
NC = S // C
NT = D // 128
NG = 16
KOFF = (NC + 1) * NG * 3
W = int(os.environ.get('W', '4'))
SKIPA = int(os.environ.get('SKIPA', '0'))
WMA, WMP, WMC = 1280, 640, 640
Q0 = int(os.environ.get('Q0', '512'))
N2 = int(os.environ.get('N2', '5'))
PRELN = int(os.environ.get('PRELN', '2'))
NOCACHE = int(os.environ.get('NOCACHE', '0'))
OUTWAIT = int(os.environ.get('OUTWAIT', '0'))
SEGS = [int(x) for x in os.environ.get('SEGS', '012345')]
SKIPB = int(os.environ.get('SKIPB', '0'))
PADK = int(os.environ.get('PADK', '0'))
KARA = int(os.environ.get('KARA', '1'))
UNR = int(os.environ.get('UNR', '2'))
HEAD = int(os.environ.get('HEAD', '250'))
TAIL = int(os.environ.get('TAIL', '450'))
DORDER = os.environ.get('DORDER', 'HaUb')
R1 = int(os.environ.get('R1', '64'))
R2 = int(os.environ.get('R2', '128'))
LEAD = int(os.environ.get('LEAD', '3'))
TS = int(os.environ.get('TS', '256'))
ONEPASS = int(os.environ.get('ONEPASS', '1'))
RSQ = int(os.environ.get('RSQ', '1'))
T2 = int(os.environ.get('T2', '512'))
EPS = 1e-5
_C0 = math.sqrt(2.0 / math.pi)
ALPHA = (_C0 * 0.044715) ** (1.0 / 3.0)
GC = _C0 / ALPHA
BETA = 0.5 / ALPHA
_fc = [int(x) for x in os.environ.get('FC', '192,512,512,512').split(',')]
F_CHUNKS = tuple((sum(_fc[:i]), _fc[i]) for i in range(len(_fc)))
assert sum(_fc) == F

f32 = jnp.float32
bf16 = jnp.bfloat16
u32 = jnp.uint32
NTDIMS = (((1,), (1,)), ((), ()))


def _cos_table(m, scale):
    mm = jnp.abs(((m + 256) & 511) - 256)
    x = (128 - mm).astype(f32) * (1.0 / 128.0)
    x2 = x * x
    h = math.pi / 2
    p = -(h ** 7) / 5040 + x2 * ((h ** 9) / 362880 - x2 * (h ** 11) / 39916800)
    p = h + x2 * (-(h ** 3) / 6 + x2 * ((h ** 5) / 120 + x2 * p))
    return (x * scale) * p


def _dft_tables():
    shape = (16, 8, 128)
    n = lax.broadcasted_iota(jnp.int32, shape, 0)
    s = lax.broadcasted_iota(jnp.int32, shape, 1)
    l = lax.broadcasted_iota(jnp.int32, shape, 2)
    fw, fu, iv = [], [], []
    wv = l >> 4
    tu = (16 * W) * (wv // W) + (2 * W) * ((l >> 1) & 7) + 2 * (wv % W) + (l & 1)
    for e in range(2):
        r = 2 * s + e
        j = 8 * n + (r & 7)
        fw.append(_cos_table((4 * j + 1) * l + (r >> 3) * 128, 1.0))
        fu.append(_cos_table((4 * j + 1) * tu + (r >> 3) * 128, 1.0))
        b = 16 * (n >> 1) + r
        col = 128 * (n & 1) + l
        iv.append(_cos_table((4 * (col >> 1) + 1) * b + (col & 1) * 128, 1.0 / 128.0))
    pk = lambda xs: pltpu.bitcast(pltpu.pack_elementwise(xs, packed_dtype=bf16), f32)
    return pk(fw), pk(iv), pk(fu)


def _gelu2a(z):
    return z * (1.0 + jnp.tanh(z * (z * z + GC)))


def _rstd(ssd, scale):
    if RSQ == 0:
        r = lax.rsqrt(ssd * (1.0 / D) + EPS)
        return r if scale == 1.0 else r * scale
    return jnp.exp2(jnp.log(ssd + D * EPS) * (-0.5 / math.log(2.0)) + math.log2(scale * math.sqrt(D)))


def _center(x, scale=1.0):
    s1 = jnp.sum(x, axis=-1, keepdims=True)
    m = s1 * (1.0 / D)
    d = x - m
    if ONEPASS:
        ssd = jnp.maximum(jnp.sum(x * x, axis=-1, keepdims=True) - s1 * m, 0.0)
    else:
        ssd = jnp.sum(d * d, axis=-1, keepdims=True)
    return d, _rstd(ssd, scale)


def _conv(us, gs, a):
    acc = None
    for c in range(a + 1):
        p = us[c] * gs[a - c]
        acc = p if acc is None else acc + p
    return acc


def _wt(ref, *idx):
    return pltpu.bitcast(ref[idx] if idx else ref[...], bf16)


def _kernel(q_hbm, k_hbm, v_hbm, sk_hbm, h_hbm, dd_hbm, w1_hbm, w2_hbm, w3_hbm, w4_hbm,
            c_hbm, wm_hbm, o_hbm,
            qbuf, kbuf, vbuf, hbuf, w1, w2, w3, w4, wm, wmp, wmc, modb, obuf, sk_s, dd_s, c_s,
            ub0, ub1, gb0, gb1, kb0, kb1, yb, xn, hh, h1, par, sems, osems):
    ubs, gbs, kbs = (ub0, ub1), (gb0, gb1), (kb0, kb1)
    cp = pltpu.make_async_copy
    HS = S // 2

    def cp_tile(j, i):
        r = i * HS
        sem = sems.at[2 * j + i]
        lanes = pl.ds(j * 128, 128)
        return [cp(h_hbm.at[lanes, pl.ds(r, HS)], hbuf.bitcast(bf16).at[j, :, pl.ds(r, HS)], sem),
                cp(k_hbm.at[0, pl.ds(r, HS), lanes], kbuf.bitcast(bf16).at[j, pl.ds(r + 16, HS), :], sem),
                cp(v_hbm.at[0, pl.ds(r, HS), lanes], vbuf.bitcast(bf16).at[j, pl.ds(r, HS), :], sem)]

    def cp_wm(i):
        return cp(wm_hbm.at[:, pl.ds(i * WMA, WMA)], wm.bitcast(bf16).at[i], sems.at[10 + i])

    cp_wmp = cp(wm_hbm.at[:, pl.ds(2 * WMA, WMP)], wmp.bitcast(bf16), sems.at[13])
    cp_wmc = cp(wm_hbm.at[:, pl.ds(2 * WMA + WMP, WMC)], wmc.bitcast(bf16), sems.at[12])
    cp_q = [cp(q_hbm.at[0, pl.ds(r0, r1 - r0), :], qbuf.at[pl.ds(r0, r1 - r0), :], sems.at[13 + i])
            for i, (r0, r1) in enumerate(((0, Q0), (Q0, S)))]
    cp_w = [cp(s_, d_.bitcast(bf16), sems.at[15 + i])
            for i, (s_, d_) in enumerate(((w1_hbm, w1), (w2_hbm, w2), (w3_hbm, w3), (w4_hbm, w4)))]
    cp_s = [cp(sk_hbm, sk_s, sems.at[19]), cp(dd_hbm, dd_s, sems.at[19]), cp(c_hbm, c_s, sems.at[19])]
    order = list(cp_s)
    for j in range(NT):
        order += cp_tile(j, 0) + cp_tile(j, 1)
    order += [cp_wm(0), cp_wm(1), cp_wmp, cp_q[0], cp_w[0], cp_w[1], cp_q[1], cp_w[2], cp_w[3], cp_wmc]
    for c_ in order:
        c_.start()

    with jax.named_scope("init"):
        fw_t, iv_t, fu_t = _dft_tables()
        for kb in kbs:
            kb[pl.ds(KOFF, 16)] = fw_t
            kb[pl.ds(KOFF + 16, 16)] = iv_t
            kb[pl.ds(KOFF + 32, 16)] = fu_t
            kb[pl.ds(0, NG * 3)] = jnp.zeros((NG * 3, 8, 128), f32)
        zeros = jnp.zeros((8, 128), f32)
        for j in range(NT):
            kbuf[j, pl.ds(0, 8), :] = jnp.zeros((8, 128), u32)
        for j in range(NT):
            h1[j, pl.ds(0, 8), :] = zeros
            h1[j, pl.ds(S + 8, 8), :] = zeros
        for c_ in cp_s:
            c_.wait()
        par[pl.ds(0, 4), :] = sk_s[...].astype(f32)
        par[pl.ds(8, 8), :] = jnp.broadcast_to(dd_s[...].astype(f32).reshape(1, D), (8, D))
        cv = c_s[...].astype(f32)
        sc = jnp.broadcast_to(cv * jax.nn.sigmoid(cv), (8, D))
        scp = pltpu.bitcast(pltpu.pack_elementwise([sc, sc], packed_dtype=bf16), f32)
        for j in range(NT):
            kb0[KOFF + 48 + j] = scp[:, 128 * j:128 * (j + 1)]

    def mkb(i, unr, off, cache):
        def b(stride, extra=0, z=None):
            if isinstance(i, int):
                return (i * unr + off) * stride + extra
            key = (stride, z)
            if key not in cache or NOCACHE:
                base = pl.multiple_of(i * (unr * stride), unr * stride)
                cache[key] = base if z is None else base + (i >> z)
            return cache[key] + (off * stride + extra)
        return b

    def dot_h(j, b, lhs):
        gb = gbs[j % 2]
        hc = hbuf[j, :, pl.ds(pl.multiple_of(b(512), 512), 512)]
        rhs_t = jnp.concatenate([hc[:, C * cc:C * (cc + 1)] for cc in range(4)], axis=0)
        g = lax.dot_general(lhs, pltpu.bitcast(rhs_t, bf16), NTDIMS, preferred_element_type=f32)
        for rg in range(2 * NG):
            for cc in range(4):
                gb[b(4, cc + rg * NC)] = g[8 * rg:8 * rg + 8, 128 * cc:128 * cc + 128]

    def dot_u(j, b, lhs):
        ub = ubs[j % 2]
        taps = [par[pl.ds(t, 1), pl.ds(j * 128, 128)] for t in range(4)]
        unp = lambda w_, e: pltpu.unpack_elementwise(w_, index=e, packed_dtype=bf16, unpacked_dtype=f32)
        cols = []
        for cc in range(4):
            words = []
            for blk in range(8 // W):
                w0 = 64 * cc + 8 * W * blk
                kw = {m: kbuf[j, pl.ds(b(256, 8 + w0 + m), 8, stride=W), :] for m in range(-2, W)}
                kk = {2 * m + e: unp(kw[m], e) for m in range(-2, W) for e in range(2) if 2 * m + e >= -3}
                for m in range(W):
                    vw = vbuf[j, pl.ds(b(256, w0 + m), 8, stride=W), :]
                    pair = []
                    for e in range(2):
                        n = 2 * m + e
                        ks = kk[n] * taps[0] + kk[n - 1] * taps[1] + kk[n - 2] * taps[2] + kk[n - 3] * taps[3]
                        pair.append(ks * unp(vw, e))
                    words.append(pltpu.pack_elementwise(pair, packed_dtype=bf16))
            cols.append(jnp.concatenate(words, axis=0))
        rhs = pltpu.bitcast(jnp.concatenate(cols, axis=1), bf16)
        u = jnp.dot(lhs, rhs, preferred_element_type=f32)
        for rg in range(2 * NG):
            for cc in range(4):
                ub[b(4, cc + rg * NC)] = u[8 * rg:8 * rg + 8, 128 * cc:128 * cc + 128]

    def dot_i(j, b, half, lhs):
        kb = kbs[j % 2]
        cols = [[], []]
        for gi in range(NG):
            prev = None
            for cc in range(-1, 2):
                k0, k1, k2 = [kb[b(4 * NG * 3, ((2 * half + cc + 1) * NG + gi) * 3 + t)] for t in range(3)]
                re, im = k0 - k2, k0 + k1
                if prev is not None:
                    cols[cc].append(pltpu.pack_elementwise([re - prev[1], im + prev[0]], packed_dtype=bf16))
                prev = (re, im)
        rhs = jnp.concatenate([jnp.concatenate(c_, axis=0) for c_ in cols], axis=1)
        y = jnp.dot(lhs, pltpu.bitcast(rhs, bf16), preferred_element_type=f32)
        for cc in range(2):
            yb[j, pl.ds(b(512, (2 * half + cc) * C), C), :] = y[:, 128 * cc:128 * cc + 128]

    def gen_m(j, b):
        ub, gb, kb = ubs[j % 2], gbs[j % 2], kbs[j % 2]
        for s in range(4):
            for t in range(3):
                z = 8 + t
                re = lambda ref, c: ref[b(8 * NC, 2 * s * NC + c, z)]
                im = lambda ref, c: ref[b(8 * NC, (2 * s + 1) * NC + c, z)]
                gre = [re(gb, c) for c in range(NC)]
                if t == 0:
                    us = [re(ub, c) + im(ub, c) for c in range(NC)]
                    gs = gre
                elif t == 1:
                    us = [re(ub, c) for c in range(NC)]
                    gs = [im(gb, c) - gre[c] for c in range(NC)]
                else:
                    us = [im(ub, c) for c in range(NC)]
                    gs = [im(gb, c) + gre[c] for c in range(NC)]

                def st(a, val):
                    kb[b(12, ((a + 1) * NG + s) * 3 + t)] = val
                if not KARA:
                    for a in range(NC):
                        st(a, _conv(us, gs, a))
                        yield 2 * a + 2
                    continue
                ue, uo, ge, go = us[0::2], us[1::2], gs[0::2], gs[1::2]
                usum = [x + y for x, y in zip(ue, uo)]
                gsum = [x + y for x, y in zip(ge, go)]
                poo_prev = None
                for a in range(NC // 2):
                    pee = _conv(ue, ge, a)
                    poo = _conv(uo, go, a)
                    pss = _conv(usum, gsum, a)
                    st(2 * a, pee if poo_prev is None else pee + poo_prev)
                    st(2 * a + 1, pss - pee - poo)
                    poo_prev = poo
                    yield 3 * (2 * a + 1) + 7

    def add_d(j):
        gb = gbs[j % 2]
        dvec = par[pl.ds(8, 8), pl.ds(j * 128, 128)]
        for gi in range(NG):
            gb[2 * gi * NC] = gb[2 * gi * NC] + dvec

    def sc_lhs():
        return pltpu.bitcast(jnp.concatenate([kb0[KOFF + 48 + j] for j in range(NT)], axis=1), bf16)

    def dot_m(i, t0, nt, rows):
        m = None
        for kt in range(NT):
            p = jnp.dot(pltpu.bitcast(rows[kt], bf16), _wt(wm, i, pl.ds(64 * kt, 64), pl.ds(128 * t0, 128 * nt)),
                        preferred_element_type=f32)
            m = p if m is None else m + p
        for t in range(nt):
            modb[i * (WMA // 128) + (t0 + t)] = m[0:8, 128 * t:128 * (t + 1)]

    def inv_lhs(tbl, n):
        return jnp.concatenate([tbl[KOFF + 16 + 2 * n], tbl[KOFF + 17 + 2 * n]], axis=1)

    PRE = dict(H=0, U=672 + 96 // W, a=192, b=192, m=0)
    POST = dict(H=0, U=0, a=4, b=4, m=2)
    NST = dict(H=16, U=16, a=8, b=8, m=5)
    MCOST = 12 * (248 if KARA else 272)

    def a_loop(jf, jm, ji, with_mod=False):
        unr = 2
        kinds = [k_ for k_ in DORDER if (jf is not None if k_ in 'HU' else ji is not None)]
        dots = [(k_, s_) for s_ in range(unr) for k_ in kinds]
        if with_mod:
            dots = [('m', (0, 4)), dots[0], ('m', (4, 4)), dots[1], ('m', (8, 2))] + dots[2:]
        native, dur = [], []
        for idx, (k_, arg) in enumerate(dots):
            nxt = PRE[dots[idx + 1][0]] if idx + 1 < len(dots) else 0
            d_ = 2.0 if k_ == 'm' else 1.0
            native += [nxt / NST[k_] + POST[k_] * d_] * NST[k_]
            dur += [d_] * NST[k_]
        tbl = kbs[jm % 2] if jm is not None else kbs[0]

        def body(i, carry):
            cache = {}
            if jm is not None:
                def chain():
                    for s_ in range(unr):
                        yield from gen_m(jm, mkb(i, unr, s_, cache))
                mg = chain()
                mtot = MCOST * unr - TAIL - HEAD
                lvl = (mtot + sum(native)) / sum(dur)
                want = [max(lvl * d_ - x, 0.0) for x, d_ in zip(native, dur)]
                scale = mtot / sum(want)
                cum, tgt = [HEAD], HEAD
                for w_ in want:
                    tgt += w_ * scale
                    cum.append(tgt)
            done = 0.0
            step = 0
            for (k_, arg) in dots:
                rows = []
                for n in range(NST[k_]):
                    if jm is not None:
                        while done < cum[step]:
                            done += next(mg)
                    step += 1
                    if k_ in 'HU':
                        rows.append(tbl[KOFF + n + (32 if k_ == 'U' else 0)])
                    elif k_ in 'ab':
                        rows.append(inv_lhs(tbl, n))
                    else:
                        rows.append(kb0[KOFF + 48 + n])
                if k_ == 'm':
                    dot_m(i, arg[0], arg[1], rows)
                    continue
                lhs = pltpu.bitcast(jnp.concatenate(rows, axis=0), bf16)
                if k_ == 'H':
                    dot_h(jf, mkb(i, unr, arg, cache), lhs)
                elif k_ == 'U':
                    dot_u(jf, mkb(i, unr, arg, cache), lhs)
                else:
                    dot_i(ji, mkb(i, unr, arg, cache), 0 if k_ == 'a' else 1, lhs)
            if jm is not None:
                for _ in mg:
                    pass

            @pl.when(i == 0)
            def _():
                for c_ in (cp_tile(jf, 1) if jf is not None else [cp_wm(1)]):
                    c_.wait()
            return carry
        for c_ in (cp_tile(jf, 0) if jf is not None else [cp_wm(0)]):
            c_.wait()
        lax.fori_loop(0, 2, body, 0)

    for seg in range(NT + 1):
        jf, jm, ji = [x if 0 <= x < NT else None for x in (seg, seg - 1, seg - 2)]
        if SKIPA or seg not in SEGS:
            for i in range(2):
                for c_ in (cp_tile(jf, i) if jf is not None else [cp_wm(i)]):
                    c_.wait()
        if SKIPA or seg not in SEGS:
            continue
        with jax.named_scope(f"A_seg{seg}"):
            a_loop(jf, jm, ji, with_mod=(seg == NT))
            if jf is not None:
                add_d(jf)

    def inv_last(bt):
        lhs = pltpu.bitcast(jnp.concatenate([inv_lhs(kb1, n) for n in range(8)], axis=0), bf16)
        for half in range(2):
            dot_i(NT - 1, mkb(0, 1, bt, None), half, lhs)

    def modrow(k_):
        return jnp.concatenate([modb[NT * k_ + j] for j in range(NT)], axis=1)

    def bc(x, p):
        return x.reshape(x.shape[0] // 8, 8, D), p[None]

    def ln_chain(r, n):
        pa, pb, pc, ps = [par[pl.ds(16 + 8 * t, 8), :][None] for t in range(4)]
        g3 = lambda x: x.reshape(n // 8, 8, D)
        q = g3(qbuf[pl.ds(r, n), :].astype(f32))
        d1, r1 = _center(q)
        y = g3(jnp.concatenate([yb[j, pl.ds(r, n), :] for j in range(NT)], axis=1))
        x = q + ((d1 * r1) * pa + pb) * y
        xn[pl.ds(r, n), :] = x.reshape(n, D)
        d2, r2 = _center(x)
        h = (d2 * r2) * pc + ps
        hh[pl.ds(r, n), :] = h.reshape(n, D)
        d3, r3 = _center(h, ALPHA)
        return (d3 * r3).reshape(n, D).astype(bf16)

    def w1_dot(r, n, l3):
        z = jnp.dot(l3, _wt(w1), preferred_element_type=f32)
        g = _gelu2a(z)
        for j in range(NT):
            h1[j, pl.ds(r + 8, n), :] = g[:, j * 128:(j + 1) * 128]

    def b2a(r, n):
        lane = lax.broadcasted_iota(jnp.int32, (n, 128), 1)

        def ld(j, off):
            return h1[j, pl.ds(r + 8 + off, n), :]
        tiles = [
            ld(0, -1),
            jnp.where(lane < 32, ld(1, -1), ld(1, 1)),
            jnp.where(lane < 64, ld(2, 1), ld(2, -2)),
            jnp.where(lane < 96, ld(3, -2), ld(3, 2)),
            ld(4, 2),
        ]
        hs = jnp.concatenate(tiles, axis=1).astype(bf16)
        x1 = hh[pl.ds(r, n), :] + jnp.dot(hs, _wt(w2), preferred_element_type=f32) * BETA
        hh[pl.ds(r, n), :] = x1

    R = R1
    l3s = {}

    def do1(p):
        w1_dot(p * R, R, l3s.pop(p) if p in l3s else ln_chain(p * R, R))

    with jax.named_scope("P1"):
        cp_wmp.wait()
        cp_q[0].wait()
        mp = jnp.dot(sc_lhs(), _wt(wmp), preferred_element_type=f32)
        for t in range(WMP // 128):
            modb[2 * WMA // 128 + t] = mp[0:8, 128 * t:128 * (t + 1)]
        sa, ca, ga, sb, cb = [modrow(k_) for k_ in range(5)]
        par[pl.ds(16, 8), :] = ga * (1.0 + ca)
        par[pl.ds(24, 8), :] = ga * sa
        par[pl.ds(32, 8), :] = 1.0 + cb
        par[pl.ds(40, 8), :] = sb
        if not SKIPA:
            for bt in range(4):
                inv_last(bt)
        for p in range(PRELN):
            l3s[p] = ln_chain(p * R, R)
    with jax.named_scope("w1wait"):
        cp_w[0].wait()
    p1 = p2 = 0
    with jax.named_scope("P2"):
        while p1 < N2:
            do1(p1)
            p1 += 1
    with jax.named_scope("w2wait"):
        cp_w[1].wait()
    with jax.named_scope("P3"):
        while p2 < Q0 // R - 3:
            b2a(p2 * R, R)
            p2 += 1
            if p1 < Q0 // R:
                do1(p1)
                p1 += 1
    with jax.named_scope("q1wait"):
        cp_q[1].wait()
    with jax.named_scope("P4"):
        for _ in range(2):
            b2a(p2 * R, R)
            p2 += 1
        while p2 < S // R and not SKIPB:
            while p1 < S // R and p1 - p2 < LEAD:
                do1(p1)
                p1 += 1
            b2a(p2 * R, R)
            p2 += 1

    def out_copy(r):
        return cp(obuf.at[pl.ds(r, TS), :], o_hbm.at[0, pl.ds(r, TS), :], osems.at[0])

    def b2_step(i):
        gbv = par[pl.ds(48, 1), :]
        for sub in range(T2 // TS):
            r = pl.multiple_of(pl.multiple_of(i * T2, T2) + sub * TS, TS)
            x1 = hh[pl.ds(r, TS), :]
            d4, r4 = _center(x1, ALPHA)
            l4 = (d4 * r4).astype(bf16)
            acc = None
            for (f0, fn) in F_CHUNKS:
                z = lax.dot_general(l4, _wt(w3, pl.ds(f0 // 2, fn // 2), slice(None)), NTDIMS, preferred_element_type=f32)
                g = _gelu2a(z).astype(bf16)
                p = jnp.dot(g, _wt(w4, pl.ds(f0 // 2, fn // 2), slice(None)), preferred_element_type=f32)
                acc = p if acc is None else acc + p
            obuf[pl.ds(r, TS), :] = (xn[pl.ds(r, TS), :] + gbv * (hh[pl.ds(r, TS), :] + BETA * acc)).astype(bf16)
            out_copy(r).start()

    with jax.named_scope("B2_wait"):
        cp_w[2].wait()
        cp_w[3].wait()
        cp_wmc.wait()
        mc = jnp.dot(sc_lhs(), _wt(wmc), preferred_element_type=f32)[0:8]
        par[pl.ds(48, 8), :] = mc
    with jax.named_scope("BII"):
        lax.fori_loop(0, S // T2, lambda i, c: (b2_step(i), c)[1], 0)
    with jax.named_scope("out_wait"):
        for i in range(S // TS):
            out_copy(i * TS).wait()


@jax.jit
def pallas_adaLN_cond__ssm_conv_h3__mixer_s_mlp__prompt_kernel(
    A_q, A_k, A_v, A_shift_k, A_ssm_k, A_ssm_D, B_x, B_w1, B_w2, B_w3, B_w4, c, w_mod,
):
    del B_x
    hbm = pl.BlockSpec(memory_space=pltpu.MemorySpace.HBM)
    return pl.pallas_call(
        _kernel,
        out_shape=jax.ShapeDtypeStruct((1, S, D), bf16),
        in_specs=[hbm] * 12,
        out_specs=hbm,
        scratch_shapes=[
            pltpu.VMEM((S, D), bf16),
            pltpu.VMEM((NT, 8 + S // 2, 128), u32),
            pltpu.VMEM((NT, S // 2, 128), u32),
            pltpu.VMEM((NT, 64, S), u32),
            pltpu.VMEM((D // 2, D), u32),
            pltpu.VMEM((D // 2, D), u32),
            pltpu.VMEM((F // 2, D), u32),
            pltpu.VMEM((F // 2, D), u32),
            pltpu.VMEM((2, D // 2, WMA), u32),
            pltpu.VMEM((D // 2, WMP), u32),
            pltpu.VMEM((D // 2, WMC), u32),
            pltpu.VMEM((26 + int(os.environ.get('PADM', '2')), 8, 128), f32),
            pltpu.VMEM((S, D), bf16),
            pltpu.VMEM((4, D), bf16),
            pltpu.VMEM((D,), bf16),
            pltpu.VMEM((1, D), bf16),
            pltpu.VMEM((NG * 2 * NC, 8, 128), f32),
            pltpu.VMEM((NG * 2 * NC, 8, 128), f32),
            pltpu.VMEM((NG * 2 * NC, 8, 128), f32),
            pltpu.VMEM((NG * 2 * NC, 8, 128), f32),
            pltpu.VMEM((KOFF + 56 + PADK, 8, 128), f32),
            pltpu.VMEM((KOFF + 56 + PADK, 8, 128), f32),
            pltpu.VMEM((NT, S, 128), f32),
            pltpu.VMEM((S, D), f32),
            pltpu.VMEM((S, D), f32),
            pltpu.VMEM((NT, S + 16, 128), f32),
            pltpu.VMEM((56, D), f32),
            pltpu.SemaphoreType.DMA((20,)),
            pltpu.SemaphoreType.DMA((1,)),
        ],
        compiler_params=pltpu.CompilerParams(vmem_limit_bytes=100 * 1024 * 1024, disable_semaphore_checks=True,
                                             disable_bounds_checks=bool(int(os.environ.get('NOBC', '0')))),
    )(A_q, A_k, A_v, A_shift_k.T, A_ssm_k, A_ssm_D, B_w1, B_w2, B_w3.T, B_w4, c, w_mod)
```

```python
import math
import os

import jax
import jax.numpy as jnp
from jax import lax
import jax.experimental.pallas as pl
import jax.experimental.pallas.tpu as pltpu

S, D, F = 2048, 640, 1728
C = 128
NC = S // C
NT = D // 128
NG = 16
KOFF = (NC + 1) * NG * 3
W = int(os.environ.get('W', '4'))
SKIPA = int(os.environ.get('SKIPA', '0'))
WMA, WMP, WMC = 1280, 640, 640
Q0 = int(os.environ.get('Q0', '512'))
N2 = int(os.environ.get('N2', '5'))
PRELN = int(os.environ.get('PRELN', '2'))
NOCACHE = int(os.environ.get('NOCACHE', '0'))
OUTWAIT = int(os.environ.get('OUTWAIT', '0'))
SEGS = [int(x) for x in os.environ.get('SEGS', '012345')]
SKIPB = int(os.environ.get('SKIPB', '0'))
PADK = int(os.environ.get('PADK', '0'))
PREW = int(os.environ.get('PREW', '0'))
SP = float(os.environ.get('SP', '0'))
MINS = int(os.environ.get('MINS', '30'))
GA = int(os.environ.get('GA', '2'))
TRT = int(os.environ.get('TRT', '1'))
LP = int(os.environ.get('LP', '1'))
FA = 1664
LPN = int(os.environ.get('LPN', '2'))
KARA = int(os.environ.get('KARA', '1'))
UNR = int(os.environ.get('UNR', '2'))
HEAD = int(os.environ.get('HEAD', '250'))
TAIL = int(os.environ.get('TAIL', '450'))
DORDER = os.environ.get('DORDER', 'HaUb')
R1 = int(os.environ.get('R1', '64'))
R2 = int(os.environ.get('R2', '128'))
LEAD = int(os.environ.get('LEAD', '4'))
TS = int(os.environ.get('TS', '256'))
ONEPASS = int(os.environ.get('ONEPASS', '1'))
RSQ = int(os.environ.get('RSQ', '1'))
T2 = int(os.environ.get('T2', '512'))
EPS = 1e-5
_C0 = math.sqrt(2.0 / math.pi)
ALPHA = (_C0 * 0.044715) ** (1.0 / 3.0)
GC = _C0 / ALPHA
BETA = 0.5 / ALPHA
_fc = [int(x) for x in os.environ.get('FC', '1728').split(',')]
F_CHUNKS = tuple((sum(_fc[:i]), _fc[i]) for i in range(len(_fc)))
assert sum(_fc) == F

f32 = jnp.float32
bf16 = jnp.bfloat16
u32 = jnp.uint32
NTDIMS = (((1,), (1,)), ((), ()))


def _cos_table(m, scale):
    mm = jnp.abs(((m + 256) & 511) - 256)
    x = (128 - mm).astype(f32) * (1.0 / 128.0)
    x2 = x * x
    h = math.pi / 2
    p = -(h ** 7) / 5040 + x2 * ((h ** 9) / 362880 - x2 * (h ** 11) / 39916800)
    p = h + x2 * (-(h ** 3) / 6 + x2 * ((h ** 5) / 120 + x2 * p))
    return (x * scale) * p


def _dft_tables():
    shape = (16, 8, 128)
    n = lax.broadcasted_iota(jnp.int32, shape, 0)
    s = lax.broadcasted_iota(jnp.int32, shape, 1)
    l = lax.broadcasted_iota(jnp.int32, shape, 2)
    fw, fu, iv = [], [], []
    wv = l >> 4
    tu = (16 * W) * (wv // W) + (2 * W) * ((l >> 1) & 7) + 2 * (wv % W) + (l & 1)
    for e in range(2):
        r = 2 * s + e
        j = 8 * n + (r & 7)
        fw.append(_cos_table((4 * j + 1) * l + (r >> 3) * 128, 1.0))
        fu.append(_cos_table((4 * j + 1) * tu + (r >> 3) * 128, 1.0))
        b = 16 * (n >> 1) + r
        col = 128 * (n & 1) + l
        iv.append(_cos_table((4 * (col >> 1) + 1) * b + (col & 1) * 128, 1.0 / 128.0))
    pk = lambda xs: pltpu.bitcast(pltpu.pack_elementwise(xs, packed_dtype=bf16), f32)
    return pk(fw), pk(iv), pk(fu)


def _gelu2a(z):
    return z * (1.0 + jnp.tanh(z * (z * z + GC)))


def _rstd(ssd, scale):
    if RSQ == 0:
        r = lax.rsqrt(ssd * (1.0 / D) + EPS)
        return r if scale == 1.0 else r * scale
    return jnp.exp2(jnp.log(ssd + D * EPS) * (-0.5 / math.log(2.0)) + math.log2(scale * math.sqrt(D)))


def _center(x, scale=1.0):
    s1 = jnp.sum(x, axis=-1, keepdims=True)
    m = s1 * (1.0 / D)
    d = x - m
    if ONEPASS:
        ssd = jnp.maximum(jnp.sum(x * x, axis=-1, keepdims=True) - s1 * m, 0.0)
    else:
        ssd = jnp.sum(d * d, axis=-1, keepdims=True)
    return d, _rstd(ssd, scale)


def _conv(us, gs, a):
    acc = None
    for c in range(a + 1):
        p = us[c] * gs[a - c]
        acc = p if acc is None else acc + p
    return acc


def _wt(ref, *idx):
    return pltpu.bitcast(ref[idx] if idx else ref[...], bf16)


def _kernel(q_hbm, k_hbm, v_hbm, sk_hbm, h_hbm, dd_hbm, w1_hbm, w2_hbm, w3_hbm, w4_hbm,
            c_hbm, wm_hbm, o_hbm,
            qbuf, kbuf, vbuf, hbuf, w1, w2, w3, w4, wm, wmp, wmc, modb, obuf, sk_s, dd_s, c_s,
            ub0, ub1, gb0, gb1, kb0, kb1, yb, xn, hh, h1, par, l4p, sems, osems):
    ubs, gbs, kbs = (ub0, ub1), (gb0, gb1), (kb0, kb1)
    cp = pltpu.make_async_copy
    HS = S // 2

    def cp_tile(j, i):
        r = i * HS
        sem = sems.at[2 * j + i]
        lanes = pl.ds(j * 128, 128)
        return [cp(h_hbm.at[lanes, pl.ds(r, HS)], hbuf.bitcast(bf16).at[j, :, pl.ds(r, HS)], sem),
                cp(k_hbm.at[0, pl.ds(r, HS), lanes], kbuf.bitcast(bf16).at[j, pl.ds(r + 16, HS), :], sem),
                cp(v_hbm.at[0, pl.ds(r, HS), lanes], vbuf.bitcast(bf16).at[j, pl.ds(r, HS), :], sem)]

    def cp_wm(i):
        return cp(wm_hbm.at[:, pl.ds(i * WMA, WMA)], wm.bitcast(bf16).at[i], sems.at[10 + i])

    cp_wmp = cp(wm_hbm.at[:, pl.ds(2 * WMA, WMP)], wmp.bitcast(bf16), sems.at[13])
    cp_wmc = cp(wm_hbm.at[:, pl.ds(2 * WMA + WMP, WMC)], wmc.bitcast(bf16), sems.at[12])
    cp_q = [cp(q_hbm.at[0, pl.ds(r0, r1 - r0), :], qbuf.at[pl.ds(r0, r1 - r0), :], sems.at[13 + i])
            for i, (r0, r1) in enumerate(((0, Q0), (Q0, S)))]
    cp_w = [cp(s_, d_.bitcast(bf16), sems.at[15 + i])
            for i, (s_, d_) in enumerate(((w1_hbm, w1), (w2_hbm, w2), (w3_hbm, w3), (w4_hbm, w4)))]
    cp_s = [cp(sk_hbm, sk_s, sems.at[19]), cp(dd_hbm, dd_s, sems.at[19]), cp(c_hbm, c_s, sems.at[19])]
    order = list(cp_s)
    for j in range(NT):
        order += cp_tile(j, 0) + cp_tile(j, 1)
    order += [cp_wm(0), cp_wm(1), cp_wmp, cp_q[0], cp_w[0], cp_w[1], cp_q[1], cp_w[2], cp_w[3], cp_wmc]
    for c_ in order:
        c_.start()

    with jax.named_scope("init"):
        fw_t, iv_t, fu_t = _dft_tables()
        for kb in kbs:
            kb[pl.ds(KOFF, 16)] = fw_t
            kb[pl.ds(KOFF + 16, 16)] = iv_t
            kb[pl.ds(KOFF + 32, 16)] = fu_t
            kb[pl.ds(0, NG * 3)] = jnp.zeros((NG * 3, 8, 128), f32)
        zeros = jnp.zeros((8, 128), f32)
        for j in range(NT):
            kbuf[j, pl.ds(0, 8), :] = jnp.zeros((8, 128), u32)
        for j in range(NT):
            h1[j, pl.ds(0, 8), :] = zeros
            h1[j, pl.ds(S + 8, 8), :] = zeros
        for c_ in cp_s:
            c_.wait()
        par[pl.ds(0, 4), :] = sk_s[...].astype(f32)
        par[pl.ds(8, 8), :] = jnp.broadcast_to(dd_s[...].astype(f32).reshape(1, D), (8, D))
        cv = c_s[...].astype(f32)
        sc = jnp.broadcast_to(cv * jax.nn.sigmoid(cv), (8, D))
        scp = pltpu.bitcast(pltpu.pack_elementwise([sc, sc], packed_dtype=bf16), f32)
        for j in range(NT):
            kb0[KOFF + 48 + j] = scp[:, 128 * j:128 * (j + 1)]

    def mkb(i, unr, off, cache):
        def b(stride, extra=0, z=None):
            if isinstance(i, int):
                return (i * unr + off) * stride + extra
            key = (stride, z)
            if key not in cache or NOCACHE:
                base = pl.multiple_of(i * (unr * stride), unr * stride)
                cache[key] = base if z is None else base + (i >> z)
            return cache[key] + (off * stride + extra)
        return b

    def dot_h(j, b, lhs):
        gb = gbs[j % 2]
        hc = hbuf[j, :, pl.ds(pl.multiple_of(b(512), 512), 512)]
        rhs_t = jnp.concatenate([hc[:, C * cc:C * (cc + 1)] for cc in range(4)], axis=0)
        g = lax.dot_general(lhs, pltpu.bitcast(rhs_t, bf16), NTDIMS, preferred_element_type=f32)
        for rg in range(2 * NG):
            for cc in range(4):
                gb[b(4, cc + rg * NC)] = g[8 * rg:8 * rg + 8, 128 * cc:128 * cc + 128]

    def dot_u(j, b, lhs):
        ub = ubs[j % 2]
        taps = [par[pl.ds(t, 1), pl.ds(j * 128, 128)] for t in range(4)]
        unp = lambda w_, e: pltpu.unpack_elementwise(w_, index=e, packed_dtype=bf16, unpacked_dtype=f32)
        cols = []
        for cc in range(4):
            words = []
            for blk in range(8 // W):
                w0 = 64 * cc + 8 * W * blk
                kw = {m: kbuf[j, pl.ds(b(256, 8 + w0 + m), 8, stride=W), :] for m in range(-2, W)}
                kk = {2 * m + e: unp(kw[m], e) for m in range(-2, W) for e in range(2) if 2 * m + e >= -3}
                for m in range(W):
                    vw = vbuf[j, pl.ds(b(256, w0 + m), 8, stride=W), :]
                    pair = []
                    for e in range(2):
                        n = 2 * m + e
                        ks = kk[n] * taps[0] + kk[n - 1] * taps[1] + kk[n - 2] * taps[2] + kk[n - 3] * taps[3]
                        pair.append(ks * unp(vw, e))
                    words.append(pltpu.pack_elementwise(pair, packed_dtype=bf16))
            cols.append(jnp.concatenate(words, axis=0))
        rhs = pltpu.bitcast(jnp.concatenate(cols, axis=1), bf16)
        u = jnp.dot(lhs, rhs, preferred_element_type=f32)
        for rg in range(2 * NG):
            for cc in range(4):
                ub[b(4, cc + rg * NC)] = u[8 * rg:8 * rg + 8, 128 * cc:128 * cc + 128]

    def dot_i(j, b, half, lhs):
        kb = kbs[j % 2]
        cols = [[], []]
        for gi in range(NG):
            prev = None
            for cc in range(-1, 2):
                k0, k1, k2 = [kb[b(4 * NG * 3, ((2 * half + cc + 1) * NG + gi) * 3 + t)] for t in range(3)]
                re, im = k0 - k2, k0 + k1
                if prev is not None:
                    cols[cc].append(pltpu.pack_elementwise([re - prev[1], im + prev[0]], packed_dtype=bf16))
                prev = (re, im)
        rhs = jnp.concatenate([jnp.concatenate(c_, axis=0) for c_ in cols], axis=1)
        y = jnp.dot(lhs, pltpu.bitcast(rhs, bf16), preferred_element_type=f32)
        for cc in range(2):
            yb[j, pl.ds(b(512, (2 * half + cc) * C), C), :] = y[:, 128 * cc:128 * cc + 128]

    def gen_m(j, b):
        ub, gb, kb = ubs[j % 2], gbs[j % 2], kbs[j % 2]
        for s in range(4):
            for t in range(3):
                z = 8 + t
                re = lambda ref, c: ref[b(8 * NC, 2 * s * NC + c, z)]
                im = lambda ref, c: ref[b(8 * NC, (2 * s + 1) * NC + c, z)]
                gre = [re(gb, c) for c in range(NC)]
                if t == 0:
                    us = [re(ub, c) + im(ub, c) for c in range(NC)]
                    gs = gre
                elif t == 1:
                    us = [re(ub, c) for c in range(NC)]
                    gs = [im(gb, c) - gre[c] for c in range(NC)]
                else:
                    us = [im(ub, c) for c in range(NC)]
                    gs = [im(gb, c) + gre[c] for c in range(NC)]

                def st(a, val):
                    kb[b(12, ((a + 1) * NG + s) * 3 + t)] = val
                if not KARA:
                    for a in range(NC):
                        st(a, _conv(us, gs, a))
                        yield 2 * a + 2
                    continue
                ue, uo, ge, go = us[0::2], us[1::2], gs[0::2], gs[1::2]
                usum = [x + y for x, y in zip(ue, uo)]
                gsum = [x + y for x, y in zip(ge, go)]
                poo_prev = None
                for a in range(NC // 2):
                    pee = _conv(ue, ge, a)
                    poo = _conv(uo, go, a)
                    pss = _conv(usum, gsum, a)
                    st(2 * a, pee if poo_prev is None else pee + poo_prev)
                    st(2 * a + 1, pss - pee - poo)
                    poo_prev = poo
                    yield 3 * (2 * a + 1) + 7

    def add_d(j):
        gb = gbs[j % 2]
        dvec = par[pl.ds(8, 8), pl.ds(j * 128, 128)]
        for gi in range(NG):
            gb[2 * gi * NC] = gb[2 * gi * NC] + dvec

    def sc_lhs():
        return pltpu.bitcast(jnp.concatenate([kb0[KOFF + 48 + j] for j in range(NT)], axis=1), bf16)

    def dot_m(i, t0, nt, rows):
        m = None
        for kt in range(NT):
            p = jnp.dot(pltpu.bitcast(rows[kt], bf16), _wt(wm, i, pl.ds(64 * kt, 64), pl.ds(128 * t0, 128 * nt)),
                        preferred_element_type=f32)
            m = p if m is None else m + p
        for t in range(nt):
            modb[i * (WMA // 128) + (t0 + t)] = m[0:8, 128 * t:128 * (t + 1)]

    def inv_lhs(tbl, n):
        return jnp.concatenate([tbl[KOFF + 16 + 2 * n], tbl[KOFF + 17 + 2 * n]], axis=1)

    PRE = dict(H=0, U=672 + 96 // W, a=192, b=192, m=0)
    POST = dict(H=0, U=0, a=4, b=4, m=2)
    NST = dict(H=16, U=16, a=8, b=8, m=5)
    MCOST = 12 * (248 if KARA else 272)

    def a_loop(jf, jm, ji, with_mod=False):
        unr = 2
        kinds = [k_ for k_ in DORDER if (jf is not None if k_ in 'HU' else ji is not None)]
        dots = [(k_, s_) for s_ in range(unr) for k_ in kinds]
        if with_mod:
            dots = [('m', (0, 4)), dots[0], ('m', (4, 4)), dots[1], ('m', (8, 2))] + dots[2:]
        native, dur = [], []
        for idx, (k_, arg) in enumerate(dots):
            nxt = PRE[dots[idx + 1][0]] if idx + 1 < len(dots) else 0
            d_ = 2.0 if k_ == 'm' else 1.0
            native += [nxt / NST[k_] + POST[k_] * d_] * NST[k_]
            dur += [d_] * NST[k_]
        tbl = kbs[jm % 2] if jm is not None else kbs[0]

        def body(i, carry):
            cache = {}
            if jm is not None:
                def chain():
                    for s_ in range(unr):
                        yield from gen_m(jm, mkb(i, unr, s_, cache))
                mg = chain()
                mtot = MCOST * unr - TAIL - HEAD
                lvl = (mtot + sum(native)) / sum(dur)
                want = [max(lvl * d_ - x, 0.0) for x, d_ in zip(native, dur)]
                scale = mtot / sum(want)
                cum, tgt = [HEAD], HEAD
                for w_ in want:
                    tgt += w_ * scale
                    cum.append(tgt)
            done = 0.0
            step = 0
            for (k_, arg) in dots:
                rows = []
                for n in range(NST[k_]):
                    if jm is not None:
                        while done < cum[step]:
                            done += next(mg)
                    step += 1
                    if k_ in 'HU':
                        rows.append(tbl[KOFF + n + (32 if k_ == 'U' else 0)])
                    elif k_ in 'ab':
                        rows.append(inv_lhs(tbl, n))
                    else:
                        rows.append(kb0[KOFF + 48 + n])
                if k_ == 'm':
                    dot_m(i, arg[0], arg[1], rows)
                    continue
                lhs = pltpu.bitcast(jnp.concatenate(rows, axis=0), bf16)
                if k_ == 'H':
                    dot_h(jf, mkb(i, unr, arg, cache), lhs)
                elif k_ == 'U':
                    dot_u(jf, mkb(i, unr, arg, cache), lhs)
                else:
                    dot_i(ji, mkb(i, unr, arg, cache), 0 if k_ == 'a' else 1, lhs)
            if jm is not None:
                for _ in mg:
                    pass

            @pl.when(i == 0)
            def _():
                for c_ in (cp_tile(jf, 1) if jf is not None else [cp_wm(1)]):
                    c_.wait()
            return carry
        for c_ in (cp_tile(jf, 0) if jf is not None else [cp_wm(0)]):
            c_.wait()
        lax.fori_loop(0, 2, body, 0)

    for seg in range(NT + 1):
        jf, jm, ji = [x if 0 <= x < NT else None for x in (seg, seg - 1, seg - 2)]
        if SKIPA or seg not in SEGS:
            for i in range(2):
                with jax.named_scope(f"W{seg}{i}"):
                    for c_ in (cp_tile(jf, i) if jf is not None else [cp_wm(i)]):
                        c_.wait()
        if SKIPA or seg not in SEGS:
            continue
        if seg == NT and PREW:
            cp_w[3].wait()
        with jax.named_scope(f"A_seg{seg}"):
            a_loop(jf, jm, ji, with_mod=(seg == NT))
            if jf is not None:
                add_d(jf)

    def inv_last(bt):
        lhs = pltpu.bitcast(jnp.concatenate([inv_lhs(kb1, n) for n in range(8)], axis=0), bf16)
        for half in range(2):
            dot_i(NT - 1, mkb(0, 1, bt, None), half, lhs)

    def modrow(k_):
        return jnp.concatenate([modb[NT * k_ + j] for j in range(NT)], axis=1)

    R = R1
    GP = R // 8

    def ln_chain(p):
        r = p * R
        pa, pb, pc, ps = [par[pl.ds(16 + 8 * t, 8), :][None] for t in range(4)]
        g3 = lambda x: x.reshape(GP, 8, D)
        q = g3(qbuf[pl.ds(r, R), :].astype(f32))
        d1, r1 = _center(q)
        y = g3(jnp.concatenate([yb[j, pl.ds(r, R), :] for j in range(NT)], axis=1))
        x = q + ((d1 * r1) * pa + pb) * y
        xn[pl.ds(r, R), :] = x.reshape(R, D)
        d2, r2 = _center(x)
        h = (d2 * r2) * pc + ps
        hh[pl.ds(r, R), :] = h.reshape(R, D)
        d3, r3 = _center(h, ALPHA)
        return (d3 * r3).reshape(R, D)

    def tied(wref, ties):
        if not ties:
            return _wt(wref)
        rows = []
        for kt in range(NT):
            rows.append(wref[pl.ds(64 * kt, 56), :])
            last = []
            for n in range(NT):
                w_ = wref[pl.ds(64 * kt + 56, 8), pl.ds(128 * n, 128)]
                vs = ties.get(5 * n + kt)
                if vs:
                    t_ = pltpu.bitcast(vs[0], u32)
                    for v_ in vs[1:]:
                        t_ = t_ | pltpu.bitcast(v_, u32)
                    w_ = w_ | (t_ & kbuf[0, pl.ds(0, 8), :])
                last.append(w_)
            rows.append(jnp.concatenate(last, axis=1))
        return pltpu.bitcast(jnp.concatenate(rows, axis=0), bf16)

    def w1_dot(p, l3, ties):
        z = jnp.dot(l3.astype(bf16), tied(w1, ties), preferred_element_type=f32)
        g = _gelu2a(z)
        for j in range(NT):
            h1[j, pl.ds(p * R + 8, R), :] = g[:, j * 128:(j + 1) * 128]

    def w2_dot(p, ties):
        r = p * R
        lane = lax.broadcasted_iota(jnp.int32, (R, 128), 1)

        def ld(j, off):
            return h1[j, pl.ds(r + 8 + off, R), :]
        tiles = [
            ld(0, -1),
            jnp.where(lane < 32, ld(1, -1), ld(1, 1)),
            jnp.where(lane < 64, ld(2, 1), ld(2, -2)),
            jnp.where(lane < 96, ld(3, -2), ld(3, 2)),
            ld(4, 2),
        ]
        hs = jnp.concatenate(tiles, axis=1).astype(bf16)
        x1 = hh[pl.ds(r, R), :] + jnp.dot(hs, tied(w2, ties), preferred_element_type=f32) * BETA
        hh[pl.ds(r, R), :] = x1

    l3s = {}

    def run_block(dots, extra=()):
        groups = []
        for d_, (k_, p) in enumerate(dots):
            if k_ == 1 and p not in l3s:
                groups += [(p, g, 25 * d_) for g in range(GP)]
        for p in extra:
            groups += [(p, g, 25 * len(dots) - 1) for g in range(GP)]
        slots = {}
        nxt = None
        for (p, g, hard) in reversed(groups):
            sl = hard if nxt is None else min(hard, nxt - (SP * GA if g % GA == GA - 1 else 0))
            sl = min(hard, max(sl, MINS))
            nxt = sl
            if sl < hard or p in extra:
                slots.setdefault(int(sl), []).append((p, g))
        for d_, (k_, p) in enumerate(dots):
            ties = {}
            for t in range(25):
                for (pp, g) in slots.get(25 * d_ + t, ()):
                    if pp not in l3s:
                        l3s[pp] = ln_chain(pp)
                    ties.setdefault(t, []).append(l3s[pp][8 * g:8 * g + 8, 0:128])
            if k_ == 1:
                if p not in l3s:
                    l3s[p] = ln_chain(p)
                w1_dot(p, l3s[p], ties)
            else:
                w2_dot(p, ties)

    with jax.named_scope("P1"):
        cp_wmp.wait()
        cp_q[0].wait()
        mp = jnp.dot(sc_lhs(), _wt(wmp), preferred_element_type=f32)
        for t in range(WMP // 128):
            modb[2 * WMA // 128 + t] = mp[0:8, 128 * t:128 * (t + 1)]
        sa, ca, ga, sb, cb = [modrow(k_) for k_ in range(5)]
        par[pl.ds(16, 8), :] = ga * (1.0 + ca)
        par[pl.ds(24, 8), :] = ga * sa
        par[pl.ds(32, 8), :] = 1.0 + cb
        par[pl.ds(40, 8), :] = sb
        if not SKIPA:
            for bt in range(4):
                inv_last(bt)
        for p in range(PRELN):
            l3s[p] = ln_chain(p)
    with jax.named_scope("w1wait"):
        cp_w[0].wait()
    p1, p2 = N2, 0
    with jax.named_scope("P2"):
        run_block([(1, p) for p in range(N2)])
    with jax.named_scope("w2wait"):
        cp_w[1].wait()
    with jax.named_scope("P3"):
        dots = []
        while p2 < Q0 // R - 3:
            dots.append((2, p2))
            p2 += 1
            if p1 < Q0 // R:
                dots.append((1, p1))
                p1 += 1
        run_block(dots)
    with jax.named_scope("q1wait"):
        cp_q[1].wait()
    with jax.named_scope("P4"):
        dots = [(2, p2), (2, p2 + 1)]
        p2 += 2
        while p2 < S // R and not SKIPB:
            while p1 < S // R and p1 - p2 < LEAD:
                dots.append((1, p1))
                p1 += 1
            dots.append((2, p2))
            p2 += 1
        run_block(dots)

    def out_copy(r):
        return cp(obuf.at[pl.ds(r, TS), :], o_hbm.at[0, pl.ds(r, TS), :], osems.at[0])

    def ln4(r):
        d4, r4 = _center(hh[pl.ds(r, TS), :], ALPHA)
        return d4 * r4

    def b2_step(i):
        gbv = par[pl.ds(48, 1), :]
        nsub = T2 // TS
        for sub in range(nsub):
            r = pl.multiple_of(pl.multiple_of(i * T2, T2) + sub * TS, TS)
            l4 = _wt(l4p) if (sub == 0 and LP) else ln4(r).astype(bf16)
            z = lax.dot_general(l4, _wt(w3, pl.ds(0, FA // 2), slice(None)), NTDIMS, preferred_element_type=f32)
            zt = lax.dot_general(_wt(w3, pl.ds(FA // 2, (F - FA) // 2), slice(None)), l4, NTDIMS,
                                 preferred_element_type=f32)
            g = jnp.concatenate([_gelu2a(z), _gelu2a(zt).T], axis=1).astype(bf16)
            if sub == nsub - 1 and LP:
                nx = ln4(pl.multiple_of(jnp.minimum(i + 1, S // T2 - 1) * T2, T2))
                l4p[...] = pltpu.bitcast(nx.astype(bf16), u32)
                t_ = pltpu.bitcast(nx[0:8, 0:128], u32)
                for gi in range(1, TS // 8):
                    t_ = t_ | pltpu.bitcast(nx[8 * gi:8 * gi + 8, 0:128], u32)
                top = [w4[pl.ds(0, 8), pl.ds(128 * n, 128)] for n in range(NT)]
                top[LPN] = top[LPN] | (t_ & kbuf[0, pl.ds(0, 8), :])
                w4v = jnp.concatenate([jnp.concatenate(top, axis=1), w4[pl.ds(8, F // 2 - 8), :]], axis=0)
            else:
                w4v = w4[...]
            acc = jnp.dot(g, pltpu.bitcast(w4v, bf16), preferred_element_type=f32)
            obuf[pl.ds(r, TS), :] = (xn[pl.ds(r, TS), :] + gbv * (hh[pl.ds(r, TS), :] + BETA * acc)).astype(bf16)
            out_copy(r).start()

    with jax.named_scope("B2_wait"):
        cp_w[2].wait()
        if not PREW:
            cp_w[3].wait()
        cp_wmc.wait()
        mc = jnp.dot(sc_lhs(), _wt(wmc), preferred_element_type=f32)[0:8]
        par[pl.ds(48, 8), :] = mc
        if LP:
            l4p[...] = pltpu.bitcast(ln4(0).astype(bf16), u32)
    with jax.named_scope("BII"):
        lax.fori_loop(0, S // T2, lambda i, c: (b2_step(i), c)[1], 0)
    with jax.named_scope("out_wait"):
        for i in range(S // TS):
            out_copy(i * TS).wait()


@jax.jit
def pallas_adaLN_cond__ssm_conv_h3__mixer_s_mlp__prompt_kernel(
    A_q, A_k, A_v, A_shift_k, A_ssm_k, A_ssm_D, B_x, B_w1, B_w2, B_w3, B_w4, c, w_mod,
):
    del B_x
    hbm = pl.BlockSpec(memory_space=pltpu.MemorySpace.HBM)
    return pl.pallas_call(
        _kernel,
        out_shape=jax.ShapeDtypeStruct((1, S, D), bf16),
        in_specs=[hbm] * 12,
        out_specs=hbm,
        scratch_shapes=[
            pltpu.VMEM((S, D), bf16),
            pltpu.VMEM((NT, 8 + S // 2, 128), u32),
            pltpu.VMEM((NT, S // 2, 128), u32),
            pltpu.VMEM((NT, 64, S), u32),
            pltpu.VMEM((D // 2, D), u32),
            pltpu.VMEM((D // 2, D), u32),
            pltpu.VMEM((F // 2, D), u32),
            pltpu.VMEM((F // 2, D), u32),
            pltpu.VMEM((2, D // 2, WMA), u32),
            pltpu.VMEM((D // 2, WMP), u32),
            pltpu.VMEM((D // 2, WMC), u32),
            pltpu.VMEM((26 + int(os.environ.get('PADM', '2')), 8, 128), f32),
            pltpu.VMEM((S, D), bf16),
            pltpu.VMEM((4, D), bf16),
            pltpu.VMEM((D,), bf16),
            pltpu.VMEM((1, D), bf16),
            pltpu.VMEM((NG * 2 * NC, 8, 128), f32),
            pltpu.VMEM((NG * 2 * NC, 8, 128), f32),
            pltpu.VMEM((NG * 2 * NC, 8, 128), f32),
            pltpu.VMEM((NG * 2 * NC, 8, 128), f32),
            pltpu.VMEM((KOFF + 56 + PADK, 8, 128), f32),
            pltpu.VMEM((KOFF + 56 + PADK, 8, 128), f32),
            pltpu.VMEM((NT, S, 128), f32),
            pltpu.VMEM((S, D), f32),
            pltpu.VMEM((S, D), f32),
            pltpu.VMEM((NT, S + 16, 128), f32),
            pltpu.VMEM((56, D), f32),
            pltpu.VMEM((TS // 2, D), u32),
            pltpu.SemaphoreType.DMA((20,)),
            pltpu.SemaphoreType.DMA((1,)),
        ],
        compiler_params=pltpu.CompilerParams(vmem_limit_bytes=100 * 1024 * 1024, disable_semaphore_checks=True,
                                             disable_bounds_checks=bool(int(os.environ.get('NOBC', '0')))),
    )(A_q, A_k, A_v, A_shift_k.T, A_ssm_k, A_ssm_D, B_w1, B_w2, B_w3.T, B_w4, c, w_mod)
```

```python
import math
import os

import jax
import jax.numpy as jnp
from jax import lax
import jax.experimental.pallas as pl
import jax.experimental.pallas.tpu as pltpu

S, D, F = 2048, 640, 1728
C = 128
NC = S // C
NT = D // 128
NG = 16
KOFF = (NC + 1) * NG * 3
W = int(os.environ.get('W', '4'))
SKIPA = int(os.environ.get('SKIPA', '0'))
WMA, WMP, WMC = 1280, 640, 640
Q0 = int(os.environ.get('Q0', '512'))
N2 = int(os.environ.get('N2', '5'))
PRELN = int(os.environ.get('PRELN', '2'))
NOCACHE = int(os.environ.get('NOCACHE', '0'))
OUTWAIT = int(os.environ.get('OUTWAIT', '0'))
SEGS = [int(x) for x in os.environ.get('SEGS', '012345')]
SKIPB = int(os.environ.get('SKIPB', '0'))
PADK = int(os.environ.get('PADK', '0'))
PREW = int(os.environ.get('PREW', '0'))
SP = float(os.environ.get('SP', '0'))
MINS = int(os.environ.get('MINS', '30'))
GA = int(os.environ.get('GA', '2'))
TRT = int(os.environ.get('TRT', '1'))
LP = int(os.environ.get('LP', '1'))
FA = 1664
LPN = int(os.environ.get('LPN', '2'))
G0 = int(os.environ.get('G0', '4'))
KARA = int(os.environ.get('KARA', '1'))
UNR = int(os.environ.get('UNR', '2'))
HEAD = int(os.environ.get('HEAD', '250'))
TAIL = int(os.environ.get('TAIL', '450'))
DORDER = os.environ.get('DORDER', 'HaUb')
R1 = int(os.environ.get('R1', '64'))
R2 = int(os.environ.get('R2', '128'))
LEAD = int(os.environ.get('LEAD', '4'))
TS = int(os.environ.get('TS', '256'))
ONEPASS = int(os.environ.get('ONEPASS', '1'))
RSQ = int(os.environ.get('RSQ', '1'))
T2 = int(os.environ.get('T2', '512'))
EPS = 1e-5
_C0 = math.sqrt(2.0 / math.pi)
ALPHA = (_C0 * 0.044715) ** (1.0 / 3.0)
GC = _C0 / ALPHA
BETA = 0.5 / ALPHA
_fc = [int(x) for x in os.environ.get('FC', '1728').split(',')]
F_CHUNKS = tuple((sum(_fc[:i]), _fc[i]) for i in range(len(_fc)))
assert sum(_fc) == F

f32 = jnp.float32
bf16 = jnp.bfloat16
u32 = jnp.uint32
NTDIMS = (((1,), (1,)), ((), ()))


def _cos_table(m, scale):
    mm = jnp.abs(((m + 256) & 511) - 256)
    x = (128 - mm).astype(f32) * (1.0 / 128.0)
    x2 = x * x
    h = math.pi / 2
    p = -(h ** 7) / 5040 + x2 * ((h ** 9) / 362880 - x2 * (h ** 11) / 39916800)
    p = h + x2 * (-(h ** 3) / 6 + x2 * ((h ** 5) / 120 + x2 * p))
    return (x * scale) * p


def _dft_tables():
    shape = (16, 8, 128)
    n = lax.broadcasted_iota(jnp.int32, shape, 0)
    s = lax.broadcasted_iota(jnp.int32, shape, 1)
    l = lax.broadcasted_iota(jnp.int32, shape, 2)
    fw, fu, iv = [], [], []
    wv = l >> 4
    tu = (16 * W) * (wv // W) + (2 * W) * ((l >> 1) & 7) + 2 * (wv % W) + (l & 1)
    for e in range(2):
        r = 2 * s + e
        j = 8 * n + (r & 7)
        fw.append(_cos_table((4 * j + 1) * l + (r >> 3) * 128, 1.0))
        fu.append(_cos_table((4 * j + 1) * tu + (r >> 3) * 128, 1.0))
        b = 16 * (n >> 1) + r
        col = 128 * (n & 1) + l
        iv.append(_cos_table((4 * (col >> 1) + 1) * b + (col & 1) * 128, 1.0 / 128.0))
    pk = lambda xs: pltpu.bitcast(pltpu.pack_elementwise(xs, packed_dtype=bf16), f32)
    return pk(fw), pk(iv), pk(fu)


def _gelu2a(z):
    return z * (1.0 + jnp.tanh(z * (z * z + GC)))


def _rstd(ssd, scale):
    if RSQ == 0:
        r = lax.rsqrt(ssd * (1.0 / D) + EPS)
        return r if scale == 1.0 else r * scale
    return jnp.exp2(jnp.log(ssd + D * EPS) * (-0.5 / math.log(2.0)) + math.log2(scale * math.sqrt(D)))


def _center(x, scale=1.0):
    s1 = jnp.sum(x, axis=-1, keepdims=True)
    m = s1 * (1.0 / D)
    d = x - m
    if ONEPASS:
        ssd = jnp.maximum(jnp.sum(x * x, axis=-1, keepdims=True) - s1 * m, 0.0)
    else:
        ssd = jnp.sum(d * d, axis=-1, keepdims=True)
    return d, _rstd(ssd, scale)


def _conv(us, gs, a):
    acc = None
    for c in range(a + 1):
        p = us[c] * gs[a - c]
        acc = p if acc is None else acc + p
    return acc


def _mult(x, n):
    return x if isinstance(x, int) else pl.multiple_of(x, n)


def _wt(ref, *idx):
    return pltpu.bitcast(ref[idx] if idx else ref[...], bf16)


def _kernel(q_hbm, k_hbm, v_hbm, sk_hbm, h_hbm, dd_hbm, w1_hbm, w2_hbm, w3_hbm, w4_hbm,
            c_hbm, wm_hbm, o_hbm,
            modb, qbuf, kbuf, vbuf, hbuf, w1, w2, w3, w4, wm, wmp, wmc, obuf,
            ub0, ub1, gb0, gb1, kb0, kb1, yb, xn, hh, h1, par, l4p, sk_s, dd_s, c_s, zs, sems, osems):
    ubs, gbs, kbs = (ub0, ub1), (gb0, gb1), (kb0, kb1)
    cp = pltpu.make_async_copy
    HS = S // 2

    def cp_h(j, c0, c1, sem):
        return cp(h_hbm.at[pl.ds(j * 128, 128), pl.ds(c0, c1 - c0)], hbuf.bitcast(bf16).at[j, :, pl.ds(c0, c1 - c0)], sem)

    def cp_kv(j, r0, r1, sem):
        r0, r1 = (r0 + 16 if r0 else 0), min(r1 + 16, S)
        lanes = pl.ds(j * 128, 128)
        return [cp(k_hbm.at[0, pl.ds(r0, r1 - r0), lanes], kbuf.bitcast(bf16).at[j, pl.ds(r0 + 16, r1 - r0), :], sem),
                cp(v_hbm.at[0, pl.ds(r0, r1 - r0), lanes], vbuf.bitcast(bf16).at[j, pl.ds(r0, r1 - r0), :], sem)]

    def cp_tile(j, i):
        sem = sems.at[2 * j + i]
        return [cp_h(j, i * HS, (i + 1) * HS, sem)] + cp_kv(j, i * HS, (i + 1) * HS, sem)

    cp_t0 = [[cp_h(0, 0, S, sems.at[0])], cp_kv(0, 0, 1024, sems.at[1]), cp_kv(0, 1024, 1536, sems.at[20]),
             cp_kv(0, 1536, S, sems.at[21])]

    def cp_wm(i):
        return cp(wm_hbm.at[:, pl.ds(i * WMA, WMA)], wm.bitcast(bf16).at[i], sems.at[10 + i])

    cp_wmp = cp(wm_hbm.at[:, pl.ds(2 * WMA, WMP)], wmp.bitcast(bf16), sems.at[13])
    cp_wmc = cp(wm_hbm.at[:, pl.ds(2 * WMA + WMP, WMC)], wmc.bitcast(bf16), sems.at[12])
    cp_q = [cp(q_hbm.at[0, pl.ds(r0, r1 - r0), :], qbuf.at[pl.ds(r0, r1 - r0), :], sems.at[13 + i])
            for i, (r0, r1) in enumerate(((0, Q0), (Q0, S)))]
    cp_w = [cp(s_, d_.bitcast(bf16), sems.at[15 + i])
            for i, (s_, d_) in enumerate(((w1_hbm, w1), (w2_hbm, w2), (w3_hbm, w3), (w4_hbm, w4)))]
    cp_s = [cp(sk_hbm, sk_s, sems.at[19]), cp(dd_hbm, dd_s, sems.at[19]), cp(c_hbm, c_s, sems.at[19])]
    order = list(cp_s)
    for grp in cp_t0:
        order += grp
    for j in range(1, NT):
        order += cp_tile(j, 0) + cp_tile(j, 1)
    order += [cp_wm(0), cp_wm(1), cp_wmp, cp_q[0], cp_w[0], cp_w[1], cp_q[1], cp_w[2], cp_w[3], cp_wmc]
    for c_ in order:
        c_.start()

    with jax.named_scope("init"):
        fw_t, iv_t, fu_t = _dft_tables()
        for kb in kbs:
            kb[pl.ds(KOFF, 16)] = fw_t
            kb[pl.ds(KOFF + 16, 16)] = iv_t
            kb[pl.ds(KOFF + 32, 16)] = fu_t
            kb[pl.ds(0, NG * 3)] = jnp.zeros((NG * 3, 8, 128), f32)
        zeros = jnp.zeros((8, 128), f32)
        for j in range(NT):
            kbuf[j, pl.ds(0, 8), :] = jnp.zeros((8, 128), u32)
            kbuf[j, pl.ds(8 + HS, 8), :] = jnp.zeros((8, 128), u32)
            vbuf[j, pl.ds(HS, 8), :] = jnp.zeros((8, 128), u32)
        for j in range(NT):
            h1[j, pl.ds(0, 8), :] = zeros
            h1[j, pl.ds(S + 8, 8), :] = zeros
        for c_ in cp_s:
            c_.wait()
        par[pl.ds(0, 4), :] = sk_s[...].astype(f32)
        par[pl.ds(8, 8), :] = jnp.broadcast_to(dd_s[...].astype(f32).reshape(1, D), (8, D))
        cv = c_s[...].astype(f32)
        sc = jnp.broadcast_to(cv * jax.nn.sigmoid(cv), (8, D))
        scp = pltpu.bitcast(pltpu.pack_elementwise([sc, sc], packed_dtype=bf16), f32)
        for j in range(NT):
            kb0[KOFF + 48 + j] = scp[:, 128 * j:128 * (j + 1)]
            kb1[KOFF + 48 + j] = scp[:, 128 * j:128 * (j + 1)]

    def mkb(i, unr, off, cache):
        def b(stride, extra=0, z=None):
            if isinstance(i, int):
                return (i * unr + off) * stride + extra
            key = (unr * stride, z)
            if key not in cache or NOCACHE:
                base = pl.multiple_of(i * (unr * stride), unr * stride)
                cache[key] = base if z is None else base + (i >> z)
            return cache[key] + (off * stride + extra)
        return b

    def dot_h(j, b, lhs):
        gb = gbs[j % 2]
        hc = hbuf[j, :, pl.ds(_mult(b(512), 512), 512)]
        rhs_t = jnp.concatenate([hc[:, C * cc:C * (cc + 1)] for cc in range(4)], axis=0)
        g = lax.dot_general(lhs, pltpu.bitcast(rhs_t, bf16), NTDIMS, preferred_element_type=f32)
        for rg in range(2 * NG):
            for cc in range(4):
                gb[b(4, cc + rg * NC)] = g[8 * rg:8 * rg + 8, 128 * cc:128 * cc + 128]

    def dot_u(j, b, lhs):
        ub = ubs[j % 2]
        taps = [par[pl.ds(t, 1), pl.ds(j * 128, 128)] for t in range(4)]
        unp = lambda w_, e: pltpu.unpack_elementwise(w_, index=e, packed_dtype=bf16, unpacked_dtype=f32)
        cols = []
        for cc in range(4):
            words = []
            for blk in range(8 // W):
                w0 = 64 * cc + 8 * W * blk
                kw = {m: kbuf[j, pl.ds(b(256, 8 + w0 + m), 8, stride=W), :] for m in range(-2, W)}
                kk = {2 * m + e: unp(kw[m], e) for m in range(-2, W) for e in range(2) if 2 * m + e >= -3}
                for m in range(W):
                    vw = vbuf[j, pl.ds(b(256, w0 + m), 8, stride=W), :]
                    pair = []
                    for e in range(2):
                        n = 2 * m + e
                        ks = kk[n] * taps[0] + kk[n - 1] * taps[1] + kk[n - 2] * taps[2] + kk[n - 3] * taps[3]
                        pair.append(ks * unp(vw, e))
                    words.append(pltpu.pack_elementwise(pair, packed_dtype=bf16))
            cols.append(jnp.concatenate(words, axis=0))
        rhs = pltpu.bitcast(jnp.concatenate(cols, axis=1), bf16)
        u = jnp.dot(lhs, rhs, preferred_element_type=f32)
        for rg in range(2 * NG):
            for cc in range(4):
                ub[b(4, cc + rg * NC)] = u[8 * rg:8 * rg + 8, 128 * cc:128 * cc + 128]

    def dot_i(j, b, half, lhs):
        kb = kbs[j % 2]
        cols = [[], []]
        for gi in range(NG):
            prev = None
            for cc in range(-1, 2):
                k0, k1, k2 = [kb[b(4 * NG * 3, ((2 * half + cc + 1) * NG + gi) * 3 + t)] for t in range(3)]
                re, im = k0 - k2, k0 + k1
                if prev is not None:
                    cols[cc].append(pltpu.pack_elementwise([re - prev[1], im + prev[0]], packed_dtype=bf16))
                prev = (re, im)
        rhs = jnp.concatenate([jnp.concatenate(c_, axis=0) for c_ in cols], axis=1)
        y = jnp.dot(lhs, pltpu.bitcast(rhs, bf16), preferred_element_type=f32)
        for cc in range(2):
            yb[j, pl.ds(b(512, (2 * half + cc) * C), C), :] = y[:, 128 * cc:128 * cc + 128]

    def gen_m(j, kb, b, ng):
        ub, gb = ubs[j % 2], gbs[j % 2]
        for s in range(ng):
            for t in range(3):
                z = 8 + t
                re = lambda ref, c: ref[b(2 * NC, 2 * s * NC + c, z)]
                im = lambda ref, c: ref[b(2 * NC, (2 * s + 1) * NC + c, z)]
                gre = [re(gb, c) for c in range(NC)]
                if t == 0:
                    us = [re(ub, c) + im(ub, c) for c in range(NC)]
                    gs = gre
                elif t == 1:
                    us = [re(ub, c) for c in range(NC)]
                    gs = [im(gb, c) - gre[c] for c in range(NC)]
                else:
                    us = [im(ub, c) for c in range(NC)]
                    gs = [im(gb, c) + gre[c] for c in range(NC)]

                def st(a, val):
                    kb[b(3, ((a + 1) * NG + s) * 3 + t)] = val
                if not KARA:
                    for a in range(NC):
                        st(a, _conv(us, gs, a))
                        yield 2 * a + 2
                    continue
                ue, uo, ge, go = us[0::2], us[1::2], gs[0::2], gs[1::2]
                usum = [x + y for x, y in zip(ue, uo)]
                gsum = [x + y for x, y in zip(ge, go)]
                poo_prev = None
                for a in range(NC // 2):
                    pee = _conv(ue, ge, a)
                    poo = _conv(uo, go, a)
                    pss = _conv(usum, gsum, a)
                    st(2 * a, pee if poo_prev is None else pee + poo_prev)
                    st(2 * a + 1, pss - pee - poo)
                    poo_prev = poo
                    yield 3 * (2 * a + 1) + 7

    def add_d(j):
        gb = gbs[j % 2]
        dvec = par[pl.ds(8, 8), pl.ds(j * 128, 128)]
        for gi in range(NG):
            gb[2 * gi * NC] = gb[2 * gi * NC] + dvec

    def sc_lhs():
        return pltpu.bitcast(jnp.concatenate([kb0[KOFF + 48 + j] for j in range(NT)], axis=1), bf16)

    def dot_m(i, t0, nt, rows):
        m = None
        for kt in range(NT):
            p = jnp.dot(pltpu.bitcast(rows[kt], bf16), _wt(wm, i, pl.ds(64 * kt, 64), pl.ds(128 * t0, 128 * nt)),
                        preferred_element_type=f32)
            m = p if m is None else m + p
        for t in range(nt):
            modb[i * (WMA // 128) + (t0 + t)] = m[0:8, 128 * t:128 * (t + 1)]

    def inv_lhs(tbl, n):
        return jnp.concatenate([tbl[KOFF + 16 + 2 * n], tbl[KOFF + 17 + 2 * n]], axis=1)

    def dot_k(kb, kt, bt, lhs):
        cols = [[] for _ in range(4)]
        for gi in range(8 * kt, 8 * kt + 8):
            prev = None
            for cc in range(-1, 4):
                k0, k1, k2 = [kb[((4 * bt + cc + 1) * NG + gi) * 3 + t] for t in range(3)]
                re, im = k0 - k2, k0 + k1
                if prev is not None:
                    cols[cc].append(pltpu.pack_elementwise([re - prev[1], im + prev[0]], packed_dtype=bf16))
                prev = (re, im)
        rhs = jnp.concatenate([jnp.concatenate(c_, axis=0) for c_ in cols], axis=1)
        y = jnp.dot(lhs, pltpu.bitcast(rhs, bf16), preferred_element_type=f32)
        for cc in range(4):
            rows = pl.ds((4 * bt + cc) * C, C)
            yc = y[:, 128 * cc:128 * cc + 128]
            yb[NT - 1, rows, :] = yc if kt == 0 else yb[NT - 1, rows, :] + yc

    PRE = dict(H=0, U=672 + 96 // W, a=192, b=192, m=0, k=176)
    POST = dict(H=0, U=0, a=4, b=4, m=2, k=0)
    NST = dict(H=16, U=16, a=8, b=8, m=5, k=8)
    GCOST = 3 * (248 if KARA else 272)

    def a_block(dots, mg=None, ng=0, tbl=kb0):
        native, dur = [], []
        for idx, (k_, _) in enumerate(dots):
            nxt = PRE[dots[idx + 1][0]] if idx + 1 < len(dots) else 0
            d_ = 2.0 if k_ == 'm' else 1.0
            native += [nxt / NST[k_] + POST[k_] * d_] * NST[k_]
            dur += [d_] * NST[k_]
        if mg is not None and dots:
            head = max(HEAD - PRE[dots[0][0]], 0)
            mtot = GCOST * ng - TAIL - head
            lvl = (mtot + sum(native)) / sum(dur)
            want = [max(lvl * d_ - x, 0.0) for x, d_ in zip(native, dur)]
            scale = mtot / sum(want)
            cum, tgt = [head], head
            for w_ in want:
                tgt += w_ * scale
                cum.append(tgt)
        done = 0.0
        step = 0
        for (k_, fn) in dots:
            rows = []
            for n in range(NST[k_]):
                if mg is not None:
                    while done < cum[step]:
                        done += next(mg)
                step += 1
                if k_ in 'HU':
                    rows.append(tbl[KOFF + n + (32 if k_ == 'U' else 0)])
                elif k_ in 'ab':
                    rows.append(inv_lhs(tbl, n))
                elif k_ == 'k':
                    rows.append(tbl[KOFF + 16 + 2 * n])
                else:
                    rows.append(tbl[KOFF + 48 + n])
            fn(rows if k_ == 'm' else pltpu.bitcast(jnp.concatenate(rows, axis=0), bf16))
        if mg is not None:
            for _ in mg:
                pass

    def fdot(k_, j, b):
        if k_ == 'H':
            return (k_, lambda lhs: dot_h(j, b, lhs))
        if k_ == 'U':
            return (k_, lambda lhs: dot_u(j, b, lhs))
        return (k_, lambda lhs: dot_i(j, b, 0 if k_ == 'a' else 1, lhs))

    def wait_all(cps):
        for c_ in cps:
            c_.wait()

    def a_loop(jf, jm, ji, g0, ng):
        kinds = [k_ for k_ in DORDER if k_ in 'HU' or ji is not None]

        def body(i, carry):
            cache = {}
            zs[i] = 0
            dots = [fdot(k_, jf if k_ in 'HU' else ji, mkb(i, 2, s_, cache)) for s_ in range(2) for k_ in kinds]
            a_block(dots, gen_m(jm, kbs[jm % 2], mkb(i, ng, g0, cache), ng), ng, kbs[jm % 2])

            @pl.when(i == 0)
            def _():
                wait_all(cp_tile(jf, 1))
            return carry
        wait_all(cp_tile(jf, 0))
        lax.fori_loop(0, 2, body, 0)
        add_d(jf)

    sb_ = lambda bt: mkb(0, 1, bt, None)
    with jax.named_scope("A_seg0"):
        wait_all(cp_t0[0])
        a_block([fdot('H', 0, sb_(bt)) for bt in range(4)])
        add_d(0)
        wait_all(cp_t0[1])
        a_block([fdot('U', 0, sb_(bt)) for bt in range(2)])
        for bt in (2, 3):
            wait_all(cp_t0[bt])
            a_block([fdot('U', 0, sb_(bt))])
    with jax.named_scope("A_m0"):
        def body_m0(i, carry):
            a_block([], gen_m(0, kb0, mkb(i, G0 // 2, 0, {}), G0 // 2))
            return carry
        if G0:
            lax.fori_loop(0, 2, body_m0, 0)
    for seg in range(1, NT):
        with jax.named_scope(f"A_seg{seg}"):
            if seg == 1:
                a_loop(1, 0, None, G0, (NG - G0) // 2)
            else:
                a_loop(seg, seg - 1, seg - 2, 0, 8)

    def mods(i):
        return [('m', lambda rows, t0=t0, nt=nt: dot_m(i, t0, nt, rows)) for (t0, nt) in ((0, 4), (4, 4), (8, 2))]

    with jax.named_scope("A_seg5a"):
        cp_wm(0).wait()
        zz = zs[1]

        @pl.when(zz == 0)
        def _():
            dots = [fdot(k_, NT - 2, sb_(bt)) for bt in range(4) for k_ in 'ab']
            mm = mods(0)
            dots = [mm[0]] + dots[0:2] + [mm[1]] + dots[2:4] + [mm[2]] + dots[4:]
            a_block(dots, gen_m(NT - 1, kb0, mkb(zz, 8, 0, {}), 8), 8, kb0)
    with jax.named_scope("A_seg5b"):
        cp_wm(1).wait()

        @pl.when(zz == 0)
        def _():
            dots = [('k', lambda lhs, bt=bt: dot_k(kb0, 0, bt, lhs)) for bt in range(4)]
            mm = mods(1)
            dots = [mm[0], dots[0], mm[1], dots[1], mm[2]] + dots[2:]
            a_block(dots, gen_m(NT - 1, kb1, mkb(zz, 8, 8, {}), 8), 8, kb1)

    def inv_last(bt):
        lhs = pltpu.bitcast(jnp.concatenate([kb0[KOFF + 17 + 2 * n] for n in range(8)], axis=0), bf16)
        dot_k(kb1, 1, bt, lhs)

    def modrow(k_):
        return jnp.concatenate([modb[NT * k_ + j] for j in range(NT)], axis=1)

    R = R1
    GP = R // 8

    def ln_chain(p):
        r = p * R
        pa, pb, pc, ps = [par[pl.ds(16 + 8 * t, 8), :][None] for t in range(4)]
        g3 = lambda x: x.reshape(GP, 8, D)
        q = g3(qbuf[pl.ds(r, R), :].astype(f32))
        d1, r1 = _center(q)
        y = g3(jnp.concatenate([yb[j, pl.ds(r, R), :] for j in range(NT)], axis=1))
        x = q + ((d1 * r1) * pa + pb) * y
        xn[pl.ds(r, R), :] = x.reshape(R, D)
        d2, r2 = _center(x)
        h = (d2 * r2) * pc + ps
        hh[pl.ds(r, R), :] = h.reshape(R, D)
        d3, r3 = _center(h, ALPHA)
        return (d3 * r3).reshape(R, D)

    def tied(wref, ties):
        if not ties:
            return _wt(wref)
        rows = []
        for kt in range(NT):
            rows.append(wref[pl.ds(64 * kt, 56), :])
            last = []
            for n in range(NT):
                w_ = wref[pl.ds(64 * kt + 56, 8), pl.ds(128 * n, 128)]
                vs = ties.get(5 * n + kt)
                if vs:
                    t_ = pltpu.bitcast(vs[0], u32)
                    for v_ in vs[1:]:
                        t_ = t_ | pltpu.bitcast(v_, u32)
                    w_ = w_ | (t_ & kbuf[0, pl.ds(0, 8), :])
                last.append(w_)
            rows.append(jnp.concatenate(last, axis=1))
        return pltpu.bitcast(jnp.concatenate(rows, axis=0), bf16)

    def w1_dot(p, l3, ties):
        z = jnp.dot(l3.astype(bf16), tied(w1, ties), preferred_element_type=f32)
        g = _gelu2a(z)
        for j in range(NT):
            h1[j, pl.ds(p * R + 8, R), :] = g[:, j * 128:(j + 1) * 128]

    def w2_dot(p, ties):
        r = p * R
        lane = lax.broadcasted_iota(jnp.int32, (R, 128), 1)

        def ld(j, off):
            return h1[j, pl.ds(r + 8 + off, R), :]
        tiles = [
            ld(0, -1),
            jnp.where(lane < 32, ld(1, -1), ld(1, 1)),
            jnp.where(lane < 64, ld(2, 1), ld(2, -2)),
            jnp.where(lane < 96, ld(3, -2), ld(3, 2)),
            ld(4, 2),
        ]
        hs = jnp.concatenate(tiles, axis=1).astype(bf16)
        x1 = hh[pl.ds(r, R), :] + jnp.dot(hs, tied(w2, ties), preferred_element_type=f32) * BETA
        hh[pl.ds(r, R), :] = x1

    l3s = {}

    def run_block(dots, extra=()):
        groups = []
        for d_, (k_, p) in enumerate(dots):
            if k_ == 1 and p not in l3s:
                groups += [(p, g, 25 * d_) for g in range(GP)]
        for p in extra:
            groups += [(p, g, 25 * len(dots) - 1) for g in range(GP)]
        slots = {}
        nxt = None
        for (p, g, hard) in reversed(groups):
            sl = hard if nxt is None else min(hard, nxt - (SP * GA if g % GA == GA - 1 else 0))
            sl = min(hard, max(sl, MINS))
            nxt = sl
            if sl < hard or p in extra:
                slots.setdefault(int(sl), []).append((p, g))
        for d_, (k_, p) in enumerate(dots):
            ties = {}
            for t in range(25):
                for (pp, g) in slots.get(25 * d_ + t, ()):
                    if pp not in l3s:
                        l3s[pp] = ln_chain(pp)
                    ties.setdefault(t, []).append(l3s[pp][8 * g:8 * g + 8, 0:128])
            if k_ == 1:
                if p not in l3s:
                    l3s[p] = ln_chain(p)
                w1_dot(p, l3s[p], ties)
            else:
                w2_dot(p, ties)

    with jax.named_scope("P1"):
        cp_wmp.wait()
        cp_q[0].wait()
        mp = jnp.dot(sc_lhs(), _wt(wmp), preferred_element_type=f32)
        for t in range(WMP // 128):
            modb[2 * WMA // 128 + t] = mp[0:8, 128 * t:128 * (t + 1)]
        sa, ca, ga, sb, cb = [modrow(k_) for k_ in range(5)]
        par[pl.ds(16, 8), :] = ga * (1.0 + ca)
        par[pl.ds(24, 8), :] = ga * sa
        par[pl.ds(32, 8), :] = 1.0 + cb
        par[pl.ds(40, 8), :] = sb
        for bt in range(4):
            inv_last(bt)
        for p in range(PRELN):
            l3s[p] = ln_chain(p)
    with jax.named_scope("w1wait"):
        cp_w[0].wait()
    p1, p2 = N2, 0
    with jax.named_scope("P2"):
        run_block([(1, p) for p in range(N2)])
    with jax.named_scope("w2wait"):
        cp_w[1].wait()
    with jax.named_scope("P3"):
        dots = []
        while p2 < Q0 // R - 3:
            dots.append((2, p2))
            p2 += 1
            if p1 < Q0 // R:
                dots.append((1, p1))
                p1 += 1
        run_block(dots)
    with jax.named_scope("q1wait"):
        cp_q[1].wait()
    with jax.named_scope("P4"):
        dots = [(2, p2), (2, p2 + 1)]
        p2 += 2
        while p2 < S // R and not SKIPB:
            while p1 < S // R and p1 - p2 < LEAD:
                dots.append((1, p1))
                p1 += 1
            dots.append((2, p2))
            p2 += 1
        run_block(dots)

    def out_copy(r):
        return cp(obuf.at[pl.ds(r, TS), :], o_hbm.at[0, pl.ds(r, TS), :], osems.at[0])

    def ln4(r):
        d4, r4 = _center(hh[pl.ds(r, TS), :], ALPHA)
        return d4 * r4

    def b2_step(i):
        gbv = par[pl.ds(48, 1), :]
        nsub = T2 // TS
        for sub in range(nsub):
            r = pl.multiple_of(pl.multiple_of(i * T2, T2) + sub * TS, TS)
            l4 = _wt(l4p, pl.ds(0, TS // 2), slice(None)) if (sub == 0 and LP) else ln4(r).astype(bf16)
            z = lax.dot_general(l4, _wt(w3, pl.ds(0, FA // 2), slice(None)), NTDIMS, preferred_element_type=f32)
            zt = lax.dot_general(_wt(w3, pl.ds(FA // 2, (F - FA) // 2), slice(None)), l4, NTDIMS,
                                 preferred_element_type=f32)
            g = jnp.concatenate([_gelu2a(z), _gelu2a(zt).T], axis=1).astype(bf16)
            if sub == nsub - 1 and LP:
                nx = ln4(pl.multiple_of(jnp.minimum(i + 1, S // T2 - 1) * T2, T2))
                l4p[pl.ds(0, TS // 2), :] = pltpu.bitcast(nx.astype(bf16), u32)
                t_ = pltpu.bitcast(nx[0:8, 0:128], u32)
                for gi in range(1, TS // 8):
                    t_ = t_ | pltpu.bitcast(nx[8 * gi:8 * gi + 8, 0:128], u32)
                top = [w4[pl.ds(0, 8), pl.ds(128 * n, 128)] for n in range(NT)]
                top[LPN] = top[LPN] | (t_ & kbuf[0, pl.ds(0, 8), :])
                w4v = jnp.concatenate([jnp.concatenate(top, axis=1), w4[pl.ds(8, F // 2 - 8), :]], axis=0)
            else:
                w4v = w4[...]
            acc = jnp.dot(g, pltpu.bitcast(w4v, bf16), preferred_element_type=f32)
            obuf[pl.ds(r, TS), :] = (xn[pl.ds(r, TS), :] + gbv * (hh[pl.ds(r, TS), :] + BETA * acc)).astype(bf16)
            out_copy(r).start()

    with jax.named_scope("B2_wait"):
        cp_w[2].wait()
        cp_w[3].wait()
        cp_wmc.wait()
        mc = jnp.dot(sc_lhs(), _wt(wmc), preferred_element_type=f32)[0:8]
        par[pl.ds(48, 8), :] = mc
        if LP:
            l4p[pl.ds(0, TS // 2), :] = pltpu.bitcast(ln4(0).astype(bf16), u32)
    with jax.named_scope("BII"):
        lax.fori_loop(0, S // T2, lambda i, c: (b2_step(i), c)[1], 0)
    with jax.named_scope("out_wait"):
        for i in range(S // TS):
            out_copy(i * TS).wait()


@jax.jit
def pallas_adaLN_cond__ssm_conv_h3__mixer_s_mlp__prompt_kernel(
    A_q, A_k, A_v, A_shift_k, A_ssm_k, A_ssm_D, B_x, B_w1, B_w2, B_w3, B_w4, c, w_mod,
):
    del B_x
    hbm = pl.BlockSpec(memory_space=pltpu.MemorySpace.HBM)
    return pl.pallas_call(
        _kernel,
        out_shape=jax.ShapeDtypeStruct((1, S, D), bf16),
        in_specs=[hbm] * 12,
        out_specs=hbm,
        scratch_shapes=[
            pltpu.VMEM((27, 8, 128), f32),
            pltpu.VMEM((S + 16 * int(os.environ.get('PADF', '0')), D), bf16),
            pltpu.VMEM((NT, 32 + S // 2, 128), u32),
            pltpu.VMEM((NT, 32 + S // 2, 128), u32),
            pltpu.VMEM((NT, 64, S), u32),
            pltpu.VMEM((D // 2, D), u32),
            pltpu.VMEM((D // 2, D), u32),
            pltpu.VMEM((F // 2, D), u32),
            pltpu.VMEM((F // 2, D), u32),
            pltpu.VMEM((2, D // 2, WMA), u32),
            pltpu.VMEM((D // 2, WMP), u32),
            pltpu.VMEM((D // 2, WMC), u32),
            pltpu.VMEM((S, D), bf16),
            pltpu.VMEM((NG * 2 * NC, 8, 128), f32),
            pltpu.VMEM((NG * 2 * NC, 8, 128), f32),
            pltpu.VMEM((NG * 2 * NC, 8, 128), f32),
            pltpu.VMEM((NG * 2 * NC, 8, 128), f32),
            pltpu.VMEM((KOFF + 56 + PADK, 8, 128), f32),
            pltpu.VMEM((KOFF + 56 + PADK, 8, 128), f32),
            pltpu.VMEM((NT, S, 128), f32),
            pltpu.VMEM((S, D), f32),
            pltpu.VMEM((S, D), f32),
            pltpu.VMEM((NT, S + 32, 128), f32),
            pltpu.VMEM((64, D), f32),
            pltpu.VMEM((TS // 2 + 8 * int(os.environ.get('PADE', '0')), D), u32),
            pltpu.VMEM((4, D), bf16),
            pltpu.VMEM((D,), bf16),
            pltpu.VMEM((1, D), bf16),
            pltpu.SMEM((2,), jnp.int32),
            pltpu.SemaphoreType.DMA((22,)),
            pltpu.SemaphoreType.DMA((1,)),
        ],
        compiler_params=pltpu.CompilerParams(vmem_limit_bytes=100 * 1024 * 1024, disable_semaphore_checks=True,
                                             disable_bounds_checks=bool(int(os.environ.get('NOBC', '0')))),
    )(A_q, A_k, A_v, A_shift_k.T, A_ssm_k, A_ssm_D, B_w1, B_w2, B_w3.T, B_w4, c, w_mod)
```

```python
import math
import os

import jax
import jax.numpy as jnp
from jax import lax
import jax.experimental.pallas as pl
import jax.experimental.pallas.tpu as pltpu

S, D, F = 2048, 640, 1728
C = 128
NC = S // C
NT = D // 128
NG = 16
KOFF = (NC + 1) * NG * 3
W = int(os.environ.get('W', '4'))
SKIPA = int(os.environ.get('SKIPA', '0'))
WMA, WMP, WMC = 1280, 640, 640
Q0 = int(os.environ.get('Q0', '384'))
N2 = int(os.environ.get('N2', '4'))
PRELN = int(os.environ.get('PRELN', '2'))
NOCACHE = int(os.environ.get('NOCACHE', '0'))
OUTWAIT = int(os.environ.get('OUTWAIT', '0'))
SEGS = [int(x) for x in os.environ.get('SEGS', '012345')]
SKIPB = int(os.environ.get('SKIPB', '0'))
PADK = int(os.environ.get('PADK', '0'))
PREW = int(os.environ.get('PREW', '0'))
SP = float(os.environ.get('SP', '0'))
MINS = int(os.environ.get('MINS', '30'))
GA = int(os.environ.get('GA', '2'))
TRT = int(os.environ.get('TRT', '1'))
LP = int(os.environ.get('LP', '1'))
FA = 1664
LPN = int(os.environ.get('LPN', '2'))
G0 = int(os.environ.get('G0', '4'))
Q1 = int(os.environ.get('Q1', '1408'))
TIE4 = int(os.environ.get('TIE4', '12'))
KARA = int(os.environ.get('KARA', '1'))
UNR = int(os.environ.get('UNR', '2'))
HEAD = int(os.environ.get('HEAD', '250'))
TAIL = int(os.environ.get('TAIL', '450'))
DORDER = os.environ.get('DORDER', 'HaUb')
R1 = int(os.environ.get('R1', '64'))
R2 = int(os.environ.get('R2', '128'))
LEAD = int(os.environ.get('LEAD', '4'))
TS = int(os.environ.get('TS', '256'))
ONEPASS = int(os.environ.get('ONEPASS', '1'))
RSQ = int(os.environ.get('RSQ', '1'))
T2 = int(os.environ.get('T2', '512'))
EPS = 1e-5
_C0 = math.sqrt(2.0 / math.pi)
ALPHA = (_C0 * 0.044715) ** (1.0 / 3.0)
GC = _C0 / ALPHA
BETA = 0.5 / ALPHA
_fc = [int(x) for x in os.environ.get('FC', '1728').split(',')]
F_CHUNKS = tuple((sum(_fc[:i]), _fc[i]) for i in range(len(_fc)))
assert sum(_fc) == F

f32 = jnp.float32
bf16 = jnp.bfloat16
u32 = jnp.uint32
NTDIMS = (((1,), (1,)), ((), ()))


def _cos_table(m, scale):
    mm = jnp.abs(((m + 256) & 511) - 256)
    x = (128 - mm).astype(f32) * (1.0 / 128.0)
    x2 = x * x
    h = math.pi / 2
    p = -(h ** 7) / 5040 + x2 * ((h ** 9) / 362880 - x2 * (h ** 11) / 39916800)
    p = h + x2 * (-(h ** 3) / 6 + x2 * ((h ** 5) / 120 + x2 * p))
    return (x * scale) * p


def _dft_tables():
    shape = (16, 8, 128)
    n = lax.broadcasted_iota(jnp.int32, shape, 0)
    s = lax.broadcasted_iota(jnp.int32, shape, 1)
    l = lax.broadcasted_iota(jnp.int32, shape, 2)
    fw, fu, iv = [], [], []
    wv = l >> 4
    tu = (16 * W) * (wv // W) + (2 * W) * ((l >> 1) & 7) + 2 * (wv % W) + (l & 1)
    for e in range(2):
        r = 2 * s + e
        j = 8 * n + (r & 7)
        fw.append(_cos_table((4 * j + 1) * l + (r >> 3) * 128, 1.0))
        fu.append(_cos_table((4 * j + 1) * tu + (r >> 3) * 128, 1.0))
        b = 16 * (n >> 1) + r
        col = 128 * (n & 1) + l
        iv.append(_cos_table((4 * (col >> 1) + 1) * b + (col & 1) * 128, 1.0 / 128.0))
    pk = lambda xs: pltpu.bitcast(pltpu.pack_elementwise(xs, packed_dtype=bf16), f32)
    return pk(fw), pk(iv), pk(fu)


def _gelu2a(z):
    return z * (1.0 + jnp.tanh(z * (z * z + GC)))


def _rstd(ssd, scale):
    if RSQ == 0:
        r = lax.rsqrt(ssd * (1.0 / D) + EPS)
        return r if scale == 1.0 else r * scale
    return jnp.exp2(jnp.log(ssd + D * EPS) * (-0.5 / math.log(2.0)) + math.log2(scale * math.sqrt(D)))


def _center(x, scale=1.0):
    s1 = jnp.sum(x, axis=-1, keepdims=True)
    m = s1 * (1.0 / D)
    d = x - m
    if ONEPASS:
        ssd = jnp.maximum(jnp.sum(x * x, axis=-1, keepdims=True) - s1 * m, 0.0)
    else:
        ssd = jnp.sum(d * d, axis=-1, keepdims=True)
    return d, _rstd(ssd, scale)


def _conv(us, gs, a):
    acc = None
    for c in range(a + 1):
        p = us[c] * gs[a - c]
        acc = p if acc is None else acc + p
    return acc


def _mult(x, n):
    return x if isinstance(x, int) else pl.multiple_of(x, n)


def _wt(ref, *idx):
    return pltpu.bitcast(ref[idx] if idx else ref[...], bf16)


def _kernel(q_hbm, k_hbm, v_hbm, sk_hbm, h_hbm, dd_hbm, w1_hbm, w2_hbm, w3_hbm, w4_hbm,
            c_hbm, wm_hbm, o_hbm,
            modb, qbuf, kbuf, vbuf, hbuf, w1, w2, w3, w4, wm, wmp, wmc, obuf,
            ub0, ub1, gb0, gb1, kb0, kb1, yb, xn, hh, h1, par, l4p, sk_s, dd_s, c_s, zs, sems, osems):
    ubs, gbs, kbs = (ub0, ub1), (gb0, gb1), (kb0, kb1)
    cp = pltpu.make_async_copy
    HS = S // 2

    def cp_h(j, c0, c1, sem):
        return cp(h_hbm.at[pl.ds(j * 128, 128), pl.ds(c0, c1 - c0)], hbuf.bitcast(bf16).at[j, :, pl.ds(c0, c1 - c0)], sem)

    def cp_kv(j, r0, r1, sem):
        r0, r1 = (r0 + 16 if r0 else 0), min(r1 + 16, S)
        lanes = pl.ds(j * 128, 128)
        return [cp(k_hbm.at[0, pl.ds(r0, r1 - r0), lanes], kbuf.bitcast(bf16).at[j, pl.ds(r0 + 16, r1 - r0), :], sem),
                cp(v_hbm.at[0, pl.ds(r0, r1 - r0), lanes], vbuf.bitcast(bf16).at[j, pl.ds(r0, r1 - r0), :], sem)]

    def cp_tile(j, i):
        sem = sems.at[2 * j + i]
        return [cp_h(j, i * HS, (i + 1) * HS, sem)] + cp_kv(j, i * HS, (i + 1) * HS, sem)

    cp_t0 = [[cp_h(0, 0, S, sems.at[0])], cp_kv(0, 0, 1024, sems.at[1]), cp_kv(0, 1024, 1536, sems.at[20]),
             cp_kv(0, 1536, S, sems.at[21])]

    def cp_wm(i):
        return cp(wm_hbm.at[:, pl.ds(i * WMA, WMA)], wm.bitcast(bf16).at[i], sems.at[10 + i])

    cp_wmp = cp(wm_hbm.at[:, pl.ds(2 * WMA, WMP)], wmp.bitcast(bf16), sems.at[13])
    cp_wmc = cp(wm_hbm.at[:, pl.ds(2 * WMA + WMP, WMC)], wmc.bitcast(bf16), sems.at[12])
    cp_q = [cp(q_hbm.at[0, pl.ds(r0, r1 - r0), :], qbuf.at[pl.ds(r0, r1 - r0), :], sems.at[sm])
            for sm, r0, r1 in ((13, 0, Q0), (14, Q0, Q1), (12, Q1, S))]
    cp_w = [cp(s_, d_.bitcast(bf16), sems.at[sm])
            for sm, s_, d_ in ((15, w1_hbm, w1), (16, w2_hbm, w2), (12, w3_hbm, w3), (12, w4_hbm, w4))]
    cp_s = [cp(sk_hbm, sk_s, sems.at[19]), cp(dd_hbm, dd_s, sems.at[19]), cp(c_hbm, c_s, sems.at[19])]
    order = list(cp_s)
    for grp in cp_t0:
        order += grp
    for j in range(1, NT):
        order += cp_tile(j, 0) + cp_tile(j, 1)
    order += [cp_wm(0), cp_wm(1), cp_wmp, cp_q[0], cp_w[0], cp_w[1], cp_q[1], cp_q[2], cp_wmc, cp_w[2], cp_w[3]]
    for c_ in order:
        c_.start()

    with jax.named_scope("init"):
        fw_t, iv_t, fu_t = _dft_tables()
        for kb in kbs:
            kb[pl.ds(KOFF, 16)] = fw_t
            kb[pl.ds(KOFF + 16, 16)] = iv_t
            kb[pl.ds(KOFF + 32, 16)] = fu_t
            kb[pl.ds(0, NG * 3)] = jnp.zeros((NG * 3, 8, 128), f32)
        zeros = jnp.zeros((8, 128), f32)
        for j in range(NT):
            kbuf[j, pl.ds(0, 8), :] = jnp.zeros((8, 128), u32)
            kbuf[j, pl.ds(8 + HS, 8), :] = jnp.zeros((8, 128), u32)
            vbuf[j, pl.ds(HS, 8), :] = jnp.zeros((8, 128), u32)
        for j in range(NT):
            h1[j, pl.ds(0, 8), :] = zeros
            h1[j, pl.ds(S + 8, 8), :] = zeros
        for c_ in cp_s:
            c_.wait()
        par[pl.ds(0, 4), :] = sk_s[...].astype(f32)
        par[pl.ds(8, 8), :] = jnp.broadcast_to(dd_s[...].astype(f32).reshape(1, D), (8, D))
        cv = c_s[...].astype(f32)
        sc = jnp.broadcast_to(cv * jax.nn.sigmoid(cv), (8, D))
        scp = pltpu.bitcast(pltpu.pack_elementwise([sc, sc], packed_dtype=bf16), f32)
        for j in range(NT):
            kb0[KOFF + 48 + j] = scp[:, 128 * j:128 * (j + 1)]
            kb1[KOFF + 48 + j] = scp[:, 128 * j:128 * (j + 1)]

    def mkb(i, unr, off, cache):
        def b(stride, extra=0, z=None):
            if isinstance(i, int):
                return (i * unr + off) * stride + extra
            key = (unr * stride, z)
            if key not in cache or NOCACHE:
                base = pl.multiple_of(i * (unr * stride), unr * stride)
                cache[key] = base if z is None else base + (i >> z)
            return cache[key] + (off * stride + extra)
        return b

    def dot_h(j, b, lhs):
        gb = gbs[j % 2]
        hc = hbuf[j, :, pl.ds(_mult(b(512), 512), 512)]
        rhs_t = jnp.concatenate([hc[:, C * cc:C * (cc + 1)] for cc in range(4)], axis=0)
        g = lax.dot_general(lhs, pltpu.bitcast(rhs_t, bf16), NTDIMS, preferred_element_type=f32)
        for rg in range(2 * NG):
            for cc in range(4):
                gb[b(4, cc + rg * NC)] = g[8 * rg:8 * rg + 8, 128 * cc:128 * cc + 128]

    def dot_u(j, b, lhs):
        ub = ubs[j % 2]
        taps = [par[pl.ds(t, 1), pl.ds(j * 128, 128)] for t in range(4)]
        unp = lambda w_, e: pltpu.unpack_elementwise(w_, index=e, packed_dtype=bf16, unpacked_dtype=f32)
        cols = []
        for cc in range(4):
            words = []
            for blk in range(8 // W):
                w0 = 64 * cc + 8 * W * blk
                kw = {m: kbuf[j, pl.ds(b(256, 8 + w0 + m), 8, stride=W), :] for m in range(-2, W)}
                kk = {2 * m + e: unp(kw[m], e) for m in range(-2, W) for e in range(2) if 2 * m + e >= -3}
                for m in range(W):
                    vw = vbuf[j, pl.ds(b(256, w0 + m), 8, stride=W), :]
                    pair = []
                    for e in range(2):
                        n = 2 * m + e
                        ks = kk[n] * taps[0] + kk[n - 1] * taps[1] + kk[n - 2] * taps[2] + kk[n - 3] * taps[3]
                        pair.append(ks * unp(vw, e))
                    words.append(pltpu.pack_elementwise(pair, packed_dtype=bf16))
            cols.append(jnp.concatenate(words, axis=0))
        rhs = pltpu.bitcast(jnp.concatenate(cols, axis=1), bf16)
        u = jnp.dot(lhs, rhs, preferred_element_type=f32)
        for rg in range(2 * NG):
            for cc in range(4):
                ub[b(4, cc + rg * NC)] = u[8 * rg:8 * rg + 8, 128 * cc:128 * cc + 128]

    def dot_i(j, b, half, lhs):
        kb = kbs[j % 2]
        cols = [[], []]
        for gi in range(NG):
            prev = None
            for cc in range(-1, 2):
                k0, k1, k2 = [kb[b(4 * NG * 3, ((2 * half + cc + 1) * NG + gi) * 3 + t)] for t in range(3)]
                re, im = k0 - k2, k0 + k1
                if prev is not None:
                    cols[cc].append(pltpu.pack_elementwise([re - prev[1], im + prev[0]], packed_dtype=bf16))
                prev = (re, im)
        rhs = jnp.concatenate([jnp.concatenate(c_, axis=0) for c_ in cols], axis=1)
        y = jnp.dot(lhs, pltpu.bitcast(rhs, bf16), preferred_element_type=f32)
        for cc in range(2):
            yb[j, pl.ds(b(512, (2 * half + cc) * C), C), :] = y[:, 128 * cc:128 * cc + 128]

    def gen_m(j, kb, b, ng):
        ub, gb = ubs[j % 2], gbs[j % 2]
        for s in range(ng):
            for t in range(3):
                z = 8 + t
                re = lambda ref, c: ref[b(2 * NC, 2 * s * NC + c, z)]
                im = lambda ref, c: ref[b(2 * NC, (2 * s + 1) * NC + c, z)]
                gre = [re(gb, c) for c in range(NC)]
                if t == 0:
                    us = [re(ub, c) + im(ub, c) for c in range(NC)]
                    gs = gre
                elif t == 1:
                    us = [re(ub, c) for c in range(NC)]
                    gs = [im(gb, c) - gre[c] for c in range(NC)]
                else:
                    us = [im(ub, c) for c in range(NC)]
                    gs = [im(gb, c) + gre[c] for c in range(NC)]

                def st(a, val):
                    kb[b(3, ((a + 1) * NG + s) * 3 + t)] = val
                if not KARA:
                    for a in range(NC):
                        st(a, _conv(us, gs, a))
                        yield 2 * a + 2
                    continue
                ue, uo, ge, go = us[0::2], us[1::2], gs[0::2], gs[1::2]
                usum = [x + y for x, y in zip(ue, uo)]
                gsum = [x + y for x, y in zip(ge, go)]
                poo_prev = None
                for a in range(NC // 2):
                    pee = _conv(ue, ge, a)
                    poo = _conv(uo, go, a)
                    pss = _conv(usum, gsum, a)
                    st(2 * a, pee if poo_prev is None else pee + poo_prev)
                    st(2 * a + 1, pss - pee - poo)
                    poo_prev = poo
                    yield 3 * (2 * a + 1) + 7

    def add_d(j):
        gb = gbs[j % 2]
        dvec = par[pl.ds(8, 8), pl.ds(j * 128, 128)]
        for gi in range(NG):
            gb[2 * gi * NC] = gb[2 * gi * NC] + dvec

    def sc_lhs():
        return pltpu.bitcast(jnp.concatenate([kb0[KOFF + 48 + j] for j in range(NT)], axis=1), bf16)

    def dot_m(i, t0, nt, rows):
        m = None
        for kt in range(NT):
            p = jnp.dot(pltpu.bitcast(rows[kt], bf16), _wt(wm, i, pl.ds(64 * kt, 64), pl.ds(128 * t0, 128 * nt)),
                        preferred_element_type=f32)
            m = p if m is None else m + p
        for t in range(nt):
            modb[i * (WMA // 128) + (t0 + t)] = m[0:8, 128 * t:128 * (t + 1)]

    def inv_lhs(tbl, n):
        return jnp.concatenate([tbl[KOFF + 16 + 2 * n], tbl[KOFF + 17 + 2 * n]], axis=1)

    def dot_k(kb, kt, bt, lhs):
        cols = [[] for _ in range(4)]
        for gi in range(8 * kt, 8 * kt + 8):
            prev = None
            for cc in range(-1, 4):
                k0, k1, k2 = [kb[((4 * bt + cc + 1) * NG + gi) * 3 + t] for t in range(3)]
                re, im = k0 - k2, k0 + k1
                if prev is not None:
                    cols[cc].append(pltpu.pack_elementwise([re - prev[1], im + prev[0]], packed_dtype=bf16))
                prev = (re, im)
        rhs = jnp.concatenate([jnp.concatenate(c_, axis=0) for c_ in cols], axis=1)
        y = jnp.dot(lhs, pltpu.bitcast(rhs, bf16), preferred_element_type=f32)
        for cc in range(4):
            rows = pl.ds((4 * bt + cc) * C, C)
            yc = y[:, 128 * cc:128 * cc + 128]
            yb[NT - 1, rows, :] = yc if kt == 0 else yb[NT - 1, rows, :] + yc

    PRE = dict(H=0, U=672 + 96 // W, a=192, b=192, m=0, k=176)
    POST = dict(H=0, U=0, a=4, b=4, m=2, k=0)
    NST = dict(H=16, U=16, a=8, b=8, m=5, k=8)
    GCOST = 3 * (248 if KARA else 272)

    def a_block(dots, mg=None, ng=0, tbl=kb0):
        native, dur = [], []
        for idx, (k_, _) in enumerate(dots):
            nxt = PRE[dots[idx + 1][0]] if idx + 1 < len(dots) else 0
            d_ = 2.0 if k_ == 'm' else 1.0
            native += [nxt / NST[k_] + POST[k_] * d_] * NST[k_]
            dur += [d_] * NST[k_]
        if mg is not None and dots:
            head = max(HEAD - PRE[dots[0][0]], 0)
            mtot = GCOST * ng - TAIL - head
            lvl = (mtot + sum(native)) / sum(dur)
            want = [max(lvl * d_ - x, 0.0) for x, d_ in zip(native, dur)]
            scale = mtot / sum(want)
            cum, tgt = [head], head
            for w_ in want:
                tgt += w_ * scale
                cum.append(tgt)
        done = 0.0
        step = 0
        for (k_, fn) in dots:
            rows = []
            for n in range(NST[k_]):
                if mg is not None:
                    while done < cum[step]:
                        done += next(mg)
                step += 1
                if k_ in 'HU':
                    rows.append(tbl[KOFF + n + (32 if k_ == 'U' else 0)])
                elif k_ in 'ab':
                    rows.append(inv_lhs(tbl, n))
                elif k_ == 'k':
                    rows.append(tbl[KOFF + 16 + 2 * n])
                else:
                    rows.append(tbl[KOFF + 48 + n])
            fn(rows if k_ == 'm' else pltpu.bitcast(jnp.concatenate(rows, axis=0), bf16))
        if mg is not None:
            for _ in mg:
                pass

    def fdot(k_, j, b):
        if k_ == 'H':
            return (k_, lambda lhs: dot_h(j, b, lhs))
        if k_ == 'U':
            return (k_, lambda lhs: dot_u(j, b, lhs))
        return (k_, lambda lhs: dot_i(j, b, 0 if k_ == 'a' else 1, lhs))

    def wait_all(cps):
        for c_ in cps:
            c_.wait()

    def a_loop(jf, jm, ji, g0, ng):
        kinds = [k_ for k_ in DORDER if k_ in 'HU' or ji is not None]

        def body(i, carry):
            cache = {}
            zs[i] = 0
            dots = [fdot(k_, jf if k_ in 'HU' else ji, mkb(i, 2, s_, cache)) for s_ in range(2) for k_ in kinds]
            a_block(dots, gen_m(jm, kbs[jm % 2], mkb(i, ng, g0, cache), ng), ng, kbs[jm % 2])

            @pl.when(i == 0)
            def _():
                wait_all(cp_tile(jf, 1))
            return carry
        wait_all(cp_tile(jf, 0))
        lax.fori_loop(0, 2, body, 0)
        add_d(jf)

    sb_ = lambda bt: mkb(0, 1, bt, None)
    with jax.named_scope("A_seg0"):
        wait_all(cp_t0[0])
        a_block([fdot('H', 0, sb_(bt)) for bt in range(4)])
        add_d(0)
        wait_all(cp_t0[1])
        a_block([fdot('U', 0, sb_(bt)) for bt in range(2)])
        for bt in (2, 3):
            wait_all(cp_t0[bt])
            a_block([fdot('U', 0, sb_(bt))])
    with jax.named_scope("A_m0"):
        def body_m0(i, carry):
            a_block([], gen_m(0, kb0, mkb(i, G0 // 2, 0, {}), G0 // 2))
            return carry
        if G0:
            lax.fori_loop(0, 2, body_m0, 0)
    for seg in range(1, NT):
        with jax.named_scope(f"A_seg{seg}"):
            if seg == 1:
                a_loop(1, 0, None, G0, (NG - G0) // 2)
            else:
                a_loop(seg, seg - 1, seg - 2, 0, 8)

    def mods(i):
        return [('m', lambda rows, t0=t0, nt=nt: dot_m(i, t0, nt, rows)) for (t0, nt) in ((0, 4), (4, 4), (8, 2))]

    with jax.named_scope("A_seg5a"):
        cp_wm(0).wait()
        zz = zs[1]

        @pl.when(zz == 0)
        def _():
            dots = [fdot(k_, NT - 2, sb_(bt)) for bt in range(4) for k_ in 'ab']
            mm = mods(0)
            dots = [mm[0]] + dots[0:2] + [mm[1]] + dots[2:4] + [mm[2]] + dots[4:]
            a_block(dots, gen_m(NT - 1, kb0, mkb(zz, 8, 0, {}), 8), 8, kb0)
    with jax.named_scope("A_seg5b"):
        cp_wm(1).wait()

        @pl.when(zz == 0)
        def _():
            dots = [('k', lambda lhs, bt=bt: dot_k(kb0, 0, bt, lhs)) for bt in range(4)]
            mm = mods(1)
            dots = [mm[0], dots[0], mm[1], dots[1], mm[2]] + dots[2:]
            a_block(dots, gen_m(NT - 1, kb1, mkb(zz, 8, 8, {}), 8), 8, kb1)

    def inv_last(bt):
        lhs = pltpu.bitcast(jnp.concatenate([kb0[KOFF + 17 + 2 * n] for n in range(8)], axis=0), bf16)
        dot_k(kb1, 1, bt, lhs)

    def modrow(k_):
        return jnp.concatenate([modb[NT * k_ + j] for j in range(NT)], axis=1)

    R = R1
    GP = R // 8

    def ln_chain(p):
        r = p * R
        pa, pb, pc, ps = [par[pl.ds(16 + 8 * t, 8), :][None] for t in range(4)]
        g3 = lambda x: x.reshape(GP, 8, D)
        q = g3(qbuf[pl.ds(r, R), :].astype(f32))
        d1, r1 = _center(q)
        y = g3(jnp.concatenate([yb[j, pl.ds(r, R), :] for j in range(NT)], axis=1))
        x = q + ((d1 * r1) * pa + pb) * y
        xn[pl.ds(r, R), :] = x.reshape(R, D)
        d2, r2 = _center(x)
        h = (d2 * r2) * pc + ps
        hh[pl.ds(r, R), :] = h.reshape(R, D)
        d3, r3 = _center(h, ALPHA)
        return (d3 * r3).reshape(R, D)

    def tied(wref, ties):
        if not ties:
            return _wt(wref)
        rows = []
        for kt in range(NT):
            rows.append(wref[pl.ds(64 * kt, 56), :])
            last = []
            for n in range(NT):
                w_ = wref[pl.ds(64 * kt + 56, 8), pl.ds(128 * n, 128)]
                vs = ties.get(5 * n + kt)
                if vs:
                    t_ = pltpu.bitcast(vs[0], u32)
                    for v_ in vs[1:]:
                        t_ = t_ | pltpu.bitcast(v_, u32)
                    w_ = w_ | (t_ & kbuf[0, pl.ds(0, 8), :])
                last.append(w_)
            rows.append(jnp.concatenate(last, axis=1))
        return pltpu.bitcast(jnp.concatenate(rows, axis=0), bf16)

    def w1_dot(p, l3, ties):
        z = jnp.dot(l3.astype(bf16), tied(w1, ties), preferred_element_type=f32)
        g = _gelu2a(z)
        for j in range(NT):
            h1[j, pl.ds(p * R + 8, R), :] = g[:, j * 128:(j + 1) * 128]

    def w2_dot(p, ties):
        r = p * R
        lane = lax.broadcasted_iota(jnp.int32, (R, 128), 1)

        def ld(j, off):
            return h1[j, pl.ds(r + 8 + off, R), :]
        tiles = [
            ld(0, -1),
            jnp.where(lane < 32, ld(1, -1), ld(1, 1)),
            jnp.where(lane < 64, ld(2, 1), ld(2, -2)),
            jnp.where(lane < 96, ld(3, -2), ld(3, 2)),
            ld(4, 2),
        ]
        hs = jnp.concatenate(tiles, axis=1).astype(bf16)
        x1 = hh[pl.ds(r, R), :] + jnp.dot(hs, tied(w2, ties), preferred_element_type=f32) * BETA
        hh[pl.ds(r, R), :] = x1

    l3s = {}

    def ln4(r, n):
        d4, r4 = _center(hh[pl.ds(r, n), :], ALPHA)
        return d4 * r4

    def run_block(dots, pre4=False):
        for d_, (k_, p) in enumerate(dots):
            ties = {}
            e = d_ - (len(dots) - TS // R)
            if pre4 and e >= 0:
                nx = ln4(e * R, R)
                l4p[pl.ds(e * R // 2, R // 2), :] = pltpu.bitcast(nx.astype(bf16), u32)
                ties[TIE4] = [nx[8 * g:8 * g + 8, 0:128] for g in range(GP)]
            if k_ == 1:
                w1_dot(p, l3s.pop(p) if p in l3s else ln_chain(p), ties)
            elif k_ == 2:
                w2_dot(p, ties)
            else:
                par[pl.ds(48, 8), :] = jnp.dot(sc_lhs(), _wt(wmc), preferred_element_type=f32)[0:8]

    with jax.named_scope("P1"):
        cp_wmp.wait()
        cp_q[0].wait()
        mp = jnp.dot(sc_lhs(), _wt(wmp), preferred_element_type=f32)
        for t in range(WMP // 128):
            modb[2 * WMA // 128 + t] = mp[0:8, 128 * t:128 * (t + 1)]
        sa, ca, ga, sb, cb = [modrow(k_) for k_ in range(5)]
        par[pl.ds(16, 8), :] = ga * (1.0 + ca)
        par[pl.ds(24, 8), :] = ga * sa
        par[pl.ds(32, 8), :] = 1.0 + cb
        par[pl.ds(40, 8), :] = sb
        for bt in range(4):
            inv_last(bt)
        for p in range(PRELN):
            l3s[p] = ln_chain(p)
    with jax.named_scope("w1wait"):
        cp_w[0].wait()
    p1, p2 = N2, 0
    with jax.named_scope("P2"):
        run_block([(1, p) for p in range(N2)])
    with jax.named_scope("w2wait"):
        cp_w[1].wait()

    def plan(lim1, hold):
        nonlocal p1, p2
        dots = []
        while p2 < p1 - 1 and len(dots) < 2:
            dots.append((2, p2))
            p2 += 1
        last2 = lim1 if lim1 == S // R else lim1 - 1 - hold
        while p2 < last2 or p1 < lim1:
            while p1 < lim1 and (p1 - p2 < LEAD or p2 >= last2):
                dots.append((1, p1))
                p1 += 1
            if p2 < last2:
                dots.append((2, p2))
                p2 += 1
        return dots

    with jax.named_scope("P3"):
        run_block(plan(Q0 // R, 2))
    with jax.named_scope("q1wait"):
        cp_q[1].wait()
    with jax.named_scope("P4"):
        run_block(plan(Q1 // R, 2))
    with jax.named_scope("q2wait"):
        wait_all([cp_q[2], cp_wmc, cp_w[2], cp_w[3]])
    with jax.named_scope("P5"):
        dots = plan(S // R, 0)
        run_block(dots[:2] + [(3, 0)] + dots[2:], pre4=True)

    def out_copy(r):
        return cp(obuf.at[pl.ds(r, TS), :], o_hbm.at[0, pl.ds(r, TS), :], osems.at[0])

    def b2_step(i):
        gbv = par[pl.ds(48, 1), :]
        nsub = T2 // TS
        for sub in range(nsub):
            r = pl.multiple_of(pl.multiple_of(i * T2, T2) + sub * TS, TS)
            l4 = _wt(l4p, pl.ds(0, TS // 2), slice(None)) if (sub == 0 and LP) else ln4(r, TS).astype(bf16)
            z = lax.dot_general(l4, _wt(w3, pl.ds(0, FA // 2), slice(None)), NTDIMS, preferred_element_type=f32)
            zt = lax.dot_general(_wt(w3, pl.ds(FA // 2, (F - FA) // 2), slice(None)), l4, NTDIMS,
                                 preferred_element_type=f32)
            g = jnp.concatenate([_gelu2a(z), _gelu2a(zt).T], axis=1).astype(bf16)
            if sub == nsub - 1 and LP:
                nx = ln4(pl.multiple_of(jnp.minimum(i + 1, S // T2 - 1) * T2, T2), TS)
                l4p[pl.ds(0, TS // 2), :] = pltpu.bitcast(nx.astype(bf16), u32)
                t_ = pltpu.bitcast(nx[0:8, 0:128], u32)
                for gi in range(1, TS // 8):
                    t_ = t_ | pltpu.bitcast(nx[8 * gi:8 * gi + 8, 0:128], u32)
                top = [w4[pl.ds(0, 8), pl.ds(128 * n, 128)] for n in range(NT)]
                top[LPN] = top[LPN] | (t_ & kbuf[0, pl.ds(0, 8), :])
                w4v = jnp.concatenate([jnp.concatenate(top, axis=1), w4[pl.ds(8, F // 2 - 8), :]], axis=0)
            else:
                w4v = w4[...]
            acc = jnp.dot(g, pltpu.bitcast(w4v, bf16), preferred_element_type=f32)
            obuf[pl.ds(r, TS), :] = (xn[pl.ds(r, TS), :] + gbv * (hh[pl.ds(r, TS), :] + BETA * acc)).astype(bf16)
            out_copy(r).start()

    with jax.named_scope("BII"):
        lax.fori_loop(0, S // T2, lambda i, c: (b2_step(i), c)[1], 0)
    with jax.named_scope("out_wait"):
        for i in range(S // TS):
            out_copy(i * TS).wait()


@jax.jit
def pallas_adaLN_cond__ssm_conv_h3__mixer_s_mlp__prompt_kernel(
    A_q, A_k, A_v, A_shift_k, A_ssm_k, A_ssm_D, B_x, B_w1, B_w2, B_w3, B_w4, c, w_mod,
):
    del B_x
    hbm = pl.BlockSpec(memory_space=pltpu.MemorySpace.HBM)
    return pl.pallas_call(
        _kernel,
        out_shape=jax.ShapeDtypeStruct((1, S, D), bf16),
        in_specs=[hbm] * 12,
        out_specs=hbm,
        scratch_shapes=[
            pltpu.VMEM((27, 8, 128), f32),
            pltpu.VMEM((S + 16 * int(os.environ.get('PADF', '0')), D), bf16),
            pltpu.VMEM((NT, 32 + S // 2, 128), u32),
            pltpu.VMEM((NT, 32 + S // 2, 128), u32),
            pltpu.VMEM((NT, 64, S), u32),
            pltpu.VMEM((D // 2, D), u32),
            pltpu.VMEM((D // 2, D), u32),
            pltpu.VMEM((F // 2, D), u32),
            pltpu.VMEM((F // 2, D), u32),
            pltpu.VMEM((2, D // 2, WMA), u32),
            pltpu.VMEM((D // 2, WMP), u32),
            pltpu.VMEM((D // 2, WMC), u32),
            pltpu.VMEM((S, D), bf16),
            pltpu.VMEM((NG * 2 * NC, 8, 128), f32),
            pltpu.VMEM((NG * 2 * NC, 8, 128), f32),
            pltpu.VMEM((NG * 2 * NC, 8, 128), f32),
            pltpu.VMEM((NG * 2 * NC, 8, 128), f32),
            pltpu.VMEM((KOFF + 56 + PADK, 8, 128), f32),
            pltpu.VMEM((KOFF + 56 + PADK, 8, 128), f32),
            pltpu.VMEM((NT, S, 128), f32),
            pltpu.VMEM((S, D), f32),
            pltpu.VMEM((S, D), f32),
            pltpu.VMEM((NT, S + 32, 128), f32),
            pltpu.VMEM((64, D), f32),
            pltpu.VMEM((TS // 2 + 8 * int(os.environ.get('PADE', '0')), D), u32),
            pltpu.VMEM((4, D), bf16),
            pltpu.VMEM((D,), bf16),
            pltpu.VMEM((1, D), bf16),
            pltpu.SMEM((2,), jnp.int32),
            pltpu.SemaphoreType.DMA((22,)),
            pltpu.SemaphoreType.DMA((1,)),
        ],
        compiler_params=pltpu.CompilerParams(vmem_limit_bytes=100 * 1024 * 1024, disable_semaphore_checks=True,
                                             disable_bounds_checks=bool(int(os.environ.get('NOBC', '0')))),
    )(A_q, A_k, A_v, A_shift_k.T, A_ssm_k, A_ssm_D, B_w1, B_w2, B_w3.T, B_w4, c, w_mod)
```

```python
import math
import os

import jax
import jax.numpy as jnp
from jax import lax
import jax.experimental.pallas as pl
import jax.experimental.pallas.tpu as pltpu

S, D, F = 2048, 640, 1728
C = 128
NC = S // C
NT = D // 128
NG = 16
KOFF = (NC + 1) * NG * 3
W = int(os.environ.get('W', '4'))
SKIPA = int(os.environ.get('SKIPA', '0'))
WMA, WMP, WMC = 1280, 640, 640
Q0 = int(os.environ.get('Q0', '384'))
N2 = int(os.environ.get('N2', '4'))
PRELN = int(os.environ.get('PRELN', '2'))
NOCACHE = int(os.environ.get('NOCACHE', '0'))
OUTWAIT = int(os.environ.get('OUTWAIT', '0'))
SEGS = [int(x) for x in os.environ.get('SEGS', '012345')]
SKIPB = int(os.environ.get('SKIPB', '0'))
PADK = int(os.environ.get('PADK', '0'))
PREW = int(os.environ.get('PREW', '0'))
SP = float(os.environ.get('SP', '0'))
MINS = int(os.environ.get('MINS', '30'))
GA = int(os.environ.get('GA', '2'))
TRT = int(os.environ.get('TRT', '1'))
LP = int(os.environ.get('LP', '1'))
FA = 1664
LPN = int(os.environ.get('LPN', '2'))
G0 = int(os.environ.get('G0', '4'))
Q1 = int(os.environ.get('Q1', '1408'))
TIE4 = int(os.environ.get('TIE4', '12'))
STAG = os.environ.get('STAG', 'w02,l0,n,n')
KARA = int(os.environ.get('KARA', '1'))
UNR = int(os.environ.get('UNR', '2'))
HEAD = int(os.environ.get('HEAD', '250'))
TAIL = int(os.environ.get('TAIL', '450'))
DORDER = os.environ.get('DORDER', 'HaUb')
R1 = int(os.environ.get('R1', '64'))
R2 = int(os.environ.get('R2', '128'))
LEAD = int(os.environ.get('LEAD', '4'))
TS = int(os.environ.get('TS', '256'))
ONEPASS = int(os.environ.get('ONEPASS', '1'))
RSQ = int(os.environ.get('RSQ', '1'))
T2 = int(os.environ.get('T2', '512'))
EPS = 1e-5
_C0 = math.sqrt(2.0 / math.pi)
ALPHA = (_C0 * 0.044715) ** (1.0 / 3.0)
GC = _C0 / ALPHA
BETA = 0.5 / ALPHA
_fc = [int(x) for x in os.environ.get('FC', '1728').split(',')]
F_CHUNKS = tuple((sum(_fc[:i]), _fc[i]) for i in range(len(_fc)))
assert sum(_fc) == F

f32 = jnp.float32
bf16 = jnp.bfloat16
u32 = jnp.uint32
NTDIMS = (((1,), (1,)), ((), ()))


def _cos_table(m, scale):
    mm = jnp.abs(((m + 256) & 511) - 256)
    x = (128 - mm).astype(f32) * (1.0 / 128.0)
    x2 = x * x
    h = math.pi / 2
    p = -(h ** 7) / 5040 + x2 * ((h ** 9) / 362880 - x2 * (h ** 11) / 39916800)
    p = h + x2 * (-(h ** 3) / 6 + x2 * ((h ** 5) / 120 + x2 * p))
    return (x * scale) * p


def _dft_tables():
    shape = (16, 8, 128)
    n = lax.broadcasted_iota(jnp.int32, shape, 0)
    s = lax.broadcasted_iota(jnp.int32, shape, 1)
    l = lax.broadcasted_iota(jnp.int32, shape, 2)
    fw, fu, iv = [], [], []
    wv = l >> 4
    tu = (16 * W) * (wv // W) + (2 * W) * ((l >> 1) & 7) + 2 * (wv % W) + (l & 1)
    for e in range(2):
        r = 2 * s + e
        j = 8 * n + (r & 7)
        fw.append(_cos_table((4 * j + 1) * l + (r >> 3) * 128, 1.0))
        fu.append(_cos_table((4 * j + 1) * tu + (r >> 3) * 128, 1.0))
        b = 16 * (n >> 1) + r
        col = 128 * (n & 1) + l
        iv.append(_cos_table((4 * (col >> 1) + 1) * b + (col & 1) * 128, 1.0 / 128.0))
    pk = lambda xs: pltpu.bitcast(pltpu.pack_elementwise(xs, packed_dtype=bf16), f32)
    return pk(fw), pk(iv), pk(fu)


def _gelu2a(z):
    return z * (1.0 + jnp.tanh(z * (z * z + GC)))


def _rstd(ssd, scale):
    if RSQ == 0:
        r = lax.rsqrt(ssd * (1.0 / D) + EPS)
        return r if scale == 1.0 else r * scale
    return jnp.exp2(jnp.log(ssd + D * EPS) * (-0.5 / math.log(2.0)) + math.log2(scale * math.sqrt(D)))


def _center(x, scale=1.0):
    s1 = jnp.sum(x, axis=-1, keepdims=True)
    m = s1 * (1.0 / D)
    d = x - m
    if ONEPASS:
        ssd = jnp.maximum(jnp.sum(x * x, axis=-1, keepdims=True) - s1 * m, 0.0)
    else:
        ssd = jnp.sum(d * d, axis=-1, keepdims=True)
    return d, _rstd(ssd, scale)


def _conv(us, gs, a):
    acc = None
    for c in range(a + 1):
        p = us[c] * gs[a - c]
        acc = p if acc is None else acc + p
    return acc


def _mult(x, n):
    return x if isinstance(x, int) else pl.multiple_of(x, n)


def _wt(ref, *idx):
    return pltpu.bitcast(ref[idx] if idx else ref[...], bf16)


def _kernel(q_hbm, k_hbm, v_hbm, sk_hbm, h_hbm, dd_hbm, w1_hbm, w2_hbm, w3_hbm, w4_hbm,
            c_hbm, wm_hbm, o_hbm,
            modb, qbuf, kbuf, vbuf, hbuf, w1, w2, w3, w4, wm, wmp, wmc, obuf,
            ub0, ub1, gb0, gb1, kb0, kb1, yb, xn, hh, h1, par, l4p, sk_s, dd_s, c_s, zs, sems, osems):
    ubs, gbs, kbs = (ub0, ub1), (gb0, gb1), (kb0, kb1)
    cp = pltpu.make_async_copy
    HS = S // 2

    def cp_h(j, c0, c1, sem):
        return cp(h_hbm.at[pl.ds(j * 128, 128), pl.ds(c0, c1 - c0)], hbuf.bitcast(bf16).at[j, :, pl.ds(c0, c1 - c0)], sem)

    def cp_kv(j, r0, r1, sem):
        r0, r1 = (r0 + 16 if r0 else 0), min(r1 + 16, S)
        lanes = pl.ds(j * 128, 128)
        return [cp(k_hbm.at[0, pl.ds(r0, r1 - r0), lanes], kbuf.bitcast(bf16).at[j, pl.ds(r0 + 16, r1 - r0), :], sem),
                cp(v_hbm.at[0, pl.ds(r0, r1 - r0), lanes], vbuf.bitcast(bf16).at[j, pl.ds(r0, r1 - r0), :], sem)]

    def cp_tile(j, i):
        sem = sems.at[2 * j + i]
        return [cp_h(j, i * HS, (i + 1) * HS, sem)] + cp_kv(j, i * HS, (i + 1) * HS, sem)

    cp_t0 = [[cp_h(0, 0, S, sems.at[0])], cp_kv(0, 0, 1024, sems.at[1]), cp_kv(0, 1024, 1536, sems.at[20]),
             cp_kv(0, 1536, S, sems.at[21])]

    def cp_wm(i):
        return cp(wm_hbm.at[:, pl.ds(i * WMA, WMA)], wm.bitcast(bf16).at[i], sems.at[10 + i])

    cp_wmp = cp(wm_hbm.at[:, pl.ds(2 * WMA, WMP)], wmp.bitcast(bf16), sems.at[13])
    cp_wmc = cp(wm_hbm.at[:, pl.ds(2 * WMA + WMP, WMC)], wmc.bitcast(bf16), sems.at[12])
    cp_q = [cp(q_hbm.at[0, pl.ds(r0, r1 - r0), :], qbuf.at[pl.ds(r0, r1 - r0), :], sems.at[sm])
            for sm, r0, r1 in ((13, 0, Q0), (14, Q0, Q1), (12, Q1, S))]
    cp_w = [cp(s_, d_.bitcast(bf16), sems.at[sm])
            for sm, s_, d_ in ((15, w1_hbm, w1), (16, w2_hbm, w2), (12, w3_hbm, w3), (12, w4_hbm, w4))]
    cp_s = [cp(sk_hbm, sk_s, sems.at[19]), cp(dd_hbm, dd_s, sems.at[19]), cp(c_hbm, c_s, sems.at[19])]
    order = list(cp_s)
    for grp in cp_t0:
        order += grp
    for j in range(1, NT):
        order += cp_tile(j, 0) + cp_tile(j, 1)
    order += [cp_wm(0), cp_wm(1), cp_wmp, cp_q[0], cp_w[0], cp_w[1], cp_q[1], cp_q[2], cp_wmc, cp_w[2], cp_w[3]]
    for c_ in order:
        c_.start()

    with jax.named_scope("init"):
        fw_t, iv_t, fu_t = _dft_tables()
        for kb in kbs:
            kb[pl.ds(KOFF, 16)] = fw_t
            kb[pl.ds(KOFF + 16, 16)] = iv_t
            kb[pl.ds(KOFF + 32, 16)] = fu_t
            kb[pl.ds(0, NG * 3)] = jnp.zeros((NG * 3, 8, 128), f32)
        zeros = jnp.zeros((8, 128), f32)
        for j in range(NT):
            kbuf[j, pl.ds(0, 8), :] = jnp.zeros((8, 128), u32)
            kbuf[j, pl.ds(8 + HS, 8), :] = jnp.zeros((8, 128), u32)
            vbuf[j, pl.ds(HS, 8), :] = jnp.zeros((8, 128), u32)
        for j in range(NT):
            h1[j, pl.ds(0, 8), :] = zeros
            h1[j, pl.ds(S + 8, 8), :] = zeros
        for c_ in cp_s:
            c_.wait()
        par[pl.ds(0, 4), :] = sk_s[...].astype(f32)
        par[pl.ds(8, 8), :] = jnp.broadcast_to(dd_s[...].astype(f32).reshape(1, D), (8, D))
        cv = c_s[...].astype(f32)
        sc = jnp.broadcast_to(cv * jax.nn.sigmoid(cv), (8, D))
        scp = pltpu.bitcast(pltpu.pack_elementwise([sc, sc], packed_dtype=bf16), f32)
        for j in range(NT):
            kb0[KOFF + 48 + j] = scp[:, 128 * j:128 * (j + 1)]
            kb1[KOFF + 48 + j] = scp[:, 128 * j:128 * (j + 1)]

    def mkb(i, unr, off, cache):
        def b(stride, extra=0, z=None):
            if isinstance(i, int):
                return (i * unr + off) * stride + extra
            key = (unr * stride, z)
            if key not in cache or NOCACHE:
                base = pl.multiple_of(i * (unr * stride), unr * stride)
                cache[key] = base if z is None else base + (i >> z)
            return cache[key] + (off * stride + extra)
        return b

    def dot_h(j, b, lhs):
        gb = gbs[j % 2]
        hc = hbuf[j, :, pl.ds(_mult(b(512), 512), 512)]
        rhs_t = jnp.concatenate([hc[:, C * cc:C * (cc + 1)] for cc in range(4)], axis=0)
        g = lax.dot_general(lhs, pltpu.bitcast(rhs_t, bf16), NTDIMS, preferred_element_type=f32)
        for rg in range(2 * NG):
            for cc in range(4):
                gb[b(4, cc + rg * NC)] = g[8 * rg:8 * rg + 8, 128 * cc:128 * cc + 128]

    def dot_u(j, b, lhs):
        ub = ubs[j % 2]
        taps = [par[pl.ds(t, 1), pl.ds(j * 128, 128)] for t in range(4)]
        unp = lambda w_, e: pltpu.unpack_elementwise(w_, index=e, packed_dtype=bf16, unpacked_dtype=f32)
        cols = []
        for cc in range(4):
            words = []
            for blk in range(8 // W):
                w0 = 64 * cc + 8 * W * blk
                kw = {m: kbuf[j, pl.ds(b(256, 8 + w0 + m), 8, stride=W), :] for m in range(-2, W)}
                kk = {2 * m + e: unp(kw[m], e) for m in range(-2, W) for e in range(2) if 2 * m + e >= -3}
                for m in range(W):
                    vw = vbuf[j, pl.ds(b(256, w0 + m), 8, stride=W), :]
                    pair = []
                    for e in range(2):
                        n = 2 * m + e
                        ks = kk[n] * taps[0] + kk[n - 1] * taps[1] + kk[n - 2] * taps[2] + kk[n - 3] * taps[3]
                        pair.append(ks * unp(vw, e))
                    words.append(pltpu.pack_elementwise(pair, packed_dtype=bf16))
            cols.append(jnp.concatenate(words, axis=0))
        rhs = pltpu.bitcast(jnp.concatenate(cols, axis=1), bf16)
        u = jnp.dot(lhs, rhs, preferred_element_type=f32)
        for rg in range(2 * NG):
            for cc in range(4):
                ub[b(4, cc + rg * NC)] = u[8 * rg:8 * rg + 8, 128 * cc:128 * cc + 128]

    def dot_i(j, b, half, lhs):
        kb = kbs[j % 2]
        cols = [[], []]
        for gi in range(NG):
            prev = None
            for cc in range(-1, 2):
                k0, k1, k2 = [kb[b(4 * NG * 3, ((2 * half + cc + 1) * NG + gi) * 3 + t)] for t in range(3)]
                re, im = k0 - k2, k0 + k1
                if prev is not None:
                    cols[cc].append(pltpu.pack_elementwise([re - prev[1], im + prev[0]], packed_dtype=bf16))
                prev = (re, im)
        rhs = jnp.concatenate([jnp.concatenate(c_, axis=0) for c_ in cols], axis=1)
        y = jnp.dot(lhs, pltpu.bitcast(rhs, bf16), preferred_element_type=f32)
        for cc in range(2):
            yb[j, pl.ds(b(512, (2 * half + cc) * C), C), :] = y[:, 128 * cc:128 * cc + 128]

    def gen_m(j, kb, b, ng):
        ub, gb = ubs[j % 2], gbs[j % 2]
        for s in range(ng):
            for t in range(3):
                z = 8 + t
                re = lambda ref, c: ref[b(2 * NC, 2 * s * NC + c, z)]
                im = lambda ref, c: ref[b(2 * NC, (2 * s + 1) * NC + c, z)]
                gre = [re(gb, c) for c in range(NC)]
                if t == 0:
                    us = [re(ub, c) + im(ub, c) for c in range(NC)]
                    gs = gre
                elif t == 1:
                    us = [re(ub, c) for c in range(NC)]
                    gs = [im(gb, c) - gre[c] for c in range(NC)]
                else:
                    us = [im(ub, c) for c in range(NC)]
                    gs = [im(gb, c) + gre[c] for c in range(NC)]

                def st(a, val):
                    kb[b(3, ((a + 1) * NG + s) * 3 + t)] = val
                if not KARA:
                    for a in range(NC):
                        st(a, _conv(us, gs, a))
                        yield 2 * a + 2
                    continue
                ue, uo, ge, go = us[0::2], us[1::2], gs[0::2], gs[1::2]
                usum = [x + y for x, y in zip(ue, uo)]
                gsum = [x + y for x, y in zip(ge, go)]
                poo_prev = None
                for a in range(NC // 2):
                    pee = _conv(ue, ge, a)
                    poo = _conv(uo, go, a)
                    pss = _conv(usum, gsum, a)
                    st(2 * a, pee if poo_prev is None else pee + poo_prev)
                    st(2 * a + 1, pss - pee - poo)
                    poo_prev = poo
                    yield 3 * (2 * a + 1) + 7

    def add_d(j):
        gb = gbs[j % 2]
        dvec = par[pl.ds(8, 8), pl.ds(j * 128, 128)]
        for gi in range(NG):
            gb[2 * gi * NC] = gb[2 * gi * NC] + dvec

    def sc_lhs():
        return pltpu.bitcast(jnp.concatenate([kb0[KOFF + 48 + j] for j in range(NT)], axis=1), bf16)

    def dot_m(i, t0, nt, rows):
        m = None
        for kt in range(NT):
            p = jnp.dot(pltpu.bitcast(rows[kt], bf16), _wt(wm, i, pl.ds(64 * kt, 64), pl.ds(128 * t0, 128 * nt)),
                        preferred_element_type=f32)
            m = p if m is None else m + p
        for t in range(nt):
            modb[i * (WMA // 128) + (t0 + t)] = m[0:8, 128 * t:128 * (t + 1)]

    def inv_lhs(tbl, n):
        return jnp.concatenate([tbl[KOFF + 16 + 2 * n], tbl[KOFF + 17 + 2 * n]], axis=1)

    def dot_k(kb, kt, bt, lhs):
        cols = [[] for _ in range(4)]
        for gi in range(8 * kt, 8 * kt + 8):
            prev = None
            for cc in range(-1, 4):
                k0, k1, k2 = [kb[((4 * bt + cc + 1) * NG + gi) * 3 + t] for t in range(3)]
                re, im = k0 - k2, k0 + k1
                if prev is not None:
                    cols[cc].append(pltpu.pack_elementwise([re - prev[1], im + prev[0]], packed_dtype=bf16))
                prev = (re, im)
        rhs = jnp.concatenate([jnp.concatenate(c_, axis=0) for c_ in cols], axis=1)
        y = jnp.dot(lhs, pltpu.bitcast(rhs, bf16), preferred_element_type=f32)
        for cc in range(4):
            rows = pl.ds((4 * bt + cc) * C, C)
            yc = y[:, 128 * cc:128 * cc + 128]
            yb[NT - 1, rows, :] = yc if kt == 0 else yb[NT - 1, rows, :] + yc

    PRE = dict(H=0, U=672 + 96 // W, a=192, b=192, m=0, k=176)
    POST = dict(H=0, U=0, a=4, b=4, m=2, k=0)
    NST = dict(H=16, U=16, a=8, b=8, m=5, k=8)
    GCOST = 3 * (248 if KARA else 272)

    def a_block(dots, mg=None, ng=0, tbl=kb0):
        native, dur = [], []
        for idx, (k_, _) in enumerate(dots):
            nxt = PRE[dots[idx + 1][0]] if idx + 1 < len(dots) else 0
            d_ = 2.0 if k_ == 'm' else 1.0
            native += [nxt / NST[k_] + POST[k_] * d_] * NST[k_]
            dur += [d_] * NST[k_]
        if mg is not None and dots:
            head = max(HEAD - PRE[dots[0][0]], 0)
            mtot = GCOST * ng - TAIL - head
            lvl = (mtot + sum(native)) / sum(dur)
            want = [max(lvl * d_ - x, 0.0) for x, d_ in zip(native, dur)]
            scale = mtot / sum(want)
            cum, tgt = [head], head
            for w_ in want:
                tgt += w_ * scale
                cum.append(tgt)
        done = 0.0
        step = 0
        for (k_, fn) in dots:
            rows = []
            for n in range(NST[k_]):
                if mg is not None:
                    while done < cum[step]:
                        done += next(mg)
                step += 1
                if k_ in 'HU':
                    rows.append(tbl[KOFF + n + (32 if k_ == 'U' else 0)])
                elif k_ in 'ab':
                    rows.append(inv_lhs(tbl, n))
                elif k_ == 'k':
                    rows.append(tbl[KOFF + 16 + 2 * n])
                else:
                    rows.append(tbl[KOFF + 48 + n])
            fn(rows if k_ == 'm' else pltpu.bitcast(jnp.concatenate(rows, axis=0), bf16))
        if mg is not None:
            for _ in mg:
                pass

    def fdot(k_, j, b):
        if k_ == 'H':
            return (k_, lambda lhs: dot_h(j, b, lhs))
        if k_ == 'U':
            return (k_, lambda lhs: dot_u(j, b, lhs))
        return (k_, lambda lhs: dot_i(j, b, 0 if k_ == 'a' else 1, lhs))

    def wait_all(cps):
        for c_ in cps:
            c_.wait()

    def a_loop(jf, jm, ji, g0, ng):
        kinds = [k_ for k_ in DORDER if k_ in 'HU' or ji is not None]

        def body(i, carry):
            cache = {}
            zs[i] = 0
            dots = [fdot(k_, jf if k_ in 'HU' else ji, mkb(i, 2, s_, cache)) for s_ in range(2) for k_ in kinds]
            a_block(dots, gen_m(jm, kbs[jm % 2], mkb(i, ng, g0, cache), ng), ng, kbs[jm % 2])

            @pl.when(i == 0)
            def _():
                wait_all(cp_tile(jf, 1))
            return carry
        wait_all(cp_tile(jf, 0))
        lax.fori_loop(0, 2, body, 0)
        add_d(jf)

    sb_ = lambda bt: mkb(0, 1, bt, None)
    if SKIPA:
        a_block = lambda *a, **k: None
    with jax.named_scope("A_seg0"):
        wait_all(cp_t0[0])
        a_block([fdot('H', 0, sb_(bt)) for bt in range(4)])
        add_d(0)
        wait_all(cp_t0[1])
        a_block([fdot('U', 0, sb_(bt)) for bt in range(2)])
        for bt in (2, 3):
            wait_all(cp_t0[bt])
            a_block([fdot('U', 0, sb_(bt))])
    with jax.named_scope("A_m0"):
        def body_m0(i, carry):
            a_block([], gen_m(0, kb0, mkb(i, G0 // 2, 0, {}), G0 // 2))
            return carry
        if G0:
            lax.fori_loop(0, 2, body_m0, 0)
    for seg in range(1, NT):
        with jax.named_scope(f"A_seg{seg}"):
            if seg == 1:
                a_loop(1, 0, None, G0, (NG - G0) // 2)
            else:
                a_loop(seg, seg - 1, seg - 2, 0, 8)

    def mods(i):
        return [('m', lambda rows, t0=t0, nt=nt: dot_m(i, t0, nt, rows)) for (t0, nt) in ((0, 4), (4, 4), (8, 2))]

    with jax.named_scope("A_seg5a"):
        cp_wm(0).wait()
        zz = zs[1]

        @pl.when(zz == 0)
        def _():
            dots = [fdot(k_, NT - 2, sb_(bt)) for bt in range(4) for k_ in 'ab']
            mm = mods(0)
            dots = [mm[0]] + dots[0:2] + [mm[1]] + dots[2:4] + [mm[2]] + dots[4:]
            a_block(dots, gen_m(NT - 1, kb0, mkb(zz, 8, 0, {}), 8), 8, kb0)
    with jax.named_scope("A_seg5b"):
        cp_wm(1).wait()

        @pl.when(zz == 0)
        def _():
            dots = [('k', lambda lhs, bt=bt: dot_k(kb0, 0, bt, lhs)) for bt in range(4)]
            mm = mods(1)
            dots = [mm[0], dots[0], mm[1], dots[1], mm[2]] + dots[2:]
            a_block(dots, gen_m(NT - 1, kb1, mkb(zz, 8, 8, {}), 8), 8, kb1)

    def inv_last(bt):
        lhs = pltpu.bitcast(jnp.concatenate([kb0[KOFF + 17 + 2 * n] for n in range(8)], axis=0), bf16)
        dot_k(kb1, 1, bt, lhs)

    def modrow(k_):
        return jnp.concatenate([modb[NT * k_ + j] for j in range(NT)], axis=1)

    R = R1
    GP = R // 8

    def ln_chain(p):
        r = p * R
        pa, pb, pc, ps = [par[pl.ds(16 + 8 * t, 8), :][None] for t in range(4)]
        g3 = lambda x: x.reshape(GP, 8, D)
        q = g3(qbuf[pl.ds(r, R), :].astype(f32))
        d1, r1 = _center(q)
        y = g3(jnp.concatenate([yb[j, pl.ds(r, R), :] for j in range(NT)], axis=1))
        x = q + ((d1 * r1) * pa + pb) * y
        xn[pl.ds(r, R), :] = x.reshape(R, D)
        d2, r2 = _center(x)
        h = (d2 * r2) * pc + ps
        hh[pl.ds(r, R), :] = h.reshape(R, D)
        d3, r3 = _center(h, ALPHA)
        return (d3 * r3).reshape(R, D)

    def tie(w_, vs):
        t_ = pltpu.bitcast(vs[0], u32)
        for v_ in vs[1:]:
            t_ = t_ | pltpu.bitcast(v_, u32)
        return w_ | (t_ & kbuf[0, pl.ds(0, 8), :])

    def tied(wref, ties):
        if not ties:
            return _wt(wref)
        rbs = sorted({8 * (t % 5) + rb for (t, rb) in ties})
        rows, pos = [], 0
        for rb in rbs:
            if rb > pos:
                rows.append(wref[pl.ds(8 * pos, 8 * (rb - pos)), :])
            blk = []
            for n in range(NT):
                w_ = wref[pl.ds(8 * rb, 8), pl.ds(128 * n, 128)]
                vs = ties.get((5 * n + rb // 8, rb % 8))
                blk.append(tie(w_, vs) if vs else w_)
            rows.append(jnp.concatenate(blk, axis=1))
            pos = rb + 1
        if pos < 40:
            rows.append(wref[pl.ds(8 * pos, 8 * (40 - pos)), :])
        return pltpu.bitcast(jnp.concatenate(rows, axis=0), bf16)

    def w1_dot(p, l3, ties, fresh):
        if fresh and STAG:
            grp = lambda g: l3[8 * g:8 * g + 8, 0:128]
            lt = {}
            for pr, spec in enumerate(STAG.split(',')):
                vs = [grp(2 * pr), grp(2 * pr + 1)]
                if spec[0] == 'w':
                    ties.setdefault((int(spec[1]), int(spec[2])), []).extend(vs)
                elif spec[0] == 'l':
                    lt.setdefault(int(spec[1]), []).extend(vs)
            for pr, vs in lt.items():
                x = pltpu.bitcast(tie(pltpu.bitcast(l3[16 * pr:16 * pr + 8, 128:256], u32), vs), f32)
                mid = jnp.concatenate([l3[16 * pr:16 * pr + 8, 0:128], x, l3[16 * pr:16 * pr + 8, 256:]], axis=1)
                l3 = jnp.concatenate(([l3[:16 * pr]] if pr else []) + [mid, l3[16 * pr + 8:]], axis=0)
        z = jnp.dot(l3.astype(bf16), tied(w1, ties), preferred_element_type=f32)
        g = _gelu2a(z)
        for j in range(NT):
            h1[j, pl.ds(p * R + 8, R), :] = g[:, j * 128:(j + 1) * 128]

    def w2_dot(p, ties):
        r = p * R
        lane = lax.broadcasted_iota(jnp.int32, (R, 128), 1)

        def ld(j, off):
            return h1[j, pl.ds(r + 8 + off, R), :]
        tiles = [
            ld(0, -1),
            jnp.where(lane < 32, ld(1, -1), ld(1, 1)),
            jnp.where(lane < 64, ld(2, 1), ld(2, -2)),
            jnp.where(lane < 96, ld(3, -2), ld(3, 2)),
            ld(4, 2),
        ]
        hs = jnp.concatenate(tiles, axis=1).astype(bf16)
        x1 = hh[pl.ds(r, R), :] + jnp.dot(hs, tied(w2, ties), preferred_element_type=f32) * BETA
        hh[pl.ds(r, R), :] = x1

    l3s = {}

    def ln4(r, n):
        d4, r4 = _center(hh[pl.ds(r, n), :], ALPHA)
        return d4 * r4

    def run_block(dots, pre4=False):
        for d_, (k_, p) in enumerate(dots):
            ties = {}
            e = d_ - (len(dots) - TS // R)
            if pre4 and e >= 0:
                nx = ln4(e * R, R)
                l4p[pl.ds(e * R // 2, R // 2), :] = pltpu.bitcast(nx.astype(bf16), u32)
                ties[(TIE4, 7)] = [nx[8 * g:8 * g + 8, 0:128] for g in range(GP)]
            if k_ == 1:
                fresh = p not in l3s
                w1_dot(p, ln_chain(p) if fresh else l3s.pop(p), ties, fresh)
            elif k_ == 2:
                w2_dot(p, ties)
            else:
                par[pl.ds(48, 8), :] = jnp.dot(sc_lhs(), _wt(wmc), preferred_element_type=f32)[0:8]

    with jax.named_scope("P1"):
        cp_wmp.wait()
        cp_q[0].wait()
        mp = jnp.dot(sc_lhs(), _wt(wmp), preferred_element_type=f32)
        for t in range(WMP // 128):
            modb[2 * WMA // 128 + t] = mp[0:8, 128 * t:128 * (t + 1)]
        sa, ca, ga, sb, cb = [modrow(k_) for k_ in range(5)]
        par[pl.ds(16, 8), :] = ga * (1.0 + ca)
        par[pl.ds(24, 8), :] = ga * sa
        par[pl.ds(32, 8), :] = 1.0 + cb
        par[pl.ds(40, 8), :] = sb
        for bt in range(4):
            inv_last(bt)
        for p in range(PRELN):
            l3s[p] = ln_chain(p)
    with jax.named_scope("w1wait"):
        cp_w[0].wait()
    p1, p2 = N2, 0
    with jax.named_scope("P2"):
        run_block([(1, p) for p in range(N2)])
    with jax.named_scope("w2wait"):
        cp_w[1].wait()

    def plan(lim1, hold):
        nonlocal p1, p2
        dots = []
        while p2 < p1 - 1 and len(dots) < 2:
            dots.append((2, p2))
            p2 += 1
        last2 = lim1 if lim1 == S // R else lim1 - 1 - hold
        while p2 < last2 or p1 < lim1:
            while p1 < lim1 and (p1 - p2 < LEAD or p2 >= last2):
                dots.append((1, p1))
                p1 += 1
            if p2 < last2:
                dots.append((2, p2))
                p2 += 1
        return dots

    with jax.named_scope("P3"):
        run_block(plan(Q0 // R, 2))
    with jax.named_scope("q1wait"):
        cp_q[1].wait()
    with jax.named_scope("P4"):
        run_block(plan(Q1 // R, 2))
    with jax.named_scope("q2wait"):
        wait_all([cp_q[2], cp_wmc, cp_w[2], cp_w[3]])
    with jax.named_scope("P5"):
        dots = plan(S // R, 0)
        run_block(dots[:2] + [(3, 0)] + dots[2:], pre4=True)

    def out_copy(r):
        return cp(obuf.at[pl.ds(r, TS), :], o_hbm.at[0, pl.ds(r, TS), :], osems.at[0])

    def b2_step(i):
        gbv = par[pl.ds(48, 1), :]
        nsub = T2 // TS
        for sub in range(nsub):
            r = pl.multiple_of(pl.multiple_of(i * T2, T2) + sub * TS, TS)
            l4 = _wt(l4p, pl.ds(0, TS // 2), slice(None)) if (sub == 0 and LP) else ln4(r, TS).astype(bf16)
            z = lax.dot_general(l4, _wt(w3, pl.ds(0, FA // 2), slice(None)), NTDIMS, preferred_element_type=f32)
            zt = lax.dot_general(_wt(w3, pl.ds(FA // 2, (F - FA) // 2), slice(None)), l4, NTDIMS,
                                 preferred_element_type=f32)
            g = jnp.concatenate([_gelu2a(z), _gelu2a(zt).T], axis=1).astype(bf16)
            if sub == nsub - 1 and LP:
                nx = ln4(pl.multiple_of(jnp.minimum(i + 1, S // T2 - 1) * T2, T2), TS)
                l4p[pl.ds(0, TS // 2), :] = pltpu.bitcast(nx.astype(bf16), u32)
                t_ = pltpu.bitcast(nx[0:8, 0:128], u32)
                for gi in range(1, TS // 8):
                    t_ = t_ | pltpu.bitcast(nx[8 * gi:8 * gi + 8, 0:128], u32)
                top = [w4[pl.ds(0, 8), pl.ds(128 * n, 128)] for n in range(NT)]
                top[LPN] = top[LPN] | (t_ & kbuf[0, pl.ds(0, 8), :])
                w4v = jnp.concatenate([jnp.concatenate(top, axis=1), w4[pl.ds(8, F // 2 - 8), :]], axis=0)
            else:
                w4v = w4[...]
            acc = jnp.dot(g, pltpu.bitcast(w4v, bf16), preferred_element_type=f32)
            obuf[pl.ds(r, TS), :] = (xn[pl.ds(r, TS), :] + gbv * (hh[pl.ds(r, TS), :] + BETA * acc)).astype(bf16)
            out_copy(r).start()

    with jax.named_scope("BII"):
        lax.fori_loop(0, S // T2, lambda i, c: (b2_step(i), c)[1], 0)
    with jax.named_scope("out_wait"):
        for i in range(S // TS):
            out_copy(i * TS).wait()


@jax.jit
def pallas_adaLN_cond__ssm_conv_h3__mixer_s_mlp__prompt_kernel(
    A_q, A_k, A_v, A_shift_k, A_ssm_k, A_ssm_D, B_x, B_w1, B_w2, B_w3, B_w4, c, w_mod,
):
    del B_x
    hbm = pl.BlockSpec(memory_space=pltpu.MemorySpace.HBM)
    return pl.pallas_call(
        _kernel,
        out_shape=jax.ShapeDtypeStruct((1, S, D), bf16),
        in_specs=[hbm] * 12,
        out_specs=hbm,
        scratch_shapes=[
            pltpu.VMEM((27, 8, 128), f32),
            pltpu.VMEM((S + 16 * int(os.environ.get('PADF', '0')), D), bf16),
            pltpu.VMEM((NT, 32 + S // 2, 128), u32),
            pltpu.VMEM((NT, 32 + S // 2, 128), u32),
            pltpu.VMEM((NT, 64, S), u32),
            pltpu.VMEM((D // 2, D), u32),
            pltpu.VMEM((D // 2, D), u32),
            pltpu.VMEM((F // 2, D), u32),
            pltpu.VMEM((F // 2, D), u32),
            pltpu.VMEM((2, D // 2, WMA), u32),
            pltpu.VMEM((D // 2, WMP), u32),
            pltpu.VMEM((D // 2, WMC), u32),
            pltpu.VMEM((S, D), bf16),
            pltpu.VMEM((NG * 2 * NC, 8, 128), f32),
            pltpu.VMEM((NG * 2 * NC, 8, 128), f32),
            pltpu.VMEM((NG * 2 * NC, 8, 128), f32),
            pltpu.VMEM((NG * 2 * NC, 8, 128), f32),
            pltpu.VMEM((KOFF + 56 + PADK, 8, 128), f32),
            pltpu.VMEM((KOFF + 56 + PADK, 8, 128), f32),
            pltpu.VMEM((NT, S, 128), f32),
            pltpu.VMEM((S, D), f32),
            pltpu.VMEM((S, D), f32),
            pltpu.VMEM((NT, S + 32, 128), f32),
            pltpu.VMEM((64, D), f32),
            pltpu.VMEM((TS // 2 + 8 * int(os.environ.get('PADE', '0')), D), u32),
            pltpu.VMEM((4, D), bf16),
            pltpu.VMEM((D,), bf16),
            pltpu.VMEM((1, D), bf16),
            pltpu.SMEM((2,), jnp.int32),
            pltpu.SemaphoreType.DMA((22,)),
            pltpu.SemaphoreType.DMA((1,)),
        ],
        compiler_params=pltpu.CompilerParams(vmem_limit_bytes=100 * 1024 * 1024, disable_semaphore_checks=True,
                                             disable_bounds_checks=bool(int(os.environ.get('NOBC', '0')))),
    )(A_q, A_k, A_v, A_shift_k.T, A_ssm_k, A_ssm_D, B_w1, B_w2, B_w3.T, B_w4, c, w_mod)
```

```python
import math
import os

import jax
import jax.numpy as jnp
from jax import lax
import jax.experimental.pallas as pl
import jax.experimental.pallas.tpu as pltpu

S, D, F = 2048, 640, 1728
C = 128
NC = S // C
NT = D // 128
NG = 16
KOFF = (NC + 1) * NG * 3
W = int(os.environ.get('W', '4'))
SKIPA = int(os.environ.get('SKIPA', '0'))
WMA, WMP, WMC = 1280, 640, 640
Q0 = int(os.environ.get('Q0', '320'))
N2 = int(os.environ.get('N2', '5'))
PRELN = int(os.environ.get('PRELN', '2'))
NOCACHE = int(os.environ.get('NOCACHE', '0'))
OUTWAIT = int(os.environ.get('OUTWAIT', '0'))
SEGS = [int(x) for x in os.environ.get('SEGS', '012345')]
SKIPB = int(os.environ.get('SKIPB', '0'))
PADK = int(os.environ.get('PADK', '0'))
PREW = int(os.environ.get('PREW', '0'))
SP = float(os.environ.get('SP', '0'))
MINS = int(os.environ.get('MINS', '30'))
GA = int(os.environ.get('GA', '2'))
TRT = int(os.environ.get('TRT', '1'))
LP = int(os.environ.get('LP', '1'))
FA = 1664
LPN = int(os.environ.get('LPN', '2'))
G0 = int(os.environ.get('G0', '4'))
Q1 = int(os.environ.get('Q1', '640'))
TIE4 = int(os.environ.get('TIE4', '12'))
STAG = os.environ.get('STAG', 'w02,l0,n,n')
OCOLS = ((0, 512), (512, 128))
KARA = int(os.environ.get('KARA', '1'))
UNR = int(os.environ.get('UNR', '2'))
HEAD = int(os.environ.get('HEAD', '250'))
TAIL = int(os.environ.get('TAIL', '450'))
DORDER = os.environ.get('DORDER', 'HaUb')
R1 = int(os.environ.get('R1', '64'))
R2 = int(os.environ.get('R2', '128'))
LEAD = int(os.environ.get('LEAD', '4'))
TS = int(os.environ.get('TS', '256'))
ONEPASS = int(os.environ.get('ONEPASS', '1'))
RSQ = int(os.environ.get('RSQ', '1'))
T2 = int(os.environ.get('T2', '512'))
EPS = 1e-5
_C0 = math.sqrt(2.0 / math.pi)
ALPHA = (_C0 * 0.044715) ** (1.0 / 3.0)
GC = _C0 / ALPHA
BETA = 0.5 / ALPHA
_fc = [int(x) for x in os.environ.get('FC', '1728').split(',')]
F_CHUNKS = tuple((sum(_fc[:i]), _fc[i]) for i in range(len(_fc)))
assert sum(_fc) == F

f32 = jnp.float32
bf16 = jnp.bfloat16
u32 = jnp.uint32
NTDIMS = (((1,), (1,)), ((), ()))


def _cos_table(m, scale):
    mm = jnp.abs(((m + 256) & 511) - 256)
    x = (128 - mm).astype(f32) * (1.0 / 128.0)
    x2 = x * x
    h = math.pi / 2
    p = -(h ** 7) / 5040 + x2 * ((h ** 9) / 362880 - x2 * (h ** 11) / 39916800)
    p = h + x2 * (-(h ** 3) / 6 + x2 * ((h ** 5) / 120 + x2 * p))
    return (x * scale) * p


def _dft_tables():
    shape = (16, 8, 128)
    n = lax.broadcasted_iota(jnp.int32, shape, 0)
    s = lax.broadcasted_iota(jnp.int32, shape, 1)
    l = lax.broadcasted_iota(jnp.int32, shape, 2)
    fw, fu, iv = [], [], []
    wv = l >> 4
    tu = (16 * W) * (wv // W) + (2 * W) * ((l >> 1) & 7) + 2 * (wv % W) + (l & 1)
    for e in range(2):
        r = 2 * s + e
        j = 8 * n + (r & 7)
        fw.append(_cos_table((4 * j + 1) * l + (r >> 3) * 128, 1.0))
        fu.append(_cos_table((4 * j + 1) * tu + (r >> 3) * 128, 1.0))
        b = 16 * (n >> 1) + r
        col = 128 * (n & 1) + l
        iv.append(_cos_table((4 * (col >> 1) + 1) * b + (col & 1) * 128, 1.0 / 128.0))
    pk = lambda xs: pltpu.bitcast(pltpu.pack_elementwise(xs, packed_dtype=bf16), f32)
    return pk(fw), pk(iv), pk(fu)


def _gelu2a(z):
    return z * (1.0 + jnp.tanh(z * (z * z + GC)))


def _rstd(ssd, scale):
    if RSQ == 0:
        r = lax.rsqrt(ssd * (1.0 / D) + EPS)
        return r if scale == 1.0 else r * scale
    return jnp.exp2(jnp.log(ssd + D * EPS) * (-0.5 / math.log(2.0)) + math.log2(scale * math.sqrt(D)))


def _center(x, scale=1.0):
    s1 = jnp.sum(x, axis=-1, keepdims=True)
    m = s1 * (1.0 / D)
    d = x - m
    if ONEPASS:
        ssd = jnp.maximum(jnp.sum(x * x, axis=-1, keepdims=True) - s1 * m, 0.0)
    else:
        ssd = jnp.sum(d * d, axis=-1, keepdims=True)
    return d, _rstd(ssd, scale)


def _conv(us, gs, a):
    acc = None
    for c in range(a + 1):
        p = us[c] * gs[a - c]
        acc = p if acc is None else acc + p
    return acc


def _mult(x, n):
    return x if isinstance(x, int) else pl.multiple_of(x, n)


def _wt(ref, *idx):
    return pltpu.bitcast(ref[idx] if idx else ref[...], bf16)


def _kernel(q_hbm, k_hbm, v_hbm, sk_hbm, h_hbm, dd_hbm, w1_hbm, w2_hbm, w3_hbm, w4_hbm,
            c_hbm, wm_hbm, o_hbm,
            modb, qbuf, kbuf, vbuf, hbuf, w1, w2, w3, w4, wm, wmp, wmc, obuf,
            ub0, ub1, gb0, gb1, kb0, kb1, yb, xn, hh, h1, par, l4p, sk_s, dd_s, c_s, zs, sems, osems):
    ubs, gbs, kbs = (ub0, ub1), (gb0, gb1), (kb0, kb1)
    cp = pltpu.make_async_copy
    HS = S // 2

    def cp_h(j, c0, c1, sem):
        return cp(h_hbm.at[pl.ds(j * 128, 128), pl.ds(c0, c1 - c0)], hbuf.bitcast(bf16).at[j, :, pl.ds(c0, c1 - c0)], sem)

    def cp_kv(j, r0, r1, sem):
        r0, r1 = (r0 + 16 if r0 else 0), min(r1 + 16, S)
        lanes = pl.ds(j * 128, 128)
        return [cp(k_hbm.at[0, pl.ds(r0, r1 - r0), lanes], kbuf.bitcast(bf16).at[j, pl.ds(r0 + 16, r1 - r0), :], sem),
                cp(v_hbm.at[0, pl.ds(r0, r1 - r0), lanes], vbuf.bitcast(bf16).at[j, pl.ds(r0, r1 - r0), :], sem)]

    def cp_tile(j, i):
        sem = sems.at[2 * j + i]
        return [cp_h(j, i * HS, (i + 1) * HS, sem)] + cp_kv(j, i * HS, (i + 1) * HS, sem)

    cp_t0 = [[cp_h(0, 0, S, sems.at[0])], cp_kv(0, 0, 1024, sems.at[1]), cp_kv(0, 1024, 1536, sems.at[20]),
             cp_kv(0, 1536, S, sems.at[21])]

    def cp_wm(i):
        return cp(wm_hbm.at[:, pl.ds(i * WMA, WMA)], wm.bitcast(bf16).at[i], sems.at[10 + i])

    cp_wmp = cp(wm_hbm.at[:, pl.ds(2 * WMA, WMP)], wmp.bitcast(bf16), sems.at[13])
    cp_wmc = cp(wm_hbm.at[:, pl.ds(2 * WMA + WMP, WMC)], wmc.bitcast(bf16), sems.at[12])
    cp_q = [cp(q_hbm.at[0, pl.ds(r0, r1 - r0), :], qbuf.at[pl.ds(r0, r1 - r0), :], sems.at[sm])
            for sm, r0, r1 in ((13, 0, Q0), (16, Q0, Q1), (12, Q1, S))]
    cp_w = [cp(s_, d_.bitcast(bf16), sems.at[sm])
            for sm, s_, d_ in ((15, w1_hbm, w1), (16, w2_hbm, w2), (14, w3_hbm, w3), (14, w4_hbm, w4))]
    cp_s = [cp(sk_hbm, sk_s, sems.at[19]), cp(dd_hbm, dd_s, sems.at[19]), cp(c_hbm, c_s, sems.at[19])]
    order = list(cp_s)
    for grp in cp_t0:
        order += grp
    for j in range(1, NT):
        order += cp_tile(j, 0) + cp_tile(j, 1)
    order += [cp_wm(0), cp_wm(1), cp_wmp, cp_q[0], cp_w[0], cp_w[1], cp_q[1], cp_q[2], cp_wmc, cp_w[2], cp_w[3]]
    for c_ in order:
        c_.start()

    with jax.named_scope("init"):
        fw_t, iv_t, fu_t = _dft_tables()
        for kb in kbs:
            kb[pl.ds(KOFF, 16)] = fw_t
            kb[pl.ds(KOFF + 16, 16)] = iv_t
            kb[pl.ds(KOFF + 32, 16)] = fu_t
            kb[pl.ds(0, NG * 3)] = jnp.zeros((NG * 3, 8, 128), f32)
        zeros = jnp.zeros((8, 128), f32)
        for j in range(NT):
            kbuf[j, pl.ds(0, 8), :] = jnp.zeros((8, 128), u32)
            kbuf[j, pl.ds(8 + HS, 8), :] = jnp.zeros((8, 128), u32)
            vbuf[j, pl.ds(HS, 8), :] = jnp.zeros((8, 128), u32)
        for j in range(NT):
            h1[j, pl.ds(0, 8), :] = zeros
            h1[j, pl.ds(S + 8, 8), :] = zeros
        for c_ in cp_s:
            c_.wait()
        par[pl.ds(0, 4), :] = sk_s[...].astype(f32)
        par[pl.ds(8, 8), :] = jnp.broadcast_to(dd_s[...].astype(f32).reshape(1, D), (8, D))
        cv = c_s[...].astype(f32)
        sc = jnp.broadcast_to(cv * jax.nn.sigmoid(cv), (8, D))
        scp = pltpu.bitcast(pltpu.pack_elementwise([sc, sc], packed_dtype=bf16), f32)
        for j in range(NT):
            kb0[KOFF + 48 + j] = scp[:, 128 * j:128 * (j + 1)]
            kb1[KOFF + 48 + j] = scp[:, 128 * j:128 * (j + 1)]

    def mkb(i, unr, off, cache):
        def b(stride, extra=0, z=None):
            if isinstance(i, int):
                return (i * unr + off) * stride + extra
            key = (unr * stride, z)
            if key not in cache or NOCACHE:
                base = pl.multiple_of(i * (unr * stride), unr * stride)
                cache[key] = base if z is None else base + (i >> z)
            return cache[key] + (off * stride + extra)
        return b

    def dot_h(j, b, lhs):
        gb = gbs[j % 2]
        hc = hbuf[j, :, pl.ds(_mult(b(512), 512), 512)]
        rhs_t = jnp.concatenate([hc[:, C * cc:C * (cc + 1)] for cc in range(4)], axis=0)
        g = lax.dot_general(lhs, pltpu.bitcast(rhs_t, bf16), NTDIMS, preferred_element_type=f32)
        for rg in range(2 * NG):
            for cc in range(4):
                gb[b(4, cc + rg * NC)] = g[8 * rg:8 * rg + 8, 128 * cc:128 * cc + 128]

    def dot_u(j, b, lhs):
        ub = ubs[j % 2]
        taps = [par[pl.ds(t, 1), pl.ds(j * 128, 128)] for t in range(4)]
        unp = lambda w_, e: pltpu.unpack_elementwise(w_, index=e, packed_dtype=bf16, unpacked_dtype=f32)
        cols = []
        for cc in range(4):
            words = []
            for blk in range(8 // W):
                w0 = 64 * cc + 8 * W * blk
                kw = {m: kbuf[j, pl.ds(b(256, 8 + w0 + m), 8, stride=W), :] for m in range(-2, W)}
                kk = {2 * m + e: unp(kw[m], e) for m in range(-2, W) for e in range(2) if 2 * m + e >= -3}
                for m in range(W):
                    vw = vbuf[j, pl.ds(b(256, w0 + m), 8, stride=W), :]
                    pair = []
                    for e in range(2):
                        n = 2 * m + e
                        ks = kk[n] * taps[0] + kk[n - 1] * taps[1] + kk[n - 2] * taps[2] + kk[n - 3] * taps[3]
                        pair.append(ks * unp(vw, e))
                    words.append(pltpu.pack_elementwise(pair, packed_dtype=bf16))
            cols.append(jnp.concatenate(words, axis=0))
        rhs = pltpu.bitcast(jnp.concatenate(cols, axis=1), bf16)
        u = jnp.dot(lhs, rhs, preferred_element_type=f32)
        for rg in range(2 * NG):
            for cc in range(4):
                ub[b(4, cc + rg * NC)] = u[8 * rg:8 * rg + 8, 128 * cc:128 * cc + 128]

    def dot_i(j, b, half, lhs):
        kb = kbs[j % 2]
        cols = [[], []]
        for gi in range(NG):
            prev = None
            for cc in range(-1, 2):
                k0, k1, k2 = [kb[b(4 * NG * 3, ((2 * half + cc + 1) * NG + gi) * 3 + t)] for t in range(3)]
                re, im = k0 - k2, k0 + k1
                if prev is not None:
                    cols[cc].append(pltpu.pack_elementwise([re - prev[1], im + prev[0]], packed_dtype=bf16))
                prev = (re, im)
        rhs = jnp.concatenate([jnp.concatenate(c_, axis=0) for c_ in cols], axis=1)
        y = jnp.dot(lhs, pltpu.bitcast(rhs, bf16), preferred_element_type=f32)
        for cc in range(2):
            yb[j, pl.ds(b(512, (2 * half + cc) * C), C), :] = y[:, 128 * cc:128 * cc + 128]

    def gen_m(j, kb, b, ng):
        ub, gb = ubs[j % 2], gbs[j % 2]
        for s in range(ng):
            for t in range(3):
                z = 8 + t
                re = lambda ref, c: ref[b(2 * NC, 2 * s * NC + c, z)]
                im = lambda ref, c: ref[b(2 * NC, (2 * s + 1) * NC + c, z)]
                gre = [re(gb, c) for c in range(NC)]
                if t == 0:
                    us = [re(ub, c) + im(ub, c) for c in range(NC)]
                    gs = gre
                elif t == 1:
                    us = [re(ub, c) for c in range(NC)]
                    gs = [im(gb, c) - gre[c] for c in range(NC)]
                else:
                    us = [im(ub, c) for c in range(NC)]
                    gs = [im(gb, c) + gre[c] for c in range(NC)]

                def st(a, val):
                    kb[b(3, ((a + 1) * NG + s) * 3 + t)] = val
                if not KARA:
                    for a in range(NC):
                        st(a, _conv(us, gs, a))
                        yield 2 * a + 2
                    continue
                ue, uo, ge, go = us[0::2], us[1::2], gs[0::2], gs[1::2]
                usum = [x + y for x, y in zip(ue, uo)]
                gsum = [x + y for x, y in zip(ge, go)]
                poo_prev = None
                for a in range(NC // 2):
                    pee = _conv(ue, ge, a)
                    poo = _conv(uo, go, a)
                    pss = _conv(usum, gsum, a)
                    st(2 * a, pee if poo_prev is None else pee + poo_prev)
                    st(2 * a + 1, pss - pee - poo)
                    poo_prev = poo
                    yield 3 * (2 * a + 1) + 7

    def add_d(j):
        gb = gbs[j % 2]
        dvec = par[pl.ds(8, 8), pl.ds(j * 128, 128)]
        for gi in range(NG):
            gb[2 * gi * NC] = gb[2 * gi * NC] + dvec

    def sc_lhs():
        return pltpu.bitcast(jnp.concatenate([kb0[KOFF + 48 + j] for j in range(NT)], axis=1), bf16)

    def dot_m(i, t0, nt, rows):
        m = None
        for kt in range(NT):
            p = jnp.dot(pltpu.bitcast(rows[kt], bf16), _wt(wm, i, pl.ds(64 * kt, 64), pl.ds(128 * t0, 128 * nt)),
                        preferred_element_type=f32)
            m = p if m is None else m + p
        for t in range(nt):
            modb[i * (WMA // 128) + (t0 + t)] = m[0:8, 128 * t:128 * (t + 1)]

    def inv_lhs(tbl, n):
        return jnp.concatenate([tbl[KOFF + 16 + 2 * n], tbl[KOFF + 17 + 2 * n]], axis=1)

    def dot_k(kb, kt, bt, lhs):
        cols = [[] for _ in range(4)]
        for gi in range(8 * kt, 8 * kt + 8):
            prev = None
            for cc in range(-1, 4):
                k0, k1, k2 = [kb[((4 * bt + cc + 1) * NG + gi) * 3 + t] for t in range(3)]
                re, im = k0 - k2, k0 + k1
                if prev is not None:
                    cols[cc].append(pltpu.pack_elementwise([re - prev[1], im + prev[0]], packed_dtype=bf16))
                prev = (re, im)
        rhs = jnp.concatenate([jnp.concatenate(c_, axis=0) for c_ in cols], axis=1)
        y = jnp.dot(lhs, pltpu.bitcast(rhs, bf16), preferred_element_type=f32)
        for cc in range(4):
            rows = pl.ds((4 * bt + cc) * C, C)
            yc = y[:, 128 * cc:128 * cc + 128]
            yb[NT - 1, rows, :] = yc if kt == 0 else yb[NT - 1, rows, :] + yc

    PRE = dict(H=0, U=672 + 96 // W, a=192, b=192, m=0, k=176)
    POST = dict(H=0, U=0, a=4, b=4, m=2, k=0)
    NST = dict(H=16, U=16, a=8, b=8, m=5, k=8)
    GCOST = 3 * (248 if KARA else 272)

    def a_block(dots, mg=None, ng=0, tbl=kb0):
        native, dur = [], []
        for idx, (k_, _) in enumerate(dots):
            nxt = PRE[dots[idx + 1][0]] if idx + 1 < len(dots) else 0
            d_ = 2.0 if k_ == 'm' else 1.0
            native += [nxt / NST[k_] + POST[k_] * d_] * NST[k_]
            dur += [d_] * NST[k_]
        if mg is not None and dots:
            head = max(HEAD - PRE[dots[0][0]], 0)
            mtot = GCOST * ng - TAIL - head
            lvl = (mtot + sum(native)) / sum(dur)
            want = [max(lvl * d_ - x, 0.0) for x, d_ in zip(native, dur)]
            scale = mtot / sum(want)
            cum, tgt = [head], head
            for w_ in want:
                tgt += w_ * scale
                cum.append(tgt)
        done = 0.0
        step = 0
        for (k_, fn) in dots:
            rows = []
            for n in range(NST[k_]):
                if mg is not None:
                    while done < cum[step]:
                        done += next(mg)
                step += 1
                if k_ in 'HU':
                    rows.append(tbl[KOFF + n + (32 if k_ == 'U' else 0)])
                elif k_ in 'ab':
                    rows.append(inv_lhs(tbl, n))
                elif k_ == 'k':
                    rows.append(tbl[KOFF + 16 + 2 * n])
                else:
                    rows.append(tbl[KOFF + 48 + n])
            fn(rows if k_ == 'm' else pltpu.bitcast(jnp.concatenate(rows, axis=0), bf16))
        if mg is not None:
            for _ in mg:
                pass

    def fdot(k_, j, b):
        if k_ == 'H':
            return (k_, lambda lhs: dot_h(j, b, lhs))
        if k_ == 'U':
            return (k_, lambda lhs: dot_u(j, b, lhs))
        return (k_, lambda lhs: dot_i(j, b, 0 if k_ == 'a' else 1, lhs))

    def wait_all(cps):
        for c_ in cps:
            c_.wait()

    def a_loop(jf, jm, ji, g0, ng):
        kinds = [k_ for k_ in DORDER if k_ in 'HU' or ji is not None]

        def body(i, carry):
            cache = {}
            zs[i] = 0
            dots = [fdot(k_, jf if k_ in 'HU' else ji, mkb(i, 2, s_, cache)) for s_ in range(2) for k_ in kinds]
            a_block(dots, gen_m(jm, kbs[jm % 2], mkb(i, ng, g0, cache), ng), ng, kbs[jm % 2])

            @pl.when(i == 0)
            def _():
                wait_all(cp_tile(jf, 1))
            return carry
        wait_all(cp_tile(jf, 0))
        lax.fori_loop(0, 2, body, 0)
        add_d(jf)

    sb_ = lambda bt: mkb(0, 1, bt, None)
    if SKIPA:
        a_block = lambda *a, **k: None
    with jax.named_scope("A_seg0"):
        wait_all(cp_t0[0])
        a_block([fdot('H', 0, sb_(bt)) for bt in range(4)])
        add_d(0)
        wait_all(cp_t0[1])
        a_block([fdot('U', 0, sb_(bt)) for bt in range(2)])
        for bt in (2, 3):
            wait_all(cp_t0[bt])
            a_block([fdot('U', 0, sb_(bt))])
    with jax.named_scope("A_m0"):
        def body_m0(i, carry):
            a_block([], gen_m(0, kb0, mkb(i, G0 // 2, 0, {}), G0 // 2))
            return carry
        if G0:
            lax.fori_loop(0, 2, body_m0, 0)
    for seg in range(1, NT):
        with jax.named_scope(f"A_seg{seg}"):
            if seg == 1:
                a_loop(1, 0, None, G0, (NG - G0) // 2)
            else:
                a_loop(seg, seg - 1, seg - 2, 0, 8)

    def mods(i):
        return [('m', lambda rows, t0=t0, nt=nt: dot_m(i, t0, nt, rows)) for (t0, nt) in ((0, 4), (4, 4), (8, 2))]

    with jax.named_scope("A_seg5a"):
        cp_wm(0).wait()
        zz = zs[1]

        @pl.when(zz == 0)
        def _():
            dots = [fdot(k_, NT - 2, sb_(bt)) for bt in range(4) for k_ in 'ab']
            mm = mods(0)
            dots = [mm[0]] + dots[0:2] + [mm[1]] + dots[2:4] + [mm[2]] + dots[4:]
            a_block(dots, gen_m(NT - 1, kb0, mkb(zz, 8, 0, {}), 8), 8, kb0)
    with jax.named_scope("A_seg5b"):
        cp_wm(1).wait()

        @pl.when(zz == 0)
        def _():
            dots = [('k', lambda lhs, bt=bt: dot_k(kb0, 0, bt, lhs)) for bt in range(4)]
            mm = mods(1)
            dots = [mm[0], dots[0], mm[1], dots[1], mm[2]] + dots[2:]
            a_block(dots, gen_m(NT - 1, kb1, mkb(zz, 8, 8, {}), 8), 8, kb1)

    def inv_last(bt):
        lhs = pltpu.bitcast(jnp.concatenate([kb0[KOFF + 17 + 2 * n] for n in range(8)], axis=0), bf16)
        dot_k(kb1, 1, bt, lhs)

    def modrow(k_):
        return jnp.concatenate([modb[NT * k_ + j] for j in range(NT)], axis=1)

    R = R1
    GP = R // 8

    def ln_chain(p):
        r = p * R
        pa, pb, pc, ps = [par[pl.ds(16 + 8 * t, 8), :][None] for t in range(4)]
        g3 = lambda x: x.reshape(GP, 8, D)
        q = g3(qbuf[pl.ds(r, R), :].astype(f32))
        d1, r1 = _center(q)
        y = g3(jnp.concatenate([yb[j, pl.ds(r, R), :] for j in range(NT)], axis=1))
        x = q + ((d1 * r1) * pa + pb) * y
        xn[pl.ds(r, R), :] = x.reshape(R, D)
        d2, r2 = _center(x)
        h = (d2 * r2) * pc + ps
        hh[pl.ds(r, R), :] = h.reshape(R, D)
        d3, r3 = _center(h, ALPHA)
        return (d3 * r3).reshape(R, D)

    def tie(w_, vs):
        t_ = pltpu.bitcast(vs[0], u32)
        for v_ in vs[1:]:
            t_ = t_ | pltpu.bitcast(v_, u32)
        return w_ | (t_ & kbuf[0, pl.ds(0, 8), :])

    def tied(wref, ties):
        if not ties:
            return _wt(wref)
        rbs = sorted({8 * (t % 5) + rb for (t, rb) in ties})
        rows, pos = [], 0
        for rb in rbs:
            if rb > pos:
                rows.append(wref[pl.ds(8 * pos, 8 * (rb - pos)), :])
            blk = []
            for n in range(NT):
                w_ = wref[pl.ds(8 * rb, 8), pl.ds(128 * n, 128)]
                vs = ties.get((5 * n + rb // 8, rb % 8))
                blk.append(tie(w_, vs) if vs else w_)
            rows.append(jnp.concatenate(blk, axis=1))
            pos = rb + 1
        if pos < 40:
            rows.append(wref[pl.ds(8 * pos, 8 * (40 - pos)), :])
        return pltpu.bitcast(jnp.concatenate(rows, axis=0), bf16)

    def w1_dot(p, l3, ties, fresh):
        if fresh and STAG:
            grp = lambda g: l3[8 * g:8 * g + 8, 0:128]
            lt = {}
            for pr, spec in enumerate(STAG.split(',')):
                vs = [grp(2 * pr), grp(2 * pr + 1)]
                if spec[0] == 'w':
                    ties.setdefault((int(spec[1]), int(spec[2])), []).extend(vs)
                elif spec[0] == 'l':
                    lt.setdefault(int(spec[1]), []).extend(vs)
            for pr, vs in lt.items():
                x = pltpu.bitcast(tie(pltpu.bitcast(l3[16 * pr:16 * pr + 8, 128:256], u32), vs), f32)
                mid = jnp.concatenate([l3[16 * pr:16 * pr + 8, 0:128], x, l3[16 * pr:16 * pr + 8, 256:]], axis=1)
                l3 = jnp.concatenate(([l3[:16 * pr]] if pr else []) + [mid, l3[16 * pr + 8:]], axis=0)
        z = jnp.dot(l3.astype(bf16), tied(w1, ties), preferred_element_type=f32)
        g = _gelu2a(z)
        for j in range(NT):
            h1[j, pl.ds(p * R + 8, R), :] = g[:, j * 128:(j + 1) * 128]

    def w2_dot(p, ties):
        r = p * R
        lane = lax.broadcasted_iota(jnp.int32, (R, 128), 1)

        def ld(j, off):
            return h1[j, pl.ds(r + 8 + off, R), :]
        tiles = [
            ld(0, -1),
            jnp.where(lane < 32, ld(1, -1), ld(1, 1)),
            jnp.where(lane < 64, ld(2, 1), ld(2, -2)),
            jnp.where(lane < 96, ld(3, -2), ld(3, 2)),
            ld(4, 2),
        ]
        hs = jnp.concatenate(tiles, axis=1).astype(bf16)
        x1 = hh[pl.ds(r, R), :] + jnp.dot(hs, tied(w2, ties), preferred_element_type=f32) * BETA
        hh[pl.ds(r, R), :] = x1

    l3s = {}

    def ln4(r, n):
        d4, r4 = _center(hh[pl.ds(r, n), :], ALPHA)
        return d4 * r4

    def run_block(dots, pre4=False):
        for d_, (k_, p) in enumerate(dots):
            ties = {}
            e = d_ - (len(dots) - TS // R)
            if pre4 and e >= 0:
                nx = ln4(e * R, R)
                l4p[pl.ds(e * R // 2, R // 2), :] = pltpu.bitcast(nx.astype(bf16), u32)
                ties[(TIE4, 7)] = [nx[8 * g:8 * g + 8, 0:128] for g in range(GP)]
            if k_ == 1:
                fresh = p not in l3s
                w1_dot(p, ln_chain(p) if fresh else l3s.pop(p), ties, fresh)
            elif k_ == 2:
                w2_dot(p, ties)
            else:
                par[pl.ds(48, 8), :] = jnp.dot(sc_lhs(), _wt(wmc), preferred_element_type=f32)[0:8]

    with jax.named_scope("P1"):
        cp_wmp.wait()
        cp_q[0].wait()
        mp = jnp.dot(sc_lhs(), _wt(wmp), preferred_element_type=f32)
        for t in range(WMP // 128):
            modb[2 * WMA // 128 + t] = mp[0:8, 128 * t:128 * (t + 1)]
        sa, ca, ga, sb, cb = [modrow(k_) for k_ in range(5)]
        par[pl.ds(16, 8), :] = ga * (1.0 + ca)
        par[pl.ds(24, 8), :] = ga * sa
        par[pl.ds(32, 8), :] = 1.0 + cb
        par[pl.ds(40, 8), :] = sb
        for bt in range(4):
            inv_last(bt)
        for p in range(PRELN):
            l3s[p] = ln_chain(p)
    with jax.named_scope("w1wait"):
        cp_w[0].wait()
    p1, p2 = N2, 0
    with jax.named_scope("P2"):
        run_block([(1, p) for p in range(N2)])
    with jax.named_scope("w2wait"):
        wait_all([cp_w[1], cp_q[1]])

    def plan(lim1, hold):
        nonlocal p1, p2
        dots = []
        while p2 < p1 - 1 and len(dots) < 2:
            dots.append((2, p2))
            p2 += 1
        last2 = lim1 if lim1 == S // R else lim1 - 1 - hold
        while p2 < last2 or p1 < lim1:
            while p1 < lim1 and (p1 - p2 < LEAD or p2 >= last2):
                dots.append((1, p1))
                p1 += 1
            if p2 < last2:
                dots.append((2, p2))
                p2 += 1
        return dots

    with jax.named_scope("P4"):
        run_block(plan(Q1 // R, 2))
    with jax.named_scope("q2wait"):
        wait_all([cp_q[2], cp_wmc])
    with jax.named_scope("P5"):
        dots = plan(S // R, 0)
        run_block(dots[:2] + [(3, 0)] + dots[2:], pre4=True)

    def out_copy(r, c0, cn):
        return cp(obuf.at[pl.ds(r, TS), pl.ds(c0, cn)], o_hbm.at[0, pl.ds(r, TS), pl.ds(c0, cn)], osems.at[0])

    def b2_step(i):
        gbv = par[pl.ds(48, 1), :]
        nsub = T2 // TS
        for sub in range(nsub):
            r = pl.multiple_of(pl.multiple_of(i * T2, T2) + sub * TS, TS)
            l4 = _wt(l4p, pl.ds(0, TS // 2), slice(None)) if (sub == 0 and LP) else ln4(r, TS).astype(bf16)
            z = lax.dot_general(l4, _wt(w3, pl.ds(0, FA // 2), slice(None)), NTDIMS, preferred_element_type=f32)
            zt = lax.dot_general(_wt(w3, pl.ds(FA // 2, (F - FA) // 2), slice(None)), l4, NTDIMS,
                                 preferred_element_type=f32)
            g = jnp.concatenate([_gelu2a(z), _gelu2a(zt).T], axis=1).astype(bf16)
            if sub == nsub - 1 and LP:
                nx = ln4(pl.multiple_of(jnp.minimum(i + 1, S // T2 - 1) * T2, T2), TS)
                l4p[pl.ds(0, TS // 2), :] = pltpu.bitcast(nx.astype(bf16), u32)
                t_ = pltpu.bitcast(nx[0:8, 0:128], u32)
                for gi in range(1, TS // 8):
                    t_ = t_ | pltpu.bitcast(nx[8 * gi:8 * gi + 8, 0:128], u32)
                top = [w4[pl.ds(0, 8), pl.ds(128 * n, 128)] for n in range(NT)]
                top[LPN] = top[LPN] | (t_ & kbuf[0, pl.ds(0, 8), :])
                w4v = jnp.concatenate([jnp.concatenate(top, axis=1), w4[pl.ds(8, F // 2 - 8), :]], axis=0)
            else:
                w4v = w4[...]
            acc = jnp.dot(g, pltpu.bitcast(w4v, bf16), preferred_element_type=f32)
            out = xn[pl.ds(r, TS), :] + gbv * (hh[pl.ds(r, TS), :] + BETA * acc)
            for (c0, cn) in OCOLS:
                obuf[pl.ds(r, TS), pl.ds(c0, cn)] = out[:, c0:c0 + cn].astype(bf16)
                out_copy(r, c0, cn).start()

    wait_all([cp_w[2], cp_w[3]])
    with jax.named_scope("BII"):
        lax.fori_loop(0, S // T2, lambda i, c: (b2_step(i), c)[1], 0)
    with jax.named_scope("out_wait"):
        for i in range(S // TS):
            for (c0, cn) in OCOLS:
                out_copy(i * TS, c0, cn).wait()


@jax.jit
def pallas_adaLN_cond__ssm_conv_h3__mixer_s_mlp__prompt_kernel(
    A_q, A_k, A_v, A_shift_k, A_ssm_k, A_ssm_D, B_x, B_w1, B_w2, B_w3, B_w4, c, w_mod,
):
    del B_x
    hbm = pl.BlockSpec(memory_space=pltpu.MemorySpace.HBM)
    return pl.pallas_call(
        _kernel,
        out_shape=jax.ShapeDtypeStruct((1, S, D), bf16),
        in_specs=[hbm] * 12,
        out_specs=hbm,
        scratch_shapes=[
            pltpu.VMEM((27, 8, 128), f32),
            pltpu.VMEM((S + 16 * int(os.environ.get('PADF', '0')), D), bf16),
            pltpu.VMEM((NT, 32 + S // 2, 128), u32),
            pltpu.VMEM((NT, 32 + S // 2, 128), u32),
            pltpu.VMEM((NT, 64, S), u32),
            pltpu.VMEM((D // 2, D), u32),
            pltpu.VMEM((D // 2, D), u32),
            pltpu.VMEM((F // 2, D), u32),
            pltpu.VMEM((F // 2, D), u32),
            pltpu.VMEM((2, D // 2, WMA), u32),
            pltpu.VMEM((D // 2, WMP), u32),
            pltpu.VMEM((D // 2, WMC), u32),
            pltpu.VMEM((S, D), bf16),
            pltpu.VMEM((NG * 2 * NC, 8, 128), f32),
            pltpu.VMEM((NG * 2 * NC, 8, 128), f32),
            pltpu.VMEM((NG * 2 * NC, 8, 128), f32),
            pltpu.VMEM((NG * 2 * NC, 8, 128), f32),
            pltpu.VMEM((KOFF + 56 + PADK, 8, 128), f32),
            pltpu.VMEM((KOFF + 56 + PADK, 8, 128), f32),
            pltpu.VMEM((NT, S, 128), f32),
            pltpu.VMEM((S, D), f32),
            pltpu.VMEM((S, D), f32),
            pltpu.VMEM((NT, S + 32, 128), f32),
            pltpu.VMEM((64, D), f32),
            pltpu.VMEM((TS // 2 + 8 * int(os.environ.get('PADE', '0')), D), u32),
            pltpu.VMEM((4, D), bf16),
            pltpu.VMEM((D,), bf16),
            pltpu.VMEM((1, D), bf16),
            pltpu.SMEM((2,), jnp.int32),
            pltpu.SemaphoreType.DMA((22,)),
            pltpu.SemaphoreType.DMA((1,)),
        ],
        compiler_params=pltpu.CompilerParams(vmem_limit_bytes=100 * 1024 * 1024, disable_semaphore_checks=True,
                                             disable_bounds_checks=bool(int(os.environ.get('NOBC', '0')))),
    )(A_q, A_k, A_v, A_shift_k.T, A_ssm_k, A_ssm_D, B_w1, B_w2, B_w3.T, B_w4, c, w_mod)
```

```python
import math
import os

import jax
import jax.numpy as jnp
from jax import lax
import jax.experimental.pallas as pl
import jax.experimental.pallas.tpu as pltpu

S, D, F = 2048, 640, 1728
C = 128
NC = S // C
NT = D // 128
NG = 16
KOFF = (NC + 1) * NG * 3
W = int(os.environ.get('W', '4'))
SKIPA = int(os.environ.get('SKIPA', '0'))
WMA, WMP, WMC = 1280, 640, 640
Q0 = int(os.environ.get('Q0', '320'))
N2 = int(os.environ.get('N2', '5'))
PRELN = int(os.environ.get('PRELN', '2'))
NOCACHE = int(os.environ.get('NOCACHE', '0'))
OUTWAIT = int(os.environ.get('OUTWAIT', '0'))
SEGS = [int(x) for x in os.environ.get('SEGS', '012345')]
SKIPB = int(os.environ.get('SKIPB', '0'))
PADK = int(os.environ.get('PADK', '0'))
PREW = int(os.environ.get('PREW', '0'))
SP = float(os.environ.get('SP', '0'))
MINS = int(os.environ.get('MINS', '30'))
GA = int(os.environ.get('GA', '2'))
TRT = int(os.environ.get('TRT', '1'))
LP = int(os.environ.get('LP', '1'))
FA = 1664
LPN = int(os.environ.get('LPN', '2'))
G0 = int(os.environ.get('G0', '4'))
Q1 = int(os.environ.get('Q1', '704'))
TIE4 = int(os.environ.get('TIE4', '12'))
STAG = os.environ.get('STAG', 'w02,l0,n,n')
OCOLS = ((0, 512), (512, 128))
FSTEP = int(os.environ.get('FSTEP', '1'))
FOFF = int(os.environ.get('FOFF', '0'))
KORD = int(os.environ.get('KORD', '0'))
CW = int(os.environ.get('CW', '128'))
NP4 = int(os.environ.get('NP4', '4'))
LNT = [int(x) for x in os.environ.get('LNT', '9,10,11,12').split(',')]
KARA = int(os.environ.get('KARA', '1'))
UNR = int(os.environ.get('UNR', '2'))
HEAD = int(os.environ.get('HEAD', '250'))
TAIL = int(os.environ.get('TAIL', '450'))
DORDER = os.environ.get('DORDER', 'aHbU')
R1 = int(os.environ.get('R1', '64'))
R2 = int(os.environ.get('R2', '128'))
LEAD = int(os.environ.get('LEAD', '4'))
TS = int(os.environ.get('TS', '512'))
ONEPASS = int(os.environ.get('ONEPASS', '1'))
RSQ = int(os.environ.get('RSQ', '1'))
T2 = int(os.environ.get('T2', '512'))
EPS = 1e-5
_C0 = math.sqrt(2.0 / math.pi)
ALPHA = (_C0 * 0.044715) ** (1.0 / 3.0)
GC = _C0 / ALPHA
BETA = 0.5 / ALPHA
_fc = [int(x) for x in os.environ.get('FC', '1728').split(',')]
F_CHUNKS = tuple((sum(_fc[:i]), _fc[i]) for i in range(len(_fc)))
assert sum(_fc) == F

f32 = jnp.float32
bf16 = jnp.bfloat16
u32 = jnp.uint32
NTDIMS = (((1,), (1,)), ((), ()))


def _cos_table(m, scale):
    mm = jnp.abs(((m + 256) & 511) - 256)
    x = (128 - mm).astype(f32) * (1.0 / 128.0)
    x2 = x * x
    h = math.pi / 2
    p = -(h ** 7) / 5040 + x2 * ((h ** 9) / 362880 - x2 * (h ** 11) / 39916800)
    p = h + x2 * (-(h ** 3) / 6 + x2 * ((h ** 5) / 120 + x2 * p))
    return (x * scale) * p


def _dft_tables():
    shape = (16, 8, 128)
    n = lax.broadcasted_iota(jnp.int32, shape, 0)
    s = lax.broadcasted_iota(jnp.int32, shape, 1)
    l = lax.broadcasted_iota(jnp.int32, shape, 2)
    fw, fu, iv = [], [], []
    wv = l >> 4
    tu = (16 * W) * (wv // W) + (2 * W) * ((l >> 1) & 7) + 2 * (wv % W) + (l & 1)
    for e in range(2):
        r = 2 * s + e
        j = 8 * n + (r & 7)
        fw.append(_cos_table((4 * j + 1) * l + (r >> 3) * 128, 1.0))
        fu.append(_cos_table((4 * j + 1) * tu + (r >> 3) * 128, 1.0))
        b = 16 * (n >> 1) + r
        col = 128 * (n & 1) + l
        iv.append(_cos_table((4 * (col >> 1) + 1) * b + (col & 1) * 128, 1.0 / 128.0))
    pk = lambda xs: pltpu.bitcast(pltpu.pack_elementwise(xs, packed_dtype=bf16), f32)
    return pk(fw), pk(iv), pk(fu)


def _gelu2a(z):
    return z * (1.0 + jnp.tanh(z * (z * z + GC)))


def _rstd(ssd, scale):
    if RSQ == 0:
        r = lax.rsqrt(ssd * (1.0 / D) + EPS)
        return r if scale == 1.0 else r * scale
    return jnp.exp2(jnp.log(ssd + D * EPS) * (-0.5 / math.log(2.0)) + math.log2(scale * math.sqrt(D)))


def _center(x, scale=1.0):
    s1 = jnp.sum(x, axis=-1, keepdims=True)
    m = s1 * (1.0 / D)
    d = x - m
    if ONEPASS:
        ssd = jnp.maximum(jnp.sum(x * x, axis=-1, keepdims=True) - s1 * m, 0.0)
    else:
        ssd = jnp.sum(d * d, axis=-1, keepdims=True)
    return d, _rstd(ssd, scale)


def _conv(us, gs, a):
    acc = None
    for c in range(a + 1):
        p = us[c] * gs[a - c]
        acc = p if acc is None else acc + p
    return acc


def _mult(x, n):
    return x if isinstance(x, int) else pl.multiple_of(x, n)


def _wt(ref, *idx):
    return pltpu.bitcast(ref[idx] if idx else ref[...], bf16)


def _kernel(q_hbm, k_hbm, v_hbm, sk_hbm, h_hbm, dd_hbm, w1_hbm, w2_hbm, w3_hbm, w4_hbm,
            c_hbm, wm_hbm, o_hbm,
            modb, qbuf, kbuf, vbuf, hbuf, w1, w2, w3, w4, wm, wmp, wmc, obuf,
            ub0, ub1, gb0, gb1, kb0, kb1, yb, xn, hh, h1, par, l4p, gs, sk_s, dd_s, c_s, zs, sems, osems):
    ubs, gbs, kbs = (ub0, ub1), (gb0, gb1), (kb0, kb1)
    cp = pltpu.make_async_copy
    HS = S // 2

    def cp_h(j, c0, c1, sem):
        return cp(h_hbm.at[pl.ds(j * 128, 128), pl.ds(c0, c1 - c0)], hbuf.bitcast(bf16).at[j, :, pl.ds(c0, c1 - c0)], sem)

    def cp_kv(j, r0, r1, sem):
        r0, r1 = (r0 + 16 if r0 else 0), min(r1 + 16, S)
        lanes = pl.ds(j * 128, 128)
        return [cp(k_hbm.at[0, pl.ds(r0, r1 - r0), lanes], kbuf.bitcast(bf16).at[j, pl.ds(r0 + 16, r1 - r0), :], sem),
                cp(v_hbm.at[0, pl.ds(r0, r1 - r0), lanes], vbuf.bitcast(bf16).at[j, pl.ds(r0, r1 - r0), :], sem)]

    def cp_tile(j, i):
        sem = sems.at[2 * j + i]
        return [cp_h(j, i * HS, (i + 1) * HS, sem)] + cp_kv(j, i * HS, (i + 1) * HS, sem)

    cp_t0 = [[cp_h(0, 0, S, sems.at[0])], cp_kv(0, 0, 1024, sems.at[1]), cp_kv(0, 1024, 1536, sems.at[20]),
             cp_kv(0, 1536, S, sems.at[21])]

    def cp_wm(i):
        return cp(wm_hbm.at[:, pl.ds(i * WMA, WMA)], wm.bitcast(bf16).at[i], sems.at[10 + i])

    cp_wmp = cp(wm_hbm.at[:, pl.ds(2 * WMA, WMP)], wmp.bitcast(bf16), sems.at[13])
    cp_wmc = cp(wm_hbm.at[:, pl.ds(2 * WMA + WMP, WMC)], wmc.bitcast(bf16), sems.at[12])
    cp_q = [cp(q_hbm.at[0, pl.ds(r0, r1 - r0), :], qbuf.at[pl.ds(r0, r1 - r0), :], sems.at[sm])
            for sm, r0, r1 in ((13, 0, Q0), (16, Q0, Q1), (12, Q1, S))]
    cp_w = [cp(s_, d_.bitcast(bf16).at[pl.ds(0, s_.shape[0]), :], sems.at[sm])
            for sm, s_, d_ in ((15, w1_hbm, w1), (16, w2_hbm, w2), (14, w3_hbm, w3), (14, w4_hbm, w4))]
    cp_s = [cp(sk_hbm, sk_s, sems.at[19]), cp(dd_hbm, dd_s, sems.at[19]), cp(c_hbm, c_s, sems.at[19])]
    order = list(cp_s)
    for grp in cp_t0:
        order += grp
    for j in range(1, NT):
        order += cp_tile(j, 0) + cp_tile(j, 1)
    order += [cp_wm(0), cp_wm(1), cp_wmp, cp_q[0], cp_w[0], cp_w[1], cp_q[1], cp_q[2], cp_wmc, cp_w[2], cp_w[3]]
    for c_ in order:
        c_.start()

    with jax.named_scope("init"):
        fw_t, iv_t, fu_t = _dft_tables()
        for kb in kbs:
            kb[pl.ds(KOFF, 16)] = fw_t
            kb[pl.ds(KOFF + 16, 16)] = iv_t
            kb[pl.ds(KOFF + 32, 16)] = fu_t
            kb[pl.ds(0, NG * 3)] = jnp.zeros((NG * 3, 8, 128), f32)
        zeros = jnp.zeros((8, 128), f32)
        w4[pl.ds(F // 2, 32), :] = jnp.zeros((32, D), u32)
        for j in range(NT):
            kbuf[j, pl.ds(0, 8), :] = jnp.zeros((8, 128), u32)
            kbuf[j, pl.ds(8 + HS, 8), :] = jnp.zeros((8, 128), u32)
            vbuf[j, pl.ds(HS, 8), :] = jnp.zeros((8, 128), u32)
        for j in range(NT):
            h1[j, pl.ds(0, 8), :] = zeros
            h1[j, pl.ds(S + 8, 8), :] = zeros
        for c_ in cp_s:
            c_.wait()
        par[pl.ds(0, 4), :] = sk_s[...].astype(f32)
        par[pl.ds(8, 8), :] = jnp.broadcast_to(dd_s[...].astype(f32).reshape(1, D), (8, D))
        cv = c_s[...].astype(f32)
        sc = jnp.broadcast_to(cv * jax.nn.sigmoid(cv), (8, D))
        scp = pltpu.bitcast(pltpu.pack_elementwise([sc, sc], packed_dtype=bf16), f32)
        for j in range(NT):
            kb0[KOFF + 48 + j] = scp[:, 128 * j:128 * (j + 1)]
            kb1[KOFF + 48 + j] = scp[:, 128 * j:128 * (j + 1)]

    def mkb(i, unr, off, cache):
        def b(stride, extra=0, z=None):
            if isinstance(i, int):
                return (i * unr + off) * stride + extra
            key = (unr * stride, z)
            if key not in cache or NOCACHE:
                base = pl.multiple_of(i * (unr * stride), unr * stride)
                cache[key] = base if z is None else base + (i >> z)
            return cache[key] + (off * stride + extra)
        return b

    def dot_h(j, b, lhs):
        gb = gbs[j % 2]
        hc = hbuf[j, :, pl.ds(_mult(b(512), 512), 512)]
        rhs_t = jnp.concatenate([hc[:, C * cc:C * (cc + 1)] for cc in range(4)], axis=0)
        g = lax.dot_general(lhs, pltpu.bitcast(rhs_t, bf16), NTDIMS, preferred_element_type=f32)
        for rg in range(2 * NG):
            for cc in range(4):
                gb[b(4, cc + rg * NC)] = g[8 * rg:8 * rg + 8, 128 * cc:128 * cc + 128]

    def dot_u(j, b, lhs):
        ub = ubs[j % 2]
        taps = [par[pl.ds(t, 1), pl.ds(j * 128, 128)] for t in range(4)]
        unp = lambda w_, e: pltpu.unpack_elementwise(w_, index=e, packed_dtype=bf16, unpacked_dtype=f32)
        cols = []
        for cc in range(4):
            words = []
            for blk in range(8 // W):
                w0 = 64 * cc + 8 * W * blk
                kw = {m: kbuf[j, pl.ds(b(256, 8 + w0 + m), 8, stride=W), :] for m in range(-2, W)}
                kk = {2 * m + e: unp(kw[m], e) for m in range(-2, W) for e in range(2) if 2 * m + e >= -3}
                for m in range(W):
                    vw = vbuf[j, pl.ds(b(256, w0 + m), 8, stride=W), :]
                    pair = []
                    for e in range(2):
                        n = 2 * m + e
                        ks = kk[n] * taps[0] + kk[n - 1] * taps[1] + kk[n - 2] * taps[2] + kk[n - 3] * taps[3]
                        pair.append(ks * unp(vw, e))
                    words.append(pltpu.pack_elementwise(pair, packed_dtype=bf16))
            cols.append(jnp.concatenate(words, axis=0))
        rhs = pltpu.bitcast(jnp.concatenate(cols, axis=1), bf16)
        u = jnp.dot(lhs, rhs, preferred_element_type=f32)
        for rg in range(2 * NG):
            for cc in range(4):
                ub[b(4, cc + rg * NC)] = u[8 * rg:8 * rg + 8, 128 * cc:128 * cc + 128]

    def dot_i(j, b, half, lhs):
        kb = kbs[j % 2]
        cols = [[], []]
        for gi in range(NG):
            prev = None
            for cc in range(-1, 2):
                k0, k1, k2 = [kb[b(4 * NG * 3, ((2 * half + cc + 1) * NG + gi) * 3 + t)] for t in range(3)]
                re, im = k0 - k2, k0 + k1
                if prev is not None:
                    cols[cc].append(pltpu.pack_elementwise([re - prev[1], im + prev[0]], packed_dtype=bf16))
                prev = (re, im)
        rhs = jnp.concatenate([jnp.concatenate(c_, axis=0) for c_ in cols], axis=1)
        y = jnp.dot(lhs, pltpu.bitcast(rhs, bf16), preferred_element_type=f32)
        for cc in range(2):
            yb[j, pl.ds(b(512, (2 * half + cc) * C), C), :] = y[:, 128 * cc:128 * cc + 128]

    def gen_m(j, kb, b, ng):
        ub, gb = ubs[j % 2], gbs[j % 2]
        for s in range(ng):
            for t in range(3):
                z = 8 + t
                re = lambda ref, c: ref[b(2 * NC, 2 * s * NC + c, z)]
                im = lambda ref, c: ref[b(2 * NC, (2 * s + 1) * NC + c, z)]
                gre = [re(gb, c) for c in range(NC)]
                if t == 0:
                    us = [re(ub, c) + im(ub, c) for c in range(NC)]
                    gs = gre
                elif t == 1:
                    us = [re(ub, c) for c in range(NC)]
                    gs = [im(gb, c) - gre[c] for c in range(NC)]
                else:
                    us = [im(ub, c) for c in range(NC)]
                    gs = [im(gb, c) + gre[c] for c in range(NC)]

                def st(a, val):
                    kb[b(3, ((a + 1) * NG + s) * 3 + t)] = val
                if not KARA:
                    for a in range(NC):
                        st(a, _conv(us, gs, a))
                        yield 2 * a + 2
                    continue
                ue, uo, ge, go = us[0::2], us[1::2], gs[0::2], gs[1::2]
                if KORD == 1:
                    usum = [x + y for x, y in zip(ue, uo)]
                    gsum = [x + y for x, y in zip(ge, go)]
                    poo = _conv(uo, go, NC // 2 - 1)
                    for a in reversed(range(NC // 2)):
                        pee = _conv(ue, ge, a)
                        pss = _conv(usum, gsum, a)
                        st(2 * a + 1, pss - pee - poo)
                        poo = _conv(uo, go, a - 1) if a else None
                        st(2 * a, pee + poo if a else pee)
                        yield 3 * (2 * a + 1) + (37 if a == NC // 2 - 1 else 3)
                    continue
                usum = [x + y for x, y in zip(ue, uo)]
                gsum = [x + y for x, y in zip(ge, go)]
                poo_prev = None
                for a in range(NC // 2):
                    pee = _conv(ue, ge, a)
                    poo = _conv(uo, go, a)
                    pss = _conv(usum, gsum, a)
                    st(2 * a, pee if poo_prev is None else pee + poo_prev)
                    st(2 * a + 1, pss - pee - poo)
                    poo_prev = poo
                    yield 3 * (2 * a + 1) + 7

    def add_d(j):
        gb = gbs[j % 2]
        dvec = par[pl.ds(8, 8), pl.ds(j * 128, 128)]
        for gi in range(NG):
            gb[2 * gi * NC] = gb[2 * gi * NC] + dvec

    def sc_lhs():
        return pltpu.bitcast(jnp.concatenate([kb0[KOFF + 48 + j] for j in range(NT)], axis=1), bf16)

    def dot_m(i, t0, nt, rows):
        m = None
        for kt in range(NT):
            p = jnp.dot(pltpu.bitcast(rows[kt], bf16), _wt(wm, i, pl.ds(64 * kt, 64), pl.ds(128 * t0, 128 * nt)),
                        preferred_element_type=f32)
            m = p if m is None else m + p
        for t in range(nt):
            modb[i * (WMA // 128) + (t0 + t)] = m[0:8, 128 * t:128 * (t + 1)]

    def inv_lhs(tbl, n):
        return jnp.concatenate([tbl[KOFF + 16 + 2 * n], tbl[KOFF + 17 + 2 * n]], axis=1)

    def dot_k(kb, kt, bt, lhs):
        cols = [[] for _ in range(4)]
        for gi in range(8 * kt, 8 * kt + 8):
            prev = None
            for cc in range(-1, 4):
                k0, k1, k2 = [kb[((4 * bt + cc + 1) * NG + gi) * 3 + t] for t in range(3)]
                re, im = k0 - k2, k0 + k1
                if prev is not None:
                    cols[cc].append(pltpu.pack_elementwise([re - prev[1], im + prev[0]], packed_dtype=bf16))
                prev = (re, im)
        rhs = jnp.concatenate([jnp.concatenate(c_, axis=0) for c_ in cols], axis=1)
        y = jnp.dot(lhs, pltpu.bitcast(rhs, bf16), preferred_element_type=f32)
        for cc in range(4):
            rows = pl.ds((4 * bt + cc) * C, C)
            yc = y[:, 128 * cc:128 * cc + 128]
            yb[NT - 1, rows, :] = yc if kt == 0 else yb[NT - 1, rows, :] + yc

    PRE = dict(H=0, U=672 + 96 // W, a=192, b=192, m=0, k=176)
    POST = dict(H=0, U=0, a=4, b=4, m=2, k=0)
    NST = dict(H=16, U=16, a=8, b=8, m=5, k=8)
    GCOST = 3 * (248 if KARA else 272)

    def a_block(dots, mg=None, ng=0, tbl=kb0):
        native, dur = [], []
        for idx, (k_, _) in enumerate(dots):
            nxt = PRE[dots[idx + 1][0]] if idx + 1 < len(dots) else 0
            d_ = 2.0 if k_ == 'm' else 1.0
            native += [nxt / NST[k_] + POST[k_] * d_] * NST[k_]
            dur += [d_] * NST[k_]
        if mg is not None and dots:
            head = max(HEAD - PRE[dots[0][0]], 0)
            mtot = GCOST * ng - TAIL - head
            lvl = (mtot + sum(native)) / sum(dur)
            want = [max(lvl * d_ - x, 0.0) for x, d_ in zip(native, dur)]
            scale = mtot / sum(want)
            cum, tgt = [head], head
            for w_ in want:
                tgt += w_ * scale
                cum.append(tgt)
        done = 0.0
        step = 0
        for (k_, fn) in dots:
            rows = []
            for n in range(NST[k_]):
                if mg is not None and (n % FSTEP == 0 or k_ == 'm'):
                    while done < cum[min(step + FOFF, len(cum) - 1)]:
                        done += next(mg)
                step += 1
                if k_ in 'HU':
                    rows.append(tbl[KOFF + n + (32 if k_ == 'U' else 0)])
                elif k_ in 'ab':
                    rows.append(inv_lhs(tbl, n))
                elif k_ == 'k':
                    rows.append(tbl[KOFF + 16 + 2 * n])
                else:
                    rows.append(tbl[KOFF + 48 + n])
            fn(rows if k_ == 'm' else pltpu.bitcast(jnp.concatenate(rows, axis=0), bf16))
        if mg is not None:
            for _ in mg:
                pass

    def fdot(k_, j, b):
        if k_ == 'H':
            return (k_, lambda lhs: dot_h(j, b, lhs))
        if k_ == 'U':
            return (k_, lambda lhs: dot_u(j, b, lhs))
        return (k_, lambda lhs: dot_i(j, b, 0 if k_ == 'a' else 1, lhs))

    def wait_all(cps):
        for c_ in cps:
            c_.wait()

    def a_loop(jf, jm, ji, g0, ng):
        kinds = [k_ for k_ in DORDER if k_ in 'HU' or ji is not None]

        def body(i, carry):
            cache = {}
            zs[i] = 0
            dots = [fdot(k_, jf if k_ in 'HU' else ji, mkb(i, 2, s_, cache)) for s_ in range(2) for k_ in kinds]
            a_block(dots, gen_m(jm, kbs[jm % 2], mkb(i, ng, g0, cache), ng), ng, kbs[jm % 2])

            @pl.when(i == 0)
            def _():
                wait_all(cp_tile(jf, 1))
            return carry
        wait_all(cp_tile(jf, 0))
        lax.fori_loop(0, 2, body, 0)
        add_d(jf)

    sb_ = lambda bt: mkb(0, 1, bt, None)
    if SKIPA:
        a_block = lambda *a, **k: None
    with jax.named_scope("A_seg0"):
        wait_all(cp_t0[0])
        a_block([fdot('H', 0, sb_(bt)) for bt in range(4)])
        add_d(0)
        wait_all(cp_t0[1])
        a_block([fdot('U', 0, sb_(bt)) for bt in range(2)])
        for bt in (2, 3):
            wait_all(cp_t0[bt])
            a_block([fdot('U', 0, sb_(bt))])
    with jax.named_scope("A_m0"):
        def body_m0(i, carry):
            a_block([], gen_m(0, kb0, mkb(i, G0 // 2, 0, {}), G0 // 2))
            return carry
        if G0:
            lax.fori_loop(0, 2, body_m0, 0)
    for seg in range(1, NT):
        with jax.named_scope(f"A_seg{seg}"):
            if seg == 1:
                a_loop(1, 0, None, G0, (NG - G0) // 2)
            else:
                a_loop(seg, seg - 1, seg - 2, 0, 8)

    def mods(i):
        return [('m', lambda rows, t0=t0, nt=nt: dot_m(i, t0, nt, rows)) for (t0, nt) in ((0, 4), (4, 4), (8, 2))]

    with jax.named_scope("A_seg5a"):
        cp_wm(0).wait()
        zz = zs[1]

        @pl.when(zz == 0)
        def _():
            dots = [fdot(k_, NT - 2, sb_(bt)) for bt in range(4) for k_ in 'ab']
            mm = mods(0)
            dots = [mm[0]] + dots[0:2] + [mm[1]] + dots[2:4] + [mm[2]] + dots[4:]
            a_block(dots, gen_m(NT - 1, kb0, mkb(zz, 8, 0, {}), 8), 8, kb0)
    with jax.named_scope("A_seg5b"):
        cp_wm(1).wait()

        @pl.when(zz == 0)
        def _():
            dots = [('k', lambda lhs, bt=bt: dot_k(kb0, 0, bt, lhs)) for bt in range(4)]
            mm = mods(1)
            dots = [mm[0], dots[0], mm[1], dots[1], mm[2]] + dots[2:]
            a_block(dots, gen_m(NT - 1, kb1, mkb(zz, 8, 8, {}), 8), 8, kb1)

    def inv_last(bt):
        lhs = pltpu.bitcast(jnp.concatenate([kb0[KOFF + 17 + 2 * n] for n in range(8)], axis=0), bf16)
        dot_k(kb1, 1, bt, lhs)

    def modrow(k_):
        return jnp.concatenate([modb[NT * k_ + j] for j in range(NT)], axis=1)

    R = R1
    GP = R // 8

    def ln_chain(p):
        r = p * R
        pa, pb, pc, ps = [par[pl.ds(16 + 8 * t, 8), :][None] for t in range(4)]
        g3 = lambda x: x.reshape(GP, 8, D)
        q = g3(qbuf[pl.ds(r, R), :].astype(f32))
        d1, r1 = _center(q)
        y = g3(jnp.concatenate([yb[j, pl.ds(r, R), :] for j in range(NT)], axis=1))
        x = q + ((d1 * r1) * pa + pb) * y
        xn[pl.ds(r, R), :] = x.reshape(R, D)
        d2, r2 = _center(x)
        h = (d2 * r2) * pc + ps
        hh[pl.ds(r, R), :] = h.reshape(R, D)
        d3, r3 = _center(h, ALPHA)
        return (d3 * r3).reshape(R, D)

    def tie(w_, vs):
        t_ = pltpu.bitcast(vs[0], u32)
        for v_ in vs[1:]:
            t_ = t_ | pltpu.bitcast(v_, u32)
        return w_ | (t_ & kbuf[0, pl.ds(0, 8), :])

    def tied(wref, ties):
        if not ties:
            return _wt(wref)
        rbs = sorted({8 * (t % 5) + rb for (t, rb) in ties})
        rows, pos = [], 0
        for rb in rbs:
            if rb > pos:
                rows.append(wref[pl.ds(8 * pos, 8 * (rb - pos)), :])
            blk = []
            for n in range(NT):
                w_ = wref[pl.ds(8 * rb, 8), pl.ds(128 * n, 128)]
                vs = ties.get((5 * n + rb // 8, rb % 8))
                blk.append(tie(w_, vs) if vs else w_)
            rows.append(jnp.concatenate(blk, axis=1))
            pos = rb + 1
        if pos < 40:
            rows.append(wref[pl.ds(8 * pos, 8 * (40 - pos)), :])
        return pltpu.bitcast(jnp.concatenate(rows, axis=0), bf16)

    def w1_dot(p, l3, ties, fresh):
        if fresh and STAG:
            grp = lambda g: l3[8 * g:8 * g + 8, 0:128]
            lt = {}
            for pr, spec in enumerate(STAG.split(',')):
                vs = [grp(2 * pr), grp(2 * pr + 1)]
                if spec[0] == 'w':
                    ties.setdefault((int(spec[1]), int(spec[2])), []).extend(vs)
                elif spec[0] == 'l':
                    lt.setdefault(int(spec[1]), []).extend(vs)
            for pr, vs in lt.items():
                x = pltpu.bitcast(tie(pltpu.bitcast(l3[16 * pr:16 * pr + 8, 128:256], u32), vs), f32)
                mid = jnp.concatenate([l3[16 * pr:16 * pr + 8, 0:128], x, l3[16 * pr:16 * pr + 8, 256:]], axis=1)
                l3 = jnp.concatenate(([l3[:16 * pr]] if pr else []) + [mid, l3[16 * pr + 8:]], axis=0)
        z = jnp.dot(l3.astype(bf16), tied(w1, ties), preferred_element_type=f32)
        g = _gelu2a(z)
        for j in range(NT):
            h1[j, pl.ds(p * R + 8, R), :] = g[:, j * 128:(j + 1) * 128]

    def w2_dot(p, ties):
        r = p * R
        lane = lax.broadcasted_iota(jnp.int32, (R, 128), 1)

        def ld(j, off):
            return h1[j, pl.ds(r + 8 + off, R), :]
        tiles = [
            ld(0, -1),
            jnp.where(lane < 32, ld(1, -1), ld(1, 1)),
            jnp.where(lane < 64, ld(2, 1), ld(2, -2)),
            jnp.where(lane < 96, ld(3, -2), ld(3, 2)),
            ld(4, 2),
        ]
        hs = jnp.concatenate(tiles, axis=1).astype(bf16)
        x1 = hh[pl.ds(r, R), :] + jnp.dot(hs, tied(w2, ties), preferred_element_type=f32) * BETA
        hh[pl.ds(r, R), :] = x1

    l3s = {}

    def ln4(r, n):
        d4, r4 = _center(hh[pl.ds(r, n), :], ALPHA)
        return d4 * r4

    def run_block(dots, pre4=False):
        for d_, (k_, p) in enumerate(dots):
            ties = {}
            e = d_ - (len(dots) - NP4)
            RP = TS // NP4
            if pre4 and e >= 0:
                nx = ln4(e * RP, RP)
                l4p[pl.ds(e * RP, RP), :] = nx
                ties[(TIE4, 7)] = [nx[8 * g:8 * g + 8, 0:128] for g in range(RP // 8)]
            if k_ == 1:
                fresh = p not in l3s
                w1_dot(p, ln_chain(p) if fresh else l3s.pop(p), ties, fresh)
            elif k_ == 2:
                w2_dot(p, ties)
            else:
                par[pl.ds(48, 8), :] = jnp.dot(sc_lhs(), _wt(wmc), preferred_element_type=f32)[0:8]

    with jax.named_scope("P1"):
        cp_wmp.wait()
        cp_q[0].wait()
        mp = jnp.dot(sc_lhs(), _wt(wmp), preferred_element_type=f32)
        for t in range(WMP // 128):
            modb[2 * WMA // 128 + t] = mp[0:8, 128 * t:128 * (t + 1)]
        sa, ca, ga, sb, cb = [modrow(k_) for k_ in range(5)]
        par[pl.ds(16, 8), :] = ga * (1.0 + ca)
        par[pl.ds(24, 8), :] = ga * sa
        par[pl.ds(32, 8), :] = 1.0 + cb
        par[pl.ds(40, 8), :] = sb
        for bt in range(4):
            inv_last(bt)
        for p in range(PRELN):
            l3s[p] = ln_chain(p)
    with jax.named_scope("w1wait"):
        cp_w[0].wait()
    p1, p2 = N2, 0
    with jax.named_scope("P2"):
        run_block([(1, p) for p in range(N2)])
    with jax.named_scope("w2wait"):
        wait_all([cp_w[1], cp_q[1]])

    def plan(lim1, hold):
        nonlocal p1, p2
        dots = []
        while p2 < p1 - 1 and len(dots) < 2:
            dots.append((2, p2))
            p2 += 1
        last2 = lim1 if lim1 == S // R else lim1 - 1 - hold
        while p2 < last2 or p1 < lim1:
            while p1 < lim1 and (p1 - p2 < LEAD or p2 >= last2):
                dots.append((1, p1))
                p1 += 1
            if p2 < last2:
                dots.append((2, p2))
                p2 += 1
        return dots

    with jax.named_scope("P4"):
        run_block(plan(Q1 // R, 2))
    with jax.named_scope("q2wait"):
        wait_all([cp_q[2], cp_wmc])
    with jax.named_scope("P5"):
        dots = plan(S // R, 0)
        run_block(dots[:2] + [(3, 0)] + dots[2:], pre4=True)

    H2 = TS // 2
    OUTS = ((0, TS, 0, 512), (0, H2, 512, 128), (H2, H2, 512, 128))

    def out_copy(r, r0, rn, c0, cn):
        rows = pl.ds(_mult(r + r0, H2), rn)
        return cp(obuf.at[rows, pl.ds(c0, cn)], o_hbm.at[0, rows, pl.ds(c0, cn)], osems.at[0])

    def wsum(x, y, sign):
        unp = lambda w_, e: pltpu.unpack_elementwise(w_, index=e, packed_dtype=bf16, unpacked_dtype=f32)
        return pltpu.pack_elementwise([unp(x, e) + unp(y, e) if sign > 0 else unp(x, e) - unp(y, e) for e in range(2)],
                                      packed_dtype=bf16)

    def strassen_lhs(a11, a12, a21, a22):
        c = lambda x: x.astype(bf16)
        return (c(a11 + a22), c(a21 + a22), c(a11), c(a22), c(a11 + a12), c(a21 - a11), c(a12 - a22))

    def strassen(ops, b11, b12, b21, b22, mm, ties=None):
        def tw(k_, w_):
            if not ties or k_ not in ties:
                return w_
            return jnp.concatenate([tie(w_[0:8], ties[k_]), w_[8:]], axis=0)
        m1 = mm(ops[0], tw(0, wsum(b11, b22, 1)))
        m4 = mm(ops[3], tw(1, wsum(b21, b11, -1)))
        m2 = mm(ops[1], tw(2, b11))
        m3 = mm(ops[2], tw(3, wsum(b12, b22, -1)))
        m5 = mm(ops[4], tw(4, b22))
        m7 = mm(ops[6], tw(5, wsum(b21, b22, 1)))
        m6 = mm(ops[5], tw(6, wsum(b11, b12, 1)))
        return (m1 + m4) + (m7 - m5), m3 + m5, m4 + m2, (m1 + (m3 - m2)) + m6

    mm_nt = lambda x, w_: lax.dot_general(x, pltpu.bitcast(w_, bf16), NTDIMS, preferred_element_type=f32)
    mm_nn = lambda x, w_: jnp.dot(x, pltpu.bitcast(w_, bf16), preferred_element_type=f32)

    def b2_step(i):
        gbv = par[pl.ds(48, 8), :]
        nsub = T2 // TS
        for sub in range(nsub):
            r = pl.multiple_of(pl.multiple_of(i * T2, T2) + sub * TS, TS)
            l4 = l4p[...] if sub == 0 else ln4(r, TS)
            lb = l4.astype(bf16)
            zt = lax.dot_general(_wt(w3, pl.ds(832, 32), slice(None)), lb, NTDIMS, preferred_element_type=f32)
            g12 = _gelu2a(mm_nt(lb, w3[pl.ds(768, 64), :]))
            gt = jnp.concatenate([_gelu2a(zt), jnp.zeros((64, TS), f32)], axis=0).T
            gs[:, pl.ds(0, 128)] = g12
            gs[:, pl.ds(896, 128)] = gt
            ops = strassen_lhs(l4[:H2, 0:256], l4[:H2, 256:512], l4[H2:, 0:256], l4[H2:, 256:512])
            lr = l4[:, 512:640].astype(bf16)
            for c in range(768 // CW):
                ra, rb = pl.ds(c * CW // 2, CW // 2), pl.ds(384 + c * CW // 2, CW // 2)
                k1, k2 = pl.ds(0, 256), pl.ds(256, 256)
                c11, c12, c21, c22 = strassen(ops, w3[ra, k1], w3[rb, k1], w3[ra, k2], w3[rb, k2], mm_nt)
                za = jnp.concatenate([c11, c21], axis=0) + mm_nt(lr, w3[ra, pl.ds(512, 128)])
                zb = jnp.concatenate([c12, c22], axis=0) + mm_nt(lr, w3[rb, pl.ds(512, 128)])
                gs[:, pl.ds(128 + c * CW, CW)] = _gelu2a(za)
                gs[:, pl.ds(1024 + c * CW, CW)] = _gelu2a(zb)
            g1, g2 = gs[:, pl.ds(0, 896)], gs[:, pl.ds(896, 896)]
            ops = strassen_lhs(g1[:H2], g2[:H2], g1[H2:], g2[H2:])

            def w4k(half, cols):
                lo, base = (768, 0) if half == 0 else (832, 384)
                return jnp.concatenate([w4[pl.ds(lo, 64), cols], w4[pl.ds(base, 384), cols]], axis=0)
            acc = [None] * 4
            ties = {}
            if sub == nsub - 1:
                rn_ = pl.multiple_of(jnp.minimum(i + 1, S // T2 - 1) * T2, T2)
                RP = TS // len(LNT)
                for e, k_ in enumerate(LNT):
                    nx = ln4(pl.multiple_of(rn_ + e * RP, RP), RP)
                    l4p[pl.ds(e * RP, RP), :] = nx
                    ties[k_] = [nx[8 * gi:8 * gi + 8, 0:128] for gi in range(RP // 8)]
            for n in range(2):
                na, nb = pl.ds(128 * n, 128), pl.ds(128 * (n + 2), 128)
                c11, c12, c21, c22 = strassen(ops, w4k(0, na), w4k(0, nb), w4k(1, na), w4k(1, nb), mm_nn,
                                              {k_ - 7 * n: v_ for k_, v_ in ties.items() if 0 <= k_ - 7 * n < 7})
                acc[n] = jnp.concatenate([c11, c21], axis=0)
                acc[n + 2] = jnp.concatenate([c12, c22], axis=0)
            wl = jnp.concatenate([w4k(0, pl.ds(512, 128)), w4k(1, pl.ds(512, 128))], axis=0)
            accs = (jnp.concatenate(acc, axis=1), mm_nn(gs[pl.ds(0, H2), :].astype(bf16), wl),
                    mm_nn(gs[pl.ds(H2, H2), :].astype(bf16), wl))
            for (r0, rn, c0, cn), ac in zip(OUTS, accs):
                rows, cols = pl.ds(_mult(r + r0, H2), rn), pl.ds(c0, cn)
                g3 = lambda x: x.reshape(rn // 8, 8, cn)
                out = g3(xn[rows, cols]) + gbv[None, :, c0:c0 + cn] * g3(hh[rows, cols] + BETA * ac)
                obuf[rows, cols] = out.reshape(rn, cn).astype(bf16)
                out_copy(r, r0, rn, c0, cn).start()

    wait_all([cp_w[2], cp_w[3]])
    with jax.named_scope("BII"):
        lax.fori_loop(0, S // T2, lambda i, c: (b2_step(i), c)[1], 0)
    with jax.named_scope("out_wait"):
        for i in range(S // TS):
            for o_ in OUTS:
                out_copy(i * TS, *o_).wait()


@jax.jit
def pallas_adaLN_cond__ssm_conv_h3__mixer_s_mlp__prompt_kernel(
    A_q, A_k, A_v, A_shift_k, A_ssm_k, A_ssm_D, B_x, B_w1, B_w2, B_w3, B_w4, c, w_mod,
):
    del B_x
    hbm = pl.BlockSpec(memory_space=pltpu.MemorySpace.HBM)
    return pl.pallas_call(
        _kernel,
        out_shape=jax.ShapeDtypeStruct((1, S, D), bf16),
        in_specs=[hbm] * 12,
        out_specs=hbm,
        scratch_shapes=[
            pltpu.VMEM((27, 8, 128), f32),
            pltpu.VMEM((S + 16 * int(os.environ.get('PADF', '0')), D), bf16),
            pltpu.VMEM((NT, 32 + S // 2, 128), u32),
            pltpu.VMEM((NT, 32 + S // 2, 128), u32),
            pltpu.VMEM((NT, 64, S), u32),
            pltpu.VMEM((D // 2, D), u32),
            pltpu.VMEM((D // 2, D), u32),
            pltpu.VMEM((F // 2, D), u32),
            pltpu.VMEM((896, D), u32),
            pltpu.VMEM((2, D // 2, WMA), u32),
            pltpu.VMEM((D // 2, WMP), u32),
            pltpu.VMEM((D // 2, WMC), u32),
            pltpu.VMEM((S, D), bf16),
            pltpu.VMEM((NG * 2 * NC, 8, 128), f32),
            pltpu.VMEM((NG * 2 * NC, 8, 128), f32),
            pltpu.VMEM((NG * 2 * NC, 8, 128), f32),
            pltpu.VMEM((NG * 2 * NC, 8, 128), f32),
            pltpu.VMEM((KOFF + 56 + PADK, 8, 128), f32),
            pltpu.VMEM((KOFF + 56 + PADK, 8, 128), f32),
            pltpu.VMEM((NT, S, 128), f32),
            pltpu.VMEM((S, D), f32),
            pltpu.VMEM((S, D), f32),
            pltpu.VMEM((NT, S + 32, 128), f32),
            pltpu.VMEM((64, D), f32),
            pltpu.VMEM((TS, D), f32),
            pltpu.VMEM((TS, 1792), f32),
            pltpu.VMEM((4, D), bf16),
            pltpu.VMEM((D,), bf16),
            pltpu.VMEM((1, D), bf16),
            pltpu.SMEM((2,), jnp.int32),
            pltpu.SemaphoreType.DMA((22,)),
            pltpu.SemaphoreType.DMA((1,)),
        ],
        compiler_params=pltpu.CompilerParams(vmem_limit_bytes=100 * 1024 * 1024, disable_semaphore_checks=True,
                                             disable_bounds_checks=bool(int(os.environ.get('NOBC', '0')))),
    )(A_q, A_k, A_v, A_shift_k.T, A_ssm_k, A_ssm_D, B_w1, B_w2, B_w3.T, B_w4, c, w_mod)
```

```python
import math
import os

import jax
import jax.numpy as jnp
from jax import lax
import jax.experimental.pallas as pl
import jax.experimental.pallas.tpu as pltpu

S, D, F = 2048, 640, 1728
C = 128
NC = S // C
NT = D // 128
NG = 16
KOFF = (NC + 1) * NG * 3
W = int(os.environ.get('W', '4'))
SKIPA = int(os.environ.get('SKIPA', '0'))
WMA, WMP, WMC = 1280, 640, 640
Q0 = int(os.environ.get('Q0', '320'))
N2 = int(os.environ.get('N2', '5'))
PRELN = int(os.environ.get('PRELN', '2'))
NOCACHE = int(os.environ.get('NOCACHE', '0'))
OUTWAIT = int(os.environ.get('OUTWAIT', '0'))
SEGS = [int(x) for x in os.environ.get('SEGS', '012345')]
SKIPB = int(os.environ.get('SKIPB', '0'))
PADK = int(os.environ.get('PADK', '0'))
PREW = int(os.environ.get('PREW', '0'))
SP = float(os.environ.get('SP', '0'))
MINS = int(os.environ.get('MINS', '30'))
GA = int(os.environ.get('GA', '2'))
TRT = int(os.environ.get('TRT', '1'))
LP = int(os.environ.get('LP', '1'))
FA = 1664
LPN = int(os.environ.get('LPN', '2'))
G0 = int(os.environ.get('G0', '4'))
Q1 = int(os.environ.get('Q1', '704'))
TIE4 = int(os.environ.get('TIE4', '12'))
STAG = os.environ.get('STAG', 'w02,l0,n,n')
OCOLS = ((0, 512), (512, 128))
FSTEP = int(os.environ.get('FSTEP', '1'))
FOFF = int(os.environ.get('FOFF', '0'))
KORD = int(os.environ.get('KORD', '0'))
CW = int(os.environ.get('CW', '128'))
NP4 = int(os.environ.get('NP4', '4'))
LNT = [int(x) for x in os.environ.get('LNT', '0,1,2,3,4,5,18,22').split(',')]
OPQ = int(os.environ.get('OPQ', '1'))
RELOAD = int(os.environ.get('RELOAD', '0'))
REMP = os.environ.get('REMP', '653765376537')
KARA = int(os.environ.get('KARA', '1'))
UNR = int(os.environ.get('UNR', '2'))
HEAD = int(os.environ.get('HEAD', '250'))
TAIL = int(os.environ.get('TAIL', '450'))
DORDER = os.environ.get('DORDER', 'aHbU')
R1 = int(os.environ.get('R1', '64'))
R2 = int(os.environ.get('R2', '128'))
LEAD = int(os.environ.get('LEAD', '4'))
TS = int(os.environ.get('TS', '512'))
ONEPASS = int(os.environ.get('ONEPASS', '1'))
RSQ = int(os.environ.get('RSQ', '1'))
T2 = int(os.environ.get('T2', '512'))
EPS = 1e-5
_C0 = math.sqrt(2.0 / math.pi)
ALPHA = (_C0 * 0.044715) ** (1.0 / 3.0)
GC = _C0 / ALPHA
BETA = 0.5 / ALPHA
_fc = [int(x) for x in os.environ.get('FC', '1728').split(',')]
F_CHUNKS = tuple((sum(_fc[:i]), _fc[i]) for i in range(len(_fc)))
assert sum(_fc) == F

f32 = jnp.float32
bf16 = jnp.bfloat16
u32 = jnp.uint32
NTDIMS = (((1,), (1,)), ((), ()))


def _cos_table(m, scale):
    mm = jnp.abs(((m + 256) & 511) - 256)
    x = (128 - mm).astype(f32) * (1.0 / 128.0)
    x2 = x * x
    h = math.pi / 2
    p = -(h ** 7) / 5040 + x2 * ((h ** 9) / 362880 - x2 * (h ** 11) / 39916800)
    p = h + x2 * (-(h ** 3) / 6 + x2 * ((h ** 5) / 120 + x2 * p))
    return (x * scale) * p


def _dft_tables():
    shape = (16, 8, 128)
    n = lax.broadcasted_iota(jnp.int32, shape, 0)
    s = lax.broadcasted_iota(jnp.int32, shape, 1)
    l = lax.broadcasted_iota(jnp.int32, shape, 2)
    fw, fu, iv = [], [], []
    wv = l >> 4
    tu = (16 * W) * (wv // W) + (2 * W) * ((l >> 1) & 7) + 2 * (wv % W) + (l & 1)
    for e in range(2):
        r = 2 * s + e
        j = 8 * n + (r & 7)
        fw.append(_cos_table((4 * j + 1) * l + (r >> 3) * 128, 1.0))
        fu.append(_cos_table((4 * j + 1) * tu + (r >> 3) * 128, 1.0))
        b = 16 * (n >> 1) + r
        col = 128 * (n & 1) + l
        iv.append(_cos_table((4 * (col >> 1) + 1) * b + (col & 1) * 128, 1.0 / 128.0))
    pk = lambda xs: pltpu.bitcast(pltpu.pack_elementwise(xs, packed_dtype=bf16), f32)
    return pk(fw), pk(iv), pk(fu)


def _gelu2a(z):
    return z * (1.0 + jnp.tanh(z * (z * z + GC)))


def _rstd(ssd, scale):
    if RSQ == 0:
        r = lax.rsqrt(ssd * (1.0 / D) + EPS)
        return r if scale == 1.0 else r * scale
    return jnp.exp2(jnp.log(ssd + D * EPS) * (-0.5 / math.log(2.0)) + math.log2(scale * math.sqrt(D)))


def _center(x, scale=1.0):
    s1 = jnp.sum(x, axis=-1, keepdims=True)
    m = s1 * (1.0 / D)
    d = x - m
    if ONEPASS:
        ssd = jnp.maximum(jnp.sum(x * x, axis=-1, keepdims=True) - s1 * m, 0.0)
    else:
        ssd = jnp.sum(d * d, axis=-1, keepdims=True)
    return d, _rstd(ssd, scale)


def _conv(us, gs, a):
    acc = None
    for c in range(a + 1):
        p = us[c] * gs[a - c]
        acc = p if acc is None else acc + p
    return acc


_SA = (lambda a, b, c, d: a + d, lambda a, b, c, d: d, lambda a, b, c, d: c + d, lambda a, b, c, d: a,
       lambda a, b, c, d: a + b, lambda a, b, c, d: b - d, lambda a, b, c, d: c - a)
_SB = (lambda a, b, c, d: a + d, lambda a, b, c, d: c - a, lambda a, b, c, d: a, lambda a, b, c, d: b - d,
       lambda a, b, c, d: d, lambda a, b, c, d: c + d, lambda a, b, c, d: a + b)


_SC = (((0, 1), (3, 1)), ((0, 1), (2, 1)), ((2, 1), (3, -1)), ((1, 1), (3, 1)), ((0, -1), (1, 1)), ((0, 1),), ((3, 1),))
_SCL = (5, 4, 2, 6)


def _comb(m):
    m1, m4, m2, m3, m5, m7, m6 = m
    return (m1 + m4) + (m7 - m5), m3 + m5, m4 + m2, (m1 + (m3 - m2)) + m6


class Lazy:
    def __init__(self, terms):
        self.terms = terms

    def __add__(self, o):
        return Lazy(self.terms + o.terms)

    def __sub__(self, o):
        return Lazy(self.terms + [(-s_, r_, c_) for (s_, r_, c_) in o.terms])

    def shift(self, dr, dc):
        return Lazy([(s_, r_ + dr, c_ + dc) for (s_, r_, c_) in self.terms])

    def load(self, ref, rn, cn):
        ts = sorted(self.terms, key=lambda t: -t[0])
        v = [ref[pl.ds(r_, rn), pl.ds(c_, cn)] for (_, r_, c_) in ts]
        acc_ = v[0]
        for (s_, _, _), x in zip(ts[1:], v[1:]):
            acc_ = acc_ + x if s_ > 0 else acc_ - x
        return acc_.astype(bf16)


def _mult(x, n):
    return x if isinstance(x, int) else pl.multiple_of(x, n)


def _wt(ref, *idx):
    return pltpu.bitcast(ref[idx] if idx else ref[...], bf16)


def _kernel(q_hbm, k_hbm, v_hbm, sk_hbm, h_hbm, dd_hbm, w1_hbm, w2_hbm, w3_hbm, w4_hbm,
            c_hbm, wm_hbm, o_hbm,
            modb, qbuf, kbuf, vbuf, hbuf, w1, w2, w3, w4, wm, wmp, wmc, obuf,
            ub0, ub1, gb0, gb1, kb0, kb1, yb, xn, hh, h1, par, l4p_, gs_, w4s, w3s, w4o, sk_s, dd_s, c_s, zs, sems, osems):
    l4p = l4p_.at[0]
    ubs, gbs, kbs = (ub0, ub1), (gb0, gb1), (kb0, kb1)
    cp = pltpu.make_async_copy
    HS = S // 2

    def cp_h(j, c0, c1, sem):
        return cp(h_hbm.at[pl.ds(j * 128, 128), pl.ds(c0, c1 - c0)], hbuf.bitcast(bf16).at[j, :, pl.ds(c0, c1 - c0)], sem)

    def cp_kv(j, r0, r1, sem):
        r0, r1 = (r0 + 16 if r0 else 0), min(r1 + 16, S)
        lanes = pl.ds(j * 128, 128)
        return [cp(k_hbm.at[0, pl.ds(r0, r1 - r0), lanes], kbuf.bitcast(bf16).at[j, pl.ds(r0 + 16, r1 - r0), :], sem),
                cp(v_hbm.at[0, pl.ds(r0, r1 - r0), lanes], vbuf.bitcast(bf16).at[j, pl.ds(r0, r1 - r0), :], sem)]

    def cp_tile(j, i):
        sem = sems.at[2 * j + i]
        return [cp_h(j, i * HS, (i + 1) * HS, sem)] + cp_kv(j, i * HS, (i + 1) * HS, sem)

    cp_t0 = [[cp_h(0, 0, S, sems.at[0])], cp_kv(0, 0, 1024, sems.at[1]), cp_kv(0, 1024, 1536, sems.at[20]),
             cp_kv(0, 1536, S, sems.at[21])]

    def cp_wm(i):
        return cp(wm_hbm.at[:, pl.ds(i * WMA, WMA)], wm.bitcast(bf16).at[i], sems.at[10 + i])

    cp_wmp = cp(wm_hbm.at[:, pl.ds(2 * WMA, WMP)], wmp.bitcast(bf16), sems.at[13])
    cp_wmc = cp(wm_hbm.at[:, pl.ds(2 * WMA + WMP, WMC)], wmc.bitcast(bf16), sems.at[12])
    cp_q = [cp(q_hbm.at[0, pl.ds(r0, r1 - r0), :], qbuf.at[pl.ds(r0, r1 - r0), :], sems.at[sm])
            for sm, r0, r1 in ((13, 0, Q0), (16, Q0, Q1), (12, Q1, S))]
    cp_w = [cp(s_, d_.bitcast(bf16).at[pl.ds(0, s_.shape[0]), :], sems.at[sm])
            for sm, s_, d_ in ((15, w1_hbm, w1), (16, w2_hbm, w2), (14, w3_hbm, w3), (14, w4_hbm, w4))]
    cp_s = [cp(sk_hbm, sk_s, sems.at[19]), cp(dd_hbm, dd_s, sems.at[19]), cp(c_hbm, c_s, sems.at[19])]
    order = list(cp_s)
    for grp in cp_t0:
        order += grp
    for j in range(1, NT):
        order += cp_tile(j, 0) + cp_tile(j, 1)
    order += [cp_wm(0), cp_wm(1), cp_wmp, cp_q[0], cp_w[0], cp_w[1], cp_q[1], cp_q[2], cp_wmc, cp_w[2], cp_w[3]]
    for c_ in order:
        c_.start()

    with jax.named_scope("init"):
        fw_t, iv_t, fu_t = _dft_tables()
        for kb in kbs:
            kb[pl.ds(KOFF, 16)] = fw_t
            kb[pl.ds(KOFF + 16, 16)] = iv_t
            kb[pl.ds(KOFF + 32, 16)] = fu_t
            kb[pl.ds(0, NG * 3)] = jnp.zeros((NG * 3, 8, 128), f32)
        zeros = jnp.zeros((8, 128), f32)
        w4[pl.ds(F // 2, 32), :] = jnp.zeros((32, D), u32)
        for j in range(NT):
            kbuf[j, pl.ds(0, 8), :] = jnp.zeros((8, 128), u32)
            kbuf[j, pl.ds(8 + HS, 8), :] = jnp.zeros((8, 128), u32)
            vbuf[j, pl.ds(HS, 8), :] = jnp.zeros((8, 128), u32)
        for j in range(NT):
            h1[j, pl.ds(0, 8), :] = zeros
            h1[j, pl.ds(S + 8, 8), :] = zeros
        for c_ in cp_s:
            c_.wait()
        par[pl.ds(0, 4), :] = sk_s[...].astype(f32)
        par[pl.ds(8, 8), :] = jnp.broadcast_to(dd_s[...].astype(f32).reshape(1, D), (8, D))
        cv = c_s[...].astype(f32)
        sc = jnp.broadcast_to(cv * jax.nn.sigmoid(cv), (8, D))
        scp = pltpu.bitcast(pltpu.pack_elementwise([sc, sc], packed_dtype=bf16), f32)
        for j in range(NT):
            kb0[KOFF + 48 + j] = scp[:, 128 * j:128 * (j + 1)]
            kb1[KOFF + 48 + j] = scp[:, 128 * j:128 * (j + 1)]

    def mkb(i, unr, off, cache):
        def b(stride, extra=0, z=None):
            if isinstance(i, int):
                return (i * unr + off) * stride + extra
            key = (unr * stride, z)
            if key not in cache or NOCACHE:
                base = pl.multiple_of(i * (unr * stride), unr * stride)
                cache[key] = base if z is None else base + (i >> z)
            return cache[key] + (off * stride + extra)
        return b

    def dot_h(j, b, lhs):
        gb = gbs[j % 2]
        hc = hbuf[j, :, pl.ds(_mult(b(512), 512), 512)]
        rhs_t = jnp.concatenate([hc[:, C * cc:C * (cc + 1)] for cc in range(4)], axis=0)
        g = lax.dot_general(lhs, pltpu.bitcast(rhs_t, bf16), NTDIMS, preferred_element_type=f32)
        for rg in range(2 * NG):
            for cc in range(4):
                gb[b(4, cc + rg * NC)] = g[8 * rg:8 * rg + 8, 128 * cc:128 * cc + 128]

    def dot_u(j, b, lhs):
        ub = ubs[j % 2]
        taps = [par[pl.ds(t, 1), pl.ds(j * 128, 128)] for t in range(4)]
        unp = lambda w_, e: pltpu.unpack_elementwise(w_, index=e, packed_dtype=bf16, unpacked_dtype=f32)
        cols = []
        for cc in range(4):
            words = []
            for blk in range(8 // W):
                w0 = 64 * cc + 8 * W * blk
                kw = {m: kbuf[j, pl.ds(b(256, 8 + w0 + m), 8, stride=W), :] for m in range(-2, W)}
                kk = {2 * m + e: unp(kw[m], e) for m in range(-2, W) for e in range(2) if 2 * m + e >= -3}
                for m in range(W):
                    vw = vbuf[j, pl.ds(b(256, w0 + m), 8, stride=W), :]
                    pair = []
                    for e in range(2):
                        n = 2 * m + e
                        ks = kk[n] * taps[0] + kk[n - 1] * taps[1] + kk[n - 2] * taps[2] + kk[n - 3] * taps[3]
                        pair.append(ks * unp(vw, e))
                    words.append(pltpu.pack_elementwise(pair, packed_dtype=bf16))
            cols.append(jnp.concatenate(words, axis=0))
        rhs = pltpu.bitcast(jnp.concatenate(cols, axis=1), bf16)
        u = jnp.dot(lhs, rhs, preferred_element_type=f32)
        for rg in range(2 * NG):
            for cc in range(4):
                ub[b(4, cc + rg * NC)] = u[8 * rg:8 * rg + 8, 128 * cc:128 * cc + 128]

    def dot_i(j, b, half, lhs):
        kb = kbs[j % 2]
        cols = [[], []]
        for gi in range(NG):
            prev = None
            for cc in range(-1, 2):
                k0, k1, k2 = [kb[b(4 * NG * 3, ((2 * half + cc + 1) * NG + gi) * 3 + t)] for t in range(3)]
                re, im = k0 - k2, k0 + k1
                if prev is not None:
                    cols[cc].append(pltpu.pack_elementwise([re - prev[1], im + prev[0]], packed_dtype=bf16))
                prev = (re, im)
        rhs = jnp.concatenate([jnp.concatenate(c_, axis=0) for c_ in cols], axis=1)
        y = jnp.dot(lhs, pltpu.bitcast(rhs, bf16), preferred_element_type=f32)
        for cc in range(2):
            yb[j, pl.ds(b(512, (2 * half + cc) * C), C), :] = y[:, 128 * cc:128 * cc + 128]

    def gen_m(j, kb, b, ng):
        ub, gb = ubs[j % 2], gbs[j % 2]
        for s in range(ng):
            for t in range(3):
                z = 8 + t
                re = lambda ref, c: ref[b(2 * NC, 2 * s * NC + c, z)]
                im = lambda ref, c: ref[b(2 * NC, (2 * s + 1) * NC + c, z)]
                gre = [re(gb, c) for c in range(NC)]
                if t == 0:
                    us = [re(ub, c) + im(ub, c) for c in range(NC)]
                    gs = gre
                elif t == 1:
                    us = [re(ub, c) for c in range(NC)]
                    gs = [im(gb, c) - gre[c] for c in range(NC)]
                else:
                    us = [im(ub, c) for c in range(NC)]
                    gs = [im(gb, c) + gre[c] for c in range(NC)]

                def st(a, val):
                    kb[b(3, ((a + 1) * NG + s) * 3 + t)] = val
                if not KARA:
                    for a in range(NC):
                        st(a, _conv(us, gs, a))
                        yield 2 * a + 2
                    continue
                ue, uo, ge, go = us[0::2], us[1::2], gs[0::2], gs[1::2]
                if KORD == 1:
                    usum = [x + y for x, y in zip(ue, uo)]
                    gsum = [x + y for x, y in zip(ge, go)]
                    poo = _conv(uo, go, NC // 2 - 1)
                    for a in reversed(range(NC // 2)):
                        pee = _conv(ue, ge, a)
                        pss = _conv(usum, gsum, a)
                        st(2 * a + 1, pss - pee - poo)
                        poo = _conv(uo, go, a - 1) if a else None
                        st(2 * a, pee + poo if a else pee)
                        yield 3 * (2 * a + 1) + (37 if a == NC // 2 - 1 else 3)
                    continue
                usum = [x + y for x, y in zip(ue, uo)]
                gsum = [x + y for x, y in zip(ge, go)]
                poo_prev = None
                for a in range(NC // 2):
                    pee = _conv(ue, ge, a)
                    poo = _conv(uo, go, a)
                    pss = _conv(usum, gsum, a)
                    st(2 * a, pee if poo_prev is None else pee + poo_prev)
                    st(2 * a + 1, pss - pee - poo)
                    poo_prev = poo
                    yield 3 * (2 * a + 1) + 7

    def add_d(j):
        gb = gbs[j % 2]
        dvec = par[pl.ds(8, 8), pl.ds(j * 128, 128)]
        for gi in range(NG):
            gb[2 * gi * NC] = gb[2 * gi * NC] + dvec

    def sc_lhs():
        return pltpu.bitcast(jnp.concatenate([kb0[KOFF + 48 + j] for j in range(NT)], axis=1), bf16)

    def dot_m(i, t0, nt, rows):
        m = None
        for kt in range(NT):
            p = jnp.dot(pltpu.bitcast(rows[kt], bf16), _wt(wm, i, pl.ds(64 * kt, 64), pl.ds(128 * t0, 128 * nt)),
                        preferred_element_type=f32)
            m = p if m is None else m + p
        for t in range(nt):
            modb[i * (WMA // 128) + (t0 + t)] = m[0:8, 128 * t:128 * (t + 1)]

    def inv_lhs(tbl, n):
        return jnp.concatenate([tbl[KOFF + 16 + 2 * n], tbl[KOFF + 17 + 2 * n]], axis=1)

    def dot_k(kb, kt, bt, lhs):
        cols = [[] for _ in range(4)]
        for gi in range(8 * kt, 8 * kt + 8):
            prev = None
            for cc in range(-1, 4):
                k0, k1, k2 = [kb[((4 * bt + cc + 1) * NG + gi) * 3 + t] for t in range(3)]
                re, im = k0 - k2, k0 + k1
                if prev is not None:
                    cols[cc].append(pltpu.pack_elementwise([re - prev[1], im + prev[0]], packed_dtype=bf16))
                prev = (re, im)
        rhs = jnp.concatenate([jnp.concatenate(c_, axis=0) for c_ in cols], axis=1)
        y = jnp.dot(lhs, pltpu.bitcast(rhs, bf16), preferred_element_type=f32)
        for cc in range(4):
            rows = pl.ds((4 * bt + cc) * C, C)
            yc = y[:, 128 * cc:128 * cc + 128]
            yb[NT - 1, rows, :] = yc if kt == 0 else yb[NT - 1, rows, :] + yc

    PRE = dict(H=0, U=672 + 96 // W, a=192, b=192, m=0, k=176)
    POST = dict(H=0, U=0, a=4, b=4, m=2, k=0)
    NST = dict(H=16, U=16, a=8, b=8, m=5, k=8)
    GCOST = 3 * (248 if KARA else 272)

    def a_block(dots, mg=None, ng=0, tbl=kb0):
        native, dur = [], []
        for idx, (k_, _) in enumerate(dots):
            nxt = PRE[dots[idx + 1][0]] if idx + 1 < len(dots) else 0
            d_ = 2.0 if k_ == 'm' else 1.0
            native += [nxt / NST[k_] + POST[k_] * d_] * NST[k_]
            dur += [d_] * NST[k_]
        if mg is not None and dots:
            head = max(HEAD - PRE[dots[0][0]], 0)
            mtot = GCOST * ng - TAIL - head
            lvl = (mtot + sum(native)) / sum(dur)
            want = [max(lvl * d_ - x, 0.0) for x, d_ in zip(native, dur)]
            scale = mtot / sum(want)
            cum, tgt = [head], head
            for w_ in want:
                tgt += w_ * scale
                cum.append(tgt)
        done = 0.0
        step = 0
        for (k_, fn) in dots:
            rows = []
            for n in range(NST[k_]):
                if mg is not None and (n % FSTEP == 0 or k_ == 'm'):
                    while done < cum[min(step + FOFF, len(cum) - 1)]:
                        done += next(mg)
                step += 1
                if k_ in 'HU':
                    rows.append(tbl[KOFF + n + (32 if k_ == 'U' else 0)])
                elif k_ in 'ab':
                    rows.append(inv_lhs(tbl, n))
                elif k_ == 'k':
                    rows.append(tbl[KOFF + 16 + 2 * n])
                else:
                    rows.append(tbl[KOFF + 48 + n])
            fn(rows if k_ == 'm' else pltpu.bitcast(jnp.concatenate(rows, axis=0), bf16))
        if mg is not None:
            for _ in mg:
                pass

    def fdot(k_, j, b):
        if k_ == 'H':
            return (k_, lambda lhs: dot_h(j, b, lhs))
        if k_ == 'U':
            return (k_, lambda lhs: dot_u(j, b, lhs))
        return (k_, lambda lhs: dot_i(j, b, 0 if k_ == 'a' else 1, lhs))

    def wait_all(cps):
        for c_ in cps:
            c_.wait()

    def a_loop(jf, jm, ji, g0, ng):
        kinds = [k_ for k_ in DORDER if k_ in 'HU' or ji is not None]

        def body(i, carry):
            cache = {}
            zs[i] = 0
            dots = [fdot(k_, jf if k_ in 'HU' else ji, mkb(i, 2, s_, cache)) for s_ in range(2) for k_ in kinds]
            a_block(dots, gen_m(jm, kbs[jm % 2], mkb(i, ng, g0, cache), ng), ng, kbs[jm % 2])

            @pl.when(i == 0)
            def _():
                wait_all(cp_tile(jf, 1))
            return carry
        wait_all(cp_tile(jf, 0))
        lax.fori_loop(0, 2, body, 0)
        add_d(jf)

    sb_ = lambda bt: mkb(0, 1, bt, None)
    if SKIPA:
        a_block = lambda *a, **k: None
    with jax.named_scope("A_seg0"):
        wait_all(cp_t0[0])
        a_block([fdot('H', 0, sb_(bt)) for bt in range(4)])
        add_d(0)
        wait_all(cp_t0[1])
        a_block([fdot('U', 0, sb_(bt)) for bt in range(2)])
        for bt in (2, 3):
            wait_all(cp_t0[bt])
            a_block([fdot('U', 0, sb_(bt))])
    with jax.named_scope("A_m0"):
        def body_m0(i, carry):
            a_block([], gen_m(0, kb0, mkb(i, G0 // 2, 0, {}), G0 // 2))
            return carry
        if G0:
            lax.fori_loop(0, 2, body_m0, 0)
    for seg in range(1, NT):
        with jax.named_scope(f"A_seg{seg}"):
            if seg == 1:
                a_loop(1, 0, None, G0, (NG - G0) // 2)
            else:
                a_loop(seg, seg - 1, seg - 2, 0, 8)

    def mods(i):
        return [('m', lambda rows, t0=t0, nt=nt: dot_m(i, t0, nt, rows)) for (t0, nt) in ((0, 4), (4, 4), (8, 2))]

    with jax.named_scope("A_seg5a"):
        cp_wm(0).wait()
        zz = zs[1]

        @pl.when(zz == 0)
        def _():
            dots = [fdot(k_, NT - 2, sb_(bt)) for bt in range(4) for k_ in 'ab']
            mm = mods(0)
            dots = [mm[0]] + dots[0:2] + [mm[1]] + dots[2:4] + [mm[2]] + dots[4:]
            a_block(dots, gen_m(NT - 1, kb0, mkb(zz, 8, 0, {}), 8), 8, kb0)
    with jax.named_scope("A_seg5b"):
        cp_wm(1).wait()

        @pl.when(zz == 0)
        def _():
            dots = [('k', lambda lhs, bt=bt: dot_k(kb0, 0, bt, lhs)) for bt in range(4)]
            mm = mods(1)
            dots = [mm[0], dots[0], mm[1], dots[1], mm[2]] + dots[2:]
            a_block(dots, gen_m(NT - 1, kb1, mkb(zz, 8, 8, {}), 8), 8, kb1)

    def inv_last(bt):
        lhs = pltpu.bitcast(jnp.concatenate([kb0[KOFF + 17 + 2 * n] for n in range(8)], axis=0), bf16)
        dot_k(kb1, 1, bt, lhs)

    def modrow(k_):
        return jnp.concatenate([modb[NT * k_ + j] for j in range(NT)], axis=1)

    R = R1
    GP = R // 8

    def ln_chain(p):
        r = p * R
        pa, pb, pc, ps = [par[pl.ds(16 + 8 * t, 8), :][None] for t in range(4)]
        g3 = lambda x: x.reshape(GP, 8, D)
        q = g3(qbuf[pl.ds(r, R), :].astype(f32))
        d1, r1 = _center(q)
        y = g3(jnp.concatenate([yb[j, pl.ds(r, R), :] for j in range(NT)], axis=1))
        x = q + ((d1 * r1) * pa + pb) * y
        xn[pl.ds(r, R), :] = x.reshape(R, D)
        d2, r2 = _center(x)
        h = (d2 * r2) * pc + ps
        hh[pl.ds(r, R), :] = h.reshape(R, D)
        d3, r3 = _center(h, ALPHA)
        return (d3 * r3).reshape(R, D)

    def tie(w_, vs):
        t_ = pltpu.bitcast(vs[0], u32)
        for v_ in vs[1:]:
            t_ = t_ | pltpu.bitcast(v_, u32)
        return w_ | (t_ & kbuf[0, pl.ds(0, 8), :])

    def tied(wref, ties):
        if not ties:
            return _wt(wref)
        rbs = sorted({8 * (t % 5) + rb for (t, rb) in ties})
        rows, pos = [], 0
        for rb in rbs:
            if rb > pos:
                rows.append(wref[pl.ds(8 * pos, 8 * (rb - pos)), :])
            blk = []
            for n in range(NT):
                w_ = wref[pl.ds(8 * rb, 8), pl.ds(128 * n, 128)]
                vs = ties.get((5 * n + rb // 8, rb % 8))
                blk.append(tie(w_, vs) if vs else w_)
            rows.append(jnp.concatenate(blk, axis=1))
            pos = rb + 1
        if pos < 40:
            rows.append(wref[pl.ds(8 * pos, 8 * (40 - pos)), :])
        return pltpu.bitcast(jnp.concatenate(rows, axis=0), bf16)

    def w1_dot(p, l3, ties, fresh):
        if fresh and STAG:
            grp = lambda g: l3[8 * g:8 * g + 8, 0:128]
            lt = {}
            for pr, spec in enumerate(STAG.split(',')):
                vs = [grp(2 * pr), grp(2 * pr + 1)]
                if spec[0] == 'w':
                    ties.setdefault((int(spec[1]), int(spec[2])), []).extend(vs)
                elif spec[0] == 'l':
                    lt.setdefault(int(spec[1]), []).extend(vs)
            for pr, vs in lt.items():
                x = pltpu.bitcast(tie(pltpu.bitcast(l3[16 * pr:16 * pr + 8, 128:256], u32), vs), f32)
                mid = jnp.concatenate([l3[16 * pr:16 * pr + 8, 0:128], x, l3[16 * pr:16 * pr + 8, 256:]], axis=1)
                l3 = jnp.concatenate(([l3[:16 * pr]] if pr else []) + [mid, l3[16 * pr + 8:]], axis=0)
        z = jnp.dot(l3.astype(bf16), tied(w1, ties), preferred_element_type=f32)
        g = _gelu2a(z)
        for j in range(NT):
            h1[j, pl.ds(p * R + 8, R), :] = g[:, j * 128:(j + 1) * 128]

    def w2_dot(p, ties):
        r = p * R
        lane = lax.broadcasted_iota(jnp.int32, (R, 128), 1)

        def ld(j, off):
            return h1[j, pl.ds(r + 8 + off, R), :]
        tiles = [
            ld(0, -1),
            jnp.where(lane < 32, ld(1, -1), ld(1, 1)),
            jnp.where(lane < 64, ld(2, 1), ld(2, -2)),
            jnp.where(lane < 96, ld(3, -2), ld(3, 2)),
            ld(4, 2),
        ]
        hs = jnp.concatenate(tiles, axis=1).astype(bf16)
        x1 = hh[pl.ds(r, R), :] + jnp.dot(hs, tied(w2, ties), preferred_element_type=f32) * BETA
        hh[pl.ds(r, R), :] = x1

    l3s = {}

    def ln4(r, n):
        d4, r4 = _center(hh[pl.ds(r, n), :], ALPHA)
        return d4 * r4

    def run_block(dots, pre4=False):
        for d_, (k_, p) in enumerate(dots):
            ties = {}
            e = d_ - (len(dots) - NP4)
            RP = TS // NP4
            if pre4 and e >= 0:
                nx = ln4(e * RP, RP)
                l4p[pl.ds(e * RP, RP), :] = nx
                ties[(TIE4, 7)] = [nx[8 * g:8 * g + 8, 0:128] for g in range(RP // 8)]
            if k_ == 1:
                fresh = p not in l3s
                w1_dot(p, ln_chain(p) if fresh else l3s.pop(p), ties, fresh)
            elif k_ == 2:
                w2_dot(p, ties)
            else:
                par[pl.ds(48, 8), :] = jnp.dot(sc_lhs(), _wt(wmc), preferred_element_type=f32)[0:8]

    with jax.named_scope("P1"):
        cp_wmp.wait()
        cp_q[0].wait()
        mp = jnp.dot(sc_lhs(), _wt(wmp), preferred_element_type=f32)
        for t in range(WMP // 128):
            modb[2 * WMA // 128 + t] = mp[0:8, 128 * t:128 * (t + 1)]
        sa, ca, ga, sb, cb = [modrow(k_) for k_ in range(5)]
        par[pl.ds(16, 8), :] = ga * (1.0 + ca)
        par[pl.ds(24, 8), :] = ga * sa
        par[pl.ds(32, 8), :] = 1.0 + cb
        par[pl.ds(40, 8), :] = sb
        for bt in range(4):
            inv_last(bt)
        for p in range(PRELN):
            l3s[p] = ln_chain(p)
    with jax.named_scope("w1wait"):
        cp_w[0].wait()
    p1, p2 = N2, 0
    with jax.named_scope("P2"):
        run_block([(1, p) for p in range(N2)])
    with jax.named_scope("w2wait"):
        wait_all([cp_w[1], cp_q[1]])

    def plan(lim1, hold):
        nonlocal p1, p2
        dots = []
        while p2 < p1 - 1 and len(dots) < 2:
            dots.append((2, p2))
            p2 += 1
        last2 = lim1 if lim1 == S // R else lim1 - 1 - hold
        while p2 < last2 or p1 < lim1:
            while p1 < lim1 and (p1 - p2 < LEAD or p2 >= last2):
                dots.append((1, p1))
                p1 += 1
            if p2 < last2:
                dots.append((2, p2))
                p2 += 1
        return dots

    with jax.named_scope("P4"):
        run_block(plan(Q1 // R, 2))
    with jax.named_scope("q2wait"):
        wait_all([cp_q[2], cp_wmc])
    with jax.named_scope("P5"):
        dots = plan(S // R, 0)
        run_block(dots[:2] + [(3, 0)] + dots[2:], pre4=True)

    H2 = TS // 2
    OUTS = ((0, H2, 512, 128), (H2, H2, 0, 256), (0, H2, 256, 256), (0, H2, 0, 256), (H2, H2, 256, 256), (H2, H2, 512, 128))

    def out_copy(r, r0, rn, c0, cn):
        rows = pl.ds(_mult(r + r0, H2), rn)
        return cp(obuf.at[rows, pl.ds(c0, cn)], o_hbm.at[0, rows, pl.ds(c0, cn)], osems.at[0])

    def wsum(x, y, sign):
        unp = lambda w_, e: pltpu.unpack_elementwise(w_, index=e, packed_dtype=bf16, unpacked_dtype=f32)
        return pltpu.pack_elementwise([unp(x, e) + unp(y, e) if sign > 0 else unp(x, e) - unp(y, e) for e in range(2)],
                                      packed_dtype=bf16)

    def strassen_lhs(a11, a12, a21, a22):
        c = lambda x: x.astype(bf16)
        return (c(a11 + a22), c(a21 + a22), c(a11), c(a22), c(a11 + a12), c(a21 - a11), c(a12 - a22))

    def strassen(ops, b11, b12, b21, b22, mm, ties=None):
        def tw(k_, w_):
            if not ties or k_ not in ties:
                return w_
            return jnp.concatenate([tie(w_[0:8], ties[k_]), w_[8:]], axis=0)
        m1 = mm(ops[0], tw(0, wsum(b11, b22, 1)))
        m4 = mm(ops[3], tw(1, wsum(b21, b11, -1)))
        m2 = mm(ops[1], tw(2, b11))
        m3 = mm(ops[2], tw(3, wsum(b12, b22, -1)))
        m5 = mm(ops[4], tw(4, b22))
        m7 = mm(ops[6], tw(5, wsum(b21, b22, 1)))
        m6 = mm(ops[5], tw(6, wsum(b11, b12, 1)))
        return (m1 + m4) + (m7 - m5), m3 + m5, m4 + m2, (m1 + (m3 - m2)) + m6

    mm_nt = lambda x, w_: lax.dot_general(x, pltpu.bitcast(w_, bf16), NTDIMS, preferred_element_type=f32)
    mm_nn = lambda x, w_: jnp.dot(x, pltpu.bitcast(w_, bf16), preferred_element_type=f32)

    def b2_step(i):
        gbv = par[pl.ds(48, 8), :]
        nsub = T2 // TS
        for sub in range(nsub):
            r = pl.multiple_of(pl.multiple_of(i * T2, T2) + sub * TS, TS)
            gs = gs_.at[i >> 8]
            l4 = l4p[...] if sub == 0 else ln4(r, TS)
            lb = l4.astype(bf16)
            zt = lax.dot_general(_wt(w3, pl.ds(832, 32), slice(None)), lb, NTDIMS, preferred_element_type=f32)
            g12 = _gelu2a(mm_nt(lb, w3[pl.ds(768, 64), :]))
            gt = jnp.concatenate([_gelu2a(zt), jnp.zeros((64, TS), f32)], axis=0).T
            gs[:, pl.ds(0, 128)] = g12
            gs[:, pl.ds(896, 128)] = gt
            lrs = [l4[:H2, 512:640].astype(bf16), l4[H2:, 512:640].astype(bf16)]
            Q = H2 // 2
            ab = [Lazy([(1, r_, c_)]) for (r_, c_) in ((0, 0), (0, 256), (H2, 0), (H2, 256))]
            opsA = {}
            rn_ = pl.multiple_of(jnp.minimum(i + 1, S // T2 - 1) * T2, T2)
            RP = TS // len(LNT)
            l4n = l4p
            for t in range(3):
                cq, left = [None] * 4, [5, 3, 3, 5]

                def add(k_, x, sg=1):
                    cq[k_] = x if cq[k_] is None else cq[k_] + x if sg > 0 else cq[k_] - x
                    left[k_] -= 1
                    if left[k_] == 0:
                        gg = _gelu2a(cq[k_])
                        for n2 in range(2):
                            gs[pl.ds(H2 * (k_ // 2), H2), pl.ds(128 + 896 * (k_ % 2) + 128 * (t + 3 * n2), 128)] = gg[:, 128 * n2:128 * (n2 + 1)]

                def rem(k_):
                    wr = jnp.concatenate([w3[pl.ds(64 * (t + 3 * (2 * (k_ % 2) + n2)), 64), pl.ds(512, 128)] for n2 in range(2)], axis=0)
                    add(k_, mm_nt(lrs[k_ // 2], wr))
                for p_ in range(8):
                    for k_ in (2, 1, 0, 3):
                        if int(REMP[4 * t + k_]) == p_:
                            rem(k_)
                    if p_ == 7:
                        break
                    a_ = _SA[p_](*ab)
                    sub_ = (a_, a_.shift(0, 128), a_.shift(Q, 0), a_.shift(Q, 128))
                    pr = []
                    for q_ in range(7):
                        n = 7 * p_ + q_
                        if n not in opsA or RELOAD:
                            opsA[n] = _SA[q_](*sub_).load(l4p_.at[(i + 4 * p_ + 32 * t) >> (9 + q_)] if RELOAD else l4p, Q, 128)
                        w_ = w3s[n, pl.ds(64 * t, 64), :]
                        pr.append(mm_nt(opsA[n], w_))
                    c11, c12, c21, c22 = _comb(pr)
                    m_ = jnp.concatenate([jnp.concatenate([c11, c12], axis=1), jnp.concatenate([c21, c22], axis=1)], axis=0)
                    for k_, sg in _SC[p_]:
                        add(k_, m_, sg)
            kord = [0, 896] + [o_ for c in (0, 3, 1, 4, 2, 5) for o_ in (128 + 128 * c, 1024 + 128 * c)]
            wrow = lambda o_: 768 if o_ == 0 else 832 if o_ == 896 else (o_ - 128) // 2 if o_ < 896 else 384 + (o_ - 1024) // 2
            wl = jnp.concatenate([w4[pl.ds(wrow(o_), 64), pl.ds(512, 128)] for o_ in kord], axis=0)
            gk = lambda r0: jnp.concatenate([gs[pl.ds(r0, H2), pl.ds(o_, 128)] for o_ in kord], axis=1).astype(bf16)
            acc_t = mm_nn(gk(0), wl)
            ties = {}
            for e, k_ in enumerate(LNT):
                nx = ln4(pl.multiple_of(rn_ + e * RP, RP), RP)
                l4n[pl.ds(e * RP, RP), :] = nx
                ties[k_] = [nx[8 * gi:8 * gi + 8, 0:128] for gi in range(RP // 8)]
            Q = H2 // 2

            blocks = [Lazy([(1, r_, c_)]) for (r_, c_) in ((0, 0), (0, 896), (H2, 0), (H2, 896))]
            ms = []
            for p_ in range(7):
                a_ = _SA[p_](*blocks)
                wo = w4o[p_]
                if p_ in ties:
                    wo = jnp.concatenate([jnp.concatenate([tie(wo[0:8, 0:128], ties[p_]), wo[0:8, 128:]], axis=1), wo[8:]], axis=0)
                m_ = mm_nn(a_.load(gs, H2, 128), wo)
                sub_ = (a_.shift(0, 128), a_.shift(0, 512), a_.shift(Q, 128), a_.shift(Q, 512))
                gref = lambda q_: gs_.at[(i + 4 * p_) >> (9 + q_)] if OPQ else gs
                c11, c12, c21, c22 = _comb([mm_nn(_SA[q_](*sub_).load(gref(q_), Q, 384), w4s[7 * p_ + q_]) for q_ in range(7)])
                ms.append(m_ + jnp.concatenate([jnp.concatenate([c11, c12], axis=1), jnp.concatenate([c21, c22], axis=1)], axis=0))
            c11, c12, c21, c22 = _comb(ms)
            for k_ in ties:
                if k_ >= 10:
                    o_ = 64 * (k_ - 10)
                    wl = jnp.concatenate([wl[:o_], tie(wl[o_:o_ + 8], ties[k_]), wl[o_ + 8:]], axis=0)
            accs = (acc_t, c21, c12, c11, c22, mm_nn(gk(H2), wl))
            for (r0, rn, c0, cn), ac in zip(OUTS, accs):
                rows, cols = pl.ds(_mult(r + r0, H2), rn), pl.ds(c0, cn)
                g3 = lambda x: x.reshape(rn // 8, 8, cn)
                out = g3(xn[rows, cols]) + gbv[None, :, c0:c0 + cn] * g3(hh[rows, cols] + BETA * ac)
                obuf[rows, cols] = out.reshape(rn, cn).astype(bf16)
                out_copy(r, r0, rn, c0, cn).start()

    wait_all([cp_w[2], cp_w[3]])

    def prep_w4(t, carry):
        unp = lambda w_, e: pltpu.unpack_elementwise(w_, index=e, packed_dtype=bf16, unpacked_dtype=f32)
        pk = lambda xs: pltpu.pack_elementwise(xs, packed_dtype=bf16)
        r0 = pl.multiple_of(t * 8, 8)
        raw = [[w4[pl.ds(r0 + 192 * kq, 8), pl.ds(128 * nq, 128)] for nq in range(4)] for kq in range(4)]
        for p_ in range(7):
            l1 = [[_SB[p_](*[unp(raw[2 * hk + k2][2 * hn + n2], e) for hk in range(2) for hn in range(2)])
                   for k2 in range(2) for n2 in range(2)] for e in range(2)]
            for q_ in range(7):
                w4s[7 * p_ + q_, pl.ds(r0, 8), :] = pk([_SB[q_](*l1[e]) for e in range(2)])
        raw = [[w3[pl.ds(r0 + 192 * nq, 8), pl.ds(128 * kq, 128)] for nq in range(4)] for kq in range(4)]
        for p_ in range(7):
            l1 = [[_SB[p_](*[unp(raw[2 * hk + k2][2 * hn + n2], e) for hk in range(2) for hn in range(2)])
                   for k2 in range(2) for n2 in range(2)] for e in range(2)]
            for q_ in range(7):
                w3s[7 * p_ + q_, pl.ds(r0, 8), :] = pk([_SB[q_](*l1[e]) for e in range(2)])
        return carry

    with jax.named_scope("prep"):
        lax.fori_loop(0, 24, prep_w4, 0)
        unp = lambda w_, e: pltpu.unpack_elementwise(w_, index=e, packed_dtype=bf16, unpacked_dtype=f32)
        bl = [w4[pl.ds(lo, 64), pl.ds(c0, 256)] for lo in (768, 832) for c0 in (0, 256)]
        for p_ in range(7):
            w4o[p_] = pltpu.pack_elementwise([_SB[p_](*[unp(x, e) for x in bl]) for e in range(2)], packed_dtype=bf16)
    with jax.named_scope("BII"):
        lax.fori_loop(0, S // T2, lambda i, c: (b2_step(i), c)[1], 0)
    with jax.named_scope("out_wait"):
        for i in range(S // TS):
            for o_ in OUTS:
                out_copy(i * TS, *o_).wait()


@jax.jit
def pallas_adaLN_cond__ssm_conv_h3__mixer_s_mlp__prompt_kernel(
    A_q, A_k, A_v, A_shift_k, A_ssm_k, A_ssm_D, B_x, B_w1, B_w2, B_w3, B_w4, c, w_mod,
):
    del B_x
    hbm = pl.BlockSpec(memory_space=pltpu.MemorySpace.HBM)
    return pl.pallas_call(
        _kernel,
        out_shape=jax.ShapeDtypeStruct((1, S, D), bf16),
        in_specs=[hbm] * 12,
        out_specs=hbm,
        scratch_shapes=[
            pltpu.VMEM((27, 8, 128), f32),
            pltpu.VMEM((S + 16 * int(os.environ.get('PADF', '0')), D), bf16),
            pltpu.VMEM((NT, 32 + S // 2, 128), u32),
            pltpu.VMEM((NT, 32 + S // 2, 128), u32),
            pltpu.VMEM((NT, 64, S), u32),
            pltpu.VMEM((D // 2, D), u32),
            pltpu.VMEM((D // 2, D), u32),
            pltpu.VMEM((F // 2, D), u32),
            pltpu.VMEM((896, D), u32),
            pltpu.VMEM((2, D // 2, WMA), u32),
            pltpu.VMEM((D // 2, WMP), u32),
            pltpu.VMEM((D // 2, WMC), u32),
            pltpu.VMEM((S, D), bf16),
            pltpu.VMEM((NG * 2 * NC, 8, 128), f32),
            pltpu.VMEM((NG * 2 * NC, 8, 128), f32),
            pltpu.VMEM((NG * 2 * NC, 8, 128), f32),
            pltpu.VMEM((NG * 2 * NC, 8, 128), f32),
            pltpu.VMEM((KOFF + 56 + PADK, 8, 128), f32),
            pltpu.VMEM((KOFF + 56 + PADK, 8, 128), f32),
            pltpu.VMEM((NT, S, 128), f32),
            pltpu.VMEM((S, D), f32),
            pltpu.VMEM((S, D), f32),
            pltpu.VMEM((NT, S + 32, 128), f32),
            pltpu.VMEM((64, D), f32),
            pltpu.VMEM((1, TS, D), f32),
            pltpu.VMEM((1, TS, 1792), f32),
            pltpu.VMEM((49, 192, 128), u32),
            pltpu.VMEM((49, 192, 128), u32),
            pltpu.VMEM((7, 64, 256), u32),
            pltpu.VMEM((4, D), bf16),
            pltpu.VMEM((D,), bf16),
            pltpu.VMEM((1, D), bf16),
            pltpu.SMEM((2,), jnp.int32),
            pltpu.SemaphoreType.DMA((22,)),
            pltpu.SemaphoreType.DMA((1,)),
        ],
        compiler_params=pltpu.CompilerParams(vmem_limit_bytes=100 * 1024 * 1024, disable_semaphore_checks=True,
                                             disable_bounds_checks=bool(int(os.environ.get('NOBC', '0')))),
    )(A_q, A_k, A_v, A_shift_k.T, A_ssm_k, A_ssm_D, B_w1, B_w2, B_w3.T, B_w4, c, w_mod)
```

```python
import functools
import math
import os

import jax
import jax.numpy as jnp
from jax import lax
import jax.experimental.pallas as pl
import jax.experimental.pallas.tpu as pltpu

S, D, F = 2048, 640, 1728
C = 128
NC = S // C
NT = D // 128
NG = 16
KOFF = (NC + 1) * NG * 3
W = int(os.environ.get('W', '4'))
SKIPA = int(os.environ.get('SKIPA', '0'))
WMA, WMP, WMC = 1280, 640, 640
Q0 = int(os.environ.get('Q0', '320'))
N2 = int(os.environ.get('N2', '5'))
PRELN = int(os.environ.get('PRELN', '2'))
NOCACHE = int(os.environ.get('NOCACHE', '0'))
OUTWAIT = int(os.environ.get('OUTWAIT', '0'))
SEGS = [int(x) for x in os.environ.get('SEGS', '012345')]
SKIPB = int(os.environ.get('SKIPB', '0'))
PADK = int(os.environ.get('PADK', '0'))
PREW = int(os.environ.get('PREW', '0'))
SP = float(os.environ.get('SP', '0'))
MINS = int(os.environ.get('MINS', '30'))
GA = int(os.environ.get('GA', '2'))
TRT = int(os.environ.get('TRT', '1'))
LP = int(os.environ.get('LP', '1'))
FA = 1664
LPN = int(os.environ.get('LPN', '2'))
G0 = int(os.environ.get('G0', '4'))
Q1 = int(os.environ.get('Q1', '768'))
TIE4 = int(os.environ.get('TIE4', '12'))
STAG = os.environ.get('STAG', 'w02,l0,n,n')
OCOLS = ((0, 512), (512, 128))
FSTEP = int(os.environ.get('FSTEP', '1'))
FOFF = int(os.environ.get('FOFF', '0'))
KORD = int(os.environ.get('KORD', '0'))
CW = int(os.environ.get('CW', '128'))
NP4 = int(os.environ.get('NP4', '2'))
LNT = [int(x) for x in os.environ.get('LNT', '0,1,2,3,4,5,18,22').split(',')]
OPQ = int(os.environ.get('OPQ', '1'))
RELOAD = int(os.environ.get('RELOAD', '0'))
REMP = os.environ.get('REMP', '653765376537')
Q2 = int(os.environ.get('Q2', '1408'))
_u0, _u1, _un = [int(x) for x in os.environ.get('ANCH', '20,58,18').split(',')]
ANCH = sorted({(_u0 + (_u1 - _u0) * i // _un) % 80 for i in range(_un)})
XRB = [int(x) for x in os.environ.get('XRB', '7420')]
KARA = int(os.environ.get('KARA', '1'))
UNR = int(os.environ.get('UNR', '2'))
HEAD = int(os.environ.get('HEAD', '250'))
TAIL = int(os.environ.get('TAIL', '450'))
DORDER = os.environ.get('DORDER', 'aHbU')
R1 = int(os.environ.get('R1', '64'))
R2 = int(os.environ.get('R2', '128'))
LEAD = int(os.environ.get('LEAD', '3'))
TS = int(os.environ.get('TS', '512'))
ONEPASS = int(os.environ.get('ONEPASS', '1'))
RSQ = int(os.environ.get('RSQ', '1'))
T2 = int(os.environ.get('T2', '512'))
EPS = 1e-5
_C0 = math.sqrt(2.0 / math.pi)
ALPHA = (_C0 * 0.044715) ** (1.0 / 3.0)
GC = _C0 / ALPHA
BETA = 0.5 / ALPHA
_fc = [int(x) for x in os.environ.get('FC', '1728').split(',')]
F_CHUNKS = tuple((sum(_fc[:i]), _fc[i]) for i in range(len(_fc)))
assert sum(_fc) == F

f32 = jnp.float32
bf16 = jnp.bfloat16
u32 = jnp.uint32
NTDIMS = (((1,), (1,)), ((), ()))


def _cos_table(m, scale):
    mm = jnp.abs(((m + 256) & 511) - 256)
    x = (128 - mm).astype(f32) * (1.0 / 128.0)
    x2 = x * x
    h = math.pi / 2
    p = -(h ** 7) / 5040 + x2 * ((h ** 9) / 362880 - x2 * (h ** 11) / 39916800)
    p = h + x2 * (-(h ** 3) / 6 + x2 * ((h ** 5) / 120 + x2 * p))
    return (x * scale) * p


def _dft_tables():
    shape = (16, 8, 128)
    n = lax.broadcasted_iota(jnp.int32, shape, 0)
    s = lax.broadcasted_iota(jnp.int32, shape, 1)
    l = lax.broadcasted_iota(jnp.int32, shape, 2)
    fw, fu, iv = [], [], []
    wv = l >> 4
    tu = (16 * W) * (wv // W) + (2 * W) * ((l >> 1) & 7) + 2 * (wv % W) + (l & 1)
    for e in range(2):
        r = 2 * s + e
        j = 8 * n + (r & 7)
        fw.append(_cos_table((4 * j + 1) * l + (r >> 3) * 128, 1.0))
        fu.append(_cos_table((4 * j + 1) * tu + (r >> 3) * 128, 1.0))
        b = 16 * (n >> 1) + r
        col = 128 * (n & 1) + l
        iv.append(_cos_table((4 * (col >> 1) + 1) * b + (col & 1) * 128, 1.0 / 128.0))
    pk = lambda xs: pltpu.bitcast(pltpu.pack_elementwise(xs, packed_dtype=bf16), f32)
    return pk(fw), pk(iv), pk(fu)


def _gelu2a(z):
    return z * (1.0 + jnp.tanh(z * (z * z + GC)))


def _rstd(ssd, scale):
    if RSQ == 0:
        r = lax.rsqrt(ssd * (1.0 / D) + EPS)
        return r if scale == 1.0 else r * scale
    return jnp.exp2(jnp.log(ssd + D * EPS) * (-0.5 / math.log(2.0)) + math.log2(scale * math.sqrt(D)))


def _center(x, scale=1.0):
    s1 = jnp.sum(x, axis=-1, keepdims=True)
    m = s1 * (1.0 / D)
    d = x - m
    if ONEPASS:
        ssd = jnp.maximum(jnp.sum(x * x, axis=-1, keepdims=True) - s1 * m, 0.0)
    else:
        ssd = jnp.sum(d * d, axis=-1, keepdims=True)
    return d, _rstd(ssd, scale)


def _conv(us, gs, a):
    acc = None
    for c in range(a + 1):
        p = us[c] * gs[a - c]
        acc = p if acc is None else acc + p
    return acc


_SA = (lambda a, b, c, d: a + d, lambda a, b, c, d: d, lambda a, b, c, d: c + d, lambda a, b, c, d: a,
       lambda a, b, c, d: a + b, lambda a, b, c, d: b - d, lambda a, b, c, d: c - a)
_SB = (lambda a, b, c, d: a + d, lambda a, b, c, d: c - a, lambda a, b, c, d: a, lambda a, b, c, d: b - d,
       lambda a, b, c, d: d, lambda a, b, c, d: c + d, lambda a, b, c, d: a + b)


_SC = (((0, 1), (3, 1)), ((0, 1), (2, 1)), ((2, 1), (3, -1)), ((1, 1), (3, 1)), ((0, -1), (1, 1)), ((0, 1),), ((3, 1),))
_SCL = (5, 4, 2, 6)


_SBU = ((1, 0, 0, 1), (1, 0, 1, 0), (1, 0, 0, 0), (0, 1, 0, 1), (0, 0, 0, 1), (0, 0, 1, 1), (1, 1, 0, 0))


def _comb(m):
    m1, m4, m2, m3, m5, m7, m6 = m
    return (m1 + m4) + (m7 - m5), m3 + m5, m4 + m2, (m1 + (m3 - m2)) + m6


class Lazy:
    def __init__(self, terms):
        self.terms = terms

    def __add__(self, o):
        return Lazy(self.terms + o.terms)

    def __sub__(self, o):
        return Lazy(self.terms + [(-s_, r_, c_) for (s_, r_, c_) in o.terms])

    def shift(self, dr, dc):
        return Lazy([(s_, r_ + dr, c_ + dc) for (s_, r_, c_) in self.terms])

    def load(self, ref, rn, cn):
        ts = sorted(self.terms, key=lambda t: -t[0])
        v = [ref[pl.ds(r_, rn), pl.ds(c_, cn)] for (_, r_, c_) in ts]
        acc_ = v[0]
        for (s_, _, _), x in zip(ts[1:], v[1:]):
            acc_ = acc_ + x if s_ > 0 else acc_ - x
        return acc_.astype(bf16)


def _mult(x, n):
    return x if isinstance(x, int) else pl.multiple_of(x, n)


def _wt(ref, *idx):
    return pltpu.bitcast(ref[idx] if idx else ref[...], bf16)


def _kernel(q_hbm, k_hbm, v_hbm, sk_hbm, h_hbm, dd_hbm, w1_hbm, w2_hbm, w3_hbm, w4_hbm,
            c_hbm, wm_hbm, o_hbm,
            modb, qbuf, kbuf, vbuf, hbuf, w1, w2, w3, w4, wm, wmp, wmc, obuf,
            ub0, ub1, gb0, gb1, kb0, kb1, yb, xn, hh, h1, par, l4p_, gs_, w4s, w3s, w4o, sk_s, dd_s, c_s, zs, sems, osems):
    l4p = l4p_.at[0]
    ubs, gbs, kbs = (ub0, ub1), (gb0, gb1), (kb0, kb1)
    cp = pltpu.make_async_copy
    HS = S // 2

    def cp_h(j, c0, c1, sem):
        return cp(h_hbm.at[pl.ds(j * 128, 128), pl.ds(c0, c1 - c0)], hbuf.bitcast(bf16).at[j, :, pl.ds(c0, c1 - c0)], sem)

    def cp_kv(j, r0, r1, sem):
        r0, r1 = (r0 + 16 if r0 else 0), min(r1 + 16, S)
        lanes = pl.ds(j * 128, 128)
        return [cp(k_hbm.at[0, pl.ds(r0, r1 - r0), lanes], kbuf.bitcast(bf16).at[j, pl.ds(r0 + 16, r1 - r0), :], sem),
                cp(v_hbm.at[0, pl.ds(r0, r1 - r0), lanes], vbuf.bitcast(bf16).at[j, pl.ds(r0, r1 - r0), :], sem)]

    def cp_tile(j, i):
        sem = sems.at[2 * j + i]
        return [cp_h(j, i * HS, (i + 1) * HS, sem)] + cp_kv(j, i * HS, (i + 1) * HS, sem)

    cp_t0 = [[cp_h(0, 0, S, sems.at[0])], cp_kv(0, 0, 1024, sems.at[1]), cp_kv(0, 1024, 1536, sems.at[20]),
             cp_kv(0, 1536, S, sems.at[21])]

    def cp_wm(i):
        return cp(wm_hbm.at[:, pl.ds(i * WMA, WMA)], wm.bitcast(bf16).at[i], sems.at[10 + i])

    cp_wmp = cp(wm_hbm.at[:, pl.ds(2 * WMA, WMP)], wmp.bitcast(bf16), sems.at[13])
    cp_wmc = cp(wm_hbm.at[:, pl.ds(2 * WMA + WMP, WMC)], wmc.bitcast(bf16), sems.at[12])
    cp_q = [cp(q_hbm.at[0, pl.ds(r0, r1 - r0), :], qbuf.at[pl.ds(r0, r1 - r0), :], sems.at[sm])
            for sm, r0, r1 in ((13, 0, Q0), (16, Q0, Q1), (14, Q1, Q2), (12, Q2, S))]
    cp_w = [cp(s_, d_.bitcast(bf16).at[pl.ds(0, s_.shape[0]), :], sems.at[sm])
            for sm, s_, d_ in ((15, w1_hbm, w1), (16, w2_hbm, w2), (12, w3_hbm, w3), (14, w4_hbm, w4))]
    cp_s = [cp(sk_hbm, sk_s, sems.at[19]), cp(dd_hbm, dd_s, sems.at[19]), cp(c_hbm, c_s, sems.at[19])]
    order = list(cp_s)
    for grp in cp_t0:
        order += grp
    for j in range(1, NT):
        order += cp_tile(j, 0) + cp_tile(j, 1)
    order += [cp_wm(0), cp_wm(1), cp_wmp, cp_q[0], cp_w[0], cp_w[1], cp_q[1], cp_q[2], cp_w[3], cp_q[3], cp_wmc, cp_w[2]]
    for c_ in order:
        c_.start()

    with jax.named_scope("init"):
        fw_t, iv_t, fu_t = _dft_tables()
        for kb in kbs:
            kb[pl.ds(KOFF, 16)] = fw_t
            kb[pl.ds(KOFF + 16, 16)] = iv_t
            kb[pl.ds(KOFF + 32, 16)] = fu_t
            kb[pl.ds(0, NG * 3)] = jnp.zeros((NG * 3, 8, 128), f32)
        zeros = jnp.zeros((8, 128), f32)
        w4[pl.ds(F // 2, 32), :] = jnp.zeros((32, D), u32)
        for j in range(NT):
            kbuf[j, pl.ds(0, 8), :] = jnp.zeros((8, 128), u32)
            kbuf[j, pl.ds(8 + HS, 8), :] = jnp.zeros((8, 128), u32)
            vbuf[j, pl.ds(HS, 8), :] = jnp.zeros((8, 128), u32)
        for j in range(NT):
            h1[j, pl.ds(0, 8), :] = zeros
            h1[j, pl.ds(S + 8, 8), :] = zeros
        for c_ in cp_s:
            c_.wait()
        par[pl.ds(0, 4), :] = sk_s[...].astype(f32)
        par[pl.ds(8, 8), :] = jnp.broadcast_to(dd_s[...].astype(f32).reshape(1, D), (8, D))
        cv = c_s[...].astype(f32)
        sc = jnp.broadcast_to(cv * jax.nn.sigmoid(cv), (8, D))
        scp = pltpu.bitcast(pltpu.pack_elementwise([sc, sc], packed_dtype=bf16), f32)
        for j in range(NT):
            kb0[KOFF + 48 + j] = scp[:, 128 * j:128 * (j + 1)]
            kb1[KOFF + 48 + j] = scp[:, 128 * j:128 * (j + 1)]

    def mkb(i, unr, off, cache):
        def b(stride, extra=0, z=None):
            if isinstance(i, int):
                return (i * unr + off) * stride + extra
            key = (unr * stride, z)
            if key not in cache or NOCACHE:
                base = pl.multiple_of(i * (unr * stride), unr * stride)
                cache[key] = base if z is None else base + (i >> z)
            return cache[key] + (off * stride + extra)
        return b

    def dot_h(j, b, lhs):
        gb = gbs[j % 2]
        hc = hbuf[j, :, pl.ds(_mult(b(512), 512), 512)]
        rhs_t = jnp.concatenate([hc[:, C * cc:C * (cc + 1)] for cc in range(4)], axis=0)
        g = lax.dot_general(lhs, pltpu.bitcast(rhs_t, bf16), NTDIMS, preferred_element_type=f32)
        for rg in range(2 * NG):
            for cc in range(4):
                gb[b(4, cc + rg * NC)] = g[8 * rg:8 * rg + 8, 128 * cc:128 * cc + 128]

    def dot_u(j, b, lhs):
        ub = ubs[j % 2]
        taps = [par[pl.ds(t, 1), pl.ds(j * 128, 128)] for t in range(4)]
        unp = lambda w_, e: pltpu.unpack_elementwise(w_, index=e, packed_dtype=bf16, unpacked_dtype=f32)
        cols = []
        for cc in range(4):
            words = []
            for blk in range(8 // W):
                w0 = 64 * cc + 8 * W * blk
                kw = {m: kbuf[j, pl.ds(b(256, 8 + w0 + m), 8, stride=W), :] for m in range(-2, W)}
                kk = {2 * m + e: unp(kw[m], e) for m in range(-2, W) for e in range(2) if 2 * m + e >= -3}
                for m in range(W):
                    vw = vbuf[j, pl.ds(b(256, w0 + m), 8, stride=W), :]
                    pair = []
                    for e in range(2):
                        n = 2 * m + e
                        ks = kk[n] * taps[0] + kk[n - 1] * taps[1] + kk[n - 2] * taps[2] + kk[n - 3] * taps[3]
                        pair.append(ks * unp(vw, e))
                    words.append(pltpu.pack_elementwise(pair, packed_dtype=bf16))
            cols.append(jnp.concatenate(words, axis=0))
        rhs = pltpu.bitcast(jnp.concatenate(cols, axis=1), bf16)
        u = jnp.dot(lhs, rhs, preferred_element_type=f32)
        for rg in range(2 * NG):
            for cc in range(4):
                ub[b(4, cc + rg * NC)] = u[8 * rg:8 * rg + 8, 128 * cc:128 * cc + 128]

    def dot_i(j, b, half, lhs):
        kb = kbs[j % 2]
        cols = [[], []]
        for gi in range(NG):
            prev = None
            for cc in range(-1, 2):
                k0, k1, k2 = [kb[b(4 * NG * 3, ((2 * half + cc + 1) * NG + gi) * 3 + t)] for t in range(3)]
                re, im = k0 - k2, k0 + k1
                if prev is not None:
                    cols[cc].append(pltpu.pack_elementwise([re - prev[1], im + prev[0]], packed_dtype=bf16))
                prev = (re, im)
        rhs = jnp.concatenate([jnp.concatenate(c_, axis=0) for c_ in cols], axis=1)
        y = jnp.dot(lhs, pltpu.bitcast(rhs, bf16), preferred_element_type=f32)
        for cc in range(2):
            yb[j, pl.ds(b(512, (2 * half + cc) * C), C), :] = y[:, 128 * cc:128 * cc + 128]

    def gen_m(j, kb, b, ng):
        ub, gb = ubs[j % 2], gbs[j % 2]
        for s in range(ng):
            for t in range(3):
                z = 8 + t
                re = lambda ref, c: ref[b(2 * NC, 2 * s * NC + c, z)]
                im = lambda ref, c: ref[b(2 * NC, (2 * s + 1) * NC + c, z)]
                gre = [re(gb, c) for c in range(NC)]
                if t == 0:
                    us = [re(ub, c) + im(ub, c) for c in range(NC)]
                    gs = gre
                elif t == 1:
                    us = [re(ub, c) for c in range(NC)]
                    gs = [im(gb, c) - gre[c] for c in range(NC)]
                else:
                    us = [im(ub, c) for c in range(NC)]
                    gs = [im(gb, c) + gre[c] for c in range(NC)]

                def st(a, val):
                    kb[b(3, ((a + 1) * NG + s) * 3 + t)] = val
                if not KARA:
                    for a in range(NC):
                        st(a, _conv(us, gs, a))
                        yield 2 * a + 2
                    continue
                ue, uo, ge, go = us[0::2], us[1::2], gs[0::2], gs[1::2]
                if KORD == 1:
                    usum = [x + y for x, y in zip(ue, uo)]
                    gsum = [x + y for x, y in zip(ge, go)]
                    poo = _conv(uo, go, NC // 2 - 1)
                    for a in reversed(range(NC // 2)):
                        pee = _conv(ue, ge, a)
                        pss = _conv(usum, gsum, a)
                        st(2 * a + 1, pss - pee - poo)
                        poo = _conv(uo, go, a - 1) if a else None
                        st(2 * a, pee + poo if a else pee)
                        yield 3 * (2 * a + 1) + (37 if a == NC // 2 - 1 else 3)
                    continue
                usum = [x + y for x, y in zip(ue, uo)]
                gsum = [x + y for x, y in zip(ge, go)]
                poo_prev = None
                for a in range(NC // 2):
                    pee = _conv(ue, ge, a)
                    poo = _conv(uo, go, a)
                    pss = _conv(usum, gsum, a)
                    st(2 * a, pee if poo_prev is None else pee + poo_prev)
                    st(2 * a + 1, pss - pee - poo)
                    poo_prev = poo
                    yield 3 * (2 * a + 1) + 7

    def add_d(j):
        gb = gbs[j % 2]
        dvec = par[pl.ds(8, 8), pl.ds(j * 128, 128)]
        for gi in range(NG):
            gb[2 * gi * NC] = gb[2 * gi * NC] + dvec

    def sc_lhs():
        return pltpu.bitcast(jnp.concatenate([kb0[KOFF + 48 + j] for j in range(NT)], axis=1), bf16)

    def dot_m(i, t0, nt, rows):
        m = None
        for kt in range(NT):
            p = jnp.dot(pltpu.bitcast(rows[kt], bf16), _wt(wm, i, pl.ds(64 * kt, 64), pl.ds(128 * t0, 128 * nt)),
                        preferred_element_type=f32)
            m = p if m is None else m + p
        for t in range(nt):
            modb[i * (WMA // 128) + (t0 + t)] = m[0:8, 128 * t:128 * (t + 1)]

    def inv_lhs(tbl, n):
        return jnp.concatenate([tbl[KOFF + 16 + 2 * n], tbl[KOFF + 17 + 2 * n]], axis=1)

    def dot_k(kb, kt, bt, lhs):
        cols = [[] for _ in range(4)]
        for gi in range(8 * kt, 8 * kt + 8):
            prev = None
            for cc in range(-1, 4):
                k0, k1, k2 = [kb[((4 * bt + cc + 1) * NG + gi) * 3 + t] for t in range(3)]
                re, im = k0 - k2, k0 + k1
                if prev is not None:
                    cols[cc].append(pltpu.pack_elementwise([re - prev[1], im + prev[0]], packed_dtype=bf16))
                prev = (re, im)
        rhs = jnp.concatenate([jnp.concatenate(c_, axis=0) for c_ in cols], axis=1)
        y = jnp.dot(lhs, pltpu.bitcast(rhs, bf16), preferred_element_type=f32)
        for cc in range(4):
            rows = pl.ds((4 * bt + cc) * C, C)
            yc = y[:, 128 * cc:128 * cc + 128]
            yb[NT - 1, rows, :] = yc if kt == 0 else yb[NT - 1, rows, :] + yc

    PRE = dict(H=0, U=672 + 96 // W, a=192, b=192, m=0, k=176)
    POST = dict(H=0, U=0, a=4, b=4, m=2, k=0)
    NST = dict(H=16, U=16, a=8, b=8, m=5, k=8)
    GCOST = 3 * (248 if KARA else 272)

    def a_block(dots, mg=None, ng=0, tbl=kb0):
        native, dur = [], []
        for idx, (k_, _) in enumerate(dots):
            nxt = PRE[dots[idx + 1][0]] if idx + 1 < len(dots) else 0
            d_ = 2.0 if k_ == 'm' else 1.0
            native += [nxt / NST[k_] + POST[k_] * d_] * NST[k_]
            dur += [d_] * NST[k_]
        if mg is not None and dots:
            head = max(HEAD - PRE[dots[0][0]], 0)
            mtot = GCOST * ng - TAIL - head
            lvl = (mtot + sum(native)) / sum(dur)
            want = [max(lvl * d_ - x, 0.0) for x, d_ in zip(native, dur)]
            scale = mtot / sum(want)
            cum, tgt = [head], head
            for w_ in want:
                tgt += w_ * scale
                cum.append(tgt)
        done = 0.0
        step = 0
        for (k_, fn) in dots:
            rows = []
            for n in range(NST[k_]):
                if mg is not None and (n % FSTEP == 0 or k_ == 'm'):
                    while done < cum[min(step + FOFF, len(cum) - 1)]:
                        done += next(mg)
                step += 1
                if k_ in 'HU':
                    rows.append(tbl[KOFF + n + (32 if k_ == 'U' else 0)])
                elif k_ in 'ab':
                    rows.append(inv_lhs(tbl, n))
                elif k_ == 'k':
                    rows.append(tbl[KOFF + 16 + 2 * n])
                else:
                    rows.append(tbl[KOFF + 48 + n])
            fn(rows if k_ == 'm' else pltpu.bitcast(jnp.concatenate(rows, axis=0), bf16))
        if mg is not None:
            for _ in mg:
                pass

    def fdot(k_, j, b):
        if k_ == 'H':
            return (k_, lambda lhs: dot_h(j, b, lhs))
        if k_ == 'U':
            return (k_, lambda lhs: dot_u(j, b, lhs))
        return (k_, lambda lhs: dot_i(j, b, 0 if k_ == 'a' else 1, lhs))

    def wait_all(cps):
        for c_ in cps:
            c_.wait()

    def a_loop(jf, jm, ji, g0, ng):
        kinds = [k_ for k_ in DORDER if k_ in 'HU' or ji is not None]

        def body(i, carry):
            cache = {}
            zs[i] = 0
            dots = [fdot(k_, jf if k_ in 'HU' else ji, mkb(i, 2, s_, cache)) for s_ in range(2) for k_ in kinds]
            a_block(dots, gen_m(jm, kbs[jm % 2], mkb(i, ng, g0, cache), ng), ng, kbs[jm % 2])

            @pl.when(i == 0)
            def _():
                wait_all(cp_tile(jf, 1))
            return carry
        wait_all(cp_tile(jf, 0))
        lax.fori_loop(0, 2, body, 0)
        add_d(jf)

    sb_ = lambda bt: mkb(0, 1, bt, None)
    if SKIPA:
        a_block = lambda *a, **k: None
    with jax.named_scope("A_seg0"):
        wait_all(cp_t0[0])
        a_block([fdot('H', 0, sb_(bt)) for bt in range(4)])
        add_d(0)
        wait_all(cp_t0[1])
        a_block([fdot('U', 0, sb_(bt)) for bt in range(2)])
        for bt in (2, 3):
            wait_all(cp_t0[bt])
            a_block([fdot('U', 0, sb_(bt))])
    with jax.named_scope("A_m0"):
        def body_m0(i, carry):
            a_block([], gen_m(0, kb0, mkb(i, G0 // 2, 0, {}), G0 // 2))
            return carry
        if G0:
            lax.fori_loop(0, 2, body_m0, 0)
    for seg in range(1, NT):
        with jax.named_scope(f"A_seg{seg}"):
            if seg == 1:
                a_loop(1, 0, None, G0, (NG - G0) // 2)
            else:
                a_loop(seg, seg - 1, seg - 2, 0, 8)

    def mods(i):
        return [('m', lambda rows, t0=t0, nt=nt: dot_m(i, t0, nt, rows)) for (t0, nt) in ((0, 4), (4, 4), (8, 2))]

    with jax.named_scope("A_seg5a"):
        cp_wm(0).wait()
        zz = zs[1]

        @pl.when(zz == 0)
        def _():
            dots = [fdot(k_, NT - 2, sb_(bt)) for bt in range(4) for k_ in 'ab']
            mm = mods(0)
            dots = [mm[0]] + dots[0:2] + [mm[1]] + dots[2:4] + [mm[2]] + dots[4:]
            a_block(dots, gen_m(NT - 1, kb0, mkb(zz, 8, 0, {}), 8), 8, kb0)
    with jax.named_scope("A_seg5b"):
        cp_wm(1).wait()

        @pl.when(zz == 0)
        def _():
            dots = [('k', lambda lhs, bt=bt: dot_k(kb0, 0, bt, lhs)) for bt in range(4)]
            mm = mods(1)
            dots = [mm[0], dots[0], mm[1], dots[1], mm[2]] + dots[2:]
            a_block(dots, gen_m(NT - 1, kb1, mkb(zz, 8, 8, {}), 8), 8, kb1)

    def inv_last(bt):
        lhs = pltpu.bitcast(jnp.concatenate([kb0[KOFF + 17 + 2 * n] for n in range(8)], axis=0), bf16)
        dot_k(kb1, 1, bt, lhs)

    def modrow(k_):
        return jnp.concatenate([modb[NT * k_ + j] for j in range(NT)], axis=1)

    R = R1
    GP = R // 8

    def ln_chain(p):
        r = p * R
        pa, pb, pc, ps = [par[pl.ds(16 + 8 * t, 8), :][None] for t in range(4)]
        g3 = lambda x: x.reshape(GP, 8, D)
        q = g3(qbuf[pl.ds(r, R), :].astype(f32))
        d1, r1 = _center(q)
        y = g3(jnp.concatenate([yb[j, pl.ds(r, R), :] for j in range(NT)], axis=1))
        x = q + ((d1 * r1) * pa + pb) * y
        xn[pl.ds(r, R), :] = x.reshape(R, D)
        d2, r2 = _center(x)
        h = (d2 * r2) * pc + ps
        hh[pl.ds(r, R), :] = h.reshape(R, D)
        d3, r3 = _center(h, ALPHA)
        return (d3 * r3).reshape(R, D)

    def tie(w_, vs):
        t_ = pltpu.bitcast(vs[0], u32)
        for v_ in vs[1:]:
            t_ = t_ | pltpu.bitcast(v_, u32)
        return w_ | (t_ & kbuf[0, pl.ds(0, 8), :])

    def tied(wref, ties):
        if not ties:
            return _wt(wref)
        rbs = sorted({8 * (t % 5) + rb for (t, rb) in ties})
        rows, pos = [], 0
        for rb in rbs:
            if rb > pos:
                rows.append(wref[pl.ds(8 * pos, 8 * (rb - pos)), :])
            blk = []
            for n in range(NT):
                w_ = wref[pl.ds(8 * rb, 8), pl.ds(128 * n, 128)]
                vs = ties.get((5 * n + rb // 8, rb % 8))
                blk.append(tie(w_, vs) if vs else w_)
            rows.append(jnp.concatenate(blk, axis=1))
            pos = rb + 1
        if pos < 40:
            rows.append(wref[pl.ds(8 * pos, 8 * (40 - pos)), :])
        return pltpu.bitcast(jnp.concatenate(rows, axis=0), bf16)

    def w1_dot(p, l3, ties, fresh):
        if fresh and STAG:
            grp = lambda g: l3[8 * g:8 * g + 8, 0:128]
            lt = {}
            for pr, spec in enumerate(STAG.split(',')):
                vs = [grp(2 * pr), grp(2 * pr + 1)]
                if spec[0] == 'w':
                    ties.setdefault((int(spec[1]), int(spec[2])), []).extend(vs)
                elif spec[0] == 'l':
                    lt.setdefault(int(spec[1]), []).extend(vs)
            for pr, vs in lt.items():
                x = pltpu.bitcast(tie(pltpu.bitcast(l3[16 * pr:16 * pr + 8, 128:256], u32), vs), f32)
                mid = jnp.concatenate([l3[16 * pr:16 * pr + 8, 0:128], x, l3[16 * pr:16 * pr + 8, 256:]], axis=1)
                l3 = jnp.concatenate(([l3[:16 * pr]] if pr else []) + [mid, l3[16 * pr + 8:]], axis=0)
        z = jnp.dot(l3.astype(bf16), tied(w1, ties), preferred_element_type=f32)
        g = _gelu2a(z)
        for j in range(NT):
            h1[j, pl.ds(p * R + 8, R), :] = g[:, j * 128:(j + 1) * 128]
        return z

    def w2_dot(p, ties):
        r = p * R
        lane = lax.broadcasted_iota(jnp.int32, (R, 128), 1)

        def ld(j, off):
            return h1[j, pl.ds(r + 8 + off, R), :]
        tiles = [
            ld(0, -1),
            jnp.where(lane < 32, ld(1, -1), ld(1, 1)),
            jnp.where(lane < 64, ld(2, 1), ld(2, -2)),
            jnp.where(lane < 96, ld(3, -2), ld(3, 2)),
            ld(4, 2),
        ]
        hs = jnp.concatenate(tiles, axis=1).astype(bf16)
        x1 = hh[pl.ds(r, R), :] + jnp.dot(hs, tied(w2, ties), preferred_element_type=f32) * BETA
        hh[pl.ds(r, R), :] = x1
        return x1

    unp = lambda w_, e: pltpu.unpack_elementwise(w_, index=e, packed_dtype=bf16, unpacked_dtype=f32)
    pk = lambda xs: pltpu.pack_elementwise(xs, packed_dtype=bf16)
    PURE = {7 * p_ + q_: 2 * i_ + j_ for i_, p_ in enumerate((2, 4)) for j_, q_ in enumerate((2, 4))}

    zoff = [pl.multiple_of((zz >> p_) * 32, 32) for p_ in range(7)]

    def prep2(src, dst, tr, t, p_, anchor):
        zero = None if anchor is None else pltpu.bitcast(anchor, u32) & kbuf[0, pl.ds(0, 8), :]
        gate = 0 if _SBU[p_][0] else 3
        l1 = [[], []]
        for k2 in range(2):
            for n2 in range(2):
                bl = []
                for b_ in range(4):
                    kq, nq = 2 * (b_ // 2) + k2, 2 * (b_ % 2) + n2
                    x = None
                    if _SBU[p_][b_]:
                        x = src[pl.ds(zoff[p_] + (8 * t + 192 * (nq if tr else kq)), 8), pl.ds(128 * (kq if tr else nq), 128)]
                        if zero is not None and b_ == gate and k2 == n2:
                            x = x | zero
                    bl.append(x)
                for e in range(2):
                    l1[e].append(_SB[p_](*[None if x is None else unp(x, e) for x in bl]))
        for q_ in range(7):
            if 7 * p_ + q_ not in PURE:
                dst[7 * p_ + q_, pl.ds(8 * t, 8), :] = pk([_SB[q_](*l1[e]) for e in range(2)])

    def prep1(t, n, anchor):
        bl = [w4[pl.ds(lo + 8 * t, 8), pl.ds(c0 + 128 * n, 128)] for lo in (768, 832) for c0 in (0, 256)]
        if anchor is not None:
            zero = pltpu.bitcast(anchor, u32) & kbuf[0, pl.ds(0, 8), :]
            bl[0], bl[3] = bl[0] | zero, bl[3] | zero
        for p_ in (0, 1, 3, 5, 6):
            w4o[p_, pl.ds(8 * t, 8), pl.ds(128 * n, 128)] = pk([_SB[p_](*[unp(x, e) for x in bl]) for e in range(2)])

    units = []
    l3s = {}

    def ln4(r, n):
        d4, r4 = _center(hh[pl.ds(r, n), :], ALPHA)
        return d4 * r4

    def run_block(dots, extra=None, pre4=False):
        for d_, (k_, p) in enumerate(dots):
            ties = {}
            e = d_ - (len(dots) - NP4)
            RP = TS // NP4
            if pre4 and e >= 0:
                nx = ln4(e * RP, RP)
                l4p[pl.ds(e * RP, RP), :] = nx
                ties[(TIE4, 7)] = [nx[8 * g:8 * g + 8, 0:128] for g in range(RP // 8)]
            if extra is not None and d_ == len(dots) - 1:
                nx = ln_chain(extra)
                for pr in range(4):
                    ties[(24, XRB[pr])] = [nx[16 * pr:16 * pr + 8, 0:128], nx[16 * pr + 8:16 * pr + 16, 0:128]]
                l3s[extra] = nx.astype(bf16)
            if k_ == 1:
                fresh = p not in l3s
                res = w1_dot(p, ln_chain(p) if fresh else l3s.pop(p), ties, fresh)
            elif k_ == 2:
                res = w2_dot(p, ties)
            else:
                par[pl.ds(48, 8), :] = jnp.dot(sc_lhs(), _wt(wmc), preferred_element_type=f32)[0:8]
            for u_ in ANCH:
                if u_ // 40 + 1 == k_ and units and d_ < len(dots) - (NP4 + 1 if pre4 else 0):
                    n, g = (u_ % 40) // 8, u_ % 8
                    units.pop(0)(res[8 * g:8 * g + 8, 128 * n:128 * (n + 1)])

    with jax.named_scope("P1"):
        cp_wmp.wait()
        cp_q[0].wait()
        mp = jnp.dot(sc_lhs(), _wt(wmp), preferred_element_type=f32)
        for t in range(WMP // 128):
            modb[2 * WMA // 128 + t] = mp[0:8, 128 * t:128 * (t + 1)]
        sa, ca, ga, sb, cb = [modrow(k_) for k_ in range(5)]
        par[pl.ds(16, 8), :] = ga * (1.0 + ca)
        par[pl.ds(24, 8), :] = ga * sa
        par[pl.ds(32, 8), :] = 1.0 + cb
        par[pl.ds(40, 8), :] = sb
        for bt in range(4):
            inv_last(bt)
        for p in range(PRELN):
            l3s[p] = ln_chain(p)
    with jax.named_scope("w1wait"):
        cp_w[0].wait()
    p1, p2 = N2, 0
    with jax.named_scope("P2"):
        run_block([(1, p) for p in range(N2)])
    with jax.named_scope("w2wait"):
        wait_all([cp_w[1], cp_q[1]])

    def plan(lim1):
        nonlocal p1, p2
        last = lim1 == S // R
        dots = []
        while p1 < (lim1 if last else lim1 - 1) or p1 - p2 >= LEAD or (last and p2 < lim1):
            if p1 - p2 < LEAD and p1 < lim1:
                dots.append((1, p1))
                p1 += 1
            else:
                dots.append((2, p2))
                p2 += 1
        return dots, (None if last else p1)

    with jax.named_scope("P4"):
        run_block(*plan(Q1 // R))
    with jax.named_scope("q2wait"):
        wait_all([cp_q[2], cp_w[3]])
    units += [functools.partial(prep2, w4, w4s, False, t, p_) for t in range(24) for p_ in range(7)]
    units += [functools.partial(prep1, t, n) for t in range(8) for n in range(2)]
    with jax.named_scope("P5"):
        run_block(*plan(Q2 // R))
    with jax.named_scope("q3wait"):
        wait_all([cp_q[3], cp_wmc, cp_w[2]])
    units += [functools.partial(prep2, w3, w3s, True, t, p_) for t in range(24) for p_ in range(7)]
    with jax.named_scope("P6"):
        dots, _ = plan(S // R)
        run_block(dots[:-NP4] + [(3, 0)] + dots[-NP4:], pre4=True)

    H2 = TS // 2
    OUTS = ((0, H2, 512, 128), (H2, H2, 0, 256), (0, H2, 256, 256), (0, H2, 0, 256), (H2, H2, 256, 256), (H2, H2, 512, 128))

    def out_copy(r, r0, rn, c0, cn):
        rows = pl.ds(_mult(r + r0, H2), rn)
        return cp(obuf.at[rows, pl.ds(c0, cn)], o_hbm.at[0, rows, pl.ds(c0, cn)], osems.at[0])

    def wsum(x, y, sign):
        unp = lambda w_, e: pltpu.unpack_elementwise(w_, index=e, packed_dtype=bf16, unpacked_dtype=f32)
        return pltpu.pack_elementwise([unp(x, e) + unp(y, e) if sign > 0 else unp(x, e) - unp(y, e) for e in range(2)],
                                      packed_dtype=bf16)

    def strassen_lhs(a11, a12, a21, a22):
        c = lambda x: x.astype(bf16)
        return (c(a11 + a22), c(a21 + a22), c(a11), c(a22), c(a11 + a12), c(a21 - a11), c(a12 - a22))

    def strassen(ops, b11, b12, b21, b22, mm, ties=None):
        def tw(k_, w_):
            if not ties or k_ not in ties:
                return w_
            return jnp.concatenate([tie(w_[0:8], ties[k_]), w_[8:]], axis=0)
        m1 = mm(ops[0], tw(0, wsum(b11, b22, 1)))
        m4 = mm(ops[3], tw(1, wsum(b21, b11, -1)))
        m2 = mm(ops[1], tw(2, b11))
        m3 = mm(ops[2], tw(3, wsum(b12, b22, -1)))
        m5 = mm(ops[4], tw(4, b22))
        m7 = mm(ops[6], tw(5, wsum(b21, b22, 1)))
        m6 = mm(ops[5], tw(6, wsum(b11, b12, 1)))
        return (m1 + m4) + (m7 - m5), m3 + m5, m4 + m2, (m1 + (m3 - m2)) + m6

    mm_nt = lambda x, w_: lax.dot_general(x, pltpu.bitcast(w_, bf16), NTDIMS, preferred_element_type=f32)
    mm_nn = lambda x, w_: jnp.dot(x, pltpu.bitcast(w_, bf16), preferred_element_type=f32)

    def b2_step(i):
        gbv = par[pl.ds(48, 8), :]
        nsub = T2 // TS
        for sub in range(nsub):
            r = pl.multiple_of(pl.multiple_of(i * T2, T2) + sub * TS, TS)
            gs = gs_.at[i >> 8]
            l4 = l4p[...] if sub == 0 else ln4(r, TS)
            lb = l4.astype(bf16)
            zt = lax.dot_general(_wt(w3, pl.ds(832, 32), slice(None)), lb, NTDIMS, preferred_element_type=f32)
            g12 = _gelu2a(mm_nt(lb, w3[pl.ds(768, 64), :]))
            gt = jnp.concatenate([_gelu2a(zt), jnp.zeros((64, TS), f32)], axis=0).T
            gs[:, pl.ds(0, 128)] = g12
            gs[:, pl.ds(896, 128)] = gt
            lrs = [l4[:H2, 512:640].astype(bf16), l4[H2:, 512:640].astype(bf16)]
            Q = H2 // 2
            ab = [Lazy([(1, r_, c_)]) for (r_, c_) in ((0, 0), (0, 256), (H2, 0), (H2, 256))]
            opsA = {}
            rn_ = pl.multiple_of(jnp.minimum(i + 1, S // T2 - 1) * T2, T2)
            RP = TS // len(LNT)
            l4n = l4p
            for t in range(3):
                cq, left = [None] * 4, [5, 3, 3, 5]

                def add(k_, x, sg=1):
                    cq[k_] = x if cq[k_] is None else cq[k_] + x if sg > 0 else cq[k_] - x
                    left[k_] -= 1
                    if left[k_] == 0:
                        gg = _gelu2a(cq[k_])
                        for n2 in range(2):
                            gs[pl.ds(H2 * (k_ // 2), H2), pl.ds(128 + 896 * (k_ % 2) + 128 * (t + 3 * n2), 128)] = gg[:, 128 * n2:128 * (n2 + 1)]

                def rem(k_):
                    wr = jnp.concatenate([w3[pl.ds(64 * (t + 3 * (2 * (k_ % 2) + n2)), 64), pl.ds(512, 128)] for n2 in range(2)], axis=0)
                    add(k_, mm_nt(lrs[k_ // 2], wr))
                for p_ in range(8):
                    for k_ in (2, 1, 0, 3):
                        if int(REMP[4 * t + k_]) == p_:
                            rem(k_)
                    if p_ == 7:
                        break
                    a_ = _SA[p_](*ab)
                    sub_ = (a_, a_.shift(0, 128), a_.shift(Q, 0), a_.shift(Q, 128))
                    pr = []
                    for q_ in range(7):
                        n = 7 * p_ + q_
                        if n not in opsA or RELOAD:
                            opsA[n] = _SA[q_](*sub_).load(l4p_.at[(i + 4 * p_ + 32 * t) >> (9 + q_)] if RELOAD else l4p, Q, 128)
                        w_ = w3[pl.ds(192 * PURE[n] + 64 * t, 64), pl.ds(128 * PURE[n], 128)] if n in PURE else w3s[n, pl.ds(64 * t, 64), :]
                        pr.append(mm_nt(opsA[n], w_))
                    c11, c12, c21, c22 = _comb(pr)
                    m_ = jnp.concatenate([jnp.concatenate([c11, c12], axis=1), jnp.concatenate([c21, c22], axis=1)], axis=0)
                    for k_, sg in _SC[p_]:
                        add(k_, m_, sg)
            kord = [0, 896] + [o_ for c in (0, 3, 1, 4, 2, 5) for o_ in (128 + 128 * c, 1024 + 128 * c)]
            wrow = lambda o_: 768 if o_ == 0 else 832 if o_ == 896 else (o_ - 128) // 2 if o_ < 896 else 384 + (o_ - 1024) // 2
            wl = jnp.concatenate([w4[pl.ds(wrow(o_), 64), pl.ds(512, 128)] for o_ in kord], axis=0)
            gk = lambda r0: jnp.concatenate([gs[pl.ds(r0, H2), pl.ds(o_, 128)] for o_ in kord], axis=1).astype(bf16)
            acc_t = mm_nn(gk(0), wl)
            ties = {}
            for e, k_ in enumerate(LNT):
                nx = ln4(pl.multiple_of(rn_ + e * RP, RP), RP)
                l4n[pl.ds(e * RP, RP), :] = nx
                ties[k_] = [nx[8 * gi:8 * gi + 8, 0:128] for gi in range(RP // 8)]
            Q = H2 // 2

            blocks = [Lazy([(1, r_, c_)]) for (r_, c_) in ((0, 0), (0, 896), (H2, 0), (H2, 896))]
            ms = []
            for p_ in range(7):
                a_ = _SA[p_](*blocks)
                wo = w4[pl.ds(768, 64), pl.ds(0, 256)] if p_ == 2 else w4[pl.ds(832, 64), pl.ds(256, 256)] if p_ == 4 else w4o[p_]
                w4n = lambda n: w4[pl.ds(192 * PURE[n], 192), pl.ds(128 * PURE[n], 128)] if n in PURE else w4s[n]
                if p_ in ties:
                    wo = jnp.concatenate([jnp.concatenate([tie(wo[0:8, 0:128], ties[p_]), wo[0:8, 128:]], axis=1), wo[8:]], axis=0)
                m_ = mm_nn(a_.load(gs, H2, 128), wo)
                sub_ = (a_.shift(0, 128), a_.shift(0, 512), a_.shift(Q, 128), a_.shift(Q, 512))
                gref = lambda q_: gs_.at[(i + 4 * p_) >> (9 + q_)] if OPQ else gs
                c11, c12, c21, c22 = _comb([mm_nn(_SA[q_](*sub_).load(gref(q_), Q, 384), w4n(7 * p_ + q_)) for q_ in range(7)])
                ms.append(m_ + jnp.concatenate([jnp.concatenate([c11, c12], axis=1), jnp.concatenate([c21, c22], axis=1)], axis=0))
            c11, c12, c21, c22 = _comb(ms)
            for k_ in ties:
                if k_ >= 10:
                    o_ = 64 * (k_ - 10)
                    wl = jnp.concatenate([wl[:o_], tie(wl[o_:o_ + 8], ties[k_]), wl[o_ + 8:]], axis=0)
            accs = (acc_t, c21, c12, c11, c22, mm_nn(gk(H2), wl))
            for (r0, rn, c0, cn), ac in zip(OUTS, accs):
                rows, cols = pl.ds(_mult(r + r0, H2), rn), pl.ds(c0, cn)
                g3 = lambda x: x.reshape(rn // 8, 8, cn)
                out = g3(xn[rows, cols]) + gbv[None, :, c0:c0 + cn] * g3(hh[rows, cols] + BETA * ac)
                obuf[rows, cols] = out.reshape(rn, cn).astype(bf16)
                out_copy(r, r0, rn, c0, cn).start()

    with jax.named_scope("prep"):
        print("left-over prep units:", len(units))
        for u_ in units:
            u_(None)
    with jax.named_scope("BII"):
        lax.fori_loop(0, S // T2, lambda i, c: (b2_step(i), c)[1], 0)
    with jax.named_scope("out_wait"):
        for i in range(S // TS):
            for o_ in OUTS:
                out_copy(i * TS, *o_).wait()


@jax.jit
def pallas_adaLN_cond__ssm_conv_h3__mixer_s_mlp__prompt_kernel(
    A_q, A_k, A_v, A_shift_k, A_ssm_k, A_ssm_D, B_x, B_w1, B_w2, B_w3, B_w4, c, w_mod,
):
    del B_x
    hbm = pl.BlockSpec(memory_space=pltpu.MemorySpace.HBM)
    return pl.pallas_call(
        _kernel,
        out_shape=jax.ShapeDtypeStruct((1, S, D), bf16),
        in_specs=[hbm] * 12,
        out_specs=hbm,
        scratch_shapes=[
            pltpu.VMEM((27, 8, 128), f32),
            pltpu.VMEM((S + 16 * int(os.environ.get('PADF', '0')), D), bf16),
            pltpu.VMEM((NT, 32 + S // 2, 128), u32),
            pltpu.VMEM((NT, 32 + S // 2, 128), u32),
            pltpu.VMEM((NT, 64, S), u32),
            pltpu.VMEM((D // 2, D), u32),
            pltpu.VMEM((D // 2, D), u32),
            pltpu.VMEM((F // 2, D), u32),
            pltpu.VMEM((896, D), u32),
            pltpu.VMEM((2, D // 2, WMA), u32),
            pltpu.VMEM((D // 2, WMP), u32),
            pltpu.VMEM((D // 2, WMC), u32),
            pltpu.VMEM((S, D), bf16),
            pltpu.VMEM((NG * 2 * NC, 8, 128), f32),
            pltpu.VMEM((NG * 2 * NC, 8, 128), f32),
            pltpu.VMEM((NG * 2 * NC, 8, 128), f32),
            pltpu.VMEM((NG * 2 * NC, 8, 128), f32),
            pltpu.VMEM((KOFF + 56 + PADK, 8, 128), f32),
            pltpu.VMEM((KOFF + 56 + PADK, 8, 128), f32),
            pltpu.VMEM((NT, S, 128), f32),
            pltpu.VMEM((S, D), f32),
            pltpu.VMEM((S, D), f32),
            pltpu.VMEM((NT, S + 32, 128), f32),
            pltpu.VMEM((64, D), f32),
            pltpu.VMEM((1, TS, D), f32),
            pltpu.VMEM((1, TS, 1792), f32),
            pltpu.VMEM((49, 192, 128), u32),
            pltpu.VMEM((49, 192, 128), u32),
            pltpu.VMEM((7, 64, 256), u32),
            pltpu.VMEM((4, D), bf16),
            pltpu.VMEM((D,), bf16),
            pltpu.VMEM((1, D), bf16),
            pltpu.SMEM((2,), jnp.int32),
            pltpu.SemaphoreType.DMA((22,)),
            pltpu.SemaphoreType.DMA((1,)),
        ],
        compiler_params=pltpu.CompilerParams(vmem_limit_bytes=100 * 1024 * 1024, disable_semaphore_checks=True,
                                             disable_bounds_checks=bool(int(os.environ.get('NOBC', '0')))),
    )(A_q, A_k, A_v, A_shift_k.T, A_ssm_k, A_ssm_D, B_w1, B_w2, B_w3.T, B_w4, c, w_mod)
```

```python
import functools
import math
import os

import jax
import jax.numpy as jnp
from jax import lax
import jax.experimental.pallas as pl
import jax.experimental.pallas.tpu as pltpu

S, D, F = 2048, 640, 1728
C = 128
NC = S // C
NT = D // 128
NG = 16
KOFF = (NC + 1) * NG * 3
W = int(os.environ.get('W', '4'))
SKIPA = int(os.environ.get('SKIPA', '0'))
WMA, WMP, WMC = 1280, 640, 640
Q0 = int(os.environ.get('Q0', '320'))
N2 = int(os.environ.get('N2', '5'))
PRELN = int(os.environ.get('PRELN', '2'))
NOCACHE = int(os.environ.get('NOCACHE', '0'))
OUTWAIT = int(os.environ.get('OUTWAIT', '0'))
SEGS = [int(x) for x in os.environ.get('SEGS', '012345')]
SKIPB = int(os.environ.get('SKIPB', '0'))
PADK = int(os.environ.get('PADK', '0'))
PREW = int(os.environ.get('PREW', '0'))
SP = float(os.environ.get('SP', '0'))
MINS = int(os.environ.get('MINS', '30'))
GA = int(os.environ.get('GA', '2'))
TRT = int(os.environ.get('TRT', '1'))
LP = int(os.environ.get('LP', '1'))
FA = 1664
LPN = int(os.environ.get('LPN', '2'))
G0 = int(os.environ.get('G0', '4'))
Q1 = int(os.environ.get('Q1', '768'))
TIE4 = int(os.environ.get('TIE4', '12'))
STAG = os.environ.get('STAG', 'w02,l0,n,n')
OCOLS = ((0, 512), (512, 128))
FSTEP = int(os.environ.get('FSTEP', '1'))
FOFF = int(os.environ.get('FOFF', '0'))
KORD = int(os.environ.get('KORD', '0'))
CW = int(os.environ.get('CW', '128'))
NP4 = int(os.environ.get('NP4', '2'))
LNT = [int(x) for x in os.environ.get('LNT', '0,1,2,3,4,5,18,22').split(',')]
OPQ = int(os.environ.get('OPQ', '1'))
RELOAD = int(os.environ.get('RELOAD', '0'))
REMP = os.environ.get('REMP', '653765376537')
Q2 = int(os.environ.get('Q2', '1408'))
_u0, _u1, _un = [int(x) for x in os.environ.get('ANCH', '20,58,18').split(',')]
ANCH = sorted({(_u0 + (_u1 - _u0) * i // _un) % 80 for i in range(_un)})
XRB = [int(x) for x in os.environ.get('XRB', '7420')]
OPQ3 = int(os.environ.get('OPQ3', '1'))
SHST = int(os.environ.get('SHST', '1'))
KARA = int(os.environ.get('KARA', '1'))
UNR = int(os.environ.get('UNR', '2'))
HEAD = int(os.environ.get('HEAD', '250'))
TAIL = int(os.environ.get('TAIL', '450'))
DORDER = os.environ.get('DORDER', 'aHbU')
R1 = int(os.environ.get('R1', '64'))
R2 = int(os.environ.get('R2', '128'))
LEAD = int(os.environ.get('LEAD', '3'))
TS = int(os.environ.get('TS', '512'))
ONEPASS = int(os.environ.get('ONEPASS', '1'))
RSQ = int(os.environ.get('RSQ', '1'))
T2 = int(os.environ.get('T2', '512'))
EPS = 1e-5
_C0 = math.sqrt(2.0 / math.pi)
ALPHA = (_C0 * 0.044715) ** (1.0 / 3.0)
GC = _C0 / ALPHA
BETA = 0.5 / ALPHA
_fc = [int(x) for x in os.environ.get('FC', '1728').split(',')]
F_CHUNKS = tuple((sum(_fc[:i]), _fc[i]) for i in range(len(_fc)))
assert sum(_fc) == F

f32 = jnp.float32
bf16 = jnp.bfloat16
u32 = jnp.uint32
NTDIMS = (((1,), (1,)), ((), ()))


def _cos_table(m, scale):
    mm = jnp.abs(((m + 256) & 511) - 256)
    x = (128 - mm).astype(f32) * (1.0 / 128.0)
    x2 = x * x
    h = math.pi / 2
    p = -(h ** 7) / 5040 + x2 * ((h ** 9) / 362880 - x2 * (h ** 11) / 39916800)
    p = h + x2 * (-(h ** 3) / 6 + x2 * ((h ** 5) / 120 + x2 * p))
    return (x * scale) * p


def _dft_tables():
    shape = (16, 8, 128)
    n = lax.broadcasted_iota(jnp.int32, shape, 0)
    s = lax.broadcasted_iota(jnp.int32, shape, 1)
    l = lax.broadcasted_iota(jnp.int32, shape, 2)
    fw, fu, iv = [], [], []
    wv = l >> 4
    tu = (16 * W) * (wv // W) + (2 * W) * ((l >> 1) & 7) + 2 * (wv % W) + (l & 1)
    for e in range(2):
        r = 2 * s + e
        j = 8 * n + (r & 7)
        fw.append(_cos_table((4 * j + 1) * l + (r >> 3) * 128, 1.0))
        fu.append(_cos_table((4 * j + 1) * tu + (r >> 3) * 128, 1.0))
        b = 16 * (n >> 1) + r
        col = 128 * (n & 1) + l
        iv.append(_cos_table((4 * (col >> 1) + 1) * b + (col & 1) * 128, 1.0 / 128.0))
    pk = lambda xs: pltpu.bitcast(pltpu.pack_elementwise(xs, packed_dtype=bf16), f32)
    return pk(fw), pk(iv), pk(fu)


def _gelu2a(z):
    return z * (1.0 + jnp.tanh(z * (z * z + GC)))


def _rstd(ssd, scale):
    if RSQ == 0:
        r = lax.rsqrt(ssd * (1.0 / D) + EPS)
        return r if scale == 1.0 else r * scale
    return jnp.exp2(jnp.log(ssd + D * EPS) * (-0.5 / math.log(2.0)) + math.log2(scale * math.sqrt(D)))


def _center(x, scale=1.0):
    s1 = jnp.sum(x, axis=-1, keepdims=True)
    m = s1 * (1.0 / D)
    d = x - m
    if ONEPASS:
        ssd = jnp.maximum(jnp.sum(x * x, axis=-1, keepdims=True) - s1 * m, 0.0)
    else:
        ssd = jnp.sum(d * d, axis=-1, keepdims=True)
    return d, _rstd(ssd, scale)


def _conv(us, gs, a):
    acc = None
    for c in range(a + 1):
        p = us[c] * gs[a - c]
        acc = p if acc is None else acc + p
    return acc


_SA = (lambda a, b, c, d: a + d, lambda a, b, c, d: d, lambda a, b, c, d: c + d, lambda a, b, c, d: a,
       lambda a, b, c, d: a + b, lambda a, b, c, d: b - d, lambda a, b, c, d: c - a)
_SB = (lambda a, b, c, d: a + d, lambda a, b, c, d: c - a, lambda a, b, c, d: a, lambda a, b, c, d: b - d,
       lambda a, b, c, d: d, lambda a, b, c, d: c + d, lambda a, b, c, d: a + b)


_SC = (((0, 1), (3, 1)), ((0, 1), (2, 1)), ((2, 1), (3, -1)), ((1, 1), (3, 1)), ((0, -1), (1, 1)), ((0, 1),), ((3, 1),))
_SCL = (5, 4, 2, 6)


_SBU = ((1, 0, 0, 1), (1, 0, 1, 0), (1, 0, 0, 0), (0, 1, 0, 1), (0, 0, 0, 1), (0, 0, 1, 1), (1, 1, 0, 0))


def _comb(m):
    m1, m4, m2, m3, m5, m7, m6 = m
    return (m1 + m4) + (m7 - m5), m3 + m5, m4 + m2, (m1 + (m3 - m2)) + m6


class Lazy:
    def __init__(self, terms):
        self.terms = terms

    def __add__(self, o):
        return Lazy(self.terms + o.terms)

    def __sub__(self, o):
        return Lazy(self.terms + [(-s_, r_, c_) for (s_, r_, c_) in o.terms])

    def shift(self, dr, dc):
        return Lazy([(s_, r_ + dr, c_ + dc) for (s_, r_, c_) in self.terms])

    def load(self, ref, rn, cn):
        ts = sorted(self.terms, key=lambda t: -t[0])
        v = [ref[pl.ds(r_, rn), pl.ds(c_, cn)] for (_, r_, c_) in ts]
        acc_ = v[0]
        for (s_, _, _), x in zip(ts[1:], v[1:]):
            acc_ = acc_ + x if s_ > 0 else acc_ - x
        return acc_.astype(bf16)


def _mult(x, n):
    return x if isinstance(x, int) else pl.multiple_of(x, n)


def _wt(ref, *idx):
    return pltpu.bitcast(ref[idx] if idx else ref[...], bf16)


def _kernel(q_hbm, k_hbm, v_hbm, sk_hbm, h_hbm, dd_hbm, w1_hbm, w2_hbm, w3_hbm, w4_hbm,
            c_hbm, wm_hbm, o_hbm,
            modb, qbuf, kbuf, vbuf, hbuf, w1, w2, w3, w4, wm, wmp, wmc, obuf,
            ub0, ub1, gb0, gb1, kb0, kb1, yb, xn, hh, h1, par, l4p_, gs_, w4s, w3s, w4o, sk_s, dd_s, c_s, zs, sems, osems):
    l4p = l4p_.at[0]
    ubs, gbs, kbs = (ub0, ub1), (gb0, gb1), (kb0, kb1)
    cp = pltpu.make_async_copy
    HS = S // 2

    def cp_h(j, c0, c1, sem):
        return cp(h_hbm.at[pl.ds(j * 128, 128), pl.ds(c0, c1 - c0)], hbuf.bitcast(bf16).at[j, :, pl.ds(c0, c1 - c0)], sem)

    def cp_kv(j, r0, r1, sem):
        r0, r1 = (r0 + 16 if r0 else 0), min(r1 + 16, S)
        lanes = pl.ds(j * 128, 128)
        return [cp(k_hbm.at[0, pl.ds(r0, r1 - r0), lanes], kbuf.bitcast(bf16).at[j, pl.ds(r0 + 16, r1 - r0), :], sem),
                cp(v_hbm.at[0, pl.ds(r0, r1 - r0), lanes], vbuf.bitcast(bf16).at[j, pl.ds(r0, r1 - r0), :], sem)]

    def cp_tile(j, i):
        sem = sems.at[2 * j + i]
        return [cp_h(j, i * HS, (i + 1) * HS, sem)] + cp_kv(j, i * HS, (i + 1) * HS, sem)

    cp_t0 = [[cp_h(0, 0, S, sems.at[0])], cp_kv(0, 0, 1024, sems.at[1]), cp_kv(0, 1024, 1536, sems.at[20]),
             cp_kv(0, 1536, S, sems.at[21])]

    def cp_wm(i):
        return cp(wm_hbm.at[:, pl.ds(i * WMA, WMA)], wm.bitcast(bf16).at[i], sems.at[10 + i])

    cp_wmp = cp(wm_hbm.at[:, pl.ds(2 * WMA, WMP)], wmp.bitcast(bf16), sems.at[13])
    cp_wmc = cp(wm_hbm.at[:, pl.ds(2 * WMA + WMP, WMC)], wmc.bitcast(bf16), sems.at[12])
    cp_q = [cp(q_hbm.at[0, pl.ds(r0, r1 - r0), :], qbuf.at[pl.ds(r0, r1 - r0), :], sems.at[sm])
            for sm, r0, r1 in ((13, 0, Q0), (16, Q0, Q1), (14, Q1, Q2), (12, Q2, S))]
    cp_w = [cp(s_, d_.bitcast(bf16).at[pl.ds(0, s_.shape[0]), :], sems.at[sm])
            for sm, s_, d_ in ((15, w1_hbm, w1), (16, w2_hbm, w2), (12, w3_hbm, w3), (14, w4_hbm, w4))]
    cp_s = [cp(sk_hbm, sk_s, sems.at[19]), cp(dd_hbm, dd_s, sems.at[19]), cp(c_hbm, c_s, sems.at[19])]
    order = list(cp_s)
    for grp in cp_t0:
        order += grp
    for j in range(1, NT):
        order += cp_tile(j, 0) + cp_tile(j, 1)
    order += [cp_wm(0), cp_wm(1), cp_wmp, cp_q[0], cp_w[0], cp_w[1], cp_q[1], cp_q[2], cp_w[3], cp_q[3], cp_wmc, cp_w[2]]
    for c_ in order:
        c_.start()

    with jax.named_scope("init"):
        fw_t, iv_t, fu_t = _dft_tables()
        for kb in kbs:
            kb[pl.ds(KOFF, 16)] = fw_t
            kb[pl.ds(KOFF + 16, 16)] = iv_t
            kb[pl.ds(KOFF + 32, 16)] = fu_t
            kb[pl.ds(0, NG * 3)] = jnp.zeros((NG * 3, 8, 128), f32)
        zeros = jnp.zeros((8, 128), f32)
        w4[pl.ds(F // 2, 32), :] = jnp.zeros((32, D), u32)
        for j in range(NT):
            kbuf[j, pl.ds(0, 8), :] = jnp.zeros((8, 128), u32)
            kbuf[j, pl.ds(8 + HS, 8), :] = jnp.zeros((8, 128), u32)
            vbuf[j, pl.ds(HS, 8), :] = jnp.zeros((8, 128), u32)
        for j in range(NT):
            h1[j, pl.ds(8 if SHST else 0, 8), :] = zeros
            h1[j, pl.ds(S if SHST else S + 8, 8), :] = zeros
        for c_ in cp_s:
            c_.wait()
        par[pl.ds(0, 4), :] = sk_s[...].astype(f32)
        par[pl.ds(8, 8), :] = jnp.broadcast_to(dd_s[...].astype(f32).reshape(1, D), (8, D))
        cv = c_s[...].astype(f32)
        sc = jnp.broadcast_to(cv * jax.nn.sigmoid(cv), (8, D))
        scp = pltpu.bitcast(pltpu.pack_elementwise([sc, sc], packed_dtype=bf16), f32)
        for j in range(NT):
            kb0[KOFF + 48 + j] = scp[:, 128 * j:128 * (j + 1)]
            kb1[KOFF + 48 + j] = scp[:, 128 * j:128 * (j + 1)]

    def mkb(i, unr, off, cache):
        def b(stride, extra=0, z=None):
            if isinstance(i, int):
                return (i * unr + off) * stride + extra
            key = (unr * stride, z)
            if key not in cache or NOCACHE:
                base = pl.multiple_of(i * (unr * stride), unr * stride)
                cache[key] = base if z is None else base + (i >> z)
            return cache[key] + (off * stride + extra)
        return b

    def dot_h(j, b, lhs):
        gb = gbs[j % 2]
        hc = hbuf[j, :, pl.ds(_mult(b(512), 512), 512)]
        rhs_t = jnp.concatenate([hc[:, C * cc:C * (cc + 1)] for cc in range(4)], axis=0)
        g = lax.dot_general(lhs, pltpu.bitcast(rhs_t, bf16), NTDIMS, preferred_element_type=f32)
        for rg in range(2 * NG):
            for cc in range(4):
                gb[b(4, cc + rg * NC)] = g[8 * rg:8 * rg + 8, 128 * cc:128 * cc + 128]

    def dot_u(j, b, lhs):
        ub = ubs[j % 2]
        taps = [par[pl.ds(t, 1), pl.ds(j * 128, 128)] for t in range(4)]
        unp = lambda w_, e: pltpu.unpack_elementwise(w_, index=e, packed_dtype=bf16, unpacked_dtype=f32)
        cols = []
        for cc in range(4):
            words = []
            for blk in range(8 // W):
                w0 = 64 * cc + 8 * W * blk
                kw = {m: kbuf[j, pl.ds(b(256, 8 + w0 + m), 8, stride=W), :] for m in range(-2, W)}
                kk = {2 * m + e: unp(kw[m], e) for m in range(-2, W) for e in range(2) if 2 * m + e >= -3}
                for m in range(W):
                    vw = vbuf[j, pl.ds(b(256, w0 + m), 8, stride=W), :]
                    pair = []
                    for e in range(2):
                        n = 2 * m + e
                        ks = kk[n] * taps[0] + kk[n - 1] * taps[1] + kk[n - 2] * taps[2] + kk[n - 3] * taps[3]
                        pair.append(ks * unp(vw, e))
                    words.append(pltpu.pack_elementwise(pair, packed_dtype=bf16))
            cols.append(jnp.concatenate(words, axis=0))
        rhs = pltpu.bitcast(jnp.concatenate(cols, axis=1), bf16)
        u = jnp.dot(lhs, rhs, preferred_element_type=f32)
        for rg in range(2 * NG):
            for cc in range(4):
                ub[b(4, cc + rg * NC)] = u[8 * rg:8 * rg + 8, 128 * cc:128 * cc + 128]

    def dot_i(j, b, half, lhs):
        kb = kbs[j % 2]
        cols = [[], []]
        for gi in range(NG):
            prev = None
            for cc in range(-1, 2):
                k0, k1, k2 = [kb[b(4 * NG * 3, ((2 * half + cc + 1) * NG + gi) * 3 + t)] for t in range(3)]
                re, im = k0 - k2, k0 + k1
                if prev is not None:
                    cols[cc].append(pltpu.pack_elementwise([re - prev[1], im + prev[0]], packed_dtype=bf16))
                prev = (re, im)
        rhs = jnp.concatenate([jnp.concatenate(c_, axis=0) for c_ in cols], axis=1)
        y = jnp.dot(lhs, pltpu.bitcast(rhs, bf16), preferred_element_type=f32)
        for cc in range(2):
            yb[j, pl.ds(b(512, (2 * half + cc) * C), C), :] = y[:, 128 * cc:128 * cc + 128]

    def gen_m(j, kb, b, ng):
        ub, gb = ubs[j % 2], gbs[j % 2]
        for s in range(ng):
            for t in range(3):
                z = 8 + t
                re = lambda ref, c: ref[b(2 * NC, 2 * s * NC + c, z)]
                im = lambda ref, c: ref[b(2 * NC, (2 * s + 1) * NC + c, z)]
                gre = [re(gb, c) for c in range(NC)]
                if t == 0:
                    us = [re(ub, c) + im(ub, c) for c in range(NC)]
                    gs = gre
                elif t == 1:
                    us = [re(ub, c) for c in range(NC)]
                    gs = [im(gb, c) - gre[c] for c in range(NC)]
                else:
                    us = [im(ub, c) for c in range(NC)]
                    gs = [im(gb, c) + gre[c] for c in range(NC)]

                def st(a, val):
                    kb[b(3, ((a + 1) * NG + s) * 3 + t)] = val
                if not KARA:
                    for a in range(NC):
                        st(a, _conv(us, gs, a))
                        yield 2 * a + 2
                    continue
                ue, uo, ge, go = us[0::2], us[1::2], gs[0::2], gs[1::2]
                if KORD == 1:
                    usum = [x + y for x, y in zip(ue, uo)]
                    gsum = [x + y for x, y in zip(ge, go)]
                    poo = _conv(uo, go, NC // 2 - 1)
                    for a in reversed(range(NC // 2)):
                        pee = _conv(ue, ge, a)
                        pss = _conv(usum, gsum, a)
                        st(2 * a + 1, pss - pee - poo)
                        poo = _conv(uo, go, a - 1) if a else None
                        st(2 * a, pee + poo if a else pee)
                        yield 3 * (2 * a + 1) + (37 if a == NC // 2 - 1 else 3)
                    continue
                usum = [x + y for x, y in zip(ue, uo)]
                gsum = [x + y for x, y in zip(ge, go)]
                poo_prev = None
                for a in range(NC // 2):
                    pee = _conv(ue, ge, a)
                    poo = _conv(uo, go, a)
                    pss = _conv(usum, gsum, a)
                    st(2 * a, pee if poo_prev is None else pee + poo_prev)
                    st(2 * a + 1, pss - pee - poo)
                    poo_prev = poo
                    yield 3 * (2 * a + 1) + 7

    def add_d(j):
        gb = gbs[j % 2]
        dvec = par[pl.ds(8, 8), pl.ds(j * 128, 128)]
        for gi in range(NG):
            gb[2 * gi * NC] = gb[2 * gi * NC] + dvec

    def sc_lhs():
        return pltpu.bitcast(jnp.concatenate([kb0[KOFF + 48 + j] for j in range(NT)], axis=1), bf16)

    def dot_m(i, t0, nt, rows):
        m = None
        for kt in range(NT):
            p = jnp.dot(pltpu.bitcast(rows[kt], bf16), _wt(wm, i, pl.ds(64 * kt, 64), pl.ds(128 * t0, 128 * nt)),
                        preferred_element_type=f32)
            m = p if m is None else m + p
        for t in range(nt):
            modb[i * (WMA // 128) + (t0 + t)] = m[0:8, 128 * t:128 * (t + 1)]

    def inv_lhs(tbl, n):
        return jnp.concatenate([tbl[KOFF + 16 + 2 * n], tbl[KOFF + 17 + 2 * n]], axis=1)

    def dot_k(kb, kt, bt, lhs):
        cols = [[] for _ in range(4)]
        for gi in range(8 * kt, 8 * kt + 8):
            prev = None
            for cc in range(-1, 4):
                k0, k1, k2 = [kb[((4 * bt + cc + 1) * NG + gi) * 3 + t] for t in range(3)]
                re, im = k0 - k2, k0 + k1
                if prev is not None:
                    cols[cc].append(pltpu.pack_elementwise([re - prev[1], im + prev[0]], packed_dtype=bf16))
                prev = (re, im)
        rhs = jnp.concatenate([jnp.concatenate(c_, axis=0) for c_ in cols], axis=1)
        y = jnp.dot(lhs, pltpu.bitcast(rhs, bf16), preferred_element_type=f32)
        for cc in range(4):
            rows = pl.ds((4 * bt + cc) * C, C)
            yc = y[:, 128 * cc:128 * cc + 128]
            yb[NT - 1, rows, :] = yc if kt == 0 else yb[NT - 1, rows, :] + yc

    PRE = dict(H=0, U=672 + 96 // W, a=192, b=192, m=0, k=176)
    POST = dict(H=0, U=0, a=4, b=4, m=2, k=0)
    NST = dict(H=16, U=16, a=8, b=8, m=5, k=8)
    GCOST = 3 * (248 if KARA else 272)

    def a_block(dots, mg=None, ng=0, tbl=kb0):
        native, dur = [], []
        for idx, (k_, _) in enumerate(dots):
            nxt = PRE[dots[idx + 1][0]] if idx + 1 < len(dots) else 0
            d_ = 2.0 if k_ == 'm' else 1.0
            native += [nxt / NST[k_] + POST[k_] * d_] * NST[k_]
            dur += [d_] * NST[k_]
        if mg is not None and dots:
            head = max(HEAD - PRE[dots[0][0]], 0)
            mtot = GCOST * ng - TAIL - head
            lvl = (mtot + sum(native)) / sum(dur)
            want = [max(lvl * d_ - x, 0.0) for x, d_ in zip(native, dur)]
            scale = mtot / sum(want)
            cum, tgt = [head], head
            for w_ in want:
                tgt += w_ * scale
                cum.append(tgt)
        done = 0.0
        step = 0
        for (k_, fn) in dots:
            rows = []
            for n in range(NST[k_]):
                if mg is not None and (n % FSTEP == 0 or k_ == 'm'):
                    while done < cum[min(step + FOFF, len(cum) - 1)]:
                        done += next(mg)
                step += 1
                if k_ in 'HU':
                    rows.append(tbl[KOFF + n + (32 if k_ == 'U' else 0)])
                elif k_ in 'ab':
                    rows.append(inv_lhs(tbl, n))
                elif k_ == 'k':
                    rows.append(tbl[KOFF + 16 + 2 * n])
                else:
                    rows.append(tbl[KOFF + 48 + n])
            fn(rows if k_ == 'm' else pltpu.bitcast(jnp.concatenate(rows, axis=0), bf16))
        if mg is not None:
            for _ in mg:
                pass

    def fdot(k_, j, b):
        if k_ == 'H':
            return (k_, lambda lhs: dot_h(j, b, lhs))
        if k_ == 'U':
            return (k_, lambda lhs: dot_u(j, b, lhs))
        return (k_, lambda lhs: dot_i(j, b, 0 if k_ == 'a' else 1, lhs))

    def wait_all(cps):
        for c_ in cps:
            c_.wait()

    def a_loop(jf, jm, ji, g0, ng):
        kinds = [k_ for k_ in DORDER if k_ in 'HU' or ji is not None]

        def body(i, carry):
            cache = {}
            zs[i] = 0
            dots = [fdot(k_, jf if k_ in 'HU' else ji, mkb(i, 2, s_, cache)) for s_ in range(2) for k_ in kinds]
            a_block(dots, gen_m(jm, kbs[jm % 2], mkb(i, ng, g0, cache), ng), ng, kbs[jm % 2])

            @pl.when(i == 0)
            def _():
                wait_all(cp_tile(jf, 1))
            return carry
        wait_all(cp_tile(jf, 0))
        lax.fori_loop(0, 2, body, 0)
        add_d(jf)

    sb_ = lambda bt: mkb(0, 1, bt, None)
    if SKIPA:
        a_block = lambda *a, **k: None
    with jax.named_scope("A_seg0"):
        wait_all(cp_t0[0])
        a_block([fdot('H', 0, sb_(bt)) for bt in range(4)])
        add_d(0)
        wait_all(cp_t0[1])
        a_block([fdot('U', 0, sb_(bt)) for bt in range(2)])
        for bt in (2, 3):
            wait_all(cp_t0[bt])
            a_block([fdot('U', 0, sb_(bt))])
    with jax.named_scope("A_m0"):
        def body_m0(i, carry):
            a_block([], gen_m(0, kb0, mkb(i, G0 // 2, 0, {}), G0 // 2))
            return carry
        if G0:
            lax.fori_loop(0, 2, body_m0, 0)
    for seg in range(1, NT):
        with jax.named_scope(f"A_seg{seg}"):
            if seg == 1:
                a_loop(1, 0, None, G0, (NG - G0) // 2)
            else:
                a_loop(seg, seg - 1, seg - 2, 0, 8)

    def mods(i):
        return [('m', lambda rows, t0=t0, nt=nt: dot_m(i, t0, nt, rows)) for (t0, nt) in ((0, 4), (4, 4), (8, 2))]

    with jax.named_scope("A_seg5a"):
        cp_wm(0).wait()
        zz = zs[1]

        @pl.when(zz == 0)
        def _():
            dots = [fdot(k_, NT - 2, sb_(bt)) for bt in range(4) for k_ in 'ab']
            mm = mods(0)
            dots = [mm[0]] + dots[0:2] + [mm[1]] + dots[2:4] + [mm[2]] + dots[4:]
            a_block(dots, gen_m(NT - 1, kb0, mkb(zz, 8, 0, {}), 8), 8, kb0)
    with jax.named_scope("A_seg5b"):
        cp_wm(1).wait()

        @pl.when(zz == 0)
        def _():
            dots = [('k', lambda lhs, bt=bt: dot_k(kb0, 0, bt, lhs)) for bt in range(4)]
            mm = mods(1)
            dots = [mm[0], dots[0], mm[1], dots[1], mm[2]] + dots[2:]
            a_block(dots, gen_m(NT - 1, kb1, mkb(zz, 8, 8, {}), 8), 8, kb1)

    def inv_last(bt):
        lhs = pltpu.bitcast(jnp.concatenate([kb0[KOFF + 17 + 2 * n] for n in range(8)], axis=0), bf16)
        dot_k(kb1, 1, bt, lhs)

    def modrow(k_):
        return jnp.concatenate([modb[NT * k_ + j] for j in range(NT)], axis=1)

    R = R1
    GP = R // 8

    def ln_chain(p):
        r = p * R
        pa, pb, pc, ps = [par[pl.ds(16 + 8 * t, 8), :][None] for t in range(4)]
        g3 = lambda x: x.reshape(GP, 8, D)
        q = g3(qbuf[pl.ds(r, R), :].astype(f32))
        d1, r1 = _center(q)
        y = g3(jnp.concatenate([yb[j, pl.ds(r, R), :] for j in range(NT)], axis=1))
        x = q + ((d1 * r1) * pa + pb) * y
        xn[pl.ds(r, R), :] = x.reshape(R, D)
        d2, r2 = _center(x)
        h = (d2 * r2) * pc + ps
        hh[pl.ds(r, R), :] = h.reshape(R, D)
        d3, r3 = _center(h, ALPHA)
        return (d3 * r3).reshape(R, D)

    def tie(w_, vs):
        t_ = pltpu.bitcast(vs[0], u32)
        for v_ in vs[1:]:
            t_ = t_ | pltpu.bitcast(v_, u32)
        return w_ | (t_ & kbuf[0, pl.ds(0, 8), :])

    def tied(wref, ties):
        if not ties:
            return _wt(wref)
        rbs = sorted({8 * (t % 5) + rb for (t, rb) in ties})
        rows, pos = [], 0
        for rb in rbs:
            if rb > pos:
                rows.append(wref[pl.ds(8 * pos, 8 * (rb - pos)), :])
            blk = []
            for n in range(NT):
                w_ = wref[pl.ds(8 * rb, 8), pl.ds(128 * n, 128)]
                vs = ties.get((5 * n + rb // 8, rb % 8))
                blk.append(tie(w_, vs) if vs else w_)
            rows.append(jnp.concatenate(blk, axis=1))
            pos = rb + 1
        if pos < 40:
            rows.append(wref[pl.ds(8 * pos, 8 * (40 - pos)), :])
        return pltpu.bitcast(jnp.concatenate(rows, axis=0), bf16)

    def w1_dot(p, l3, ties, fresh):
        if fresh and STAG:
            grp = lambda g: l3[8 * g:8 * g + 8, 0:128]
            lt = {}
            for pr, spec in enumerate(STAG.split(',')):
                vs = [grp(2 * pr), grp(2 * pr + 1)]
                if spec[0] == 'w':
                    ties.setdefault((int(spec[1]), int(spec[2])), []).extend(vs)
                elif spec[0] == 'l':
                    lt.setdefault(int(spec[1]), []).extend(vs)
            for pr, vs in lt.items():
                x = pltpu.bitcast(tie(pltpu.bitcast(l3[16 * pr:16 * pr + 8, 128:256], u32), vs), f32)
                mid = jnp.concatenate([l3[16 * pr:16 * pr + 8, 0:128], x, l3[16 * pr:16 * pr + 8, 256:]], axis=1)
                l3 = jnp.concatenate(([l3[:16 * pr]] if pr else []) + [mid, l3[16 * pr + 8:]], axis=0)
        z = jnp.dot(l3.astype(bf16), tied(w1, ties), preferred_element_type=f32)
        g = _gelu2a(z)
        if SHST:
            lane = lax.broadcasted_iota(jnp.int32, (R, 128), 1)
            for j, (o1, cut, o2) in enumerate(((1, 128, 0), (1, 32, -1), (-1, 64, 2), (2, 96, -2), (-2, 128, 0))):
                gj = g[:, j * 128:(j + 1) * 128]
                if cut == 128:
                    h1[j, pl.ds(p * R + 8 + o1, R), :] = gj
                else:
                    pltpu.store(h1.at[j, pl.ds(p * R + 8 + o1, R), :], gj, mask=lane < cut)
                    pltpu.store(h1.at[j, pl.ds(p * R + 8 + o2, R), :], gj, mask=lane >= cut)
            return z
        for j in range(NT):
            h1[j, pl.ds(p * R + 8, R), :] = g[:, j * 128:(j + 1) * 128]
        return z

    def w2_dot(p, ties):
        r = p * R
        lane = lax.broadcasted_iota(jnp.int32, (R, 128), 1)

        def ld(j, off):
            return h1[j, pl.ds(r + 8 + off, R), :]
        tiles = [
            ld(0, -1),
            jnp.where(lane < 32, ld(1, -1), ld(1, 1)),
            jnp.where(lane < 64, ld(2, 1), ld(2, -2)),
            jnp.where(lane < 96, ld(3, -2), ld(3, 2)),
            ld(4, 2),
        ]
        if SHST:
            tiles = [ld(j, 0) for j in range(NT)]
        hs = jnp.concatenate(tiles, axis=1).astype(bf16)
        x1 = hh[pl.ds(r, R), :] + jnp.dot(hs, tied(w2, ties), preferred_element_type=f32) * BETA
        hh[pl.ds(r, R), :] = x1
        return x1

    unp = lambda w_, e: pltpu.unpack_elementwise(w_, index=e, packed_dtype=bf16, unpacked_dtype=f32)
    pk = lambda xs: pltpu.pack_elementwise(xs, packed_dtype=bf16)
    PURE = {7 * p_ + q_: 2 * i_ + j_ for i_, p_ in enumerate((2, 4)) for j_, q_ in enumerate((2, 4))}

    zoff = [pl.multiple_of((zz >> p_) * 32, 32) for p_ in range(7)]

    def prep2(src, dst, tr, t, p_, anchor):
        zero = None if anchor is None else pltpu.bitcast(anchor, u32) & kbuf[0, pl.ds(0, 8), :]
        gate = 0 if _SBU[p_][0] else 3
        l1 = [[], []]
        for k2 in range(2):
            for n2 in range(2):
                bl = []
                for b_ in range(4):
                    kq, nq = 2 * (b_ // 2) + k2, 2 * (b_ % 2) + n2
                    x = None
                    if _SBU[p_][b_]:
                        x = src[pl.ds(zoff[p_] + (8 * t + 192 * (nq if tr else kq)), 8), pl.ds(128 * (kq if tr else nq), 128)]
                        if zero is not None and b_ == gate and k2 == n2:
                            x = x | zero
                    bl.append(x)
                for e in range(2):
                    l1[e].append(_SB[p_](*[None if x is None else unp(x, e) for x in bl]))
        for q_ in range(7):
            if 7 * p_ + q_ not in PURE:
                dst[7 * p_ + q_, pl.ds(8 * t, 8), :] = pk([_SB[q_](*l1[e]) for e in range(2)])

    def prep1(t, n, anchor):
        bl = [w4[pl.ds(lo + 8 * t, 8), pl.ds(c0 + 128 * n, 128)] for lo in (768, 832) for c0 in (0, 256)]
        if anchor is not None:
            zero = pltpu.bitcast(anchor, u32) & kbuf[0, pl.ds(0, 8), :]
            bl[0], bl[3] = bl[0] | zero, bl[3] | zero
        for p_ in (0, 1, 3, 5, 6):
            w4o[p_, pl.ds(8 * t, 8), pl.ds(128 * n, 128)] = pk([_SB[p_](*[unp(x, e) for x in bl]) for e in range(2)])

    units = []
    l3s = {}

    def ln4(r, n):
        d4, r4 = _center(hh[pl.ds(r, n), :], ALPHA)
        return d4 * r4

    def run_block(dots, extra=None, pre4=False):
        for d_, (k_, p) in enumerate(dots):
            ties = {}
            e = d_ - (len(dots) - NP4)
            RP = TS // NP4
            if pre4 and e >= 0:
                nx = ln4(e * RP, RP)
                l4p[pl.ds(e * RP, RP), :] = nx
                ties[(TIE4, 7)] = [nx[8 * g:8 * g + 8, 0:128] for g in range(RP // 8)]
            if extra is not None and d_ == len(dots) - 1:
                nx = ln_chain(extra)
                for pr in range(4):
                    ties[(24, XRB[pr])] = [nx[16 * pr:16 * pr + 8, 0:128], nx[16 * pr + 8:16 * pr + 16, 0:128]]
                l3s[extra] = nx.astype(bf16)
            if k_ == 1:
                fresh = p not in l3s
                res = w1_dot(p, ln_chain(p) if fresh else l3s.pop(p), ties, fresh)
            elif k_ == 2:
                res = w2_dot(p, ties)
            else:
                par[pl.ds(48, 8), :] = jnp.dot(sc_lhs(), _wt(wmc), preferred_element_type=f32)[0:8]
            for u_ in ANCH:
                if u_ // 40 + 1 == k_ and units and d_ < len(dots) - (NP4 + 1 if pre4 else 0):
                    n, g = (u_ % 40) // 8, u_ % 8
                    units.pop(0)(res[8 * g:8 * g + 8, 128 * n:128 * (n + 1)])

    with jax.named_scope("P1"):
        cp_wmp.wait()
        cp_q[0].wait()
        mp = jnp.dot(sc_lhs(), _wt(wmp), preferred_element_type=f32)
        for t in range(WMP // 128):
            modb[2 * WMA // 128 + t] = mp[0:8, 128 * t:128 * (t + 1)]
        sa, ca, ga, sb, cb = [modrow(k_) for k_ in range(5)]
        par[pl.ds(16, 8), :] = ga * (1.0 + ca)
        par[pl.ds(24, 8), :] = ga * sa
        par[pl.ds(32, 8), :] = 1.0 + cb
        par[pl.ds(40, 8), :] = sb
        for bt in range(4):
            inv_last(bt)
        for p in range(PRELN):
            l3s[p] = ln_chain(p)
    with jax.named_scope("w1wait"):
        cp_w[0].wait()
    p1, p2 = N2, 0
    with jax.named_scope("P2"):
        run_block([(1, p) for p in range(N2)])
    with jax.named_scope("w2wait"):
        wait_all([cp_w[1], cp_q[1]])

    def plan(lim1):
        nonlocal p1, p2
        last = lim1 == S // R
        dots = []
        while p1 < (lim1 if last else lim1 - 1) or p1 - p2 >= LEAD or (last and p2 < lim1):
            if p1 - p2 < LEAD and p1 < lim1:
                dots.append((1, p1))
                p1 += 1
            else:
                dots.append((2, p2))
                p2 += 1
        return dots, (None if last else p1)

    with jax.named_scope("P4"):
        run_block(*plan(Q1 // R))
    with jax.named_scope("q2wait"):
        wait_all([cp_q[2], cp_w[3]])
    units += [functools.partial(prep2, w4, w4s, False, t, p_) for t in range(24) for p_ in range(7)]
    units += [functools.partial(prep1, t, n) for t in range(8) for n in range(2)]
    with jax.named_scope("P5"):
        run_block(*plan(Q2 // R))
    with jax.named_scope("q3wait"):
        wait_all([cp_q[3], cp_wmc, cp_w[2]])
    units += [functools.partial(prep2, w3, w3s, True, t, p_) for t in range(24) for p_ in range(7)]
    with jax.named_scope("P6"):
        dots, _ = plan(S // R)
        run_block(dots[:-NP4] + [(3, 0)] + dots[-NP4:], pre4=True)

    H2 = TS // 2
    OUTS = ((0, H2, 512, 128), (H2, H2, 0, 256), (0, H2, 256, 256), (0, H2, 0, 256), (H2, H2, 256, 256), (H2, H2, 512, 128))

    def out_copy(r, r0, rn, c0, cn):
        rows = pl.ds(_mult(r + r0, H2), rn)
        return cp(obuf.at[rows, pl.ds(c0, cn)], o_hbm.at[0, rows, pl.ds(c0, cn)], osems.at[0])

    def wsum(x, y, sign):
        unp = lambda w_, e: pltpu.unpack_elementwise(w_, index=e, packed_dtype=bf16, unpacked_dtype=f32)
        return pltpu.pack_elementwise([unp(x, e) + unp(y, e) if sign > 0 else unp(x, e) - unp(y, e) for e in range(2)],
                                      packed_dtype=bf16)

    def strassen_lhs(a11, a12, a21, a22):
        c = lambda x: x.astype(bf16)
        return (c(a11 + a22), c(a21 + a22), c(a11), c(a22), c(a11 + a12), c(a21 - a11), c(a12 - a22))

    def strassen(ops, b11, b12, b21, b22, mm, ties=None):
        def tw(k_, w_):
            if not ties or k_ not in ties:
                return w_
            return jnp.concatenate([tie(w_[0:8], ties[k_]), w_[8:]], axis=0)
        m1 = mm(ops[0], tw(0, wsum(b11, b22, 1)))
        m4 = mm(ops[3], tw(1, wsum(b21, b11, -1)))
        m2 = mm(ops[1], tw(2, b11))
        m3 = mm(ops[2], tw(3, wsum(b12, b22, -1)))
        m5 = mm(ops[4], tw(4, b22))
        m7 = mm(ops[6], tw(5, wsum(b21, b22, 1)))
        m6 = mm(ops[5], tw(6, wsum(b11, b12, 1)))
        return (m1 + m4) + (m7 - m5), m3 + m5, m4 + m2, (m1 + (m3 - m2)) + m6

    mm_nt = lambda x, w_: lax.dot_general(x, pltpu.bitcast(w_, bf16), NTDIMS, preferred_element_type=f32)
    mm_nn = lambda x, w_: jnp.dot(x, pltpu.bitcast(w_, bf16), preferred_element_type=f32)

    def b2_step(i):
        gbv = par[pl.ds(48, 8), :]
        nsub = T2 // TS
        for sub in range(nsub):
            r = pl.multiple_of(pl.multiple_of(i * T2, T2) + sub * TS, TS)
            gs = gs_.at[i >> 8]
            l4 = l4p[...] if sub == 0 else ln4(r, TS)
            lb = l4.astype(bf16)
            zt = lax.dot_general(_wt(w3, pl.ds(832, 32), slice(None)), lb, NTDIMS, preferred_element_type=f32)
            g12 = _gelu2a(mm_nt(lb, w3[pl.ds(768, 64), :]))
            gt = jnp.concatenate([_gelu2a(zt), jnp.zeros((64, TS), f32)], axis=0).T
            gs[:, pl.ds(0, 128)] = g12
            gs[:, pl.ds(896, 128)] = gt
            lrs = [l4[:H2, 512:640].astype(bf16), l4[H2:, 512:640].astype(bf16)]
            Q = H2 // 2
            ab = [Lazy([(1, r_, c_)]) for (r_, c_) in ((0, 0), (0, 256), (H2, 0), (H2, 256))]
            opsA = {}
            rn_ = pl.multiple_of(jnp.minimum(i + 1, S // T2 - 1) * T2, T2)
            RP = TS // len(LNT)
            l4n = l4p
            for t in range(3):
                cq, left = [None] * 4, [5, 3, 3, 5]

                def add(k_, x, sg=1):
                    cq[k_] = x if cq[k_] is None else cq[k_] + x if sg > 0 else cq[k_] - x
                    left[k_] -= 1
                    if left[k_] == 0:
                        gg = _gelu2a(cq[k_])
                        for n2 in range(2):
                            gs[pl.ds(H2 * (k_ // 2), H2), pl.ds(128 + 896 * (k_ % 2) + 128 * (t + 3 * n2), 128)] = gg[:, 128 * n2:128 * (n2 + 1)]

                def rem(k_):
                    wr = jnp.concatenate([w3[pl.ds(64 * (t + 3 * (2 * (k_ % 2) + n2)), 64), pl.ds(512, 128)] for n2 in range(2)], axis=0)
                    add(k_, mm_nt(lrs[k_ // 2], wr))
                for p_ in range(8):
                    for k_ in (2, 1, 0, 3):
                        if int(REMP[4 * t + k_]) == p_:
                            rem(k_)
                    if p_ == 7:
                        break
                    a_ = _SA[p_](*ab)
                    sub_ = (a_, a_.shift(0, 128), a_.shift(Q, 0), a_.shift(Q, 128))
                    pr = []
                    for q_ in range(7):
                        n = 7 * p_ + q_
                        if n not in opsA or RELOAD:
                            opsA[n] = _SA[q_](*sub_).load(l4p_.at[(i + 4 * p_ + 32 * t) >> (9 + q_)] if RELOAD or OPQ3 else l4p, Q, 128)
                        w_ = w3[pl.ds(192 * PURE[n] + 64 * t, 64), pl.ds(128 * PURE[n], 128)] if n in PURE else w3s[n, pl.ds(64 * t, 64), :]
                        pr.append(mm_nt(opsA[n], w_))
                    c11, c12, c21, c22 = _comb(pr)
                    m_ = jnp.concatenate([jnp.concatenate([c11, c12], axis=1), jnp.concatenate([c21, c22], axis=1)], axis=0)
                    for k_, sg in _SC[p_]:
                        add(k_, m_, sg)
            kord = [0, 896] + [o_ for c in (0, 3, 1, 4, 2, 5) for o_ in (128 + 128 * c, 1024 + 128 * c)]
            wrow = lambda o_: 768 if o_ == 0 else 832 if o_ == 896 else (o_ - 128) // 2 if o_ < 896 else 384 + (o_ - 1024) // 2
            wl = jnp.concatenate([w4[pl.ds(wrow(o_), 64), pl.ds(512, 128)] for o_ in kord], axis=0)
            gk = lambda r0: jnp.concatenate([gs[pl.ds(r0, H2), pl.ds(o_, 128)] for o_ in kord], axis=1).astype(bf16)
            acc_t = mm_nn(gk(0), wl)
            ties = {}
            for e, k_ in enumerate(LNT):
                nx = ln4(pl.multiple_of(rn_ + e * RP, RP), RP)
                l4n[pl.ds(e * RP, RP), :] = nx
                ties[k_] = [nx[8 * gi:8 * gi + 8, 0:128] for gi in range(RP // 8)]
            Q = H2 // 2

            blocks = [Lazy([(1, r_, c_)]) for (r_, c_) in ((0, 0), (0, 896), (H2, 0), (H2, 896))]
            ms = []
            for p_ in range(7):
                a_ = _SA[p_](*blocks)
                wo = w4[pl.ds(768, 64), pl.ds(0, 256)] if p_ == 2 else w4[pl.ds(832, 64), pl.ds(256, 256)] if p_ == 4 else w4o[p_]
                w4n = lambda n: w4[pl.ds(192 * PURE[n], 192), pl.ds(128 * PURE[n], 128)] if n in PURE else w4s[n, pl.ds(0, 192), :]
                if p_ in ties:
                    wo = jnp.concatenate([jnp.concatenate([tie(wo[0:8, 0:128], ties[p_]), wo[0:8, 128:]], axis=1), wo[8:]], axis=0)
                m_ = mm_nn(a_.load(gs, H2, 128), wo)
                sub_ = (a_.shift(0, 128), a_.shift(0, 512), a_.shift(Q, 128), a_.shift(Q, 512))
                gref = lambda q_: gs_.at[(i + 4 * p_) >> (9 + q_)] if OPQ else gs
                c11, c12, c21, c22 = _comb([mm_nn(_SA[q_](*sub_).load(gref(q_), Q, 384), w4n(7 * p_ + q_)) for q_ in range(7)])
                ms.append(m_ + jnp.concatenate([jnp.concatenate([c11, c12], axis=1), jnp.concatenate([c21, c22], axis=1)], axis=0))
            c11, c12, c21, c22 = _comb(ms)
            for k_ in ties:
                if k_ >= 10:
                    o_ = 64 * (k_ - 10)
                    wl = jnp.concatenate([wl[:o_], tie(wl[o_:o_ + 8], ties[k_]), wl[o_ + 8:]], axis=0)
            accs = (acc_t, c21, c12, c11, c22, mm_nn(gk(H2), wl))
            for (r0, rn, c0, cn), ac in zip(OUTS, accs):
                rows, cols = pl.ds(_mult(r + r0, H2), rn), pl.ds(c0, cn)
                g3 = lambda x: x.reshape(rn // 8, 8, cn)
                out = g3(xn[rows, cols]) + gbv[None, :, c0:c0 + cn] * g3(hh[rows, cols] + BETA * ac)
                obuf[rows, cols] = out.reshape(rn, cn).astype(bf16)
                out_copy(r, r0, rn, c0, cn).start()

    with jax.named_scope("prep"):
        print("left-over prep units:", len(units))
        for u_ in units:
            u_(None)
    with jax.named_scope("BII"):
        lax.fori_loop(0, S // T2, lambda i, c: (b2_step(i), c)[1], 0)
    with jax.named_scope("out_wait"):
        for i in range(S // TS):
            for o_ in OUTS:
                out_copy(i * TS, *o_).wait()


@jax.jit
def pallas_adaLN_cond__ssm_conv_h3__mixer_s_mlp__prompt_kernel(
    A_q, A_k, A_v, A_shift_k, A_ssm_k, A_ssm_D, B_x, B_w1, B_w2, B_w3, B_w4, c, w_mod,
):
    del B_x
    hbm = pl.BlockSpec(memory_space=pltpu.MemorySpace.HBM)
    return pl.pallas_call(
        _kernel,
        out_shape=jax.ShapeDtypeStruct((1, S, D), bf16),
        in_specs=[hbm] * 12,
        out_specs=hbm,
        scratch_shapes=[
            pltpu.VMEM((27, 8, 128), f32),
            pltpu.VMEM((S + 16 * int(os.environ.get('PADF', '0')), D), bf16),
            pltpu.VMEM((NT, 32 + S // 2, 128), u32),
            pltpu.VMEM((NT, 32 + S // 2, 128), u32),
            pltpu.VMEM((NT, 64, S), u32),
            pltpu.VMEM((D // 2, D), u32),
            pltpu.VMEM((D // 2, D), u32),
            pltpu.VMEM((F // 2, D), u32),
            pltpu.VMEM((896, D), u32),
            pltpu.VMEM((2, D // 2, WMA), u32),
            pltpu.VMEM((D // 2, WMP), u32),
            pltpu.VMEM((D // 2, WMC), u32),
            pltpu.VMEM((S, D), bf16),
            pltpu.VMEM((NG * 2 * NC, 8, 128), f32),
            pltpu.VMEM((NG * 2 * NC, 8, 128), f32),
            pltpu.VMEM((NG * 2 * NC, 8, 128), f32),
            pltpu.VMEM((NG * 2 * NC, 8, 128), f32),
            pltpu.VMEM((KOFF + 56 + PADK, 8, 128), f32),
            pltpu.VMEM((KOFF + 56 + PADK, 8, 128), f32),
            pltpu.VMEM((NT, S, 128), f32),
            pltpu.VMEM((S, D), f32),
            pltpu.VMEM((S, D), f32),
            pltpu.VMEM((NT, S + 32, 128), f32),
            pltpu.VMEM((64, D), f32),
            pltpu.VMEM((1, TS, D), f32),
            pltpu.VMEM((1, TS, 1792), f32),
            pltpu.VMEM((52, 200, 128), u32),
            pltpu.VMEM((52, 200, 128), u32),
            pltpu.VMEM((7, 64, 256), u32),
            pltpu.VMEM((4, D), bf16),
            pltpu.VMEM((D,), bf16),
            pltpu.VMEM((1, D), bf16),
            pltpu.SMEM((2,), jnp.int32),
            pltpu.SemaphoreType.DMA((22,)),
            pltpu.SemaphoreType.DMA((1,)),
        ],
        compiler_params=pltpu.CompilerParams(vmem_limit_bytes=100 * 1024 * 1024, disable_semaphore_checks=True,
                                             disable_bounds_checks=bool(int(os.environ.get('NOBC', '0')))),
    )(A_q, A_k, A_v, A_shift_k.T, A_ssm_k, A_ssm_D, B_w1, B_w2, B_w3.T, B_w4, c, w_mod)
```

```python
import functools
import math
import os

import jax
import jax.numpy as jnp
from jax import lax
import jax.experimental.pallas as pl
import jax.experimental.pallas.tpu as pltpu

S, D, F = 2048, 640, 1728
C = 128
NC = S // C
NT = D // 128
NG = 16
KOFF = (NC + 1) * NG * 3
W = int(os.environ.get('W', '4'))
SKIPA = int(os.environ.get('SKIPA', '0'))
WMA, WMP, WMC = 1280, 640, 640
Q0 = int(os.environ.get('Q0', '320'))
N2 = int(os.environ.get('N2', '5'))
PRELN = int(os.environ.get('PRELN', '2'))
NOCACHE = int(os.environ.get('NOCACHE', '0'))
OUTWAIT = int(os.environ.get('OUTWAIT', '0'))
SEGS = [int(x) for x in os.environ.get('SEGS', '012345')]
SKIPB = int(os.environ.get('SKIPB', '0'))
PADK = int(os.environ.get('PADK', '0'))
PREW = int(os.environ.get('PREW', '0'))
SP = float(os.environ.get('SP', '0'))
MINS = int(os.environ.get('MINS', '30'))
GA = int(os.environ.get('GA', '2'))
TRT = int(os.environ.get('TRT', '1'))
LP = int(os.environ.get('LP', '1'))
FA = 1664
LPN = int(os.environ.get('LPN', '2'))
G0 = int(os.environ.get('G0', '4'))
Q1 = int(os.environ.get('Q1', '768'))
TIE4 = int(os.environ.get('TIE4', '12'))
STAG = os.environ.get('STAG', 'w02,l0,n,n')
OCOLS = ((0, 512), (512, 128))
FSTEP = int(os.environ.get('FSTEP', '1'))
FOFF = int(os.environ.get('FOFF', '0'))
KORD = int(os.environ.get('KORD', '0'))
CW = int(os.environ.get('CW', '128'))
NP4 = int(os.environ.get('NP4', '2'))
LNT = [int(x) for x in os.environ.get('LNT', '0,1,2,3,4,5,18,22').split(',')]
OPQ = int(os.environ.get('OPQ', '1'))
RELOAD = int(os.environ.get('RELOAD', '0'))
REMP = os.environ.get('REMP', '653765376537')
Q2 = int(os.environ.get('Q2', '1408'))
_u0, _u1, _un = [int(x) for x in os.environ.get('ANCH', '20,58,18').split(',')]
ANCH = sorted({(_u0 + (_u1 - _u0) * i // _un) % 80 for i in range(_un)})
XRB = [int(x) for x in os.environ.get('XRB', '7420')]
OPQ3 = int(os.environ.get('OPQ3', '1'))
SHST = int(os.environ.get('SHST', '1'))
KARA = int(os.environ.get('KARA', '1'))
UNR = int(os.environ.get('UNR', '2'))
HEAD = int(os.environ.get('HEAD', '250'))
TAIL = int(os.environ.get('TAIL', '450'))
DORDER = os.environ.get('DORDER', 'aHbU')
R1 = int(os.environ.get('R1', '64'))
R2 = int(os.environ.get('R2', '128'))
LEAD = int(os.environ.get('LEAD', '3'))
TS = int(os.environ.get('TS', '512'))
ONEPASS = int(os.environ.get('ONEPASS', '1'))
RSQ = int(os.environ.get('RSQ', '1'))
T2 = int(os.environ.get('T2', '512'))
EPS = 1e-5
_C0 = math.sqrt(2.0 / math.pi)
ALPHA = (_C0 * 0.044715) ** (1.0 / 3.0)
GC = _C0 / ALPHA
BETA = 0.5 / ALPHA
_fc = [int(x) for x in os.environ.get('FC', '1728').split(',')]
F_CHUNKS = tuple((sum(_fc[:i]), _fc[i]) for i in range(len(_fc)))
assert sum(_fc) == F

f32 = jnp.float32
bf16 = jnp.bfloat16
u32 = jnp.uint32
NTDIMS = (((1,), (1,)), ((), ()))


def _cos_table(m, scale):
    mm = jnp.abs(((m + 256) & 511) - 256)
    x = (128 - mm).astype(f32) * (1.0 / 128.0)
    x2 = x * x
    h = math.pi / 2
    p = -(h ** 7) / 5040 + x2 * ((h ** 9) / 362880 - x2 * (h ** 11) / 39916800)
    p = h + x2 * (-(h ** 3) / 6 + x2 * ((h ** 5) / 120 + x2 * p))
    return (x * scale) * p


def _dft_tables():
    shape = (16, 8, 128)
    n = lax.broadcasted_iota(jnp.int32, shape, 0)
    s = lax.broadcasted_iota(jnp.int32, shape, 1)
    l = lax.broadcasted_iota(jnp.int32, shape, 2)
    fw, fu, iv = [], [], []
    wv = l >> 4
    tu = (16 * W) * (wv // W) + (2 * W) * ((l >> 1) & 7) + 2 * (wv % W) + (l & 1)
    for e in range(2):
        r = 2 * s + e
        j = 8 * n + (r & 7)
        fw.append(_cos_table((4 * j + 1) * l + (r >> 3) * 128, 1.0))
        fu.append(_cos_table((4 * j + 1) * tu + (r >> 3) * 128, 1.0))
        b = 16 * (n >> 1) + r
        col = 128 * (n & 1) + l
        iv.append(_cos_table((4 * (col >> 1) + 1) * b + (col & 1) * 128, 1.0 / 128.0))
    pk = lambda xs: pltpu.bitcast(pltpu.pack_elementwise(xs, packed_dtype=bf16), f32)
    return pk(fw), pk(iv), pk(fu)


def _gelu2a(z):
    return z * (1.0 + jnp.tanh(z * (z * z + GC)))


def _rstd(ssd, scale):
    if RSQ == 0:
        r = lax.rsqrt(ssd * (1.0 / D) + EPS)
        return r if scale == 1.0 else r * scale
    return jnp.exp2(jnp.log(ssd + D * EPS) * (-0.5 / math.log(2.0)) + math.log2(scale * math.sqrt(D)))


def _center(x, scale=1.0):
    s1 = jnp.sum(x, axis=-1, keepdims=True)
    m = s1 * (1.0 / D)
    d = x - m
    if ONEPASS:
        ssd = jnp.maximum(jnp.sum(x * x, axis=-1, keepdims=True) - s1 * m, 0.0)
    else:
        ssd = jnp.sum(d * d, axis=-1, keepdims=True)
    return d, _rstd(ssd, scale)


def _conv(us, gs, a):
    acc = None
    for c in range(a + 1):
        p = us[c] * gs[a - c]
        acc = p if acc is None else acc + p
    return acc


_SA = (lambda a, b, c, d: a + d, lambda a, b, c, d: d, lambda a, b, c, d: c + d, lambda a, b, c, d: a,
       lambda a, b, c, d: a + b, lambda a, b, c, d: b - d, lambda a, b, c, d: c - a)
_SB = (lambda a, b, c, d: a + d, lambda a, b, c, d: c - a, lambda a, b, c, d: a, lambda a, b, c, d: b - d,
       lambda a, b, c, d: d, lambda a, b, c, d: c + d, lambda a, b, c, d: a + b)


_SC = (((0, 1), (3, 1)), ((0, 1), (2, 1)), ((2, 1), (3, -1)), ((1, 1), (3, 1)), ((0, -1), (1, 1)), ((0, 1),), ((3, 1),))
_SCL = (5, 4, 2, 6)


_SBU = ((1, 0, 0, 1), (1, 0, 1, 0), (1, 0, 0, 0), (0, 1, 0, 1), (0, 0, 0, 1), (0, 0, 1, 1), (1, 1, 0, 0))


def _comb(m):
    m1, m4, m2, m3, m5, m7, m6 = m
    return (m1 + m4) + (m7 - m5), m3 + m5, m4 + m2, (m1 + (m3 - m2)) + m6


class Lazy:
    def __init__(self, terms):
        self.terms = terms

    def __add__(self, o):
        return Lazy(self.terms + o.terms)

    def __sub__(self, o):
        return Lazy(self.terms + [(-s_, r_, c_) for (s_, r_, c_) in o.terms])

    def shift(self, dr, dc):
        return Lazy([(s_, r_ + dr, c_ + dc) for (s_, r_, c_) in self.terms])

    def load(self, ref, rn, cn):
        ts = sorted(self.terms, key=lambda t: -t[0])
        v = [ref[pl.ds(r_, rn), pl.ds(c_, cn)] for (_, r_, c_) in ts]
        acc_ = v[0]
        for (s_, _, _), x in zip(ts[1:], v[1:]):
            acc_ = acc_ + x if s_ > 0 else acc_ - x
        return acc_.astype(bf16)


def _mult(x, n):
    return x if isinstance(x, int) else pl.multiple_of(x, n)


def _wt(ref, *idx):
    return pltpu.bitcast(ref[idx] if idx else ref[...], bf16)


def _kernel(q_hbm, k_hbm, v_hbm, sk_hbm, h_hbm, dd_hbm, w1_hbm, w2_hbm, w3_hbm, w4_hbm,
            c_hbm, wm_hbm, o_hbm,
            modb, qbuf, kbuf, vbuf, hbuf, w1, w2, w3, w4, wm, wmp, wmc, obuf,
            ub0, ub1, gb0, gb1, kb0, kb1, yb, xn, hh, h1, par, l4p_, gs_, w4s, w3s, w4o, w3o, sk_s, dd_s, c_s, zs, sems, osems):
    l4p = l4p_.at[0]
    ubs, gbs, kbs = (ub0, ub1), (gb0, gb1), (kb0, kb1)
    cp = pltpu.make_async_copy
    HS = S // 2

    def cp_h(j, c0, c1, sem):
        return cp(h_hbm.at[pl.ds(j * 128, 128), pl.ds(c0, c1 - c0)], hbuf.bitcast(bf16).at[j, :, pl.ds(c0, c1 - c0)], sem)

    def cp_kv(j, r0, r1, sem):
        r0, r1 = (r0 + 16 if r0 else 0), min(r1 + 16, S)
        lanes = pl.ds(j * 128, 128)
        return [cp(k_hbm.at[0, pl.ds(r0, r1 - r0), lanes], kbuf.bitcast(bf16).at[j, pl.ds(r0 + 16, r1 - r0), :], sem),
                cp(v_hbm.at[0, pl.ds(r0, r1 - r0), lanes], vbuf.bitcast(bf16).at[j, pl.ds(r0, r1 - r0), :], sem)]

    def cp_tile(j, i):
        sem = sems.at[2 * j + i]
        return [cp_h(j, i * HS, (i + 1) * HS, sem)] + cp_kv(j, i * HS, (i + 1) * HS, sem)

    cp_t0 = [[cp_h(0, 0, S, sems.at[0])], cp_kv(0, 0, 1024, sems.at[1]), cp_kv(0, 1024, 1536, sems.at[20]),
             cp_kv(0, 1536, S, sems.at[21])]

    def cp_wm(i):
        return cp(wm_hbm.at[:, pl.ds(i * WMA, WMA)], wm.bitcast(bf16).at[i], sems.at[10 + i])

    cp_wmp = cp(wm_hbm.at[:, pl.ds(2 * WMA, WMP)], wmp.bitcast(bf16), sems.at[13])
    cp_wmc = cp(wm_hbm.at[:, pl.ds(2 * WMA + WMP, WMC)], wmc.bitcast(bf16), sems.at[12])
    cp_q = [cp(q_hbm.at[0, pl.ds(r0, r1 - r0), :], qbuf.at[pl.ds(r0, r1 - r0), :], sems.at[sm])
            for sm, r0, r1 in ((13, 0, Q0), (16, Q0, Q1), (14, Q1, Q2), (12, Q2, S))]
    cp_w = [cp(s_, d_.bitcast(bf16).at[pl.ds(0, s_.shape[0]), :], sems.at[sm])
            for sm, s_, d_ in ((15, w1_hbm, w1), (16, w2_hbm, w2), (12, w3_hbm, w3), (14, w4_hbm, w4))]
    cp_s = [cp(sk_hbm, sk_s, sems.at[19]), cp(dd_hbm, dd_s, sems.at[19]), cp(c_hbm, c_s, sems.at[19])]
    order = list(cp_s)
    for grp in cp_t0:
        order += grp
    for j in range(1, NT):
        order += cp_tile(j, 0) + cp_tile(j, 1)
    order += [cp_wm(0), cp_wm(1), cp_wmp, cp_q[0], cp_w[0], cp_w[1], cp_q[1], cp_q[2], cp_w[3], cp_q[3], cp_wmc, cp_w[2]]
    for c_ in order:
        c_.start()

    with jax.named_scope("init"):
        fw_t, iv_t, fu_t = _dft_tables()
        for kb in kbs:
            kb[pl.ds(KOFF, 16)] = fw_t
            kb[pl.ds(KOFF + 16, 16)] = iv_t
            kb[pl.ds(KOFF + 32, 16)] = fu_t
            kb[pl.ds(0, NG * 3)] = jnp.zeros((NG * 3, 8, 128), f32)
        zeros = jnp.zeros((8, 128), f32)
        w4[pl.ds(F // 2, 32), :] = jnp.zeros((32, D), u32)
        for j in range(NT):
            kbuf[j, pl.ds(0, 8), :] = jnp.zeros((8, 128), u32)
            kbuf[j, pl.ds(8 + HS, 8), :] = jnp.zeros((8, 128), u32)
            vbuf[j, pl.ds(HS, 8), :] = jnp.zeros((8, 128), u32)
        for j in range(NT):
            h1[j, pl.ds(8 if SHST else 0, 8), :] = zeros
            h1[j, pl.ds(S if SHST else S + 8, 8), :] = zeros
        for c_ in cp_s:
            c_.wait()
        par[pl.ds(0, 4), :] = sk_s[...].astype(f32)
        par[pl.ds(8, 8), :] = jnp.broadcast_to(dd_s[...].astype(f32).reshape(1, D), (8, D))
        cv = c_s[...].astype(f32)
        sc = jnp.broadcast_to(cv * jax.nn.sigmoid(cv), (8, D))
        scp = pltpu.bitcast(pltpu.pack_elementwise([sc, sc], packed_dtype=bf16), f32)
        for j in range(NT):
            kb0[KOFF + 48 + j] = scp[:, 128 * j:128 * (j + 1)]
            kb1[KOFF + 48 + j] = scp[:, 128 * j:128 * (j + 1)]

    def mkb(i, unr, off, cache):
        def b(stride, extra=0, z=None):
            if isinstance(i, int):
                return (i * unr + off) * stride + extra
            key = (unr * stride, z)
            if key not in cache or NOCACHE:
                base = pl.multiple_of(i * (unr * stride), unr * stride)
                cache[key] = base if z is None else base + (i >> z)
            return cache[key] + (off * stride + extra)
        return b

    def dot_h(j, b, lhs):
        gb = gbs[j % 2]
        hc = hbuf[j, :, pl.ds(_mult(b(512), 512), 512)]
        rhs_t = jnp.concatenate([hc[:, C * cc:C * (cc + 1)] for cc in range(4)], axis=0)
        g = lax.dot_general(lhs, pltpu.bitcast(rhs_t, bf16), NTDIMS, preferred_element_type=f32)
        for rg in range(2 * NG):
            for cc in range(4):
                gb[b(4, cc + rg * NC)] = g[8 * rg:8 * rg + 8, 128 * cc:128 * cc + 128]

    def dot_u(j, b, lhs):
        ub = ubs[j % 2]
        taps = [par[pl.ds(t, 1), pl.ds(j * 128, 128)] for t in range(4)]
        unp = lambda w_, e: pltpu.unpack_elementwise(w_, index=e, packed_dtype=bf16, unpacked_dtype=f32)
        cols = []
        for cc in range(4):
            words = []
            for blk in range(8 // W):
                w0 = 64 * cc + 8 * W * blk
                kw = {m: kbuf[j, pl.ds(b(256, 8 + w0 + m), 8, stride=W), :] for m in range(-2, W)}
                kk = {2 * m + e: unp(kw[m], e) for m in range(-2, W) for e in range(2) if 2 * m + e >= -3}
                for m in range(W):
                    vw = vbuf[j, pl.ds(b(256, w0 + m), 8, stride=W), :]
                    pair = []
                    for e in range(2):
                        n = 2 * m + e
                        ks = kk[n] * taps[0] + kk[n - 1] * taps[1] + kk[n - 2] * taps[2] + kk[n - 3] * taps[3]
                        pair.append(ks * unp(vw, e))
                    words.append(pltpu.pack_elementwise(pair, packed_dtype=bf16))
            cols.append(jnp.concatenate(words, axis=0))
        rhs = pltpu.bitcast(jnp.concatenate(cols, axis=1), bf16)
        u = jnp.dot(lhs, rhs, preferred_element_type=f32)
        for rg in range(2 * NG):
            for cc in range(4):
                ub[b(4, cc + rg * NC)] = u[8 * rg:8 * rg + 8, 128 * cc:128 * cc + 128]

    def dot_i(j, b, half, lhs):
        kb = kbs[j % 2]
        cols = [[], []]
        for gi in range(NG):
            prev = None
            for cc in range(-1, 2):
                k0, k1, k2 = [kb[b(4 * NG * 3, ((2 * half + cc + 1) * NG + gi) * 3 + t)] for t in range(3)]
                re, im = k0 - k2, k0 + k1
                if prev is not None:
                    cols[cc].append(pltpu.pack_elementwise([re - prev[1], im + prev[0]], packed_dtype=bf16))
                prev = (re, im)
        rhs = jnp.concatenate([jnp.concatenate(c_, axis=0) for c_ in cols], axis=1)
        y = jnp.dot(lhs, pltpu.bitcast(rhs, bf16), preferred_element_type=f32)
        for cc in range(2):
            yb[j, pl.ds(b(512, (2 * half + cc) * C), C), :] = y[:, 128 * cc:128 * cc + 128]

    def gen_m(j, kb, b, ng):
        ub, gb = ubs[j % 2], gbs[j % 2]
        for s in range(ng):
            for t in range(3):
                z = 8 + t
                re = lambda ref, c: ref[b(2 * NC, 2 * s * NC + c, z)]
                im = lambda ref, c: ref[b(2 * NC, (2 * s + 1) * NC + c, z)]
                gre = [re(gb, c) for c in range(NC)]
                if t == 0:
                    us = [re(ub, c) + im(ub, c) for c in range(NC)]
                    gs = gre
                elif t == 1:
                    us = [re(ub, c) for c in range(NC)]
                    gs = [im(gb, c) - gre[c] for c in range(NC)]
                else:
                    us = [im(ub, c) for c in range(NC)]
                    gs = [im(gb, c) + gre[c] for c in range(NC)]

                def st(a, val):
                    kb[b(3, ((a + 1) * NG + s) * 3 + t)] = val
                if not KARA:
                    for a in range(NC):
                        st(a, _conv(us, gs, a))
                        yield 2 * a + 2
                    continue
                ue, uo, ge, go = us[0::2], us[1::2], gs[0::2], gs[1::2]
                if KORD == 1:
                    usum = [x + y for x, y in zip(ue, uo)]
                    gsum = [x + y for x, y in zip(ge, go)]
                    poo = _conv(uo, go, NC // 2 - 1)
                    for a in reversed(range(NC // 2)):
                        pee = _conv(ue, ge, a)
                        pss = _conv(usum, gsum, a)
                        st(2 * a + 1, pss - pee - poo)
                        poo = _conv(uo, go, a - 1) if a else None
                        st(2 * a, pee + poo if a else pee)
                        yield 3 * (2 * a + 1) + (37 if a == NC // 2 - 1 else 3)
                    continue
                usum = [x + y for x, y in zip(ue, uo)]
                gsum = [x + y for x, y in zip(ge, go)]
                poo_prev = None
                for a in range(NC // 2):
                    pee = _conv(ue, ge, a)
                    poo = _conv(uo, go, a)
                    pss = _conv(usum, gsum, a)
                    st(2 * a, pee if poo_prev is None else pee + poo_prev)
                    st(2 * a + 1, pss - pee - poo)
                    poo_prev = poo
                    yield 3 * (2 * a + 1) + 7

    def add_d(j):
        gb = gbs[j % 2]
        dvec = par[pl.ds(8, 8), pl.ds(j * 128, 128)]
        for gi in range(NG):
            gb[2 * gi * NC] = gb[2 * gi * NC] + dvec

    def sc_lhs():
        return pltpu.bitcast(jnp.concatenate([kb0[KOFF + 48 + j] for j in range(NT)], axis=1), bf16)

    def dot_m(i, t0, nt, rows):
        m = None
        for kt in range(NT):
            p = jnp.dot(pltpu.bitcast(rows[kt], bf16), _wt(wm, i, pl.ds(64 * kt, 64), pl.ds(128 * t0, 128 * nt)),
                        preferred_element_type=f32)
            m = p if m is None else m + p
        for t in range(nt):
            modb[i * (WMA // 128) + (t0 + t)] = m[0:8, 128 * t:128 * (t + 1)]

    def inv_lhs(tbl, n):
        return jnp.concatenate([tbl[KOFF + 16 + 2 * n], tbl[KOFF + 17 + 2 * n]], axis=1)

    def dot_k(kb, kt, bt, lhs):
        cols = [[] for _ in range(4)]
        for gi in range(8 * kt, 8 * kt + 8):
            prev = None
            for cc in range(-1, 4):
                k0, k1, k2 = [kb[((4 * bt + cc + 1) * NG + gi) * 3 + t] for t in range(3)]
                re, im = k0 - k2, k0 + k1
                if prev is not None:
                    cols[cc].append(pltpu.pack_elementwise([re - prev[1], im + prev[0]], packed_dtype=bf16))
                prev = (re, im)
        rhs = jnp.concatenate([jnp.concatenate(c_, axis=0) for c_ in cols], axis=1)
        y = jnp.dot(lhs, pltpu.bitcast(rhs, bf16), preferred_element_type=f32)
        for cc in range(4):
            rows = pl.ds((4 * bt + cc) * C, C)
            yc = y[:, 128 * cc:128 * cc + 128]
            yb[NT - 1, rows, :] = yc if kt == 0 else yb[NT - 1, rows, :] + yc

    PRE = dict(H=0, U=672 + 96 // W, a=192, b=192, m=0, k=176)
    POST = dict(H=0, U=0, a=4, b=4, m=2, k=0)
    NST = dict(H=16, U=16, a=8, b=8, m=5, k=8)
    GCOST = 3 * (248 if KARA else 272)

    def a_block(dots, mg=None, ng=0, tbl=kb0):
        native, dur = [], []
        for idx, (k_, _) in enumerate(dots):
            nxt = PRE[dots[idx + 1][0]] if idx + 1 < len(dots) else 0
            d_ = 2.0 if k_ == 'm' else 1.0
            native += [nxt / NST[k_] + POST[k_] * d_] * NST[k_]
            dur += [d_] * NST[k_]
        if mg is not None and dots:
            head = max(HEAD - PRE[dots[0][0]], 0)
            mtot = GCOST * ng - TAIL - head
            lvl = (mtot + sum(native)) / sum(dur)
            want = [max(lvl * d_ - x, 0.0) for x, d_ in zip(native, dur)]
            scale = mtot / sum(want)
            cum, tgt = [head], head
            for w_ in want:
                tgt += w_ * scale
                cum.append(tgt)
        done = 0.0
        step = 0
        for (k_, fn) in dots:
            rows = []
            for n in range(NST[k_]):
                if mg is not None and (n % FSTEP == 0 or k_ == 'm'):
                    while done < cum[min(step + FOFF, len(cum) - 1)]:
                        done += next(mg)
                step += 1
                if k_ in 'HU':
                    rows.append(tbl[KOFF + n + (32 if k_ == 'U' else 0)])
                elif k_ in 'ab':
                    rows.append(inv_lhs(tbl, n))
                elif k_ == 'k':
                    rows.append(tbl[KOFF + 16 + 2 * n])
                else:
                    rows.append(tbl[KOFF + 48 + n])
            fn(rows if k_ == 'm' else pltpu.bitcast(jnp.concatenate(rows, axis=0), bf16))
        if mg is not None:
            for _ in mg:
                pass

    def fdot(k_, j, b):
        if k_ == 'H':
            return (k_, lambda lhs: dot_h(j, b, lhs))
        if k_ == 'U':
            return (k_, lambda lhs: dot_u(j, b, lhs))
        return (k_, lambda lhs: dot_i(j, b, 0 if k_ == 'a' else 1, lhs))

    def wait_all(cps):
        for c_ in cps:
            c_.wait()

    def a_loop(jf, jm, ji, g0, ng):
        kinds = [k_ for k_ in DORDER if k_ in 'HU' or ji is not None]

        def body(i, carry):
            cache = {}
            zs[i] = 0
            dots = [fdot(k_, jf if k_ in 'HU' else ji, mkb(i, 2, s_, cache)) for s_ in range(2) for k_ in kinds]
            a_block(dots, gen_m(jm, kbs[jm % 2], mkb(i, ng, g0, cache), ng), ng, kbs[jm % 2])

            @pl.when(i == 0)
            def _():
                wait_all(cp_tile(jf, 1))
            return carry
        wait_all(cp_tile(jf, 0))
        lax.fori_loop(0, 2, body, 0)
        add_d(jf)

    sb_ = lambda bt: mkb(0, 1, bt, None)
    if SKIPA:
        a_block = lambda *a, **k: None
    with jax.named_scope("A_seg0"):
        wait_all(cp_t0[0])
        a_block([fdot('H', 0, sb_(bt)) for bt in range(4)])
        add_d(0)
        wait_all(cp_t0[1])
        a_block([fdot('U', 0, sb_(bt)) for bt in range(2)])
        for bt in (2, 3):
            wait_all(cp_t0[bt])
            a_block([fdot('U', 0, sb_(bt))])
    with jax.named_scope("A_m0"):
        def body_m0(i, carry):
            a_block([], gen_m(0, kb0, mkb(i, G0 // 2, 0, {}), G0 // 2))
            return carry
        if G0:
            lax.fori_loop(0, 2, body_m0, 0)
    for seg in range(1, NT):
        with jax.named_scope(f"A_seg{seg}"):
            if seg == 1:
                a_loop(1, 0, None, G0, (NG - G0) // 2)
            else:
                a_loop(seg, seg - 1, seg - 2, 0, 8)

    def mods(i):
        return [('m', lambda rows, t0=t0, nt=nt: dot_m(i, t0, nt, rows)) for (t0, nt) in ((0, 4), (4, 4), (8, 2))]

    with jax.named_scope("A_seg5a"):
        cp_wm(0).wait()
        zz = zs[1]

        @pl.when(zz == 0)
        def _():
            dots = [fdot(k_, NT - 2, sb_(bt)) for bt in range(4) for k_ in 'ab']
            mm = mods(0)
            dots = [mm[0]] + dots[0:2] + [mm[1]] + dots[2:4] + [mm[2]] + dots[4:]
            a_block(dots, gen_m(NT - 1, kb0, mkb(zz, 8, 0, {}), 8), 8, kb0)
    with jax.named_scope("A_seg5b"):
        cp_wm(1).wait()

        @pl.when(zz == 0)
        def _():
            dots = [('k', lambda lhs, bt=bt: dot_k(kb0, 0, bt, lhs)) for bt in range(4)]
            mm = mods(1)
            dots = [mm[0], dots[0], mm[1], dots[1], mm[2]] + dots[2:]
            a_block(dots, gen_m(NT - 1, kb1, mkb(zz, 8, 8, {}), 8), 8, kb1)

    def inv_last(bt):
        lhs = pltpu.bitcast(jnp.concatenate([kb0[KOFF + 17 + 2 * n] for n in range(8)], axis=0), bf16)
        dot_k(kb1, 1, bt, lhs)

    def modrow(k_):
        return jnp.concatenate([modb[NT * k_ + j] for j in range(NT)], axis=1)

    R = R1
    GP = R // 8

    def ln_chain(p):
        r = p * R
        pa, pb, pc, ps = [par[pl.ds(16 + 8 * t, 8), :][None] for t in range(4)]
        g3 = lambda x: x.reshape(GP, 8, D)
        q = g3(qbuf[pl.ds(r, R), :].astype(f32))
        d1, r1 = _center(q)
        y = g3(jnp.concatenate([yb[j, pl.ds(r, R), :] for j in range(NT)], axis=1))
        x = q + ((d1 * r1) * pa + pb) * y
        xn[pl.ds(r, R), :] = x.reshape(R, D)
        d2, r2 = _center(x)
        h = (d2 * r2) * pc + ps
        hh[pl.ds(r, R), :] = h.reshape(R, D)
        d3, r3 = _center(h, ALPHA)
        return (d3 * r3).reshape(R, D)

    def tie(w_, vs):
        t_ = pltpu.bitcast(vs[0], u32)
        for v_ in vs[1:]:
            t_ = t_ | pltpu.bitcast(v_, u32)
        return w_ | (t_ & kbuf[0, pl.ds(0, 8), :])

    def tied(wref, ties):
        if not ties:
            return _wt(wref)
        rbs = sorted({8 * (t % 5) + rb for (t, rb) in ties})
        rows, pos = [], 0
        for rb in rbs:
            if rb > pos:
                rows.append(wref[pl.ds(8 * pos, 8 * (rb - pos)), :])
            blk = []
            for n in range(NT):
                w_ = wref[pl.ds(8 * rb, 8), pl.ds(128 * n, 128)]
                vs = ties.get((5 * n + rb // 8, rb % 8))
                blk.append(tie(w_, vs) if vs else w_)
            rows.append(jnp.concatenate(blk, axis=1))
            pos = rb + 1
        if pos < 40:
            rows.append(wref[pl.ds(8 * pos, 8 * (40 - pos)), :])
        return pltpu.bitcast(jnp.concatenate(rows, axis=0), bf16)

    def w1_dot(p, l3, ties, fresh):
        if fresh and STAG:
            grp = lambda g: l3[8 * g:8 * g + 8, 0:128]
            lt = {}
            for pr, spec in enumerate(STAG.split(',')):
                vs = [grp(2 * pr), grp(2 * pr + 1)]
                if spec[0] == 'w':
                    ties.setdefault((int(spec[1]), int(spec[2])), []).extend(vs)
                elif spec[0] == 'l':
                    lt.setdefault(int(spec[1]), []).extend(vs)
            for pr, vs in lt.items():
                x = pltpu.bitcast(tie(pltpu.bitcast(l3[16 * pr:16 * pr + 8, 128:256], u32), vs), f32)
                mid = jnp.concatenate([l3[16 * pr:16 * pr + 8, 0:128], x, l3[16 * pr:16 * pr + 8, 256:]], axis=1)
                l3 = jnp.concatenate(([l3[:16 * pr]] if pr else []) + [mid, l3[16 * pr + 8:]], axis=0)
        z = jnp.dot(l3.astype(bf16), tied(w1, ties), preferred_element_type=f32)
        g = _gelu2a(z)
        if SHST:
            lane = lax.broadcasted_iota(jnp.int32, (R, 128), 1)
            for j, (o1, cut, o2) in enumerate(((1, 128, 0), (1, 32, -1), (-1, 64, 2), (2, 96, -2), (-2, 128, 0))):
                gj = g[:, j * 128:(j + 1) * 128]
                if cut == 128:
                    h1[j, pl.ds(p * R + 8 + o1, R), :] = gj
                else:
                    pltpu.store(h1.at[j, pl.ds(p * R + 8 + o1, R), :], gj, mask=lane < cut)
                    pltpu.store(h1.at[j, pl.ds(p * R + 8 + o2, R), :], gj, mask=lane >= cut)
            return z
        for j in range(NT):
            h1[j, pl.ds(p * R + 8, R), :] = g[:, j * 128:(j + 1) * 128]
        return z

    def w2_dot(p, ties):
        r = p * R
        lane = lax.broadcasted_iota(jnp.int32, (R, 128), 1)

        def ld(j, off):
            return h1[j, pl.ds(r + 8 + off, R), :]
        tiles = [
            ld(0, -1),
            jnp.where(lane < 32, ld(1, -1), ld(1, 1)),
            jnp.where(lane < 64, ld(2, 1), ld(2, -2)),
            jnp.where(lane < 96, ld(3, -2), ld(3, 2)),
            ld(4, 2),
        ]
        if SHST:
            tiles = [ld(j, 0) for j in range(NT)]
        hs = jnp.concatenate(tiles, axis=1).astype(bf16)
        x1 = hh[pl.ds(r, R), :] + jnp.dot(hs, tied(w2, ties), preferred_element_type=f32) * BETA
        hh[pl.ds(r, R), :] = x1
        return x1

    unp = lambda w_, e: pltpu.unpack_elementwise(w_, index=e, packed_dtype=bf16, unpacked_dtype=f32)
    pk = lambda xs: pltpu.pack_elementwise(xs, packed_dtype=bf16)
    PURE = {7 * p_ + q_: 2 * i_ + j_ for i_, p_ in enumerate((2, 4)) for j_, q_ in enumerate((2, 4))}

    zoff = [pl.multiple_of((zz >> p_) * 32, 32) for p_ in range(7)]

    def prep2(src, dst, tr, t, p_, anchor):
        zero = None if anchor is None else pltpu.bitcast(anchor, u32) & kbuf[0, pl.ds(0, 8), :]
        gate = 0 if _SBU[p_][0] else 3
        l1 = [[], []]
        for k2 in range(2):
            for n2 in range(2):
                bl = []
                for b_ in range(4):
                    kq, nq = 2 * (b_ // 2) + k2, 2 * (b_ % 2) + n2
                    x = None
                    if _SBU[p_][b_]:
                        x = src[pl.ds(zoff[p_] + (8 * t + 192 * (nq if tr else kq)), 8), pl.ds(128 * (kq if tr else nq), 128)]
                        if zero is not None and b_ == gate and k2 == n2:
                            x = x | zero
                    bl.append(x)
                for e in range(2):
                    l1[e].append(_SB[p_](*[None if x is None else unp(x, e) for x in bl]))
        for q_ in range(7):
            if 7 * p_ + q_ not in PURE:
                dst[7 * p_ + q_, pl.ds(8 * t, 8), :] = pk([_SB[q_](*l1[e]) for e in range(2)])

    def prep1(t, n, anchor):
        bl = [w4[pl.ds(lo + 8 * t, 8), pl.ds(c0 + 128 * n, 128)] for lo in (768, 832) for c0 in (0, 256)]
        if anchor is not None:
            zero = pltpu.bitcast(anchor, u32) & kbuf[0, pl.ds(0, 8), :]
            bl[0], bl[3] = bl[0] | zero, bl[3] | zero
        for p_ in (0, 1, 3, 5, 6):
            w4o[p_, pl.ds(8 * t, 8), pl.ds(128 * n, 128)] = pk([_SB[p_](*[unp(x, e) for x in bl]) for e in range(2)])

    def prep3(t, n, anchor):
        bl = [w3[pl.ds(lo + 8 * t, 8), pl.ds(c0 + 128 * n, 128)] for lo in (768, 816) for c0 in (0, 256)]
        if anchor is not None:
            zero = pltpu.bitcast(anchor, u32) & kbuf[0, pl.ds(0, 8), :]
            bl[0], bl[3] = bl[0] | zero, bl[3] | zero
        for p_ in (0, 2, 4, 5, 6):
            w3o[p_, pl.ds(8 * t, 8), pl.ds(128 * n, 128)] = pk([_SA[p_](*[unp(x, e) for x in bl]) for e in range(2)])

    units = []
    l3s = {}

    def ln4(r, n):
        d4, r4 = _center(hh[pl.ds(r, n), :], ALPHA)
        return d4 * r4

    def run_block(dots, extra=None, pre4=False):
        for d_, (k_, p) in enumerate(dots):
            ties = {}
            e = d_ - (len(dots) - NP4)
            RP = TS // NP4
            if pre4 and e >= 0:
                nx = ln4(e * RP, RP)
                l4p[pl.ds(e * RP, RP), :] = nx
                ties[(TIE4, 7)] = [nx[8 * g:8 * g + 8, 0:128] for g in range(RP // 8)]
            if extra is not None and d_ == len(dots) - 1:
                nx = ln_chain(extra)
                for pr in range(4):
                    ties[(24, XRB[pr])] = [nx[16 * pr:16 * pr + 8, 0:128], nx[16 * pr + 8:16 * pr + 16, 0:128]]
                l3s[extra] = nx.astype(bf16)
            if k_ == 1:
                fresh = p not in l3s
                res = w1_dot(p, ln_chain(p) if fresh else l3s.pop(p), ties, fresh)
            elif k_ == 2:
                res = w2_dot(p, ties)
            else:
                par[pl.ds(48, 8), :] = jnp.dot(sc_lhs(), _wt(wmc), preferred_element_type=f32)[0:8]
            for u_ in ANCH:
                if u_ // 40 + 1 == k_ and units and d_ < len(dots) - (NP4 + 1 if pre4 else 0):
                    n, g = (u_ % 40) // 8, u_ % 8
                    units.pop(0)(res[8 * g:8 * g + 8, 128 * n:128 * (n + 1)])

    with jax.named_scope("P1"):
        cp_wmp.wait()
        cp_q[0].wait()
        mp = jnp.dot(sc_lhs(), _wt(wmp), preferred_element_type=f32)
        for t in range(WMP // 128):
            modb[2 * WMA // 128 + t] = mp[0:8, 128 * t:128 * (t + 1)]
        sa, ca, ga, sb, cb = [modrow(k_) for k_ in range(5)]
        par[pl.ds(16, 8), :] = ga * (1.0 + ca)
        par[pl.ds(24, 8), :] = ga * sa
        par[pl.ds(32, 8), :] = 1.0 + cb
        par[pl.ds(40, 8), :] = sb
        for bt in range(4):
            inv_last(bt)
        for p in range(PRELN):
            l3s[p] = ln_chain(p)
    with jax.named_scope("w1wait"):
        cp_w[0].wait()
    p1, p2 = N2, 0
    with jax.named_scope("P2"):
        run_block([(1, p) for p in range(N2)])
    with jax.named_scope("w2wait"):
        wait_all([cp_w[1], cp_q[1]])

    def plan(lim1):
        nonlocal p1, p2
        last = lim1 == S // R
        dots = []
        while p1 < (lim1 if last else lim1 - 1) or p1 - p2 >= LEAD or (last and p2 < lim1):
            if p1 - p2 < LEAD and p1 < lim1:
                dots.append((1, p1))
                p1 += 1
            else:
                dots.append((2, p2))
                p2 += 1
        return dots, (None if last else p1)

    with jax.named_scope("P4"):
        run_block(*plan(Q1 // R))
    with jax.named_scope("q2wait"):
        wait_all([cp_q[2], cp_w[3]])
    units += [functools.partial(prep2, w4, w4s, False, t, p_) for t in range(24) for p_ in range(7)]
    units += [functools.partial(prep1, t, n) for t in range(8) for n in range(2)]
    with jax.named_scope("P5"):
        run_block(*plan(Q2 // R))
    with jax.named_scope("q3wait"):
        wait_all([cp_q[3], cp_wmc, cp_w[2]])
    units += [functools.partial(prep2, w3, w3s, True, t, p_) for t in range(24) for p_ in range(7)]
    units += [functools.partial(prep3, t, n) for t in range(6) for n in range(2)]
    with jax.named_scope("P6"):
        dots, _ = plan(S // R)
        run_block(dots[:-NP4] + [(3, 0)] + dots[-NP4:], pre4=True)

    H2 = TS // 2
    OUTS = ((0, H2, 512, 128), (H2, H2, 0, 256), (0, H2, 256, 256), (0, H2, 0, 256), (H2, H2, 256, 256), (H2, H2, 512, 128))

    def out_copy(r, r0, rn, c0, cn):
        rows = pl.ds(_mult(r + r0, H2), rn)
        return cp(obuf.at[rows, pl.ds(c0, cn)], o_hbm.at[0, rows, pl.ds(c0, cn)], osems.at[0])

    def wsum(x, y, sign):
        unp = lambda w_, e: pltpu.unpack_elementwise(w_, index=e, packed_dtype=bf16, unpacked_dtype=f32)
        return pltpu.pack_elementwise([unp(x, e) + unp(y, e) if sign > 0 else unp(x, e) - unp(y, e) for e in range(2)],
                                      packed_dtype=bf16)

    def strassen_lhs(a11, a12, a21, a22):
        c = lambda x: x.astype(bf16)
        return (c(a11 + a22), c(a21 + a22), c(a11), c(a22), c(a11 + a12), c(a21 - a11), c(a12 - a22))

    def strassen(ops, b11, b12, b21, b22, mm, ties=None):
        def tw(k_, w_):
            if not ties or k_ not in ties:
                return w_
            return jnp.concatenate([tie(w_[0:8], ties[k_]), w_[8:]], axis=0)
        m1 = mm(ops[0], tw(0, wsum(b11, b22, 1)))
        m4 = mm(ops[3], tw(1, wsum(b21, b11, -1)))
        m2 = mm(ops[1], tw(2, b11))
        m3 = mm(ops[2], tw(3, wsum(b12, b22, -1)))
        m5 = mm(ops[4], tw(4, b22))
        m7 = mm(ops[6], tw(5, wsum(b21, b22, 1)))
        m6 = mm(ops[5], tw(6, wsum(b11, b12, 1)))
        return (m1 + m4) + (m7 - m5), m3 + m5, m4 + m2, (m1 + (m3 - m2)) + m6

    mm_nt = lambda x, w_: lax.dot_general(x, pltpu.bitcast(w_, bf16), NTDIMS, preferred_element_type=f32)
    mm_nn = lambda x, w_: jnp.dot(x, pltpu.bitcast(w_, bf16), preferred_element_type=f32)

    def b2_step(i):
        gbv = par[pl.ds(48, 8), :]
        nsub = T2 // TS
        for sub in range(nsub):
            r = pl.multiple_of(pl.multiple_of(i * T2, T2) + sub * TS, TS)
            gs = gs_.at[i >> 8]
            l4 = l4p[...] if sub == 0 else ln4(r, TS)
            lt_ = [Lazy([(1, r_, c_)]) for (r_, c_) in ((0, 0), (H2, 0), (0, 256), (H2, 256))]
            nt_ = lambda w_, x: lax.dot_general(pltpu.bitcast(w_, bf16), x, NTDIMS, preferred_element_type=f32)
            w3a = lambda p_: (w3[pl.ds(816, 48), pl.ds(256, 256)] if p_ == 1 else w3[pl.ds(768, 48), pl.ds(0, 256)] if p_ == 3
                              else w3o[p_])
            zr = nt_(w3[pl.ds(768, 96), pl.ds(512, 128)], l4[:, 512:640].astype(bf16))
            c11, c12, c21, c22 = _comb([nt_(w3a(p_), _SB[p_](*lt_).load(l4p_.at[i >> (20 + p_)], H2, 256)) for p_ in range(7)])
            zt = zr + jnp.concatenate([jnp.concatenate([c11, c12], axis=1), jnp.concatenate([c21, c22], axis=1)], axis=0)
            gt = jnp.concatenate([_gelu2a(zt), jnp.zeros((64, TS), f32)], axis=0)
            gs[:, pl.ds(0, 128)] = gt[:128].T
            gs[:, pl.ds(896, 128)] = gt[128:].T
            lrs = [l4[:H2, 512:640].astype(bf16), l4[H2:, 512:640].astype(bf16)]
            Q = H2 // 2
            ab = [Lazy([(1, r_, c_)]) for (r_, c_) in ((0, 0), (0, 256), (H2, 0), (H2, 256))]
            opsA = {}
            rn_ = pl.multiple_of(jnp.minimum(i + 1, S // T2 - 1) * T2, T2)
            RP = TS // len(LNT)
            l4n = l4p
            for t in range(3):
                cq, left = [None] * 4, [5, 3, 3, 5]

                def add(k_, x, sg=1):
                    cq[k_] = x if cq[k_] is None else cq[k_] + x if sg > 0 else cq[k_] - x
                    left[k_] -= 1
                    if left[k_] == 0:
                        gg = _gelu2a(cq[k_])
                        for n2 in range(2):
                            gs[pl.ds(H2 * (k_ // 2), H2), pl.ds(128 + 896 * (k_ % 2) + 128 * (t + 3 * n2), 128)] = gg[:, 128 * n2:128 * (n2 + 1)]

                def rem(k_):
                    wr = jnp.concatenate([w3[pl.ds(64 * (t + 3 * (2 * (k_ % 2) + n2)), 64), pl.ds(512, 128)] for n2 in range(2)], axis=0)
                    add(k_, mm_nt(lrs[k_ // 2], wr))
                for p_ in range(8):
                    for k_ in (2, 1, 0, 3):
                        if int(REMP[4 * t + k_]) == p_:
                            rem(k_)
                    if p_ == 7:
                        break
                    a_ = _SA[p_](*ab)
                    sub_ = (a_, a_.shift(0, 128), a_.shift(Q, 0), a_.shift(Q, 128))
                    pr = []
                    for q_ in range(7):
                        n = 7 * p_ + q_
                        if n not in opsA or RELOAD:
                            opsA[n] = _SA[q_](*sub_).load(l4p_.at[(i + 4 * p_ + 32 * t) >> (9 + q_)] if RELOAD or OPQ3 else l4p, Q, 128)
                        w_ = w3[pl.ds(192 * PURE[n] + 64 * t, 64), pl.ds(128 * PURE[n], 128)] if n in PURE else w3s[n, pl.ds(64 * t, 64), :]
                        pr.append(mm_nt(opsA[n], w_))
                    c11, c12, c21, c22 = _comb(pr)
                    m_ = jnp.concatenate([jnp.concatenate([c11, c12], axis=1), jnp.concatenate([c21, c22], axis=1)], axis=0)
                    for k_, sg in _SC[p_]:
                        add(k_, m_, sg)
            kord = [0, 896] + [o_ for c in (0, 3, 1, 4, 2, 5) for o_ in (128 + 128 * c, 1024 + 128 * c)]
            wrow = lambda o_: 768 if o_ == 0 else 832 if o_ == 896 else (o_ - 128) // 2 if o_ < 896 else 384 + (o_ - 1024) // 2
            wl = jnp.concatenate([w4[pl.ds(wrow(o_), 64), pl.ds(512, 128)] for o_ in kord], axis=0)
            gk = lambda r0: jnp.concatenate([gs[pl.ds(r0, H2), pl.ds(o_, 128)] for o_ in kord], axis=1).astype(bf16)
            acc_t = mm_nn(gk(0), wl)
            ties = {}
            for e, k_ in enumerate(LNT):
                nx = ln4(pl.multiple_of(rn_ + e * RP, RP), RP)
                l4n[pl.ds(e * RP, RP), :] = nx
                ties[k_] = [nx[8 * gi:8 * gi + 8, 0:128] for gi in range(RP // 8)]
            Q = H2 // 2

            blocks = [Lazy([(1, r_, c_)]) for (r_, c_) in ((0, 0), (0, 896), (H2, 0), (H2, 896))]
            ms = []
            for p_ in range(7):
                a_ = _SA[p_](*blocks)
                wo = w4[pl.ds(768, 64), pl.ds(0, 256)] if p_ == 2 else w4[pl.ds(832, 64), pl.ds(256, 256)] if p_ == 4 else w4o[p_]
                w4n = lambda n: w4[pl.ds(192 * PURE[n], 192), pl.ds(128 * PURE[n], 128)] if n in PURE else w4s[n, pl.ds(0, 192), :]
                if p_ in ties:
                    wo = jnp.concatenate([jnp.concatenate([tie(wo[0:8, 0:128], ties[p_]), wo[0:8, 128:]], axis=1), wo[8:]], axis=0)
                m_ = mm_nn(a_.load(gs, H2, 128), wo)
                sub_ = (a_.shift(0, 128), a_.shift(0, 512), a_.shift(Q, 128), a_.shift(Q, 512))
                gref = lambda q_: gs_.at[(i + 4 * p_) >> (9 + q_)] if OPQ else gs
                c11, c12, c21, c22 = _comb([mm_nn(_SA[q_](*sub_).load(gref(q_), Q, 384), w4n(7 * p_ + q_)) for q_ in range(7)])
                ms.append(m_ + jnp.concatenate([jnp.concatenate([c11, c12], axis=1), jnp.concatenate([c21, c22], axis=1)], axis=0))
            c11, c12, c21, c22 = _comb(ms)
            for k_ in ties:
                if k_ >= 10:
                    o_ = 64 * (k_ - 10)
                    wl = jnp.concatenate([wl[:o_], tie(wl[o_:o_ + 8], ties[k_]), wl[o_ + 8:]], axis=0)
            accs = (acc_t, c21, c12, c11, c22, mm_nn(gk(H2), wl))
            for (r0, rn, c0, cn), ac in zip(OUTS, accs):
                rows, cols = pl.ds(_mult(r + r0, H2), rn), pl.ds(c0, cn)
                g3 = lambda x: x.reshape(rn // 8, 8, cn)
                out = g3(xn[rows, cols]) + gbv[None, :, c0:c0 + cn] * g3(hh[rows, cols] + BETA * ac)
                obuf[rows, cols] = out.reshape(rn, cn).astype(bf16)
                out_copy(r, r0, rn, c0, cn).start()

    with jax.named_scope("prep"):
        print("left-over prep units:", len(units))
        for u_ in units:
            u_(None)
    with jax.named_scope("BII"):
        lax.fori_loop(0, S // T2, lambda i, c: (b2_step(i), c)[1], 0)
    with jax.named_scope("out_wait"):
        for i in range(S // TS):
            for o_ in OUTS:
                out_copy(i * TS, *o_).wait()


@jax.jit
def pallas_adaLN_cond__ssm_conv_h3__mixer_s_mlp__prompt_kernel(
    A_q, A_k, A_v, A_shift_k, A_ssm_k, A_ssm_D, B_x, B_w1, B_w2, B_w3, B_w4, c, w_mod,
):
    del B_x
    hbm = pl.BlockSpec(memory_space=pltpu.MemorySpace.HBM)
    return pl.pallas_call(
        _kernel,
        out_shape=jax.ShapeDtypeStruct((1, S, D), bf16),
        in_specs=[hbm] * 12,
        out_specs=hbm,
        scratch_shapes=[
            pltpu.VMEM((27, 8, 128), f32),
            pltpu.VMEM((S + 16 * int(os.environ.get('PADF', '0')), D), bf16),
            pltpu.VMEM((NT, 32 + S // 2, 128), u32),
            pltpu.VMEM((NT, 32 + S // 2, 128), u32),
            pltpu.VMEM((NT, 64, S), u32),
            pltpu.VMEM((D // 2, D), u32),
            pltpu.VMEM((D // 2, D), u32),
            pltpu.VMEM((F // 2, D), u32),
            pltpu.VMEM((896, D), u32),
            pltpu.VMEM((2, D // 2, WMA), u32),
            pltpu.VMEM((D // 2, WMP), u32),
            pltpu.VMEM((D // 2, WMC), u32),
            pltpu.VMEM((S, D), bf16),
            pltpu.VMEM((NG * 2 * NC, 8, 128), f32),
            pltpu.VMEM((NG * 2 * NC, 8, 128), f32),
            pltpu.VMEM((NG * 2 * NC, 8, 128), f32),
            pltpu.VMEM((NG * 2 * NC, 8, 128), f32),
            pltpu.VMEM((KOFF + 56 + PADK, 8, 128), f32),
            pltpu.VMEM((KOFF + 56 + PADK, 8, 128), f32),
            pltpu.VMEM((NT, S, 128), f32),
            pltpu.VMEM((S, D), f32),
            pltpu.VMEM((S, D), f32),
            pltpu.VMEM((NT, S + 32, 128), f32),
            pltpu.VMEM((64, D), f32),
            pltpu.VMEM((1, TS, D), f32),
            pltpu.VMEM((1, TS, 1792), f32),
            pltpu.VMEM((52, 200, 128), u32),
            pltpu.VMEM((52, 200, 128), u32),
            pltpu.VMEM((7, 64, 256), u32),
            pltpu.VMEM((7, 48, 256), u32),
            pltpu.VMEM((4, D), bf16),
            pltpu.VMEM((D,), bf16),
            pltpu.VMEM((1, D), bf16),
            pltpu.SMEM((2,), jnp.int32),
            pltpu.SemaphoreType.DMA((22,)),
            pltpu.SemaphoreType.DMA((1,)),
        ],
        compiler_params=pltpu.CompilerParams(vmem_limit_bytes=100 * 1024 * 1024, disable_semaphore_checks=True,
                                             disable_bounds_checks=bool(int(os.environ.get('NOBC', '0')))),
    )(A_q, A_k, A_v, A_shift_k.T, A_ssm_k, A_ssm_D, B_w1, B_w2, B_w3.T, B_w4, c, w_mod)
```

```python
import functools
import math

import jax
import jax.numpy as jnp
from jax import lax
import jax.experimental.pallas as pl
import jax.experimental.pallas.tpu as pltpu

S, D, F = 2048, 640, 1728
EPS = 1e-5
NT = D // 128
HS = S // 2

C = 128
NC = S // C
NG = 16
KOFF = (NC + 1) * NG * 3
W = 4
G0 = 4
HEAD, TAIL = 250, 450
DORDER = 'aHbU'
WMA, WMP, WMC = 1280, 640, 640
R = 64
Q0, Q1, Q2 = 320, 768, 1408
N2, PRELN, LEAD, NP4, TIE4 = 5, 2, 3, 2, 12
XRB = (7, 4, 2, 0)
ANCH = (20, 58, 18)
TS = 512
H2, Q4 = TS // 2, TS // 4
LNT = (0, 1, 2, 3, 4, 5, 18, 22)
REMP = (6, 5, 3, 7)
ORD4 = (0, 1, 2, 3, 4, 5, 6)
SKIPA = 0

_C0 = math.sqrt(2.0 / math.pi)
ALPHA = (_C0 * 0.044715) ** (1.0 / 3.0)
GC = _C0 / ALPHA
BETA = 0.5 / ALPHA

f32 = jnp.float32
bf16 = jnp.bfloat16
u32 = jnp.uint32
NTDIMS = (((1,), (1,)), ((), ()))

_SA = (lambda a, b, c, d: a + d, lambda a, b, c, d: d, lambda a, b, c, d: c + d, lambda a, b, c, d: a,
       lambda a, b, c, d: a + b, lambda a, b, c, d: b - d, lambda a, b, c, d: c - a)
_SB = (lambda a, b, c, d: a + d, lambda a, b, c, d: c - a, lambda a, b, c, d: a, lambda a, b, c, d: b - d,
       lambda a, b, c, d: d, lambda a, b, c, d: c + d, lambda a, b, c, d: a + b)
_SBU = ((1, 0, 0, 1), (1, 0, 1, 0), (1, 0, 0, 0), (0, 1, 0, 1), (0, 0, 0, 1), (0, 0, 1, 1), (1, 1, 0, 0))
_SC = (((0, 1), (3, 1)), ((0, 1), (2, 1)), ((2, 1), (3, -1)), ((1, 1), (3, 1)), ((0, -1), (1, 1)), ((0, 1),), ((3, 1),))
_PURE = {7 * p + q: 2 * i + j for i, p in enumerate((2, 4)) for j, q in enumerate((2, 4))}


def _comb(m):
    m1, m4, m2, m3, m5, m7, m6 = m
    return (m1 + m4) + (m7 - m5), m3 + m5, m4 + m2, (m1 + (m3 - m2)) + m6


def _quad(c):
    return jnp.concatenate([jnp.concatenate(c[0:2], axis=1), jnp.concatenate(c[2:4], axis=1)], axis=0)


class _Lazy:
    def __init__(self, terms):
        self.terms = terms

    def __add__(self, o):
        return _Lazy(self.terms + o.terms)

    def __sub__(self, o):
        return _Lazy(self.terms + [(-s, r, c) for (s, r, c) in o.terms])

    def shift(self, dr, dc):
        return _Lazy([(s, r + dr, c + dc) for (s, r, c) in self.terms])

    def load(self, ref, rn, cn):
        ts = sorted(self.terms, key=lambda t: -t[0])
        acc = None
        for (s, r, c) in ts:
            x = ref[pl.ds(r, rn), pl.ds(c, cn)]
            acc = x if acc is None else acc + x if s > 0 else acc - x
        return acc.astype(bf16)


def _blocks(*offsets):
    return [_Lazy([(1, r, c)]) for (r, c) in offsets]


def _unp(w, e):
    return pltpu.unpack_elementwise(w, index=e, packed_dtype=bf16, unpacked_dtype=f32)


def _pk(xs):
    return pltpu.pack_elementwise(xs, packed_dtype=bf16)


def _as_bf16(w):
    return pltpu.bitcast(w, bf16)


def _mm(x, w):
    return jnp.dot(x, _as_bf16(w), preferred_element_type=f32)


def _mm_nt(x, w):
    return lax.dot_general(x, w, NTDIMS, preferred_element_type=f32)


def _mult(x, n):
    return x if isinstance(x, int) else pl.multiple_of(x, n)


def _cos_table(m, scale):
    mm = jnp.abs(((m + 256) & 511) - 256)
    x = (128 - mm).astype(f32) * (1.0 / 128.0)
    x2 = x * x
    h = math.pi / 2
    p = -(h ** 7) / 5040 + x2 * ((h ** 9) / 362880 - x2 * (h ** 11) / 39916800)
    p = h + x2 * (-(h ** 3) / 6 + x2 * ((h ** 5) / 120 + x2 * p))
    return (x * scale) * p


def _dft_tables():
    shape = (16, 8, 128)
    n = lax.broadcasted_iota(jnp.int32, shape, 0)
    s = lax.broadcasted_iota(jnp.int32, shape, 1)
    l = lax.broadcasted_iota(jnp.int32, shape, 2)
    fw, fu, iv = [], [], []
    wv = l >> 4
    tu = (16 * W) * (wv // W) + (2 * W) * ((l >> 1) & 7) + 2 * (wv % W) + (l & 1)
    for e in range(2):
        r = 2 * s + e
        j = 8 * n + (r & 7)
        fw.append(_cos_table((4 * j + 1) * l + (r >> 3) * 128, 1.0))
        fu.append(_cos_table((4 * j + 1) * tu + (r >> 3) * 128, 1.0))
        b = 16 * (n >> 1) + r
        col = 128 * (n & 1) + l
        iv.append(_cos_table((4 * (col >> 1) + 1) * b + (col & 1) * 128, 1.0 / 128.0))
    return [pltpu.bitcast(_pk(x), f32) for x in (fw, iv, fu)]


def _gelu2a(z):
    return z * (1.0 + jnp.tanh(z * (z * z + GC)))


def _center(x, scale=1.0):
    s1 = jnp.sum(x, axis=-1, keepdims=True)
    m = s1 * (1.0 / D)
    ssd = jnp.maximum(jnp.sum(x * x, axis=-1, keepdims=True) - s1 * m, 0.0)
    rstd = jnp.exp2(jnp.log(ssd + D * EPS) * (-0.5 / math.log(2.0)) + math.log2(scale * math.sqrt(D)))
    return x - m, rstd


def _conv(us, gs, a):
    acc = None
    for c in range(a + 1):
        p = us[c] * gs[a - c]
        acc = p if acc is None else acc + p
    return acc


def _kernel(q_hbm, k_hbm, v_hbm, sk_hbm, h_hbm, dd_hbm, w1_hbm, w2_hbm, w3_hbm, w4_hbm, c_hbm, wm_hbm, o_hbm,
            modb, qbuf, kbuf, vbuf, hbuf, w1, w2, w3, w4, wm, wmp, wmc, obuf, ub0, ub1, gb0, gb1, kb0, kb1,
            yb, xn, hh, h1, par, l4p_, gs_, w4s, w3s, w4o, w3o, sk_s, dd_s, c_s, zs, sems, osem):
    l4p = l4p_.at[0]
    ubs, gbs, kbs = (ub0, ub1), (gb0, gb1), (kb0, kb1)
    cp = pltpu.make_async_copy

    def cp_h(j, c0, c1, sem):
        cols = pl.ds(c0, c1 - c0)
        return cp(h_hbm.at[pl.ds(j * 128, 128), cols], hbuf.bitcast(bf16).at[j, :, cols], sem)

    def cp_kv(j, r0, r1, sem):
        r0, r1 = (r0 + 16 if r0 else 0), min(r1 + 16, S)
        lanes = pl.ds(j * 128, 128)
        return [cp(k_hbm.at[0, pl.ds(r0, r1 - r0), lanes], kbuf.bitcast(bf16).at[j, pl.ds(r0 + 16, r1 - r0), :], sem),
                cp(v_hbm.at[0, pl.ds(r0, r1 - r0), lanes], vbuf.bitcast(bf16).at[j, pl.ds(r0, r1 - r0), :], sem)]

    def cp_tile(j, i):
        sem = sems.at[2 * j + i]
        return [cp_h(j, i * HS, (i + 1) * HS, sem)] + cp_kv(j, i * HS, (i + 1) * HS, sem)

    def cp_wm(i):
        return cp(wm_hbm.at[:, pl.ds(i * WMA, WMA)], wm.bitcast(bf16).at[i], sems.at[10 + i])

    def wait_all(cps):
        for c_ in cps:
            c_.wait()

    cp_t0 = [[cp_h(0, 0, S, sems.at[0])], cp_kv(0, 0, 1024, sems.at[1]), cp_kv(0, 1024, 1536, sems.at[17]),
             cp_kv(0, 1536, S, sems.at[18])]
    cp_wmp = cp(wm_hbm.at[:, pl.ds(2 * WMA, WMP)], wmp.bitcast(bf16), sems.at[13])
    cp_wmc = cp(wm_hbm.at[:, pl.ds(2 * WMA + WMP, WMC)], wmc.bitcast(bf16), sems.at[12])
    cp_q = [cp(q_hbm.at[0, pl.ds(r0, r1 - r0), :], qbuf.at[pl.ds(r0, r1 - r0), :], sems.at[sm])
            for sm, r0, r1 in ((13, 0, Q0), (16, Q0, Q1), (14, Q1, Q2), (12, Q2, S))]
    cp_w = [cp(s_, d_.bitcast(bf16).at[pl.ds(0, s_.shape[0]), :], sems.at[sm])
            for sm, s_, d_ in ((15, w1_hbm, w1), (16, w2_hbm, w2), (12, w3_hbm, w3), (14, w4_hbm, w4))]
    cp_s = [cp(sk_hbm, sk_s, sems.at[19]), cp(dd_hbm, dd_s, sems.at[19]), cp(c_hbm, c_s, sems.at[19])]
    order = list(cp_s)
    for grp in cp_t0:
        order += grp
    for j in range(1, NT):
        order += cp_tile(j, 0) + cp_tile(j, 1)
    order += [cp_wm(0), cp_wm(1), cp_wmp, cp_q[0], cp_w[0], cp_w[1], cp_q[1], cp_q[2], cp_w[3], cp_q[3], cp_wmc, cp_w[2]]
    for c_ in order:
        c_.start()

    with jax.named_scope("init"):
        tables = _dft_tables()
        for kb in kbs:
            for i, tb in enumerate(tables):
                kb[pl.ds(KOFF + 16 * i, 16)] = tb
            kb[pl.ds(0, NG * 3)] = jnp.zeros((NG * 3, 8, 128), f32)
        w4[pl.ds(F // 2, 32), :] = jnp.zeros((32, D), u32)
        for j in range(NT):
            kbuf[j, pl.ds(0, 8), :] = jnp.zeros((8, 128), u32)
            kbuf[j, pl.ds(8 + HS, 8), :] = jnp.zeros((8, 128), u32)
            vbuf[j, pl.ds(HS, 8), :] = jnp.zeros((8, 128), u32)
            h1[j, pl.ds(8, 8), :] = jnp.zeros((8, 128), f32)
            h1[j, pl.ds(S, 8), :] = jnp.zeros((8, 128), f32)
        wait_all(cp_s)
        par[pl.ds(0, 4), :] = sk_s[...].astype(f32)
        par[pl.ds(8, 8), :] = jnp.broadcast_to(dd_s[...].astype(f32).reshape(1, D), (8, D))
        cv = c_s[...].astype(f32)
        sc = jnp.broadcast_to(cv * jax.nn.sigmoid(cv), (8, D))
        scp = pltpu.bitcast(_pk([sc, sc]), f32)
        for kb in kbs:
            for j in range(NT):
                kb[KOFF + 48 + j] = scp[:, 128 * j:128 * (j + 1)]

    def mkb(i, unr, off, cache):
        def b(stride, extra=0, z=None):
            if isinstance(i, int):
                return (i * unr + off) * stride + extra
            key = (unr * stride, z)
            if key not in cache:
                base = pl.multiple_of(i * (unr * stride), unr * stride)
                cache[key] = base if z is None else base + (i >> z)
            return cache[key] + (off * stride + extra)
        return b

    def store_spec(ref, b, x):
        for rg in range(2 * NG):
            for cc in range(4):
                ref[b(4, cc + rg * NC)] = x[8 * rg:8 * rg + 8, 128 * cc:128 * cc + 128]

    def dot_h(j, b, lhs):
        hc = hbuf[j, :, pl.ds(_mult(b(512), 512), 512)]
        rhs_t = jnp.concatenate([hc[:, C * cc:C * (cc + 1)] for cc in range(4)], axis=0)
        store_spec(gbs[j % 2], b, _mm_nt(lhs, _as_bf16(rhs_t)))

    def dot_u(j, b, lhs):
        taps = [par[pl.ds(t, 1), pl.ds(j * 128, 128)] for t in range(4)]
        cols = []
        for cc in range(4):
            words = []
            for blk in range(8 // W):
                w0 = 64 * cc + 8 * W * blk
                kw = {m: kbuf[j, pl.ds(b(256, 8 + w0 + m), 8, stride=W), :] for m in range(-2, W)}
                kk = {2 * m + e: _unp(kw[m], e) for m in range(-2, W) for e in range(2) if 2 * m + e >= -3}
                for m in range(W):
                    vw = vbuf[j, pl.ds(b(256, w0 + m), 8, stride=W), :]
                    pair = []
                    for e in range(2):
                        n = 2 * m + e
                        ks = kk[n] * taps[0] + kk[n - 1] * taps[1] + kk[n - 2] * taps[2] + kk[n - 3] * taps[3]
                        pair.append(ks * _unp(vw, e))
                    words.append(_pk(pair))
            cols.append(jnp.concatenate(words, axis=0))
        store_spec(ubs[j % 2], b, _mm(lhs, jnp.concatenate(cols, axis=1)))

    def out_spec(kidx, groups, nc):
        cols = [[] for _ in range(nc)]
        for gi in groups:
            prev = None
            for cc in range(-1, nc):
                k0, k1, k2 = [kidx(((cc + 1) * NG + gi) * 3 + t) for t in range(3)]
                re, im = k0 - k2, k0 + k1
                if prev is not None:
                    cols[cc].append(_pk([re - prev[1], im + prev[0]]))
                prev = (re, im)
        return jnp.concatenate([jnp.concatenate(c_, axis=0) for c_ in cols], axis=1)

    def dot_i(j, b, half, lhs):
        y = _mm(lhs, out_spec(lambda o: kbs[j % 2][b(4 * NG * 3, 2 * half * NG * 3 + o)], range(NG), 2))
        for cc in range(2):
            yb[j, pl.ds(b(512, (2 * half + cc) * C), C), :] = y[:, 128 * cc:128 * cc + 128]

    def dot_k(kb, kt, bt, lhs):
        y = _mm(lhs, out_spec(lambda o: kb[4 * bt * NG * 3 + o], range(8 * kt, 8 * kt + 8), 4))
        for cc in range(4):
            rows = pl.ds((4 * bt + cc) * C, C)
            yc = y[:, 128 * cc:128 * cc + 128]
            yb[NT - 1, rows, :] = yc if kt == 0 else yb[NT - 1, rows, :] + yc

    def gen_m(j, kb, b, ng):
        ub, gb = ubs[j % 2], gbs[j % 2]
        for s in range(ng):
            for t in range(3):
                re = lambda ref, c: ref[b(2 * NC, 2 * s * NC + c, 8 + t)]
                im = lambda ref, c: ref[b(2 * NC, (2 * s + 1) * NC + c, 8 + t)]
                gre = [re(gb, c) for c in range(NC)]
                if t == 0:
                    us, gs = [re(ub, c) + im(ub, c) for c in range(NC)], gre
                elif t == 1:
                    us, gs = [re(ub, c) for c in range(NC)], [im(gb, c) - gre[c] for c in range(NC)]
                else:
                    us, gs = [im(ub, c) for c in range(NC)], [im(gb, c) + gre[c] for c in range(NC)]
                ue, uo, ge, go = us[0::2], us[1::2], gs[0::2], gs[1::2]
                usum = [x + y for x, y in zip(ue, uo)]
                gsum = [x + y for x, y in zip(ge, go)]
                poo_prev = None
                for a in range(NC // 2):
                    pee, poo, pss = _conv(ue, ge, a), _conv(uo, go, a), _conv(usum, gsum, a)
                    kb[b(3, ((2 * a + 1) * NG + s) * 3 + t)] = pee if poo_prev is None else pee + poo_prev
                    kb[b(3, ((2 * a + 2) * NG + s) * 3 + t)] = pss - pee - poo
                    poo_prev = poo
                    yield 3 * (2 * a + 1) + 7

    def add_d(j):
        gb = gbs[j % 2]
        dvec = par[pl.ds(8, 8), pl.ds(j * 128, 128)]
        for gi in range(NG):
            gb[2 * gi * NC] = gb[2 * gi * NC] + dvec

    def dot_m(i, t0, nt, rows):
        m = None
        for kt in range(NT):
            p = _mm(_as_bf16(rows[kt]), wm[i, pl.ds(64 * kt, 64), pl.ds(128 * t0, 128 * nt)])
            m = p if m is None else m + p
        for t in range(nt):
            modb[i * (WMA // 128) + (t0 + t)] = m[0:8, 128 * t:128 * (t + 1)]

    pre = dict(H=0, U=672 + 96 // W, a=192, b=192, m=0, k=176)
    post = dict(H=0, U=0, a=4, b=4, m=2, k=0)
    nst = dict(H=16, U=16, a=8, b=8, m=5, k=8)

    def a_block(dots, mg=None, ng=0, tbl=kb0):
        if SKIPA:
            return
        native, dur = [], []
        for idx, (k_, _) in enumerate(dots):
            nxt = pre[dots[idx + 1][0]] if idx + 1 < len(dots) else 0
            d_ = 2.0 if k_ == 'm' else 1.0
            native += [nxt / nst[k_] + post[k_] * d_] * nst[k_]
            dur += [d_] * nst[k_]
        if mg is not None and dots:
            head = max(HEAD - pre[dots[0][0]], 0)
            mtot = 744 * ng - TAIL - head
            lvl = (mtot + sum(native)) / sum(dur)
            want = [max(lvl * d_ - x, 0.0) for x, d_ in zip(native, dur)]
            cum = [head]
            for w_ in want:
                cum.append(cum[-1] + w_ * mtot / sum(want))
        done, step = 0.0, 0
        for (k_, fn) in dots:
            rows = []
            for n in range(nst[k_]):
                while mg is not None and done < cum[step]:
                    done += next(mg)
                step += 1
                if k_ in 'ab':
                    rows.append(jnp.concatenate([tbl[KOFF + 16 + 2 * n], tbl[KOFF + 17 + 2 * n]], axis=1))
                else:
                    rows.append(tbl[KOFF + dict(H=n, U=32 + n, k=16 + 2 * n, m=48 + n)[k_]])
            fn(rows if k_ == 'm' else _as_bf16(jnp.concatenate(rows, axis=0)))
        for _ in (mg or ()):
            pass

    def fdot(k_, j, b):
        if k_ in 'HU':
            return (k_, functools.partial(dot_h if k_ == 'H' else dot_u, j, b))
        return (k_, functools.partial(dot_i, j, b, 0 if k_ == 'a' else 1))

    def a_loop(jf, jm, ji, g0, ng):
        kinds = [k_ for k_ in DORDER if k_ in 'HU' or ji is not None]

        def body(i, carry):
            cache = {}
            zs[i] = 0
            dots = [fdot(k_, jf if k_ in 'HU' else ji, mkb(i, 2, s_, cache)) for s_ in range(2) for k_ in kinds]
            a_block(dots, gen_m(jm, kbs[jm % 2], mkb(i, ng, g0, cache), ng), ng, kbs[jm % 2])

            @pl.when(i == 0)
            def _():
                wait_all(cp_tile(jf, 1))
            return carry
        wait_all(cp_tile(jf, 0))
        lax.fori_loop(0, 2, body, 0)
        add_d(jf)

    sb_ = lambda bt: mkb(0, 1, bt, None)
    with jax.named_scope("A_seg0"):
        wait_all(cp_t0[0])
        a_block([fdot('H', 0, sb_(bt)) for bt in range(4)])
        add_d(0)
        wait_all(cp_t0[1])
        a_block([fdot('U', 0, sb_(bt)) for bt in range(2)])
        for bt in (2, 3):
            wait_all(cp_t0[bt])
            a_block([fdot('U', 0, sb_(bt))])
    with jax.named_scope("A_m0"):
        def body_m0(i, carry):
            a_block([], gen_m(0, kb0, mkb(i, G0 // 2, 0, {}), G0 // 2))
            return carry
        lax.fori_loop(0, 2, body_m0, 0)
    for seg in range(1, NT):
        with jax.named_scope(f"A_seg{seg}"):
            if seg == 1:
                a_loop(1, 0, None, G0, (NG - G0) // 2)
            else:
                a_loop(seg, seg - 1, seg - 2, 0, 8)

    def with_mod(i, dots, step):
        mm = [('m', functools.partial(dot_m, i, t0, nt)) for (t0, nt) in ((0, 4), (4, 4), (8, 2))]
        return [mm[0]] + dots[:step] + [mm[1]] + dots[step:2 * step] + [mm[2]] + dots[2 * step:]

    with jax.named_scope("A_seg5a"):
        cp_wm(0).wait()
        zz = zs[1]

        @pl.when(zz == 0)
        def _():
            dots = [fdot(k_, NT - 2, sb_(bt)) for bt in range(4) for k_ in 'ab']
            a_block(with_mod(0, dots, 2), gen_m(NT - 1, kb0, mkb(zz, 8, 0, {}), 8), 8, kb0)
    with jax.named_scope("A_seg5b"):
        cp_wm(1).wait()

        @pl.when(zz == 0)
        def _():
            dots = [('k', functools.partial(dot_k, kb0, 0, bt)) for bt in range(4)]
            a_block(with_mod(1, dots, 1), gen_m(NT - 1, kb1, mkb(zz, 8, 8, {}), 8), 8, kb1)

    def zero_of(vs):
        t_ = pltpu.bitcast(vs[0], u32)
        for v_ in vs[1:]:
            t_ = t_ | pltpu.bitcast(v_, u32)
        return t_ & kbuf[0, pl.ds(0, 8), :]

    def tie_at(w_, r0, c0, vs):
        mid = [w_[r0:r0 + 8, :c0]] if c0 else []
        mid.append(w_[r0:r0 + 8, c0:c0 + 128] | zero_of(vs))
        if c0 + 128 < w_.shape[1]:
            mid.append(w_[r0:r0 + 8, c0 + 128:])
        parts = ([w_[:r0]] if r0 else []) + [jnp.concatenate(mid, axis=1)] + ([w_[r0 + 8:]] if r0 + 8 < w_.shape[0] else [])
        return jnp.concatenate(parts, axis=0)

    def tied(wref, ties):
        w_ = wref[...]
        for (t, rb), vs in ties.items():
            w_ = tie_at(w_, 64 * (t % 5) + 8 * rb, 128 * (t // 5), vs)
        return w_

    def firsts(x):
        return [x[8 * g:8 * g + 8, 0:128] for g in range(x.shape[0] // 8)]

    def ln_chain(p):
        rows = pl.ds(p * R, R)
        pa, pb, pc, ps = [par[pl.ds(16 + 8 * t, 8), :][None] for t in range(4)]
        g3 = lambda x: x.reshape(R // 8, 8, D)
        q = g3(qbuf[rows, :].astype(f32))
        d1, r1 = _center(q)
        y = g3(jnp.concatenate([yb[j, rows, :] for j in range(NT)], axis=1))
        x = q + ((d1 * r1) * pa + pb) * y
        xn[rows, :] = x.reshape(R, D)
        d2, r2 = _center(x)
        h = (d2 * r2) * pc + ps
        hh[rows, :] = h.reshape(R, D)
        d3, r3 = _center(h, ALPHA)
        return (d3 * r3).reshape(R, D)

    def w1_dot(p, l3, ties, fresh):
        if fresh:
            ties[(0, 2)] = firsts(l3)[0:2]
            l3 = pltpu.bitcast(tie_at(pltpu.bitcast(l3, u32), 0, 128, firsts(l3)[2:4]), f32)
        z = _mm(l3.astype(bf16), tied(w1, ties))
        g = _gelu2a(z)
        lane = lax.broadcasted_iota(jnp.int32, (R, 128), 1)
        for j, (o1, cut, o2) in enumerate(((1, 128, 0), (1, 32, -1), (-1, 64, 2), (2, 96, -2), (-2, 128, 0))):
            gj = g[:, j * 128:(j + 1) * 128]
            if cut == 128:
                h1[j, pl.ds(p * R + 8 + o1, R), :] = gj
            else:
                pltpu.store(h1.at[j, pl.ds(p * R + 8 + o1, R), :], gj, mask=lane < cut)
                pltpu.store(h1.at[j, pl.ds(p * R + 8 + o2, R), :], gj, mask=lane >= cut)
        return z

    def w2_dot(p, ties):
        rows = pl.ds(p * R, R)
        hs = jnp.concatenate([h1[j, pl.ds(p * R + 8, R), :] for j in range(NT)], axis=1).astype(bf16)
        x1 = hh[rows, :] + _mm(hs, tied(w2, ties)) * BETA
        hh[rows, :] = x1
        return x1

    def ln4(r, n):
        d4, r4 = _center(hh[pl.ds(r, n), :], ALPHA)
        return d4 * r4

    zoff = [pl.multiple_of((zz >> p_) * 32, 32) for p_ in range(7)]

    def prep2(src, dst, tr, t, p_, anchor):
        zero = zero_of([anchor])
        gate = 0 if _SBU[p_][0] else 3
        l1 = [[], []]
        for k2 in range(2):
            for n2 in range(2):
                bl = []
                for b_ in range(4):
                    kq, nq = 2 * (b_ // 2) + k2, 2 * (b_ % 2) + n2
                    x = None
                    if _SBU[p_][b_]:
                        x = src[pl.ds(zoff[p_] + (8 * t + 192 * (nq if tr else kq)), 8), pl.ds(128 * (kq if tr else nq), 128)]
                        if b_ == gate and k2 == n2:
                            x = x | zero
                    bl.append(x)
                for e in range(2):
                    l1[e].append(_SB[p_](*[None if x is None else _unp(x, e) for x in bl]))
        for q_ in range(7):
            if 7 * p_ + q_ not in _PURE:
                dst[7 * p_ + q_, pl.ds(8 * t, 8), :] = _pk([_SB[q_](*l1[e]) for e in range(2)])

    def prep1(src, dst, r1, fs, ps_, t, n, anchor):
        bl = [src[pl.ds(lo + 8 * t, 8), pl.ds(c0 + 128 * n, 128)] for lo in (768, r1) for c0 in (0, 256)]
        zero = zero_of([anchor])
        bl[0], bl[3] = bl[0] | zero, bl[3] | zero
        for p_ in ps_:
            dst[p_, pl.ds(8 * t, 8), pl.ds(128 * n, 128)] = _pk([fs[p_](*[_unp(x, e) for x in bl]) for e in range(2)])

    def sc_lhs():
        return _as_bf16(jnp.concatenate([kb0[KOFF + 48 + j] for j in range(NT)], axis=1))

    units, l3s = [], {}
    anch = sorted({(ANCH[0] + (ANCH[1] - ANCH[0]) * i // ANCH[2]) % 80 for i in range(ANCH[2])})

    def run_block(dots, extra=None, pre4=False):
        for d_, (k_, p) in enumerate(dots):
            ties = {}
            e, rp = d_ - (len(dots) - NP4), TS // NP4
            if pre4 and e >= 0:
                nx = ln4(e * rp, rp)
                l4p[pl.ds(e * rp, rp), :] = nx
                ties[(TIE4, 7)] = firsts(nx)
            if extra is not None and d_ == len(dots) - 1:
                nx = ln_chain(extra)
                for pr in range(4):
                    ties[(24, XRB[pr])] = firsts(nx)[2 * pr:2 * pr + 2]
                l3s[extra] = nx.astype(bf16)
            if k_ == 1:
                fresh = p not in l3s
                res = w1_dot(p, ln_chain(p) if fresh else l3s.pop(p), ties, fresh)
            elif k_ == 2:
                res = w2_dot(p, ties)
            else:
                par[pl.ds(48, 8), :] = _mm(sc_lhs(), wmc[...])[0:8]
            for u_ in anch:
                if u_ // 40 + 1 == k_ and units and d_ < len(dots) - (NP4 + 1 if pre4 else 0):
                    n, g = (u_ % 40) // 8, u_ % 8
                    units.pop(0)(res[8 * g:8 * g + 8, 128 * n:128 * (n + 1)])

    pos = [N2, 0]

    def plan(lim1):
        last = lim1 == S // R
        dots = []
        while pos[0] < (lim1 if last else lim1 - 1) or pos[0] - pos[1] >= LEAD or (last and pos[1] < lim1):
            k_ = 0 if pos[0] - pos[1] < LEAD and pos[0] < lim1 else 1
            dots.append((k_ + 1, pos[k_]))
            pos[k_] += 1
        return dots, (None if last else pos[0])

    with jax.named_scope("P1"):
        wait_all([cp_wmp, cp_q[0]])
        mp = _mm(sc_lhs(), wmp[...])
        for t in range(WMP // 128):
            modb[2 * WMA // 128 + t] = mp[0:8, 128 * t:128 * (t + 1)]
        sa, ca, ga, sb, cb = [jnp.concatenate([modb[NT * k_ + j] for j in range(NT)], axis=1) for k_ in range(5)]
        par[pl.ds(16, 8), :] = ga * (1.0 + ca)
        par[pl.ds(24, 8), :] = ga * sa
        par[pl.ds(32, 8), :] = 1.0 + cb
        par[pl.ds(40, 8), :] = sb
        for bt in range(4):
            dot_k(kb1, 1, bt, _as_bf16(jnp.concatenate([kb0[KOFF + 17 + 2 * n] for n in range(8)], axis=0)))
        for p in range(PRELN):
            l3s[p] = ln_chain(p)
    with jax.named_scope("w1wait"):
        cp_w[0].wait()
    with jax.named_scope("P2"):
        run_block([(1, p) for p in range(N2)])
    with jax.named_scope("w2wait"):
        wait_all([cp_w[1], cp_q[1]])
    with jax.named_scope("P4"):
        run_block(*plan(Q1 // R))
    with jax.named_scope("q2wait"):
        wait_all([cp_q[2], cp_w[3]])
    units += [functools.partial(prep2, w4, w4s, False, t, p_) for t in range(24) for p_ in range(7)]
    units += [functools.partial(prep1, w4, w4o, 832, _SB, (0, 1, 3, 5, 6), t, n) for t in range(8) for n in range(2)]
    with jax.named_scope("P5"):
        run_block(*plan(Q2 // R))
    with jax.named_scope("q3wait"):
        wait_all([cp_q[3], cp_wmc, cp_w[2]])
    units += [functools.partial(prep2, w3, w3s, True, t, p_) for t in range(24) for p_ in range(7)]
    units += [functools.partial(prep1, w3, w3o, 816, _SA, (0, 2, 4, 5, 6), t, n) for t in range(6) for n in range(2)]
    with jax.named_scope("P6"):
        dots, _ = plan(S // R)
        run_block(dots[:-NP4] + [(3, 0)] + dots[-NP4:], pre4=True)
    assert not units

    quads = ((0, 0), (0, 256), (H2, 0), (H2, 256))
    done_at = [max(i for i, p_ in enumerate(ORD4) if any(k_ == kq for k_, _ in _SC[p_])) for kq in range(4)]
    qorder = sorted(range(4), key=lambda kq: done_at[kq])
    outs = [(0, 512, 128)] + [quads[kq] + (256,) for kq in qorder] + [(H2, 512, 128)]

    def out_copy(r, r0, c0, cn):
        rows = pl.ds(_mult(r + r0, H2), H2)
        return cp(obuf.at[rows, pl.ds(c0, cn)], o_hbm.at[0, rows, pl.ds(c0, cn)], osem.at[0])

    def b2_step(i, carry):
        r = pl.multiple_of(i * TS, TS)
        gs = gs_.at[i >> 8]
        lr = l4p[:, pl.ds(512, 128)]
        w3a = lambda p_: (w3[pl.ds(816, 48), pl.ds(256, 256)] if p_ == 1 else
                          w3[pl.ds(768, 48), pl.ds(0, 256)] if p_ == 3 else w3o[p_])
        lt_ = _blocks((0, 0), (H2, 0), (0, 256), (H2, 256))
        zt = _mm_nt(_as_bf16(w3[pl.ds(768, 96), pl.ds(512, 128)]), lr.astype(bf16))
        zt = zt + _quad(_comb([_mm_nt(_as_bf16(w3a(p_)), _SB[p_](*lt_).load(l4p_.at[i >> (20 + p_)], H2, 256))
                               for p_ in range(7)]))
        gt = jnp.concatenate([_gelu2a(zt), jnp.zeros((64, TS), f32)], axis=0)
        gs[:, pl.ds(0, 128)] = gt[:128].T
        gs[:, pl.ds(896, 128)] = gt[128:].T
        lrs = [lr[:H2].astype(bf16), lr[H2:].astype(bf16)]
        ab = _blocks(*quads)
        ops = {}
        for t in range(3):
            cq, left = [None] * 4, [5, 3, 3, 5]

            def add(k_, x, sg=1):
                cq[k_] = x if cq[k_] is None else cq[k_] + x if sg > 0 else cq[k_] - x
                left[k_] -= 1
                if left[k_] == 0:
                    gg = _gelu2a(cq[k_])
                    for n2 in range(2):
                        cols = pl.ds(128 + 896 * (k_ % 2) + 128 * (t + 3 * n2), 128)
                        gs[pl.ds(H2 * (k_ // 2), H2), cols] = gg[:, 128 * n2:128 * (n2 + 1)]

            for p_ in range(8):
                for k_ in (2, 1, 0, 3):
                    if REMP[k_] == p_:
                        wr = [w3[pl.ds(64 * (t + 3 * (2 * (k_ % 2) + n2)), 64), pl.ds(512, 128)] for n2 in range(2)]
                        add(k_, _mm_nt(lrs[k_ // 2], _as_bf16(jnp.concatenate(wr, axis=0))))
                if p_ == 7:
                    break
                a_ = _SA[p_](*ab)
                sub_ = (a_, a_.shift(0, 128), a_.shift(Q4, 0), a_.shift(Q4, 128))
                pr = []
                for q_ in range(7):
                    n = 7 * p_ + q_
                    if n not in ops:
                        ops[n] = _SA[q_](*sub_).load(l4p_.at[(i + 4 * p_) >> (9 + q_)], Q4, 128)
                    w_ = (w3[pl.ds(192 * _PURE[n] + 64 * t, 64), pl.ds(128 * _PURE[n], 128)] if n in _PURE
                          else w3s[n, pl.ds(64 * t, 64), :])
                    pr.append(_mm_nt(ops[n], _as_bf16(w_)))
                m_ = _quad(_comb(pr))
                for k_, sg in _SC[p_]:
                    add(k_, m_, sg)
        kord = [(0, 768), (896, 832)] + [x for c in (0, 3, 1, 4, 2, 5)
                                         for x in ((128 + 128 * c, 64 * c), (1024 + 128 * c, 384 + 64 * c))]
        wl = jnp.concatenate([w4[pl.ds(wr_, 64), pl.ds(512, 128)] for _, wr_ in kord], axis=0)
        gk = lambda r0: jnp.concatenate([gs[pl.ds(r0, H2), pl.ds(o_, 128)] for o_, _ in kord], axis=1).astype(bf16)
        acc_t = _mm(gk(0), wl)
        rn_ = pl.multiple_of(jnp.minimum(i + 1, S // TS - 1) * TS, TS)
        rp = TS // len(LNT)
        ties = {}
        for e, k_ in enumerate(LNT):
            nx = ln4(pl.multiple_of(rn_ + e * rp, rp), rp)
            l4p[pl.ds(e * rp, rp), :] = nx
            ties[k_] = firsts(nx)
        gb_ = _blocks((0, 0), (0, 896), (H2, 0), (H2, 896))
        ms = [None] * 7
        for idx, p_ in enumerate(ORD4):
            a_ = _SA[p_](*gb_)
            wo = (w4[pl.ds(768, 64), pl.ds(0, 256)] if p_ == 2 else
                  w4[pl.ds(832, 64), pl.ds(256, 256)] if p_ == 4 else w4o[p_])
            if idx in ties:
                wo = tie_at(wo, 0, 0, ties[idx])
            m_ = _mm(a_.load(gs, H2, 128), wo)
            sub_ = (a_.shift(0, 128), a_.shift(0, 512), a_.shift(Q4, 128), a_.shift(Q4, 512))
            pr = []
            for q_ in range(7):
                n = 7 * p_ + q_
                w_ = (w4[pl.ds(192 * _PURE[n], 192), pl.ds(128 * _PURE[n], 128)] if n in _PURE
                      else w4s[n, pl.ds(0, 192), :])
                pr.append(_mm(_SA[q_](*sub_).load(gs_.at[(i + 4 * p_) >> (9 + q_)], Q4, 384), w_))
            ms[p_] = m_ + _quad(_comb(pr))
        cs = _comb(ms)
        for k_ in ties:
            if k_ >= 10:
                wl = tie_at(wl, 64 * (k_ - 10), 0, ties[k_])
        accs = [acc_t] + [cs[kq] for kq in qorder] + [_mm(gk(H2), wl)]
        gbv = par[pl.ds(48, 8), :]
        for (r0, c0, cn), ac in zip(outs, accs):
            rows, cols = pl.ds(_mult(r + r0, H2), H2), pl.ds(c0, cn)
            g3 = lambda x: x.reshape(H2 // 8, 8, cn)
            out = g3(xn[rows, cols]) + gbv[None, :, c0:c0 + cn] * g3(hh[rows, cols] + BETA * ac)
            obuf[rows, cols] = out.reshape(H2, cn).astype(bf16)
            out_copy(r, r0, c0, cn).start()
        return carry

    with jax.named_scope("BII"):
        lax.fori_loop(0, S // TS, b2_step, 0)
    with jax.named_scope("out_wait"):
        for i in range(S // TS):
            for o_ in outs:
                out_copy(i * TS, *o_).wait()


@jax.jit
def pallas_adaLN_cond__ssm_conv_h3__mixer_s_mlp__prompt_kernel(
    A_q: jax.Array,
    A_k: jax.Array,
    A_v: jax.Array,
    A_shift_k: jax.Array,
    A_ssm_k: jax.Array,
    A_ssm_D: jax.Array,
    B_x: jax.Array,
    B_w1: jax.Array,
    B_w2: jax.Array,
    B_w3: jax.Array,
    B_w4: jax.Array,
    c: jax.Array,
    w_mod: jax.Array,
):
    del B_x
    hbm = pl.BlockSpec(memory_space=pltpu.MemorySpace.HBM)
    spec = pltpu.VMEM((NG * 2 * NC, 8, 128), f32)
    part = pltpu.VMEM((KOFF + 56, 8, 128), f32)
    return pl.pallas_call(
        _kernel,
        out_shape=jax.ShapeDtypeStruct((1, S, D), bf16),
        in_specs=[hbm] * 12,
        out_specs=hbm,
        scratch_shapes=[
            pltpu.VMEM((27, 8, 128), f32),
            pltpu.VMEM((S, D), bf16),
            pltpu.VMEM((NT, 32 + HS, 128), u32),
            pltpu.VMEM((NT, 32 + HS, 128), u32),
            pltpu.VMEM((NT, 64, S), u32),
            pltpu.VMEM((D // 2, D), u32),
            pltpu.VMEM((D // 2, D), u32),
            pltpu.VMEM((F // 2, D), u32),
            pltpu.VMEM((896, D), u32),
            pltpu.VMEM((2, D // 2, WMA), u32),
            pltpu.VMEM((D // 2, WMP), u32),
            pltpu.VMEM((D // 2, WMC), u32),
            pltpu.VMEM((S, D), bf16),
            spec, spec, spec, spec,
            part, part,
            pltpu.VMEM((NT, S, 128), f32),
            pltpu.VMEM((S, D), f32),
            pltpu.VMEM((S, D), f32),
            pltpu.VMEM((NT, S + 32, 128), f32),
            pltpu.VMEM((64, D), f32),
            pltpu.VMEM((1, TS, D), f32),
            pltpu.VMEM((1, TS, 1792), f32),
            pltpu.VMEM((52, 200, 128), u32),
            pltpu.VMEM((52, 200, 128), u32),
            pltpu.VMEM((7, 64, 256), u32),
            pltpu.VMEM((7, 48, 256), u32),
            pltpu.VMEM((4, D), bf16),
            pltpu.VMEM((D,), bf16),
            pltpu.VMEM((1, D), bf16),
            pltpu.SMEM((2,), jnp.int32),
            pltpu.SemaphoreType.DMA((20,)),
            pltpu.SemaphoreType.DMA((1,)),
        ],
        compiler_params=pltpu.CompilerParams(vmem_limit_bytes=100 * 1024 * 1024, disable_semaphore_checks=True),
    )(A_q, A_k, A_v, A_shift_k.T, A_ssm_k, A_ssm_D, B_w1, B_w2, B_w3.T, B_w4, c, w_mod)
```

```python
import functools
import math

import jax
import jax.numpy as jnp
from jax import lax
import jax.experimental.pallas as pl
import jax.experimental.pallas.tpu as pltpu

S, D, F = 2048, 640, 1728
EPS = 1e-5
NT = D // 128
HS = S // 2

C = 128
NC = S // C
NG = 16
KOFF = (NC + 1) * NG * 3
W = 4
G0 = 4
HEAD, TAIL = 250, 450
DORDER = 'aHbU'
WMA, WMP, WMC = 1280, 640, 640
R = 64
Q0, Q1, Q2 = 320, 768, 1408
N2, PRELN, LEAD, NP4, TIE4 = 5, 2, 3, 2, 12
XRB = (7, 4, 2, 0)
ANCH = (20, 58, 18)
TS = 512
H2, Q4 = TS // 2, TS // 4
LNT = (0, 1, 2, 3, 4, 5, 18, 22)
REMP = (6, 5, 3, 7)
ORD4 = (0, 5, 4, 1, 3, 2, 6)
SKIPA = 0
ZM = 4
NOBC = True
GBP = 1

_C0 = math.sqrt(2.0 / math.pi)
ALPHA = (_C0 * 0.044715) ** (1.0 / 3.0)
GC = _C0 / ALPHA
BETA = 0.5 / ALPHA

f32 = jnp.float32
bf16 = jnp.bfloat16
u32 = jnp.uint32
NTDIMS = (((1,), (1,)), ((), ()))

_SA = (lambda a, b, c, d: a + d, lambda a, b, c, d: d, lambda a, b, c, d: c + d, lambda a, b, c, d: a,
       lambda a, b, c, d: a + b, lambda a, b, c, d: b - d, lambda a, b, c, d: c - a)
_SB = (lambda a, b, c, d: a + d, lambda a, b, c, d: c - a, lambda a, b, c, d: a, lambda a, b, c, d: b - d,
       lambda a, b, c, d: d, lambda a, b, c, d: c + d, lambda a, b, c, d: a + b)
_SBU = ((1, 0, 0, 1), (1, 0, 1, 0), (1, 0, 0, 0), (0, 1, 0, 1), (0, 0, 0, 1), (0, 0, 1, 1), (1, 1, 0, 0))
_SC = (((0, 1), (3, 1)), ((0, 1), (2, 1)), ((2, 1), (3, -1)), ((1, 1), (3, 1)), ((0, -1), (1, 1)), ((0, 1),), ((3, 1),))
_PURE = {7 * p + q: 2 * i + j for i, p in enumerate((2, 4)) for j, q in enumerate((2, 4))}


def _comb(m):
    m1, m4, m2, m3, m5, m7, m6 = m
    return (m1 + m4) + (m7 - m5), m3 + m5, m4 + m2, (m1 + (m3 - m2)) + m6


def _quad(c):
    return jnp.concatenate([jnp.concatenate(c[0:2], axis=1), jnp.concatenate(c[2:4], axis=1)], axis=0)


class _Lazy:
    def __init__(self, terms):
        self.terms = terms

    def __add__(self, o):
        return _Lazy(self.terms + o.terms)

    def __sub__(self, o):
        return _Lazy(self.terms + [(-s, r, c) for (s, r, c) in o.terms])

    def shift(self, dr, dc):
        return _Lazy([(s, r + dr, c + dc) for (s, r, c) in self.terms])

    def load(self, ref, rn, cn):
        ts = sorted(self.terms, key=lambda t: -t[0])
        acc = None
        for (s, r, c) in ts:
            x = ref[pl.ds(r, rn), pl.ds(c, cn)]
            acc = x if acc is None else acc + x if s > 0 else acc - x
        return acc.astype(bf16)


def _blocks(*offsets):
    return [_Lazy([(1, r, c)]) for (r, c) in offsets]


def _unp(w, e):
    return pltpu.unpack_elementwise(w, index=e, packed_dtype=bf16, unpacked_dtype=f32)


def _pk(xs):
    return pltpu.pack_elementwise(xs, packed_dtype=bf16)


def _as_bf16(w):
    return pltpu.bitcast(w, bf16)


def _mm(x, w):
    return jnp.dot(x, _as_bf16(w), preferred_element_type=f32)


def _mm_nt(x, w):
    return lax.dot_general(x, w, NTDIMS, preferred_element_type=f32)


def _mult(x, n):
    return x if isinstance(x, int) else pl.multiple_of(x, n)


def _cos_table(m, scale):
    mm = jnp.abs(((m + 256) & 511) - 256)
    x = (128 - mm).astype(f32) * (1.0 / 128.0)
    x2 = x * x
    h = math.pi / 2
    p = -(h ** 7) / 5040 + x2 * ((h ** 9) / 362880 - x2 * (h ** 11) / 39916800)
    p = h + x2 * (-(h ** 3) / 6 + x2 * ((h ** 5) / 120 + x2 * p))
    return (x * scale) * p


def _dft_tables():
    shape = (16, 8, 128)
    n = lax.broadcasted_iota(jnp.int32, shape, 0)
    s = lax.broadcasted_iota(jnp.int32, shape, 1)
    l = lax.broadcasted_iota(jnp.int32, shape, 2)
    fw, fu, iv = [], [], []
    wv = l >> 4
    tu = (16 * W) * (wv // W) + (2 * W) * ((l >> 1) & 7) + 2 * (wv % W) + (l & 1)
    for e in range(2):
        r = 2 * s + e
        j = 8 * n + (r & 7)
        fw.append(_cos_table((4 * j + 1) * l + (r >> 3) * 128, 1.0))
        fu.append(_cos_table((4 * j + 1) * tu + (r >> 3) * 128, 1.0))
        b = 16 * (n >> 1) + r
        col = 128 * (n & 1) + l
        iv.append(_cos_table((4 * (col >> 1) + 1) * b + (col & 1) * 128, 1.0 / 128.0))
    return [pltpu.bitcast(_pk(x), f32) for x in (fw, iv, fu)]


def _gelu2a(z):
    return z * (1.0 + jnp.tanh(z * (z * z + GC)))


def _center(x, scale=1.0):
    s1 = jnp.sum(x, axis=-1, keepdims=True)
    m = s1 * (1.0 / D)
    ssd = jnp.maximum(jnp.sum(x * x, axis=-1, keepdims=True) - s1 * m, 0.0)
    rstd = jnp.exp2(jnp.log(ssd + D * EPS) * (-0.5 / math.log(2.0)) + math.log2(scale * math.sqrt(D)))
    return x - m, rstd


def _conv(us, gs, a):
    acc = None
    for c in range(a + 1):
        p = us[c] * gs[a - c]
        acc = p if acc is None else acc + p
    return acc


def _kernel(q_hbm, k_hbm, v_hbm, sk_hbm, h_hbm, dd_hbm, w1_hbm, w2_hbm, w3_hbm, w4_hbm, c_hbm, wm_hbm, o_hbm,
            modb, qbuf, kbuf, vbuf, hbuf, w1, w2, w3_, w4_, wm, wmp, wmc, obuf, ub0, ub1, gb0, gb1, kb0, kb1,
            yb, xn, hh, h1, par, l4p_, gs_, w4s, w3s, w4o, w3o, sk_s, dd_s, c_s, zs, sems, osem):
    l4p, w3, w4 = l4p_.at[0], w3_.at[0], w4_.at[0]
    ubs, gbs, kbs = (ub0, ub1), (gb0, gb1), (kb0, kb1)
    cp = pltpu.make_async_copy

    def cp_h(j, c0, c1, sem):
        cols = pl.ds(c0, c1 - c0)
        return cp(h_hbm.at[pl.ds(j * 128, 128), cols], hbuf.bitcast(bf16).at[j, :, cols], sem)

    def cp_kv(j, r0, r1, sem):
        r0, r1 = (r0 + 16 if r0 else 0), min(r1 + 16, S)
        lanes = pl.ds(j * 128, 128)
        return [cp(k_hbm.at[0, pl.ds(r0, r1 - r0), lanes], kbuf.bitcast(bf16).at[j, pl.ds(r0 + 16, r1 - r0), :], sem),
                cp(v_hbm.at[0, pl.ds(r0, r1 - r0), lanes], vbuf.bitcast(bf16).at[j, pl.ds(r0, r1 - r0), :], sem)]

    def cp_tile(j, i):
        sem = sems.at[2 * j + i]
        return [cp_h(j, i * HS, (i + 1) * HS, sem)] + cp_kv(j, i * HS, (i + 1) * HS, sem)

    def cp_wm(i):
        return cp(wm_hbm.at[:, pl.ds(i * WMA, WMA)], wm.bitcast(bf16).at[i], sems.at[10 + i])

    def wait_all(cps):
        for c_ in cps:
            c_.wait()

    cp_t0 = [[cp_h(0, 0, S, sems.at[0])], cp_kv(0, 0, 1024, sems.at[1]), cp_kv(0, 1024, 1536, sems.at[17]),
             cp_kv(0, 1536, S, sems.at[18])]
    cp_wmp = cp(wm_hbm.at[:, pl.ds(2 * WMA, WMP)], wmp.bitcast(bf16), sems.at[13])
    cp_wmc = cp(wm_hbm.at[:, pl.ds(2 * WMA + WMP, WMC)], wmc.bitcast(bf16), sems.at[12])
    cp_q = [cp(q_hbm.at[0, pl.ds(r0, r1 - r0), :], qbuf.at[pl.ds(r0, r1 - r0), :], sems.at[sm])
            for sm, r0, r1 in ((13, 0, Q0), (16, Q0, Q1), (14, Q1, Q2), (12, Q2, S))]
    cp_w = [cp(w1_hbm, w1.bitcast(bf16), sems.at[15]), cp(w2_hbm, w2.bitcast(bf16), sems.at[16]),
            cp(w3_hbm, w3_.bitcast(bf16).at[0], sems.at[12]),
            cp(w4_hbm, w4_.bitcast(bf16).at[0, pl.ds(0, F), :], sems.at[14])]
    cp_s = [cp(sk_hbm, sk_s, sems.at[19]), cp(dd_hbm, dd_s, sems.at[19]), cp(c_hbm, c_s, sems.at[19])]
    order = list(cp_s)
    for grp in cp_t0:
        order += grp
    for j in range(1, NT):
        order += cp_tile(j, 0) + cp_tile(j, 1)
    order += [cp_wm(0), cp_wm(1), cp_wmp, cp_q[0], cp_w[0], cp_w[1], cp_q[1], cp_q[2], cp_w[3], cp_q[3], cp_wmc, cp_w[2]]
    for c_ in order:
        c_.start()

    with jax.named_scope("init"):
        tables = _dft_tables()
        for kb in kbs:
            for i, tb in enumerate(tables):
                kb[pl.ds(KOFF + 16 * i, 16)] = tb
            kb[pl.ds(0, NG * 3)] = jnp.zeros((NG * 3, 8, 128), f32)
        w4[pl.ds(F // 2, 32), :] = jnp.zeros((32, D), u32)
        for j in range(NT):
            kbuf[j, pl.ds(0, 8), :] = jnp.zeros((8, 128), u32)
            kbuf[j, pl.ds(8 + HS, 8), :] = jnp.zeros((8, 128), u32)
            vbuf[j, pl.ds(HS, 8), :] = jnp.zeros((8, 128), u32)
            h1[j, pl.ds(8, 8), :] = jnp.zeros((8, 128), f32)
            h1[j, pl.ds(S, 8), :] = jnp.zeros((8, 128), f32)
        wait_all(cp_s)
        par[pl.ds(0, 4), :] = sk_s[...].astype(f32)
        par[pl.ds(8, 8), :] = jnp.broadcast_to(dd_s[...].astype(f32).reshape(1, D), (8, D))
        cv = c_s[...].astype(f32)
        sc = jnp.broadcast_to(cv * jax.nn.sigmoid(cv), (8, D))
        scp = pltpu.bitcast(_pk([sc, sc]), f32)
        for kb in kbs:
            for j in range(NT):
                kb[KOFF + 48 + j] = scp[:, 128 * j:128 * (j + 1)]

    def mkb(i, unr, off, cache):
        def b(stride, extra=0, z=None):
            if isinstance(i, int):
                return (i * unr + off) * stride + extra
            key = (unr * stride, z)
            if key not in cache:
                base = pl.multiple_of(i * (unr * stride), unr * stride)
                cache[key] = base if z is None else pl.multiple_of(base + (i >> z) * ZM, ZM)
            return cache[key] + (off * stride + extra)
        return b

    def store_spec(ref, b, x):
        for rg in range(2 * NG):
            for cc in range(4):
                ref[b(4, cc + rg * NC)] = x[8 * rg:8 * rg + 8, 128 * cc:128 * cc + 128]

    def dot_h(j, b, lhs):
        hc = hbuf[j, :, pl.ds(_mult(b(512), 512), 512)]
        rhs_t = jnp.concatenate([hc[:, C * cc:C * (cc + 1)] for cc in range(4)], axis=0)
        store_spec(gbs[j % 2], b, _mm_nt(lhs, _as_bf16(rhs_t)))

    def dot_u(j, b, lhs):
        taps = [par[pl.ds(t, 1), pl.ds(j * 128, 128)] for t in range(4)]
        cols = []
        for cc in range(4):
            words = []
            for blk in range(8 // W):
                w0 = 64 * cc + 8 * W * blk
                kw = {m: kbuf[j, pl.ds(b(256, 8 + w0 + m), 8, stride=W), :] for m in range(-2, W)}
                kk = {2 * m + e: _unp(kw[m], e) for m in range(-2, W) for e in range(2) if 2 * m + e >= -3}
                for m in range(W):
                    vw = vbuf[j, pl.ds(b(256, w0 + m), 8, stride=W), :]
                    pair = []
                    for e in range(2):
                        n = 2 * m + e
                        ks = kk[n] * taps[0] + kk[n - 1] * taps[1] + kk[n - 2] * taps[2] + kk[n - 3] * taps[3]
                        pair.append(ks * _unp(vw, e))
                    words.append(_pk(pair))
            cols.append(jnp.concatenate(words, axis=0))
        store_spec(ubs[j % 2], b, _mm(lhs, jnp.concatenate(cols, axis=1)))

    def out_spec(kidx, groups, nc):
        cols = [[] for _ in range(nc)]
        for gi in groups:
            prev = None
            for cc in range(-1, nc):
                k0, k1, k2 = [kidx(((cc + 1) * NG + gi) * 3 + t) for t in range(3)]
                re, im = k0 - k2, k0 + k1
                if prev is not None:
                    cols[cc].append(_pk([re - prev[1], im + prev[0]]))
                prev = (re, im)
        return jnp.concatenate([jnp.concatenate(c_, axis=0) for c_ in cols], axis=1)

    def dot_i(j, b, half, lhs):
        y = _mm(lhs, out_spec(lambda o: kbs[j % 2][b(4 * NG * 3, 2 * half * NG * 3 + o)], range(NG), 2))
        for cc in range(2):
            yb[j, pl.ds(b(512, (2 * half + cc) * C), C), :] = y[:, 128 * cc:128 * cc + 128]

    def dot_k(kb, kt, bt, lhs):
        y = _mm(lhs, out_spec(lambda o: kb[4 * bt * NG * 3 + o], range(8 * kt, 8 * kt + 8), 4))
        for cc in range(4):
            rows = pl.ds((4 * bt + cc) * C, C)
            yc = y[:, 128 * cc:128 * cc + 128]
            yb[NT - 1, rows, :] = yc if kt == 0 else yb[NT - 1, rows, :] + yc

    def gen_m(j, kb, b, ng):
        ub, gb = ubs[j % 2], gbs[j % 2]
        for s in range(ng):
            for t in range(3):
                re = lambda ref, c: ref[b(2 * NC, 2 * s * NC + c, 8 + t)]
                im = lambda ref, c: ref[b(2 * NC, (2 * s + 1) * NC + c, 8 + t)]
                gre = [re(gb, c) for c in range(NC)]
                if t == 0:
                    us, gs = [re(ub, c) + im(ub, c) for c in range(NC)], gre
                elif t == 1:
                    us, gs = [re(ub, c) for c in range(NC)], [im(gb, c) - gre[c] for c in range(NC)]
                else:
                    us, gs = [im(ub, c) for c in range(NC)], [im(gb, c) + gre[c] for c in range(NC)]
                ue, uo, ge, go = us[0::2], us[1::2], gs[0::2], gs[1::2]
                usum = [x + y for x, y in zip(ue, uo)]
                gsum = [x + y for x, y in zip(ge, go)]
                poo_prev = None
                for a in range(NC // 2):
                    pee, poo, pss = _conv(ue, ge, a), _conv(uo, go, a), _conv(usum, gsum, a)
                    kb[b(3, ((2 * a + 1) * NG + s) * 3 + t)] = pee if poo_prev is None else pee + poo_prev
                    kb[b(3, ((2 * a + 2) * NG + s) * 3 + t)] = pss - pee - poo
                    poo_prev = poo
                    yield 3 * (2 * a + 1) + 7

    def add_d(j):
        gb = gbs[j % 2]
        dvec = par[pl.ds(8, 8), pl.ds(j * 128, 128)]
        for gi in range(NG):
            gb[2 * gi * NC] = gb[2 * gi * NC] + dvec

    def dot_m(i, t0, nt, rows):
        m = None
        for kt in range(NT):
            p = _mm(_as_bf16(rows[kt]), wm[i, pl.ds(64 * kt, 64), pl.ds(128 * t0, 128 * nt)])
            m = p if m is None else m + p
        for t in range(nt):
            modb[i * (WMA // 128) + (t0 + t)] = m[0:8, 128 * t:128 * (t + 1)]

    pre = dict(H=0, U=672 + 96 // W, a=192, b=192, m=0, k=176)
    post = dict(H=0, U=0, a=4, b=4, m=2, k=0)
    nst = dict(H=16, U=16, a=8, b=8, m=5, k=8)

    def a_block(dots, mg=None, ng=0, tbl=kb0):
        if SKIPA:
            return
        native, dur = [], []
        for idx, (k_, _) in enumerate(dots):
            nxt = pre[dots[idx + 1][0]] if idx + 1 < len(dots) else 0
            d_ = 2.0 if k_ == 'm' else 1.0
            native += [nxt / nst[k_] + post[k_] * d_] * nst[k_]
            dur += [d_] * nst[k_]
        if mg is not None and dots:
            head = max(HEAD - pre[dots[0][0]], 0)
            mtot = 744 * ng - TAIL - head
            lvl = (mtot + sum(native)) / sum(dur)
            want = [max(lvl * d_ - x, 0.0) for x, d_ in zip(native, dur)]
            cum = [head]
            for w_ in want:
                cum.append(cum[-1] + w_ * mtot / sum(want))
        done, step = 0.0, 0
        for (k_, fn) in dots:
            rows = []
            for n in range(nst[k_]):
                while mg is not None and done < cum[step]:
                    done += next(mg)
                step += 1
                if k_ in 'ab':
                    rows.append(jnp.concatenate([tbl[KOFF + 16 + 2 * n], tbl[KOFF + 17 + 2 * n]], axis=1))
                else:
                    rows.append(tbl[KOFF + dict(H=n, U=32 + n, k=16 + 2 * n, m=48 + n)[k_]])
            fn(rows if k_ == 'm' else _as_bf16(jnp.concatenate(rows, axis=0)))
        for _ in (mg or ()):
            pass

    def fdot(k_, j, b):
        if k_ in 'HU':
            return (k_, functools.partial(dot_h if k_ == 'H' else dot_u, j, b))
        return (k_, functools.partial(dot_i, j, b, 0 if k_ == 'a' else 1))

    def a_loop(jf, jm, ji, g0, ng):
        kinds = [k_ for k_ in DORDER if k_ in 'HU' or ji is not None]

        def body(i, carry):
            cache = {}
            zs[i] = 0
            dots = [fdot(k_, jf if k_ in 'HU' else ji, mkb(i, 2, s_, cache)) for s_ in range(2) for k_ in kinds]
            a_block(dots, gen_m(jm, kbs[jm % 2], mkb(i, ng, g0, cache), ng), ng, kbs[jm % 2])

            @pl.when(i == 0)
            def _():
                wait_all(cp_tile(jf, 1))
            return carry
        wait_all(cp_tile(jf, 0))
        lax.fori_loop(0, 2, body, 0)
        add_d(jf)

    sb_ = lambda bt: mkb(0, 1, bt, None)
    with jax.named_scope("A_seg0"):
        wait_all(cp_t0[0])
        a_block([fdot('H', 0, sb_(bt)) for bt in range(4)])
        add_d(0)
        wait_all(cp_t0[1])
        a_block([fdot('U', 0, sb_(bt)) for bt in range(2)])
        for bt in (2, 3):
            wait_all(cp_t0[bt])
            a_block([fdot('U', 0, sb_(bt))])
    with jax.named_scope("A_m0"):
        def body_m0(i, carry):
            a_block([], gen_m(0, kb0, mkb(i, G0 // 2, 0, {}), G0 // 2))
            return carry
        lax.fori_loop(0, 2, body_m0, 0)
    for seg in range(1, NT):
        with jax.named_scope(f"A_seg{seg}"):
            if seg == 1:
                a_loop(1, 0, None, G0, (NG - G0) // 2)
            else:
                a_loop(seg, seg - 1, seg - 2, 0, 8)

    def with_mod(i, dots, step):
        mm = [('m', functools.partial(dot_m, i, t0, nt)) for (t0, nt) in ((0, 4), (4, 4), (8, 2))]
        return [mm[0]] + dots[:step] + [mm[1]] + dots[step:2 * step] + [mm[2]] + dots[2 * step:]

    with jax.named_scope("A_seg5a"):
        cp_wm(0).wait()
        zz = zs[1]

        @pl.when(zz == 0)
        def _():
            dots = [fdot(k_, NT - 2, sb_(bt)) for bt in range(4) for k_ in 'ab']
            a_block(with_mod(0, dots, 2), gen_m(NT - 1, kb0, mkb(zz, 8, 0, {}), 8), 8, kb0)
    with jax.named_scope("A_seg5b"):
        cp_wm(1).wait()

        @pl.when(zz == 0)
        def _():
            dots = [('k', functools.partial(dot_k, kb0, 0, bt)) for bt in range(4)]
            a_block(with_mod(1, dots, 1), gen_m(NT - 1, kb1, mkb(zz, 8, 8, {}), 8), 8, kb1)

    def zero_of(vs):
        t_ = pltpu.bitcast(vs[0], u32)
        for v_ in vs[1:]:
            t_ = t_ | pltpu.bitcast(v_, u32)
        return t_ & kbuf[0, pl.ds(0, 8), :]

    def tie_at(w_, r0, c0, vs):
        mid = [w_[r0:r0 + 8, :c0]] if c0 else []
        mid.append(w_[r0:r0 + 8, c0:c0 + 128] | zero_of(vs))
        if c0 + 128 < w_.shape[1]:
            mid.append(w_[r0:r0 + 8, c0 + 128:])
        parts = ([w_[:r0]] if r0 else []) + [jnp.concatenate(mid, axis=1)] + ([w_[r0 + 8:]] if r0 + 8 < w_.shape[0] else [])
        return jnp.concatenate(parts, axis=0)

    def tied(wref, ties):
        w_ = wref[...]
        for (t, rb), vs in ties.items():
            w_ = tie_at(w_, 64 * (t % 5) + 8 * rb, 128 * (t // 5), vs)
        return w_

    def firsts(x):
        return [x[8 * g:8 * g + 8, 0:128] for g in range(x.shape[0] // 8)]

    def ln_chain(p):
        rows = pl.ds(p * R, R)
        pa, pb, pc, ps = [par[pl.ds(16 + 8 * t, 8), :][None] for t in range(4)]
        g3 = lambda x: x.reshape(R // 8, 8, D)
        q = g3(qbuf[rows, :].astype(f32))
        d1, r1 = _center(q)
        y = g3(jnp.concatenate([yb[j, rows, :] for j in range(NT)], axis=1))
        x = q + ((d1 * r1) * pa + pb) * y
        xn[rows, :] = x.reshape(R, D)
        d2, r2 = _center(x)
        h = (d2 * r2) * pc + ps
        hh[rows, :] = h.reshape(R, D)
        d3, r3 = _center(h, ALPHA)
        return (d3 * r3).reshape(R, D)

    def w1_dot(p, l3, ties, fresh):
        if fresh:
            ties[(0, 2)] = firsts(l3)[0:2]
            l3 = pltpu.bitcast(tie_at(pltpu.bitcast(l3, u32), 0, 128, firsts(l3)[2:4]), f32)
        z = _mm(l3.astype(bf16), tied(w1, ties))
        g = _gelu2a(z)
        lane = lax.broadcasted_iota(jnp.int32, (R, 128), 1)
        for j, (o1, cut, o2) in enumerate(((1, 128, 0), (1, 32, -1), (-1, 64, 2), (2, 96, -2), (-2, 128, 0))):
            gj = g[:, j * 128:(j + 1) * 128]
            if cut == 128:
                h1[j, pl.ds(p * R + 8 + o1, R), :] = gj
            else:
                pltpu.store(h1.at[j, pl.ds(p * R + 8 + o1, R), :], gj, mask=lane < cut)
                pltpu.store(h1.at[j, pl.ds(p * R + 8 + o2, R), :], gj, mask=lane >= cut)
        return z

    def w2_dot(p, ties):
        rows = pl.ds(p * R, R)
        hs = jnp.concatenate([h1[j, pl.ds(p * R + 8, R), :] for j in range(NT)], axis=1).astype(bf16)
        x1 = hh[rows, :] + _mm(hs, tied(w2, ties)) * BETA
        hh[rows, :] = x1
        return x1

    def ln4(r, n):
        d4, r4 = _center(hh[pl.ds(r, n), :], ALPHA)
        return d4 * r4

    zoff = [zz >> p_ for p_ in range(7)]

    def prep2(src, dst, tr, t, p_, anchor):
        zero = zero_of([anchor])
        gate = 0 if _SBU[p_][0] else 3
        l1 = [[], []]
        for k2 in range(2):
            for n2 in range(2):
                bl = []
                for b_ in range(4):
                    kq, nq = 2 * (b_ // 2) + k2, 2 * (b_ % 2) + n2
                    x = None
                    if _SBU[p_][b_]:
                        x = src[zoff[p_], pl.ds(8 * t + 192 * (nq if tr else kq), 8), pl.ds(128 * (kq if tr else nq), 128)]
                        if b_ == gate and k2 == n2:
                            x = x | zero
                    bl.append(x)
                for e in range(2):
                    l1[e].append(_SB[p_](*[None if x is None else _unp(x, e) for x in bl]))
        for q_ in range(7):
            if 7 * p_ + q_ not in _PURE:
                dst[7 * p_ + q_, pl.ds(8 * t, 8), :] = _pk([_SB[q_](*l1[e]) for e in range(2)])

    def prep1(src, dst, r1, fs, ps_, t, n, anchor):
        bl = [src[pl.ds(lo + 8 * t, 8), pl.ds(c0 + 128 * n, 128)] for lo in (768, r1) for c0 in (0, 256)]
        zero = zero_of([anchor])
        bl[0], bl[3] = bl[0] | zero, bl[3] | zero
        for p_ in ps_:
            dst[p_, pl.ds(8 * t, 8), pl.ds(128 * n, 128)] = _pk([fs[p_](*[_unp(x, e) for x in bl]) for e in range(2)])

    def sc_lhs():
        return _as_bf16(jnp.concatenate([kb0[KOFF + 48 + j] for j in range(NT)], axis=1))

    units, l3s = [], {}
    anch = sorted({(ANCH[0] + (ANCH[1] - ANCH[0]) * i // ANCH[2]) % 80 for i in range(ANCH[2])})

    def run_block(dots, extra=None, pre4=False):
        for d_, (k_, p) in enumerate(dots):
            ties = {}
            e, rp = d_ - (len(dots) - NP4), TS // NP4
            if pre4 and e >= 0:
                nx = ln4(e * rp, rp)
                l4p[pl.ds(e * rp, rp), :] = nx
                ties[(TIE4, 7)] = firsts(nx)
            if extra is not None and d_ == len(dots) - 1:
                nx = ln_chain(extra)
                for pr in range(4):
                    ties[(24, XRB[pr])] = firsts(nx)[2 * pr:2 * pr + 2]
                l3s[extra] = nx.astype(bf16)
            if k_ == 1:
                fresh = p not in l3s
                res = w1_dot(p, ln_chain(p) if fresh else l3s.pop(p), ties, fresh)
            elif k_ == 2:
                res = w2_dot(p, ties)
            else:
                par[pl.ds(48, 8), :] = _mm(sc_lhs(), wmc[...])[0:8]
            for u_ in anch:
                if u_ // 40 + 1 == k_ and units and d_ < len(dots) - (NP4 + 1 if pre4 else 0):
                    n, g = (u_ % 40) // 8, u_ % 8
                    units.pop(0)(res[8 * g:8 * g + 8, 128 * n:128 * (n + 1)])

    pos = [N2, 0]

    def plan(lim1):
        last = lim1 == S // R
        dots = []
        while pos[0] < (lim1 if last else lim1 - 1) or pos[0] - pos[1] >= LEAD or (last and pos[1] < lim1):
            k_ = 0 if pos[0] - pos[1] < LEAD and pos[0] < lim1 else 1
            dots.append((k_ + 1, pos[k_]))
            pos[k_] += 1
        return dots, (None if last else pos[0])

    with jax.named_scope("P1"):
        wait_all([cp_wmp, cp_q[0]])
        mp = _mm(sc_lhs(), wmp[...])
        for t in range(WMP // 128):
            modb[2 * WMA // 128 + t] = mp[0:8, 128 * t:128 * (t + 1)]
        sa, ca, ga, sb, cb = [jnp.concatenate([modb[NT * k_ + j] for j in range(NT)], axis=1) for k_ in range(5)]
        par[pl.ds(16, 8), :] = ga * (1.0 + ca)
        par[pl.ds(24, 8), :] = ga * sa
        par[pl.ds(32, 8), :] = 1.0 + cb
        par[pl.ds(40, 8), :] = sb
        for bt in range(4):
            dot_k(kb1, 1, bt, _as_bf16(jnp.concatenate([kb0[KOFF + 17 + 2 * n] for n in range(8)], axis=0)))
        for p in range(PRELN):
            l3s[p] = ln_chain(p)
    with jax.named_scope("w1wait"):
        cp_w[0].wait()
    with jax.named_scope("P2"):
        run_block([(1, p) for p in range(N2)])
    with jax.named_scope("w2wait"):
        wait_all([cp_w[1], cp_q[1]])
    with jax.named_scope("P4"):
        run_block(*plan(Q1 // R))
    with jax.named_scope("q2wait"):
        wait_all([cp_q[2], cp_w[3]])
    units += [functools.partial(prep2, w4_, w4s, False, t, p_) for t in range(24) for p_ in range(7)]
    units += [functools.partial(prep1, w4, w4o, 832, _SB, (0, 1, 3, 5, 6), t, n) for t in range(8) for n in range(2)]
    with jax.named_scope("P5"):
        run_block(*plan(Q2 // R))
    with jax.named_scope("q3wait"):
        wait_all([cp_q[3], cp_wmc, cp_w[2]])
    units += [functools.partial(prep2, w3_, w3s, True, t, p_) for t in range(24) for p_ in range(7)]
    units += [functools.partial(prep1, w3, w3o, 816, _SA, (0, 2, 4, 5, 6), t, n) for t in range(6) for n in range(2)]
    with jax.named_scope("P6"):
        dots, _ = plan(S // R)
        gp = len(dots) - NP4 if GBP else 3
        run_block(dots[:gp] + [(3, 0)] + dots[gp:], pre4=True)
    assert not units

    quads = ((0, 0), (0, 256), (H2, 0), (H2, 256))
    done_at = [max(i for i, p_ in enumerate(ORD4) if any(k_ == kq for k_, _ in _SC[p_])) for kq in range(4)]
    qorder = sorted(range(4), key=lambda kq: done_at[kq])
    outs = [(0, 512, 128)] + [quads[kq] + (256,) for kq in qorder] + [(H2, 512, 128)]
    assert qorder == [0, 1, 2, 3]
    copies = {2: (0, 0, D), 4: (H2, 0, 512), 5: (H2, 512, 128)}

    def out_copy(r, r0, c0, cn):
        rows = pl.ds(_mult(r + r0, H2), H2)
        return cp(obuf.at[rows, pl.ds(c0, cn)], o_hbm.at[0, rows, pl.ds(c0, cn)], osem.at[0])

    def b2_step(i, carry):
        r = pl.multiple_of(i * TS, TS)
        gs = gs_.at[i >> 8]
        lr = l4p[:, pl.ds(512, 128)]
        w3a = lambda p_: (w3[pl.ds(816, 48), pl.ds(256, 256)] if p_ == 1 else
                          w3[pl.ds(768, 48), pl.ds(0, 256)] if p_ == 3 else w3o[p_])
        lt_ = _blocks((0, 0), (H2, 0), (0, 256), (H2, 256))
        zt = _mm_nt(_as_bf16(w3[pl.ds(768, 96), pl.ds(512, 128)]), lr.astype(bf16))
        zt = zt + _quad(_comb([_mm_nt(_as_bf16(w3a(p_)), _SB[p_](*lt_).load(l4p_.at[i >> (20 + p_)], H2, 256))
                               for p_ in range(7)]))
        gt = jnp.concatenate([_gelu2a(zt), jnp.zeros((64, TS), f32)], axis=0)
        gs[:, pl.ds(0, 128)] = gt[:128].T
        gs[:, pl.ds(896, 128)] = gt[128:].T
        lrs = [lr[:H2].astype(bf16), lr[H2:].astype(bf16)]
        ab = _blocks(*quads)
        ops = {}
        for t in range(3):
            cq, left = [None] * 4, [5, 3, 3, 5]

            def add(k_, x, sg=1):
                cq[k_] = x if cq[k_] is None else cq[k_] + x if sg > 0 else cq[k_] - x
                left[k_] -= 1
                if left[k_] == 0:
                    gg = _gelu2a(cq[k_])
                    for n2 in range(2):
                        cols = pl.ds(128 + 896 * (k_ % 2) + 128 * (t + 3 * n2), 128)
                        gs[pl.ds(H2 * (k_ // 2), H2), cols] = gg[:, 128 * n2:128 * (n2 + 1)]

            for p_ in range(8):
                for k_ in (2, 1, 0, 3):
                    if REMP[k_] == p_:
                        wr = [w3[pl.ds(64 * (t + 3 * (2 * (k_ % 2) + n2)), 64), pl.ds(512, 128)] for n2 in range(2)]
                        add(k_, _mm_nt(lrs[k_ // 2], _as_bf16(jnp.concatenate(wr, axis=0))))
                if p_ == 7:
                    break
                a_ = _SA[p_](*ab)
                sub_ = (a_, a_.shift(0, 128), a_.shift(Q4, 0), a_.shift(Q4, 128))
                pr = []
                for q_ in range(7):
                    n = 7 * p_ + q_
                    if n not in ops:
                        ops[n] = _SA[q_](*sub_).load(l4p_.at[(i + 4 * p_) >> (9 + q_)], Q4, 128)
                    w_ = (w3[pl.ds(192 * _PURE[n] + 64 * t, 64), pl.ds(128 * _PURE[n], 128)] if n in _PURE
                          else w3s[n, pl.ds(64 * t, 64), :])
                    pr.append(_mm_nt(ops[n], _as_bf16(w_)))
                m_ = _quad(_comb(pr))
                for k_, sg in _SC[p_]:
                    add(k_, m_, sg)
        kord = [(0, 768), (896, 832)] + [x for c in (0, 3, 1, 4, 2, 5)
                                         for x in ((128 + 128 * c, 64 * c), (1024 + 128 * c, 384 + 64 * c))]
        wl = jnp.concatenate([w4[pl.ds(wr_, 64), pl.ds(512, 128)] for _, wr_ in kord], axis=0)
        gk = lambda r0: jnp.concatenate([gs[pl.ds(r0, H2), pl.ds(o_, 128)] for o_, _ in kord], axis=1).astype(bf16)
        acc_t = _mm(gk(0), wl)
        rn_ = pl.multiple_of(jnp.minimum(i + 1, S // TS - 1) * TS, TS)
        rp = TS // len(LNT)
        ties = {}
        for e, k_ in enumerate(LNT):
            nx = ln4(pl.multiple_of(rn_ + e * rp, rp), rp)
            l4p[pl.ds(e * rp, rp), :] = nx
            ties[k_] = firsts(nx)
        gb_ = _blocks((0, 0), (0, 896), (H2, 0), (H2, 896))
        ms = [None] * 7
        for idx, p_ in enumerate(ORD4):
            a_ = _SA[p_](*gb_)
            wo = (w4[pl.ds(768, 64), pl.ds(0, 256)] if p_ == 2 else
                  w4[pl.ds(832, 64), pl.ds(256, 256)] if p_ == 4 else w4o[p_])
            if idx in ties:
                wo = tie_at(wo, 0, 0, ties[idx])
            m_ = _mm(a_.load(gs, H2, 128), wo)
            sub_ = (a_.shift(0, 128), a_.shift(0, 512), a_.shift(Q4, 128), a_.shift(Q4, 512))
            pr = []
            for q_ in range(7):
                n = 7 * p_ + q_
                w_ = (w4[pl.ds(192 * _PURE[n], 192), pl.ds(128 * _PURE[n], 128)] if n in _PURE
                      else w4s[n, pl.ds(0, 192), :])
                pr.append(_mm(_SA[q_](*sub_).load(gs_.at[(i + 4 * p_) >> (9 + q_)], Q4, 384), w_))
            ms[p_] = m_ + _quad(_comb(pr))
        cs = _comb(ms)
        for k_ in ties:
            if k_ >= 10:
                wl = tie_at(wl, 64 * (k_ - 10), 0, ties[k_])
        accs = [acc_t] + [cs[kq] for kq in qorder] + [_mm(gk(H2), wl)]
        gbv = par[pl.ds(48, 8), :]
        for oi, ((r0, c0, cn), ac) in enumerate(zip(outs, accs)):
            rows, cols = pl.ds(_mult(r + r0, H2), H2), pl.ds(c0, cn)
            g3 = lambda x: x.reshape(H2 // 8, 8, cn)
            out = g3(xn[rows, cols]) + gbv[None, :, c0:c0 + cn] * g3(hh[rows, cols] + BETA * ac)
            obuf[rows, cols] = out.reshape(H2, cn).astype(bf16)
            if oi in copies:
                out_copy(r, *copies[oi]).start()
        return carry

    with jax.named_scope("BII"):
        lax.fori_loop(0, S // TS, b2_step, 0)
    with jax.named_scope("out_wait"):
        for i in range(S // TS):
            for o_ in copies.values():
                out_copy(i * TS, *o_).wait()


@jax.jit
def pallas_adaLN_cond__ssm_conv_h3__mixer_s_mlp__prompt_kernel(
    A_q: jax.Array,
    A_k: jax.Array,
    A_v: jax.Array,
    A_shift_k: jax.Array,
    A_ssm_k: jax.Array,
    A_ssm_D: jax.Array,
    B_x: jax.Array,
    B_w1: jax.Array,
    B_w2: jax.Array,
    B_w3: jax.Array,
    B_w4: jax.Array,
    c: jax.Array,
    w_mod: jax.Array,
):
    del B_x
    hbm = pl.BlockSpec(memory_space=pltpu.MemorySpace.HBM)
    spec = pltpu.VMEM((NG * 2 * NC, 8, 128), f32)
    part = pltpu.VMEM((KOFF + 56, 8, 128), f32)
    return pl.pallas_call(
        _kernel,
        out_shape=jax.ShapeDtypeStruct((1, S, D), bf16),
        in_specs=[hbm] * 12,
        out_specs=hbm,
        scratch_shapes=[
            pltpu.VMEM((27, 8, 128), f32),
            pltpu.VMEM((S, D), bf16),
            pltpu.VMEM((NT, 32 + HS, 128), u32),
            pltpu.VMEM((NT, 32 + HS, 128), u32),
            pltpu.VMEM((NT, 64, S), u32),
            pltpu.VMEM((D // 2, D), u32),
            pltpu.VMEM((D // 2, D), u32),
            pltpu.VMEM((1, F // 2, D), u32),
            pltpu.VMEM((1, 896, D), u32),
            pltpu.VMEM((2, D // 2, WMA), u32),
            pltpu.VMEM((D // 2, WMP), u32),
            pltpu.VMEM((D // 2, WMC), u32),
            pltpu.VMEM((S, D), bf16),
            spec, spec, spec, spec,
            part, part,
            pltpu.VMEM((NT, S, 128), f32),
            pltpu.VMEM((S, D), f32),
            pltpu.VMEM((S, D), f32),
            pltpu.VMEM((NT, S + 32, 128), f32),
            pltpu.VMEM((64, D), f32),
            pltpu.VMEM((1, TS, D), f32),
            pltpu.VMEM((1, TS, 1792), f32),
            pltpu.VMEM((52, 200, 128), u32),
            pltpu.VMEM((52, 200, 128), u32),
            pltpu.VMEM((7, 64, 256), u32),
            pltpu.VMEM((7, 48, 256), u32),
            pltpu.VMEM((4, D), bf16),
            pltpu.VMEM((D,), bf16),
            pltpu.VMEM((1, D), bf16),
            pltpu.SMEM((2,), jnp.int32),
            pltpu.SemaphoreType.DMA((20,)),
            pltpu.SemaphoreType.DMA((1,)),
        ],
        compiler_params=pltpu.CompilerParams(vmem_limit_bytes=100 * 1024 * 1024, disable_semaphore_checks=True,
                                             disable_bounds_checks=NOBC),
    )(A_q, A_k, A_v, A_shift_k.T, A_ssm_k, A_ssm_D, B_w1, B_w2, B_w3.T, B_w4, c, w_mod)
```

```python
import functools
import math

import jax
import jax.numpy as jnp
from jax import lax
import jax.experimental.pallas as pl
import jax.experimental.pallas.tpu as pltpu

S, D, F = 2048, 640, 1728
EPS = 1e-5
NT = D // 128
HS = S // 2

C = 128
NC = S // C
NG = 16
KOFF = (NC + 1) * NG * 3
W = 4
G0 = 4
HEAD, TAIL = 250, 450
DORDER = 'aHbU'
WMA, WMP, WMC = 1280, 640, 640
R = 64
Q0, Q1, Q2 = 320, 768, 1408
N2, PRELN, LEAD, NP4, TIE4 = 5, 2, 3, 2, 12
XRB = (7, 4, 2, 0)
ANCH = (20, 58, 18)
TS = 512
H2, Q4 = TS // 2, TS // 4
LNT = (0, 1, 2, 3, 4, 5, 18, 22)
REMP = (6, 5, 3, 7)
ORD4 = (0, 5, 4, 1, 3, 2, 6)

_C0 = math.sqrt(2.0 / math.pi)
ALPHA = (_C0 * 0.044715) ** (1.0 / 3.0)
GC = _C0 / ALPHA
BETA = 0.5 / ALPHA

f32 = jnp.float32
bf16 = jnp.bfloat16
u32 = jnp.uint32
NTDIMS = (((1,), (1,)), ((), ()))

_SA = (lambda a, b, c, d: a + d, lambda a, b, c, d: d, lambda a, b, c, d: c + d, lambda a, b, c, d: a,
       lambda a, b, c, d: a + b, lambda a, b, c, d: b - d, lambda a, b, c, d: c - a)
_SB = (lambda a, b, c, d: a + d, lambda a, b, c, d: c - a, lambda a, b, c, d: a, lambda a, b, c, d: b - d,
       lambda a, b, c, d: d, lambda a, b, c, d: c + d, lambda a, b, c, d: a + b)
_SBU = ((1, 0, 0, 1), (1, 0, 1, 0), (1, 0, 0, 0), (0, 1, 0, 1), (0, 0, 0, 1), (0, 0, 1, 1), (1, 1, 0, 0))
_SC = (((0, 1), (3, 1)), ((0, 1), (2, 1)), ((2, 1), (3, -1)), ((1, 1), (3, 1)), ((0, -1), (1, 1)), ((0, 1),), ((3, 1),))
_PURE = {7 * p + q: 2 * i + j for i, p in enumerate((2, 4)) for j, q in enumerate((2, 4))}


def _comb(m):
    m1, m4, m2, m3, m5, m7, m6 = m
    return (m1 + m4) + (m7 - m5), m3 + m5, m4 + m2, (m1 + (m3 - m2)) + m6


def _quad(c):
    return jnp.concatenate([jnp.concatenate(c[0:2], axis=1), jnp.concatenate(c[2:4], axis=1)], axis=0)


class _Lazy:
    def __init__(self, terms):
        self.terms = terms

    def __add__(self, o):
        return _Lazy(self.terms + o.terms)

    def __sub__(self, o):
        return _Lazy(self.terms + [(-s, r, c) for (s, r, c) in o.terms])

    def shift(self, dr, dc):
        return _Lazy([(s, r + dr, c + dc) for (s, r, c) in self.terms])

    def load(self, ref, rn, cn):
        ts = sorted(self.terms, key=lambda t: -t[0])
        acc = None
        for (s, r, c) in ts:
            x = ref[pl.ds(r, rn), pl.ds(c, cn)]
            acc = x if acc is None else acc + x if s > 0 else acc - x
        return acc.astype(bf16)


def _blocks(*offsets):
    return [_Lazy([(1, r, c)]) for (r, c) in offsets]


def _unp(w, e):
    return pltpu.unpack_elementwise(w, index=e, packed_dtype=bf16, unpacked_dtype=f32)


def _pk(xs):
    return pltpu.pack_elementwise(xs, packed_dtype=bf16)


def _as_bf16(w):
    return pltpu.bitcast(w, bf16)


def _mm(x, w):
    return jnp.dot(x, _as_bf16(w), preferred_element_type=f32)


def _mm_nt(x, w):
    return lax.dot_general(x, w, NTDIMS, preferred_element_type=f32)


def _mult(x, n):
    return x if isinstance(x, int) else pl.multiple_of(x, n)


def _cos_table(m, scale):
    mm = jnp.abs(((m + 256) & 511) - 256)
    x = (128 - mm).astype(f32) * (1.0 / 128.0)
    x2 = x * x
    h = math.pi / 2
    p = -(h ** 7) / 5040 + x2 * ((h ** 9) / 362880 - x2 * (h ** 11) / 39916800)
    p = h + x2 * (-(h ** 3) / 6 + x2 * ((h ** 5) / 120 + x2 * p))
    return (x * scale) * p


def _dft_tables():
    shape = (16, 8, 128)
    n = lax.broadcasted_iota(jnp.int32, shape, 0)
    s = lax.broadcasted_iota(jnp.int32, shape, 1)
    l = lax.broadcasted_iota(jnp.int32, shape, 2)
    fw, fu, iv = [], [], []
    wv = l >> 4
    tu = (16 * W) * (wv // W) + (2 * W) * ((l >> 1) & 7) + 2 * (wv % W) + (l & 1)
    for e in range(2):
        r = 2 * s + e
        j = 8 * n + (r & 7)
        fw.append(_cos_table((4 * j + 1) * l + (r >> 3) * 128, 1.0))
        fu.append(_cos_table((4 * j + 1) * tu + (r >> 3) * 128, 1.0))
        b = 16 * (n >> 1) + r
        col = 128 * (n & 1) + l
        iv.append(_cos_table((4 * (col >> 1) + 1) * b + (col & 1) * 128, 1.0 / 128.0))
    return [pltpu.bitcast(_pk(x), f32) for x in (fw, iv, fu)]


def _gelu2a(z):
    return z * (1.0 + jnp.tanh(z * (z * z + GC)))


def _center(x, scale=1.0):
    s1 = jnp.sum(x, axis=-1, keepdims=True)
    m = s1 * (1.0 / D)
    ssd = jnp.maximum(jnp.sum(x * x, axis=-1, keepdims=True) - s1 * m, 0.0)
    rstd = jnp.exp2(jnp.log(ssd + D * EPS) * (-0.5 / math.log(2.0)) + math.log2(scale * math.sqrt(D)))
    return x - m, rstd


def _conv(us, gs, a):
    acc = None
    for c in range(a + 1):
        p = us[c] * gs[a - c]
        acc = p if acc is None else acc + p
    return acc


def _kernel(q_hbm, k_hbm, v_hbm, sk_hbm, h_hbm, dd_hbm, w1_hbm, w2_hbm, w3_hbm, w4_hbm, c_hbm, wm_hbm, o_hbm,
            modb, qbuf, kbuf, vbuf, hbuf, w1, w2, w3_, w4_, wm, wmp, wmc, obuf, ub0, ub1, gb0, gb1, kb0, kb1,
            yb, xn, hh, h1, par, l4p_, gs_, w4s, w3s, w4o, w3o, sk_s, dd_s, c_s, zs, sems, osem):
    l4p, w3, w4 = l4p_.at[0], w3_.at[0], w4_.at[0]
    ubs, gbs, kbs = (ub0, ub1), (gb0, gb1), (kb0, kb1)
    cp = pltpu.make_async_copy

    def cp_h(j, c0, c1, sem):
        cols = pl.ds(c0, c1 - c0)
        return cp(h_hbm.at[pl.ds(j * 128, 128), cols], hbuf.bitcast(bf16).at[j, :, cols], sem)

    def cp_kv(j, r0, r1, sem):
        r0, r1 = (r0 + 16 if r0 else 0), min(r1 + 16, S)
        lanes = pl.ds(j * 128, 128)
        return [cp(k_hbm.at[0, pl.ds(r0, r1 - r0), lanes], kbuf.bitcast(bf16).at[j, pl.ds(r0 + 16, r1 - r0), :], sem),
                cp(v_hbm.at[0, pl.ds(r0, r1 - r0), lanes], vbuf.bitcast(bf16).at[j, pl.ds(r0, r1 - r0), :], sem)]

    def cp_tile(j, i):
        sem = sems.at[2 * j + i]
        return [cp_h(j, i * HS, (i + 1) * HS, sem)] + cp_kv(j, i * HS, (i + 1) * HS, sem)

    def cp_wm(i):
        return cp(wm_hbm.at[:, pl.ds(i * WMA, WMA)], wm.bitcast(bf16).at[i], sems.at[10 + i])

    def wait_all(cps):
        for c_ in cps:
            c_.wait()

    cp_t0 = [[cp_h(0, 0, S, sems.at[0])], cp_kv(0, 0, 1024, sems.at[1]), cp_kv(0, 1024, 1536, sems.at[17]),
             cp_kv(0, 1536, S, sems.at[18])]
    cp_wmp = cp(wm_hbm.at[:, pl.ds(2 * WMA, WMP)], wmp.bitcast(bf16), sems.at[13])
    cp_wmc = cp(wm_hbm.at[:, pl.ds(2 * WMA + WMP, WMC)], wmc.bitcast(bf16), sems.at[12])
    cp_q = [cp(q_hbm.at[0, pl.ds(r0, r1 - r0), :], qbuf.at[pl.ds(r0, r1 - r0), :], sems.at[sm])
            for sm, r0, r1 in ((13, 0, Q0), (16, Q0, Q1), (14, Q1, Q2), (12, Q2, S))]
    cp_w = [cp(w1_hbm, w1.bitcast(bf16), sems.at[15]), cp(w2_hbm, w2.bitcast(bf16), sems.at[16]),
            cp(w3_hbm, w3_.bitcast(bf16).at[0], sems.at[12]),
            cp(w4_hbm, w4_.bitcast(bf16).at[0, pl.ds(0, F), :], sems.at[14])]
    cp_s = [cp(sk_hbm, sk_s, sems.at[19]), cp(dd_hbm, dd_s, sems.at[19]), cp(c_hbm, c_s, sems.at[19])]
    order = list(cp_s)
    for grp in cp_t0:
        order += grp
    for j in range(1, NT):
        order += cp_tile(j, 0) + cp_tile(j, 1)
    order += [cp_wm(0), cp_wm(1), cp_wmp, cp_q[0], cp_w[0], cp_w[1], cp_q[1], cp_q[2], cp_w[3], cp_q[3], cp_wmc, cp_w[2]]
    for c_ in order:
        c_.start()

    with jax.named_scope("init"):
        tables = _dft_tables()
        for kb in kbs:
            for i, tb in enumerate(tables):
                kb[pl.ds(KOFF + 16 * i, 16)] = tb
            kb[pl.ds(0, NG * 3)] = jnp.zeros((NG * 3, 8, 128), f32)
        w4[pl.ds(F // 2, 32), :] = jnp.zeros((32, D), u32)
        for j in range(NT):
            kbuf[j, pl.ds(0, 8), :] = jnp.zeros((8, 128), u32)
            kbuf[j, pl.ds(8 + HS, 8), :] = jnp.zeros((8, 128), u32)
            vbuf[j, pl.ds(HS, 8), :] = jnp.zeros((8, 128), u32)
            h1[j, pl.ds(8, 8), :] = jnp.zeros((8, 128), f32)
            h1[j, pl.ds(S, 8), :] = jnp.zeros((8, 128), f32)
        wait_all(cp_s)
        par[pl.ds(0, 4), :] = sk_s[...].astype(f32)
        par[pl.ds(8, 8), :] = jnp.broadcast_to(dd_s[...].astype(f32).reshape(1, D), (8, D))
        cv = c_s[...].astype(f32)
        sc = jnp.broadcast_to(cv * jax.nn.sigmoid(cv), (8, D))
        scp = pltpu.bitcast(_pk([sc, sc]), f32)
        for kb in kbs:
            for j in range(NT):
                kb[KOFF + 48 + j] = scp[:, 128 * j:128 * (j + 1)]

    def mkb(i, unr, off, cache):
        def b(stride, extra=0, z=None):
            if isinstance(i, int):
                return (i * unr + off) * stride + extra
            key = (unr * stride, z)
            if key not in cache:
                base = pl.multiple_of(i * (unr * stride), unr * stride)
                cache[key] = base if z is None else pl.multiple_of(base + (i >> z) * 4, 4)
            return cache[key] + (off * stride + extra)
        return b

    def store_spec(ref, b, x):
        for rg in range(2 * NG):
            for cc in range(4):
                ref[b(4, cc + rg * NC)] = x[8 * rg:8 * rg + 8, 128 * cc:128 * cc + 128]

    def dot_h(j, b, lhs):
        hc = hbuf[j, :, pl.ds(_mult(b(512), 512), 512)]
        rhs_t = jnp.concatenate([hc[:, C * cc:C * (cc + 1)] for cc in range(4)], axis=0)
        store_spec(gbs[j % 2], b, _mm_nt(lhs, _as_bf16(rhs_t)))

    def dot_u(j, b, lhs):
        taps = [par[pl.ds(t, 1), pl.ds(j * 128, 128)] for t in range(4)]
        cols = []
        for cc in range(4):
            words = []
            for blk in range(8 // W):
                w0 = 64 * cc + 8 * W * blk
                kw = {m: kbuf[j, pl.ds(b(256, 8 + w0 + m), 8, stride=W), :] for m in range(-2, W)}
                kk = {2 * m + e: _unp(kw[m], e) for m in range(-2, W) for e in range(2) if 2 * m + e >= -3}
                for m in range(W):
                    vw = vbuf[j, pl.ds(b(256, w0 + m), 8, stride=W), :]
                    pair = []
                    for e in range(2):
                        n = 2 * m + e
                        ks = kk[n] * taps[0] + kk[n - 1] * taps[1] + kk[n - 2] * taps[2] + kk[n - 3] * taps[3]
                        pair.append(ks * _unp(vw, e))
                    words.append(_pk(pair))
            cols.append(jnp.concatenate(words, axis=0))
        store_spec(ubs[j % 2], b, _mm(lhs, jnp.concatenate(cols, axis=1)))

    def out_spec(kidx, groups, nc):
        cols = [[] for _ in range(nc)]
        for gi in groups:
            prev = None
            for cc in range(-1, nc):
                k0, k1, k2 = [kidx(((cc + 1) * NG + gi) * 3 + t) for t in range(3)]
                re, im = k0 - k2, k0 + k1
                if prev is not None:
                    cols[cc].append(_pk([re - prev[1], im + prev[0]]))
                prev = (re, im)
        return jnp.concatenate([jnp.concatenate(c_, axis=0) for c_ in cols], axis=1)

    def dot_i(j, b, half, lhs):
        y = _mm(lhs, out_spec(lambda o: kbs[j % 2][b(4 * NG * 3, 2 * half * NG * 3 + o)], range(NG), 2))
        for cc in range(2):
            yb[j, pl.ds(b(512, (2 * half + cc) * C), C), :] = y[:, 128 * cc:128 * cc + 128]

    def dot_k(kb, kt, bt, lhs):
        y = _mm(lhs, out_spec(lambda o: kb[4 * bt * NG * 3 + o], range(8 * kt, 8 * kt + 8), 4))
        for cc in range(4):
            rows = pl.ds((4 * bt + cc) * C, C)
            yc = y[:, 128 * cc:128 * cc + 128]
            yb[NT - 1, rows, :] = yc if kt == 0 else yb[NT - 1, rows, :] + yc

    def gen_m(j, kb, b, ng):
        ub, gb = ubs[j % 2], gbs[j % 2]
        for s in range(ng):
            for t in range(3):
                re = lambda ref, c: ref[b(2 * NC, 2 * s * NC + c, 8 + t)]
                im = lambda ref, c: ref[b(2 * NC, (2 * s + 1) * NC + c, 8 + t)]
                gre = [re(gb, c) for c in range(NC)]
                if t == 0:
                    us, gs = [re(ub, c) + im(ub, c) for c in range(NC)], gre
                elif t == 1:
                    us, gs = [re(ub, c) for c in range(NC)], [im(gb, c) - gre[c] for c in range(NC)]
                else:
                    us, gs = [im(ub, c) for c in range(NC)], [im(gb, c) + gre[c] for c in range(NC)]
                ue, uo, ge, go = us[0::2], us[1::2], gs[0::2], gs[1::2]
                usum = [x + y for x, y in zip(ue, uo)]
                gsum = [x + y for x, y in zip(ge, go)]
                poo_prev = None
                for a in range(NC // 2):
                    pee, poo, pss = _conv(ue, ge, a), _conv(uo, go, a), _conv(usum, gsum, a)
                    kb[b(3, ((2 * a + 1) * NG + s) * 3 + t)] = pee if poo_prev is None else pee + poo_prev
                    kb[b(3, ((2 * a + 2) * NG + s) * 3 + t)] = pss - pee - poo
                    poo_prev = poo
                    yield 3 * (2 * a + 1) + 7

    def add_d(j):
        gb = gbs[j % 2]
        dvec = par[pl.ds(8, 8), pl.ds(j * 128, 128)]
        for gi in range(NG):
            gb[2 * gi * NC] = gb[2 * gi * NC] + dvec

    def dot_m(i, t0, nt, rows):
        m = None
        for kt in range(NT):
            p = _mm(_as_bf16(rows[kt]), wm[i, pl.ds(64 * kt, 64), pl.ds(128 * t0, 128 * nt)])
            m = p if m is None else m + p
        for t in range(nt):
            modb[i * (WMA // 128) + (t0 + t)] = m[0:8, 128 * t:128 * (t + 1)]

    pre = dict(H=0, U=672 + 96 // W, a=192, b=192, m=0, k=176)
    post = dict(H=0, U=0, a=4, b=4, m=2, k=0)
    nst = dict(H=16, U=16, a=8, b=8, m=5, k=8)

    def a_block(dots, mg=None, ng=0, tbl=kb0):
        native, dur = [], []
        for idx, (k_, _) in enumerate(dots):
            nxt = pre[dots[idx + 1][0]] if idx + 1 < len(dots) else 0
            d_ = 2.0 if k_ == 'm' else 1.0
            native += [nxt / nst[k_] + post[k_] * d_] * nst[k_]
            dur += [d_] * nst[k_]
        if mg is not None and dots:
            head = max(HEAD - pre[dots[0][0]], 0)
            mtot = 744 * ng - TAIL - head
            lvl = (mtot + sum(native)) / sum(dur)
            want = [max(lvl * d_ - x, 0.0) for x, d_ in zip(native, dur)]
            cum = [head]
            for w_ in want:
                cum.append(cum[-1] + w_ * mtot / sum(want))
        done, step = 0.0, 0
        for (k_, fn) in dots:
            rows = []
            for n in range(nst[k_]):
                while mg is not None and done < cum[step]:
                    done += next(mg)
                step += 1
                if k_ in 'ab':
                    rows.append(jnp.concatenate([tbl[KOFF + 16 + 2 * n], tbl[KOFF + 17 + 2 * n]], axis=1))
                else:
                    rows.append(tbl[KOFF + dict(H=n, U=32 + n, k=16 + 2 * n, m=48 + n)[k_]])
            fn(rows if k_ == 'm' else _as_bf16(jnp.concatenate(rows, axis=0)))
        for _ in (mg or ()):
            pass

    def fdot(k_, j, b):
        if k_ in 'HU':
            return (k_, functools.partial(dot_h if k_ == 'H' else dot_u, j, b))
        return (k_, functools.partial(dot_i, j, b, 0 if k_ == 'a' else 1))

    def a_loop(jf, jm, ji, g0, ng):
        kinds = [k_ for k_ in DORDER if k_ in 'HU' or ji is not None]

        def body(i, carry):
            cache = {}
            zs[i] = 0
            dots = [fdot(k_, jf if k_ in 'HU' else ji, mkb(i, 2, s_, cache)) for s_ in range(2) for k_ in kinds]
            a_block(dots, gen_m(jm, kbs[jm % 2], mkb(i, ng, g0, cache), ng), ng, kbs[jm % 2])

            @pl.when(i == 0)
            def _():
                wait_all(cp_tile(jf, 1))
            return carry
        wait_all(cp_tile(jf, 0))
        lax.fori_loop(0, 2, body, 0)
        add_d(jf)

    sb_ = lambda bt: mkb(0, 1, bt, None)
    with jax.named_scope("A_seg0"):
        wait_all(cp_t0[0])
        a_block([fdot('H', 0, sb_(bt)) for bt in range(4)])
        add_d(0)
        wait_all(cp_t0[1])
        a_block([fdot('U', 0, sb_(bt)) for bt in range(2)])
        for bt in (2, 3):
            wait_all(cp_t0[bt])
            a_block([fdot('U', 0, sb_(bt))])
    with jax.named_scope("A_m0"):
        def body_m0(i, carry):
            a_block([], gen_m(0, kb0, mkb(i, G0 // 2, 0, {}), G0 // 2))
            return carry
        lax.fori_loop(0, 2, body_m0, 0)
    for seg in range(1, NT):
        with jax.named_scope(f"A_seg{seg}"):
            if seg == 1:
                a_loop(1, 0, None, G0, (NG - G0) // 2)
            else:
                a_loop(seg, seg - 1, seg - 2, 0, 8)

    def with_mod(i, dots, step):
        mm = [('m', functools.partial(dot_m, i, t0, nt)) for (t0, nt) in ((0, 4), (4, 4), (8, 2))]
        return [mm[0]] + dots[:step] + [mm[1]] + dots[step:2 * step] + [mm[2]] + dots[2 * step:]

    with jax.named_scope("A_seg5a"):
        cp_wm(0).wait()
        zz = zs[1]

        @pl.when(zz == 0)
        def _():
            dots = [fdot(k_, NT - 2, sb_(bt)) for bt in range(4) for k_ in 'ab']
            a_block(with_mod(0, dots, 2), gen_m(NT - 1, kb0, mkb(zz, 8, 0, {}), 8), 8, kb0)
    with jax.named_scope("A_seg5b"):
        cp_wm(1).wait()

        @pl.when(zz == 0)
        def _():
            dots = [('k', functools.partial(dot_k, kb0, 0, bt)) for bt in range(4)]
            a_block(with_mod(1, dots, 1), gen_m(NT - 1, kb1, mkb(zz, 8, 8, {}), 8), 8, kb1)

    def zero_of(vs):
        t_ = pltpu.bitcast(vs[0], u32)
        for v_ in vs[1:]:
            t_ = t_ | pltpu.bitcast(v_, u32)
        return t_ & kbuf[0, pl.ds(0, 8), :]

    def tie_at(w_, r0, c0, vs):
        mid = [w_[r0:r0 + 8, :c0]] if c0 else []
        mid.append(w_[r0:r0 + 8, c0:c0 + 128] | zero_of(vs))
        if c0 + 128 < w_.shape[1]:
            mid.append(w_[r0:r0 + 8, c0 + 128:])
        parts = ([w_[:r0]] if r0 else []) + [jnp.concatenate(mid, axis=1)] + ([w_[r0 + 8:]] if r0 + 8 < w_.shape[0] else [])
        return jnp.concatenate(parts, axis=0)

    def tied(wref, ties):
        w_ = wref[...]
        for (t, rb), vs in ties.items():
            w_ = tie_at(w_, 64 * (t % 5) + 8 * rb, 128 * (t // 5), vs)
        return w_

    def firsts(x):
        return [x[8 * g:8 * g + 8, 0:128] for g in range(x.shape[0] // 8)]

    def ln_chain(p):
        rows = pl.ds(p * R, R)
        pa, pb, pc, ps = [par[pl.ds(16 + 8 * t, 8), :][None] for t in range(4)]
        g3 = lambda x: x.reshape(R // 8, 8, D)
        q = g3(qbuf[rows, :].astype(f32))
        d1, r1 = _center(q)
        y = g3(jnp.concatenate([yb[j, rows, :] for j in range(NT)], axis=1))
        x = q + ((d1 * r1) * pa + pb) * y
        xn[rows, :] = x.reshape(R, D)
        d2, r2 = _center(x)
        h = (d2 * r2) * pc + ps
        hh[rows, :] = h.reshape(R, D)
        d3, r3 = _center(h, ALPHA)
        return (d3 * r3).reshape(R, D)

    def w1_dot(p, l3, ties, fresh):
        if fresh:
            ties[(0, 2)] = firsts(l3)[0:2]
            l3 = pltpu.bitcast(tie_at(pltpu.bitcast(l3, u32), 0, 128, firsts(l3)[2:4]), f32)
        z = _mm(l3.astype(bf16), tied(w1, ties))
        g = _gelu2a(z)
        lane = lax.broadcasted_iota(jnp.int32, (R, 128), 1)
        for j, (o1, cut, o2) in enumerate(((1, 128, 0), (1, 32, -1), (-1, 64, 2), (2, 96, -2), (-2, 128, 0))):
            gj = g[:, j * 128:(j + 1) * 128]
            if cut == 128:
                h1[j, pl.ds(p * R + 8 + o1, R), :] = gj
            else:
                pltpu.store(h1.at[j, pl.ds(p * R + 8 + o1, R), :], gj, mask=lane < cut)
                pltpu.store(h1.at[j, pl.ds(p * R + 8 + o2, R), :], gj, mask=lane >= cut)
        return z

    def w2_dot(p, ties):
        rows = pl.ds(p * R, R)
        hs = jnp.concatenate([h1[j, pl.ds(p * R + 8, R), :] for j in range(NT)], axis=1).astype(bf16)
        x1 = hh[rows, :] + _mm(hs, tied(w2, ties)) * BETA
        hh[rows, :] = x1
        return x1

    def ln4(r, n):
        d4, r4 = _center(hh[pl.ds(r, n), :], ALPHA)
        return d4 * r4

    zoff = [zz >> p_ for p_ in range(7)]

    def prep2(src, dst, tr, t, p_, anchor):
        zero = zero_of([anchor])
        gate = 0 if _SBU[p_][0] else 3
        l1 = [[], []]
        for k2 in range(2):
            for n2 in range(2):
                bl = []
                for b_ in range(4):
                    kq, nq = 2 * (b_ // 2) + k2, 2 * (b_ % 2) + n2
                    x = None
                    if _SBU[p_][b_]:
                        x = src[zoff[p_], pl.ds(8 * t + 192 * (nq if tr else kq), 8), pl.ds(128 * (kq if tr else nq), 128)]
                        if b_ == gate and k2 == n2:
                            x = x | zero
                    bl.append(x)
                for e in range(2):
                    l1[e].append(_SB[p_](*[None if x is None else _unp(x, e) for x in bl]))
        for q_ in range(7):
            if 7 * p_ + q_ not in _PURE:
                dst[7 * p_ + q_, pl.ds(8 * t, 8), :] = _pk([_SB[q_](*l1[e]) for e in range(2)])

    def prep1(src, dst, r1, fs, ps_, t, n, anchor):
        bl = [src[pl.ds(lo + 8 * t, 8), pl.ds(c0 + 128 * n, 128)] for lo in (768, r1) for c0 in (0, 256)]
        zero = zero_of([anchor])
        bl[0], bl[3] = bl[0] | zero, bl[3] | zero
        for p_ in ps_:
            dst[p_, pl.ds(8 * t, 8), pl.ds(128 * n, 128)] = _pk([fs[p_](*[_unp(x, e) for x in bl]) for e in range(2)])

    def sc_lhs():
        return _as_bf16(jnp.concatenate([kb0[KOFF + 48 + j] for j in range(NT)], axis=1))

    units, l3s = [], {}
    anch = sorted({(ANCH[0] + (ANCH[1] - ANCH[0]) * i // ANCH[2]) % 80 for i in range(ANCH[2])})

    def run_block(dots, extra=None, pre4=False):
        for d_, (k_, p) in enumerate(dots):
            ties = {}
            e, rp = d_ - (len(dots) - NP4), TS // NP4
            if pre4 and e >= 0:
                nx = ln4(e * rp, rp)
                l4p[pl.ds(e * rp, rp), :] = nx
                ties[(TIE4, 7)] = firsts(nx)
            if extra is not None and d_ == len(dots) - 1:
                nx = ln_chain(extra)
                for pr in range(4):
                    ties[(24, XRB[pr])] = firsts(nx)[2 * pr:2 * pr + 2]
                l3s[extra] = nx.astype(bf16)
            if k_ == 1:
                fresh = p not in l3s
                res = w1_dot(p, ln_chain(p) if fresh else l3s.pop(p), ties, fresh)
            elif k_ == 2:
                res = w2_dot(p, ties)
            else:
                par[pl.ds(48, 8), :] = _mm(sc_lhs(), wmc[...])[0:8]
            for u_ in anch:
                if u_ // 40 + 1 == k_ and units and d_ < len(dots) - (NP4 + 1 if pre4 else 0):
                    n, g = (u_ % 40) // 8, u_ % 8
                    units.pop(0)(res[8 * g:8 * g + 8, 128 * n:128 * (n + 1)])

    pos = [N2, 0]

    def plan(lim1):
        last = lim1 == S // R
        dots = []
        while pos[0] < (lim1 if last else lim1 - 1) or pos[0] - pos[1] >= LEAD or (last and pos[1] < lim1):
            k_ = 0 if pos[0] - pos[1] < LEAD and pos[0] < lim1 else 1
            dots.append((k_ + 1, pos[k_]))
            pos[k_] += 1
        return dots, (None if last else pos[0])

    with jax.named_scope("P1"):
        wait_all([cp_wmp, cp_q[0]])
        mp = _mm(sc_lhs(), wmp[...])
        for t in range(WMP // 128):
            modb[2 * WMA // 128 + t] = mp[0:8, 128 * t:128 * (t + 1)]
        sa, ca, ga, sb, cb = [jnp.concatenate([modb[NT * k_ + j] for j in range(NT)], axis=1) for k_ in range(5)]
        par[pl.ds(16, 8), :] = ga * (1.0 + ca)
        par[pl.ds(24, 8), :] = ga * sa
        par[pl.ds(32, 8), :] = 1.0 + cb
        par[pl.ds(40, 8), :] = sb
        for bt in range(4):
            dot_k(kb1, 1, bt, _as_bf16(jnp.concatenate([kb0[KOFF + 17 + 2 * n] for n in range(8)], axis=0)))
        for p in range(PRELN):
            l3s[p] = ln_chain(p)
    with jax.named_scope("w1wait"):
        cp_w[0].wait()
    with jax.named_scope("P2"):
        run_block([(1, p) for p in range(N2)])
    with jax.named_scope("w2wait"):
        wait_all([cp_w[1], cp_q[1]])
    with jax.named_scope("P4"):
        run_block(*plan(Q1 // R))
    with jax.named_scope("q2wait"):
        wait_all([cp_q[2], cp_w[3]])
    units += [functools.partial(prep2, w4_, w4s, False, t, p_) for t in range(24) for p_ in range(7)]
    units += [functools.partial(prep1, w4, w4o, 832, _SB, (0, 1, 3, 5, 6), t, n) for t in range(8) for n in range(2)]
    with jax.named_scope("P5"):
        run_block(*plan(Q2 // R))
    with jax.named_scope("q3wait"):
        wait_all([cp_q[3], cp_wmc, cp_w[2]])
    units += [functools.partial(prep2, w3_, w3s, True, t, p_) for t in range(24) for p_ in range(7)]
    units += [functools.partial(prep1, w3, w3o, 816, _SA, (0, 2, 4, 5, 6), t, n) for t in range(6) for n in range(2)]
    with jax.named_scope("P6"):
        dots, _ = plan(S // R)
        run_block(dots[:-NP4] + [(3, 0)] + dots[-NP4:], pre4=True)
    assert not units

    quads = ((0, 0), (0, 256), (H2, 0), (H2, 256))
    done_at = [max(i for i, p_ in enumerate(ORD4) if any(k_ == kq for k_, _ in _SC[p_])) for kq in range(4)]
    qorder = sorted(range(4), key=lambda kq: done_at[kq])
    outs = [(0, 512, 128)] + [quads[kq] + (256,) for kq in qorder] + [(H2, 512, 128)]
    assert qorder == [0, 1, 2, 3]
    copies = {2: (0, 0, D), 4: (H2, 0, 512), 5: (H2, 512, 128)}

    def out_copy(r, r0, c0, cn):
        rows = pl.ds(_mult(r + r0, H2), H2)
        return cp(obuf.at[rows, pl.ds(c0, cn)], o_hbm.at[0, rows, pl.ds(c0, cn)], osem.at[0])

    def b2_step(i, carry):
        r = pl.multiple_of(i * TS, TS)
        gs = gs_.at[i >> 8]
        lr = l4p[:, pl.ds(512, 128)]
        w3a = lambda p_: (w3[pl.ds(816, 48), pl.ds(256, 256)] if p_ == 1 else
                          w3[pl.ds(768, 48), pl.ds(0, 256)] if p_ == 3 else w3o[p_])
        lt_ = _blocks((0, 0), (H2, 0), (0, 256), (H2, 256))
        zt = _mm_nt(_as_bf16(w3[pl.ds(768, 96), pl.ds(512, 128)]), lr.astype(bf16))
        zt = zt + _quad(_comb([_mm_nt(_as_bf16(w3a(p_)), _SB[p_](*lt_).load(l4p_.at[i >> (20 + p_)], H2, 256))
                               for p_ in range(7)]))
        gt = jnp.concatenate([_gelu2a(zt), jnp.zeros((64, TS), f32)], axis=0)
        gs[:, pl.ds(0, 128)] = gt[:128].T
        gs[:, pl.ds(896, 128)] = gt[128:].T
        lrs = [lr[:H2].astype(bf16), lr[H2:].astype(bf16)]
        ab = _blocks(*quads)
        ops = {}
        for t in range(3):
            cq, left = [None] * 4, [5, 3, 3, 5]

            def add(k_, x, sg=1):
                cq[k_] = x if cq[k_] is None else cq[k_] + x if sg > 0 else cq[k_] - x
                left[k_] -= 1
                if left[k_] == 0:
                    gg = _gelu2a(cq[k_])
                    for n2 in range(2):
                        cols = pl.ds(128 + 896 * (k_ % 2) + 128 * (t + 3 * n2), 128)
                        gs[pl.ds(H2 * (k_ // 2), H2), cols] = gg[:, 128 * n2:128 * (n2 + 1)]

            for p_ in range(8):
                for k_ in (2, 1, 0, 3):
                    if REMP[k_] == p_:
                        wr = [w3[pl.ds(64 * (t + 3 * (2 * (k_ % 2) + n2)), 64), pl.ds(512, 128)] for n2 in range(2)]
                        add(k_, _mm_nt(lrs[k_ // 2], _as_bf16(jnp.concatenate(wr, axis=0))))
                if p_ == 7:
                    break
                a_ = _SA[p_](*ab)
                sub_ = (a_, a_.shift(0, 128), a_.shift(Q4, 0), a_.shift(Q4, 128))
                pr = []
                for q_ in range(7):
                    n = 7 * p_ + q_
                    if n not in ops:
                        ops[n] = _SA[q_](*sub_).load(l4p_.at[(i + 4 * p_) >> (9 + q_)], Q4, 128)
                    w_ = (w3[pl.ds(192 * _PURE[n] + 64 * t, 64), pl.ds(128 * _PURE[n], 128)] if n in _PURE
                          else w3s[n, pl.ds(64 * t, 64), :])
                    pr.append(_mm_nt(ops[n], _as_bf16(w_)))
                m_ = _quad(_comb(pr))
                for k_, sg in _SC[p_]:
                    add(k_, m_, sg)
        kord = [(0, 768), (896, 832)] + [x for c in (0, 3, 1, 4, 2, 5)
                                         for x in ((128 + 128 * c, 64 * c), (1024 + 128 * c, 384 + 64 * c))]
        wl = jnp.concatenate([w4[pl.ds(wr_, 64), pl.ds(512, 128)] for _, wr_ in kord], axis=0)
        gk = lambda r0: jnp.concatenate([gs[pl.ds(r0, H2), pl.ds(o_, 128)] for o_, _ in kord], axis=1).astype(bf16)
        acc_t = _mm(gk(0), wl)
        rn_ = pl.multiple_of(jnp.minimum(i + 1, S // TS - 1) * TS, TS)
        rp = TS // len(LNT)
        ties = {}
        for e, k_ in enumerate(LNT):
            nx = ln4(pl.multiple_of(rn_ + e * rp, rp), rp)
            l4p[pl.ds(e * rp, rp), :] = nx
            ties[k_] = firsts(nx)
        gb_ = _blocks((0, 0), (0, 896), (H2, 0), (H2, 896))
        ms = [None] * 7
        for idx, p_ in enumerate(ORD4):
            a_ = _SA[p_](*gb_)
            wo = (w4[pl.ds(768, 64), pl.ds(0, 256)] if p_ == 2 else
                  w4[pl.ds(832, 64), pl.ds(256, 256)] if p_ == 4 else w4o[p_])
            if idx in ties:
                wo = tie_at(wo, 0, 0, ties[idx])
            m_ = _mm(a_.load(gs, H2, 128), wo)
            sub_ = (a_.shift(0, 128), a_.shift(0, 512), a_.shift(Q4, 128), a_.shift(Q4, 512))
            pr = []
            for q_ in range(7):
                n = 7 * p_ + q_
                w_ = (w4[pl.ds(192 * _PURE[n], 192), pl.ds(128 * _PURE[n], 128)] if n in _PURE
                      else w4s[n, pl.ds(0, 192), :])
                pr.append(_mm(_SA[q_](*sub_).load(gs_.at[(i + 4 * p_) >> (9 + q_)], Q4, 384), w_))
            ms[p_] = m_ + _quad(_comb(pr))
        cs = _comb(ms)
        for k_ in ties:
            if k_ >= 10:
                wl = tie_at(wl, 64 * (k_ - 10), 0, ties[k_])
        accs = [acc_t] + [cs[kq] for kq in qorder] + [_mm(gk(H2), wl)]
        gbv = par[pl.ds(48, 8), :]
        for oi, ((r0, c0, cn), ac) in enumerate(zip(outs, accs)):
            rows, cols = pl.ds(_mult(r + r0, H2), H2), pl.ds(c0, cn)
            g3 = lambda x: x.reshape(H2 // 8, 8, cn)
            out = g3(xn[rows, cols]) + gbv[None, :, c0:c0 + cn] * g3(hh[rows, cols] + BETA * ac)
            obuf[rows, cols] = out.reshape(H2, cn).astype(bf16)
            if oi in copies:
                out_copy(r, *copies[oi]).start()
        return carry

    with jax.named_scope("BII"):
        lax.fori_loop(0, S // TS, b2_step, 0)
    with jax.named_scope("out_wait"):
        for i in range(S // TS):
            for o_ in copies.values():
                out_copy(i * TS, *o_).wait()


@jax.jit
def pallas_adaLN_cond__ssm_conv_h3__mixer_s_mlp__prompt_kernel(
    A_q: jax.Array,
    A_k: jax.Array,
    A_v: jax.Array,
    A_shift_k: jax.Array,
    A_ssm_k: jax.Array,
    A_ssm_D: jax.Array,
    B_x: jax.Array,
    B_w1: jax.Array,
    B_w2: jax.Array,
    B_w3: jax.Array,
    B_w4: jax.Array,
    c: jax.Array,
    w_mod: jax.Array,
):
    del B_x
    hbm = pl.BlockSpec(memory_space=pltpu.MemorySpace.HBM)
    spec = pltpu.VMEM((NG * 2 * NC, 8, 128), f32)
    part = pltpu.VMEM((KOFF + 56, 8, 128), f32)
    return pl.pallas_call(
        _kernel,
        out_shape=jax.ShapeDtypeStruct((1, S, D), bf16),
        in_specs=[hbm] * 12,
        out_specs=hbm,
        scratch_shapes=[
            pltpu.VMEM((27, 8, 128), f32),
            pltpu.VMEM((S, D), bf16),
            pltpu.VMEM((NT, 32 + HS, 128), u32),
            pltpu.VMEM((NT, 32 + HS, 128), u32),
            pltpu.VMEM((NT, 64, S), u32),
            pltpu.VMEM((D // 2, D), u32),
            pltpu.VMEM((D // 2, D), u32),
            pltpu.VMEM((1, F // 2, D), u32),
            pltpu.VMEM((1, 896, D), u32),
            pltpu.VMEM((2, D // 2, WMA), u32),
            pltpu.VMEM((D // 2, WMP), u32),
            pltpu.VMEM((D // 2, WMC), u32),
            pltpu.VMEM((S, D), bf16),
            spec, spec, spec, spec,
            part, part,
            pltpu.VMEM((NT, S, 128), f32),
            pltpu.VMEM((S, D), f32),
            pltpu.VMEM((S, D), f32),
            pltpu.VMEM((NT, S + 32, 128), f32),
            pltpu.VMEM((64, D), f32),
            pltpu.VMEM((1, TS, D), f32),
            pltpu.VMEM((1, TS, 1792), f32),
            pltpu.VMEM((52, 200, 128), u32),
            pltpu.VMEM((52, 200, 128), u32),
            pltpu.VMEM((7, 64, 256), u32),
            pltpu.VMEM((7, 48, 256), u32),
            pltpu.VMEM((4, D), bf16),
            pltpu.VMEM((D,), bf16),
            pltpu.VMEM((1, D), bf16),
            pltpu.SMEM((2,), jnp.int32),
            pltpu.SemaphoreType.DMA((20,)),
            pltpu.SemaphoreType.DMA((1,)),
        ],
        compiler_params=pltpu.CompilerParams(vmem_limit_bytes=100 * 1024 * 1024, disable_semaphore_checks=True,
                                             disable_bounds_checks=True),
    )(A_q, A_k, A_v, A_shift_k.T, A_ssm_k, A_ssm_D, B_w1, B_w2, B_w3.T, B_w4, c, w_mod)
```

```python
import functools
import math

import jax
import jax.numpy as jnp
from jax import lax
import jax.experimental.pallas as pl
import jax.experimental.pallas.tpu as pltpu

S, D, F = 2048, 640, 1728
EPS = 1e-5
NT = D // 128
HS = S // 2

C = 128
NC = S // C
NG = 16
KOFF = (NC + 1) * NG * 3
W = 4
G0 = 4
HEAD, TAIL = 250, 450
DORDER = 'aHbU'
WMA, WMP, WMC = 1280, 640, 640
R = 64
Q0, Q1, Q2 = 320, 768, 1408
N2, PRELN, LEAD, NP4, TIE4 = 5, 2, 3, 2, 12
XRB = (7, 4, 2, 0)
ANCH = (20, 58, 18)
TS = 512
H2, Q4 = TS // 2, TS // 4
LNT = (0, 1, 2, 3, 4, 5, 18, 22)
REMP = (6, 5, 3, 7)
ORD4 = (0, 5, 4, 1, 3, 2, 6)

_C0 = math.sqrt(2.0 / math.pi)
ALPHA = (_C0 * 0.044715) ** (1.0 / 3.0)
GC = _C0 / ALPHA
BETA = 0.5 / ALPHA

f32 = jnp.float32
bf16 = jnp.bfloat16
u32 = jnp.uint32
NTDIMS = (((1,), (1,)), ((), ()))

_SA = (lambda a, b, c, d: a + d, lambda a, b, c, d: d, lambda a, b, c, d: c + d, lambda a, b, c, d: a,
       lambda a, b, c, d: a + b, lambda a, b, c, d: b - d, lambda a, b, c, d: c - a)
_SB = (lambda a, b, c, d: a + d, lambda a, b, c, d: c - a, lambda a, b, c, d: a, lambda a, b, c, d: b - d,
       lambda a, b, c, d: d, lambda a, b, c, d: c + d, lambda a, b, c, d: a + b)
_SBU = ((1, 0, 0, 1), (1, 0, 1, 0), (1, 0, 0, 0), (0, 1, 0, 1), (0, 0, 0, 1), (0, 0, 1, 1), (1, 1, 0, 0))
_SC = (((0, 1), (3, 1)), ((0, 1), (2, 1)), ((2, 1), (3, -1)), ((1, 1), (3, 1)), ((0, -1), (1, 1)), ((0, 1),), ((3, 1),))
_PURE = {7 * p + q: 2 * i + j for i, p in enumerate((2, 4)) for j, q in enumerate((2, 4))}


def _comb(m):
    m1, m4, m2, m3, m5, m7, m6 = m
    return (m1 + m4) + (m7 - m5), m3 + m5, m4 + m2, (m1 + (m3 - m2)) + m6


def _quad(c):
    return jnp.concatenate([jnp.concatenate(c[0:2], axis=1), jnp.concatenate(c[2:4], axis=1)], axis=0)


class _Lazy:
    def __init__(self, terms):
        self.terms = terms

    def __add__(self, o):
        return _Lazy(self.terms + o.terms)

    def __sub__(self, o):
        return _Lazy(self.terms + [(-s, r, c) for (s, r, c) in o.terms])

    def shift(self, dr, dc):
        return _Lazy([(s, r + dr, c + dc) for (s, r, c) in self.terms])

    def load(self, ref, rn, cn):
        ts = sorted(self.terms, key=lambda t: -t[0])
        acc = None
        for (s, r, c) in ts:
            x = ref[pl.ds(r, rn), pl.ds(c, cn)]
            acc = x if acc is None else acc + x if s > 0 else acc - x
        return acc.astype(bf16)


def _blocks(*offsets):
    return [_Lazy([(1, r, c)]) for (r, c) in offsets]


def _unp(w, e):
    return pltpu.bitcast(w & jnp.uint32(0xFFFF0000) if e else w << 16, f32)


def _as_bf16(w):
    return pltpu.bitcast(w, bf16)


def _mm(x, w):
    return jnp.dot(x, w if w.dtype == bf16 else _as_bf16(w), preferred_element_type=f32)


def _mm_nt(x, w):
    return lax.dot_general(x, w, NTDIMS, preferred_element_type=f32)


def _mult(x, n):
    return x if isinstance(x, int) else pl.multiple_of(x, n)


def _cos_table(m, scale):
    mm = jnp.abs(((m + 256) & 511) - 256)
    x = (128 - mm).astype(f32) * (1.0 / 128.0)
    x2 = x * x
    h = math.pi / 2
    p = -(h ** 7) / 5040 + x2 * ((h ** 9) / 362880 - x2 * (h ** 11) / 39916800)
    p = h + x2 * (-(h ** 3) / 6 + x2 * ((h ** 5) / 120 + x2 * p))
    return (x * scale) * p


def _dft_tables():
    r = lax.broadcasted_iota(jnp.int32, (256, 128), 0)
    l = lax.broadcasted_iota(jnp.int32, (256, 128), 1)
    phase = lambda f, t: (4 * (8 * (f >> 4) + (f & 7)) + 1) * t + ((f >> 3) & 1) * 128
    wv = l >> 4
    tu = (16 * W) * (wv // W) + (2 * W) * (l & 7) + 2 * (wv % W) + ((l >> 3) & 1)
    tb = 16 * (r >> 5) + (r & 15)
    tabs = (_cos_table(phase(r, l), 1.0), _cos_table(phase(128 * ((r >> 4) & 1) + l, tb), 1.0 / 128.0),
            _cos_table(phase(r, tu), 1.0))
    return [pltpu.bitcast(x.astype(bf16), f32).reshape(16, 8, 128) for x in tabs]


def _gelu2a(z):
    return z * (1.0 + jnp.tanh(z * (z * z + GC)))


def _center(x, scale=1.0):
    s1 = jnp.sum(x, axis=-1, keepdims=True)
    m = s1 * (1.0 / D)
    ssd = jnp.maximum(jnp.sum(x * x, axis=-1, keepdims=True) - s1 * m, 0.0)
    rstd = jnp.exp2(jnp.log(ssd + D * EPS) * (-0.5 / math.log(2.0)) + math.log2(scale * math.sqrt(D)))
    return x - m, rstd


def _conv(us, gs, a):
    acc = None
    for c in range(a + 1):
        p = us[c] * gs[a - c]
        acc = p if acc is None else acc + p
    return acc


def _kernel(q_hbm, k_hbm, v_hbm, sk_hbm, h_hbm, dd_hbm, w1_hbm, w2_hbm, w3_hbm, w4_hbm, c_hbm, wm_hbm, o_hbm,
            modb, qbuf, kbuf, vbuf, hbuf, w1, w2, w3_, w4_, wm, wmp, wmc, obuf, ub0, ub1, gb0, gb1, kb0, kb1,
            yb, xn, hh, h1, par, l4p_, gs_, w4s, w3s, w4o, w3o, sk_s, dd_s, c_s, zs, sems, osem):
    l4p, w3, w4 = l4p_.at[0], w3_.at[0], w4_.at[0]
    ubs, gbs, kbs = (ub0, ub1), (gb0, gb1), (kb0, kb1)
    cp = pltpu.make_async_copy

    def cp_h(j, c0, c1, sem):
        cols = pl.ds(c0, c1 - c0)
        return cp(h_hbm.at[pl.ds(j * 128, 128), cols], hbuf.bitcast(bf16).at[j, :, cols], sem)

    def cp_kv(j, r0, r1, sem):
        r0, r1 = (r0 + 16 if r0 else 0), min(r1 + 16, S)
        lanes = pl.ds(j * 128, 128)
        return [cp(k_hbm.at[0, pl.ds(r0, r1 - r0), lanes], kbuf.bitcast(bf16).at[j, pl.ds(r0 + 16, r1 - r0), :], sem),
                cp(v_hbm.at[0, pl.ds(r0, r1 - r0), lanes], vbuf.bitcast(bf16).at[j, pl.ds(r0, r1 - r0), :], sem)]

    def cp_tile(j, i):
        sem = sems.at[2 * j + i]
        return [cp_h(j, i * HS, (i + 1) * HS, sem)] + cp_kv(j, i * HS, (i + 1) * HS, sem)

    def cp_wm(i):
        return cp(wm_hbm.at[:, pl.ds(i * WMA, WMA)], wm.bitcast(bf16).at[i], sems.at[10 + i])

    def wait_all(cps):
        for c_ in cps:
            c_.wait()

    cp_t0 = [[cp_h(0, 0, S, sems.at[0])], cp_kv(0, 0, 1024, sems.at[1]), cp_kv(0, 1024, 1536, sems.at[17]),
             cp_kv(0, 1536, S, sems.at[18])]
    cp_wmp = cp(wm_hbm.at[:, pl.ds(2 * WMA, WMP)], wmp.bitcast(bf16), sems.at[13])
    cp_wmc = cp(wm_hbm.at[:, pl.ds(2 * WMA + WMP, WMC)], wmc.bitcast(bf16), sems.at[12])
    cp_q = [cp(q_hbm.at[0, pl.ds(r0, r1 - r0), :], qbuf.at[pl.ds(r0, r1 - r0), :], sems.at[sm])
            for sm, r0, r1 in ((13, 0, Q0), (16, Q0, Q1), (14, Q1, Q2), (12, Q2, S))]
    cp_w = [cp(w1_hbm, w1.bitcast(bf16), sems.at[15]), cp(w2_hbm, w2.bitcast(bf16), sems.at[16]),
            cp(w3_hbm, w3_.bitcast(bf16).at[0], sems.at[12]),
            cp(w4_hbm, w4_.bitcast(bf16).at[0, pl.ds(0, F), :], sems.at[14])]
    cp_s = [cp(sk_hbm, sk_s, sems.at[19]), cp(dd_hbm, dd_s, sems.at[19]), cp(c_hbm, c_s, sems.at[19])]
    order = list(cp_s)
    for grp in cp_t0:
        order += grp
    for j in range(1, NT):
        order += cp_tile(j, 0) + cp_tile(j, 1)
    order += [cp_wm(0), cp_wm(1), cp_wmp, cp_q[0], cp_w[0], cp_w[1], cp_q[1], cp_q[2], cp_w[3], cp_q[3], cp_wmc, cp_w[2]]
    for c_ in order:
        c_.start()

    with jax.named_scope("init"):
        tables = _dft_tables()
        for kb in kbs:
            for i, tb in enumerate(tables):
                kb[pl.ds(KOFF + 16 * i, 16)] = tb
            kb[pl.ds(0, NG * 3)] = jnp.zeros((NG * 3, 8, 128), f32)
        w4[pl.ds(F // 2, 32), :] = jnp.zeros((32, D), u32)
        for j in range(NT):
            kbuf[j, pl.ds(0, 8), :] = jnp.zeros((8, 128), u32)
            kbuf[j, pl.ds(8 + HS, 8), :] = jnp.zeros((8, 128), u32)
            vbuf[j, pl.ds(HS, 8), :] = jnp.zeros((8, 128), u32)
            h1[j, pl.ds(8, 8), :] = jnp.zeros((8, 128), f32)
            h1[j, pl.ds(S, 8), :] = jnp.zeros((8, 128), f32)
        wait_all(cp_s)
        par[pl.ds(0, 4), :] = sk_s[...].astype(f32)
        par[pl.ds(8, 8), :] = jnp.broadcast_to(dd_s[...].astype(f32).reshape(1, D), (8, D))
        cv = c_s[...].astype(f32)
        scp = pltpu.bitcast(jnp.broadcast_to(cv * jax.nn.sigmoid(cv), (16, D)).astype(bf16), f32)
        for kb in kbs:
            for j in range(NT):
                kb[KOFF + 48 + j] = scp[:, 128 * j:128 * (j + 1)]

    def mkb(i, unr, off, cache):
        def b(stride, extra=0, z=None):
            if isinstance(i, int):
                return (i * unr + off) * stride + extra
            key = (unr * stride, z)
            if key not in cache:
                base = pl.multiple_of(i * (unr * stride), unr * stride)
                cache[key] = base if z is None else pl.multiple_of(base + (i >> z) * 4, 4)
            return cache[key] + (off * stride + extra)
        return b

    def store_spec(ref, b, x):
        for rg in range(2 * NG):
            for cc in range(4):
                ref[b(4, cc + rg * NC)] = x[8 * rg:8 * rg + 8, 128 * cc:128 * cc + 128]

    def dot_h(j, b, lhs):
        hc = hbuf[j, :, pl.ds(_mult(b(512), 512), 512)]
        rhs_t = jnp.concatenate([hc[:, C * cc:C * (cc + 1)] for cc in range(4)], axis=0)
        store_spec(gbs[j % 2], b, _mm_nt(lhs, _as_bf16(rhs_t)))

    def dot_u(j, b, lhs):
        taps = [par[pl.ds(t, 1), pl.ds(j * 128, 128)] for t in range(4)]
        cols = []
        for cc in range(4):
            words = []
            for blk in range(8 // W):
                w0 = 64 * cc + 8 * W * blk
                kw = {m: kbuf[j, pl.ds(b(256, 8 + w0 + m), 8, stride=W), :] for m in range(-2, W)}
                kk = {2 * m + e: _unp(kw[m], e) for m in range(-2, W) for e in range(2) if 2 * m + e >= -3}
                for m in range(W):
                    vw = vbuf[j, pl.ds(b(256, w0 + m), 8, stride=W), :]
                    for e in range(2):
                        n = 2 * m + e
                        ks = kk[n] * taps[0] + kk[n - 1] * taps[1] + kk[n - 2] * taps[2] + kk[n - 3] * taps[3]
                        words.append(ks * _unp(vw, e))
            cols.append(jnp.concatenate(words, axis=0))
        store_spec(ubs[j % 2], b, _mm(lhs, jnp.concatenate(cols, axis=1).astype(bf16)))

    def out_spec(kidx, groups, nc):
        cols = [[] for _ in range(nc)]
        for gi in groups:
            prev = None
            for cc in range(-1, nc):
                k0, k1, k2 = [kidx(((cc + 1) * NG + gi) * 3 + t) for t in range(3)]
                re, im = k0 - k2, k0 + k1
                if prev is not None:
                    cols[cc] += [re - prev[1], im + prev[0]]
                prev = (re, im)
        return jnp.concatenate([jnp.concatenate(c_, axis=0) for c_ in cols], axis=1).astype(bf16)

    def dot_i(j, b, half, lhs):
        y = _mm(lhs, out_spec(lambda o: kbs[j % 2][b(4 * NG * 3, 2 * half * NG * 3 + o)], range(NG), 2))
        for cc in range(2):
            yb[j, pl.ds(b(512, (2 * half + cc) * C), C), :] = y[:, 128 * cc:128 * cc + 128]

    def dot_k(kb, kt, bt, lhs):
        y = _mm(lhs, out_spec(lambda o: kb[4 * bt * NG * 3 + o], range(8 * kt, 8 * kt + 8), 4))
        for cc in range(4):
            rows = pl.ds((4 * bt + cc) * C, C)
            yc = y[:, 128 * cc:128 * cc + 128]
            yb[NT - 1, rows, :] = yc if kt == 0 else yb[NT - 1, rows, :] + yc

    def gen_m(j, kb, b, ng):
        ub, gb = ubs[j % 2], gbs[j % 2]
        for s in range(ng):
            for t in range(3):
                re = lambda ref, c: ref[b(2 * NC, 2 * s * NC + c, 8 + t)]
                im = lambda ref, c: ref[b(2 * NC, (2 * s + 1) * NC + c, 8 + t)]
                gre = [re(gb, c) for c in range(NC)]
                if t == 0:
                    us, gs = [re(ub, c) + im(ub, c) for c in range(NC)], gre
                elif t == 1:
                    us, gs = [re(ub, c) for c in range(NC)], [im(gb, c) - gre[c] for c in range(NC)]
                else:
                    us, gs = [im(ub, c) for c in range(NC)], [im(gb, c) + gre[c] for c in range(NC)]
                ue, uo, ge, go = us[0::2], us[1::2], gs[0::2], gs[1::2]
                usum = [x + y for x, y in zip(ue, uo)]
                gsum = [x + y for x, y in zip(ge, go)]
                poo_prev = None
                for a in range(NC // 2):
                    pee, poo, pss = _conv(ue, ge, a), _conv(uo, go, a), _conv(usum, gsum, a)
                    kb[b(3, ((2 * a + 1) * NG + s) * 3 + t)] = pee if poo_prev is None else pee + poo_prev
                    kb[b(3, ((2 * a + 2) * NG + s) * 3 + t)] = pss - pee - poo
                    poo_prev = poo
                    yield 3 * (2 * a + 1) + 7

    def add_d(j):
        gb = gbs[j % 2]
        dvec = par[pl.ds(8, 8), pl.ds(j * 128, 128)]
        for gi in range(NG):
            gb[2 * gi * NC] = gb[2 * gi * NC] + dvec

    def dot_m(i, t0, nt, rows):
        m = None
        for kt in range(NT):
            p = _mm(_as_bf16(rows[kt]), wm[i, pl.ds(64 * kt, 64), pl.ds(128 * t0, 128 * nt)])
            m = p if m is None else m + p
        for t in range(nt):
            modb[i * (WMA // 128) + (t0 + t)] = m[0:8, 128 * t:128 * (t + 1)]

    pre = dict(H=0, U=672 + 96 // W, a=192, b=192, m=0, k=176)
    post = dict(H=0, U=0, a=4, b=4, m=2, k=0)
    nst = dict(H=16, U=16, a=8, b=8, m=5, k=8)

    def a_block(dots, mg=None, ng=0, tbl=kb0):
        native, dur = [], []
        for idx, (k_, _) in enumerate(dots):
            nxt = pre[dots[idx + 1][0]] if idx + 1 < len(dots) else 0
            d_ = 2.0 if k_ == 'm' else 1.0
            native += [nxt / nst[k_] + post[k_] * d_] * nst[k_]
            dur += [d_] * nst[k_]
        if mg is not None and dots:
            head = max(HEAD - pre[dots[0][0]], 0)
            mtot = 744 * ng - TAIL - head
            lvl = (mtot + sum(native)) / sum(dur)
            want = [max(lvl * d_ - x, 0.0) for x, d_ in zip(native, dur)]
            cum = [head]
            for w_ in want:
                cum.append(cum[-1] + w_ * mtot / sum(want))
        done, step = 0.0, 0
        for (k_, fn) in dots:
            rows = []
            for n in range(nst[k_]):
                while mg is not None and done < cum[step]:
                    done += next(mg)
                step += 1
                if k_ in 'ab':
                    rows.append(jnp.concatenate([tbl[KOFF + 16 + 2 * n], tbl[KOFF + 17 + 2 * n]], axis=1))
                else:
                    rows.append(tbl[KOFF + dict(H=n, U=32 + n, k=16 + 2 * n, m=48 + n)[k_]])
            fn(rows if k_ == 'm' else _as_bf16(jnp.concatenate(rows, axis=0)))
        for _ in (mg or ()):
            pass

    def fdot(k_, j, b):
        if k_ in 'HU':
            return (k_, functools.partial(dot_h if k_ == 'H' else dot_u, j, b))
        return (k_, functools.partial(dot_i, j, b, 0 if k_ == 'a' else 1))

    def a_loop(jf, jm, ji, g0, ng):
        kinds = [k_ for k_ in DORDER if k_ in 'HU' or ji is not None]

        def body(i, carry):
            cache = {}
            zs[i] = 0
            dots = [fdot(k_, jf if k_ in 'HU' else ji, mkb(i, 2, s_, cache)) for s_ in range(2) for k_ in kinds]
            a_block(dots, gen_m(jm, kbs[jm % 2], mkb(i, ng, g0, cache), ng), ng, kbs[jm % 2])

            @pl.when(i == 0)
            def _():
                wait_all(cp_tile(jf, 1))
            return carry
        wait_all(cp_tile(jf, 0))
        lax.fori_loop(0, 2, body, 0)
        add_d(jf)

    sb_ = lambda bt: mkb(0, 1, bt, None)
    with jax.named_scope("A_seg0"):
        wait_all(cp_t0[0])
        a_block([fdot('H', 0, sb_(bt)) for bt in range(4)])
        add_d(0)
        wait_all(cp_t0[1])
        a_block([fdot('U', 0, sb_(bt)) for bt in range(2)])
        for bt in (2, 3):
            wait_all(cp_t0[bt])
            a_block([fdot('U', 0, sb_(bt))])
    with jax.named_scope("A_m0"):
        def body_m0(i, carry):
            a_block([], gen_m(0, kb0, mkb(i, G0 // 2, 0, {}), G0 // 2))
            return carry
        lax.fori_loop(0, 2, body_m0, 0)
    for seg in range(1, NT):
        with jax.named_scope(f"A_seg{seg}"):
            if seg == 1:
                a_loop(1, 0, None, G0, (NG - G0) // 2)
            else:
                a_loop(seg, seg - 1, seg - 2, 0, 8)

    def with_mod(i, dots, step):
        mm = [('m', functools.partial(dot_m, i, t0, nt)) for (t0, nt) in ((0, 4), (4, 4), (8, 2))]
        return [mm[0]] + dots[:step] + [mm[1]] + dots[step:2 * step] + [mm[2]] + dots[2 * step:]

    with jax.named_scope("A_seg5a"):
        cp_wm(0).wait()
        zz = zs[1]

        @pl.when(zz == 0)
        def _():
            dots = [fdot(k_, NT - 2, sb_(bt)) for bt in range(4) for k_ in 'ab']
            a_block(with_mod(0, dots, 2), gen_m(NT - 1, kb0, mkb(zz, 8, 0, {}), 8), 8, kb0)
    with jax.named_scope("A_seg5b"):
        cp_wm(1).wait()

        @pl.when(zz == 0)
        def _():
            dots = [('k', functools.partial(dot_k, kb0, 0, bt)) for bt in range(4)]
            a_block(with_mod(1, dots, 1), gen_m(NT - 1, kb1, mkb(zz, 8, 8, {}), 8), 8, kb1)

    def zero_of(vs):
        t_ = pltpu.bitcast(vs[0], u32)
        for v_ in vs[1:]:
            t_ = t_ | pltpu.bitcast(v_, u32)
        return t_ & kbuf[0, pl.ds(0, 8), :]

    def tie_at(w_, r0, c0, vs):
        mid = [w_[r0:r0 + 8, :c0]] if c0 else []
        mid.append(w_[r0:r0 + 8, c0:c0 + 128] | zero_of(vs))
        if c0 + 128 < w_.shape[1]:
            mid.append(w_[r0:r0 + 8, c0 + 128:])
        parts = ([w_[:r0]] if r0 else []) + [jnp.concatenate(mid, axis=1)] + ([w_[r0 + 8:]] if r0 + 8 < w_.shape[0] else [])
        return jnp.concatenate(parts, axis=0)

    def tied(wref, ties):
        w_ = wref[...]
        for (t, rb), vs in ties.items():
            w_ = tie_at(w_, 64 * (t % 5) + 8 * rb, 128 * (t // 5), vs)
        return w_

    def firsts(x):
        return [x[8 * g:8 * g + 8, 0:128] for g in range(x.shape[0] // 8)]

    def ln_chain(p):
        rows = pl.ds(p * R, R)
        pa, pb, pc, ps = [par[pl.ds(16 + 8 * t, 8), :][None] for t in range(4)]
        g3 = lambda x: x.reshape(R // 8, 8, D)
        q = g3(qbuf[rows, :].astype(f32))
        d1, r1 = _center(q)
        y = g3(jnp.concatenate([yb[j, rows, :] for j in range(NT)], axis=1))
        x = q + ((d1 * r1) * pa + pb) * y
        xn[rows, :] = x.reshape(R, D)
        d2, r2 = _center(x)
        h = (d2 * r2) * pc + ps
        hh[rows, :] = h.reshape(R, D)
        d3, r3 = _center(h, ALPHA)
        return (d3 * r3).reshape(R, D)

    def w1_dot(p, l3, ties, fresh):
        if fresh:
            ties[(0, 2)] = firsts(l3)[0:2]
            l3 = pltpu.bitcast(tie_at(pltpu.bitcast(l3, u32), 0, 128, firsts(l3)[2:4]), f32)
        z = _mm(l3.astype(bf16), tied(w1, ties))
        g = _gelu2a(z)
        lane = lax.broadcasted_iota(jnp.int32, (R, 128), 1)
        for j, (o1, cut, o2) in enumerate(((1, 128, 0), (1, 32, -1), (-1, 64, 2), (2, 96, -2), (-2, 128, 0))):
            gj = g[:, j * 128:(j + 1) * 128]
            if cut == 128:
                h1[j, pl.ds(p * R + 8 + o1, R), :] = gj
            else:
                pltpu.store(h1.at[j, pl.ds(p * R + 8 + o1, R), :], gj, mask=lane < cut)
                pltpu.store(h1.at[j, pl.ds(p * R + 8 + o2, R), :], gj, mask=lane >= cut)
        return z

    def w2_dot(p, ties):
        rows = pl.ds(p * R, R)
        hs = jnp.concatenate([h1[j, pl.ds(p * R + 8, R), :] for j in range(NT)], axis=1).astype(bf16)
        x1 = hh[rows, :] + _mm(hs, tied(w2, ties)) * BETA
        hh[rows, :] = x1
        return x1

    def ln4(r, n):
        d4, r4 = _center(hh[pl.ds(r, n), :], ALPHA)
        return d4 * r4

    zoff = [zz >> p_ for p_ in range(7)]

    def prep2(src, dst, tr, t, p_, anchor):
        zero = zero_of([anchor])
        gate = 0 if _SBU[p_][0] else 3
        l1 = []
        for k2 in range(2):
            for n2 in range(2):
                bl = []
                for b_ in range(4):
                    kq, nq = 2 * (b_ // 2) + k2, 2 * (b_ % 2) + n2
                    x = None
                    if _SBU[p_][b_]:
                        x = src[zoff[p_], pl.ds(8 * t + 192 * (nq if tr else kq), 8), pl.ds(128 * (kq if tr else nq), 128)]
                        if b_ == gate and k2 == n2:
                            x = x | zero
                        x = _as_bf16(x).astype(f32)
                    bl.append(x)
                l1.append(_SB[p_](*bl))
        for q_ in range(7):
            if 7 * p_ + q_ not in _PURE:
                dst[7 * p_ + q_, pl.ds(16 * t, 16), :] = _SB[q_](*l1).astype(bf16)

    def prep1(src, dst, r1, fs, ps_, t, n, anchor):
        bl = [src[pl.ds(lo + 8 * t, 8), pl.ds(c0 + 128 * n, 128)] for lo in (768, r1) for c0 in (0, 256)]
        zero = zero_of([anchor])
        bl[0], bl[3] = bl[0] | zero, bl[3] | zero
        bl = [_as_bf16(x).astype(f32) for x in bl]
        for p_ in ps_:
            dst[2 * p_ + n, pl.ds(16 * t, 16), :] = fs[p_](*bl).astype(bf16)

    def sc_lhs():
        return _as_bf16(jnp.concatenate([kb0[KOFF + 48 + j] for j in range(NT)], axis=1))

    units, l3s = [], {}
    anch = sorted({(ANCH[0] + (ANCH[1] - ANCH[0]) * i // ANCH[2]) % 80 for i in range(ANCH[2])})

    def run_block(dots, extra=None, pre4=False):
        for d_, (k_, p) in enumerate(dots):
            ties = {}
            e, rp = d_ - (len(dots) - NP4), TS // NP4
            if pre4 and e >= 0:
                nx = ln4(e * rp, rp)
                l4p[pl.ds(e * rp, rp), :] = nx
                ties[(TIE4, 7)] = firsts(nx)
            if extra is not None and d_ == len(dots) - 1:
                nx = ln_chain(extra)
                for pr in range(4):
                    ties[(24, XRB[pr])] = firsts(nx)[2 * pr:2 * pr + 2]
                l3s[extra] = nx.astype(bf16)
            if k_ == 1:
                fresh = p not in l3s
                res = w1_dot(p, ln_chain(p) if fresh else l3s.pop(p), ties, fresh)
            elif k_ == 2:
                res = w2_dot(p, ties)
            else:
                par[pl.ds(48, 8), :] = _mm(sc_lhs(), wmc[...])[0:8]
            for u_ in anch:
                if u_ // 40 + 1 == k_ and units and d_ < len(dots) - (NP4 + 1 if pre4 else 0):
                    n, g = (u_ % 40) // 8, u_ % 8
                    units.pop(0)(res[8 * g:8 * g + 8, 128 * n:128 * (n + 1)])

    pos = [N2, 0]

    def plan(lim1):
        last = lim1 == S // R
        dots = []
        while pos[0] < (lim1 if last else lim1 - 1) or pos[0] - pos[1] >= LEAD or (last and pos[1] < lim1):
            k_ = 0 if pos[0] - pos[1] < LEAD and pos[0] < lim1 else 1
            dots.append((k_ + 1, pos[k_]))
            pos[k_] += 1
        return dots, (None if last else pos[0])

    with jax.named_scope("P1"):
        wait_all([cp_wmp, cp_q[0]])
        mp = _mm(sc_lhs(), wmp[...])
        for t in range(WMP // 128):
            modb[2 * WMA // 128 + t] = mp[0:8, 128 * t:128 * (t + 1)]
        sa, ca, ga, sb, cb = [jnp.concatenate([modb[NT * k_ + j] for j in range(NT)], axis=1) for k_ in range(5)]
        par[pl.ds(16, 8), :] = ga * (1.0 + ca)
        par[pl.ds(24, 8), :] = ga * sa
        par[pl.ds(32, 8), :] = 1.0 + cb
        par[pl.ds(40, 8), :] = sb
        for bt in range(4):
            dot_k(kb1, 1, bt, _as_bf16(jnp.concatenate([kb0[KOFF + 17 + 2 * n] for n in range(8)], axis=0)))
        for p in range(PRELN):
            l3s[p] = ln_chain(p)
    with jax.named_scope("w1wait"):
        cp_w[0].wait()
    with jax.named_scope("P2"):
        run_block([(1, p) for p in range(N2)])
    with jax.named_scope("w2wait"):
        wait_all([cp_w[1], cp_q[1]])
    with jax.named_scope("P4"):
        run_block(*plan(Q1 // R))
    with jax.named_scope("q2wait"):
        wait_all([cp_q[2], cp_w[3]])
    units += [functools.partial(prep2, w4_, w4s, False, t, p_) for t in range(24) for p_ in range(7)]
    units += [functools.partial(prep1, w4, w4o, 832, _SB, (0, 1, 3, 5, 6), t, n) for t in range(8) for n in range(2)]
    with jax.named_scope("P5"):
        run_block(*plan(Q2 // R))
    with jax.named_scope("q3wait"):
        wait_all([cp_q[3], cp_wmc, cp_w[2]])
    units += [functools.partial(prep2, w3_, w3s, True, t, p_) for t in range(24) for p_ in range(7)]
    units += [functools.partial(prep1, w3, w3o, 816, _SA, (0, 2, 4, 5, 6), t, n) for t in range(6) for n in range(2)]
    with jax.named_scope("P6"):
        dots, _ = plan(S // R)
        run_block(dots[:-NP4] + [(3, 0)] + dots[-NP4:], pre4=True)
    assert not units

    quads = ((0, 0), (0, 256), (H2, 0), (H2, 256))
    done_at = [max(i for i, p_ in enumerate(ORD4) if any(k_ == kq for k_, _ in _SC[p_])) for kq in range(4)]
    qorder = sorted(range(4), key=lambda kq: done_at[kq])
    outs = [(0, 512, 128)] + [quads[kq] + (256,) for kq in qorder] + [(H2, 512, 128)]
    assert qorder == [0, 1, 2, 3]
    copies = {2: (0, 0, D), 4: (H2, 0, 512), 5: (H2, 512, 128)}

    def out_copy(r, r0, c0, cn):
        rows = pl.ds(_mult(r + r0, H2), H2)
        return cp(obuf.at[rows, pl.ds(c0, cn)], o_hbm.at[0, rows, pl.ds(c0, cn)], osem.at[0])

    def b2_step(i, carry):
        r = pl.multiple_of(i * TS, TS)
        gs = gs_.at[i >> 8]
        lr = l4p[:, pl.ds(512, 128)]
        w3u, w4u = w3s.bitcast(u32), w4s.bitcast(u32)
        two = lambda ref, p_: jnp.concatenate([ref.bitcast(u32)[2 * p_], ref.bitcast(u32)[2 * p_ + 1]], axis=1)
        w3a = lambda p_: (w3[pl.ds(816, 48), pl.ds(256, 256)] if p_ == 1 else
                          w3[pl.ds(768, 48), pl.ds(0, 256)] if p_ == 3 else two(w3o, p_))
        lt_ = _blocks((0, 0), (H2, 0), (0, 256), (H2, 256))
        zt = _mm_nt(_as_bf16(w3[pl.ds(768, 96), pl.ds(512, 128)]), lr.astype(bf16))
        zt = zt + _quad(_comb([_mm_nt(_as_bf16(w3a(p_)), _SB[p_](*lt_).load(l4p_.at[i >> (20 + p_)], H2, 256))
                               for p_ in range(7)]))
        gt = jnp.concatenate([_gelu2a(zt), jnp.zeros((64, TS), f32)], axis=0)
        gs[:, pl.ds(0, 128)] = gt[:128].T
        gs[:, pl.ds(896, 128)] = gt[128:].T
        lrs = [lr[:H2].astype(bf16), lr[H2:].astype(bf16)]
        ab = _blocks(*quads)
        ops = {}
        for t in range(3):
            cq, left = [None] * 4, [5, 3, 3, 5]

            def add(k_, x, sg=1):
                cq[k_] = x if cq[k_] is None else cq[k_] + x if sg > 0 else cq[k_] - x
                left[k_] -= 1
                if left[k_] == 0:
                    gg = _gelu2a(cq[k_])
                    for n2 in range(2):
                        cols = pl.ds(128 + 896 * (k_ % 2) + 128 * (t + 3 * n2), 128)
                        gs[pl.ds(H2 * (k_ // 2), H2), cols] = gg[:, 128 * n2:128 * (n2 + 1)]

            for p_ in range(8):
                for k_ in (2, 1, 0, 3):
                    if REMP[k_] == p_:
                        wr = [w3[pl.ds(64 * (t + 3 * (2 * (k_ % 2) + n2)), 64), pl.ds(512, 128)] for n2 in range(2)]
                        add(k_, _mm_nt(lrs[k_ // 2], _as_bf16(jnp.concatenate(wr, axis=0))))
                if p_ == 7:
                    break
                a_ = _SA[p_](*ab)
                sub_ = (a_, a_.shift(0, 128), a_.shift(Q4, 0), a_.shift(Q4, 128))
                pr = []
                for q_ in range(7):
                    n = 7 * p_ + q_
                    if n not in ops:
                        ops[n] = _SA[q_](*sub_).load(l4p_.at[(i + 4 * p_) >> (9 + q_)], Q4, 128)
                    w_ = (w3[pl.ds(192 * _PURE[n] + 64 * t, 64), pl.ds(128 * _PURE[n], 128)] if n in _PURE
                          else w3u[n, pl.ds(64 * t, 64), :])
                    pr.append(_mm_nt(ops[n], _as_bf16(w_)))
                m_ = _quad(_comb(pr))
                for k_, sg in _SC[p_]:
                    add(k_, m_, sg)
        kord = [(0, 768), (896, 832)] + [x for c in (0, 3, 1, 4, 2, 5)
                                         for x in ((128 + 128 * c, 64 * c), (1024 + 128 * c, 384 + 64 * c))]
        wl = jnp.concatenate([w4[pl.ds(wr_, 64), pl.ds(512, 128)] for _, wr_ in kord], axis=0)
        gk = lambda r0: jnp.concatenate([gs[pl.ds(r0, H2), pl.ds(o_, 128)] for o_, _ in kord], axis=1).astype(bf16)
        acc_t = _mm(gk(0), wl)
        rn_ = pl.multiple_of(jnp.minimum(i + 1, S // TS - 1) * TS, TS)
        rp = TS // len(LNT)
        ties = {}
        for e, k_ in enumerate(LNT):
            nx = ln4(pl.multiple_of(rn_ + e * rp, rp), rp)
            l4p[pl.ds(e * rp, rp), :] = nx
            ties[k_] = firsts(nx)
        gb_ = _blocks((0, 0), (0, 896), (H2, 0), (H2, 896))
        ms = [None] * 7
        for idx, p_ in enumerate(ORD4):
            a_ = _SA[p_](*gb_)
            wo = (w4[pl.ds(768, 64), pl.ds(0, 256)] if p_ == 2 else
                  w4[pl.ds(832, 64), pl.ds(256, 256)] if p_ == 4 else two(w4o, p_))
            if idx in ties:
                wo = tie_at(wo, 0, 0, ties[idx])
            m_ = _mm(a_.load(gs, H2, 128), wo)
            sub_ = (a_.shift(0, 128), a_.shift(0, 512), a_.shift(Q4, 128), a_.shift(Q4, 512))
            pr = []
            for q_ in range(7):
                n = 7 * p_ + q_
                w_ = (w4[pl.ds(192 * _PURE[n], 192), pl.ds(128 * _PURE[n], 128)] if n in _PURE
                      else w4u[n, pl.ds(0, 192), :])
                pr.append(_mm(_SA[q_](*sub_).load(gs_.at[(i + 4 * p_) >> (9 + q_)], Q4, 384), w_))
            ms[p_] = m_ + _quad(_comb(pr))
        cs = _comb(ms)
        for k_ in ties:
            if k_ >= 10:
                wl = tie_at(wl, 64 * (k_ - 10), 0, ties[k_])
        accs = [acc_t] + [cs[kq] for kq in qorder] + [_mm(gk(H2), wl)]
        gbv = par[pl.ds(48, 8), :]
        for oi, ((r0, c0, cn), ac) in enumerate(zip(outs, accs)):
            rows, cols = pl.ds(_mult(r + r0, H2), H2), pl.ds(c0, cn)
            g3 = lambda x: x.reshape(H2 // 8, 8, cn)
            out = g3(xn[rows, cols]) + gbv[None, :, c0:c0 + cn] * g3(hh[rows, cols] + BETA * ac)
            obuf[rows, cols] = out.reshape(H2, cn).astype(bf16)
            if oi in copies:
                out_copy(r, *copies[oi]).start()
        return carry

    with jax.named_scope("BII"):
        lax.fori_loop(0, S // TS, b2_step, 0)
    with jax.named_scope("out_wait"):
        for i in range(S // TS):
            for o_ in copies.values():
                out_copy(i * TS, *o_).wait()


@jax.jit
def pallas_adaLN_cond__ssm_conv_h3__mixer_s_mlp__prompt_kernel(
    A_q: jax.Array,
    A_k: jax.Array,
    A_v: jax.Array,
    A_shift_k: jax.Array,
    A_ssm_k: jax.Array,
    A_ssm_D: jax.Array,
    B_x: jax.Array,
    B_w1: jax.Array,
    B_w2: jax.Array,
    B_w3: jax.Array,
    B_w4: jax.Array,
    c: jax.Array,
    w_mod: jax.Array,
):
    del B_x
    hbm = pl.BlockSpec(memory_space=pltpu.MemorySpace.HBM)
    spec = pltpu.VMEM((NG * 2 * NC, 8, 128), f32)
    part = pltpu.VMEM((KOFF + 56, 8, 128), f32)
    return pl.pallas_call(
        _kernel,
        out_shape=jax.ShapeDtypeStruct((1, S, D), bf16),
        in_specs=[hbm] * 12,
        out_specs=hbm,
        scratch_shapes=[
            pltpu.VMEM((27, 8, 128), f32),
            pltpu.VMEM((S, D), bf16),
            pltpu.VMEM((NT, 32 + HS, 128), u32),
            pltpu.VMEM((NT, 32 + HS, 128), u32),
            pltpu.VMEM((NT, 64, S), u32),
            pltpu.VMEM((D // 2, D), u32),
            pltpu.VMEM((D // 2, D), u32),
            pltpu.VMEM((1, F // 2, D), u32),
            pltpu.VMEM((1, 896, D), u32),
            pltpu.VMEM((2, D // 2, WMA), u32),
            pltpu.VMEM((D // 2, WMP), u32),
            pltpu.VMEM((D // 2, WMC), u32),
            pltpu.VMEM((S, D), bf16),
            spec, spec, spec, spec,
            part, part,
            pltpu.VMEM((NT, S, 128), f32),
            pltpu.VMEM((S, D), f32),
            pltpu.VMEM((S, D), f32),
            pltpu.VMEM((NT, S + 32, 128), f32),
            pltpu.VMEM((64, D), f32),
            pltpu.VMEM((1, TS, D), f32),
            pltpu.VMEM((1, TS, 1792), f32),
            pltpu.VMEM((52, 400, 128), bf16),
            pltpu.VMEM((52, 400, 128), bf16),
            pltpu.VMEM((14, 128, 128), bf16),
            pltpu.VMEM((14, 96, 128), bf16),
            pltpu.VMEM((4, D), bf16),
            pltpu.VMEM((D,), bf16),
            pltpu.VMEM((1, D), bf16),
            pltpu.SMEM((2,), jnp.int32),
            pltpu.SemaphoreType.DMA((20,)),
            pltpu.SemaphoreType.DMA((1,)),
        ],
        compiler_params=pltpu.CompilerParams(vmem_limit_bytes=100 * 1024 * 1024, disable_semaphore_checks=True,
                                             disable_bounds_checks=True),
    )(A_q, A_k, A_v, A_shift_k.T, A_ssm_k, A_ssm_D, B_w1, B_w2, B_w3.T, B_w4, c, w_mod)
```

```python
import functools
import math

import jax
import jax.numpy as jnp
from jax import lax
import jax.experimental.pallas as pl
import jax.experimental.pallas.tpu as pltpu

S, D, F = 2048, 640, 1728
EPS = 1e-5
NT = D // 128
HS = S // 2

C = 128
NC = S // C
NG = 16
KOFF = (NC + 1) * NG * 3
W = 4
G0 = 4
HEAD, TAIL = 250, 450
DORDER = 'aHbU'
WMA, WMP, WMC = 1280, 640, 640
R = 64
Q0, Q1, Q2 = 320, 768, 1408
N2, PRELN, LEAD, NP4, TIE4 = 5, 2, 3, 2, 12
XRB = (7, 4, 2, 0)
ANCH = (20, 58, 18)
TS = 512
H2, Q4 = TS // 2, TS // 4
LNT = (0, 1, 2, 3, 4, 5, 18, 22)
REMP = (6, 5, 3, 7)
ORD4 = (0, 5, 4, 1, 3, 2, 6)

_C0 = math.sqrt(2.0 / math.pi)
ALPHA = (_C0 * 0.044715) ** (1.0 / 3.0)
GC = _C0 / ALPHA
BETA = 0.5 / ALPHA

f32 = jnp.float32
bf16 = jnp.bfloat16
u32 = jnp.uint32
NTDIMS = (((1,), (1,)), ((), ()))

_SA = (lambda a, b, c, d: a + d, lambda a, b, c, d: d, lambda a, b, c, d: c + d, lambda a, b, c, d: a,
       lambda a, b, c, d: a + b, lambda a, b, c, d: b - d, lambda a, b, c, d: c - a)
_SB = (lambda a, b, c, d: a + d, lambda a, b, c, d: c - a, lambda a, b, c, d: a, lambda a, b, c, d: b - d,
       lambda a, b, c, d: d, lambda a, b, c, d: c + d, lambda a, b, c, d: a + b)
_SBU = ((1, 0, 0, 1), (1, 0, 1, 0), (1, 0, 0, 0), (0, 1, 0, 1), (0, 0, 0, 1), (0, 0, 1, 1), (1, 1, 0, 0))
_SC = (((0, 1), (3, 1)), ((0, 1), (2, 1)), ((2, 1), (3, -1)), ((1, 1), (3, 1)), ((0, -1), (1, 1)), ((0, 1),), ((3, 1),))
_PURE = {7 * p + q: 2 * i + j for i, p in enumerate((2, 4)) for j, q in enumerate((2, 4))}


def _comb(m):
    m1, m4, m2, m3, m5, m7, m6 = m
    return (m1 + m4) + (m7 - m5), m3 + m5, m4 + m2, (m1 + (m3 - m2)) + m6


def _quad(c):
    return jnp.concatenate([jnp.concatenate(c[0:2], axis=1), jnp.concatenate(c[2:4], axis=1)], axis=0)


class _Lazy:
    def __init__(self, terms):
        self.terms = terms

    def __add__(self, o):
        return _Lazy(self.terms + o.terms)

    def __sub__(self, o):
        return _Lazy(self.terms + [(-s, r, c) for (s, r, c) in o.terms])

    def shift(self, dr, dc):
        return _Lazy([(s, r + dr, c + dc) for (s, r, c) in self.terms])

    def load(self, ref, rn, cn):
        ts = sorted(self.terms, key=lambda t: -t[0])
        acc = None
        for (s, r, c) in ts:
            x = ref[pl.ds(r, rn), pl.ds(c, cn)]
            acc = x if acc is None else acc + x if s > 0 else acc - x
        return acc.astype(bf16)


def _blocks(*offsets):
    return [_Lazy([(1, r, c)]) for (r, c) in offsets]


def _unp(w, e):
    return pltpu.bitcast(w & jnp.uint32(0xFFFF0000) if e else w << 16, f32)


def _as_bf16(w):
    return pltpu.bitcast(w, bf16)


def _mm(x, w):
    return jnp.dot(x, w if w.dtype == bf16 else _as_bf16(w), preferred_element_type=f32)


def _mm_nt(x, w):
    return lax.dot_general(x, w, NTDIMS, preferred_element_type=f32)


def _mult(x, n):
    return x if isinstance(x, int) else pl.multiple_of(x, n)


def _cos_table(m, scale):
    mm = jnp.abs(((m + 256) & 511) - 256)
    x = (128 - mm).astype(f32) * (1.0 / 128.0)
    x2 = x * x
    h = math.pi / 2
    p = -(h ** 7) / 5040 + x2 * ((h ** 9) / 362880 - x2 * (h ** 11) / 39916800)
    p = h + x2 * (-(h ** 3) / 6 + x2 * ((h ** 5) / 120 + x2 * p))
    return (x * scale) * p


def _dft_tables():
    r = lax.broadcasted_iota(jnp.int32, (256, 128), 0)
    l = lax.broadcasted_iota(jnp.int32, (256, 128), 1)
    phase = lambda f, t: (4 * (8 * (f >> 4) + (f & 7)) + 1) * t + ((f >> 3) & 1) * 128
    wv = l >> 4
    tu = (16 * W) * (wv // W) + (2 * W) * (l & 7) + 2 * (wv % W) + ((l >> 3) & 1)
    tb = 16 * (r >> 5) + (r & 15)
    tabs = (_cos_table(phase(r, l), 1.0), _cos_table(phase(128 * ((r >> 4) & 1) + l, tb), 1.0 / 128.0),
            _cos_table(phase(r, tu), 1.0))
    return [pltpu.bitcast(x.astype(bf16), f32).reshape(16, 8, 128) for x in tabs]


def _gelu2a(z):
    return z * (1.0 + jnp.tanh(z * (z * z + GC)))


def _center(x, mlp_in=False):
    s1 = jnp.sum(x, axis=-1, keepdims=True)
    m = s1 * (1.0 / D)
    ssd = jnp.maximum(jnp.sum(x * x, axis=-1, keepdims=True) - s1 * m, 0.0)
    lg = jnp.log(ssd + D * EPS / (BETA * BETA if mlp_in else 1.0)) * (-0.5 / math.log(2.0))
    return x - m, jnp.exp2(lg + math.log2(ALPHA * math.sqrt(D)) if mlp_in else lg)


def _conv(us, gs, a):
    acc = None
    for c in range(a + 1):
        p = us[c] * gs[a - c]
        acc = p if acc is None else acc + p
    return acc


def _kernel(q_hbm, k_hbm, v_hbm, sk_hbm, h_hbm, dd_hbm, w1_hbm, w2_hbm, w3_hbm, w4_hbm, c_hbm, wm_hbm, o_hbm,
            modb, qbuf, kbuf, vbuf, hbuf, w1, w2, w3_, w4_, wm, wmp, wmc, obuf, ub0, ub1, gb0, gb1, kb0, kb1,
            yb, xn, hh, h1, par, l4p_, gs_, w4s, w3s, w4o, w3o, sk_s, dd_s, c_s, zs, sems, osem):
    l4p, w3, w4 = l4p_.at[0], w3_.at[0], w4_.at[0]
    ubs, gbs, kbs = (ub0, ub1), (gb0, gb1), (kb0, kb1)
    cp = pltpu.make_async_copy

    def cp_h(j, c0, c1, sem):
        cols = pl.ds(c0, c1 - c0)
        return cp(h_hbm.at[pl.ds(j * 128, 128), cols], hbuf.bitcast(bf16).at[j, :, cols], sem)

    def cp_kv(j, r0, r1, sem):
        r0, r1 = (r0 + 16 if r0 else 0), min(r1 + 16, S)
        lanes = pl.ds(j * 128, 128)
        return [cp(k_hbm.at[0, pl.ds(r0, r1 - r0), lanes], kbuf.bitcast(bf16).at[j, pl.ds(r0 + 16, r1 - r0), :], sem),
                cp(v_hbm.at[0, pl.ds(r0, r1 - r0), lanes], vbuf.bitcast(bf16).at[j, pl.ds(r0, r1 - r0), :], sem)]

    def cp_tile(j, i):
        sem = sems.at[2 * j + i]
        return [cp_h(j, i * HS, (i + 1) * HS, sem)] + cp_kv(j, i * HS, (i + 1) * HS, sem)

    def cp_wm(i):
        return cp(wm_hbm.at[:, pl.ds(i * WMA, WMA)], wm.bitcast(bf16).at[i], sems.at[10 + i])

    def wait_all(cps):
        for c_ in cps:
            c_.wait()

    cp_t0 = [[cp_h(0, 0, S, sems.at[0])], cp_kv(0, 0, 1024, sems.at[1]), cp_kv(0, 1024, 1536, sems.at[17]),
             cp_kv(0, 1536, S, sems.at[18])]
    cp_wmp = cp(wm_hbm.at[:, pl.ds(2 * WMA, WMP)], wmp.bitcast(bf16), sems.at[13])
    cp_wmc = cp(wm_hbm.at[:, pl.ds(2 * WMA + WMP, WMC)], wmc.bitcast(bf16), sems.at[12])
    cp_q = [cp(q_hbm.at[0, pl.ds(r0, r1 - r0), :], qbuf.at[pl.ds(r0, r1 - r0), :], sems.at[sm])
            for sm, r0, r1 in ((13, 0, Q0), (16, Q0, Q1), (14, Q1, Q2), (12, Q2, S))]
    cp_w = [cp(w1_hbm, w1.bitcast(bf16), sems.at[15]), cp(w2_hbm, w2.bitcast(bf16), sems.at[16]),
            cp(w3_hbm, w3_.bitcast(bf16).at[0], sems.at[12]),
            cp(w4_hbm, w4_.bitcast(bf16).at[0, pl.ds(0, F), :], sems.at[14])]
    cp_s = [cp(sk_hbm, sk_s, sems.at[19]), cp(dd_hbm, dd_s, sems.at[19]), cp(c_hbm, c_s, sems.at[19])]
    order = list(cp_s)
    for grp in cp_t0:
        order += grp
    for j in range(1, NT):
        order += cp_tile(j, 0) + cp_tile(j, 1)
    order += [cp_wm(0), cp_wm(1), cp_wmp, cp_q[0], cp_w[0], cp_w[1], cp_q[1], cp_q[2], cp_w[3], cp_q[3], cp_wmc, cp_w[2]]
    for c_ in order:
        c_.start()

    with jax.named_scope("init"):
        tables = _dft_tables()
        for kb in kbs:
            for i, tb in enumerate(tables):
                kb[pl.ds(KOFF + 16 * i, 16)] = tb
            kb[pl.ds(0, NG * 3)] = jnp.zeros((NG * 3, 8, 128), f32)
        w4[pl.ds(F // 2, 32), :] = jnp.zeros((32, D), u32)
        for j in range(NT):
            kbuf[j, pl.ds(0, 8), :] = jnp.zeros((8, 128), u32)
            kbuf[j, pl.ds(8 + HS, 8), :] = jnp.zeros((8, 128), u32)
            vbuf[j, pl.ds(HS, 8), :] = jnp.zeros((8, 128), u32)
            h1[j, pl.ds(8, 8), :] = jnp.zeros((8, 128), f32)
            h1[j, pl.ds(S, 8), :] = jnp.zeros((8, 128), f32)
        wait_all(cp_s)
        par[pl.ds(0, 4), :] = sk_s[...].astype(f32)
        par[pl.ds(8, 8), :] = jnp.broadcast_to(dd_s[...].astype(f32).reshape(1, D), (8, D))
        cv = c_s[...].astype(f32)
        scp = pltpu.bitcast(jnp.broadcast_to(cv * jax.nn.sigmoid(cv), (16, D)).astype(bf16), f32)
        for kb in kbs:
            for j in range(NT):
                kb[KOFF + 48 + j] = scp[:, 128 * j:128 * (j + 1)]

    def mkb(i, unr, off, cache):
        def b(stride, extra=0, z=None):
            if isinstance(i, int):
                return (i * unr + off) * stride + extra
            key = (unr * stride, z)
            if key not in cache:
                base = pl.multiple_of(i * (unr * stride), unr * stride)
                cache[key] = base if z is None else pl.multiple_of(base + (i >> z) * 4, 4)
            return cache[key] + (off * stride + extra)
        return b

    def store_spec(ref, b, x):
        for rg in range(2 * NG):
            for cc in range(4):
                ref[b(4, cc + rg * NC)] = x[8 * rg:8 * rg + 8, 128 * cc:128 * cc + 128]

    def dot_h(j, b, lhs):
        hc = hbuf[j, :, pl.ds(_mult(b(512), 512), 512)]
        rhs_t = jnp.concatenate([hc[:, C * cc:C * (cc + 1)] for cc in range(4)], axis=0)
        store_spec(gbs[j % 2], b, _mm_nt(lhs, _as_bf16(rhs_t)))

    def dot_u(j, b, lhs):
        taps = [par[pl.ds(t, 1), pl.ds(j * 128, 128)] for t in range(4)]
        cols = []
        for cc in range(4):
            words = []
            for blk in range(8 // W):
                w0 = 64 * cc + 8 * W * blk
                kw = {m: kbuf[j, pl.ds(b(256, 8 + w0 + m), 8, stride=W), :] for m in range(-2, W)}
                kk = {2 * m + e: _unp(kw[m], e) for m in range(-2, W) for e in range(2) if 2 * m + e >= -3}
                for m in range(W):
                    vw = vbuf[j, pl.ds(b(256, w0 + m), 8, stride=W), :]
                    for e in range(2):
                        n = 2 * m + e
                        ks = kk[n] * taps[0] + kk[n - 1] * taps[1] + kk[n - 2] * taps[2] + kk[n - 3] * taps[3]
                        words.append(ks * _unp(vw, e))
            cols.append(jnp.concatenate(words, axis=0))
        store_spec(ubs[j % 2], b, _mm(lhs, jnp.concatenate(cols, axis=1).astype(bf16)))

    def out_spec(kidx, groups, nc):
        cols = [[] for _ in range(nc)]
        for gi in groups:
            prev = None
            for cc in range(-1, nc):
                k0, k1, k2 = [kidx(((cc + 1) * NG + gi) * 3 + t) for t in range(3)]
                re, im = k0 - k2, k0 + k1
                if prev is not None:
                    cols[cc] += [re - prev[1], im + prev[0]]
                prev = (re, im)
        return jnp.concatenate([jnp.concatenate(c_, axis=0) for c_ in cols], axis=1).astype(bf16)

    def dot_i(j, b, half, lhs):
        y = _mm(lhs, out_spec(lambda o: kbs[j % 2][b(4 * NG * 3, 2 * half * NG * 3 + o)], range(NG), 2))
        for cc in range(2):
            yb[j, pl.ds(b(512, (2 * half + cc) * C), C), :] = y[:, 128 * cc:128 * cc + 128]

    def dot_k(kb, kt, bt, lhs):
        y = _mm(lhs, out_spec(lambda o: kb[4 * bt * NG * 3 + o], range(8 * kt, 8 * kt + 8), 4))
        for cc in range(4):
            rows = pl.ds((4 * bt + cc) * C, C)
            yc = y[:, 128 * cc:128 * cc + 128]
            yb[NT - 1, rows, :] = yc if kt == 0 else yb[NT - 1, rows, :] + yc

    def gen_m(j, kb, b, ng):
        ub, gb = ubs[j % 2], gbs[j % 2]
        for s in range(ng):
            for t in range(3):
                re = lambda ref, c: ref[b(2 * NC, 2 * s * NC + c, 8 + t)]
                im = lambda ref, c: ref[b(2 * NC, (2 * s + 1) * NC + c, 8 + t)]
                gre = [re(gb, c) for c in range(NC)]
                if t == 0:
                    us, gs = [re(ub, c) + im(ub, c) for c in range(NC)], gre
                elif t == 1:
                    us, gs = [re(ub, c) for c in range(NC)], [im(gb, c) - gre[c] for c in range(NC)]
                else:
                    us, gs = [im(ub, c) for c in range(NC)], [im(gb, c) + gre[c] for c in range(NC)]
                ue, uo, ge, go = us[0::2], us[1::2], gs[0::2], gs[1::2]
                usum = [x + y for x, y in zip(ue, uo)]
                gsum = [x + y for x, y in zip(ge, go)]
                poo_prev = None
                for a in range(NC // 2):
                    pee, poo, pss = _conv(ue, ge, a), _conv(uo, go, a), _conv(usum, gsum, a)
                    kb[b(3, ((2 * a + 1) * NG + s) * 3 + t)] = pee if poo_prev is None else pee + poo_prev
                    kb[b(3, ((2 * a + 2) * NG + s) * 3 + t)] = pss - pee - poo
                    poo_prev = poo
                    yield 3 * (2 * a + 1) + 7

    def add_d(j):
        gb = gbs[j % 2]
        dvec = par[pl.ds(8, 8), pl.ds(j * 128, 128)]
        for gi in range(NG):
            gb[2 * gi * NC] = gb[2 * gi * NC] + dvec

    def dot_m(i, t0, nt, rows):
        m = None
        for kt in range(NT):
            p = _mm(_as_bf16(rows[kt]), wm[i, pl.ds(64 * kt, 64), pl.ds(128 * t0, 128 * nt)])
            m = p if m is None else m + p
        for t in range(nt):
            modb[i * (WMA // 128) + (t0 + t)] = m[0:8, 128 * t:128 * (t + 1)]

    pre = dict(H=0, U=672 + 96 // W, a=192, b=192, m=0, k=176)
    post = dict(H=0, U=0, a=4, b=4, m=2, k=0)
    nst = dict(H=16, U=16, a=8, b=8, m=5, k=8)

    def a_block(dots, mg=None, ng=0, tbl=kb0):
        native, dur = [], []
        for idx, (k_, _) in enumerate(dots):
            nxt = pre[dots[idx + 1][0]] if idx + 1 < len(dots) else 0
            d_ = 2.0 if k_ == 'm' else 1.0
            native += [nxt / nst[k_] + post[k_] * d_] * nst[k_]
            dur += [d_] * nst[k_]
        if mg is not None and dots:
            head = max(HEAD - pre[dots[0][0]], 0)
            mtot = 744 * ng - TAIL - head
            lvl = (mtot + sum(native)) / sum(dur)
            want = [max(lvl * d_ - x, 0.0) for x, d_ in zip(native, dur)]
            cum = [head]
            for w_ in want:
                cum.append(cum[-1] + w_ * mtot / sum(want))
        done, step = 0.0, 0
        for (k_, fn) in dots:
            rows = []
            for n in range(nst[k_]):
                while mg is not None and done < cum[step]:
                    done += next(mg)
                step += 1
                if k_ in 'ab':
                    rows.append(jnp.concatenate([tbl[KOFF + 16 + 2 * n], tbl[KOFF + 17 + 2 * n]], axis=1))
                else:
                    rows.append(tbl[KOFF + dict(H=n, U=32 + n, k=16 + 2 * n, m=48 + n)[k_]])
            fn(rows if k_ == 'm' else _as_bf16(jnp.concatenate(rows, axis=0)))
        for _ in (mg or ()):
            pass

    def fdot(k_, j, b):
        if k_ in 'HU':
            return (k_, functools.partial(dot_h if k_ == 'H' else dot_u, j, b))
        return (k_, functools.partial(dot_i, j, b, 0 if k_ == 'a' else 1))

    def a_loop(jf, jm, ji, g0, ng):
        kinds = [k_ for k_ in DORDER if k_ in 'HU' or ji is not None]

        def body(i, carry):
            cache = {}
            zs[i] = 0
            dots = [fdot(k_, jf if k_ in 'HU' else ji, mkb(i, 2, s_, cache)) for s_ in range(2) for k_ in kinds]
            a_block(dots, gen_m(jm, kbs[jm % 2], mkb(i, ng, g0, cache), ng), ng, kbs[jm % 2])

            @pl.when(i == 0)
            def _():
                wait_all(cp_tile(jf, 1))
            return carry
        wait_all(cp_tile(jf, 0))
        lax.fori_loop(0, 2, body, 0)
        add_d(jf)

    sb_ = lambda bt: mkb(0, 1, bt, None)
    with jax.named_scope("A_seg0"):
        wait_all(cp_t0[0])
        a_block([fdot('H', 0, sb_(bt)) for bt in range(4)])
        add_d(0)
        wait_all(cp_t0[1])
        a_block([fdot('U', 0, sb_(bt)) for bt in range(2)])
        for bt in (2, 3):
            wait_all(cp_t0[bt])
            a_block([fdot('U', 0, sb_(bt))])
    with jax.named_scope("A_m0"):
        def body_m0(i, carry):
            a_block([], gen_m(0, kb0, mkb(i, G0 // 2, 0, {}), G0 // 2))
            return carry
        lax.fori_loop(0, 2, body_m0, 0)
    for seg in range(1, NT):
        with jax.named_scope(f"A_seg{seg}"):
            if seg == 1:
                a_loop(1, 0, None, G0, (NG - G0) // 2)
            else:
                a_loop(seg, seg - 1, seg - 2, 0, 8)

    def with_mod(i, dots, step):
        mm = [('m', functools.partial(dot_m, i, t0, nt)) for (t0, nt) in ((0, 4), (4, 4), (8, 2))]
        return [mm[0]] + dots[:step] + [mm[1]] + dots[step:2 * step] + [mm[2]] + dots[2 * step:]

    with jax.named_scope("A_seg5a"):
        cp_wm(0).wait()
        zz = zs[1]

        @pl.when(zz == 0)
        def _():
            dots = [fdot(k_, NT - 2, sb_(bt)) for bt in range(4) for k_ in 'ab']
            a_block(with_mod(0, dots, 2), gen_m(NT - 1, kb0, mkb(zz, 8, 0, {}), 8), 8, kb0)
    with jax.named_scope("A_seg5b"):
        cp_wm(1).wait()

        @pl.when(zz == 0)
        def _():
            dots = [('k', functools.partial(dot_k, kb0, 0, bt)) for bt in range(4)]
            a_block(with_mod(1, dots, 1), gen_m(NT - 1, kb1, mkb(zz, 8, 8, {}), 8), 8, kb1)

    def zero_of(vs):
        t_ = pltpu.bitcast(vs[0], u32)
        for v_ in vs[1:]:
            t_ = t_ | pltpu.bitcast(v_, u32)
        return t_ & kbuf[0, pl.ds(0, 8), :]

    def tie_at(w_, r0, c0, vs):
        mid = [w_[r0:r0 + 8, :c0]] if c0 else []
        mid.append(w_[r0:r0 + 8, c0:c0 + 128] | zero_of(vs))
        if c0 + 128 < w_.shape[1]:
            mid.append(w_[r0:r0 + 8, c0 + 128:])
        parts = ([w_[:r0]] if r0 else []) + [jnp.concatenate(mid, axis=1)] + ([w_[r0 + 8:]] if r0 + 8 < w_.shape[0] else [])
        return jnp.concatenate(parts, axis=0)

    def tied(wref, ties):
        w_ = wref[...]
        for (t, rb), vs in ties.items():
            w_ = tie_at(w_, 64 * (t % 5) + 8 * rb, 128 * (t // 5), vs)
        return w_

    def firsts(x):
        return [x[8 * g:8 * g + 8, 0:128] for g in range(x.shape[0] // 8)]

    def ln_chain(p):
        rows = pl.ds(p * R, R)
        pa, pb, pc, ps = [par[pl.ds(16 + 8 * t, 8), :][None] for t in range(4)]
        g3 = lambda x: x.reshape(R // 8, 8, D)
        q = g3(qbuf[rows, :].astype(f32))
        d1, r1 = _center(q)
        y = g3(jnp.concatenate([yb[j, rows, :] for j in range(NT)], axis=1))
        x = q + ((d1 * r1) * pa + pb) * y
        xn[rows, :] = x.reshape(R, D)
        d2, r2 = _center(x)
        h = (d2 * r2) * pc + ps
        hh[rows, :] = h.reshape(R, D)
        d3, r3 = _center(h, True)
        return (d3 * r3).reshape(R, D)

    def w1_dot(p, l3, ties, fresh):
        if fresh:
            ties[(0, 2)] = firsts(l3)[0:2]
            l3 = pltpu.bitcast(tie_at(pltpu.bitcast(l3, u32), 0, 128, firsts(l3)[2:4]), f32)
        z = _mm(l3.astype(bf16), tied(w1, ties))
        g = _gelu2a(z)
        lane = lax.broadcasted_iota(jnp.int32, (R, 128), 1)
        for j, (o1, cut, o2) in enumerate(((1, 128, 0), (1, 32, -1), (-1, 64, 2), (2, 96, -2), (-2, 128, 0))):
            gj = g[:, j * 128:(j + 1) * 128]
            if cut == 128:
                h1[j, pl.ds(p * R + 8 + o1, R), :] = gj
            else:
                pltpu.store(h1.at[j, pl.ds(p * R + 8 + o1, R), :], gj, mask=lane < cut)
                pltpu.store(h1.at[j, pl.ds(p * R + 8 + o2, R), :], gj, mask=lane >= cut)
        return z

    def w2_dot(p, ties):
        rows = pl.ds(p * R, R)
        hs = jnp.concatenate([h1[j, pl.ds(p * R + 8, R), :] for j in range(NT)], axis=1).astype(bf16)
        x1 = hh[rows, :] + _mm(hs, tied(w2, ties))
        hh[rows, :] = x1
        return x1

    def ln4(r, n):
        d4, r4 = _center(hh[pl.ds(r, n), :], True)
        return d4 * r4

    zoff = [zz >> p_ for p_ in range(7)]

    def prep2(src, dst, tr, t, p_, anchor):
        zero = zero_of([anchor])
        gate = 0 if _SBU[p_][0] else 3
        l1 = []
        for k2 in range(2):
            for n2 in range(2):
                bl = []
                for b_ in range(4):
                    kq, nq = 2 * (b_ // 2) + k2, 2 * (b_ % 2) + n2
                    x = None
                    if _SBU[p_][b_]:
                        x = src[zoff[p_], pl.ds(8 * t + 192 * (nq if tr else kq), 8), pl.ds(128 * (kq if tr else nq), 128)]
                        if b_ == gate and k2 == n2:
                            x = x | zero
                        x = _as_bf16(x).astype(f32)
                    bl.append(x)
                l1.append(_SB[p_](*bl))
        for q_ in range(7):
            if 7 * p_ + q_ not in _PURE:
                dst[7 * p_ + q_, pl.ds(16 * t, 16), :] = _SB[q_](*l1).astype(bf16)

    def prep1(src, dst, r1, fs, ps_, t, n, anchor):
        bl = [src[pl.ds(lo + 8 * t, 8), pl.ds(c0 + 128 * n, 128)] for lo in (768, r1) for c0 in (0, 256)]
        zero = zero_of([anchor])
        bl[0], bl[3] = bl[0] | zero, bl[3] | zero
        bl = [_as_bf16(x).astype(f32) for x in bl]
        for p_ in ps_:
            dst[2 * p_ + n, pl.ds(16 * t, 16), :] = fs[p_](*bl).astype(bf16)

    def sc_lhs():
        return _as_bf16(jnp.concatenate([kb0[KOFF + 48 + j] for j in range(NT)], axis=1))

    units, l3s = [], {}
    anch = sorted({(ANCH[0] + (ANCH[1] - ANCH[0]) * i // ANCH[2]) % 80 for i in range(ANCH[2])})

    def run_block(dots, extra=None, pre4=False):
        for d_, (k_, p) in enumerate(dots):
            ties = {}
            e, rp = d_ - (len(dots) - NP4), TS // NP4
            if pre4 and e >= 0:
                nx = ln4(e * rp, rp)
                l4p[pl.ds(e * rp, rp), :] = nx
                ties[(TIE4, 7)] = firsts(nx)
            if extra is not None and d_ == len(dots) - 1:
                nx = ln_chain(extra)
                for pr in range(4):
                    ties[(24, XRB[pr])] = firsts(nx)[2 * pr:2 * pr + 2]
                l3s[extra] = nx.astype(bf16)
            if k_ == 1:
                fresh = p not in l3s
                res = w1_dot(p, ln_chain(p) if fresh else l3s.pop(p), ties, fresh)
            elif k_ == 2:
                res = w2_dot(p, ties)
            else:
                par[pl.ds(48, 8), :] = _mm(sc_lhs(), wmc[...])[0:8] * BETA
            for u_ in anch:
                if u_ // 40 + 1 == k_ and units and d_ < len(dots) - (NP4 + 1 if pre4 else 0):
                    n, g = (u_ % 40) // 8, u_ % 8
                    units.pop(0)(res[8 * g:8 * g + 8, 128 * n:128 * (n + 1)])

    pos = [N2, 0]

    def plan(lim1):
        last = lim1 == S // R
        dots = []
        while pos[0] < (lim1 if last else lim1 - 1) or pos[0] - pos[1] >= LEAD or (last and pos[1] < lim1):
            k_ = 0 if pos[0] - pos[1] < LEAD and pos[0] < lim1 else 1
            dots.append((k_ + 1, pos[k_]))
            pos[k_] += 1
        return dots, (None if last else pos[0])

    with jax.named_scope("P1"):
        wait_all([cp_wmp, cp_q[0]])
        mp = _mm(sc_lhs(), wmp[...])
        for t in range(WMP // 128):
            modb[2 * WMA // 128 + t] = mp[0:8, 128 * t:128 * (t + 1)]
        sa, ca, ga, sb, cb = [jnp.concatenate([modb[NT * k_ + j] for j in range(NT)], axis=1) for k_ in range(5)]
        par[pl.ds(16, 8), :] = ga * (1.0 + ca) * math.sqrt(D)
        par[pl.ds(24, 8), :] = ga * sa
        par[pl.ds(32, 8), :] = (1.0 + cb) * (math.sqrt(D) / BETA)
        par[pl.ds(40, 8), :] = sb * (1.0 / BETA)
        for bt in range(4):
            dot_k(kb1, 1, bt, _as_bf16(jnp.concatenate([kb0[KOFF + 17 + 2 * n] for n in range(8)], axis=0)))
        for p in range(PRELN):
            l3s[p] = ln_chain(p)
    with jax.named_scope("w1wait"):
        cp_w[0].wait()
    with jax.named_scope("P2"):
        run_block([(1, p) for p in range(N2)])
    with jax.named_scope("w2wait"):
        wait_all([cp_w[1], cp_q[1]])
    with jax.named_scope("P4"):
        run_block(*plan(Q1 // R))
    with jax.named_scope("q2wait"):
        wait_all([cp_q[2], cp_w[3]])
    units += [functools.partial(prep2, w4_, w4s, False, t, p_) for t in range(24) for p_ in range(7)]
    units += [functools.partial(prep1, w4, w4o, 832, _SB, (0, 1, 3, 5, 6), t, n) for t in range(8) for n in range(2)]
    with jax.named_scope("P5"):
        run_block(*plan(Q2 // R))
    with jax.named_scope("q3wait"):
        wait_all([cp_q[3], cp_wmc, cp_w[2]])
    units += [functools.partial(prep2, w3_, w3s, True, t, p_) for t in range(24) for p_ in range(7)]
    units += [functools.partial(prep1, w3, w3o, 816, _SA, (0, 2, 4, 5, 6), t, n) for t in range(6) for n in range(2)]
    with jax.named_scope("P6"):
        dots, _ = plan(S // R)
        run_block(dots[:-NP4] + [(3, 0)] + dots[-NP4:], pre4=True)
    assert not units

    quads = ((0, 0), (0, 256), (H2, 0), (H2, 256))
    done_at = [max(i for i, p_ in enumerate(ORD4) if any(k_ == kq for k_, _ in _SC[p_])) for kq in range(4)]
    qorder = sorted(range(4), key=lambda kq: done_at[kq])
    outs = [(0, 512, 128)] + [quads[kq] + (256,) for kq in qorder] + [(H2, 512, 128)]
    assert qorder == [0, 1, 2, 3]
    copies = {2: (0, 0, D), 4: (H2, 0, 512), 5: (H2, 512, 128)}

    def out_copy(r, r0, c0, cn):
        rows = pl.ds(_mult(r + r0, H2), H2)
        return cp(obuf.at[rows, pl.ds(c0, cn)], o_hbm.at[0, rows, pl.ds(c0, cn)], osem.at[0])

    def b2_step(i, carry):
        r = pl.multiple_of(i * TS, TS)
        gs = gs_.at[i >> 8]
        lr = l4p[:, pl.ds(512, 128)]
        w3u, w4u = w3s.bitcast(u32), w4s.bitcast(u32)
        two = lambda ref, p_: jnp.concatenate([ref.bitcast(u32)[2 * p_], ref.bitcast(u32)[2 * p_ + 1]], axis=1)
        w3a = lambda p_: (w3[pl.ds(816, 48), pl.ds(256, 256)] if p_ == 1 else
                          w3[pl.ds(768, 48), pl.ds(0, 256)] if p_ == 3 else two(w3o, p_))
        lt_ = _blocks((0, 0), (H2, 0), (0, 256), (H2, 256))
        zt = _mm_nt(_as_bf16(w3[pl.ds(768, 96), pl.ds(512, 128)]), lr.astype(bf16))
        zt = zt + _quad(_comb([_mm_nt(_as_bf16(w3a(p_)), _SB[p_](*lt_).load(l4p_.at[i >> (20 + p_)], H2, 256))
                               for p_ in range(7)]))
        gt = jnp.concatenate([_gelu2a(zt), jnp.zeros((64, TS), f32)], axis=0)
        gs[:, pl.ds(0, 128)] = gt[:128].T
        gs[:, pl.ds(896, 128)] = gt[128:].T
        lrs = [lr[:H2].astype(bf16), lr[H2:].astype(bf16)]
        ab = _blocks(*quads)
        ops = {}
        for t in range(3):
            cq, left = [None] * 4, [5, 3, 3, 5]

            def add(k_, x, sg=1):
                cq[k_] = x if cq[k_] is None else cq[k_] + x if sg > 0 else cq[k_] - x
                left[k_] -= 1
                if left[k_] == 0:
                    gg = _gelu2a(cq[k_])
                    for n2 in range(2):
                        cols = pl.ds(128 + 896 * (k_ % 2) + 128 * (t + 3 * n2), 128)
                        gs[pl.ds(H2 * (k_ // 2), H2), cols] = gg[:, 128 * n2:128 * (n2 + 1)]

            for p_ in range(8):
                for k_ in (2, 1, 0, 3):
                    if REMP[k_] == p_:
                        wr = [w3[pl.ds(64 * (t + 3 * (2 * (k_ % 2) + n2)), 64), pl.ds(512, 128)] for n2 in range(2)]
                        add(k_, _mm_nt(lrs[k_ // 2], _as_bf16(jnp.concatenate(wr, axis=0))))
                if p_ == 7:
                    break
                a_ = _SA[p_](*ab)
                sub_ = (a_, a_.shift(0, 128), a_.shift(Q4, 0), a_.shift(Q4, 128))
                pr = []
                for q_ in range(7):
                    n = 7 * p_ + q_
                    if n not in ops:
                        ops[n] = _SA[q_](*sub_).load(l4p_.at[(i + 4 * p_) >> (9 + q_)], Q4, 128)
                    w_ = (w3[pl.ds(192 * _PURE[n] + 64 * t, 64), pl.ds(128 * _PURE[n], 128)] if n in _PURE
                          else w3u[n, pl.ds(64 * t, 64), :])
                    pr.append(_mm_nt(ops[n], _as_bf16(w_)))
                m_ = _quad(_comb(pr))
                for k_, sg in _SC[p_]:
                    add(k_, m_, sg)
        kord = [(0, 768), (896, 832)] + [x for c in (0, 3, 1, 4, 2, 5)
                                         for x in ((128 + 128 * c, 64 * c), (1024 + 128 * c, 384 + 64 * c))]
        wl = jnp.concatenate([w4[pl.ds(wr_, 64), pl.ds(512, 128)] for _, wr_ in kord], axis=0)
        gk = lambda r0: jnp.concatenate([gs[pl.ds(r0, H2), pl.ds(o_, 128)] for o_, _ in kord], axis=1).astype(bf16)
        acc_t = _mm(gk(0), wl)
        rn_ = pl.multiple_of(jnp.minimum(i + 1, S // TS - 1) * TS, TS)
        rp = TS // len(LNT)
        ties = {}
        for e, k_ in enumerate(LNT):
            nx = ln4(pl.multiple_of(rn_ + e * rp, rp), rp)
            l4p[pl.ds(e * rp, rp), :] = nx
            ties[k_] = firsts(nx)
        gb_ = _blocks((0, 0), (0, 896), (H2, 0), (H2, 896))
        ms = [None] * 7
        for idx, p_ in enumerate(ORD4):
            a_ = _SA[p_](*gb_)
            wo = (w4[pl.ds(768, 64), pl.ds(0, 256)] if p_ == 2 else
                  w4[pl.ds(832, 64), pl.ds(256, 256)] if p_ == 4 else two(w4o, p_))
            if idx in ties:
                wo = tie_at(wo, 0, 0, ties[idx])
            m_ = _mm(a_.load(gs, H2, 128), wo)
            sub_ = (a_.shift(0, 128), a_.shift(0, 512), a_.shift(Q4, 128), a_.shift(Q4, 512))
            pr = []
            for q_ in range(7):
                n = 7 * p_ + q_
                w_ = (w4[pl.ds(192 * _PURE[n], 192), pl.ds(128 * _PURE[n], 128)] if n in _PURE
                      else w4u[n, pl.ds(0, 192), :])
                pr.append(_mm(_SA[q_](*sub_).load(gs_.at[(i + 4 * p_) >> (9 + q_)], Q4, 384), w_))
            ms[p_] = m_ + _quad(_comb(pr))
        cs = _comb(ms)
        for k_ in ties:
            if k_ >= 10:
                wl = tie_at(wl, 64 * (k_ - 10), 0, ties[k_])
        accs = [acc_t] + [cs[kq] for kq in qorder] + [_mm(gk(H2), wl)]
        gbv = par[pl.ds(48, 8), :]
        for oi, ((r0, c0, cn), ac) in enumerate(zip(outs, accs)):
            rows, cols = pl.ds(_mult(r + r0, H2), H2), pl.ds(c0, cn)
            g3 = lambda x: x.reshape(H2 // 8, 8, cn)
            out = g3(xn[rows, cols]) + gbv[None, :, c0:c0 + cn] * g3(hh[rows, cols] + ac)
            obuf[rows, cols] = out.reshape(H2, cn).astype(bf16)
            if oi in copies:
                out_copy(r, *copies[oi]).start()
        return carry

    with jax.named_scope("BII"):
        lax.fori_loop(0, S // TS, b2_step, 0)
    with jax.named_scope("out_wait"):
        for i in range(S // TS):
            for o_ in copies.values():
                out_copy(i * TS, *o_).wait()


@jax.jit
def pallas_adaLN_cond__ssm_conv_h3__mixer_s_mlp__prompt_kernel(
    A_q: jax.Array,
    A_k: jax.Array,
    A_v: jax.Array,
    A_shift_k: jax.Array,
    A_ssm_k: jax.Array,
    A_ssm_D: jax.Array,
    B_x: jax.Array,
    B_w1: jax.Array,
    B_w2: jax.Array,
    B_w3: jax.Array,
    B_w4: jax.Array,
    c: jax.Array,
    w_mod: jax.Array,
):
    del B_x
    hbm = pl.BlockSpec(memory_space=pltpu.MemorySpace.HBM)
    spec = pltpu.VMEM((NG * 2 * NC, 8, 128), f32)
    part = pltpu.VMEM((KOFF + 56, 8, 128), f32)
    return pl.pallas_call(
        _kernel,
        out_shape=jax.ShapeDtypeStruct((1, S, D), bf16),
        in_specs=[hbm] * 12,
        out_specs=hbm,
        scratch_shapes=[
            pltpu.VMEM((27, 8, 128), f32),
            pltpu.VMEM((S, D), bf16),
            pltpu.VMEM((NT, 32 + HS, 128), u32),
            pltpu.VMEM((NT, 32 + HS, 128), u32),
            pltpu.VMEM((NT, 64, S), u32),
            pltpu.VMEM((D // 2, D), u32),
            pltpu.VMEM((D // 2, D), u32),
            pltpu.VMEM((1, F // 2, D), u32),
            pltpu.VMEM((1, 896, D), u32),
            pltpu.VMEM((2, D // 2, WMA), u32),
            pltpu.VMEM((D // 2, WMP), u32),
            pltpu.VMEM((D // 2, WMC), u32),
            pltpu.VMEM((S, D), bf16),
            spec, spec, spec, spec,
            part, part,
            pltpu.VMEM((NT, S, 128), f32),
            pltpu.VMEM((S, D), f32),
            pltpu.VMEM((S, D), f32),
            pltpu.VMEM((NT, S + 32, 128), f32),
            pltpu.VMEM((64, D), f32),
            pltpu.VMEM((1, TS, D), f32),
            pltpu.VMEM((1, TS, 1792), f32),
            pltpu.VMEM((52, 400, 128), bf16),
            pltpu.VMEM((52, 400, 128), bf16),
            pltpu.VMEM((14, 128, 128), bf16),
            pltpu.VMEM((14, 96, 128), bf16),
            pltpu.VMEM((4, D), bf16),
            pltpu.VMEM((D,), bf16),
            pltpu.VMEM((1, D), bf16),
            pltpu.SMEM((2,), jnp.int32),
            pltpu.SemaphoreType.DMA((20,)),
            pltpu.SemaphoreType.DMA((1,)),
        ],
        compiler_params=pltpu.CompilerParams(vmem_limit_bytes=100 * 1024 * 1024, disable_semaphore_checks=True,
                                             disable_bounds_checks=True),
    )(A_q, A_k, A_v, A_shift_k.T, A_ssm_k, A_ssm_D, B_w1, B_w2, B_w3.T, B_w4, c, w_mod)
```

```python
import functools
import math

import jax
import jax.numpy as jnp
from jax import lax
import jax.experimental.pallas as pl
import jax.experimental.pallas.tpu as pltpu

S, D, F = 2048, 640, 1728
EPS = 1e-5
NT = D // 128
HS = S // 2

C = 128
NC = S // C
NG = 16
KOFF = (NC + 1) * NG * 3
W = 4
G0 = 4
HEAD, TAIL = 250, 450
DORDER = 'aHbU'
WMA, WMP, WMC = 1280, 640, 640
R = 64
Q0, Q1, Q2 = 320, 768, 1408
N2, PRELN, LEAD, NP4, TIE4 = 5, 2, 3, 2, 12
XRB = (7, 4, 2, 0)
ANCH = (20, 58, 18)
TS = 512
H2, Q4 = TS // 2, TS // 4
LNT = (0, 1, 2, 3, 4, 5, 6, 22)
REMP = (6, 5, 3, 7)
ORD4 = (0, 5, 4, 1, 3, 2, 6)
TPOS = (0, 1, 2, 3, 4, 5, 6, 9)

_C0 = math.sqrt(2.0 / math.pi)
ALPHA = (_C0 * 0.044715) ** (1.0 / 3.0)
GC = _C0 / ALPHA
BETA = 0.5 / ALPHA

f32 = jnp.float32
bf16 = jnp.bfloat16
u32 = jnp.uint32
NTDIMS = (((1,), (1,)), ((), ()))

_SA = (lambda a, b, c, d: a + d, lambda a, b, c, d: d, lambda a, b, c, d: c + d, lambda a, b, c, d: a,
       lambda a, b, c, d: a + b, lambda a, b, c, d: b - d, lambda a, b, c, d: c - a)
_SB = (lambda a, b, c, d: a + d, lambda a, b, c, d: c - a, lambda a, b, c, d: a, lambda a, b, c, d: b - d,
       lambda a, b, c, d: d, lambda a, b, c, d: c + d, lambda a, b, c, d: a + b)
_SBU = ((1, 0, 0, 1), (1, 0, 1, 0), (1, 0, 0, 0), (0, 1, 0, 1), (0, 0, 0, 1), (0, 0, 1, 1), (1, 1, 0, 0))
_SC = (((0, 1), (3, 1)), ((0, 1), (2, 1)), ((2, 1), (3, -1)), ((1, 1), (3, 1)), ((0, -1), (1, 1)), ((0, 1),), ((3, 1),))
_PURE = {7 * p + q: 2 * i + j for i, p in enumerate((2, 4)) for j, q in enumerate((2, 4))}


def _comb(m):
    m1, m4, m2, m3, m5, m7, m6 = m
    return (m1 + m4) + (m7 - m5), m3 + m5, m4 + m2, (m1 + (m3 - m2)) + m6


def _quad(c):
    return jnp.concatenate([jnp.concatenate(c[0:2], axis=1), jnp.concatenate(c[2:4], axis=1)], axis=0)


class _Lazy:
    def __init__(self, terms):
        self.terms = terms

    def __add__(self, o):
        return _Lazy(self.terms + o.terms)

    def __sub__(self, o):
        return _Lazy(self.terms + [(-s, r, c) for (s, r, c) in o.terms])

    def shift(self, dr, dc):
        return _Lazy([(s, r + dr, c + dc) for (s, r, c) in self.terms])

    def load(self, ref, rn, cn):
        ts = sorted(self.terms, key=lambda t: -t[0])
        acc = None
        for (s, r, c) in ts:
            x = ref[pl.ds(r, rn), pl.ds(c, cn)]
            acc = x if acc is None else acc + x if s > 0 else acc - x
        return acc.astype(bf16)


def _blocks(*offsets):
    return [_Lazy([(1, r, c)]) for (r, c) in offsets]


def _unp(w, e):
    return pltpu.bitcast(w & jnp.uint32(0xFFFF0000) if e else w << 16, f32)


def _as_bf16(w):
    return pltpu.bitcast(w, bf16)


def _mm(x, w):
    return jnp.dot(x, w if w.dtype == bf16 else _as_bf16(w), preferred_element_type=f32)


def _mm_nt(x, w):
    return lax.dot_general(x, w, NTDIMS, preferred_element_type=f32)


def _mult(x, n):
    return x if isinstance(x, int) else pl.multiple_of(x, n)


def _cos_table(m, scale):
    mm = jnp.abs(((m + 256) & 511) - 256)
    x = (128 - mm).astype(f32) * (1.0 / 128.0)
    x2 = x * x
    h = math.pi / 2
    p = -(h ** 7) / 5040 + x2 * ((h ** 9) / 362880 - x2 * (h ** 11) / 39916800)
    p = h + x2 * (-(h ** 3) / 6 + x2 * ((h ** 5) / 120 + x2 * p))
    return (x * scale) * p


def _dft_tables():
    r = lax.broadcasted_iota(jnp.int32, (256, 128), 0)
    l = lax.broadcasted_iota(jnp.int32, (256, 128), 1)
    phase = lambda f, t: (4 * (8 * (f >> 4) + (f & 7)) + 1) * t + ((f >> 3) & 1) * 128
    wv = l >> 4
    tu = (16 * W) * (wv // W) + (2 * W) * (l & 7) + 2 * (wv % W) + ((l >> 3) & 1)
    tb = 16 * (r >> 5) + (r & 15)
    tabs = (_cos_table(phase(r, l), 1.0), _cos_table(phase(128 * ((r >> 4) & 1) + l, tb), 1.0 / 128.0),
            _cos_table(phase(r, tu), 1.0))
    return [pltpu.bitcast(x.astype(bf16), f32).reshape(16, 8, 128) for x in tabs]


def _gelu2a(z):
    return z * (1.0 + jnp.tanh(z * (z * z + GC)))


def _center(x, mlp_in=False):
    s1 = jnp.sum(x, axis=-1, keepdims=True)
    m = s1 * (1.0 / D)
    ssd = jnp.maximum(jnp.sum(x * x, axis=-1, keepdims=True) - s1 * m, 0.0)
    lg = jnp.log(ssd + D * EPS / (BETA * BETA if mlp_in else 1.0)) * (-0.5 / math.log(2.0))
    return x - m, jnp.exp2(lg + math.log2(ALPHA * math.sqrt(D)) if mlp_in else lg)


def _conv(us, gs, a):
    acc = None
    for c in range(a + 1):
        p = us[c] * gs[a - c]
        acc = p if acc is None else acc + p
    return acc


def _kernel(q_hbm, k_hbm, v_hbm, sk_hbm, h_hbm, dd_hbm, w1_hbm, w2_hbm, w3_hbm, w4_hbm, c_hbm, wm_hbm, o_hbm,
            modb, qbuf, kbuf, vbuf, hbuf, w1, w2, w3_, w4_, wm, wmp, wmc, obuf, ub0, ub1, gb0, gb1, kb0, kb1,
            yb, xn, hh, h1, par, l4p_, gs_, w4s, w3s, w4o, w3o, sk_s, dd_s, c_s, zs, sems, osem):
    l4p, w3, w4 = l4p_.at[0], w3_.at[0], w4_.at[0]
    ubs, gbs, kbs = (ub0, ub1), (gb0, gb1), (kb0, kb1)
    cp = pltpu.make_async_copy

    def cp_h(j, c0, c1, sem):
        cols = pl.ds(c0, c1 - c0)
        return cp(h_hbm.at[pl.ds(j * 128, 128), cols], hbuf.bitcast(bf16).at[j, :, cols], sem)

    def cp_kv(j, r0, r1, sem):
        r0, r1 = (r0 + 16 if r0 else 0), min(r1 + 16, S)
        lanes = pl.ds(j * 128, 128)
        return [cp(k_hbm.at[0, pl.ds(r0, r1 - r0), lanes], kbuf.bitcast(bf16).at[j, pl.ds(r0 + 16, r1 - r0), :], sem),
                cp(v_hbm.at[0, pl.ds(r0, r1 - r0), lanes], vbuf.bitcast(bf16).at[j, pl.ds(r0, r1 - r0), :], sem)]

    def cp_tile(j, i):
        sem = sems.at[2 * j + i]
        return [cp_h(j, i * HS, (i + 1) * HS, sem)] + cp_kv(j, i * HS, (i + 1) * HS, sem)

    def cp_wm(i):
        return cp(wm_hbm.at[:, pl.ds(i * WMA, WMA)], wm.bitcast(bf16).at[i], sems.at[10 + i])

    def wait_all(cps):
        for c_ in cps:
            c_.wait()

    cp_t0 = [[cp_h(0, 0, S, sems.at[0])], cp_kv(0, 0, 1024, sems.at[1]), cp_kv(0, 1024, 1536, sems.at[17]),
             cp_kv(0, 1536, S, sems.at[18])]
    cp_wmp = cp(wm_hbm.at[:, pl.ds(2 * WMA, WMP)], wmp.bitcast(bf16), sems.at[13])
    cp_wmc = cp(wm_hbm.at[:, pl.ds(2 * WMA + WMP, WMC)], wmc.bitcast(bf16), sems.at[12])
    cp_q = [cp(q_hbm.at[0, pl.ds(r0, r1 - r0), :], qbuf.at[pl.ds(r0, r1 - r0), :], sems.at[sm])
            for sm, r0, r1 in ((13, 0, Q0), (16, Q0, Q1), (14, Q1, Q2), (12, Q2, S))]
    cp_w = [cp(w1_hbm, w1.bitcast(bf16), sems.at[15]), cp(w2_hbm, w2.bitcast(bf16), sems.at[16]),
            cp(w3_hbm, w3_.bitcast(bf16).at[0], sems.at[12]),
            cp(w4_hbm, w4_.bitcast(bf16).at[0, pl.ds(0, F), :], sems.at[14])]
    cp_s = [cp(sk_hbm, sk_s, sems.at[19]), cp(dd_hbm, dd_s, sems.at[19]), cp(c_hbm, c_s, sems.at[19])]
    order = list(cp_s)
    for grp in cp_t0:
        order += grp
    for j in range(1, NT):
        order += cp_tile(j, 0) + cp_tile(j, 1)
    order += [cp_wm(0), cp_wm(1), cp_wmp, cp_q[0], cp_w[0], cp_w[1], cp_q[1], cp_q[2], cp_w[3], cp_q[3], cp_wmc, cp_w[2]]
    for c_ in order:
        c_.start()

    with jax.named_scope("init"):
        tables = _dft_tables()
        for kb in kbs:
            for i, tb in enumerate(tables):
                kb[pl.ds(KOFF + 16 * i, 16)] = tb
            kb[pl.ds(0, NG * 3)] = jnp.zeros((NG * 3, 8, 128), f32)
        w4[pl.ds(F // 2, 32), :] = jnp.zeros((32, D), u32)
        for j in range(NT):
            kbuf[j, pl.ds(0, 8), :] = jnp.zeros((8, 128), u32)
            kbuf[j, pl.ds(8 + HS, 8), :] = jnp.zeros((8, 128), u32)
            vbuf[j, pl.ds(HS, 8), :] = jnp.zeros((8, 128), u32)
            h1[j, pl.ds(8, 8), :] = jnp.zeros((8, 128), f32)
            h1[j, pl.ds(S, 8), :] = jnp.zeros((8, 128), f32)
        wait_all(cp_s)
        par[pl.ds(0, 4), :] = sk_s[...].astype(f32)
        par[pl.ds(8, 8), :] = jnp.broadcast_to(dd_s[...].astype(f32).reshape(1, D), (8, D))
        cv = c_s[...].astype(f32)
        scp = pltpu.bitcast(jnp.broadcast_to(cv * jax.nn.sigmoid(cv), (16, D)).astype(bf16), f32)
        for kb in kbs:
            for j in range(NT):
                kb[KOFF + 48 + j] = scp[:, 128 * j:128 * (j + 1)]

    def mkb(i, unr, off, cache):
        def b(stride, extra=0, z=None):
            if isinstance(i, int):
                return (i * unr + off) * stride + extra
            key = (unr * stride, z)
            if key not in cache:
                base = pl.multiple_of(i * (unr * stride), unr * stride)
                cache[key] = base if z is None else pl.multiple_of(base + (i >> z) * 4, 4)
            return cache[key] + (off * stride + extra)
        return b

    def store_spec(ref, b, x):
        for rg in range(2 * NG):
            for cc in range(4):
                ref[b(4, cc + rg * NC)] = x[8 * rg:8 * rg + 8, 128 * cc:128 * cc + 128]

    def dot_h(j, b, lhs):
        hc = hbuf[j, :, pl.ds(_mult(b(512), 512), 512)]
        rhs_t = jnp.concatenate([hc[:, C * cc:C * (cc + 1)] for cc in range(4)], axis=0)
        store_spec(gbs[j % 2], b, _mm_nt(lhs, _as_bf16(rhs_t)))

    def dot_u(j, b, lhs):
        taps = [par[pl.ds(t, 1), pl.ds(j * 128, 128)] for t in range(4)]
        cols = []
        for cc in range(4):
            words = []
            for blk in range(8 // W):
                w0 = 64 * cc + 8 * W * blk
                kw = {m: kbuf[j, pl.ds(b(256, 8 + w0 + m), 8, stride=W), :] for m in range(-2, W)}
                kk = {2 * m + e: _unp(kw[m], e) for m in range(-2, W) for e in range(2) if 2 * m + e >= -3}
                for m in range(W):
                    vw = vbuf[j, pl.ds(b(256, w0 + m), 8, stride=W), :]
                    for e in range(2):
                        n = 2 * m + e
                        ks = kk[n] * taps[0] + kk[n - 1] * taps[1] + kk[n - 2] * taps[2] + kk[n - 3] * taps[3]
                        words.append(ks * _unp(vw, e))
            cols.append(jnp.concatenate(words, axis=0))
        store_spec(ubs[j % 2], b, _mm(lhs, jnp.concatenate(cols, axis=1).astype(bf16)))

    def out_spec(kidx, groups, nc):
        cols = [[] for _ in range(nc)]
        for gi in groups:
            prev = None
            for cc in range(-1, nc):
                k0, k1, k2 = [kidx(((cc + 1) * NG + gi) * 3 + t) for t in range(3)]
                re, im = k0 - k2, k0 + k1
                if prev is not None:
                    cols[cc] += [re - prev[1], im + prev[0]]
                prev = (re, im)
        return jnp.concatenate([jnp.concatenate(c_, axis=0) for c_ in cols], axis=1).astype(bf16)

    def dot_i(j, b, half, lhs):
        y = _mm(lhs, out_spec(lambda o: kbs[j % 2][b(4 * NG * 3, 2 * half * NG * 3 + o)], range(NG), 2))
        for cc in range(2):
            yb[j, pl.ds(b(512, (2 * half + cc) * C), C), :] = y[:, 128 * cc:128 * cc + 128]

    def dot_k(kb, kt, bt, lhs):
        y = _mm(lhs, out_spec(lambda o: kb[4 * bt * NG * 3 + o], range(8 * kt, 8 * kt + 8), 4))
        for cc in range(4):
            rows = pl.ds((4 * bt + cc) * C, C)
            yc = y[:, 128 * cc:128 * cc + 128]
            yb[NT - 1, rows, :] = yc if kt == 0 else yb[NT - 1, rows, :] + yc

    def gen_m(j, kb, b, ng):
        ub, gb = ubs[j % 2], gbs[j % 2]
        for s in range(ng):
            for t in range(3):
                re = lambda ref, c: ref[b(2 * NC, 2 * s * NC + c, 8 + t)]
                im = lambda ref, c: ref[b(2 * NC, (2 * s + 1) * NC + c, 8 + t)]
                gre = [re(gb, c) for c in range(NC)]
                if t == 0:
                    us, gs = [re(ub, c) + im(ub, c) for c in range(NC)], gre
                elif t == 1:
                    us, gs = [re(ub, c) for c in range(NC)], [im(gb, c) - gre[c] for c in range(NC)]
                else:
                    us, gs = [im(ub, c) for c in range(NC)], [im(gb, c) + gre[c] for c in range(NC)]
                ue, uo, ge, go = us[0::2], us[1::2], gs[0::2], gs[1::2]
                usum = [x + y for x, y in zip(ue, uo)]
                gsum = [x + y for x, y in zip(ge, go)]
                poo_prev = None
                for a in range(NC // 2):
                    pee, poo, pss = _conv(ue, ge, a), _conv(uo, go, a), _conv(usum, gsum, a)
                    kb[b(3, ((2 * a + 1) * NG + s) * 3 + t)] = pee if poo_prev is None else pee + poo_prev
                    kb[b(3, ((2 * a + 2) * NG + s) * 3 + t)] = pss - pee - poo
                    poo_prev = poo
                    yield 3 * (2 * a + 1) + 7

    def add_d(j):
        gb = gbs[j % 2]
        dvec = par[pl.ds(8, 8), pl.ds(j * 128, 128)]
        for gi in range(NG):
            gb[2 * gi * NC] = gb[2 * gi * NC] + dvec

    def dot_m(i, t0, nt, rows):
        m = None
        for kt in range(NT):
            p = _mm(_as_bf16(rows[kt]), wm[i, pl.ds(64 * kt, 64), pl.ds(128 * t0, 128 * nt)])
            m = p if m is None else m + p
        for t in range(nt):
            modb[i * (WMA // 128) + (t0 + t)] = m[0:8, 128 * t:128 * (t + 1)]

    pre = dict(H=0, U=672 + 96 // W, a=192, b=192, m=0, k=176)
    post = dict(H=0, U=0, a=4, b=4, m=2, k=0)
    nst = dict(H=16, U=16, a=8, b=8, m=5, k=8)

    def a_block(dots, mg=None, ng=0, tbl=kb0):
        native, dur = [], []
        for idx, (k_, _) in enumerate(dots):
            nxt = pre[dots[idx + 1][0]] if idx + 1 < len(dots) else 0
            d_ = 2.0 if k_ == 'm' else 1.0
            native += [nxt / nst[k_] + post[k_] * d_] * nst[k_]
            dur += [d_] * nst[k_]
        if mg is not None and dots:
            head = max(HEAD - pre[dots[0][0]], 0)
            mtot = 744 * ng - TAIL - head
            lvl = (mtot + sum(native)) / sum(dur)
            want = [max(lvl * d_ - x, 0.0) for x, d_ in zip(native, dur)]
            cum = [head]
            for w_ in want:
                cum.append(cum[-1] + w_ * mtot / sum(want))
        done, step = 0.0, 0
        for (k_, fn) in dots:
            rows = []
            for n in range(nst[k_]):
                while mg is not None and done < cum[step]:
                    done += next(mg)
                step += 1
                if k_ in 'ab':
                    rows.append(jnp.concatenate([tbl[KOFF + 16 + 2 * n], tbl[KOFF + 17 + 2 * n]], axis=1))
                else:
                    rows.append(tbl[KOFF + dict(H=n, U=32 + n, k=16 + 2 * n, m=48 + n)[k_]])
            fn(rows if k_ == 'm' else _as_bf16(jnp.concatenate(rows, axis=0)))
        for _ in (mg or ()):
            pass

    def fdot(k_, j, b):
        if k_ in 'HU':
            return (k_, functools.partial(dot_h if k_ == 'H' else dot_u, j, b))
        return (k_, functools.partial(dot_i, j, b, 0 if k_ == 'a' else 1))

    def a_loop(jf, jm, ji, g0, ng):
        kinds = [k_ for k_ in DORDER if k_ in 'HU' or ji is not None]

        def body(i, carry):
            cache = {}
            zs[i] = 0
            dots = [fdot(k_, jf if k_ in 'HU' else ji, mkb(i, 2, s_, cache)) for s_ in range(2) for k_ in kinds]
            a_block(dots, gen_m(jm, kbs[jm % 2], mkb(i, ng, g0, cache), ng), ng, kbs[jm % 2])

            @pl.when(i == 0)
            def _():
                wait_all(cp_tile(jf, 1))
            return carry
        wait_all(cp_tile(jf, 0))
        lax.fori_loop(0, 2, body, 0)
        add_d(jf)

    sb_ = lambda bt: mkb(0, 1, bt, None)
    with jax.named_scope("A_seg0"):
        wait_all(cp_t0[0])
        a_block([fdot('H', 0, sb_(bt)) for bt in range(4)])
        add_d(0)
        wait_all(cp_t0[1])
        a_block([fdot('U', 0, sb_(bt)) for bt in range(2)])
        for bt in (2, 3):
            wait_all(cp_t0[bt])
            a_block([fdot('U', 0, sb_(bt))])
    with jax.named_scope("A_m0"):
        def body_m0(i, carry):
            a_block([], gen_m(0, kb0, mkb(i, G0 // 2, 0, {}), G0 // 2))
            return carry
        lax.fori_loop(0, 2, body_m0, 0)
    for seg in range(1, NT):
        with jax.named_scope(f"A_seg{seg}"):
            if seg == 1:
                a_loop(1, 0, None, G0, (NG - G0) // 2)
            else:
                a_loop(seg, seg - 1, seg - 2, 0, 8)

    def with_mod(i, dots, step):
        mm = [('m', functools.partial(dot_m, i, t0, nt)) for (t0, nt) in ((0, 4), (4, 4), (8, 2))]
        return [mm[0]] + dots[:step] + [mm[1]] + dots[step:2 * step] + [mm[2]] + dots[2 * step:]

    with jax.named_scope("A_seg5a"):
        cp_wm(0).wait()
        zz = zs[1]

        @pl.when(zz == 0)
        def _():
            dots = [fdot(k_, NT - 2, sb_(bt)) for bt in range(4) for k_ in 'ab']
            a_block(with_mod(0, dots, 2), gen_m(NT - 1, kb0, mkb(zz, 8, 0, {}), 8), 8, kb0)
    with jax.named_scope("A_seg5b"):
        cp_wm(1).wait()

        @pl.when(zz == 0)
        def _():
            dots = [('k', functools.partial(dot_k, kb0, 0, bt)) for bt in range(4)]
            a_block(with_mod(1, dots, 1), gen_m(NT - 1, kb1, mkb(zz, 8, 8, {}), 8), 8, kb1)

    def zero_of(vs):
        t_ = pltpu.bitcast(vs[0], u32)
        for v_ in vs[1:]:
            t_ = t_ | pltpu.bitcast(v_, u32)
        return t_ & kbuf[0, pl.ds(0, 8), :]

    def tie_at(w_, r0, c0, vs):
        mid = [w_[r0:r0 + 8, :c0]] if c0 else []
        mid.append(w_[r0:r0 + 8, c0:c0 + 128] | zero_of(vs))
        if c0 + 128 < w_.shape[1]:
            mid.append(w_[r0:r0 + 8, c0 + 128:])
        parts = ([w_[:r0]] if r0 else []) + [jnp.concatenate(mid, axis=1)] + ([w_[r0 + 8:]] if r0 + 8 < w_.shape[0] else [])
        return jnp.concatenate(parts, axis=0)

    def tied(wref, ties):
        w_ = wref[...]
        for (t, rb), vs in ties.items():
            w_ = tie_at(w_, 64 * (t % 5) + 8 * rb, 128 * (t // 5), vs)
        return w_

    def firsts(x):
        return [x[8 * g:8 * g + 8, 0:128] for g in range(x.shape[0] // 8)]

    def ln_chain(p):
        rows = pl.ds(p * R, R)
        pa, pb, pc, ps = [par[pl.ds(16 + 8 * t, 8), :][None] for t in range(4)]
        g3 = lambda x: x.reshape(R // 8, 8, D)
        q = g3(qbuf[rows, :].astype(f32))
        d1, r1 = _center(q)
        y = g3(jnp.concatenate([yb[j, rows, :] for j in range(NT)], axis=1))
        x = q + ((d1 * r1) * pa + pb) * y
        xn[rows, :] = x.reshape(R, D)
        d2, r2 = _center(x)
        h = (d2 * r2) * pc + ps
        hh[rows, :] = h.reshape(R, D)
        d3, r3 = _center(h, True)
        return (d3 * r3).reshape(R, D)

    def w1_dot(p, l3, ties, fresh):
        if fresh:
            ties[(0, 2)] = firsts(l3)[0:2]
            l3 = pltpu.bitcast(tie_at(pltpu.bitcast(l3, u32), 0, 128, firsts(l3)[2:4]), f32)
        z = _mm(l3.astype(bf16), tied(w1, ties))
        g = _gelu2a(z)
        lane = lax.broadcasted_iota(jnp.int32, (R, 128), 1)
        for j, (o1, cut, o2) in enumerate(((1, 128, 0), (1, 32, -1), (-1, 64, 2), (2, 96, -2), (-2, 128, 0))):
            gj = g[:, j * 128:(j + 1) * 128]
            if cut == 128:
                h1[j, pl.ds(p * R + 8 + o1, R), :] = gj
            else:
                pltpu.store(h1.at[j, pl.ds(p * R + 8 + o1, R), :], gj, mask=lane < cut)
                pltpu.store(h1.at[j, pl.ds(p * R + 8 + o2, R), :], gj, mask=lane >= cut)
        return z

    def w2_dot(p, ties):
        rows = pl.ds(p * R, R)
        hs = jnp.concatenate([h1[j, pl.ds(p * R + 8, R), :] for j in range(NT)], axis=1).astype(bf16)
        x1 = hh[rows, :] + _mm(hs, tied(w2, ties))
        hh[rows, :] = x1
        return x1

    def ln4(r, n):
        d4, r4 = _center(hh[pl.ds(r, n), :], True)
        return d4 * r4

    zoff = [zz >> p_ for p_ in range(7)]

    def prep2(src, dst, tr, t, p_, anchor):
        zero = zero_of([anchor])
        gate = 0 if _SBU[p_][0] else 3
        l1 = []
        for k2 in range(2):
            for n2 in range(2):
                bl = []
                for b_ in range(4):
                    kq, nq = 2 * (b_ // 2) + k2, 2 * (b_ % 2) + n2
                    x = None
                    if _SBU[p_][b_]:
                        x = src[zoff[p_], pl.ds(8 * t + 192 * (nq if tr else kq), 8), pl.ds(128 * (kq if tr else nq), 128)]
                        if b_ == gate and k2 == n2:
                            x = x | zero
                        x = _as_bf16(x).astype(f32)
                    bl.append(x)
                l1.append(_SB[p_](*bl))
        for q_ in range(7):
            if 7 * p_ + q_ not in _PURE:
                dst[7 * p_ + q_, pl.ds(16 * t, 16), :] = _SB[q_](*l1).astype(bf16)

    def prep1(src, dst, r1, fs, ps_, t, n, anchor):
        bl = [src[pl.ds(lo + 8 * t, 8), pl.ds(c0 + 128 * n, 128)] for lo in (768, r1) for c0 in (0, 256)]
        zero = zero_of([anchor])
        bl[0], bl[3] = bl[0] | zero, bl[3] | zero
        bl = [_as_bf16(x).astype(f32) for x in bl]
        for p_ in ps_:
            dst[2 * p_ + n, pl.ds(16 * t, 16), :] = fs[p_](*bl).astype(bf16)

    def sc_lhs():
        return _as_bf16(jnp.concatenate([kb0[KOFF + 48 + j] for j in range(NT)], axis=1))

    units, l3s = [], {}
    anch = sorted({(ANCH[0] + (ANCH[1] - ANCH[0]) * i // ANCH[2]) % 80 for i in range(ANCH[2])})

    def run_block(dots, extra=None, pre4=False):
        for d_, (k_, p) in enumerate(dots):
            ties = {}
            e, rp = d_ - (len(dots) - NP4), TS // NP4
            if pre4 and e >= 0:
                nx = ln4(e * rp, rp)
                l4p[pl.ds(e * rp, rp), :] = nx
                ties[(TIE4, 7)] = firsts(nx)
            if extra is not None and d_ == len(dots) - 1:
                nx = ln_chain(extra)
                for pr in range(4):
                    ties[(24, XRB[pr])] = firsts(nx)[2 * pr:2 * pr + 2]
                l3s[extra] = nx.astype(bf16)
            if k_ == 1:
                fresh = p not in l3s
                res = w1_dot(p, ln_chain(p) if fresh else l3s.pop(p), ties, fresh)
            elif k_ == 2:
                res = w2_dot(p, ties)
            else:
                par[pl.ds(48, 8), :] = _mm(sc_lhs(), wmc[...])[0:8] * BETA
            for u_ in anch:
                if u_ // 40 + 1 == k_ and units and d_ < len(dots) - (NP4 + 1 if pre4 else 0):
                    n, g = (u_ % 40) // 8, u_ % 8
                    units.pop(0)(res[8 * g:8 * g + 8, 128 * n:128 * (n + 1)])

    pos = [N2, 0]

    def plan(lim1):
        last = lim1 == S // R
        dots = []
        while pos[0] < (lim1 if last else lim1 - 1) or pos[0] - pos[1] >= LEAD or (last and pos[1] < lim1):
            k_ = 0 if pos[0] - pos[1] < LEAD and pos[0] < lim1 else 1
            dots.append((k_ + 1, pos[k_]))
            pos[k_] += 1
        return dots, (None if last else pos[0])

    with jax.named_scope("P1"):
        wait_all([cp_wmp, cp_q[0]])
        mp = _mm(sc_lhs(), wmp[...])
        for t in range(WMP // 128):
            modb[2 * WMA // 128 + t] = mp[0:8, 128 * t:128 * (t + 1)]
        sa, ca, ga, sb, cb = [jnp.concatenate([modb[NT * k_ + j] for j in range(NT)], axis=1) for k_ in range(5)]
        par[pl.ds(16, 8), :] = ga * (1.0 + ca) * math.sqrt(D)
        par[pl.ds(24, 8), :] = ga * sa
        par[pl.ds(32, 8), :] = (1.0 + cb) * (math.sqrt(D) / BETA)
        par[pl.ds(40, 8), :] = sb * (1.0 / BETA)
        for bt in range(4):
            dot_k(kb1, 1, bt, _as_bf16(jnp.concatenate([kb0[KOFF + 17 + 2 * n] for n in range(8)], axis=0)))
        for p in range(PRELN):
            l3s[p] = ln_chain(p)
    with jax.named_scope("w1wait"):
        cp_w[0].wait()
    with jax.named_scope("P2"):
        run_block([(1, p) for p in range(N2)])
    with jax.named_scope("w2wait"):
        wait_all([cp_w[1], cp_q[1]])
    with jax.named_scope("P4"):
        run_block(*plan(Q1 // R))
    with jax.named_scope("q2wait"):
        wait_all([cp_q[2], cp_w[3]])
    units += [functools.partial(prep2, w4_, w4s, False, t, p_) for t in range(24) for p_ in range(7)]
    units += [functools.partial(prep1, w4, w4o, 832, _SB, (0, 1, 3, 5, 6), t, n) for t in range(8) for n in range(2)]
    with jax.named_scope("P5"):
        run_block(*plan(Q2 // R))
    with jax.named_scope("q3wait"):
        wait_all([cp_q[3], cp_wmc, cp_w[2]])
    units += [functools.partial(prep2, w3_, w3s, True, t, p_) for t in range(24) for p_ in range(7)]
    units += [functools.partial(prep1, w3, w3o, 816, _SA, (0, 2, 4, 5, 6), t, n) for t in range(6) for n in range(2)]
    with jax.named_scope("P6"):
        dots, _ = plan(S // R)
        run_block(dots[:-NP4] + [(3, 0)] + dots[-NP4:], pre4=True)
    assert not units

    quads = ((0, 0), (0, 256), (H2, 0), (H2, 256))
    done_at = [max(i for i, p_ in enumerate(ORD4) if any(k_ == kq for k_, _ in _SC[p_])) for kq in range(4)]
    qorder = sorted(range(4), key=lambda kq: done_at[kq])
    outs = [(0, 512, 128)] + [quads[kq] + (256,) for kq in qorder] + [(H2, 512, 128)]
    assert qorder == [0, 1, 2, 3]
    copies = {2: (0, 0, D), 4: (H2, 0, 512), 5: (H2, 512, 128)}

    def out_copy(r, r0, c0, cn):
        rows = pl.ds(_mult(r + r0, H2), H2)
        return cp(obuf.at[rows, pl.ds(c0, cn)], o_hbm.at[0, rows, pl.ds(c0, cn)], osem.at[0])

    def b2_step(i, carry):
        r = pl.multiple_of(i * TS, TS)
        gs = gs_.at[i >> 8]
        lr = l4p[:, pl.ds(512, 128)]
        w3u, w4u = w3s.bitcast(u32), w4s.bitcast(u32)
        two = lambda ref, p_: jnp.concatenate([ref.bitcast(u32)[2 * p_], ref.bitcast(u32)[2 * p_ + 1]], axis=1)
        w3a = lambda p_: (w3[pl.ds(816, 48), pl.ds(256, 256)] if p_ == 1 else
                          w3[pl.ds(768, 48), pl.ds(0, 256)] if p_ == 3 else two(w3o, p_))
        lt_ = _blocks((0, 0), (H2, 0), (0, 256), (H2, 256))
        tz = []

        def tdots(pos_):
            for k_, at in enumerate(TPOS):
                if at != pos_:
                    continue
                if k_ == 0:
                    tz.append(_mm_nt(_as_bf16(w3[pl.ds(768, 96), pl.ds(512, 128)]), lr.astype(bf16)))
                else:
                    tz.append(_mm_nt(_as_bf16(w3a(k_ - 1)), _SB[k_ - 1](*lt_).load(l4p_.at[i >> (19 + k_)], H2, 256)))
                if k_ == 7:
                    gt = jnp.concatenate([_gelu2a(tz[0] + _quad(_comb(tz[1:]))), jnp.zeros((64, TS), f32)], axis=0)
                    gs[:, pl.ds(0, 128)] = gt[:128].T
                    gs[:, pl.ds(896, 128)] = gt[128:].T
        lrs = [lr[:H2].astype(bf16), lr[H2:].astype(bf16)]
        ab = _blocks(*quads)
        ops = {}
        for t in range(3):
            cq, left = [None] * 4, [5, 3, 3, 5]

            def add(k_, x, sg=1):
                cq[k_] = x if cq[k_] is None else cq[k_] + x if sg > 0 else cq[k_] - x
                left[k_] -= 1
                if left[k_] == 0:
                    gg = _gelu2a(cq[k_])
                    for n2 in range(2):
                        cols = pl.ds(128 + 896 * (k_ % 2) + 128 * (t + 3 * n2), 128)
                        gs[pl.ds(H2 * (k_ // 2), H2), cols] = gg[:, 128 * n2:128 * (n2 + 1)]

            for p_ in range(8):
                for k_ in (2, 1, 0, 3):
                    if REMP[k_] == p_:
                        wr = [w3[pl.ds(64 * (t + 3 * (2 * (k_ % 2) + n2)), 64), pl.ds(512, 128)] for n2 in range(2)]
                        add(k_, _mm_nt(lrs[k_ // 2], _as_bf16(jnp.concatenate(wr, axis=0))))
                tdots(8 * t + p_)
                if p_ == 7:
                    break
                a_ = _SA[p_](*ab)
                sub_ = (a_, a_.shift(0, 128), a_.shift(Q4, 0), a_.shift(Q4, 128))
                pr = []
                for q_ in range(7):
                    n = 7 * p_ + q_
                    if n not in ops:
                        ops[n] = _SA[q_](*sub_).load(l4p_.at[(i + 4 * p_) >> (9 + q_)], Q4, 128)
                    w_ = (w3[pl.ds(192 * _PURE[n] + 64 * t, 64), pl.ds(128 * _PURE[n], 128)] if n in _PURE
                          else w3u[n, pl.ds(64 * t, 64), :])
                    pr.append(_mm_nt(ops[n], _as_bf16(w_)))
                m_ = _quad(_comb(pr))
                for k_, sg in _SC[p_]:
                    add(k_, m_, sg)
        kord = [(0, 768), (896, 832)] + [x for c in (0, 3, 1, 4, 2, 5)
                                         for x in ((128 + 128 * c, 64 * c), (1024 + 128 * c, 384 + 64 * c))]
        wl = jnp.concatenate([w4[pl.ds(wr_, 64), pl.ds(512, 128)] for _, wr_ in kord], axis=0)
        gk = lambda r0: jnp.concatenate([gs[pl.ds(r0, H2), pl.ds(o_, 128)] for o_, _ in kord], axis=1).astype(bf16)
        acc_t = _mm(gk(0), wl)
        rn_ = pl.multiple_of(jnp.minimum(i + 1, S // TS - 1) * TS, TS)
        rp = TS // len(LNT)
        ties = {}
        for e, k_ in enumerate(LNT):
            nx = ln4(pl.multiple_of(rn_ + e * rp, rp), rp)
            l4p[pl.ds(e * rp, rp), :] = nx
            ties[k_] = firsts(nx)
        gb_ = _blocks((0, 0), (0, 896), (H2, 0), (H2, 896))
        ms = [None] * 7
        for idx, p_ in enumerate(ORD4):
            a_ = _SA[p_](*gb_)
            wo = (w4[pl.ds(768, 64), pl.ds(0, 256)] if p_ == 2 else
                  w4[pl.ds(832, 64), pl.ds(256, 256)] if p_ == 4 else two(w4o, p_))
            if idx in ties:
                wo = tie_at(wo, 0, 0, ties[idx])
            m_ = _mm(a_.load(gs, H2, 128), wo)
            sub_ = (a_.shift(0, 128), a_.shift(0, 512), a_.shift(Q4, 128), a_.shift(Q4, 512))
            pr = []
            for q_ in range(7):
                n = 7 * p_ + q_
                w_ = (w4[pl.ds(192 * _PURE[n], 192), pl.ds(128 * _PURE[n], 128)] if n in _PURE
                      else w4u[n, pl.ds(0, 192), :])
                pr.append(_mm(_SA[q_](*sub_).load(gs_.at[(i + 4 * p_) >> (9 + q_)], Q4, 384), w_))
            ms[p_] = m_ + _quad(_comb(pr))
        cs = _comb(ms)
        for k_ in ties:
            if k_ >= 10:
                wl = tie_at(wl, 64 * (k_ - 10), 0, ties[k_])
        accs = [acc_t] + [cs[kq] for kq in qorder] + [_mm(gk(H2), wl)]
        gbv = par[pl.ds(48, 8), :]
        for oi, ((r0, c0, cn), ac) in enumerate(zip(outs, accs)):
            rows, cols = pl.ds(_mult(r + r0, H2), H2), pl.ds(c0, cn)
            g3 = lambda x: x.reshape(H2 // 8, 8, cn)
            out = g3(xn[rows, cols]) + gbv[None, :, c0:c0 + cn] * g3(hh[rows, cols] + ac)
            obuf[rows, cols] = out.reshape(H2, cn).astype(bf16)
            if oi in copies:
                out_copy(r, *copies[oi]).start()
        return carry

    with jax.named_scope("BII"):
        lax.fori_loop(0, S // TS, b2_step, 0)
    with jax.named_scope("out_wait"):
        for i in range(S // TS):
            for o_ in copies.values():
                out_copy(i * TS, *o_).wait()


@jax.jit
def pallas_adaLN_cond__ssm_conv_h3__mixer_s_mlp__prompt_kernel(
    A_q: jax.Array,
    A_k: jax.Array,
    A_v: jax.Array,
    A_shift_k: jax.Array,
    A_ssm_k: jax.Array,
    A_ssm_D: jax.Array,
    B_x: jax.Array,
    B_w1: jax.Array,
    B_w2: jax.Array,
    B_w3: jax.Array,
    B_w4: jax.Array,
    c: jax.Array,
    w_mod: jax.Array,
):
    del B_x
    hbm = pl.BlockSpec(memory_space=pltpu.MemorySpace.HBM)
    spec = pltpu.VMEM((NG * 2 * NC, 8, 128), f32)
    part = pltpu.VMEM((KOFF + 56, 8, 128), f32)
    return pl.pallas_call(
        _kernel,
        out_shape=jax.ShapeDtypeStruct((1, S, D), bf16),
        in_specs=[hbm] * 12,
        out_specs=hbm,
        scratch_shapes=[
            pltpu.VMEM((27, 8, 128), f32),
            pltpu.VMEM((S, D), bf16),
            pltpu.VMEM((NT, 32 + HS, 128), u32),
            pltpu.VMEM((NT, 32 + HS, 128), u32),
            pltpu.VMEM((NT, 64, S), u32),
            pltpu.VMEM((D // 2, D), u32),
            pltpu.VMEM((D // 2, D), u32),
            pltpu.VMEM((1, F // 2, D), u32),
            pltpu.VMEM((1, 896, D), u32),
            pltpu.VMEM((2, D // 2, WMA), u32),
            pltpu.VMEM((D // 2, WMP), u32),
            pltpu.VMEM((D // 2, WMC), u32),
            pltpu.VMEM((S, D), bf16),
            spec, spec, spec, spec,
            part, part,
            pltpu.VMEM((NT, S, 128), f32),
            pltpu.VMEM((S, D), f32),
            pltpu.VMEM((S, D), f32),
            pltpu.VMEM((NT, S + 32, 128), f32),
            pltpu.VMEM((64, D), f32),
            pltpu.VMEM((1, TS, D), f32),
            pltpu.VMEM((1, TS, 1792), f32),
            pltpu.VMEM((52, 400, 128), bf16),
            pltpu.VMEM((52, 400, 128), bf16),
            pltpu.VMEM((14, 128, 128), bf16),
            pltpu.VMEM((14, 96, 128), bf16),
            pltpu.VMEM((4, D), bf16),
            pltpu.VMEM((D,), bf16),
            pltpu.VMEM((1, D), bf16),
            pltpu.SMEM((2,), jnp.int32),
            pltpu.SemaphoreType.DMA((20,)),
            pltpu.SemaphoreType.DMA((1,)),
        ],
        compiler_params=pltpu.CompilerParams(vmem_limit_bytes=100 * 1024 * 1024, disable_semaphore_checks=True,
                                             disable_bounds_checks=True),
    )(A_q, A_k, A_v, A_shift_k.T, A_ssm_k, A_ssm_D, B_w1, B_w2, B_w3.T, B_w4, c, w_mod)
```

```python
import functools
import math

import jax
import jax.numpy as jnp
from jax import lax
import jax.experimental.pallas as pl
import jax.experimental.pallas.tpu as pltpu

S, D, F = 2048, 640, 1728
EPS = 1e-5
NT = D // 128
HS = S // 2

C = 128
NC = S // C
NG = 16
KOFF = (NC + 1) * NG * 3
W = 4
G0 = 4
HEAD, TAIL = 250, 450
DORDER = 'aHbU'
WMA, WMP, WMC = 1280, 640, 640
R = 64
Q0, Q1, Q2 = 320, 768, 1408
N2, PRELN, LEAD, NP4, TIE4 = 5, 2, 3, 2, 12
XRB = (7, 4, 2, 0)
ANCH = (20, 58, 17)
TS = 512
H2, Q4 = TS // 2, TS // 4
LNT = (0, 7, 14, 21, 28, 35, 42, 110)
REMP = (6, 5, 3, 7)
ORD4 = (0, 5, 4, 1, 3, 2, 6)
TPOS = (0, 1, 2, 3, 4, 5, 6, 9)

_C0 = math.sqrt(2.0 / math.pi)
ALPHA = (_C0 * 0.044715) ** (1.0 / 3.0)
GC = _C0 / ALPHA
BETA = 0.5 / ALPHA

f32 = jnp.float32
bf16 = jnp.bfloat16
u32 = jnp.uint32
NTDIMS = (((1,), (1,)), ((), ()))

_SA = (lambda a, b, c, d: a + d, lambda a, b, c, d: d, lambda a, b, c, d: c + d, lambda a, b, c, d: a,
       lambda a, b, c, d: a + b, lambda a, b, c, d: b - d, lambda a, b, c, d: c - a)
_SB = (lambda a, b, c, d: a + d, lambda a, b, c, d: c - a, lambda a, b, c, d: a, lambda a, b, c, d: b - d,
       lambda a, b, c, d: d, lambda a, b, c, d: c + d, lambda a, b, c, d: a + b)
_SBU = ((1, 0, 0, 1), (1, 0, 1, 0), (1, 0, 0, 0), (0, 1, 0, 1), (0, 0, 0, 1), (0, 0, 1, 1), (1, 1, 0, 0))
_SC = (((0, 1), (3, 1)), ((0, 1), (2, 1)), ((2, 1), (3, -1)), ((1, 1), (3, 1)), ((0, -1), (1, 1)), ((0, 1),), ((3, 1),))
_PURE = {7 * p + q: 2 * i + j for i, p in enumerate((2, 4)) for j, q in enumerate((2, 4))}


def _comb(m):
    m1, m4, m2, m3, m5, m7, m6 = m
    return (m1 + m4) + (m7 - m5), m3 + m5, m4 + m2, (m1 + (m3 - m2)) + m6


def _quad(c):
    return jnp.concatenate([jnp.concatenate(c[0:2], axis=1), jnp.concatenate(c[2:4], axis=1)], axis=0)


class _Lazy:
    def __init__(self, terms):
        self.terms = terms

    def __add__(self, o):
        return _Lazy(self.terms + o.terms)

    def __sub__(self, o):
        return _Lazy(self.terms + [(-s, r, c) for (s, r, c) in o.terms])

    def shift(self, dr, dc):
        return _Lazy([(s, r + dr, c + dc) for (s, r, c) in self.terms])

    def load(self, ref, rn, cn):
        ts = sorted(self.terms, key=lambda t: -t[0])
        acc = None
        for (s, r, c) in ts:
            x = ref[pl.ds(r, rn), pl.ds(c, cn)]
            acc = x if acc is None else acc + x if s > 0 else acc - x
        return acc.astype(bf16)


def _blocks(*offsets):
    return [_Lazy([(1, r, c)]) for (r, c) in offsets]


def _unp(w, e):
    return pltpu.bitcast(w & jnp.uint32(0xFFFF0000) if e else w << 16, f32)


def _as_bf16(w):
    return pltpu.bitcast(w, bf16)


def _mm(x, w):
    return jnp.dot(x, w if w.dtype == bf16 else _as_bf16(w), preferred_element_type=f32)


def _mm_nt(x, w):
    return lax.dot_general(x, w, NTDIMS, preferred_element_type=f32)


def _mult(x, n):
    return x if isinstance(x, int) else pl.multiple_of(x, n)


def _cos_table(m, scale):
    mm = jnp.abs(((m + 256) & 511) - 256)
    x = (128 - mm).astype(f32) * (1.0 / 128.0)
    x2 = x * x
    h = math.pi / 2
    p = -(h ** 7) / 5040 + x2 * ((h ** 9) / 362880 - x2 * (h ** 11) / 39916800)
    p = h + x2 * (-(h ** 3) / 6 + x2 * ((h ** 5) / 120 + x2 * p))
    return (x * scale) * p


def _dft_tables():
    r = lax.broadcasted_iota(jnp.int32, (256, 128), 0)
    l = lax.broadcasted_iota(jnp.int32, (256, 128), 1)
    phase = lambda f, t: (4 * (8 * (f >> 4) + (f & 7)) + 1) * t + ((f >> 3) & 1) * 128
    wv = l >> 4
    tu = (16 * W) * (wv // W) + (2 * W) * (l & 7) + 2 * (wv % W) + ((l >> 3) & 1)
    tb = 16 * (r >> 5) + (r & 15)
    tabs = (_cos_table(phase(r, l), 1.0), _cos_table(phase(128 * ((r >> 4) & 1) + l, tb), 1.0 / 128.0),
            _cos_table(phase(r, tu), 1.0))
    return [pltpu.bitcast(x.astype(bf16), f32).reshape(16, 8, 128) for x in tabs]


def _gelu2a(z):
    return z * (1.0 + jnp.tanh(z * (z * z + GC)))


def _center(x, mlp_in=False):
    s1 = jnp.sum(x, axis=-1, keepdims=True)
    m = s1 * (1.0 / D)
    ssd = jnp.maximum(jnp.sum(x * x, axis=-1, keepdims=True) - s1 * m, 0.0)
    lg = jnp.log(ssd + D * EPS / (BETA * BETA if mlp_in else 1.0)) * (-0.5 / math.log(2.0))
    return x - m, jnp.exp2(lg + math.log2(ALPHA * math.sqrt(D)) if mlp_in else lg)


def _conv(us, gs, a):
    acc = None
    for c in range(a + 1):
        p = us[c] * gs[a - c]
        acc = p if acc is None else acc + p
    return acc


def _kernel(q_hbm, k_hbm, v_hbm, sk_hbm, h_hbm, dd_hbm, w1_hbm, w2_hbm, w3_hbm, w4_hbm, c_hbm, wm_hbm, o_hbm,
            modb, qbuf, kbuf, vbuf, hbuf, w1, w2, w3_, w4_, wm, wmp, wmc, obuf, ub0, ub1, gb0, gb1, kb0, kb1,
            yb, xn, hh, h1, par, l4p_, gs_, w4s, w3s, w3o, sk_s, dd_s, c_s, zs, sems, osem):
    l4p, w3, w4 = l4p_.at[0], w3_.at[0], w4_.at[0]
    ubs, gbs, kbs = (ub0, ub1), (gb0, gb1), (kb0, kb1)
    cp = pltpu.make_async_copy

    def cp_h(j, c0, c1, sem):
        cols = pl.ds(c0, c1 - c0)
        return cp(h_hbm.at[pl.ds(j * 128, 128), cols], hbuf.bitcast(bf16).at[j, :, cols], sem)

    def cp_kv(j, r0, r1, sem):
        r0, r1 = (r0 + 16 if r0 else 0), min(r1 + 16, S)
        lanes = pl.ds(j * 128, 128)
        return [cp(k_hbm.at[0, pl.ds(r0, r1 - r0), lanes], kbuf.bitcast(bf16).at[j, pl.ds(r0 + 16, r1 - r0), :], sem),
                cp(v_hbm.at[0, pl.ds(r0, r1 - r0), lanes], vbuf.bitcast(bf16).at[j, pl.ds(r0, r1 - r0), :], sem)]

    def cp_tile(j, i):
        sem = sems.at[2 * j + i]
        return [cp_h(j, i * HS, (i + 1) * HS, sem)] + cp_kv(j, i * HS, (i + 1) * HS, sem)

    def cp_wm(i):
        return cp(wm_hbm.at[:, pl.ds(i * WMA, WMA)], wm.bitcast(bf16).at[i], sems.at[10 + i])

    def wait_all(cps):
        for c_ in cps:
            c_.wait()

    cp_t0 = [[cp_h(0, 0, S, sems.at[0])], cp_kv(0, 0, 1024, sems.at[1]), cp_kv(0, 1024, 1536, sems.at[17]),
             cp_kv(0, 1536, S, sems.at[18])]
    cp_wmp = cp(wm_hbm.at[:, pl.ds(2 * WMA, WMP)], wmp.bitcast(bf16), sems.at[13])
    cp_wmc = cp(wm_hbm.at[:, pl.ds(2 * WMA + WMP, WMC)], wmc.bitcast(bf16), sems.at[12])
    cp_q = [cp(q_hbm.at[0, pl.ds(r0, r1 - r0), :], qbuf.at[pl.ds(r0, r1 - r0), :], sems.at[sm])
            for sm, r0, r1 in ((13, 0, Q0), (16, Q0, Q1), (14, Q1, Q2), (12, Q2, S))]
    cp_w = [cp(w1_hbm, w1.bitcast(bf16), sems.at[15]), cp(w2_hbm, w2.bitcast(bf16), sems.at[16]),
            cp(w3_hbm, w3_.bitcast(bf16).at[0], sems.at[12]),
            cp(w4_hbm, w4_.bitcast(bf16).at[0], sems.at[14])]
    cp_s = [cp(sk_hbm, sk_s, sems.at[19]), cp(dd_hbm, dd_s, sems.at[19]), cp(c_hbm, c_s, sems.at[19])]
    order = list(cp_s)
    for grp in cp_t0:
        order += grp
    for j in range(1, NT):
        order += cp_tile(j, 0) + cp_tile(j, 1)
    order += [cp_wm(0), cp_wm(1), cp_wmp, cp_q[0], cp_w[0], cp_w[1], cp_q[1], cp_q[2], cp_w[3], cp_q[3], cp_wmc, cp_w[2]]
    for c_ in order:
        c_.start()

    with jax.named_scope("init"):
        tables = _dft_tables()
        for kb in kbs:
            for i, tb in enumerate(tables):
                kb[pl.ds(KOFF + 16 * i, 16)] = tb
            kb[pl.ds(0, NG * 3)] = jnp.zeros((NG * 3, 8, 128), f32)
        for j in range(NT):
            kbuf[j, pl.ds(0, 8), :] = jnp.zeros((8, 128), u32)
            kbuf[j, pl.ds(8 + HS, 8), :] = jnp.zeros((8, 128), u32)
            vbuf[j, pl.ds(HS, 8), :] = jnp.zeros((8, 128), u32)
            h1[j, pl.ds(8, 8), :] = jnp.zeros((8, 128), f32)
            h1[j, pl.ds(S, 8), :] = jnp.zeros((8, 128), f32)
        wait_all(cp_s)
        par[pl.ds(0, 4), :] = sk_s[...].astype(f32)
        par[pl.ds(8, 8), :] = jnp.broadcast_to(dd_s[...].astype(f32).reshape(1, D), (8, D))
        cv = c_s[...].astype(f32)
        scp = pltpu.bitcast(jnp.broadcast_to(cv * jax.nn.sigmoid(cv), (16, D)).astype(bf16), f32)
        for kb in kbs:
            for j in range(NT):
                kb[KOFF + 48 + j] = scp[:, 128 * j:128 * (j + 1)]

    def mkb(i, unr, off, cache):
        def b(stride, extra=0, z=None):
            if isinstance(i, int):
                return (i * unr + off) * stride + extra
            key = (unr * stride, z)
            if key not in cache:
                base = pl.multiple_of(i * (unr * stride), unr * stride)
                cache[key] = base if z is None else pl.multiple_of(base + (i >> z) * 4, 4)
            return cache[key] + (off * stride + extra)
        return b

    def store_spec(ref, b, x):
        for rg in range(2 * NG):
            for cc in range(4):
                ref[b(4, cc + rg * NC)] = x[8 * rg:8 * rg + 8, 128 * cc:128 * cc + 128]

    def dot_h(j, b, lhs):
        hc = hbuf[j, :, pl.ds(_mult(b(512), 512), 512)]
        rhs_t = jnp.concatenate([hc[:, C * cc:C * (cc + 1)] for cc in range(4)], axis=0)
        store_spec(gbs[j % 2], b, _mm_nt(lhs, _as_bf16(rhs_t)))

    def dot_u(j, b, lhs):
        taps = [par[pl.ds(t, 1), pl.ds(j * 128, 128)] for t in range(4)]
        cols = []
        for cc in range(4):
            words = []
            for blk in range(8 // W):
                w0 = 64 * cc + 8 * W * blk
                kw = {m: kbuf[j, pl.ds(b(256, 8 + w0 + m), 8, stride=W), :] for m in range(-2, W)}
                kk = {2 * m + e: _unp(kw[m], e) for m in range(-2, W) for e in range(2) if 2 * m + e >= -3}
                for m in range(W):
                    vw = vbuf[j, pl.ds(b(256, w0 + m), 8, stride=W), :]
                    for e in range(2):
                        n = 2 * m + e
                        ks = kk[n] * taps[0] + kk[n - 1] * taps[1] + kk[n - 2] * taps[2] + kk[n - 3] * taps[3]
                        words.append(ks * _unp(vw, e))
            cols.append(jnp.concatenate(words, axis=0))
        store_spec(ubs[j % 2], b, _mm(lhs, jnp.concatenate(cols, axis=1).astype(bf16)))

    def out_spec(kidx, groups, nc):
        cols = [[] for _ in range(nc)]
        for gi in groups:
            prev = None
            for cc in range(-1, nc):
                k0, k1, k2 = [kidx(((cc + 1) * NG + gi) * 3 + t) for t in range(3)]
                re, im = k0 - k2, k0 + k1
                if prev is not None:
                    cols[cc] += [re - prev[1], im + prev[0]]
                prev = (re, im)
        return jnp.concatenate([jnp.concatenate(c_, axis=0) for c_ in cols], axis=1).astype(bf16)

    def dot_i(j, b, half, lhs):
        y = _mm(lhs, out_spec(lambda o: kbs[j % 2][b(4 * NG * 3, 2 * half * NG * 3 + o)], range(NG), 2))
        for cc in range(2):
            yb[j, pl.ds(b(512, (2 * half + cc) * C), C), :] = y[:, 128 * cc:128 * cc + 128]

    def dot_k(kb, kt, bt, lhs):
        y = _mm(lhs, out_spec(lambda o: kb[4 * bt * NG * 3 + o], range(8 * kt, 8 * kt + 8), 4))
        for cc in range(4):
            rows = pl.ds((4 * bt + cc) * C, C)
            yc = y[:, 128 * cc:128 * cc + 128]
            yb[NT - 1, rows, :] = yc if kt == 0 else yb[NT - 1, rows, :] + yc

    def gen_m(j, kb, b, ng):
        ub, gb = ubs[j % 2], gbs[j % 2]
        for s in range(ng):
            for t in range(3):
                re = lambda ref, c: ref[b(2 * NC, 2 * s * NC + c, 8 + t)]
                im = lambda ref, c: ref[b(2 * NC, (2 * s + 1) * NC + c, 8 + t)]
                gre = [re(gb, c) for c in range(NC)]
                if t == 0:
                    us, gs = [re(ub, c) + im(ub, c) for c in range(NC)], gre
                elif t == 1:
                    us, gs = [re(ub, c) for c in range(NC)], [im(gb, c) - gre[c] for c in range(NC)]
                else:
                    us, gs = [im(ub, c) for c in range(NC)], [im(gb, c) + gre[c] for c in range(NC)]
                ue, uo, ge, go = us[0::2], us[1::2], gs[0::2], gs[1::2]
                usum = [x + y for x, y in zip(ue, uo)]
                gsum = [x + y for x, y in zip(ge, go)]
                poo_prev = None
                for a in range(NC // 2):
                    pee, poo, pss = _conv(ue, ge, a), _conv(uo, go, a), _conv(usum, gsum, a)
                    kb[b(3, ((2 * a + 1) * NG + s) * 3 + t)] = pee if poo_prev is None else pee + poo_prev
                    kb[b(3, ((2 * a + 2) * NG + s) * 3 + t)] = pss - pee - poo
                    poo_prev = poo
                    yield 3 * (2 * a + 1) + 7

    def add_d(j):
        gb = gbs[j % 2]
        dvec = par[pl.ds(8, 8), pl.ds(j * 128, 128)]
        for gi in range(NG):
            gb[2 * gi * NC] = gb[2 * gi * NC] + dvec

    def dot_m(i, t0, nt, rows):
        m = None
        for kt in range(NT):
            p = _mm(_as_bf16(rows[kt]), wm[i, pl.ds(64 * kt, 64), pl.ds(128 * t0, 128 * nt)])
            m = p if m is None else m + p
        for t in range(nt):
            modb[i * (WMA // 128) + (t0 + t)] = m[0:8, 128 * t:128 * (t + 1)]

    pre = dict(H=0, U=672 + 96 // W, a=192, b=192, m=0, k=176)
    post = dict(H=0, U=0, a=4, b=4, m=2, k=0)
    nst = dict(H=16, U=16, a=8, b=8, m=5, k=8)

    def a_block(dots, mg=None, ng=0, tbl=kb0):
        native, dur = [], []
        for idx, (k_, _) in enumerate(dots):
            nxt = pre[dots[idx + 1][0]] if idx + 1 < len(dots) else 0
            d_ = 2.0 if k_ == 'm' else 1.0
            native += [nxt / nst[k_] + post[k_] * d_] * nst[k_]
            dur += [d_] * nst[k_]
        if mg is not None and dots:
            head = max(HEAD - pre[dots[0][0]], 0)
            mtot = 744 * ng - TAIL - head
            lvl = (mtot + sum(native)) / sum(dur)
            want = [max(lvl * d_ - x, 0.0) for x, d_ in zip(native, dur)]
            cum = [head]
            for w_ in want:
                cum.append(cum[-1] + w_ * mtot / sum(want))
        done, step = 0.0, 0
        for (k_, fn) in dots:
            rows = []
            for n in range(nst[k_]):
                while mg is not None and done < cum[step]:
                    done += next(mg)
                step += 1
                if k_ in 'ab':
                    rows.append(jnp.concatenate([tbl[KOFF + 16 + 2 * n], tbl[KOFF + 17 + 2 * n]], axis=1))
                else:
                    rows.append(tbl[KOFF + dict(H=n, U=32 + n, k=16 + 2 * n, m=48 + n)[k_]])
            fn(rows if k_ == 'm' else _as_bf16(jnp.concatenate(rows, axis=0)))
        for _ in (mg or ()):
            pass

    def fdot(k_, j, b):
        if k_ in 'HU':
            return (k_, functools.partial(dot_h if k_ == 'H' else dot_u, j, b))
        return (k_, functools.partial(dot_i, j, b, 0 if k_ == 'a' else 1))

    def a_loop(jf, jm, ji, g0, ng):
        kinds = [k_ for k_ in DORDER if k_ in 'HU' or ji is not None]

        def body(i, carry):
            cache = {}
            zs[i] = 0
            dots = [fdot(k_, jf if k_ in 'HU' else ji, mkb(i, 2, s_, cache)) for s_ in range(2) for k_ in kinds]
            a_block(dots, gen_m(jm, kbs[jm % 2], mkb(i, ng, g0, cache), ng), ng, kbs[jm % 2])

            @pl.when(i == 0)
            def _():
                wait_all(cp_tile(jf, 1))
            return carry
        wait_all(cp_tile(jf, 0))
        lax.fori_loop(0, 2, body, 0)
        add_d(jf)

    sb_ = lambda bt: mkb(0, 1, bt, None)
    with jax.named_scope("A_seg0"):
        wait_all(cp_t0[0])
        a_block([fdot('H', 0, sb_(bt)) for bt in range(4)])
        add_d(0)
        wait_all(cp_t0[1])
        a_block([fdot('U', 0, sb_(bt)) for bt in range(2)])
        for bt in (2, 3):
            wait_all(cp_t0[bt])
            a_block([fdot('U', 0, sb_(bt))])
    with jax.named_scope("A_m0"):
        def body_m0(i, carry):
            a_block([], gen_m(0, kb0, mkb(i, G0 // 2, 0, {}), G0 // 2))
            return carry
        lax.fori_loop(0, 2, body_m0, 0)
    for seg in range(1, NT):
        with jax.named_scope(f"A_seg{seg}"):
            if seg == 1:
                a_loop(1, 0, None, G0, (NG - G0) // 2)
            else:
                a_loop(seg, seg - 1, seg - 2, 0, 8)

    def with_mod(i, dots, step):
        mm = [('m', functools.partial(dot_m, i, t0, nt)) for (t0, nt) in ((0, 4), (4, 4), (8, 2))]
        return [mm[0]] + dots[:step] + [mm[1]] + dots[step:2 * step] + [mm[2]] + dots[2 * step:]

    with jax.named_scope("A_seg5a"):
        cp_wm(0).wait()
        zz = zs[1]

        @pl.when(zz == 0)
        def _():
            dots = [fdot(k_, NT - 2, sb_(bt)) for bt in range(4) for k_ in 'ab']
            a_block(with_mod(0, dots, 2), gen_m(NT - 1, kb0, mkb(zz, 8, 0, {}), 8), 8, kb0)
    with jax.named_scope("A_seg5b"):
        cp_wm(1).wait()

        @pl.when(zz == 0)
        def _():
            dots = [('k', functools.partial(dot_k, kb0, 0, bt)) for bt in range(4)]
            a_block(with_mod(1, dots, 1), gen_m(NT - 1, kb1, mkb(zz, 8, 8, {}), 8), 8, kb1)

    def zero_of(vs):
        t_ = pltpu.bitcast(vs[0], u32)
        for v_ in vs[1:]:
            t_ = t_ | pltpu.bitcast(v_, u32)
        return t_ & kbuf[0, pl.ds(0, 8), :]

    def tie_at(w_, r0, c0, vs):
        mid = [w_[r0:r0 + 8, :c0]] if c0 else []
        mid.append(w_[r0:r0 + 8, c0:c0 + 128] | zero_of(vs))
        if c0 + 128 < w_.shape[1]:
            mid.append(w_[r0:r0 + 8, c0 + 128:])
        parts = ([w_[:r0]] if r0 else []) + [jnp.concatenate(mid, axis=1)] + ([w_[r0 + 8:]] if r0 + 8 < w_.shape[0] else [])
        return jnp.concatenate(parts, axis=0)

    def tied(wref, ties):
        w_ = wref[...]
        for (t, rb), vs in ties.items():
            w_ = tie_at(w_, 64 * (t % 5) + 8 * rb, 128 * (t // 5), vs)
        return w_

    def firsts(x):
        return [x[8 * g:8 * g + 8, 0:128] for g in range(x.shape[0] // 8)]

    def ln_chain(p):
        rows = pl.ds(p * R, R)
        pa, pb, pc, ps = [par[pl.ds(16 + 8 * t, 8), :][None] for t in range(4)]
        g3 = lambda x: x.reshape(R // 8, 8, D)
        q = g3(qbuf[rows, :].astype(f32))
        d1, r1 = _center(q)
        y = g3(jnp.concatenate([yb[j, rows, :] for j in range(NT)], axis=1))
        x = q + ((d1 * r1) * pa + pb) * y
        xn[rows, :] = x.reshape(R, D)
        d2, r2 = _center(x)
        h = (d2 * r2) * pc + ps
        hh[rows, :] = h.reshape(R, D)
        d3, r3 = _center(h, True)
        return (d3 * r3).reshape(R, D)

    def w1_dot(p, l3, ties, fresh):
        if fresh:
            ties[(0, 2)] = firsts(l3)[0:2]
            l3 = pltpu.bitcast(tie_at(pltpu.bitcast(l3, u32), 0, 128, firsts(l3)[2:4]), f32)
        z = _mm(l3.astype(bf16), tied(w1, ties))
        g = _gelu2a(z)
        lane = lax.broadcasted_iota(jnp.int32, (R, 128), 1)
        for j, (o1, cut, o2) in enumerate(((1, 128, 0), (1, 32, -1), (-1, 64, 2), (2, 96, -2), (-2, 128, 0))):
            gj = g[:, j * 128:(j + 1) * 128]
            if cut == 128:
                h1[j, pl.ds(p * R + 8 + o1, R), :] = gj
            else:
                pltpu.store(h1.at[j, pl.ds(p * R + 8 + o1, R), :], gj, mask=lane < cut)
                pltpu.store(h1.at[j, pl.ds(p * R + 8 + o2, R), :], gj, mask=lane >= cut)
        return z

    def w2_dot(p, ties):
        rows = pl.ds(p * R, R)
        hs = jnp.concatenate([h1[j, pl.ds(p * R + 8, R), :] for j in range(NT)], axis=1).astype(bf16)
        x1 = hh[rows, :] + _mm(hs, tied(w2, ties))
        hh[rows, :] = x1
        return x1

    def ln4(r, n):
        d4, r4 = _center(hh[pl.ds(r, n), :], True)
        return d4 * r4

    zoff = [zz >> p_ for p_ in range(7)]

    def prep2(src, dst, tr, t, p_, anchor):
        zero = zero_of([anchor])
        gate = 0 if _SBU[p_][0] else 3
        l1 = []
        for k2 in range(2):
            for n2 in range(2):
                bl = []
                for b_ in range(4):
                    kq, nq = 2 * (b_ // 2) + k2, 2 * (b_ % 2) + n2
                    x = None
                    if _SBU[p_][b_]:
                        x = src[zoff[p_], pl.ds(8 * t + 192 * (nq if tr else kq), 8), pl.ds(128 * (kq if tr else nq), 128)]
                        if b_ == gate and k2 == n2:
                            x = x | zero
                        x = _as_bf16(x).astype(f32)
                    bl.append(x)
                l1.append(_SB[p_](*bl))
        for q_ in range(7):
            if 7 * p_ + q_ not in _PURE:
                dst[7 * p_ + q_, pl.ds(16 * t, 16), :] = _SB[q_](*l1).astype(bf16)

    def prep1(t, n, anchor):
        bl = [w3[pl.ds(lo + 8 * t, 8), pl.ds(c0 + 128 * n, 128)] for lo in (768, 816) for c0 in (0, 256)]
        zero = zero_of([anchor])
        bl[0], bl[3] = bl[0] | zero, bl[3] | zero
        bl = [_as_bf16(x).astype(f32) for x in bl]
        for p_ in (0, 2, 4, 5, 6):
            w3o[2 * p_ + n, pl.ds(16 * t, 16), :] = _SA[p_](*bl).astype(bf16)

    def sc_lhs():
        return _as_bf16(jnp.concatenate([kb0[KOFF + 48 + j] for j in range(NT)], axis=1))

    units, l3s = [], {}
    anch = sorted({(ANCH[0] + (ANCH[1] - ANCH[0]) * i // ANCH[2]) % 80 for i in range(ANCH[2])})

    def run_block(dots, extra=None, pre4=False):
        for d_, (k_, p) in enumerate(dots):
            ties = {}
            e, rp = d_ - (len(dots) - NP4), TS // NP4
            if pre4 and e >= 0:
                nx = ln4(e * rp, rp)
                l4p[pl.ds(e * rp, rp), :] = nx
                ties[(TIE4, 7)] = firsts(nx)
            if extra is not None and d_ == len(dots) - 1:
                nx = ln_chain(extra)
                for pr in range(4):
                    ties[(24, XRB[pr])] = firsts(nx)[2 * pr:2 * pr + 2]
                l3s[extra] = nx.astype(bf16)
            if k_ == 1:
                fresh = p not in l3s
                res = w1_dot(p, ln_chain(p) if fresh else l3s.pop(p), ties, fresh)
            elif k_ == 2:
                res = w2_dot(p, ties)
            else:
                par[pl.ds(48, 8), :] = _mm(sc_lhs(), wmc[...])[0:8] * BETA
            for u_ in anch:
                if u_ // 40 + 1 == k_ and units and d_ < len(dots) - (NP4 + 1 if pre4 else 0):
                    n, g = (u_ % 40) // 8, u_ % 8
                    units.pop(0)(res[8 * g:8 * g + 8, 128 * n:128 * (n + 1)])

    pos = [N2, 0]

    def plan(lim1):
        last = lim1 == S // R
        dots = []
        while pos[0] < (lim1 if last else lim1 - 1) or pos[0] - pos[1] >= LEAD or (last and pos[1] < lim1):
            k_ = 0 if pos[0] - pos[1] < LEAD and pos[0] < lim1 else 1
            dots.append((k_ + 1, pos[k_]))
            pos[k_] += 1
        return dots, (None if last else pos[0])

    with jax.named_scope("P1"):
        wait_all([cp_wmp, cp_q[0]])
        mp = _mm(sc_lhs(), wmp[...])
        for t in range(WMP // 128):
            modb[2 * WMA // 128 + t] = mp[0:8, 128 * t:128 * (t + 1)]
        sa, ca, ga, sb, cb = [jnp.concatenate([modb[NT * k_ + j] for j in range(NT)], axis=1) for k_ in range(5)]
        par[pl.ds(16, 8), :] = ga * (1.0 + ca) * math.sqrt(D)
        par[pl.ds(24, 8), :] = ga * sa
        par[pl.ds(32, 8), :] = (1.0 + cb) * (math.sqrt(D) / BETA)
        par[pl.ds(40, 8), :] = sb * (1.0 / BETA)
        for bt in range(4):
            dot_k(kb1, 1, bt, _as_bf16(jnp.concatenate([kb0[KOFF + 17 + 2 * n] for n in range(8)], axis=0)))
        for p in range(PRELN):
            l3s[p] = ln_chain(p)
    with jax.named_scope("w1wait"):
        cp_w[0].wait()
    with jax.named_scope("P2"):
        run_block([(1, p) for p in range(N2)])
    with jax.named_scope("w2wait"):
        wait_all([cp_w[1], cp_q[1]])
    with jax.named_scope("P4"):
        run_block(*plan(Q1 // R))
    with jax.named_scope("q2wait"):
        wait_all([cp_q[2], cp_w[3]])
    units += [functools.partial(prep2, w4_, w4s, False, t, p_) for t in range(24) for p_ in range(7)]
    with jax.named_scope("P5"):
        run_block(*plan(Q2 // R))
    with jax.named_scope("q3wait"):
        wait_all([cp_q[3], cp_wmc, cp_w[2]])
    units += [functools.partial(prep2, w3_, w3s, True, t, p_) for t in range(24) for p_ in range(7)]
    units += [functools.partial(prep1, t, n) for t in range(6) for n in range(2)]
    with jax.named_scope("P6"):
        dots, _ = plan(S // R)
        run_block(dots[:-NP4] + [(3, 0)] + dots[-NP4:], pre4=True)
    assert not units

    quads = ((0, 0), (0, 256), (H2, 0), (H2, 256))
    done_at = [max(i for i, p_ in enumerate(ORD4) if any(k_ == kq for k_, _ in _SC[p_])) for kq in range(4)]
    qorder = sorted(range(4), key=lambda kq: done_at[kq])
    outs = [(0, 512, 128)] + [quads[kq] + (256,) for kq in qorder] + [(H2, 512, 128)]
    assert qorder == [0, 1, 2, 3]
    copies = {2: (0, 0, D), 4: (H2, 0, 512), 5: (H2, 512, 128)}

    def out_copy(r, r0, c0, cn):
        rows = pl.ds(_mult(r + r0, H2), H2)
        return cp(obuf.at[rows, pl.ds(c0, cn)], o_hbm.at[0, rows, pl.ds(c0, cn)], osem.at[0])

    def b2_step(i, carry):
        r = pl.multiple_of(i * TS, TS)
        gs = gs_.at[i >> 8]
        lr = l4p[:, pl.ds(512, 128)]
        w3u, w4u = w3s.bitcast(u32), w4s.bitcast(u32)
        two = lambda ref, p_: jnp.concatenate([ref.bitcast(u32)[2 * p_], ref.bitcast(u32)[2 * p_ + 1]], axis=1)
        w3a = lambda p_: (w3[pl.ds(816, 48), pl.ds(256, 256)] if p_ == 1 else
                          w3[pl.ds(768, 48), pl.ds(0, 256)] if p_ == 3 else two(w3o, p_))
        lt_ = _blocks((0, 0), (H2, 0), (0, 256), (H2, 256))
        tz = []

        def tdots(pos_):
            for k_, at in enumerate(TPOS):
                if at != pos_:
                    continue
                if k_ == 0:
                    tz.append(_mm_nt(_as_bf16(w3[pl.ds(768, 96), pl.ds(512, 128)]), lr.astype(bf16)))
                else:
                    tz.append(_mm_nt(_as_bf16(w3a(k_ - 1)), _SB[k_ - 1](*lt_).load(l4p_.at[i >> (19 + k_)], H2, 256)))
                if k_ == 7:
                    gt = _gelu2a(tz[0] + _quad(_comb(tz[1:])))
                    t1, t2, t3 = [gt[64 * c:64 * (c + 1), :H2] for c in range(3)]
                    u1, u2, u3 = [gt[64 * c:64 * (c + 1), H2:] for c in range(3)]
                    for c, pr_ in enumerate(((t2, u3), (t1, t3 - u3), (u1, u2 - t2))):
                        gs[pl.ds(H2 * (c % 2), H2), pl.ds(1536 + 128 * (c // 2), 128)] = jnp.concatenate(pr_, axis=0).T
        lrs = [lr[:H2].astype(bf16), lr[H2:].astype(bf16)]
        ab = _blocks(*quads)
        ops = {}
        for t in range(3):
            cq, left = [None] * 4, [5, 3, 3, 5]

            def add(k_, x, sg=1):
                cq[k_] = x if cq[k_] is None else cq[k_] + x if sg > 0 else cq[k_] - x
                left[k_] -= 1
                if left[k_] == 0:
                    gg = _gelu2a(cq[k_])
                    for n2 in range(2):
                        cols = pl.ds(768 * (k_ % 2) + 128 * (t + 3 * n2), 128)
                        gs[pl.ds(H2 * (k_ // 2), H2), cols] = gg[:, 128 * n2:128 * (n2 + 1)]

            for p_ in range(8):
                for k_ in (2, 1, 0, 3):
                    if REMP[k_] == p_:
                        wr = [w3[pl.ds(64 * (t + 3 * (2 * (k_ % 2) + n2)), 64), pl.ds(512, 128)] for n2 in range(2)]
                        add(k_, _mm_nt(lrs[k_ // 2], _as_bf16(jnp.concatenate(wr, axis=0))))
                tdots(8 * t + p_)
                if p_ == 7:
                    break
                a_ = _SA[p_](*ab)
                sub_ = (a_, a_.shift(0, 128), a_.shift(Q4, 0), a_.shift(Q4, 128))
                pr = []
                for q_ in range(7):
                    n = 7 * p_ + q_
                    if n not in ops:
                        ops[n] = _SA[q_](*sub_).load(l4p_.at[(i + 4 * p_) >> (9 + q_)], Q4, 128)
                    w_ = (w3[pl.ds(192 * _PURE[n] + 64 * t, 64), pl.ds(128 * _PURE[n], 128)] if n in _PURE
                          else w3u[n, pl.ds(64 * t, 64), :])
                    pr.append(_mm_nt(ops[n], _as_bf16(w_)))
                m_ = _quad(_comb(pr))
                for k_, sg in _SC[p_]:
                    add(k_, m_, sg)
        kord = [c + 3 * n for c in range(3) for n in range(4)]
        gx = lambda c: gs[pl.ds(H2 * (c % 2), H2), pl.ds(1536 + 128 * (c // 2), 128)]
        wx = lambda c, c0, cn: [w4[pl.ds(768 + 32 * b_, 32), pl.ds(c0, cn)] for b_ in ((1, 2), (0, 2), (0, 1))[c]]
        gxs = {}

        def xdot(c, c0, cn):
            if c not in gxs:
                gxs[c] = [gx(c)[Q4 * h_:Q4 * (h_ + 1)].astype(bf16) for h_ in range(2)]
            w_ = jnp.concatenate(wx(c, c0, cn), axis=0)
            return jnp.concatenate([_mm(x, w_) for x in gxs[c]], axis=0)
        wl = jnp.concatenate([w4[pl.ds(64 * k_, 64), pl.ds(512, 128)] for k_ in kord], axis=0)
        gk = lambda r0: jnp.concatenate([gs[pl.ds(r0, H2), pl.ds(128 * k_, 128)] for k_ in kord], axis=1).astype(bf16)
        zs_ = {512: xdot(0, 512, 128)}
        accs = [(zs_[512] + xdot(1, 512, 128)) + _mm(gk(0), wl)]
        rn_ = pl.multiple_of(jnp.minimum(i + 1, S // TS - 1) * TS, TS)
        rp = TS // len(LNT)
        ties = {}
        for e, k_ in enumerate(LNT):
            nx = ln4(pl.multiple_of(rn_ + e * rp, rp), rp)
            l4p[pl.ds(e * rp, rp), :] = nx
            ties[k_] = ties.get(k_, []) + firsts(nx)
        gb_ = _blocks((0, 0), (0, 768), (H2, 0), (H2, 768))
        ms = [None] * 7
        for idx, p_ in enumerate(ORD4):
            a_ = _SA[p_](*gb_)
            sub_ = (a_, a_.shift(0, 384), a_.shift(Q4, 0), a_.shift(Q4, 384))
            pr = []
            for q_ in range(7):
                n = 7 * p_ + q_
                w_ = (w4[pl.ds(192 * _PURE[n], 192), pl.ds(128 * _PURE[n], 128)] if n in _PURE
                      else w4u[n, pl.ds(0, 192), :])
                if 7 * idx + q_ in ties:
                    w_ = tie_at(w_, 0, 0, ties[7 * idx + q_])
                pr.append(_mm(_SA[q_](*sub_).load(gs_.at[(i + 4 * p_) >> (9 + q_)], Q4, 384), w_))
            ms[p_] = _quad(_comb(pr))
            for kq in range(4):
                if done_at[kq] == idx:
                    r0, c0 = quads[kq]
                    if c0 not in zs_:
                        zs_[c0] = xdot(0, c0, 256)
                    acc = zs_[c0]
                    for pp in ORD4[:idx + 1]:
                        for k_, sg in _SC[pp]:
                            if k_ == kq:
                                acc = acc + ms[pp] if sg > 0 else acc - ms[pp]
                    accs.append(acc + xdot(2 if r0 else 1, c0, 256))
        wb = wl
        xb = zs_[512] + xdot(2, 512, 128)
        for k_ in ties:
            if k_ >= 100:
                wb = tie_at(wb, 64 * (k_ - 100), 0, ties[k_])
        accs.append(xb + _mm(gk(H2), wb))
        gbv = par[pl.ds(48, 8), :]
        for oi, ((r0, c0, cn), ac) in enumerate(zip(outs, accs)):
            rows, cols = pl.ds(_mult(r + r0, H2), H2), pl.ds(c0, cn)
            g3 = lambda x: x.reshape(H2 // 8, 8, cn)
            out = g3(xn[rows, cols]) + gbv[None, :, c0:c0 + cn] * g3(hh[rows, cols] + ac)
            obuf[rows, cols] = out.reshape(H2, cn).astype(bf16)
            if oi in copies:
                out_copy(r, *copies[oi]).start()
        return carry

    with jax.named_scope("BII"):
        lax.fori_loop(0, S // TS, b2_step, 0)
    with jax.named_scope("out_wait"):
        for i in range(S // TS):
            for o_ in copies.values():
                out_copy(i * TS, *o_).wait()


@jax.jit
def pallas_adaLN_cond__ssm_conv_h3__mixer_s_mlp__prompt_kernel(
    A_q: jax.Array,
    A_k: jax.Array,
    A_v: jax.Array,
    A_shift_k: jax.Array,
    A_ssm_k: jax.Array,
    A_ssm_D: jax.Array,
    B_x: jax.Array,
    B_w1: jax.Array,
    B_w2: jax.Array,
    B_w3: jax.Array,
    B_w4: jax.Array,
    c: jax.Array,
    w_mod: jax.Array,
):
    del B_x
    hbm = pl.BlockSpec(memory_space=pltpu.MemorySpace.HBM)
    spec = pltpu.VMEM((NG * 2 * NC, 8, 128), f32)
    part = pltpu.VMEM((KOFF + 56, 8, 128), f32)
    return pl.pallas_call(
        _kernel,
        out_shape=jax.ShapeDtypeStruct((1, S, D), bf16),
        in_specs=[hbm] * 12,
        out_specs=hbm,
        scratch_shapes=[
            pltpu.VMEM((27, 8, 128), f32),
            pltpu.VMEM((S, D), bf16),
            pltpu.VMEM((NT, 32 + HS, 128), u32),
            pltpu.VMEM((NT, 32 + HS, 128), u32),
            pltpu.VMEM((NT, 64, S), u32),
            pltpu.VMEM((D // 2, D), u32),
            pltpu.VMEM((D // 2, D), u32),
            pltpu.VMEM((1, F // 2, D), u32),
            pltpu.VMEM((1, F // 2, D), u32),
            pltpu.VMEM((2, D // 2, WMA), u32),
            pltpu.VMEM((D // 2, WMP), u32),
            pltpu.VMEM((D // 2, WMC), u32),
            pltpu.VMEM((S, D), bf16),
            spec, spec, spec, spec,
            part, part,
            pltpu.VMEM((NT, S, 128), f32),
            pltpu.VMEM((S, D), f32),
            pltpu.VMEM((S, D), f32),
            pltpu.VMEM((NT, S + 32, 128), f32),
            pltpu.VMEM((64, D), f32),
            pltpu.VMEM((1, TS, D), f32),
            pltpu.VMEM((1, TS, 1792), f32),
            pltpu.VMEM((52, 400, 128), bf16),
            pltpu.VMEM((52, 400, 128), bf16),
            pltpu.VMEM((14, 96, 128), bf16),
            pltpu.VMEM((4, D), bf16),
            pltpu.VMEM((D,), bf16),
            pltpu.VMEM((1, D), bf16),
            pltpu.SMEM((2,), jnp.int32),
            pltpu.SemaphoreType.DMA((20,)),
            pltpu.SemaphoreType.DMA((1,)),
        ],
        compiler_params=pltpu.CompilerParams(vmem_limit_bytes=100 * 1024 * 1024, disable_semaphore_checks=True,
                                             disable_bounds_checks=True),
    )(A_q, A_k, A_v, A_shift_k.T, A_ssm_k, A_ssm_D, B_w1, B_w2, B_w3.T, B_w4, c, w_mod)
```

```python
import functools
import math

import jax
import jax.numpy as jnp
from jax import lax
import jax.experimental.pallas as pl
import jax.experimental.pallas.tpu as pltpu

S, D, F = 2048, 640, 1728
EPS = 1e-5
NT = D // 128
HS = S // 2

C = 128
NC = S // C
NG = 16
KOFF = (NC + 1) * NG * 3
W = 4
G0 = 4
HEAD, TAIL = 250, 450
DORDER = 'aHbU'
WMA, WMP, WMC = 1280, 640, 640
R = 64
Q0, Q1, Q2 = 320, 768, 1408
N2, PRELN, LEAD, NP4, TIE4 = 5, 2, 3, 2, 18
XRB = (7, 4, 2, 0)
ANCH = (20, 58, 19)
TS = 512
H2, Q4 = TS // 2, TS // 4
LNT = (0, 7, 14, 21, 28, 35, 42, 110)
REMP = (6, 5, 3, 7)
ORD4 = (0, 5, 4, 1, 3, 2, 6)
TPOS = (0, 1, 2, 3, 4, 5, 6, 9)

_C0 = math.sqrt(2.0 / math.pi)
ALPHA = (_C0 * 0.044715) ** (1.0 / 3.0)
GC = _C0 / ALPHA
BETA = 0.5 / ALPHA

f32 = jnp.float32
bf16 = jnp.bfloat16
u32 = jnp.uint32
NTDIMS = (((1,), (1,)), ((), ()))

_SA = (lambda a, b, c, d: a + d, lambda a, b, c, d: d, lambda a, b, c, d: c + d, lambda a, b, c, d: a,
       lambda a, b, c, d: a + b, lambda a, b, c, d: b - d, lambda a, b, c, d: c - a)
_SB = (lambda a, b, c, d: a + d, lambda a, b, c, d: c - a, lambda a, b, c, d: a, lambda a, b, c, d: b - d,
       lambda a, b, c, d: d, lambda a, b, c, d: c + d, lambda a, b, c, d: a + b)
_SBU = ((1, 0, 0, 1), (1, 0, 1, 0), (1, 0, 0, 0), (0, 1, 0, 1), (0, 0, 0, 1), (0, 0, 1, 1), (1, 1, 0, 0))
_SC = (((0, 1), (3, 1)), ((0, 1), (2, 1)), ((2, 1), (3, -1)), ((1, 1), (3, 1)), ((0, -1), (1, 1)), ((0, 1),), ((3, 1),))
_PURE = {7 * p + q: 2 * i + j for i, p in enumerate((2, 4)) for j, q in enumerate((2, 4))}


def _comb(m):
    m1, m4, m2, m3, m5, m7, m6 = m
    return (m1 + m4) + (m7 - m5), m3 + m5, m4 + m2, (m1 + (m3 - m2)) + m6


def _quad(c):
    return jnp.concatenate([jnp.concatenate(c[0:2], axis=1), jnp.concatenate(c[2:4], axis=1)], axis=0)


class _Lazy:
    def __init__(self, terms):
        self.terms = terms

    def __add__(self, o):
        return _Lazy(self.terms + o.terms)

    def __sub__(self, o):
        return _Lazy(self.terms + [(-s, r, c) for (s, r, c) in o.terms])

    def shift(self, dr, dc):
        return _Lazy([(s, r + dr, c + dc) for (s, r, c) in self.terms])

    def load(self, ref, rn, cn):
        ts = sorted(self.terms, key=lambda t: -t[0])
        acc = None
        for (s, r, c) in ts:
            x = ref[pl.ds(r, rn), pl.ds(c, cn)]
            acc = x if acc is None else acc + x if s > 0 else acc - x
        return acc.astype(bf16)


def _blocks(*offsets):
    return [_Lazy([(1, r, c)]) for (r, c) in offsets]


def _unp(w, e):
    return pltpu.bitcast(w & jnp.uint32(0xFFFF0000) if e else w << 16, f32)


def _as_bf16(w):
    return pltpu.bitcast(w, bf16)


def _mm(x, w):
    return jnp.dot(x, w if w.dtype == bf16 else _as_bf16(w), preferred_element_type=f32)


def _mm_nt(x, w):
    return lax.dot_general(x, w, NTDIMS, preferred_element_type=f32)


def _mult(x, n):
    return x if isinstance(x, int) else pl.multiple_of(x, n)


def _cos_table(m, scale):
    mm = jnp.abs(((m + 256) & 511) - 256)
    x = (128 - mm).astype(f32) * (1.0 / 128.0)
    x2 = x * x
    h = math.pi / 2
    p = -(h ** 7) / 5040 + x2 * ((h ** 9) / 362880 - x2 * (h ** 11) / 39916800)
    p = h + x2 * (-(h ** 3) / 6 + x2 * ((h ** 5) / 120 + x2 * p))
    return (x * scale) * p


def _dft_tables():
    r = lax.broadcasted_iota(jnp.int32, (256, 128), 0)
    l = lax.broadcasted_iota(jnp.int32, (256, 128), 1)
    phase = lambda f, t: (4 * (8 * (f >> 4) + (f & 7)) + 1) * t + ((f >> 3) & 1) * 128
    wv = l >> 4
    tu = (16 * W) * (wv // W) + (2 * W) * (l & 7) + 2 * (wv % W) + ((l >> 3) & 1)
    tb = 16 * (r >> 5) + (r & 15)
    tabs = (_cos_table(phase(r, l), 1.0), _cos_table(phase(128 * ((r >> 4) & 1) + l, tb), 1.0 / 128.0),
            _cos_table(phase(r, tu), 1.0))
    return [pltpu.bitcast(x.astype(bf16), f32).reshape(16, 8, 128) for x in tabs]


def _gelu2a(z):
    return z * (1.0 + jnp.tanh(z * (z * z + GC)))


def _center(x, mlp_in=False):
    s1 = jnp.sum(x, axis=-1, keepdims=True)
    m = s1 * (1.0 / D)
    ssd = jnp.maximum(jnp.sum(x * x, axis=-1, keepdims=True) - s1 * m, 0.0)
    lg = jnp.log(ssd + D * EPS / (BETA * BETA if mlp_in else 1.0)) * (-0.5 / math.log(2.0))
    return x - m, jnp.exp2(lg + math.log2(ALPHA * math.sqrt(D)) if mlp_in else lg)


def _conv(us, gs, a):
    acc = None
    for c in range(a + 1):
        p = us[c] * gs[a - c]
        acc = p if acc is None else acc + p
    return acc


def _kernel(q_hbm, k_hbm, v_hbm, sk_hbm, h_hbm, dd_hbm, w1_hbm, w2_hbm, w3_hbm, w4_hbm, c_hbm, wm_hbm, o_hbm,
            modb, qbuf, kbuf, vbuf, hbuf, w1, w2, w3_, w4_, wm, wmp, wmc, obuf, ub0, ub1, gb0, gb1, kb0, kb1,
            yb, xn, hh, h1, par, l4p_, gs_, w4s, w3s, w3o, sct, sk_s, dd_s, c_s, zs, sems, osem):
    l4p, w3, w4 = l4p_.at[0], w3_.at[0], w4_.at[0]
    ubs, gbs, kbs = (ub0, ub1), (gb0, gb1), (kb0, kb1)
    cp = pltpu.make_async_copy

    def cp_h(j, c0, c1, sem):
        cols = pl.ds(c0, c1 - c0)
        return cp(h_hbm.at[pl.ds(j * 128, 128), cols], hbuf.bitcast(bf16).at[j, :, cols], sem)

    def cp_kv(j, r0, r1, sem):
        r0, r1 = (r0 + 16 if r0 else 0), min(r1 + 16, S)
        lanes = pl.ds(j * 128, 128)
        return [cp(k_hbm.at[0, pl.ds(r0, r1 - r0), lanes], kbuf.bitcast(bf16).at[j, pl.ds(r0 + 16, r1 - r0), :], sem),
                cp(v_hbm.at[0, pl.ds(r0, r1 - r0), lanes], vbuf.bitcast(bf16).at[j, pl.ds(r0, r1 - r0), :], sem)]

    def cp_tile(j, i):
        sem = sems.at[2 * j + i]
        return [cp_h(j, i * HS, (i + 1) * HS, sem)] + cp_kv(j, i * HS, (i + 1) * HS, sem)

    def cp_wm(i):
        return cp(wm_hbm.at[:, pl.ds(i * WMA, WMA)], wm.bitcast(bf16).at[i], sems.at[10 + i])

    def wait_all(cps):
        for c_ in cps:
            c_.wait()

    cp_t0 = [[cp_h(0, 0, S, sems.at[0])], cp_kv(0, 0, 1024, sems.at[1]), cp_kv(0, 1024, 1536, sems.at[17]),
             cp_kv(0, 1536, S, sems.at[18])]
    cp_wmp = cp(wm_hbm.at[:, pl.ds(2 * WMA, WMP)], wmp.bitcast(bf16), sems.at[13])
    cp_wmc = cp(wm_hbm.at[:, pl.ds(2 * WMA + WMP, WMC)], wmc.bitcast(bf16), sems.at[12])
    cp_q = [cp(q_hbm.at[0, pl.ds(r0, r1 - r0), :], qbuf.at[pl.ds(r0, r1 - r0), :], sems.at[sm])
            for sm, r0, r1 in ((13, 0, Q0), (16, Q0, Q1), (14, Q1, Q2), (12, Q2, S))]
    cp_w = [cp(w1_hbm, w1.bitcast(bf16), sems.at[15]), cp(w2_hbm, w2.bitcast(bf16), sems.at[16]),
            cp(w3_hbm, w3_.bitcast(bf16).at[0], sems.at[12]),
            cp(w4_hbm, w4_.bitcast(bf16).at[0], sems.at[14])]
    cp_s = [cp(sk_hbm, sk_s, sems.at[19]), cp(dd_hbm, dd_s, sems.at[19]), cp(c_hbm, c_s, sems.at[19])]
    order = list(cp_s)
    for grp in cp_t0:
        order += grp
    for j in range(1, NT):
        order += cp_tile(j, 0) + cp_tile(j, 1)
    order += [cp_wm(0), cp_wm(1), cp_wmp, cp_q[0], cp_w[0], cp_w[1], cp_q[1], cp_q[2], cp_w[3], cp_q[3], cp_wmc, cp_w[2]]
    for c_ in order:
        c_.start()

    with jax.named_scope("init"):
        tables = _dft_tables()
        for kb in kbs:
            for i, tb in enumerate(tables):
                kb[pl.ds(KOFF + 16 * i, 16)] = tb
            kb[pl.ds(0, NG * 3)] = jnp.zeros((NG * 3, 8, 128), f32)
        for j in range(NT):
            kbuf[j, pl.ds(0, 8), :] = jnp.zeros((8, 128), u32)
            kbuf[j, pl.ds(8 + HS, 8), :] = jnp.zeros((8, 128), u32)
            vbuf[j, pl.ds(HS, 8), :] = jnp.zeros((8, 128), u32)
            h1[j, pl.ds(8, 8), :] = jnp.zeros((8, 128), f32)
            h1[j, pl.ds(S, 8), :] = jnp.zeros((8, 128), f32)
        wait_all(cp_s)
        par[pl.ds(0, 4), :] = sk_s[...].astype(f32)
        par[pl.ds(8, 8), :] = jnp.broadcast_to(dd_s[...].astype(f32).reshape(1, D), (8, D))
        cv = c_s[...].astype(f32)
        sil = cv * jax.nn.sigmoid(cv)
        scp = pltpu.bitcast(jnp.broadcast_to(sil, (16, D)).astype(bf16), f32)
        sct[...] = jnp.broadcast_to(sil.astype(bf16).astype(f32) * BETA, (128, D)).T
        for kb in kbs:
            for j in range(NT):
                kb[KOFF + 48 + j] = scp[:, 128 * j:128 * (j + 1)]

    def mkb(i, unr, off, cache):
        def b(stride, extra=0, z=None):
            if isinstance(i, int):
                return (i * unr + off) * stride + extra
            key = (unr * stride, z)
            if key not in cache:
                base = pl.multiple_of(i * (unr * stride), unr * stride)
                cache[key] = base if z is None else pl.multiple_of(base + (i >> z) * 4, 4)
            return cache[key] + (off * stride + extra)
        return b

    def store_spec(ref, b, x):
        for rg in range(2 * NG):
            for cc in range(4):
                ref[b(4, cc + rg * NC)] = x[8 * rg:8 * rg + 8, 128 * cc:128 * cc + 128]

    def dot_h(j, b, lhs):
        hc = hbuf[j, :, pl.ds(_mult(b(512), 512), 512)]
        rhs_t = jnp.concatenate([hc[:, C * cc:C * (cc + 1)] for cc in range(4)], axis=0)
        store_spec(gbs[j % 2], b, _mm_nt(lhs, _as_bf16(rhs_t)))

    def dot_u(j, b, lhs):
        taps = [par[pl.ds(t, 1), pl.ds(j * 128, 128)] for t in range(4)]
        cols = []
        for cc in range(4):
            words = []
            for blk in range(8 // W):
                w0 = 64 * cc + 8 * W * blk
                kw = {m: kbuf[j, pl.ds(b(256, 8 + w0 + m), 8, stride=W), :] for m in range(-2, W)}
                kk = {2 * m + e: _unp(kw[m], e) for m in range(-2, W) for e in range(2) if 2 * m + e >= -3}
                for m in range(W):
                    vw = vbuf[j, pl.ds(b(256, w0 + m), 8, stride=W), :]
                    for e in range(2):
                        n = 2 * m + e
                        ks = kk[n] * taps[0] + kk[n - 1] * taps[1] + kk[n - 2] * taps[2] + kk[n - 3] * taps[3]
                        words.append(ks * _unp(vw, e))
            cols.append(jnp.concatenate(words, axis=0))
        store_spec(ubs[j % 2], b, _mm(lhs, jnp.concatenate(cols, axis=1).astype(bf16)))

    def out_spec(kidx, groups, nc):
        cols = [[] for _ in range(nc)]
        for gi in groups:
            prev = None
            for cc in range(-1, nc):
                k0, k1, k2 = [kidx(((cc + 1) * NG + gi) * 3 + t) for t in range(3)]
                re, im = k0 - k2, k0 + k1
                if prev is not None:
                    cols[cc] += [re - prev[1], im + prev[0]]
                prev = (re, im)
        return jnp.concatenate([jnp.concatenate(c_, axis=0) for c_ in cols], axis=1).astype(bf16)

    def dot_i(j, b, half, lhs):
        y = _mm(lhs, out_spec(lambda o: kbs[j % 2][b(4 * NG * 3, 2 * half * NG * 3 + o)], range(NG), 2))
        for cc in range(2):
            yb[j, pl.ds(b(512, (2 * half + cc) * C), C), :] = y[:, 128 * cc:128 * cc + 128]

    def dot_k(kb, kt, bt, lhs):
        y = _mm(lhs, out_spec(lambda o: kb[4 * bt * NG * 3 + o], range(8 * kt, 8 * kt + 8), 4))
        for cc in range(4):
            rows = pl.ds((4 * bt + cc) * C, C)
            yc = y[:, 128 * cc:128 * cc + 128]
            yb[NT - 1, rows, :] = yc if kt == 0 else yb[NT - 1, rows, :] + yc

    def gen_m(j, kb, b, ng):
        ub, gb = ubs[j % 2], gbs[j % 2]
        for s in range(ng):
            for t in range(3):
                re = lambda ref, c: ref[b(2 * NC, 2 * s * NC + c, 8 + t)]
                im = lambda ref, c: ref[b(2 * NC, (2 * s + 1) * NC + c, 8 + t)]
                gre = [re(gb, c) for c in range(NC)]
                if t == 0:
                    us, gs = [re(ub, c) + im(ub, c) for c in range(NC)], gre
                elif t == 1:
                    us, gs = [re(ub, c) for c in range(NC)], [im(gb, c) - gre[c] for c in range(NC)]
                else:
                    us, gs = [im(ub, c) for c in range(NC)], [im(gb, c) + gre[c] for c in range(NC)]
                ue, uo, ge, go = us[0::2], us[1::2], gs[0::2], gs[1::2]
                usum = [x + y for x, y in zip(ue, uo)]
                gsum = [x + y for x, y in zip(ge, go)]
                poo_prev = None
                for a in range(NC // 2):
                    pee, poo, pss = _conv(ue, ge, a), _conv(uo, go, a), _conv(usum, gsum, a)
                    kb[b(3, ((2 * a + 1) * NG + s) * 3 + t)] = pee if poo_prev is None else pee + poo_prev
                    kb[b(3, ((2 * a + 2) * NG + s) * 3 + t)] = pss - pee - poo
                    poo_prev = poo
                    yield 3 * (2 * a + 1) + 7

    def add_d(j):
        gb = gbs[j % 2]
        dvec = par[pl.ds(8, 8), pl.ds(j * 128, 128)]
        for gi in range(NG):
            gb[2 * gi * NC] = gb[2 * gi * NC] + dvec

    def dot_m(i, t0, nt, rows):
        m = None
        for kt in range(NT):
            p = _mm(_as_bf16(rows[kt]), wm[i, pl.ds(64 * kt, 64), pl.ds(128 * t0, 128 * nt)])
            m = p if m is None else m + p
        for t in range(nt):
            modb[i * (WMA // 128) + (t0 + t)] = m[0:8, 128 * t:128 * (t + 1)]

    pre = dict(H=0, U=672 + 96 // W, a=192, b=192, m=0, k=176)
    post = dict(H=0, U=0, a=4, b=4, m=2, k=0)
    nst = dict(H=16, U=16, a=8, b=8, m=5, k=8)

    def a_block(dots, mg=None, ng=0, tbl=kb0):
        native, dur = [], []
        for idx, (k_, _) in enumerate(dots):
            nxt = pre[dots[idx + 1][0]] if idx + 1 < len(dots) else 0
            d_ = 2.0 if k_ == 'm' else 1.0
            native += [nxt / nst[k_] + post[k_] * d_] * nst[k_]
            dur += [d_] * nst[k_]
        if mg is not None and dots:
            head = max(HEAD - pre[dots[0][0]], 0)
            mtot = 744 * ng - TAIL - head
            lvl = (mtot + sum(native)) / sum(dur)
            want = [max(lvl * d_ - x, 0.0) for x, d_ in zip(native, dur)]
            cum = [head]
            for w_ in want:
                cum.append(cum[-1] + w_ * mtot / sum(want))
        done, step = 0.0, 0
        for (k_, fn) in dots:
            rows = []
            for n in range(nst[k_]):
                while mg is not None and done < cum[step]:
                    done += next(mg)
                step += 1
                if k_ in 'ab':
                    rows.append(jnp.concatenate([tbl[KOFF + 16 + 2 * n], tbl[KOFF + 17 + 2 * n]], axis=1))
                else:
                    rows.append(tbl[KOFF + dict(H=n, U=32 + n, k=16 + 2 * n, m=48 + n)[k_]])
            fn(rows if k_ == 'm' else _as_bf16(jnp.concatenate(rows, axis=0)))
        for _ in (mg or ()):
            pass

    def fdot(k_, j, b):
        if k_ in 'HU':
            return (k_, functools.partial(dot_h if k_ == 'H' else dot_u, j, b))
        return (k_, functools.partial(dot_i, j, b, 0 if k_ == 'a' else 1))

    def a_loop(jf, jm, ji, g0, ng):
        kinds = [k_ for k_ in DORDER if k_ in 'HU' or ji is not None]

        def body(i, carry):
            cache = {}
            zs[i] = 0
            dots = [fdot(k_, jf if k_ in 'HU' else ji, mkb(i, 2, s_, cache)) for s_ in range(2) for k_ in kinds]
            a_block(dots, gen_m(jm, kbs[jm % 2], mkb(i, ng, g0, cache), ng), ng, kbs[jm % 2])

            @pl.when(i == 0)
            def _():
                wait_all(cp_tile(jf, 1))
            return carry
        wait_all(cp_tile(jf, 0))
        lax.fori_loop(0, 2, body, 0)
        add_d(jf)

    sb_ = lambda bt: mkb(0, 1, bt, None)
    with jax.named_scope("A_seg0"):
        wait_all(cp_t0[0])
        a_block([fdot('H', 0, sb_(bt)) for bt in range(4)])
        add_d(0)
        wait_all(cp_t0[1])
        a_block([fdot('U', 0, sb_(bt)) for bt in range(2)])
        for bt in (2, 3):
            wait_all(cp_t0[bt])
            a_block([fdot('U', 0, sb_(bt))])
    with jax.named_scope("A_m0"):
        def body_m0(i, carry):
            a_block([], gen_m(0, kb0, mkb(i, G0 // 2, 0, {}), G0 // 2))
            return carry
        lax.fori_loop(0, 2, body_m0, 0)
    for seg in range(1, NT):
        with jax.named_scope(f"A_seg{seg}"):
            if seg == 1:
                a_loop(1, 0, None, G0, (NG - G0) // 2)
            else:
                a_loop(seg, seg - 1, seg - 2, 0, 8)

    def with_mod(i, dots, step):
        mm = [('m', functools.partial(dot_m, i, t0, nt)) for (t0, nt) in ((0, 4), (4, 4), (8, 2))]
        return [mm[0]] + dots[:step] + [mm[1]] + dots[step:2 * step] + [mm[2]] + dots[2 * step:]

    with jax.named_scope("A_seg5a"):
        cp_wm(0).wait()
        zz = zs[1]

        @pl.when(zz == 0)
        def _():
            dots = [fdot(k_, NT - 2, sb_(bt)) for bt in range(4) for k_ in 'ab']
            a_block(with_mod(0, dots, 2), gen_m(NT - 1, kb0, mkb(zz, 8, 0, {}), 8), 8, kb0)
    with jax.named_scope("A_seg5b"):
        cp_wm(1).wait()

        @pl.when(zz == 0)
        def _():
            dots = [('k', functools.partial(dot_k, kb0, 0, bt)) for bt in range(4)]
            a_block(with_mod(1, dots, 1), gen_m(NT - 1, kb1, mkb(zz, 8, 8, {}), 8), 8, kb1)

    def zero_of(vs):
        t_ = pltpu.bitcast(vs[0], u32)
        for v_ in vs[1:]:
            t_ = t_ | pltpu.bitcast(v_, u32)
        return t_ & kbuf[0, pl.ds(0, 8), :]

    def tie_at(w_, r0, c0, vs):
        mid = [w_[r0:r0 + 8, :c0]] if c0 else []
        mid.append(w_[r0:r0 + 8, c0:c0 + 128] | zero_of(vs))
        if c0 + 128 < w_.shape[1]:
            mid.append(w_[r0:r0 + 8, c0 + 128:])
        parts = ([w_[:r0]] if r0 else []) + [jnp.concatenate(mid, axis=1)] + ([w_[r0 + 8:]] if r0 + 8 < w_.shape[0] else [])
        return jnp.concatenate(parts, axis=0)

    def tied(wref, ties):
        w_ = wref[...]
        for (t, rb), vs in ties.items():
            w_ = tie_at(w_, 64 * (t % 5) + 8 * rb, 128 * (t // 5), vs)
        return w_

    def firsts(x):
        return [x[8 * g:8 * g + 8, 0:128] for g in range(x.shape[0] // 8)]

    def ln_chain(p):
        rows = pl.ds(p * R, R)
        pa, pb, pc, ps = [par[pl.ds(16 + 8 * t, 8), :][None] for t in range(4)]
        g3 = lambda x: x.reshape(R // 8, 8, D)
        q = g3(qbuf[rows, :].astype(f32))
        d1, r1 = _center(q)
        y = g3(jnp.concatenate([yb[j, rows, :] for j in range(NT)], axis=1))
        x = q + ((d1 * r1) * pa + pb) * y
        xn[rows, :] = x.reshape(R, D)
        d2, r2 = _center(x)
        h = (d2 * r2) * pc + ps
        hh[rows, :] = h.reshape(R, D)
        d3, r3 = _center(h, True)
        return (d3 * r3).reshape(R, D)

    def w1_dot(p, l3, ties, fresh):
        if fresh:
            ties[(0, 2)] = firsts(l3)[0:2]
            l3 = pltpu.bitcast(tie_at(pltpu.bitcast(l3, u32), 0, 128, firsts(l3)[2:4]), f32)
        z = _mm(l3.astype(bf16), tied(w1, ties))
        g = _gelu2a(z)
        lane = lax.broadcasted_iota(jnp.int32, (R, 128), 1)
        for j, (o1, cut, o2) in enumerate(((1, 128, 0), (1, 32, -1), (-1, 64, 2), (2, 96, -2), (-2, 128, 0))):
            gj = g[:, j * 128:(j + 1) * 128]
            if cut == 128:
                h1[j, pl.ds(p * R + 8 + o1, R), :] = gj
            else:
                pltpu.store(h1.at[j, pl.ds(p * R + 8 + o1, R), :], gj, mask=lane < cut)
                pltpu.store(h1.at[j, pl.ds(p * R + 8 + o2, R), :], gj, mask=lane >= cut)
        return z

    def w2_dot(p, ties):
        rows = pl.ds(p * R, R)
        hs = jnp.concatenate([h1[j, pl.ds(p * R + 8, R), :] for j in range(NT)], axis=1).astype(bf16)
        x1 = hh[rows, :] + _mm(hs, tied(w2, ties))
        hh[rows, :] = x1
        return x1

    def ln4(r, n):
        d4, r4 = _center(hh[pl.ds(r, n), :], True)
        return d4 * r4

    zoff = [zz >> p_ for p_ in range(7)]

    def prep2(src, dst, tr, t, p_, anchor):
        zero = zero_of([anchor])
        gate = 0 if _SBU[p_][0] else 3
        l1 = []
        for k2 in range(2):
            for n2 in range(2):
                bl = []
                for b_ in range(4):
                    kq, nq = 2 * (b_ // 2) + k2, 2 * (b_ % 2) + n2
                    x = None
                    if _SBU[p_][b_]:
                        x = src[zoff[p_], pl.ds(8 * t + 192 * (nq if tr else kq), 8), pl.ds(128 * (kq if tr else nq), 128)]
                        if b_ == gate and k2 == n2:
                            x = x | zero
                        x = _as_bf16(x).astype(f32)
                    bl.append(x)
                l1.append(_SB[p_](*bl))
        for q_ in range(7):
            if 7 * p_ + q_ not in _PURE:
                dst[7 * p_ + q_, pl.ds(16 * t, 16), :] = _SB[q_](*l1).astype(bf16)

    def prep1(t, n, anchor):
        bl = [w3[pl.ds(lo + 8 * t, 8), pl.ds(c0 + 128 * n, 128)] for lo in (768, 816) for c0 in (0, 256)]
        zero = zero_of([anchor])
        bl[0], bl[3] = bl[0] | zero, bl[3] | zero
        bl = [_as_bf16(x).astype(f32) for x in bl]
        for p_ in (0, 2, 4, 5, 6):
            w3o[2 * p_ + n, pl.ds(16 * t, 16), :] = _SA[p_](*bl).astype(bf16)

    def gb_part(kt, n, anchor):
        acc = None
        for t in range(8):
            w_ = wmc[pl.ds(64 * kt + 8 * t, 8), pl.ds(128 * n, 128)]
            if t == 0:
                w_ = w_ | zero_of([anchor])
            p_ = _as_bf16(w_).astype(f32) * sct[pl.ds(128 * kt + 16 * t, 16), :]
            acc = p_ if acc is None else acc + p_
        modb[NT * n + kt] = acc[0:8] + acc[8:16]

    def sc_lhs():
        return _as_bf16(jnp.concatenate([kb0[KOFF + 48 + j] for j in range(NT)], axis=1))

    units, l3s = [], {}
    anch = sorted({(ANCH[0] + (ANCH[1] - ANCH[0]) * i // ANCH[2]) % 80 for i in range(ANCH[2])})

    def run_block(dots, extra=None, pre4=False):
        for d_, (k_, p) in enumerate(dots):
            ties = {}
            e, rp = d_ - (len(dots) - NP4), TS // NP4
            if pre4 and e >= 0:
                nx = ln4(e * rp, rp)
                l4p[pl.ds(e * rp, rp), :] = nx
                ties[(TIE4, 7)] = firsts(nx)
            if extra is not None and d_ == len(dots) - 1:
                nx = ln_chain(extra)
                for pr in range(4):
                    ties[(24, XRB[pr])] = firsts(nx)[2 * pr:2 * pr + 2]
                l3s[extra] = nx.astype(bf16)
            if k_ == 1:
                fresh = p not in l3s
                res = w1_dot(p, ln_chain(p) if fresh else l3s.pop(p), ties, fresh)
            elif k_ == 2:
                res = w2_dot(p, ties)
            for u_ in anch:
                if u_ // 40 + 1 == k_ and units and d_ < len(dots) - (NP4 if pre4 else 0):
                    n, g = (u_ % 40) // 8, u_ % 8
                    units.pop(0)(res[8 * g:8 * g + 8, 128 * n:128 * (n + 1)])

    pos = [N2, 0]

    def plan(lim1):
        last = lim1 == S // R
        dots = []
        while pos[0] < (lim1 if last else lim1 - 1) or pos[0] - pos[1] >= LEAD or (last and pos[1] < lim1):
            k_ = 0 if pos[0] - pos[1] < LEAD and pos[0] < lim1 else 1
            dots.append((k_ + 1, pos[k_]))
            pos[k_] += 1
        return dots, (None if last else pos[0])

    with jax.named_scope("P1"):
        wait_all([cp_wmp, cp_q[0]])
        mp = _mm(sc_lhs(), wmp[...])
        for t in range(WMP // 128):
            modb[2 * WMA // 128 + t] = mp[0:8, 128 * t:128 * (t + 1)]
        sa, ca, ga, sb, cb = [jnp.concatenate([modb[NT * k_ + j] for j in range(NT)], axis=1) for k_ in range(5)]
        par[pl.ds(16, 8), :] = ga * (1.0 + ca) * math.sqrt(D)
        par[pl.ds(24, 8), :] = ga * sa
        par[pl.ds(32, 8), :] = (1.0 + cb) * (math.sqrt(D) / BETA)
        par[pl.ds(40, 8), :] = sb * (1.0 / BETA)
        for bt in range(4):
            dot_k(kb1, 1, bt, _as_bf16(jnp.concatenate([kb0[KOFF + 17 + 2 * n] for n in range(8)], axis=0)))
        for p in range(PRELN):
            l3s[p] = ln_chain(p)
    with jax.named_scope("w1wait"):
        cp_w[0].wait()
    with jax.named_scope("P2"):
        run_block([(1, p) for p in range(N2)])
    with jax.named_scope("w2wait"):
        wait_all([cp_w[1], cp_q[1]])
    with jax.named_scope("P4"):
        run_block(*plan(Q1 // R))
    with jax.named_scope("q2wait"):
        wait_all([cp_q[2], cp_w[3]])
    units += [functools.partial(prep2, w4_, w4s, False, t, p_) for t in range(24) for p_ in range(7)]
    with jax.named_scope("P5"):
        run_block(*plan(Q2 // R))
    with jax.named_scope("q3wait"):
        wait_all([cp_q[3], cp_wmc, cp_w[2]])
    units += [functools.partial(prep2, w3_, w3s, True, t, p_) for t in range(24) for p_ in range(7)]
    units += [functools.partial(prep1, t, n) for t in range(6) for n in range(2)]
    units += [functools.partial(gb_part, kt, n) for n in range(NT) for kt in range(NT)]
    with jax.named_scope("P6"):
        dots, _ = plan(S // R)
        run_block(dots, pre4=True)
        for n in range(NT):
            gsum = sum(modb[NT * n + kt] for kt in range(1, NT)) + modb[NT * n]
            par[pl.ds(48, 8), pl.ds(128 * n, 128)] = jnp.broadcast_to(jnp.sum(gsum, axis=0, keepdims=True), (8, 128))
    assert not units

    quads = ((0, 0), (0, 256), (H2, 0), (H2, 256))
    done_at = [max(i for i, p_ in enumerate(ORD4) if any(k_ == kq for k_, _ in _SC[p_])) for kq in range(4)]
    qorder = sorted(range(4), key=lambda kq: done_at[kq])
    outs = [(0, 512, 128)] + [quads[kq] + (256,) for kq in qorder] + [(H2, 512, 128)]
    assert qorder == [0, 1, 2, 3]
    copies = {2: (0, 0, D), 4: (H2, 0, 512), 5: (H2, 512, 128)}

    def out_copy(r, r0, c0, cn):
        rows = pl.ds(_mult(r + r0, H2), H2)
        return cp(obuf.at[rows, pl.ds(c0, cn)], o_hbm.at[0, rows, pl.ds(c0, cn)], osem.at[0])

    def b2_step(i, carry):
        r = pl.multiple_of(i * TS, TS)
        gs = gs_.at[i >> 8]
        lr = l4p[:, pl.ds(512, 128)]
        w3u, w4u = w3s.bitcast(u32), w4s.bitcast(u32)
        two = lambda ref, p_: jnp.concatenate([ref.bitcast(u32)[2 * p_], ref.bitcast(u32)[2 * p_ + 1]], axis=1)
        w3a = lambda p_: (w3[pl.ds(816, 48), pl.ds(256, 256)] if p_ == 1 else
                          w3[pl.ds(768, 48), pl.ds(0, 256)] if p_ == 3 else two(w3o, p_))
        lt_ = _blocks((0, 0), (H2, 0), (0, 256), (H2, 256))
        tz = []

        def tdots(pos_):
            for k_, at in enumerate(TPOS):
                if at != pos_:
                    continue
                if k_ == 0:
                    tz.append(_mm_nt(_as_bf16(w3[pl.ds(768, 96), pl.ds(512, 128)]), lr.astype(bf16)))
                else:
                    tz.append(_mm_nt(_as_bf16(w3a(k_ - 1)), _SB[k_ - 1](*lt_).load(l4p_.at[i >> (19 + k_)], H2, 256)))
                if k_ == 7:
                    gt = _gelu2a(tz[0] + _quad(_comb(tz[1:])))
                    t1, t2, t3 = [gt[64 * c:64 * (c + 1), :H2] for c in range(3)]
                    u1, u2, u3 = [gt[64 * c:64 * (c + 1), H2:] for c in range(3)]
                    for c, pr_ in enumerate(((t2, u3), (t1, t3 - u3), (u1, u2 - t2))):
                        gs[pl.ds(H2 * (c % 2), H2), pl.ds(1536 + 128 * (c // 2), 128)] = jnp.concatenate(pr_, axis=0).T
        lrs = [lr[:H2].astype(bf16), lr[H2:].astype(bf16)]
        ab = _blocks(*quads)
        ops = {}
        for t in range(3):
            cq, left = [None] * 4, [5, 3, 3, 5]

            def add(k_, x, sg=1):
                cq[k_] = x if cq[k_] is None else cq[k_] + x if sg > 0 else cq[k_] - x
                left[k_] -= 1
                if left[k_] == 0:
                    gg = _gelu2a(cq[k_])
                    for n2 in range(2):
                        cols = pl.ds(768 * (k_ % 2) + 128 * (t + 3 * n2), 128)
                        gs[pl.ds(H2 * (k_ // 2), H2), cols] = gg[:, 128 * n2:128 * (n2 + 1)]

            for p_ in range(8):
                for k_ in (2, 1, 0, 3):
                    if REMP[k_] == p_:
                        wr = [w3[pl.ds(64 * (t + 3 * (2 * (k_ % 2) + n2)), 64), pl.ds(512, 128)] for n2 in range(2)]
                        add(k_, _mm_nt(lrs[k_ // 2], _as_bf16(jnp.concatenate(wr, axis=0))))
                tdots(8 * t + p_)
                if p_ == 7:
                    break
                a_ = _SA[p_](*ab)
                sub_ = (a_, a_.shift(0, 128), a_.shift(Q4, 0), a_.shift(Q4, 128))
                pr = []
                for q_ in range(7):
                    n = 7 * p_ + q_
                    if n not in ops:
                        ops[n] = _SA[q_](*sub_).load(l4p_.at[(i + 4 * p_) >> (9 + q_)], Q4, 128)
                    w_ = (w3[pl.ds(192 * _PURE[n] + 64 * t, 64), pl.ds(128 * _PURE[n], 128)] if n in _PURE
                          else w3u[n, pl.ds(64 * t, 64), :])
                    pr.append(_mm_nt(ops[n], _as_bf16(w_)))
                m_ = _quad(_comb(pr))
                for k_, sg in _SC[p_]:
                    add(k_, m_, sg)
        kord = [c + 3 * n for c in range(3) for n in range(4)]
        gx = lambda c: gs[pl.ds(H2 * (c % 2), H2), pl.ds(1536 + 128 * (c // 2), 128)]
        wx = lambda c, c0, cn: [w4[pl.ds(768 + 32 * b_, 32), pl.ds(c0, cn)] for b_ in ((1, 2), (0, 2), (0, 1))[c]]
        gxs = {}

        def xdot(c, c0, cn):
            if c not in gxs:
                gxs[c] = [gx(c)[Q4 * h_:Q4 * (h_ + 1)].astype(bf16) for h_ in range(2)]
            w_ = jnp.concatenate(wx(c, c0, cn), axis=0)
            return jnp.concatenate([_mm(x, w_) for x in gxs[c]], axis=0)
        wl = jnp.concatenate([w4[pl.ds(64 * k_, 64), pl.ds(512, 128)] for k_ in kord], axis=0)
        gk = lambda r0: jnp.concatenate([gs[pl.ds(r0, H2), pl.ds(128 * k_, 128)] for k_ in kord], axis=1).astype(bf16)
        zs_ = {512: xdot(0, 512, 128)}
        accs = [(zs_[512] + xdot(1, 512, 128)) + _mm(gk(0), wl)]
        rn_ = pl.multiple_of(jnp.minimum(i + 1, S // TS - 1) * TS, TS)
        rp = TS // len(LNT)
        ties = {}
        for e, k_ in enumerate(LNT):
            nx = ln4(pl.multiple_of(rn_ + e * rp, rp), rp)
            l4p[pl.ds(e * rp, rp), :] = nx
            ties[k_] = ties.get(k_, []) + firsts(nx)
        gb_ = _blocks((0, 0), (0, 768), (H2, 0), (H2, 768))
        ms = [None] * 7
        for idx, p_ in enumerate(ORD4):
            a_ = _SA[p_](*gb_)
            sub_ = (a_, a_.shift(0, 384), a_.shift(Q4, 0), a_.shift(Q4, 384))
            pr = []
            for q_ in range(7):
                n = 7 * p_ + q_
                w_ = (w4[pl.ds(192 * _PURE[n], 192), pl.ds(128 * _PURE[n], 128)] if n in _PURE
                      else w4u[n, pl.ds(0, 192), :])
                if 7 * idx + q_ in ties:
                    w_ = tie_at(w_, 0, 0, ties[7 * idx + q_])
                pr.append(_mm(_SA[q_](*sub_).load(gs_.at[(i + 4 * p_) >> (9 + q_)], Q4, 384), w_))
            ms[p_] = _quad(_comb(pr))
            for kq in range(4):
                if done_at[kq] == idx:
                    r0, c0 = quads[kq]
                    if c0 not in zs_:
                        zs_[c0] = xdot(0, c0, 256)
                    acc = zs_[c0]
                    for pp in ORD4[:idx + 1]:
                        for k_, sg in _SC[pp]:
                            if k_ == kq:
                                acc = acc + ms[pp] if sg > 0 else acc - ms[pp]
                    accs.append(acc + xdot(2 if r0 else 1, c0, 256))
        wb = wl
        xb = zs_[512] + xdot(2, 512, 128)
        for k_ in ties:
            if k_ >= 100:
                wb = tie_at(wb, 64 * (k_ - 100), 0, ties[k_])
        accs.append(xb + _mm(gk(H2), wb))
        gbv = par[pl.ds(48, 8), :]
        for oi, ((r0, c0, cn), ac) in enumerate(zip(outs, accs)):
            rows, cols = pl.ds(_mult(r + r0, H2), H2), pl.ds(c0, cn)
            g3 = lambda x: x.reshape(H2 // 8, 8, cn)
            out = g3(xn[rows, cols]) + gbv[None, :, c0:c0 + cn] * g3(hh[rows, cols] + ac)
            obuf[rows, cols] = out.reshape(H2, cn).astype(bf16)
            if oi in copies:
                out_copy(r, *copies[oi]).start()
        return carry

    with jax.named_scope("BII"):
        lax.fori_loop(0, S // TS, b2_step, 0)
    with jax.named_scope("out_wait"):
        for i in range(S // TS):
            for o_ in copies.values():
                out_copy(i * TS, *o_).wait()


@jax.jit
def pallas_adaLN_cond__ssm_conv_h3__mixer_s_mlp__prompt_kernel(
    A_q: jax.Array,
    A_k: jax.Array,
    A_v: jax.Array,
    A_shift_k: jax.Array,
    A_ssm_k: jax.Array,
    A_ssm_D: jax.Array,
    B_x: jax.Array,
    B_w1: jax.Array,
    B_w2: jax.Array,
    B_w3: jax.Array,
    B_w4: jax.Array,
    c: jax.Array,
    w_mod: jax.Array,
):
    del B_x
    hbm = pl.BlockSpec(memory_space=pltpu.MemorySpace.HBM)
    spec = pltpu.VMEM((NG * 2 * NC, 8, 128), f32)
    part = pltpu.VMEM((KOFF + 56, 8, 128), f32)
    return pl.pallas_call(
        _kernel,
        out_shape=jax.ShapeDtypeStruct((1, S, D), bf16),
        in_specs=[hbm] * 12,
        out_specs=hbm,
        scratch_shapes=[
            pltpu.VMEM((27, 8, 128), f32),
            pltpu.VMEM((S, D), bf16),
            pltpu.VMEM((NT, 32 + HS, 128), u32),
            pltpu.VMEM((NT, 32 + HS, 128), u32),
            pltpu.VMEM((NT, 64, S), u32),
            pltpu.VMEM((D // 2, D), u32),
            pltpu.VMEM((D // 2, D), u32),
            pltpu.VMEM((1, F // 2, D), u32),
            pltpu.VMEM((1, F // 2, D), u32),
            pltpu.VMEM((2, D // 2, WMA), u32),
            pltpu.VMEM((D // 2, WMP), u32),
            pltpu.VMEM((D // 2, WMC), u32),
            pltpu.VMEM((S, D), bf16),
            spec, spec, spec, spec,
            part, part,
            pltpu.VMEM((NT, S, 128), f32),
            pltpu.VMEM((S, D), f32),
            pltpu.VMEM((S, D), f32),
            pltpu.VMEM((NT, S + 32, 128), f32),
            pltpu.VMEM((64, D), f32),
            pltpu.VMEM((1, TS, D), f32),
            pltpu.VMEM((1, TS, 1792), f32),
            pltpu.VMEM((52, 400, 128), bf16),
            pltpu.VMEM((52, 400, 128), bf16),
            pltpu.VMEM((14, 96, 128), bf16),
            pltpu.VMEM((D, 128), f32),
            pltpu.VMEM((4, D), bf16),
            pltpu.VMEM((D,), bf16),
            pltpu.VMEM((1, D), bf16),
            pltpu.SMEM((2,), jnp.int32),
            pltpu.SemaphoreType.DMA((20,)),
            pltpu.SemaphoreType.DMA((1,)),
        ],
        compiler_params=pltpu.CompilerParams(vmem_limit_bytes=100 * 1024 * 1024, disable_semaphore_checks=True,
                                             disable_bounds_checks=True),
    )(A_q, A_k, A_v, A_shift_k.T, A_ssm_k, A_ssm_D, B_w1, B_w2, B_w3.T, B_w4, c, w_mod)
```
